```python
import jax
import jax.numpy as jnp

def _softmax(x, axis=-1):
    return jax.nn.softmax(x, axis=axis)
def _gelu(x):
    return jax.nn.gelu(x, approximate=True)
def _silu(x):
    return jax.nn.silu(x)
def _sigmoid(x):
    return jax.nn.sigmoid(x)
def _layernorm(x, axis=-1, eps=1e-5):
    m = jnp.mean(x, axis=axis, keepdims=True)
    v = jnp.var(x, axis=axis, keepdims=True)
    return (x - m) / jnp.sqrt(v + eps)
def _scatter_add(tgt, idx, src, axis=0):
    return tgt.at[idx].add(src)
def _segment_sum(src, seg, n):
    return jax.ops.segment_sum(src, seg, n)
class _Rng:
    def __init__(self, key):
        self._k = key
    def _next(self):
        self._k, sub = jax.random.split(self._k)
        return sub
    def normal(self, shape):
        return jax.random.normal(self._next(), shape, dtype=jnp.bfloat16)
    def randint(self, lo, hi, shape):
        return jax.random.randint(self._next(), shape, lo, hi, dtype=jnp.int32)
    def uniform(self, shape, lo=0.0, hi=1.0):
        return jax.random.uniform(self._next(), shape, jnp.bfloat16, lo, hi)
    def permutation(self, n):
        return jax.random.permutation(self._next(), n)


kernel_name = 'sequential_preLN__linear_kernel_hedgehog__moe_arch_mod__prompt'

def setup_inputs():
    _rng = _Rng(jax.random.key(int.from_bytes(__import__("os").urandom(4), "little")))
    _w = (lambda a: (lambda t: t.astype(jnp.bfloat16) if jnp.issubdtype(t.dtype, jnp.floating) else t)(jnp.asarray(a)))
    def _A_setup():
        B, S, D, H = 1, 2048, 1024, 32
        Dh = D // H
        return {
            "x": _w((lambda *s: _rng.normal(s) * 0.05)(B, S, D)),
            "wqkv": _w((lambda *s: _rng.normal(s) * 0.05)(D, 3 * D)),
            "w_phi": _w((lambda *s: _rng.normal(s) * 0.05)(H, Dh, Dh) * (Dh ** -0.5)),
            "wo": _w((lambda *s: _rng.normal(s) * 0.05)(D, D)),
        }
    _A_in = _A_setup()

    def _B_setup():
        B, S, D, F, C = 1, 2048, 1024, 3584, 1
        return {
            "x": _w((lambda *s: _rng.normal(s) * 0.05)(B, S, D)),
            "w_r": _w((lambda *s: _rng.normal(s) * 0.05)(D)),
            "w_gate": _w((lambda *s: _rng.normal(s) * 0.05)(D, F)),
            "w_up": _w((lambda *s: _rng.normal(s) * 0.05)(D, F)),
            "w_down": _w((lambda *s: _rng.normal(s) * 0.05)(F, D)),
        }
    _B_in = _B_setup()

    return {
        "A_x": _A_in["x"],
        "A_wqkv": _A_in["wqkv"],
        "A_w_phi": _A_in["w_phi"],
        "A_wo": _A_in["wo"],
        "B_x": _B_in["x"],
        "B_w_r": _B_in["w_r"],
        "B_w_gate": _B_in["w_gate"],
        "B_w_up": _B_in["w_up"],
        "B_w_down": _B_in["w_down"],
    }

def reference(A_x, A_wqkv, A_w_phi, A_wo, B_x, B_w_r, B_w_gate, B_w_up, B_w_down):
    def _A_ref(x, wqkv, w_phi, wo):
        B, S, D = x.shape
        H = 32; Dh = D // H
        qkv = (lambda x, *d: x.transpose(*d))((x @ wqkv).reshape(B, S, 3, H, Dh), 2, 0, 3, 1, 4)
        q, k, v = qkv[0], qkv[1], qkv[2]
        pq = jnp.einsum("bhsd,hdf->bhsf", q, w_phi)
        pk = jnp.einsum("bhsd,hdf->bhsf", k, w_phi)
        phi_q = jnp.concatenate([_softmax(pq, axis=-1), _softmax(-pq, axis=-1)], axis=-1)
        phi_k = jnp.concatenate([_softmax(pk, axis=-1), _softmax(-pk, axis=-1)], axis=-1)
        kv = jnp.einsum("bhsf,bhsd->bhfd", phi_k, v)
        z  = jnp.einsum("bhsf->bhf", phi_k)
        num = jnp.einsum("bhqf,bhfd->bhqd", phi_q, kv)
        den = jnp.einsum("bhqf,bhf->bhq", phi_q, z)[..., None] + 1e-6
        o = num / den
        return (lambda x, *d: x.transpose(*d))(o, 0, 2, 1, 3).reshape(B, S, D) @ wo

    def _B_ref(x, w_r, w_gate, w_up, w_down):
        B, S, D = x.shape
        C = 1
        r = x @ w_r
        idx = jnp.argsort(-r, axis=-1)[:, :C]
        idx_e = jnp.repeat(idx.reshape(B, C, 1), D, axis=2)
        x_sel = jnp.take_along_axis(x, idx_e, axis=1)
        g = _silu(x_sel @ w_gate)
        u = x_sel @ w_up
        y = (g * u) @ w_down
        r_sel = _sigmoid(jnp.take_along_axis(r, idx, axis=1))
        y = y * r_sel.reshape(B, C, 1)
        b_off = (jnp.arange(B) * S).reshape(B, 1)
        flat_idx = (idx + b_off).reshape(B * C)
        zero = (x * 0.0).reshape(B * S, D)
        upd = _scatter_add(zero, flat_idx, y.reshape(B * C, D), axis=0)
        return x + upd.reshape(B, S, D)

    x = A_x
    h = x + _A_ref(_layernorm(x, axis=-1), A_wqkv, A_w_phi, A_wo)
    h2 = h + _B_ref(_layernorm(h, axis=-1), B_w_r, B_w_gate, B_w_up, B_w_down)
    return h2
```

```python
import functools

import jax
import jax.numpy as jnp
from jax import lax
import jax.experimental.pallas as pl
import jax.experimental.pallas.tpu as pltpu

F32 = jnp.float32
BF16 = jnp.bfloat16
U32 = jnp.uint32

S = 2048
D = 1024
H = 32
DH = 32
FF = 3584
NPAIR = H // 2
KVROWS = 80
LOG2E = 1.4426950408889634
LN_EPS = 1e-5

T1 = 256
T2 = 256
RC = 256
XT = 256
WD_PAD = 128

NN = (((1,), (0,)), ((), ()))
NT = (((1,), (1,)), ((), ()))
TN = (((0,), (0,)), ((), ()))


def _dot(a, b, dims):
    return lax.dot_general(a, b, dims, preferred_element_type=F32)


def _layernorm(x):
    m = jnp.mean(x, axis=-1, keepdims=True)
    xc = x - m
    v = jnp.mean(xc * xc, axis=-1, keepdims=True)
    return xc * lax.rsqrt(v + LN_EPS)


def _pair_allreduce(a, op):
    a = op(a, pltpu.roll(a, 2, 0))
    return op(a, pltpu.roll(a, 4, 0))


def _tree(op, xs):
    xs = list(xs)
    while len(xs) > 1:
        nxt = [op(xs[i], xs[i + 1]) for i in range(0, len(xs) - 1, 2)]
        if len(xs) % 2:
            nxt.append(xs[-1])
        xs = nxt
    return xs[0]


def _dual_softmax(p):
    sl = [p[8 * i:8 * i + 8, :] for i in range(8)]
    mx = _pair_allreduce(_tree(jnp.maximum, sl), jnp.maximum)
    mn = _pair_allreduce(_tree(jnp.minimum, sl), jnp.minimum)
    ep = [jnp.exp2(s - mx) for s in sl]
    en = [jnp.exp2(mn - s) for s in sl]
    rp = 1.0 / _pair_allreduce(_tree(jnp.add, ep), jnp.add)
    rn = 1.0 / _pair_allreduce(_tree(jnp.add, en), jnp.add)
    out = [e * rp for e in ep] + [e * rn for e in en]
    return jnp.concatenate(out, axis=0).astype(BF16)


def _kernel(x_hbm, wqkv_hbm, wphi_ref, wo_hbm, wr_ref, wg_hbm, wu_hbm, wd_hbm, out_hbm,
            x_v, xn_v, wraw_v, wt_v, wo_v, kvacc_v, kvbf_v, h_v, o_v, wg_v, wu_v, wd_v, patch_v,
            sem_x, sem_w, sem_o, sem_m):
    n_xt = S // XT

    def x_copy(i):
        return pltpu.make_async_copy(x_hbm.at[pl.ds(i * XT, XT), :], x_v.at[pl.ds(i * XT, XT), :], sem_x.at[i])

    def w_copy(j):
        return pltpu.make_async_copy(wqkv_hbm.at[:, pl.ds(j * D, D)], wraw_v.at[j], sem_w.at[j])

    wo_copy = pltpu.make_async_copy(wo_hbm, wo_v, sem_w.at[3])
    wg_copy = pltpu.make_async_copy(wg_hbm, wg_v, sem_m.at[0])
    wu_copy = pltpu.make_async_copy(wu_hbm, wu_v, sem_m.at[1])
    wd_copy = pltpu.make_async_copy(wd_hbm, wd_v.at[:, pl.ds(0, D)], sem_m.at[2])

    w_copy(1).start()
    x_copy(0).start()
    w_copy(2).start()
    for i in range(1, n_xt):
        x_copy(i).start()
    w_copy(0).start()
    wo_copy.start()
    wg_copy.start()
    wu_copy.start()
    wd_copy.start()

    row = lax.broadcasted_iota(jnp.int32, (128, DH), 0)
    col = lax.broadcasted_iota(jnp.int32, (128, DH), 1)
    expand = jnp.where(((row & 63) >> 1) == col, 1.0, 0.0).astype(BF16)
    a_all = _dot(expand, wphi_ref[...], NT)
    row = lax.broadcasted_iota(jnp.int32, (128, D), 0)
    col = lax.broadcasted_iota(jnp.int32, (128, D), 1)
    a_all = jnp.where((2 * (row >> 6) + (row & 1)) == ((col >> 5) & 3), a_all, 0.0).astype(BF16)

    def fold(j):
        for g in range(8):
            w = wraw_v[j, :, g * 128:(g + 1) * 128]
            if j == 2:
                wt = w.T
            else:
                wt = (_dot(a_all[:, g * 128:(g + 1) * 128], w, NT) * LOG2E).astype(BF16)
            r0 = (j * D + g * 128) // 2
            wt_v[r0:r0 + 64, :] = pltpu.bitcast(wt, U32)

    def wt_rows(r0, n):
        return pltpu.bitcast(wt_v[r0 // 2:(r0 + n) // 2, :], BF16)

    w_copy(1).wait()
    fold(1)
    w_copy(2).wait()
    fold(2)
    kvacc_v[...] = jnp.zeros_like(kvacc_v)

    def phase1(t, carry):
        r0 = pl.multiple_of(t * T1, T1)
        for i in range(T1 // XT):
            x_copy(t * (T1 // XT) + i).wait()
        xn = _layernorm(x_v[pl.ds(r0, T1), :].astype(F32)).astype(BF16)
        xn_v[pl.ds(r0, T1), :] = xn
        phis = []
        for c in range(D // RC):
            pk = _dot(wt_rows(D + c * RC, RC), xn, NT)
            for j in range(RC // 64):
                phis.append(_dual_softmax(pk[64 * j:64 * j + 64, :]))
        ones = jnp.ones((16, T1), BF16)
        for c in range(D // RC):
            vt = _dot(wt_rows(2 * D + c * RC, RC), xn, NT).astype(BF16)
            for j in range(RC // 64):
                pr = c * (RC // 64) + j
                vext = jnp.concatenate([vt[64 * j:64 * j + 64, :], ones], axis=0)
                kvacc_v[pr] += _dot(vext, phis[pr], NT)
        return carry

    lax.fori_loop(0, S // T1, phase1, 0)

    row = lax.broadcasted_iota(jnp.int32, (KVROWS, 128), 0)
    col = lax.broadcasted_iota(jnp.int32, (KVROWS, 128), 1)
    rowhead = jnp.where(row < 64, row >> 5, (row - 64) >> 3)
    keep = rowhead == (col & 1)
    for pr in range(NPAIR):
        kvbf_v[pr] = jnp.where(keep, kvacc_v[pr], 0.0).astype(BF16)

    w_copy(0).wait()
    fold(0)
    wo_copy.wait()

    def o_copy(t):
        r0 = pl.multiple_of(t * T2, T2)
        return pltpu.make_async_copy(o_v.at[pl.ds(r0, T2), :], out_hbm.at[pl.ds(r0, T2), :], sem_o.at[t])

    wr = wr_ref[...].astype(F32)

    def phase2(t, carry):
        best, besti = carry
        r0 = pl.multiple_of(t * T2, T2)
        xn = xn_v[pl.ds(r0, T2), :]
        ots = []
        for c in range(D // RC):
            pq = _dot(wt_rows(c * RC, RC), xn, NT)
            for j in range(RC // 64):
                pr = c * (RC // 64) + j
                phi = _dual_softmax(pq[64 * j:64 * j + 64, :])
                res = _dot(kvbf_v[pr], phi, NN)
                i0 = 1.0 / (res[64:72, :] + 1e-6)
                i1 = 1.0 / (res[72:80, :] + 1e-6)
                parts = [res[8 * i:8 * i + 8, :] * (i0 if i < 4 else i1) for i in range(8)]
                ots.append(jnp.concatenate(parts, axis=0).astype(BF16))
        ot = jnp.concatenate(ots, axis=0)
        h = x_v[pl.ds(r0, T2), :].astype(F32) + _dot(ot, wo_v[...], TN)
        h_v[pl.ds(r0, T2), :] = h
        hn = _layernorm(h)
        o_v[pl.ds(r0, T2), :] = (h + hn).astype(BF16)
        o_copy(t).start()
        r = jnp.sum(hn * wr, axis=-1, keepdims=True).astype(BF16).astype(F32)
        sub = lax.broadcasted_iota(jnp.int32, (8, 1), 0)
        for i in range(T2 // 8):
            ri = r[8 * i:8 * i + 8, :]
            better = ri > best
            best = jnp.where(better, ri, best)
            besti = jnp.where(better, sub + (r0 + 8 * i), besti)
        return best, besti

    best, besti = lax.fori_loop(
        0, S // T2, phase2,
        (jnp.full((8, 1), -jnp.inf, F32), jnp.zeros((8, 1), jnp.int32)))

    rmax = jnp.max(best, axis=0, keepdims=True)
    idx = jnp.min(jnp.where(best == rmax, besti, S), axis=0, keepdims=True)
    idx_s = jnp.clip(idx[0, 0], 0, S - 1)
    blk = pl.multiple_of((idx_s >> 4) << 4, 16)
    hb = h_v[pl.ds(blk, 16), :]
    hnb = _layernorm(hb)
    xs = hnb.astype(BF16)
    wg_copy.wait()
    wu_copy.wait()
    wd_copy.wait()
    g = _dot(xs, wg_v[...], NN)
    u = _dot(xs, wu_v[...], NN)
    a = (g * jax.nn.sigmoid(g) * u).astype(BF16)
    y = _dot(a, wd_v[:, 0:D], NN) * jax.nn.sigmoid(rmax)
    sel = lax.broadcasted_iota(jnp.int32, (16, 1), 0) == (idx_s - blk)
    patch_v[...] = (hb + hnb + jnp.where(sel, y, 0.0)).astype(BF16)
    for t in range(S // T2):
        o_copy(t).wait()
    pc = pltpu.make_async_copy(patch_v, out_hbm.at[pl.ds(blk, 16), :], sem_m.at[3])
    pc.start()
    pc.wait()


@jax.jit
def pallas_sequential_preLN__linear_kernel_hedgehog__moe_arch_mod__prompt_kernel(
    A_x: jax.Array,
    A_wqkv: jax.Array,
    A_w_phi: jax.Array,
    A_wo: jax.Array,
    B_x: jax.Array,
    B_w_r: jax.Array,
    B_w_gate: jax.Array,
    B_w_up: jax.Array,
    B_w_down: jax.Array,
):
    del B_x
    hbm = pl.BlockSpec(memory_space=pl.ANY)
    vmem = pl.BlockSpec(memory_space=pltpu.VMEM)
    out = pl.pallas_call(
        _kernel,
        out_shape=jax.ShapeDtypeStruct((S, D), BF16),
        in_specs=[hbm, hbm, vmem, hbm, vmem, hbm, hbm, hbm],
        out_specs=hbm,
        scratch_shapes=[
            pltpu.VMEM((S, D), BF16),
            pltpu.VMEM((S, D), BF16),
            pltpu.VMEM((3, D, D), BF16),
            pltpu.VMEM((3 * D // 2, D), U32),
            pltpu.VMEM((D, D), BF16),
            pltpu.VMEM((NPAIR, KVROWS, 128), F32),
            pltpu.VMEM((NPAIR, KVROWS, 128), BF16),
            pltpu.VMEM((S, D), F32),
            pltpu.VMEM((S, D), BF16),
            pltpu.VMEM((D, FF), BF16),
            pltpu.VMEM((D, FF), BF16),
            pltpu.VMEM((FF, D + WD_PAD), BF16),
            pltpu.VMEM((16, D), BF16),
            pltpu.SemaphoreType.DMA((S // XT,)),
            pltpu.SemaphoreType.DMA((4,)),
            pltpu.SemaphoreType.DMA((S // T2,)),
            pltpu.SemaphoreType.DMA((4,)),
        ],
        compiler_params=pltpu.CompilerParams(vmem_limit_bytes=100 * 1024 * 1024),
        name="hedgehog_mod",
    )(
        A_x.reshape(S, D),
        A_wqkv,
        A_w_phi.reshape(H * DH, DH),
        A_wo,
        B_w_r.reshape(1, D),
        B_w_gate,
        B_w_up,
        B_w_down,
    )
    return out.reshape(1, S, D)
```

```python
import jax
import jax.numpy as jnp
from jax import lax
import jax.experimental.pallas as pl
import jax.experimental.pallas.tpu as pltpu

F32 = jnp.float32
BF16 = jnp.bfloat16
U32 = jnp.uint32

S = 2048
D = 1024
H = 32
DH = 32
FF = 3584
NPAIR = H // 2
LOG2E = 1.4426950408889634
LN_EPS = 1e-5

T = 256
NT_ = S // T
RC = 256
NC = D // RC
PPC = RC // 64
WD_PAD = 128

NN = (((1,), (0,)), ((), ()))
NT = (((1,), (1,)), ((), ()))
TN = (((0,), (0,)), ((), ()))


def _dot(a, b, dims):
    return lax.dot_general(a, b, dims, preferred_element_type=F32)


def _layernorm(x):
    m = jnp.mean(x, axis=-1, keepdims=True)
    xc = x - m
    v = jnp.mean(xc * xc, axis=-1, keepdims=True)
    return xc * lax.rsqrt(v + LN_EPS)


def _pair_allreduce(a, op):
    a = op(a, pltpu.roll(a, 2, 0))
    return op(a, pltpu.roll(a, 4, 0))


def _tree(op, xs):
    xs = list(xs)
    while len(xs) > 1:
        nxt = [op(xs[i], xs[i + 1]) for i in range(0, len(xs) - 1, 2)]
        if len(xs) % 2:
            nxt.append(xs[-1])
        xs = nxt
    return xs[0]


def _dual_exp(p):
    sl = [p[8 * i:8 * i + 8, :] for i in range(8)]
    mx = _pair_allreduce(_tree(jnp.maximum, sl), jnp.maximum)
    mn = _pair_allreduce(_tree(jnp.minimum, sl), jnp.minimum)
    ep = [jnp.exp2(s - mx) for s in sl]
    en = [jnp.exp2(mn - s) for s in sl]
    rp = 1.0 / _pair_allreduce(_tree(jnp.add, ep), jnp.add)
    rn = 1.0 / _pair_allreduce(_tree(jnp.add, en), jnp.add)
    return ep, en, rp, rn


def _lane_fold(a):
    return _tree(jnp.add, [a[:, 128 * i:128 * i + 128] for i in range(a.shape[1] // 128)])


def _lane_tile(a, n):
    return a if n == 1 else jnp.concatenate([a] * n, axis=1)


def _kernel(x_hbm, wqkv_hbm, wphi_hbm, wo_hbm, wr_hbm, wg_hbm, wu_hbm, wd_hbm, out_hbm,
            x_v, xn_v, wraw_v, wt_v, wphi_v, wo_v, wr_v, kvacc_v, kvbf_v, z_v, h_v, o_v,
            wg_v, wu_v, wd_v, patch_v,
            sem_x, sem_w, sem_o, sem_m):

    def x_copy(i):
        return pltpu.make_async_copy(x_hbm.at[pl.ds(i * T, T), :], x_v.at[pl.ds(i * T, T), :], sem_x.at[i])

    def w_copy(j, c):
        return pltpu.make_async_copy(wqkv_hbm.at[:, pl.ds(j * D + c * RC, RC)], wraw_v.at[j * NC + c],
                                     sem_w.at[j * NC + c])

    wphi_copy = pltpu.make_async_copy(wphi_hbm, wphi_v, sem_m.at[4])
    wr_copy = pltpu.make_async_copy(wr_hbm, wr_v, sem_m.at[5])
    wo_copy = pltpu.make_async_copy(wo_hbm, wo_v, sem_m.at[6])
    wg_copy = pltpu.make_async_copy(wg_hbm, wg_v, sem_m.at[0])
    wu_copy = pltpu.make_async_copy(wu_hbm, wu_v, sem_m.at[1])
    wd_copy = pltpu.make_async_copy(wd_hbm, wd_v.at[:, pl.ds(0, D)], sem_m.at[2])

    wphi_copy.start()
    x_copy(0).start()
    for c in range(NC):
        w_copy(1, c).start()
    for c in range(NC):
        w_copy(2, c).start()
    x_copy(1).start()

    def ln_tile(t):
        r0 = t * T if isinstance(t, int) else pl.multiple_of(t * T, T)
        xn = _layernorm(x_v[pl.ds(r0, T), :].astype(F32)).astype(BF16)
        xn_v[pl.ds(r0, T), :] = xn
        return xn

    wphi_copy.wait()
    x_copy(0).wait()
    for i in range(2, NT_):
        x_copy(i).start()

    row = lax.broadcasted_iota(jnp.int32, (128, DH), 0)
    col = lax.broadcasted_iota(jnp.int32, (128, DH), 1)
    expand = jnp.where(((row & 63) >> 1) == col, 1.0, 0.0).astype(BF16)
    a_all = _dot(expand, wphi_v[...].reshape(H * DH, DH), NT)
    row = lax.broadcasted_iota(jnp.int32, (128, D), 0)
    col = lax.broadcasted_iota(jnp.int32, (128, D), 1)
    a_all = jnp.where((2 * (row >> 6) + (row & 1)) == ((col >> 5) & 3), a_all, 0.0).astype(BF16)
    xn0 = ln_tile(0)
    h_v[0:T, :] = jnp.zeros((T, D), F32)

    def fold(j, c):
        out = []
        for s in range(RC // 128):
            g = c * (RC // 128) + s
            w = wraw_v[j * NC + c, :, s * 128:(s + 1) * 128]
            if j == 2:
                wt = w.T
            else:
                wt = (_dot(a_all[:, g * 128:(g + 1) * 128], w, NT) * LOG2E).astype(BF16)
            r0 = (j * D + g * 128) // 2
            wt_v[r0:r0 + 64, :] = pltpu.bitcast(wt, U32)
            out.append(wt)
        return out

    def wt_rows(r0, n):
        return pltpu.bitcast(wt_v[r0 // 2:(r0 + n) // 2, :], BF16)

    def k_features(pk, c, first):
        phis = []
        for j in range(PPC):
            pr = c * PPC + j
            ep, en, rp, rn = _dual_exp(pk[64 * j:64 * j + 64, :])
            phi = jnp.concatenate([e * rp for e in ep] + [e * rn for e in en], axis=0)
            zs = _lane_fold(phi)
            z_v[pr] = zs if first else z_v[pr] + zs
            phis.append(phi.astype(BF16))
        return phis

    def kv_update(vt, phis, c, first):
        vt = vt.astype(BF16)
        for j in range(PPC):
            pr = c * PPC + j
            upd = _dot(vt[64 * j:64 * j + 64, :], phis[j], NT)
            kvacc_v[pr] = upd if first else kvacc_v[pr] + upd

    def proj(ws, xn):
        return jnp.concatenate([_dot(w, xn, NT) for w in ws], axis=0)

    phis = [None] * NC
    w_copy(1, 0).wait()
    for c in range(NC):
        w_copy(0, c).start()
    pk0 = proj(fold(1, 0), xn0)
    w_copy(1, 1).wait()
    wo_copy.start()
    wr_copy.start()
    pk1 = proj(fold(1, 1), xn0)
    phis[0] = k_features(pk0, 0, True)
    w_copy(1, 2).wait()
    w_copy(1, 3).wait()
    wg_copy.start()
    wu_copy.start()
    wd_copy.start()
    wk2 = fold(1, 2)
    wk3 = fold(1, 3)
    pk2 = proj(wk2, xn0)
    phis[1] = k_features(pk1, 1, True)
    w_copy(2, 0).wait()
    w_copy(2, 1).wait()
    pk3 = proj(wk3, xn0)
    wv0 = fold(2, 0)
    wv1 = fold(2, 1)
    phis[2] = k_features(pk2, 2, True)
    vt0 = proj(wv0, xn0)
    phis[3] = k_features(pk3, 3, True)
    w_copy(2, 2).wait()
    w_copy(2, 3).wait()
    vt1 = proj(wv1, xn0)
    wv2 = fold(2, 2)
    wv3 = fold(2, 3)
    kv_update(vt0, phis[0], 0, True)
    vt2 = proj(wv2, xn0)
    x_copy(1).wait()
    vt3 = proj(wv3, xn0)
    kv_update(vt1, phis[1], 1, True)
    kv_update(vt2, phis[2], 2, True)
    kv_update(vt3, phis[3], 3, True)
    ln_tile(1)

    def phase1(t, carry):
        r0 = pl.multiple_of(t * T, T)
        tn = jnp.minimum(t + 1, NT_ - 1)

        @pl.when(t + 1 < NT_)
        def _():
            x_copy(tn).wait()

        xn = xn_v[pl.ds(r0, T), :]
        phis = []
        for c in range(NC):
            pk = _dot(wt_rows(D + c * RC, RC), xn, NT)
            phis.append(k_features(pk, c, False))
        vts = []
        for c in range(NC):
            vts.append(_dot(wt_rows(2 * D + c * RC, RC), xn, NT))
            if c > 0:
                kv_update(vts[c - 1], phis[c - 1], c - 1, False)
        kv_update(vts[NC - 1], phis[NC - 1], NC - 1, False)
        ln_tile(tn)
        return carry

    lax.fori_loop(1, NT_, phase1, 0)

    for c in range(NC):
        w_copy(0, c).wait()
    wo_copy.wait()
    wr_copy.wait()
    row = lax.broadcasted_iota(jnp.int32, (64, 128), 0)
    col = lax.broadcasted_iota(jnp.int32, (64, 128), 1)
    keep = (row >> 5) == (col & 1)
    for pr in range(NPAIR):
        kvbf_v[pr] = jnp.where(keep, kvacc_v[pr], 0.0).astype(BF16)
        z_v[pr] = jnp.broadcast_to(jnp.sum(z_v[pr], axis=-1, keepdims=True), (128, 128))
    for c in range(NC):
        fold(0, c)

    def o_copy(t):
        r0 = t * T if isinstance(t, int) else pl.multiple_of(t * T, T)
        return pltpu.make_async_copy(o_v.at[pl.ds(r0, T), :], out_hbm.at[pl.ds(r0, T), :], sem_o.at[t])

    def finish_tile(t, valid, best, besti):
        r0 = t * T if isinstance(t, int) else pl.multiple_of(t * T, T)
        wr = wr_v[...].reshape(1, D).astype(F32)
        h = h_v[pl.ds(r0, T), :]
        hn = _layernorm(h)
        o_v[pl.ds(r0, T), :] = (h + hn).astype(BF16)
        r = jnp.sum(hn * wr, axis=-1, keepdims=True).astype(BF16).astype(F32)
        if valid is not None:
            r = jnp.where(valid, r, -jnp.inf)
        sub = lax.broadcasted_iota(jnp.int32, (8, 1), 0)
        for i in range(T // 8):
            ri = r[8 * i:8 * i + 8, :]
            better = ri > best
            best = jnp.where(better, ri, best)
            besti = jnp.where(better, sub + (r0 + 8 * i), besti)
        return best, besti

    def q_features(pq, c):
        phis = []
        for j in range(PPC):
            pr = c * PPC + j
            ep, en, rp, rn = _dual_exp(pq[64 * j:64 * j + 64, :])
            zz = [_lane_tile(z_v[pr, 8 * i:8 * i + 8, :], T // 128) for i in range(16)]
            ap = _pair_allreduce(_tree(jnp.add, [ep[i] * zz[i] for i in range(8)]), jnp.add)
            an = _pair_allreduce(_tree(jnp.add, [en[i] * zz[8 + i] for i in range(8)]), jnp.add)
            inv = 1.0 / (rp * ap + rn * an + 1e-6)
            sp = rp * inv
            sn = rn * inv
            phis.append(jnp.concatenate([e * sp for e in ep] + [e * sn for e in en], axis=0).astype(BF16))
        return phis

    def attn_rows(phis, c):
        return jnp.concatenate(
            [_dot(kvbf_v[c * PPC + j], phis[j], NN).astype(BF16) for j in range(PPC)], axis=0)

    def phase2(t, carry):
        best, besti = carry
        r0 = pl.multiple_of(t * T, T)
        tp = jnp.maximum(t - 1, 0)
        best, besti = finish_tile(tp, t > 0, best, besti)
        xn = xn_v[pl.ds(r0, T), :]
        phis, ots = [], []
        for c in range(NC):
            pq = _dot(wt_rows(c * RC, RC), xn, NT)
            phis.append(q_features(pq, c))
            if c > 0:
                ots.append(attn_rows(phis[c - 1], c - 1))
        o1 = jnp.concatenate(ots[:NC // 2], axis=0).T
        ha = _dot(o1, wo_v[0:D // 2, 0:D // 2], NN)
        ots.append(attn_rows(phis[NC - 1], NC - 1))
        hb = _dot(o1, wo_v[0:D // 2, D // 2:D], NN)
        o2 = jnp.concatenate(ots[NC // 2:], axis=0).T
        h = (x_v[pl.ds(r0, T), :].astype(F32) + jnp.concatenate([ha, hb], axis=1)
             + _dot(o2, wo_v[D // 2:D, :], NN))
        h_v[pl.ds(r0, T), :] = h

        @pl.when(t > 0)
        def _():
            o_copy(tp).start()

        return best, besti

    best, besti = lax.fori_loop(
        0, NT_, phase2,
        (jnp.full((8, 1), -jnp.inf, F32), jnp.zeros((8, 1), jnp.int32)))
    wg_copy.wait()
    wu_copy.wait()
    wd_copy.wait()
    best, besti = finish_tile(NT_ - 1, None, best, besti)
    o_copy(NT_ - 1).start()

    rmax = jnp.max(best, axis=0, keepdims=True)
    idx = jnp.min(jnp.where(best == rmax, besti, S), axis=0, keepdims=True)
    idx_s = jnp.clip(idx[0, 0], 0, S - 1)
    blk = pl.multiple_of((idx_s >> 4) << 4, 16)
    hb = h_v[pl.ds(blk, 16), :]
    hnb = _layernorm(hb)
    xs = hnb.astype(BF16)
    g = _dot(xs, wg_v[...], NN)
    u = _dot(xs, wu_v[...], NN)
    a = (g * jax.nn.sigmoid(g) * u).astype(BF16)
    y = _dot(a, wd_v[:, 0:D], NN) * jax.nn.sigmoid(rmax)
    sel = lax.broadcasted_iota(jnp.int32, (16, 1), 0) == (idx_s - blk)
    patch_v[...] = (hb + hnb + jnp.where(sel, y, 0.0)).astype(BF16)
    for t in range(NT_):
        o_copy(t).wait()
    pc = pltpu.make_async_copy(patch_v, out_hbm.at[pl.ds(blk, 16), :], sem_m.at[3])
    pc.start()
    pc.wait()


@jax.jit
def pallas_sequential_preLN__linear_kernel_hedgehog__moe_arch_mod__prompt_kernel(
    A_x: jax.Array,
    A_wqkv: jax.Array,
    A_w_phi: jax.Array,
    A_wo: jax.Array,
    B_x: jax.Array,
    B_w_r: jax.Array,
    B_w_gate: jax.Array,
    B_w_up: jax.Array,
    B_w_down: jax.Array,
):
    del B_x
    hbm = pl.BlockSpec(memory_space=pl.ANY)
    out = pl.pallas_call(
        _kernel,
        out_shape=jax.ShapeDtypeStruct((S, D), BF16),
        in_specs=[hbm] * 8,
        out_specs=hbm,
        scratch_shapes=[
            pltpu.VMEM((S, D), BF16),
            pltpu.VMEM((S, D), BF16),
            pltpu.VMEM((3 * NC, D, RC), BF16),
            pltpu.VMEM((3 * D // 2, D), U32),
            pltpu.VMEM((H, DH, DH), BF16),
            pltpu.VMEM((D, D), BF16),
            pltpu.VMEM((D,), BF16),
            pltpu.VMEM((NPAIR, 64, 128), F32),
            pltpu.VMEM((NPAIR, 64, 128), BF16),
            pltpu.VMEM((NPAIR, 128, 128), F32),
            pltpu.VMEM((S, D), F32),
            pltpu.VMEM((S, D), BF16),
            pltpu.VMEM((D, FF), BF16),
            pltpu.VMEM((D, FF), BF16),
            pltpu.VMEM((FF, D + WD_PAD), BF16),
            pltpu.VMEM((16, D), BF16),
            pltpu.SemaphoreType.DMA((NT_,)),
            pltpu.SemaphoreType.DMA((3 * NC,)),
            pltpu.SemaphoreType.DMA((NT_,)),
            pltpu.SemaphoreType.DMA((7,)),
        ],
        compiler_params=pltpu.CompilerParams(vmem_limit_bytes=100 * 1024 * 1024),
        name="hedgehog_mod",
    )(
        A_x.reshape(S, D),
        A_wqkv,
        A_w_phi,
        A_wo,
        B_w_r,
        B_w_gate,
        B_w_up,
        B_w_down,
    )
    return out.reshape(1, S, D)
```

```python
import jax
import jax.numpy as jnp
from jax import lax
import jax.experimental.pallas as pl
import jax.experimental.pallas.tpu as pltpu

F32 = jnp.float32
BF16 = jnp.bfloat16
U32 = jnp.uint32

S = 2048
D = 1024
H = 32
DH = 32
FF = 3584
NPAIR = H // 2
LOG2E = 1.4426950408889634
LN_EPS = 1e-5

T = 256
NT_ = S // T
RC = 256
NC = D // RC
PPC = RC // 64
LNC = 16
LN1_SPAN = 13
LN2_SPAN = 20
WD_PAD = 128

NN = (((1,), (0,)), ((), ()))
NT = (((1,), (1,)), ((), ()))
TN = (((0,), (0,)), ((), ()))


def _dot(a, b, dims):
    return lax.dot_general(a, b, dims, preferred_element_type=F32)


def _layernorm(x):
    m = jnp.mean(x, axis=-1, keepdims=True)
    xc = x - m
    v = jnp.mean(xc * xc, axis=-1, keepdims=True)
    return xc * lax.rsqrt(v + LN_EPS)


def _pair_allreduce(a, op):
    a = op(a, pltpu.roll(a, 2, 0))
    return op(a, pltpu.roll(a, 4, 0))


def _tree(op, xs):
    xs = list(xs)
    while len(xs) > 1:
        nxt = [op(xs[i], xs[i + 1]) for i in range(0, len(xs) - 1, 2)]
        if len(xs) % 2:
            nxt.append(xs[-1])
        xs = nxt
    return xs[0]


def _dual_exp(p):
    sl = [p[8 * i:8 * i + 8, :] for i in range(8)]
    mx = _pair_allreduce(_tree(jnp.maximum, sl), jnp.maximum)
    mn = _pair_allreduce(_tree(jnp.minimum, sl), jnp.minimum)
    ep = [jnp.exp2(s - mx) for s in sl]
    en = [jnp.exp2(mn - s) for s in sl]
    rp = 1.0 / _pair_allreduce(_tree(jnp.add, ep), jnp.add)
    rn = 1.0 / _pair_allreduce(_tree(jnp.add, en), jnp.add)
    return ep, en, rp, rn


def _tie(x, never, anchor):
    if anchor is None:
        return x
    d = jnp.concatenate([anchor] * (x.shape[0] // 8), axis=0)
    return jnp.concatenate([jnp.where(never, d, x[:, :128]), x[:, 128:]], axis=1)


def _anchors(res):
    m, n = res.shape
    return [res[r:r + 8, c:c + 128] for c in range(0, n, 128) for r in (m // 2 - 8, m - 8)]


def _lane_fold(a):
    return _tree(jnp.add, [a[:, 128 * i:128 * i + 128] for i in range(a.shape[1] // 128)])


def _lane_tile(a, n):
    return a if n == 1 else jnp.concatenate([a] * n, axis=1)


def _kernel(x_hbm, wqkv_hbm, wphi_hbm, wo_hbm, wr_hbm, wg_hbm, wu_hbm, wd_hbm, out_hbm,
            x_v, xn_v, wraw_v, wt_v, wphi_v, wo_v, wr_v, kvacc_v, kvbf_v, z_v, h_v, o_v,
            wg_v, wu_v, wd_v, patch_v,
            sem):
    SX, SW, SO, SM = 0, NT_, NT_ + 3 * NC, 2 * NT_ + 3 * NC

    def x_copy(i):
        return pltpu.make_async_copy(x_hbm.at[pl.ds(i * T, T), :], x_v.at[pl.ds(i * T, T), :], sem.at[SX + i])

    def w_copy(j, c):
        return pltpu.make_async_copy(wqkv_hbm.at[:, pl.ds(j * D + c * RC, RC)], wraw_v.at[j * NC + c],
                                     sem.at[SW + j * NC + c])

    wphi_copy = pltpu.make_async_copy(wphi_hbm, wphi_v, sem.at[SM + 4])
    wr_copy = pltpu.make_async_copy(wr_hbm, wr_v, sem.at[SM + 5])
    wo_copy = pltpu.make_async_copy(wo_hbm, wo_v, sem.at[SM + 6])
    wg_copy = pltpu.make_async_copy(wg_hbm, wg_v, sem.at[SM + 0])
    wu_copy = pltpu.make_async_copy(wu_hbm, wu_v, sem.at[SM + 1])
    wd_copy = pltpu.make_async_copy(wd_hbm, wd_v.at[:, pl.ds(0, D)], sem.at[SM + 2])

    wphi_copy.start()
    x_copy(0).start()
    for c in range(NC):
        w_copy(1, c).start()
    for c in range(NC):
        w_copy(2, c).start()
    x_copy(1).start()

    def ln_rows(r0, n, never=None, anchor=None):
        rows = pl.ds(r0, n)
        xn = _layernorm(_tie(x_v[rows, :].astype(F32), never, anchor)).astype(BF16)
        xn_v[rows, :] = xn
        return xn

    wphi_copy.wait()
    x_copy(0).wait()
    for i in range(2, NT_):
        x_copy(i).start()

    row = lax.broadcasted_iota(jnp.int32, (128, DH), 0)
    col = lax.broadcasted_iota(jnp.int32, (128, DH), 1)
    expand = jnp.where(((row & 63) >> 1) == col, 1.0, 0.0).astype(BF16)
    a_all = _dot(expand, wphi_v[...].reshape(H * DH, DH), NT)
    row = lax.broadcasted_iota(jnp.int32, (128, D), 0)
    col = lax.broadcasted_iota(jnp.int32, (128, D), 1)
    a_all = jnp.where((2 * (row >> 6) + (row & 1)) == ((col >> 5) & 3), a_all, 0.0).astype(BF16)
    xn0 = ln_rows(0, T)
    h_v[0:T, :] = jnp.zeros((T, D), F32)

    def fold(j, c):
        out = []
        for s in range(RC // 128):
            g = c * (RC // 128) + s
            w = wraw_v[j * NC + c, :, s * 128:(s + 1) * 128]
            if j == 2:
                wt = w.T
            else:
                wt = (_dot(a_all[:, g * 128:(g + 1) * 128], w, NT) * LOG2E).astype(BF16)
            r0 = (j * D + g * 128) // 2
            wt_v[r0:r0 + 64, :] = pltpu.bitcast(wt, U32)
            out.append(wt)
        return out

    def wt_rows(r0, n):
        return pltpu.bitcast(wt_v[r0 // 2:(r0 + n) // 2, :], BF16)

    def k_features(pk, c, first):
        phis = []
        for j in range(PPC):
            pr = c * PPC + j
            ep, en, rp, rn = _dual_exp(pk[64 * j:64 * j + 64, :])
            phi = jnp.concatenate([e * rp for e in ep] + [e * rn for e in en], axis=0)
            zs = _lane_fold(phi)
            z_v[pr] = zs if first else z_v[pr] + zs
            phis.append(phi.astype(BF16))
        return phis

    def kv_update(vt, phis, c, first):
        vt = vt.astype(BF16)
        for j in range(PPC):
            pr = c * PPC + j
            upd = _dot(vt[64 * j:64 * j + 64, :], phis[j], NT)
            kvacc_v[pr] = upd if first else kvacc_v[pr] + upd

    def proj(ws, xn):
        return jnp.concatenate([_dot(w, xn, NT) for w in ws], axis=0)

    phis = [None] * NC
    w_copy(1, 0).wait()
    for c in range(NC):
        w_copy(0, c).start()
    pk0 = proj(fold(1, 0), xn0)
    w_copy(1, 1).wait()
    wo_copy.start()
    wr_copy.start()
    pk1 = proj(fold(1, 1), xn0)
    phis[0] = k_features(pk0, 0, True)
    w_copy(1, 2).wait()
    w_copy(1, 3).wait()
    wg_copy.start()
    wu_copy.start()
    wd_copy.start()
    wk2 = fold(1, 2)
    wk3 = fold(1, 3)
    pk2 = proj(wk2, xn0)
    phis[1] = k_features(pk1, 1, True)
    w_copy(2, 0).wait()
    w_copy(2, 1).wait()
    pk3 = proj(wk3, xn0)
    wv0 = fold(2, 0)
    wv1 = fold(2, 1)
    phis[2] = k_features(pk2, 2, True)
    vt0 = proj(wv0, xn0)
    phis[3] = k_features(pk3, 3, True)
    w_copy(2, 2).wait()
    w_copy(2, 3).wait()
    vt1 = proj(wv1, xn0)
    wv2 = fold(2, 2)
    wv3 = fold(2, 3)
    kv_update(vt0, phis[0], 0, True)
    vt2 = proj(wv2, xn0)
    x_copy(1).wait()
    vt3 = proj(wv3, xn0)
    kv_update(vt1, phis[1], 1, True)
    kv_update(vt2, phis[2], 2, True)
    kv_update(vt3, phis[3], 3, True)
    ln_rows(T, T)

    def phase1(t, carry):
        r0 = pl.multiple_of(t * T, T)
        tn = jnp.minimum(t + 1, NT_ - 1)
        never = t < 0

        @pl.when(t + 1 < NT_)
        def _():
            x_copy(tn).wait()

        xn = xn_v[pl.ds(r0, T), :]
        phis = []
        for c in range(NC):
            pk = _dot(wt_rows(D + c * RC, RC), xn, NT)
            phis.append(k_features(pk, c, False))
        vts = []
        anchors = [pk[RC - 8:RC, T - 128:T]]
        for c in range(NC):
            vts.append(_dot(wt_rows(2 * D + c * RC, RC), xn, NT))
            anchors += _anchors(vts[c])
            if c > 0:
                kv_update(vts[c - 1], phis[c - 1], c - 1, False)
        kv_update(vts[NC - 1], phis[NC - 1], NC - 1, False)
        rn = pl.multiple_of(tn * T, T)
        for k in range(T // LNC):
            ln_rows(rn + k * LNC, LNC, never, anchors[(k * LN1_SPAN) // (T // LNC)])
        return carry

    lax.fori_loop(1, NT_, phase1, 0)

    for c in range(NC):
        w_copy(0, c).wait()
    wo_copy.wait()
    wr_copy.wait()
    row = lax.broadcasted_iota(jnp.int32, (64, 128), 0)
    col = lax.broadcasted_iota(jnp.int32, (64, 128), 1)
    keep = (row >> 5) == (col & 1)
    for pr in range(NPAIR):
        kvbf_v[pr] = jnp.where(keep, kvacc_v[pr], 0.0).astype(BF16)
        z_v[pr] = jnp.broadcast_to(jnp.sum(z_v[pr], axis=-1, keepdims=True), (128, 128))
    for c in range(NC):
        fold(0, c)

    def o_copy(t):
        r0 = t * T if isinstance(t, int) else pl.multiple_of(t * T, T)
        return pltpu.make_async_copy(o_v.at[pl.ds(r0, T), :], out_hbm.at[pl.ds(r0, T), :], sem.at[SO + t])

    def finish_tile(t, valid, best, besti, never=None, anchors=None):
        r0 = t * T if isinstance(t, int) else pl.multiple_of(t * T, T)
        wr = wr_v[...].reshape(1, D).astype(F32)
        sub = lax.broadcasted_iota(jnp.int32, (8, 1), 0)
        for k in range(T // LNC):
            rows = pl.ds(r0 + k * LNC, LNC)
            anchor = None if anchors is None else anchors[(k * LN2_SPAN) // (T // LNC)]
            h = _tie(h_v[rows, :], never, anchor)
            m = jnp.mean(h, axis=-1, keepdims=True)
            hc = h - m
            rstd = lax.rsqrt(jnp.mean(hc * hc, axis=-1, keepdims=True) + LN_EPS)
            r = (jnp.sum(hc * wr, axis=-1, keepdims=True) * rstd).astype(BF16).astype(F32)
            o_v[rows, :] = (hc * (1.0 + rstd) + m).astype(BF16)
            if valid is not None:
                r = jnp.where(valid, r, -jnp.inf)
            for i in range(LNC // 8):
                ri = r[8 * i:8 * i + 8, :]
                better = ri > best
                best = jnp.where(better, ri, best)
                besti = jnp.where(better, sub + (r0 + k * LNC + 8 * i), besti)
        return best, besti

    def q_features(pq, c):
        phis = []
        for j in range(PPC):
            pr = c * PPC + j
            ep, en, rp, rn = _dual_exp(pq[64 * j:64 * j + 64, :])
            zz = [_lane_tile(z_v[pr, 8 * i:8 * i + 8, :], T // 128) for i in range(16)]
            ap = _pair_allreduce(_tree(jnp.add, [ep[i] * zz[i] for i in range(8)]), jnp.add)
            an = _pair_allreduce(_tree(jnp.add, [en[i] * zz[8 + i] for i in range(8)]), jnp.add)
            inv = 1.0 / (rp * ap + rn * an + 1e-6)
            sp = rp * inv
            sn = rn * inv
            phis.append(jnp.concatenate([e * sp for e in ep] + [e * sn for e in en], axis=0).astype(BF16))
        return phis

    def attn_rows(phis, c):
        return jnp.concatenate(
            [_dot(kvbf_v[c * PPC + j], phis[j], NN).astype(BF16) for j in range(PPC)], axis=0)

    def phase2(t, carry):
        best, besti = carry
        r0 = pl.multiple_of(t * T, T)
        tp = jnp.maximum(t - 1, 0)
        never = t < 0
        xn = xn_v[pl.ds(r0, T), :]
        phis, ots, anchors = [], [], []
        for c in range(NC):
            pq = _dot(wt_rows(c * RC, RC), xn, NT)
            anchors += _anchors(pq)
            phis.append(q_features(pq, c))
            if c > 0:
                ots.append(attn_rows(phis[c - 1], c - 1))
        o1 = jnp.concatenate(ots[:NC // 2], axis=0).T
        ha = _dot(o1, wo_v[0:D // 2, 0:D // 2], NN)
        ots.append(attn_rows(phis[NC - 1], NC - 1))
        hb = _dot(o1, wo_v[0:D // 2, D // 2:D], NN)
        anchors += _anchors(ha)[1::2] + _anchors(hb)[1::2]
        best, besti = finish_tile(tp, t > 0, best, besti, never, anchors)
        o2 = jnp.concatenate(ots[NC // 2:], axis=0).T
        h = (x_v[pl.ds(r0, T), :].astype(F32) + jnp.concatenate([ha, hb], axis=1)
             + _dot(o2, wo_v[D // 2:D, :], NN))
        h_v[pl.ds(r0, T), :] = h

        @pl.when(t > 0)
        def _():
            o_copy(tp).start()

        return best, besti

    best, besti = lax.fori_loop(
        0, NT_, phase2,
        (jnp.full((8, 1), -jnp.inf, F32), jnp.zeros((8, 1), jnp.int32)))
    wg_copy.wait()
    wu_copy.wait()
    wd_copy.wait()
    best, besti = finish_tile(NT_ - 1, None, best, besti)
    o_copy(NT_ - 1).start()

    rmax = jnp.max(best, axis=0, keepdims=True)
    idx = jnp.min(jnp.where(best == rmax, besti, S), axis=0, keepdims=True)
    idx_s = jnp.clip(idx[0, 0], 0, S - 1)
    blk = pl.multiple_of((idx_s >> 4) << 4, 16)
    hb = h_v[pl.ds(blk, 16), :]
    hnb = _layernorm(hb)
    xs = hnb.astype(BF16)
    g = _dot(xs, wg_v[...], NN)
    u = _dot(xs, wu_v[...], NN)
    a = (g * jax.nn.sigmoid(g) * u).astype(BF16)
    y = _dot(a, wd_v[:, 0:D], NN) * jax.nn.sigmoid(rmax)
    sel = lax.broadcasted_iota(jnp.int32, (16, 1), 0) == (idx_s - blk)
    patch_v[...] = (hb + hnb + jnp.where(sel, y, 0.0)).astype(BF16)
    for t in range(NT_):
        o_copy(t).wait()
    pc = pltpu.make_async_copy(patch_v, out_hbm.at[pl.ds(blk, 16), :], sem.at[SM + 3])
    pc.start()
    pc.wait()


@jax.jit
def pallas_sequential_preLN__linear_kernel_hedgehog__moe_arch_mod__prompt_kernel(
    A_x: jax.Array,
    A_wqkv: jax.Array,
    A_w_phi: jax.Array,
    A_wo: jax.Array,
    B_x: jax.Array,
    B_w_r: jax.Array,
    B_w_gate: jax.Array,
    B_w_up: jax.Array,
    B_w_down: jax.Array,
):
    del B_x
    hbm = pl.BlockSpec(memory_space=pl.ANY)
    out = pl.pallas_call(
        _kernel,
        out_shape=jax.ShapeDtypeStruct((S, D), BF16),
        in_specs=[hbm] * 8,
        out_specs=hbm,
        scratch_shapes=[
            pltpu.VMEM((S, D), BF16),
            pltpu.VMEM((S, D), BF16),
            pltpu.VMEM((3 * NC, D, RC), BF16),
            pltpu.VMEM((3 * D // 2, D), U32),
            pltpu.VMEM((H, DH, DH), BF16),
            pltpu.VMEM((D, D), BF16),
            pltpu.VMEM((D,), BF16),
            pltpu.VMEM((NPAIR, 64, 128), F32),
            pltpu.VMEM((NPAIR, 64, 128), BF16),
            pltpu.VMEM((NPAIR, 128, 128), F32),
            pltpu.VMEM((S, D), F32),
            pltpu.VMEM((S, D), BF16),
            pltpu.VMEM((D, FF), BF16),
            pltpu.VMEM((D, FF), BF16),
            pltpu.VMEM((FF, D + WD_PAD), BF16),
            pltpu.VMEM((16, D), BF16),
            pltpu.SemaphoreType.DMA((2 * NT_ + 3 * NC + 7,)),
        ],
        compiler_params=pltpu.CompilerParams(vmem_limit_bytes=100 * 1024 * 1024),
        name="hedgehog_mod",
    )(
        A_x.reshape(S, D),
        A_wqkv,
        A_w_phi,
        A_wo,
        B_w_r,
        B_w_gate,
        B_w_up,
        B_w_down,
    )
    return out.reshape(1, S, D)
```

```python
import jax
import jax.numpy as jnp
from jax import lax
import jax.experimental.pallas as pl
import jax.experimental.pallas.tpu as pltpu

F32 = jnp.float32
BF16 = jnp.bfloat16
U32 = jnp.uint32

S = 2048
D = 1024
H = 32
DH = 32
FF = 3584
NPAIR = H // 2
LOG2E = 1.4426950408889634
LN_EPS = 1e-5

T = 256
TH = T // 2
NT_ = S // T
RC = 256
NC = D // RC
PPC = RC // 64
LNC = 16
WD_PAD = 128

LN1_PLAN = tuple((k * 12 // 16, k * 12 // 16 + 3) for k in range(16))
LN2B_PLAN = ((None, 0), (None, 0), (None, 0), (1, 6), (3, 8), (5, 10), (7, 12), (9, 14))
LN2A_PLAN = ((None, 18), (None, 18), (16, 19), (17, 20), (18, 21), (19, 22), (20, 23), (21, None))
PARTS = "all"

NN = (((1,), (0,)), ((), ()))
NT = (((1,), (1,)), ((), ()))


def _dot(a, b, dims):
    return lax.dot_general(a, b, dims, preferred_element_type=F32)


def _recip(x):
    return pl.reciprocal(x, approx=False, full_range=False)


def _pack(x):
    return pltpu.bitcast(x, U32)


def _unpack(x):
    return pltpu.bitcast(x, BF16)


def _pair_allreduce(a, op):
    a = op(a, pltpu.roll(a, 2, 0))
    return op(a, pltpu.roll(a, 4, 0))


def _tree(op, xs):
    xs = list(xs)
    while len(xs) > 1:
        nxt = [op(xs[i], xs[i + 1]) for i in range(0, len(xs) - 1, 2)]
        if len(xs) % 2:
            nxt.append(xs[-1])
        xs = nxt
    return xs[0]


def _dual_exp(p):
    sl = [p[8 * i:8 * i + 8, :] for i in range(8)]
    mx = _pair_allreduce(_tree(jnp.maximum, sl), jnp.maximum)
    mn = _pair_allreduce(_tree(jnp.minimum, sl), jnp.minimum)
    ep = [jnp.exp2(s - mx) for s in sl]
    en = [jnp.exp2(mn - s) for s in sl]
    sp = _pair_allreduce(_tree(jnp.add, ep), jnp.add)
    sn = _pair_allreduce(_tree(jnp.add, en), jnp.add)
    return ep, en, sp, sn


def _after(x, never, anchor):
    if anchor is None:
        return x
    d = jnp.concatenate([anchor] * (x.shape[0] // 8), axis=0)
    return jnp.concatenate([jnp.where(never, d, x[:, :128]), x[:, 128:]], axis=1)


def _gate(x, never, deps):
    for i, dep in enumerate(deps):
        d = jnp.broadcast_to(dep, (8, 128))
        if x.dtype != F32:
            d = pltpu.bitcast(d, x.dtype)
        blk = jnp.where(never, d, x[8 * i:8 * i + 8, :128])
        if x.shape[1] > 128:
            blk = jnp.concatenate([blk, x[8 * i:8 * i + 8, 128:]], axis=1)
        parts = ([x[:8 * i, :]] if i else []) + [blk, x[8 * i + 8:, :]]
        x = jnp.concatenate(parts, axis=0)
    return x


def _lane_fold(a):
    return _tree(jnp.add, [a[:, 128 * i:128 * i + 128] for i in range(a.shape[1] // 128)])


def _row_sum(a):
    return jnp.sum(_lane_fold(a), axis=-1, keepdims=True)


def _lane_tile(a, n):
    return a if n == 1 else jnp.concatenate([a] * n, axis=1)


class _Side:
    def __init__(self, never):
        self.never = never
        self.jobs = []
        self.deps = {}

    def add(self, plan, fn):
        for k, (rel, due) in enumerate(plan):
            if rel is None:
                self._run(due, fn, k, None)
            else:
                self.jobs.append((rel, due, fn, k))

    def _run(self, due, fn, k, anchor):
        dep = fn(k, anchor)
        if due is not None:
            self.deps.setdefault(due, []).append(dep)

    def gate(self, step, x):
        return _gate(x, self.never, self.deps.pop(step, []))

    def done(self, step, res):
        anchor = res[res.shape[0] - 8:, res.shape[1] - 128:]
        for job in [j for j in self.jobs if j[0] == step]:
            self.jobs.remove(job)
            self._run(job[1], job[2], job[3], anchor)


def _kernel(x_hbm, wqkv_hbm, wphi_hbm, wo_hbm, wr_hbm, wg_hbm, wu_hbm, wd_hbm, out_hbm,
            x_v, xn_v, wraw_v, wt_v, wphi_v, woraw_v, wo_v, wrraw_v, wr_v, kvacc_v, kvbf_v, z_v, phi_v,
            ha_v, hb_v, hn_v, o_v, wg_v, wu_v, wd_v, patch_v,
            sem):
    SX, SW, SO, SM = 0, NT_, NT_ + 3 * NC, 2 * NT_ + 3 * NC + 1

    def x_copy(i):
        return pltpu.make_async_copy(x_hbm.at[pl.ds(i * T, T), :], x_v.at[pl.ds(i * T, T), :], sem.at[SX + i])

    def w_copy(j, c):
        return pltpu.make_async_copy(wqkv_hbm.at[:, pl.ds(j * D + c * RC, RC)], wraw_v.at[j * NC + c],
                                     sem.at[SW + j * NC + c])

    wphi_copy = pltpu.make_async_copy(wphi_hbm, wphi_v, sem.at[SM + 4])
    wr_copy = pltpu.make_async_copy(wr_hbm, wrraw_v, sem.at[SM + 5])
    wo_copy = pltpu.make_async_copy(wo_hbm, woraw_v, sem.at[SM + 6])
    wg_copy = pltpu.make_async_copy(wg_hbm, wg_v, sem.at[SM + 0])
    wu_copy = pltpu.make_async_copy(wu_hbm, wu_v, sem.at[SM + 1])
    wd_copy = pltpu.make_async_copy(wd_hbm, wd_v.at[:, pl.ds(0, D)], sem.at[SM + 2])

    wphi_copy.start()
    x_copy(0).start()
    for c in range(NC):
        w_copy(1, c).start()
    for c in range(NC):
        w_copy(2, c).start()
    x_copy(1).start()

    def half(r):
        return r // 2 if isinstance(r, int) else pl.multiple_of(r // 2, LNC // 2)

    def ln_rows(r0, n, never=None, anchor=None):
        x = _after(x_v[pl.ds(r0, n), :].astype(F32), never, anchor)
        xc = x - _row_sum(x) * (1.0 / D)
        rstd = lax.rsqrt(_row_sum(xc * xc) * (1.0 / D) + LN_EPS)
        xn_v[pl.ds(half(r0), n // 2), :] = _pack((xc * rstd).astype(BF16))
        return _tree(jnp.add, [rstd[8 * i:8 * i + 8, :] for i in range(min(n, LNC) // 8)])

    def xn_tile(r0):
        return _unpack(xn_v[pl.ds(half(r0), T // 2), :])

    wphi_copy.wait()
    x_copy(0).wait()
    for i in range(2, NT_):
        x_copy(i).start()

    row = lax.broadcasted_iota(jnp.int32, (128, DH), 0)
    col = lax.broadcasted_iota(jnp.int32, (128, DH), 1)
    expand = jnp.where(((row & 63) >> 1) == col, 1.0, 0.0).astype(BF16)
    a_all = _dot(expand, wphi_v[...].reshape(H * DH, DH), NT)
    row = lax.broadcasted_iota(jnp.int32, (128, 128), 0)
    col = lax.broadcasted_iota(jnp.int32, (128, 128), 1)
    a_keep = (2 * (row >> 6) + (row & 1)) == (col >> 5)
    a_mats = [jnp.where(a_keep, a_all[:, g * 128:(g + 1) * 128], 0.0).astype(BF16) for g in range(8)]
    ln_rows(0, T)
    hb_v[...] = jnp.zeros((TH, D), F32)

    def fold(j, c):
        for s in range(RC // 128):
            g = c * (RC // 128) + s
            w = wraw_v[j * NC + c, :, s * 128:(s + 1) * 128]
            if j == 2:
                wt = w.T
            else:
                wt = (_dot(a_mats[g], w, NT) * LOG2E).astype(BF16)
            r0 = (j * D + g * 128) // 2
            wt_v[r0:r0 + 64, :] = _pack(wt)

    def wt_rows(j, c):
        r0 = (j * D + c * RC) // 2
        return wt_v[r0:r0 + RC // 2, :]

    def k_features(pk, c, first):
        for j in range(PPC):
            pr = c * PPC + j
            ep, en, sp, sn = _dual_exp(pk[64 * j:64 * j + 64, :])
            inv = _recip(sp * sn)
            rp = sn * inv
            rn = sp * inv
            phi = jnp.concatenate([e * rp for e in ep] + [e * rn for e in en], axis=0)
            zs = _lane_fold(phi)
            z_v[pr] = zs if first else z_v[pr] + zs
            phi_v[64 * pr:64 * pr + 64, :] = _pack(phi.astype(BF16))

    def kv_update(vt, c, first):
        for j in range(PPC):
            pr = c * PPC + j
            upd = _dot(vt[64 * j:64 * j + 64, :].astype(BF16), _unpack(phi_v[64 * pr:64 * pr + 64, :]), NT)
            kvacc_v[pr] = upd if first else kvacc_v[pr] + upd

    def proj0(j, c):
        return _dot(_unpack(wt_rows(j, c)), xn_tile(0), NT)

    w_copy(1, 0).wait()
    for c in range(NC):
        w_copy(0, c).start()
    fold(1, 0)
    pk0 = proj0(1, 0)
    w_copy(1, 1).wait()
    wo_copy.start()
    wr_copy.start()
    fold(1, 1)
    pk1 = proj0(1, 1)
    k_features(pk0, 0, True)
    w_copy(1, 2).wait()
    w_copy(1, 3).wait()
    wg_copy.start()
    wu_copy.start()
    wd_copy.start()
    fold(1, 2)
    fold(1, 3)
    pk2 = proj0(1, 2)
    k_features(pk1, 1, True)
    w_copy(2, 0).wait()
    w_copy(2, 1).wait()
    pk3 = proj0(1, 3)
    fold(2, 0)
    fold(2, 1)
    k_features(pk2, 2, True)
    vt0 = proj0(2, 0)
    k_features(pk3, 3, True)
    w_copy(2, 2).wait()
    w_copy(2, 3).wait()
    vt1 = proj0(2, 1)
    fold(2, 2)
    fold(2, 3)
    kv_update(vt0, 0, True)
    vt2 = proj0(2, 2)
    x_copy(1).wait()
    vt3 = proj0(2, 3)
    kv_update(vt1, 1, True)
    kv_update(vt2, 2, True)
    kv_update(vt3, 3, True)
    ln_rows(T, T)

    def phase1(t, carry):
        r0 = pl.multiple_of(t * T, T)
        tn = jnp.minimum(t + 1, NT_ - 1)
        rn = pl.multiple_of(tn * T, T)
        side = _Side(t < 0)

        @pl.when(t + 1 < NT_)
        def _():
            x_copy(tn).wait()

        xn = xn_tile(r0)
        for c in range(NC):
            pk = _dot(_unpack(wt_rows(1, c)), xn, NT)
            k_features(pk, c, False)
        side.add(LN1_PLAN, lambda k, a: ln_rows(rn + k * LNC, LNC, side.never, a))
        side.done(0, pk)
        vts = []
        for c in range(NC):
            w = wt_rows(2, c)
            quarters = []
            for n in range(2):
                for m in range(2):
                    step = 4 * c + 2 * n + m + 1
                    wq = side.gate(step, w[m * (RC // 4):(m + 1) * (RC // 4), :])
                    res = _dot(_unpack(wq), xn[n * TH:(n + 1) * TH, :], NT)
                    side.done(step, res)
                    quarters.append(res)
            vts.append(jnp.concatenate(
                [jnp.concatenate([quarters[0], quarters[2]], axis=1),
                 jnp.concatenate([quarters[1], quarters[3]], axis=1)], axis=0))
            if c > 0:
                kv_update(vts[c - 1], c - 1, False)
        kv_update(vts[NC - 1], NC - 1, False)
        return carry

    lax.fori_loop(1, NT_, phase1, 0)

    for c in range(NC):
        w_copy(0, c).wait()
    wo_copy.wait()
    wr_copy.wait()
    row = lax.broadcasted_iota(jnp.int32, (64, 128), 0)
    col = lax.broadcasted_iota(jnp.int32, (64, 128), 1)
    keep = (row >> 5) == (col & 1)
    for pr in range(NPAIR):
        kvbf_v[32 * pr:32 * pr + 32, :] = _pack(jnp.where(keep, kvacc_v[pr], 0.0).astype(BF16))
        z_v[pr] = jnp.broadcast_to(jnp.sum(z_v[pr], axis=-1, keepdims=True), (128, 128))
    for c in range(NC):
        fold(0, c)
    wo_v[...] = _pack(woraw_v[...])
    wr_v[...] = jnp.broadcast_to(wrraw_v[...].reshape(1, D).astype(F32), (8, D))

    def o_copy(r0, n, i):
        return pltpu.make_async_copy(o_v.at[pl.ds(r0, n), :], out_hbm.at[pl.ds(r0, n), :], sem.at[SO + i])

    def finish_rows(h_ref, k, r0, valid, st, never=None, anchor=None):
        best, besti = st["route"]
        wr = jnp.concatenate([wr_v[...]] * (LNC // 8), axis=0)
        sub = lax.broadcasted_iota(jnp.int32, (8, 1), 0)
        h = _after(h_ref[k * LNC:(k + 1) * LNC, :], never, anchor)
        m = _row_sum(h) * (1.0 / D)
        hc = h - m
        rstd = lax.rsqrt(_row_sum(hc * hc) * (1.0 / D) + LN_EPS)
        r = (_row_sum(hc * wr) * rstd).astype(BF16).astype(F32)
        hn = hc * rstd
        hn_v[pl.ds(half(r0), LNC // 2), :] = _pack(hn.astype(BF16))
        o_v[pl.ds(r0, LNC), :] = (hn + h).astype(BF16)
        if valid is not None:
            r = jnp.where(valid, r, -jnp.inf)
        for i in range(LNC // 8):
            ri = r[8 * i:8 * i + 8, :]
            better = ri > best
            best = jnp.where(better, ri, best)
            besti = jnp.where(better, sub + (r0 + 8 * i), besti)
        st["route"] = (best, besti)
        return best

    def q_features(pq, c):
        for j in range(PPC):
            pr = c * PPC + j
            ep, en, sp, sn = _dual_exp(pq[64 * j:64 * j + 64, :])
            zz = [_lane_tile(z_v[pr, 8 * i:8 * i + 8, :], pq.shape[1] // 128) for i in range(16)]
            ap = _pair_allreduce(_tree(jnp.add, [ep[i] * zz[i] for i in range(8)]), jnp.add)
            an = _pair_allreduce(_tree(jnp.add, [en[i] * zz[8 + i] for i in range(8)]), jnp.add)
            inv = _recip(ap * sn + (an + 1e-6 * sn) * sp)
            rp = sn * inv
            rn = sp * inv
            phi = jnp.concatenate([e * rp for e in ep] + [e * rn for e in en], axis=0)
            phi_v[64 * pr:64 * pr + 64, :] = _pack(phi.astype(BF16))

    def attn_rows(c, lo, hi):
        res = jnp.concatenate(
            [_dot(_unpack(kvbf_v[32 * pr:32 * pr + 32, :]), _unpack(phi_v[64 * pr:64 * pr + 64, lo:hi]), NN)
             for pr in range(c * PPC, (c + 1) * PPC)], axis=0)
        return res.astype(BF16).T

    def out_proj(side, step0, o, k0, k1):
        cols = []
        for n in range(D // 128):
            w = side.gate(step0 + n, wo_v[k0 // 2:k1 // 2, n * 128:(n + 1) * 128])
            res = _dot(o, _unpack(w), NN)
            side.done(step0 + n, res)
            cols.append(res)
        return jnp.concatenate(cols, axis=1)

    def phase2(t, carry):
        r0 = pl.multiple_of(t * T, T)
        rb = pl.multiple_of(jnp.maximum(r0 - TH, 0), TH)
        side = _Side(t < 0)
        st = {"route": carry}
        side.add(LN2B_PLAN, lambda k, a: finish_rows(hb_v, k, rb + k * LNC, t > 0, st, side.never, a))

        xn = xn_tile(r0)
        os_ = []
        for c in range(NC):
            pq = _dot(_unpack(wt_rows(0, c)), xn, NT)
            if c == 0:
                pq = side.gate(0, pq)
            q_features(pq, c)
            if c > 0:
                os_.append(attn_rows(c - 1, 0, T))
        o3a = attn_rows(NC - 1, 0, TH)
        ha = out_proj(side, 0, jnp.concatenate([o[0:TH, :] for o in os_[:2]], axis=1), 0, D // 2)
        o3b = attn_rows(NC - 1, TH, T)
        ha = ha + x_v[pl.ds(r0, TH), :].astype(F32)
        ha_v[...] = ha + out_proj(side, 8, jnp.concatenate([os_[2][0:TH, :], o3a], axis=1), D // 2, D)
        side.add(LN2A_PLAN, lambda k, a: finish_rows(ha_v, k, r0 + k * LNC, None, st, side.never, a))
        ob = jnp.concatenate([o[TH:T, :] for o in os_] + [o3b], axis=1)
        hb_v[...] = x_v[pl.ds(r0 + TH, TH), :].astype(F32) + out_proj(side, 16, ob, 0, D)

        @pl.when(t == 0)
        def _():
            o_copy(0, TH, 0).start()

        @pl.when(t > 0)
        def _():
            o_copy(rb, T, t).start()

        return st["route"]

    route = lax.fori_loop(
        0, NT_, phase2,
        (jnp.full((8, 1), -jnp.inf, F32), jnp.zeros((8, 1), jnp.int32)))
    wg_copy.wait()
    wu_copy.wait()
    wd_copy.wait()
    st = {"route": route}
    for k in range(TH // LNC):
        finish_rows(hb_v, k, S - TH + k * LNC, None, st)
    best, besti = st["route"]
    o_copy(S - TH, TH, NT_).start()

    rmax = jnp.max(best, axis=0, keepdims=True)
    idx = jnp.min(jnp.where(best == rmax, besti, S), axis=0, keepdims=True)
    idx_s = jnp.clip(idx[0, 0], 0, S - 1)
    blk = pl.multiple_of((idx_s >> 4) << 4, 16)
    xs = _unpack(hn_v[pl.ds(pl.multiple_of(blk >> 1, 8), 8), :])
    g = _dot(xs, wg_v[...], NN)
    u = _dot(xs, wu_v[...], NN)
    a = (g * jax.nn.sigmoid(g) * u).astype(BF16)
    y = _dot(a, wd_v[:, 0:D], NN) * jax.nn.sigmoid(rmax)
    sel = lax.broadcasted_iota(jnp.int32, (16, 1), 0) == (idx_s - blk)
    patch_v[...] = (o_v[pl.ds(blk, 16), :].astype(F32) + jnp.where(sel, y, 0.0)).astype(BF16)
    o_copy(0, TH, 0).wait()
    for t in range(1, NT_):
        o_copy(t * T - TH, T, t).wait()
    o_copy(S - TH, TH, NT_).wait()
    pc = pltpu.make_async_copy(patch_v, out_hbm.at[pl.ds(blk, 16), :], sem.at[SM + 3])
    pc.start()
    pc.wait()


@jax.jit
def pallas_sequential_preLN__linear_kernel_hedgehog__moe_arch_mod__prompt_kernel(
    A_x: jax.Array,
    A_wqkv: jax.Array,
    A_w_phi: jax.Array,
    A_wo: jax.Array,
    B_x: jax.Array,
    B_w_r: jax.Array,
    B_w_gate: jax.Array,
    B_w_up: jax.Array,
    B_w_down: jax.Array,
):
    del B_x
    hbm = pl.BlockSpec(memory_space=pl.ANY)
    out = pl.pallas_call(
        _kernel,
        out_shape=jax.ShapeDtypeStruct((S, D), BF16),
        in_specs=[hbm] * 8,
        out_specs=hbm,
        scratch_shapes=[
            pltpu.VMEM((S, D), BF16),
            pltpu.VMEM((S // 2, D), U32),
            pltpu.VMEM((3 * NC, D, RC), BF16),
            pltpu.VMEM((3 * D // 2, D), U32),
            pltpu.VMEM((H, DH, DH), BF16),
            pltpu.VMEM((D, D), BF16),
            pltpu.VMEM((D // 2, D), U32),
            pltpu.VMEM((D,), BF16),
            pltpu.VMEM((8, D), F32),
            pltpu.VMEM((NPAIR, 64, 128), F32),
            pltpu.VMEM((NPAIR * 32, 128), U32),
            pltpu.VMEM((NPAIR, 128, 128), F32),
            pltpu.VMEM((NPAIR * 64, T), U32),
            pltpu.VMEM((TH, D), F32),
            pltpu.VMEM((TH, D), F32),
            pltpu.VMEM((S // 2, D), U32),
            pltpu.VMEM((S, D), BF16),
            pltpu.VMEM((D, FF), BF16),
            pltpu.VMEM((D, FF), BF16),
            pltpu.VMEM((FF, D + WD_PAD), BF16),
            pltpu.VMEM((16, D), BF16),
            pltpu.SemaphoreType.DMA((2 * NT_ + 3 * NC + 8,)),
        ],
        compiler_params=pltpu.CompilerParams(vmem_limit_bytes=100 * 1024 * 1024),
        name="hedgehog_mod",
    )(
        A_x.reshape(S, D),
        A_wqkv,
        A_w_phi,
        A_wo,
        B_w_r,
        B_w_gate,
        B_w_up,
        B_w_down,
    )
    return out.reshape(1, S, D)
```

```python
import jax
import jax.numpy as jnp
from jax import lax
import jax.experimental.pallas as pl
import jax.experimental.pallas.tpu as pltpu

F32 = jnp.float32
BF16 = jnp.bfloat16
U32 = jnp.uint32

S = 2048
D = 1024
H = 32
DH = 32
FF = 3584
NPAIR = H // 2
LOG2E = 1.4426950408889634
LN_EPS = 1e-5

T = 256
TH = T // 2
NT_ = S // T
RC = 256
NC = D // RC
PPC = RC // 64
LNC = 16
WD_PAD = 128

LN1_PLAN = tuple((k * 12 // 16, k * 12 // 16 + 3) for k in range(16))
LN2B_PLAN = ((None, 0), (None, 0), (None, 0), (1, 6), (3, 8), (5, 10), (7, 12), (9, 14))
LN2A_PLAN = ((None, 18), (None, 18), (16, 19), (17, 20), (18, 21), (19, 22), (20, 23), (21, None))
UNROLL2 = 2

NN = (((1,), (0,)), ((), ()))
NT = (((1,), (1,)), ((), ()))


def _dot(a, b, dims):
    return lax.dot_general(a, b, dims, preferred_element_type=F32)


def _recip(x):
    return pl.reciprocal(x, approx=False, full_range=False)


def _pack(x):
    return pltpu.bitcast(x, U32)


def _unpack(x):
    return pltpu.bitcast(x, BF16)


def _pair_allreduce(a, op):
    a = op(a, pltpu.roll(a, 2, 0))
    return op(a, pltpu.roll(a, 4, 0))


def _tree(op, xs):
    xs = list(xs)
    while len(xs) > 1:
        nxt = [op(xs[i], xs[i + 1]) for i in range(0, len(xs) - 1, 2)]
        if len(xs) % 2:
            nxt.append(xs[-1])
        xs = nxt
    return xs[0]


def _dual_exp(p):
    sl = [p[8 * i:8 * i + 8, :] for i in range(8)]
    mx = _pair_allreduce(_tree(jnp.maximum, sl), jnp.maximum)
    mn = _pair_allreduce(_tree(jnp.minimum, sl), jnp.minimum)
    ep = [jnp.exp2(s - mx) for s in sl]
    en = [jnp.exp2(mn - s) for s in sl]
    sp = _pair_allreduce(_tree(jnp.add, ep), jnp.add)
    sn = _pair_allreduce(_tree(jnp.add, en), jnp.add)
    return ep, en, sp, sn


def _after(x, never, anchor):
    if anchor is None:
        return x
    d = jnp.concatenate([anchor] * (x.shape[0] // 8), axis=0)
    return jnp.concatenate([jnp.where(never, d, x[:, :128]), x[:, 128:]], axis=1)


def _gate(x, never, deps):
    for i, dep in enumerate(deps):
        d = jnp.broadcast_to(dep, (8, 128))
        if x.dtype != F32:
            d = pltpu.bitcast(d, x.dtype)
        blk = jnp.where(never, d, x[8 * i:8 * i + 8, :128])
        if x.shape[1] > 128:
            blk = jnp.concatenate([blk, x[8 * i:8 * i + 8, 128:]], axis=1)
        parts = ([x[:8 * i, :]] if i else []) + [blk, x[8 * i + 8:, :]]
        x = jnp.concatenate(parts, axis=0)
    return x


def _lane_fold(a):
    return _tree(jnp.add, [a[:, 128 * i:128 * i + 128] for i in range(a.shape[1] // 128)])


def _row_sum(a):
    return jnp.sum(_lane_fold(a), axis=-1, keepdims=True)


def _lane_tile(a, n):
    return a if n == 1 else jnp.concatenate([a] * n, axis=1)


class _Side:
    def __init__(self, never):
        self.never = never
        self.jobs = []
        self.deps = {}

    def add(self, plan, fn):
        for k, (rel, due) in enumerate(plan):
            if rel is None:
                self._run(due, fn, k, None)
            else:
                self.jobs.append((rel, due, fn, k))

    def _run(self, due, fn, k, anchor):
        dep = fn(k, anchor)
        if due is not None:
            self.deps.setdefault(due, []).append(dep)

    def gate(self, step, x):
        return _gate(x, self.never, self.deps.pop(step, []))

    def done(self, step, res):
        anchor = res[res.shape[0] - 8:, res.shape[1] - 128:]
        for job in [j for j in self.jobs if j[0] == step]:
            self.jobs.remove(job)
            self._run(job[1], job[2], job[3], anchor)


def _kernel(x_hbm, wqkv_hbm, wphi_hbm, wo_hbm, wr_hbm, wg_hbm, wu_hbm, wd_hbm, out_hbm,
            x_v, xn_v, wraw_v, wt_v, wphi_v, woraw_v, wo_v, wrraw_v, wr_v, kvacc_v, kvbf_v, z_v, phi_v,
            ha_v, hb_v, hn_v, o_v, wg_v, wu_v, wd_v, patch_v,
            sem):
    SX, SW, SO, SM = 0, NT_, NT_ + 3 * NC, 2 * NT_ + 3 * NC + 1

    def x_copy(i):
        return pltpu.make_async_copy(x_hbm.at[pl.ds(i * T, T), :], x_v.at[pl.ds(i * T, T), :], sem.at[SX + i])

    def w_copy(j, c):
        return pltpu.make_async_copy(wqkv_hbm.at[:, pl.ds(j * D + c * RC, RC)], wraw_v.at[j * NC + c],
                                     sem.at[SW + j * NC + c])

    wphi_copy = pltpu.make_async_copy(wphi_hbm, wphi_v, sem.at[SM + 4])
    wr_copy = pltpu.make_async_copy(wr_hbm, wrraw_v, sem.at[SM + 5])
    wo_copy = pltpu.make_async_copy(wo_hbm, woraw_v, sem.at[SM + 6])
    wg_copy = pltpu.make_async_copy(wg_hbm, wg_v, sem.at[SM + 0])
    wu_copy = pltpu.make_async_copy(wu_hbm, wu_v, sem.at[SM + 1])
    wd_copy = pltpu.make_async_copy(wd_hbm, wd_v.at[:, pl.ds(0, D)], sem.at[SM + 2])

    wphi_copy.start()
    x_copy(0).start()
    for c in range(NC):
        w_copy(1, c).start()
    for c in range(NC):
        w_copy(2, c).start()
    x_copy(1).start()

    def half(r):
        return r // 2 if isinstance(r, int) else pl.multiple_of(r // 2, LNC // 2)

    def ln_rows(r0, n, never=None, anchor=None):
        x = _after(x_v[pl.ds(r0, n), :].astype(F32), never, anchor)
        xc = x - _row_sum(x) * (1.0 / D)
        rstd = lax.rsqrt(_row_sum(xc * xc) * (1.0 / D) + LN_EPS)
        xn_v[pl.ds(half(r0), n // 2), :] = _pack((xc * rstd).astype(BF16))
        return _tree(jnp.add, [rstd[8 * i:8 * i + 8, :] for i in range(min(n, LNC) // 8)])

    def xn_tile(r0):
        return _unpack(xn_v[pl.ds(half(r0), T // 2), :])

    wphi_copy.wait()
    x_copy(0).wait()
    for i in range(2, NT_):
        x_copy(i).start()

    row = lax.broadcasted_iota(jnp.int32, (128, DH), 0)
    col = lax.broadcasted_iota(jnp.int32, (128, DH), 1)
    expand = jnp.where(((row & 63) >> 1) == col, 1.0, 0.0).astype(BF16)
    a_all = _dot(expand, wphi_v[...].reshape(H * DH, DH), NT)
    row = lax.broadcasted_iota(jnp.int32, (128, 128), 0)
    col = lax.broadcasted_iota(jnp.int32, (128, 128), 1)
    a_keep = (2 * (row >> 6) + (row & 1)) == (col >> 5)
    a_mats = [jnp.where(a_keep, a_all[:, g * 128:(g + 1) * 128], 0.0).astype(BF16) for g in range(8)]
    ln_rows(0, T)
    hb_v[...] = jnp.zeros((TH, D), F32)

    def fold(j, c):
        for s in range(RC // 128):
            g = c * (RC // 128) + s
            w = wraw_v[j * NC + c, :, s * 128:(s + 1) * 128]
            if j == 2:
                wt = w.T
            else:
                wt = (_dot(a_mats[g], w, NT) * LOG2E).astype(BF16)
            r0 = (j * D + g * 128) // 2
            wt_v[r0:r0 + 64, :] = _pack(wt)

    def wt_rows(j, c):
        r0 = (j * D + c * RC) // 2
        return wt_v[r0:r0 + RC // 2, :]

    def k_features(pk, c, first):
        for j in range(PPC):
            pr = c * PPC + j
            ep, en, sp, sn = _dual_exp(pk[64 * j:64 * j + 64, :])
            inv = _recip(sp * sn)
            rp = sn * inv
            rn = sp * inv
            phi = jnp.concatenate([e * rp for e in ep] + [e * rn for e in en], axis=0)
            zs = _lane_fold(phi)
            z_v[pr] = zs if first else z_v[pr] + zs
            phi_v[64 * pr:64 * pr + 64, :] = _pack(phi.astype(BF16))

    def kv_update(vt, c, first):
        for j in range(PPC):
            pr = c * PPC + j
            upd = _dot(vt[64 * j:64 * j + 64, :].astype(BF16), _unpack(phi_v[64 * pr:64 * pr + 64, :]), NT)
            kvacc_v[pr] = upd if first else kvacc_v[pr] + upd

    def proj0(j, c):
        return _dot(_unpack(wt_rows(j, c)), xn_tile(0), NT)

    w_copy(1, 0).wait()
    for c in range(NC):
        w_copy(0, c).start()
    fold(1, 0)
    pk0 = proj0(1, 0)
    w_copy(1, 1).wait()
    wo_copy.start()
    wr_copy.start()
    fold(1, 1)
    pk1 = proj0(1, 1)
    k_features(pk0, 0, True)
    w_copy(1, 2).wait()
    w_copy(1, 3).wait()
    wg_copy.start()
    wu_copy.start()
    wd_copy.start()
    fold(1, 2)
    fold(1, 3)
    pk2 = proj0(1, 2)
    k_features(pk1, 1, True)
    w_copy(2, 0).wait()
    w_copy(2, 1).wait()
    pk3 = proj0(1, 3)
    fold(2, 0)
    fold(2, 1)
    k_features(pk2, 2, True)
    vt0 = proj0(2, 0)
    k_features(pk3, 3, True)
    w_copy(2, 2).wait()
    w_copy(2, 3).wait()
    vt1 = proj0(2, 1)
    fold(2, 2)
    fold(2, 3)
    kv_update(vt0, 0, True)
    vt2 = proj0(2, 2)
    x_copy(1).wait()
    vt3 = proj0(2, 3)
    kv_update(vt1, 1, True)
    kv_update(vt2, 2, True)
    kv_update(vt3, 3, True)
    ln_rows(T, T)

    def phase1(t, carry):
        r0 = pl.multiple_of(t * T, T)
        tn = jnp.minimum(t + 1, NT_ - 1)
        rn = pl.multiple_of(tn * T, T)
        side = _Side(t < 0)

        @pl.when(t + 1 < NT_)
        def _():
            x_copy(tn).wait()

        xn = xn_tile(r0)
        for c in range(NC):
            pk = _dot(_unpack(wt_rows(1, c)), xn, NT)
            k_features(pk, c, False)
        side.add(LN1_PLAN, lambda k, a: ln_rows(rn + k * LNC, LNC, side.never, a))
        side.done(0, pk)
        vts = []
        for c in range(NC):
            w = wt_rows(2, c)
            quarters = []
            for n in range(2):
                for m in range(2):
                    step = 4 * c + 2 * n + m + 1
                    wq = side.gate(step, w[m * (RC // 4):(m + 1) * (RC // 4), :])
                    res = _dot(_unpack(wq), xn[n * TH:(n + 1) * TH, :], NT)
                    side.done(step, res)
                    quarters.append(res)
            vts.append(jnp.concatenate(
                [jnp.concatenate([quarters[0], quarters[2]], axis=1),
                 jnp.concatenate([quarters[1], quarters[3]], axis=1)], axis=0))
            if c > 0:
                kv_update(vts[c - 1], c - 1, False)
        kv_update(vts[NC - 1], NC - 1, False)
        return carry

    lax.fori_loop(1, NT_, phase1, 0)

    for c in range(NC):
        w_copy(0, c).wait()
    wo_copy.wait()
    wr_copy.wait()
    row = lax.broadcasted_iota(jnp.int32, (64, 128), 0)
    col = lax.broadcasted_iota(jnp.int32, (64, 128), 1)
    keep = (row >> 5) == (col & 1)
    for pr in range(NPAIR):
        kvbf_v[32 * pr:32 * pr + 32, :] = _pack(jnp.where(keep, kvacc_v[pr], 0.0).astype(BF16))
        z_v[pr] = jnp.broadcast_to(jnp.sum(z_v[pr], axis=-1, keepdims=True), (128, 128))
    for c in range(NC):
        fold(0, c)
    wo_v[...] = _pack(woraw_v[...])
    wr_v[...] = jnp.broadcast_to(wrraw_v[...].reshape(1, D).astype(F32), (8, D))

    def o_copy(r0, n, i):
        return pltpu.make_async_copy(o_v.at[pl.ds(r0, n), :], out_hbm.at[pl.ds(r0, n), :], sem.at[SO + i])

    def finish_rows(h_ref, k, r0, valid, st, never=None, anchor=None):
        best, besti = st["route"]
        wr = jnp.concatenate([wr_v[...]] * (LNC // 8), axis=0)
        sub = lax.broadcasted_iota(jnp.int32, (8, 1), 0)
        h = _after(h_ref[k * LNC:(k + 1) * LNC, :], never, anchor)
        m = _row_sum(h) * (1.0 / D)
        hc = h - m
        rstd = lax.rsqrt(_row_sum(hc * hc) * (1.0 / D) + LN_EPS)
        r = (_row_sum(hc * wr) * rstd).astype(BF16).astype(F32)
        hn = hc * rstd
        hn_v[pl.ds(half(r0), LNC // 2), :] = _pack(hn.astype(BF16))
        o_v[pl.ds(r0, LNC), :] = (hn + h).astype(BF16)
        if valid is not None:
            r = jnp.where(valid, r, -jnp.inf)
        for i in range(LNC // 8):
            ri = r[8 * i:8 * i + 8, :]
            better = ri > best
            best = jnp.where(better, ri, best)
            besti = jnp.where(better, sub + (r0 + 8 * i), besti)
        st["route"] = (best, besti)
        return best

    def q_features(pq, c):
        for j in range(PPC):
            pr = c * PPC + j
            ep, en, sp, sn = _dual_exp(pq[64 * j:64 * j + 64, :])
            zz = [_lane_tile(z_v[pr, 8 * i:8 * i + 8, :], pq.shape[1] // 128) for i in range(16)]
            ap = _pair_allreduce(_tree(jnp.add, [ep[i] * zz[i] for i in range(8)]), jnp.add)
            an = _pair_allreduce(_tree(jnp.add, [en[i] * zz[8 + i] for i in range(8)]), jnp.add)
            inv = _recip(ap * sn + (an + 1e-6 * sn) * sp)
            rp = sn * inv
            rn = sp * inv
            phi = jnp.concatenate([e * rp for e in ep] + [e * rn for e in en], axis=0)
            phi_v[64 * pr:64 * pr + 64, :] = _pack(phi.astype(BF16))

    def attn_rows(c, lo, hi):
        res = jnp.concatenate(
            [_dot(_unpack(kvbf_v[32 * pr:32 * pr + 32, :]), _unpack(phi_v[64 * pr:64 * pr + 64, lo:hi]), NN)
             for pr in range(c * PPC, (c + 1) * PPC)], axis=0)
        return res.astype(BF16).T

    def out_proj(side, step0, o, k0, k1):
        cols = []
        for n in range(D // 128):
            w = side.gate(step0 + n, wo_v[k0 // 2:k1 // 2, n * 128:(n + 1) * 128])
            res = _dot(o, _unpack(w), NN)
            side.done(step0 + n, res)
            cols.append(res)
        return jnp.concatenate(cols, axis=1)

    def phase2(u, carry):
        for i in range(UNROLL2):
            carry = phase2_tile(u * UNROLL2 + i, carry, u < 0)

        r0 = pl.multiple_of(u * (UNROLL2 * T), T)

        @pl.when(u == 0)
        def _():
            o_copy(0, UNROLL2 * T - TH, 0).start()

        @pl.when(u > 0)
        def _():
            o_copy(pl.multiple_of(jnp.maximum(r0 - TH, 0), TH), UNROLL2 * T, u).start()

        return carry

    def phase2_tile(t, carry, never):
        r0 = pl.multiple_of(t * T, T)
        rb = pl.multiple_of(jnp.maximum(r0 - TH, 0), TH)
        side = _Side(never)
        st = {"route": carry}
        side.add(LN2B_PLAN, lambda k, a: finish_rows(hb_v, k, rb + k * LNC, t > 0, st, side.never, a))

        xn = xn_tile(r0)
        os_ = []
        for c in range(NC):
            pq = _dot(_unpack(wt_rows(0, c)), xn, NT)
            if c == 0:
                pq = side.gate(0, pq)
            q_features(pq, c)
            if c > 0:
                os_.append(attn_rows(c - 1, 0, T))
        o3a = attn_rows(NC - 1, 0, TH)
        ha = out_proj(side, 0, jnp.concatenate([o[0:TH, :] for o in os_[:2]], axis=1), 0, D // 2)
        o3b = attn_rows(NC - 1, TH, T)
        ha = ha + x_v[pl.ds(r0, TH), :].astype(F32)
        ha_v[...] = ha + out_proj(side, 8, jnp.concatenate([os_[2][0:TH, :], o3a], axis=1), D // 2, D)
        side.add(LN2A_PLAN, lambda k, a: finish_rows(ha_v, k, r0 + k * LNC, None, st, side.never, a))
        ob = jnp.concatenate([o[TH:T, :] for o in os_] + [o3b], axis=1)
        hb_v[...] = x_v[pl.ds(r0 + TH, TH), :].astype(F32) + out_proj(side, 16, ob, 0, D)
        return st["route"]

    route = lax.fori_loop(
        0, NT_ // UNROLL2, phase2,
        (jnp.full((8, 1), -jnp.inf, F32), jnp.zeros((8, 1), jnp.int32)))
    wg_copy.wait()
    wu_copy.wait()
    wd_copy.wait()
    st = {"route": route}
    for k in range(TH // LNC):
        finish_rows(hb_v, k, S - TH + k * LNC, None, st)
    best, besti = st["route"]
    o_copy(S - TH, TH, NT_).start()

    rmax = jnp.max(best, axis=0, keepdims=True)
    idx = jnp.min(jnp.where(best == rmax, besti, S), axis=0, keepdims=True)
    idx_s = jnp.clip(idx[0, 0], 0, S - 1)
    blk = pl.multiple_of((idx_s >> 4) << 4, 16)
    xs = _unpack(hn_v[pl.ds(pl.multiple_of(blk >> 1, 8), 8), :])
    g = _dot(xs, wg_v[...], NN)
    u = _dot(xs, wu_v[...], NN)
    a = (g * jax.nn.sigmoid(g) * u).astype(BF16)
    y = _dot(a, wd_v[:, 0:D], NN) * jax.nn.sigmoid(rmax)
    sel = lax.broadcasted_iota(jnp.int32, (16, 1), 0) == (idx_s - blk)
    patch_v[...] = (o_v[pl.ds(blk, 16), :].astype(F32) + jnp.where(sel, y, 0.0)).astype(BF16)
    o_copy(0, UNROLL2 * T - TH, 0).wait()
    for u in range(1, NT_ // UNROLL2):
        o_copy(u * UNROLL2 * T - TH, UNROLL2 * T, u).wait()
    o_copy(S - TH, TH, NT_).wait()
    pc = pltpu.make_async_copy(patch_v, out_hbm.at[pl.ds(blk, 16), :], sem.at[SM + 3])
    pc.start()
    pc.wait()


@jax.jit
def pallas_sequential_preLN__linear_kernel_hedgehog__moe_arch_mod__prompt_kernel(
    A_x: jax.Array,
    A_wqkv: jax.Array,
    A_w_phi: jax.Array,
    A_wo: jax.Array,
    B_x: jax.Array,
    B_w_r: jax.Array,
    B_w_gate: jax.Array,
    B_w_up: jax.Array,
    B_w_down: jax.Array,
):
    del B_x
    hbm = pl.BlockSpec(memory_space=pl.ANY)
    out = pl.pallas_call(
        _kernel,
        out_shape=jax.ShapeDtypeStruct((S, D), BF16),
        in_specs=[hbm] * 8,
        out_specs=hbm,
        scratch_shapes=[
            pltpu.VMEM((S, D), BF16),
            pltpu.VMEM((S // 2, D), U32),
            pltpu.VMEM((3 * NC, D, RC), BF16),
            pltpu.VMEM((3 * D // 2, D), U32),
            pltpu.VMEM((H, DH, DH), BF16),
            pltpu.VMEM((D, D), BF16),
            pltpu.VMEM((D // 2, D), U32),
            pltpu.VMEM((D,), BF16),
            pltpu.VMEM((8, D), F32),
            pltpu.VMEM((NPAIR, 64, 128), F32),
            pltpu.VMEM((NPAIR * 32, 128), U32),
            pltpu.VMEM((NPAIR, 128, 128), F32),
            pltpu.VMEM((NPAIR * 64, T), U32),
            pltpu.VMEM((TH, D), F32),
            pltpu.VMEM((TH, D), F32),
            pltpu.VMEM((S // 2, D), U32),
            pltpu.VMEM((S, D), BF16),
            pltpu.VMEM((D, FF), BF16),
            pltpu.VMEM((D, FF), BF16),
            pltpu.VMEM((FF, D + WD_PAD), BF16),
            pltpu.VMEM((16, D), BF16),
            pltpu.SemaphoreType.DMA((2 * NT_ + 3 * NC + 8,)),
        ],
        compiler_params=pltpu.CompilerParams(vmem_limit_bytes=100 * 1024 * 1024),
        name="hedgehog_mod",
    )(
        A_x.reshape(S, D),
        A_wqkv,
        A_w_phi,
        A_wo,
        B_w_r,
        B_w_gate,
        B_w_up,
        B_w_down,
    )
    return out.reshape(1, S, D)
```

```python
import jax
import jax.numpy as jnp
from jax import lax
import jax.experimental.pallas as pl
import jax.experimental.pallas.tpu as pltpu

F32 = jnp.float32
BF16 = jnp.bfloat16
U32 = jnp.uint32

S = 2048
D = 1024
H = 32
DH = 32
FF = 3584
NPAIR = H // 2
LOG2E = 1.4426950408889634
LN_EPS = 1e-5

T = 256
TH = T // 2
NT_ = S // T
RC = 256
NC = D // RC
PPC = RC // 64
LNC = 16
WD_PAD = 128

LN1_PLAN = tuple((k * 12 // 16, k * 12 // 16 + 3) for k in range(16))
LN2B_PLAN = ((None, 0), (None, 0), (None, 0), (1, 6), (3, 8), (5, 10), (7, 12), (9, 14))
LN2A_PLAN = ((None, 18), (None, 18), (16, 19), (17, 20), (18, 21), (19, 22), (20, 23), (21, None))
UNROLL2 = 2
G3_AT = 4

NN = (((1,), (0,)), ((), ()))
NT = (((1,), (1,)), ((), ()))


def _dot(a, b, dims):
    return lax.dot_general(a, b, dims, preferred_element_type=F32)


def _recip(x):
    return pl.reciprocal(x, approx=False, full_range=False)


def _pack(x):
    return pltpu.bitcast(x, U32)


def _unpack(x):
    return pltpu.bitcast(x, BF16)


def _pair_allreduce(a, op):
    a = op(a, pltpu.roll(a, 2, 0))
    return op(a, pltpu.roll(a, 4, 0))


def _tree(op, xs):
    xs = list(xs)
    while len(xs) > 1:
        nxt = [op(xs[i], xs[i + 1]) for i in range(0, len(xs) - 1, 2)]
        if len(xs) % 2:
            nxt.append(xs[-1])
        xs = nxt
    return xs[0]


def _dual_exp(p):
    sl = [p[8 * i:8 * i + 8, :] for i in range(8)]
    mx = _pair_allreduce(_tree(jnp.maximum, sl), jnp.maximum)
    mn = _pair_allreduce(_tree(jnp.minimum, sl), jnp.minimum)
    ep = [jnp.exp2(s - mx) for s in sl]
    en = [jnp.exp2(mn - s) for s in sl]
    sp = _pair_allreduce(_tree(jnp.add, ep), jnp.add)
    sn = _pair_allreduce(_tree(jnp.add, en), jnp.add)
    return ep, en, sp, sn


def _after(x, never, anchor):
    if anchor is None:
        return x
    d = jnp.concatenate([anchor] * (x.shape[0] // 8), axis=0)
    return jnp.concatenate([jnp.where(never, d, x[:, :128]), x[:, 128:]], axis=1)


def _gate(x, never, deps):
    for i, dep in enumerate(deps):
        d = jnp.broadcast_to(dep, (8, 128))
        if x.dtype != F32:
            d = pltpu.bitcast(d, x.dtype)
        blk = jnp.where(never, d, x[8 * i:8 * i + 8, :128])
        if x.shape[1] > 128:
            blk = jnp.concatenate([blk, x[8 * i:8 * i + 8, 128:]], axis=1)
        parts = ([x[:8 * i, :]] if i else []) + [blk, x[8 * i + 8:, :]]
        x = jnp.concatenate(parts, axis=0)
    return x


def _lane_fold(a):
    return _tree(jnp.add, [a[:, 128 * i:128 * i + 128] for i in range(a.shape[1] // 128)])


def _row_sum(a):
    return jnp.sum(_lane_fold(a), axis=-1, keepdims=True)


def _lane_tile(a, n):
    return a if n == 1 else jnp.concatenate([a] * n, axis=1)


class _Side:
    def __init__(self, never):
        self.never = never
        self.jobs = []
        self.deps = {}

    def add(self, plan, fn):
        for k, (rel, due) in enumerate(plan):
            if rel is None:
                self._run(due, fn, k, None)
            else:
                self.jobs.append((rel, due, fn, k))

    def _run(self, due, fn, k, anchor):
        dep = fn(k, anchor)
        if due is not None:
            self.deps.setdefault(due, []).append(dep)

    def gate(self, step, x):
        return _gate(x, self.never, self.deps.pop(step, []))

    def done(self, step, res):
        anchor = res[res.shape[0] - 8:, res.shape[1] - 128:]
        for job in [j for j in self.jobs if j[0] == step]:
            self.jobs.remove(job)
            self._run(job[1], job[2], job[3], anchor)


def _kernel(x_hbm, wqkv_hbm, wphi_hbm, wo_hbm, wr_hbm, wg_hbm, wu_hbm, wd_hbm, out_hbm,
            x_v, xn_v, wraw_v, wt_v, wphi_v, woraw_v, wo_v, wrraw_v, wr_v, kvacc_v, kvbf_v, z_v, phi_v,
            ha_v, hb_v, hn_v, o_v, wg_v, wu_v, wd_v, patch_v,
            sem):
    SX, SW, SO, SM = 0, NT_, NT_ + 3 * NC, 2 * NT_ + 3 * NC + 1

    def x_copy(i):
        return pltpu.make_async_copy(x_hbm.at[pl.ds(i * T, T), :], x_v.at[pl.ds(i * T, T), :], sem.at[SX + i])

    def w_copy(j, c):
        return pltpu.make_async_copy(wqkv_hbm.at[:, pl.ds(j * D + c * RC, RC)], wraw_v.at[j * NC + c],
                                     sem.at[SW + j * NC + c])

    wphi_copy = pltpu.make_async_copy(wphi_hbm, wphi_v, sem.at[SM + 4])
    wr_copy = pltpu.make_async_copy(wr_hbm, wrraw_v, sem.at[SM + 5])
    wo_copy = pltpu.make_async_copy(wo_hbm, woraw_v, sem.at[SM + 6])
    wg_copy = pltpu.make_async_copy(wg_hbm, wg_v, sem.at[SM + 0])
    wu_copy = pltpu.make_async_copy(wu_hbm, wu_v, sem.at[SM + 1])
    wd_copy = pltpu.make_async_copy(wd_hbm, wd_v.at[:, pl.ds(0, D)], sem.at[SM + 2])

    wphi_copy.start()
    x_copy(0).start()
    for c in range(NC):
        w_copy(1, c).start()
    for c in range(NC):
        w_copy(2, c).start()
    x_copy(1).start()

    def half(r):
        return r // 2 if isinstance(r, int) else pl.multiple_of(r // 2, LNC // 2)

    def ln_rows(r0, n, never=None, anchor=None):
        x = _after(x_v[pl.ds(r0, n), :].astype(F32), never, anchor)
        xc = x - _row_sum(x) * (1.0 / D)
        rstd = lax.rsqrt(_row_sum(xc * xc) * (1.0 / D) + LN_EPS)
        xn_v[pl.ds(half(r0), n // 2), :] = _pack((xc * rstd).astype(BF16))
        return _tree(jnp.add, [rstd[8 * i:8 * i + 8, :] for i in range(min(n, LNC) // 8)])

    def xn_tile(r0):
        return _unpack(xn_v[pl.ds(half(r0), T // 2), :])

    wphi_copy.wait()
    x_copy(0).wait()
    for i in range(2, NT_):
        x_copy(i).start()

    row = lax.broadcasted_iota(jnp.int32, (128, DH), 0)
    col = lax.broadcasted_iota(jnp.int32, (128, DH), 1)
    expand = jnp.where(((row & 63) >> 1) == col, 1.0, 0.0).astype(BF16)
    a_all = _dot(expand, wphi_v[...].reshape(H * DH, DH), NT)
    row = lax.broadcasted_iota(jnp.int32, (128, 128), 0)
    col = lax.broadcasted_iota(jnp.int32, (128, 128), 1)
    a_keep = (2 * (row >> 6) + (row & 1)) == (col >> 5)
    a_mats = [jnp.where(a_keep, a_all[:, g * 128:(g + 1) * 128], 0.0).astype(BF16) for g in range(8)]
    ln_rows(0, T)
    hb_v[...] = jnp.zeros((TH, D), F32)

    def fold(j, c):
        for s in range(RC // 128):
            g = c * (RC // 128) + s
            w = wraw_v[j * NC + c, :, s * 128:(s + 1) * 128]
            if j == 2:
                wt = w.T
            else:
                wt = (_dot(a_mats[g], w, NT) * LOG2E).astype(BF16)
            r0 = (j * D + g * 128) // 2
            wt_v[r0:r0 + 64, :] = _pack(wt)

    def wt_rows(j, c):
        r0 = (j * D + c * RC) // 2
        return wt_v[r0:r0 + RC // 2, :]

    def k_features(pk, c, first):
        for j in range(PPC):
            pr = c * PPC + j
            ep, en, sp, sn = _dual_exp(pk[64 * j:64 * j + 64, :])
            inv = _recip(sp * sn)
            rp = sn * inv
            rn = sp * inv
            phi = jnp.concatenate([e * rp for e in ep] + [e * rn for e in en], axis=0)
            zs = _lane_fold(phi)
            z_v[pr] = zs if first else z_v[pr] + zs
            phi_v[64 * pr:64 * pr + 64, :] = _pack(phi.astype(BF16))

    def kv_update(vt, c, first):
        for j in range(PPC):
            pr = c * PPC + j
            upd = _dot(vt[64 * j:64 * j + 64, :].astype(BF16), _unpack(phi_v[64 * pr:64 * pr + 64, :]), NT)
            kvacc_v[pr] = upd if first else kvacc_v[pr] + upd

    def proj0(j, c):
        return _dot(_unpack(wt_rows(j, c)), xn_tile(0), NT)

    w_copy(1, 0).wait()
    for c in range(NC):
        w_copy(0, c).start()
    fold(1, 0)
    pk0 = proj0(1, 0)
    w_copy(1, 1).wait()
    wo_copy.start()
    wr_copy.start()
    fold(1, 1)
    pk1 = proj0(1, 1)
    k_features(pk0, 0, True)
    w_copy(1, 2).wait()
    w_copy(1, 3).wait()
    wg_copy.start()
    wu_copy.start()
    wd_copy.start()
    fold(1, 2)
    fold(1, 3)
    pk2 = proj0(1, 2)
    k_features(pk1, 1, True)
    w_copy(2, 0).wait()
    w_copy(2, 1).wait()
    pk3 = proj0(1, 3)
    fold(2, 0)
    fold(2, 1)
    k_features(pk2, 2, True)
    vt0 = proj0(2, 0)
    k_features(pk3, 3, True)
    w_copy(2, 2).wait()
    w_copy(2, 3).wait()
    vt1 = proj0(2, 1)
    fold(2, 2)
    fold(2, 3)
    kv_update(vt0, 0, True)
    vt2 = proj0(2, 2)
    x_copy(1).wait()
    vt3 = proj0(2, 3)
    kv_update(vt1, 1, True)
    kv_update(vt2, 2, True)
    kv_update(vt3, 3, True)
    ln_rows(T, T)

    def phase1(t, carry):
        r0 = pl.multiple_of(t * T, T)
        tn = jnp.minimum(t + 1, NT_ - 1)
        rn = pl.multiple_of(tn * T, T)
        side = _Side(t < 0)

        @pl.when(t + 1 < NT_)
        def _():
            x_copy(tn).wait()

        xn = xn_tile(r0)
        for c in range(NC):
            pk = _dot(_unpack(wt_rows(1, c)), xn, NT)
            k_features(pk, c, False)
        side.add(LN1_PLAN, lambda k, a: ln_rows(rn + k * LNC, LNC, side.never, a))
        side.done(0, pk)
        vts = []
        for c in range(NC):
            w = wt_rows(2, c)
            quarters = []
            for n in range(2):
                for m in range(2):
                    step = 4 * c + 2 * n + m + 1
                    wq = side.gate(step, w[m * (RC // 4):(m + 1) * (RC // 4), :])
                    res = _dot(_unpack(wq), xn[n * TH:(n + 1) * TH, :], NT)
                    side.done(step, res)
                    quarters.append(res)
            vts.append(jnp.concatenate(
                [jnp.concatenate([quarters[0], quarters[2]], axis=1),
                 jnp.concatenate([quarters[1], quarters[3]], axis=1)], axis=0))
            if c > 0:
                kv_update(vts[c - 1], c - 1, False)
        kv_update(vts[NC - 1], NC - 1, False)
        return carry

    lax.fori_loop(1, NT_, phase1, 0)

    for c in range(NC):
        w_copy(0, c).wait()
    wo_copy.wait()
    wr_copy.wait()
    row = lax.broadcasted_iota(jnp.int32, (64, 128), 0)
    col = lax.broadcasted_iota(jnp.int32, (64, 128), 1)
    keep = (row >> 5) == (col & 1)
    for pr in range(NPAIR):
        kvbf_v[32 * pr:32 * pr + 32, :] = _pack(jnp.where(keep, kvacc_v[pr], 0.0).astype(BF16))
        z_v[pr] = jnp.broadcast_to(jnp.sum(z_v[pr], axis=-1, keepdims=True), (128, 128))
    for c in range(NC):
        fold(0, c)
    wo_v[...] = _pack(woraw_v[...])
    wr_v[...] = jnp.broadcast_to(wrraw_v[...].reshape(1, D).astype(F32), (8, D))

    def o_copy(r0, n, i):
        return pltpu.make_async_copy(o_v.at[pl.ds(r0, n), :], out_hbm.at[pl.ds(r0, n), :], sem.at[SO + i])

    def finish_rows(h_ref, k, r0, valid, st, never=None, anchor=None):
        best, besti = st["route"]
        wr = jnp.concatenate([wr_v[...]] * (LNC // 8), axis=0)
        sub = lax.broadcasted_iota(jnp.int32, (8, 1), 0)
        h = _after(h_ref[k * LNC:(k + 1) * LNC, :], never, anchor)
        m = _row_sum(h) * (1.0 / D)
        hc = h - m
        rstd = lax.rsqrt(_row_sum(hc * hc) * (1.0 / D) + LN_EPS)
        r = (_row_sum(hc * wr) * rstd).astype(BF16).astype(F32)
        hn = hc * rstd
        hn_v[pl.ds(half(r0), LNC // 2), :] = _pack(hn.astype(BF16))
        o_v[pl.ds(r0, LNC), :] = (hn + h).astype(BF16)
        if valid is not None:
            r = jnp.where(valid, r, -jnp.inf)
        for i in range(LNC // 8):
            ri = r[8 * i:8 * i + 8, :]
            better = ri > best
            best = jnp.where(better, ri, best)
            besti = jnp.where(better, sub + (r0 + 8 * i), besti)
        st["route"] = (best, besti)
        return best

    def q_features(pq, c):
        for j in range(PPC):
            pr = c * PPC + j
            ep, en, sp, sn = _dual_exp(pq[64 * j:64 * j + 64, :])
            zz = [_lane_tile(z_v[pr, 8 * i:8 * i + 8, :], pq.shape[1] // 128) for i in range(16)]
            ap = _pair_allreduce(_tree(jnp.add, [ep[i] * zz[i] for i in range(8)]), jnp.add)
            an = _pair_allreduce(_tree(jnp.add, [en[i] * zz[8 + i] for i in range(8)]), jnp.add)
            inv = _recip(ap * sn + (an + 1e-6 * sn) * sp)
            rp = sn * inv
            rn = sp * inv
            phi = jnp.concatenate([e * rp for e in ep] + [e * rn for e in en], axis=0)
            phi_v[64 * pr:64 * pr + 64, :] = _pack(phi.astype(BF16))

    def attn_rows(c, lo, hi):
        res = jnp.concatenate(
            [_dot(_unpack(kvbf_v[32 * pr:32 * pr + 32, :]), _unpack(phi_v[64 * pr:64 * pr + 64, lo:hi]), NN)
             for pr in range(c * PPC, (c + 1) * PPC)], axis=0)
        return res.astype(BF16).T

    def out_proj(side, step0, o, k0, k1, n0=0, n1=D // 128):
        cols = []
        for n in range(n0, n1):
            w = side.gate(step0 + n, wo_v[k0 // 2:k1 // 2, n * 128:(n + 1) * 128])
            res = _dot(o, _unpack(w), NN)
            side.done(step0 + n, res)
            cols.append(res)
        return jnp.concatenate(cols, axis=1)

    def phase2(u, carry):
        for i in range(UNROLL2):
            carry = phase2_tile(u * UNROLL2 + i, carry, u < 0)

        r0 = pl.multiple_of(u * (UNROLL2 * T), T)

        @pl.when(u == 0)
        def _():
            o_copy(0, UNROLL2 * T - TH, 0).start()

        @pl.when(u > 0)
        def _():
            o_copy(pl.multiple_of(jnp.maximum(r0 - TH, 0), TH), UNROLL2 * T, u).start()

        return carry

    def phase2_tile(t, carry, never):
        r0 = pl.multiple_of(t * T, T)
        rb = pl.multiple_of(jnp.maximum(r0 - TH, 0), TH)
        side = _Side(never)
        st = {"route": carry}
        side.add(LN2B_PLAN, lambda k, a: finish_rows(hb_v, k, rb + k * LNC, t > 0, st, side.never, a))

        xn = xn_tile(r0)
        os_ = []
        for c in range(NC):
            pq = _dot(_unpack(wt_rows(0, c)), xn, NT)
            if c == 0:
                pq = side.gate(0, pq)
            q_features(pq, c)
            if c > 0:
                os_.append(attn_rows(c - 1, 0, T))
        oa = jnp.concatenate([o[0:TH, :] for o in os_[:2]], axis=1)
        ha0 = out_proj(side, 0, oa, 0, D // 2, 0, G3_AT)
        os_.append(attn_rows(NC - 1, 0, T))
        ha1 = out_proj(side, 0, oa, 0, D // 2, G3_AT, D // 128)
        ha = jnp.concatenate([ha0, ha1], axis=1) + x_v[pl.ds(r0, TH), :].astype(F32)
        ha_v[...] = ha + out_proj(side, 8, jnp.concatenate([o[0:TH, :] for o in os_[2:]], axis=1), D // 2, D)
        side.add(LN2A_PLAN, lambda k, a: finish_rows(ha_v, k, r0 + k * LNC, None, st, side.never, a))
        ob = jnp.concatenate([o[TH:T, :] for o in os_], axis=1)
        hb_v[...] = x_v[pl.ds(r0 + TH, TH), :].astype(F32) + out_proj(side, 16, ob, 0, D)
        return st["route"]

    route = lax.fori_loop(
        0, NT_ // UNROLL2, phase2,
        (jnp.full((8, 1), -jnp.inf, F32), jnp.zeros((8, 1), jnp.int32)))
    wg_copy.wait()
    wu_copy.wait()
    wd_copy.wait()
    st = {"route": route}
    for k in range(TH // LNC):
        finish_rows(hb_v, k, S - TH + k * LNC, None, st)
    best, besti = st["route"]
    o_copy(S - TH, TH, NT_).start()

    rmax = jnp.max(best, axis=0, keepdims=True)
    idx = jnp.min(jnp.where(best == rmax, besti, S), axis=0, keepdims=True)
    idx_s = jnp.clip(idx[0, 0], 0, S - 1)
    blk = pl.multiple_of((idx_s >> 4) << 4, 16)
    xs = _unpack(hn_v[pl.ds(pl.multiple_of(blk >> 1, 8), 8), :])
    g = _dot(xs, wg_v[...], NN)
    u = _dot(xs, wu_v[...], NN)
    a = (g * jax.nn.sigmoid(g) * u).astype(BF16)
    y = _dot(a, wd_v[:, 0:D], NN) * jax.nn.sigmoid(rmax)
    sel = lax.broadcasted_iota(jnp.int32, (16, 1), 0) == (idx_s - blk)
    patch_v[...] = (o_v[pl.ds(blk, 16), :].astype(F32) + jnp.where(sel, y, 0.0)).astype(BF16)
    o_copy(0, UNROLL2 * T - TH, 0).wait()
    for u in range(1, NT_ // UNROLL2):
        o_copy(u * UNROLL2 * T - TH, UNROLL2 * T, u).wait()
    o_copy(S - TH, TH, NT_).wait()
    pc = pltpu.make_async_copy(patch_v, out_hbm.at[pl.ds(blk, 16), :], sem.at[SM + 3])
    pc.start()
    pc.wait()


@jax.jit
def pallas_sequential_preLN__linear_kernel_hedgehog__moe_arch_mod__prompt_kernel(
    A_x: jax.Array,
    A_wqkv: jax.Array,
    A_w_phi: jax.Array,
    A_wo: jax.Array,
    B_x: jax.Array,
    B_w_r: jax.Array,
    B_w_gate: jax.Array,
    B_w_up: jax.Array,
    B_w_down: jax.Array,
):
    del B_x
    hbm = pl.BlockSpec(memory_space=pl.ANY)
    out = pl.pallas_call(
        _kernel,
        out_shape=jax.ShapeDtypeStruct((S, D), BF16),
        in_specs=[hbm] * 8,
        out_specs=hbm,
        scratch_shapes=[
            pltpu.VMEM((S, D), BF16),
            pltpu.VMEM((S // 2, D), U32),
            pltpu.VMEM((3 * NC, D, RC), BF16),
            pltpu.VMEM((3 * D // 2, D), U32),
            pltpu.VMEM((H, DH, DH), BF16),
            pltpu.VMEM((D, D), BF16),
            pltpu.VMEM((D // 2, D), U32),
            pltpu.VMEM((D,), BF16),
            pltpu.VMEM((8, D), F32),
            pltpu.VMEM((NPAIR, 64, 128), F32),
            pltpu.VMEM((NPAIR * 32, 128), U32),
            pltpu.VMEM((NPAIR, 128, 128), F32),
            pltpu.VMEM((NPAIR * 64, T), U32),
            pltpu.VMEM((TH, D), F32),
            pltpu.VMEM((TH, D), F32),
            pltpu.VMEM((S // 2, D), U32),
            pltpu.VMEM((S, D), BF16),
            pltpu.VMEM((D, FF), BF16),
            pltpu.VMEM((D, FF), BF16),
            pltpu.VMEM((FF, D + WD_PAD), BF16),
            pltpu.VMEM((16, D), BF16),
            pltpu.SemaphoreType.DMA((2 * NT_ + 3 * NC + 8,)),
        ],
        compiler_params=pltpu.CompilerParams(vmem_limit_bytes=100 * 1024 * 1024,
                                             disable_semaphore_checks=True, disable_bounds_checks=True),
        name="hedgehog_mod",
    )(
        A_x.reshape(S, D),
        A_wqkv,
        A_w_phi,
        A_wo,
        B_w_r,
        B_w_gate,
        B_w_up,
        B_w_down,
    )
    return out.reshape(1, S, D)
```

```python
import jax
import jax.numpy as jnp
from jax import lax
import jax.experimental.pallas as pl
import jax.experimental.pallas.tpu as pltpu

F32 = jnp.float32
BF16 = jnp.bfloat16
U32 = jnp.uint32

S = 2048
D = 1024
H = 32
DH = 32
FF = 3584
NPAIR = H // 2
LOG2E = 1.4426950408889634
LN_EPS = 1e-5

T = 256
TH = T // 2
NT_ = S // T
RC = 256
NC = D // RC
PPC = RC // 64
LNC = 16
WD_PAD = 128

LN1_PLAN = tuple((k * 12 // 16, k * 12 // 16 + 3) for k in range(16))
LN2B_PLAN = ((None, 0), (None, 0), (None, 0), (1, 6), (3, 8), (5, 10), (7, 12), (9, 14))
LN2A_PLAN = ((None, 18), (None, 18), (16, 19), (17, 20), (18, 21), (19, 22), (20, 23), (21, None))
PRO_LN1_PLAN = tuple((k * 5 // 16 - 1 if k * 5 // 16 else None, None) for k in range(16))
WO_ROWS = 352
WO_PLAN = tuple((k + 1, None) for k in range(11))
Z_PLAN = tuple((1 + k * 12 // 16, 1 + k * 12 // 16 + 3) for k in range(16))
UNROLL2 = 2
G3_AT = 4

NN = (((1,), (0,)), ((), ()))
NT = (((1,), (1,)), ((), ()))


def _dot(a, b, dims):
    return lax.dot_general(a, b, dims, preferred_element_type=F32)


def _recip(x):
    return pl.reciprocal(x, approx=False, full_range=False)


def _pack(x):
    return pltpu.bitcast(x, U32)


def _unpack(x):
    return pltpu.bitcast(x, BF16)


def _pair_allreduce(a, op):
    a = op(a, pltpu.roll(a, 2, 0))
    return op(a, pltpu.roll(a, 4, 0))


def _tree(op, xs):
    xs = list(xs)
    while len(xs) > 1:
        nxt = [op(xs[i], xs[i + 1]) for i in range(0, len(xs) - 1, 2)]
        if len(xs) % 2:
            nxt.append(xs[-1])
        xs = nxt
    return xs[0]


def _dual_exp(p):
    sl = [p[8 * i:8 * i + 8, :] for i in range(8)]
    mx = _pair_allreduce(_tree(jnp.maximum, sl), jnp.maximum)
    mn = _pair_allreduce(_tree(jnp.minimum, sl), jnp.minimum)
    ep = [jnp.exp2(s - mx) for s in sl]
    en = [jnp.exp2(mn - s) for s in sl]
    sp = _pair_allreduce(_tree(jnp.add, ep), jnp.add)
    sn = _pair_allreduce(_tree(jnp.add, en), jnp.add)
    return ep, en, sp, sn


def _after(x, never, anchor):
    if anchor is None:
        return x
    d = jnp.concatenate([anchor] * (x.shape[0] // 8), axis=0)
    if x.shape[1] == 128:
        return jnp.where(never, d, x)
    return jnp.concatenate([jnp.where(never, d, x[:, :128]), x[:, 128:]], axis=1)


def _gate(x, never, deps):
    for i, dep in enumerate(deps):
        d = jnp.broadcast_to(dep, (8, 128))
        if x.dtype != F32:
            d = pltpu.bitcast(d, x.dtype)
        blk = jnp.where(never, d, x[8 * i:8 * i + 8, :128])
        if x.shape[1] > 128:
            blk = jnp.concatenate([blk, x[8 * i:8 * i + 8, 128:]], axis=1)
        parts = ([x[:8 * i, :]] if i else []) + [blk, x[8 * i + 8:, :]]
        x = jnp.concatenate(parts, axis=0)
    return x


def _lane_fold(a):
    return _tree(jnp.add, [a[:, 128 * i:128 * i + 128] for i in range(a.shape[1] // 128)])


def _row_sum(a):
    return jnp.sum(_lane_fold(a), axis=-1, keepdims=True)


def _lane_tile(a, n):
    return a if n == 1 else jnp.concatenate([a] * n, axis=1)


class _Side:
    def __init__(self, never):
        self.never = never
        self.jobs = []
        self.deps = {}

    def add(self, plan, fn):
        for k, (rel, due) in enumerate(plan):
            if rel is None:
                self._run(due, fn, k, None)
            else:
                self.jobs.append((rel, due, fn, k))

    def _run(self, due, fn, k, anchor):
        dep = fn(k, anchor)
        if due is not None:
            self.deps.setdefault(due, []).append(dep)

    def gate(self, step, x):
        return _gate(x, self.never, self.deps.pop(step, []))

    def done(self, step, res):
        anchor = res[res.shape[0] - 8:, res.shape[1] - 128:]
        for job in [j for j in self.jobs if j[0] == step]:
            self.jobs.remove(job)
            self._run(job[1], job[2], job[3], anchor)


def _kernel(x_hbm, wqkv_hbm, wphi_hbm, wo_hbm, wr_hbm, wg_hbm, wu_hbm, wd_hbm, out_hbm,
            x_v, xn_v, wraw_v, wt_v, wphi_v, a_v, woraw_v, wo_v, wrraw_v, wr_v, kvacc_v, kvbf_v,
            z_v, zb_v, phi_v, ha_v, hb_v, hn_v, o_v, wg_v, wu_v, wd_v, patch_v,
            sem):
    SX, SW, SO, SM = 0, 5, 5 + 3 * NC, 5 + 3 * NC + NT_ + 1

    def x_copy(i):
        t0, t1 = ((0, 1), (1, 2), (2, 3), (3, 5), (5, NT_))[i]
        rows = pl.ds(t0 * T, (t1 - t0) * T)
        return pltpu.make_async_copy(x_hbm.at[rows, :], x_v.at[rows, :], sem.at[SX + i])

    def w_copy(j, c):
        return pltpu.make_async_copy(wqkv_hbm.at[:, pl.ds(j * D + c * RC, RC)], wraw_v.at[j * NC + c],
                                     sem.at[SW + j * NC + c])

    wphi_copy = pltpu.make_async_copy(wphi_hbm, wphi_v, sem.at[SM + 4])
    wr_copy = pltpu.make_async_copy(wr_hbm, wrraw_v, sem.at[SM + 5])
    wo_copy = pltpu.make_async_copy(wo_hbm, woraw_v, sem.at[SM + 6])
    wg_copy = pltpu.make_async_copy(wg_hbm, wg_v, sem.at[SM + 0])
    wu_copy = pltpu.make_async_copy(wu_hbm, wu_v, sem.at[SM + 1])
    wd_copy = pltpu.make_async_copy(wd_hbm, wd_v.at[:, pl.ds(0, D)], sem.at[SM + 2])

    wphi_copy.start()
    x_copy(0).start()
    w_copy(1, 0).start()
    w_copy(1, 1).start()
    x_copy(1).start()
    w_copy(1, 2).start()

    def half(r):
        return r // 2 if isinstance(r, int) else pl.multiple_of(r // 2, LNC // 2)

    def ln_rows(r0, n, never=None, anchor=None):
        x = _after(x_v[pl.ds(r0, n), :].astype(F32), never, anchor)
        xc = x - _row_sum(x) * (1.0 / D)
        rstd = lax.rsqrt(_row_sum(xc * xc) * (1.0 / D) + LN_EPS)
        xn_v[pl.ds(half(r0), n // 2), :] = _pack((xc * rstd).astype(BF16))
        return _tree(jnp.add, [rstd[8 * i:8 * i + 8, :] for i in range(min(n, LNC) // 8)])

    def xn_tile(r0):
        return _unpack(xn_v[pl.ds(half(r0), T // 2), :])

    wphi_copy.wait()
    x_copy(0).wait()
    w_copy(1, 3).start()
    for c in range(NC):
        w_copy(2, c).start()
    x_copy(2).start()

    row = lax.broadcasted_iota(jnp.int32, (128, DH), 0)
    col = lax.broadcasted_iota(jnp.int32, (128, DH), 1)
    expand = jnp.where(((row & 63) >> 1) == col, 1.0, 0.0).astype(BF16)
    a_all = _dot(expand, wphi_v[...].reshape(H * DH, DH), NT)
    row = lax.broadcasted_iota(jnp.int32, (128, 128), 0)
    col = lax.broadcasted_iota(jnp.int32, (128, 128), 1)
    a_keep = (2 * (row >> 6) + (row & 1)) == (col >> 5)
    for g in range(8):
        a_v[64 * g:64 * g + 64, :] = _pack(jnp.where(a_keep, a_all[:, g * 128:(g + 1) * 128], 0.0).astype(BF16))
    never0 = ln_rows(0, T)[0, 0] < 0.0
    hb_v[...] = jnp.zeros((TH, D), F32)

    def fold(j, c, side=None, step0=None):
        for s in range(RC // 128):
            g = c * (RC // 128) + s
            w = wraw_v[j * NC + c, :, s * 128:(s + 1) * 128]
            g0 = 64 * g if isinstance(g, int) else pl.multiple_of(64 * g, 64)
            if j == 2:
                wt = w.T
            else:
                res = _dot(_unpack(a_v[pl.ds(g0, 64), :]), w, NT)
                if side is not None:
                    side.done(step0 + s, res)
                wt = (res * LOG2E).astype(BF16)
            wt_v[j][pl.ds(g0, 64), :] = _pack(wt)

    def wt_rows(j, c):
        return wt_v[j][c * RC // 2:(c + 1) * RC // 2, :]

    def k_features(pk, slot, c, first, ties=None):
        for j in range(PPC):
            pr = c * PPC + j
            p = pk[64 * j:64 * j + 64, :]
            if ties is not None:
                p = jnp.concatenate([jnp.where(ties[0], _lane_tile(ties[1][j], T // 128), p[0:8, :]), p[8:, :]], axis=0)
            ep, en, sp, sn = _dual_exp(p)
            inv = _recip(sp * sn)
            rp = sn * inv
            rn = sp * inv
            phi = jnp.concatenate([e * rp for e in ep] + [e * rn for e in en], axis=0)
            zs = _lane_fold(phi)
            z_v[pr] = zs if first else z_v[pr] + zs
            phi_v[slot][64 * pr:64 * pr + 64, :] = _pack(phi.astype(BF16))

    row = lax.broadcasted_iota(jnp.int32, (64, 128), 0)
    col = lax.broadcasted_iota(jnp.int32, (64, 128), 1)
    kv_keep = (row >> 5) == (col & 1)

    def kv_update(vt, slot, c, first, publish=False):
        for j in range(PPC):
            pr = c * PPC + j
            upd = _dot(vt[64 * j:64 * j + 64, :].astype(BF16), _unpack(phi_v[slot][64 * pr:64 * pr + 64, :]), NT)
            acc = upd if first else kvacc_v[pr] + upd
            kvacc_v[pr] = acc
            if publish:
                kvbf_v[32 * pr:32 * pr + 32, :] = _pack(jnp.where(kv_keep, acc, 0.0).astype(BF16))

    def proj(j, c, r0):
        return _dot(_unpack(wt_rows(j, c)), xn_tile(r0), NT)

    def proj_steps(side, step0, j, c, xn):
        w = wt_rows(j, c)
        quarters = []
        for n in range(2):
            for m in range(2):
                step = step0 + 2 * n + m
                wq = side.gate(step, w[m * (RC // 4):(m + 1) * (RC // 4), :])
                res = _dot(_unpack(wq), xn[n * TH:(n + 1) * TH, :], NT)
                side.done(step, res)
                quarters.append(res)
        return jnp.concatenate(
            [jnp.concatenate([quarters[0], quarters[2]], axis=1),
             jnp.concatenate([quarters[1], quarters[3]], axis=1)], axis=0)

    def spots(res, n):
        m, w = res.shape
        allp = [res[r:r + 8, c:c + 128] for c in range(0, w, 128) for r in range(56, m, 64)]
        return [allp[(i * len(allp)) // n] for i in range(n)]

    w_copy(1, 0).wait()
    for c in range(NC):
        w_copy(0, c).start()
    x_copy(3).start()
    fold(1, 0)
    pk00 = proj(1, 0, 0)

    w_copy(1, 1).wait()
    wo_copy.start()
    wr_copy.start()
    x_copy(4).start()
    fold(1, 1)
    pk01 = proj(1, 1, 0)
    k_features(pk00, 0, 0, True)

    x_copy(1).wait()
    w_copy(1, 2).wait()
    wg_copy.start()
    wu_copy.start()
    wd_copy.start()
    side = _Side(never0)
    side.add(PRO_LN1_PLAN, lambda k, a: ln_rows(T + k * LNC, LNC, never0, a))
    fold(1, 2, side, 0)
    pk02 = proj_steps(side, 2, 1, 2, xn_tile(0))
    pk10 = proj(1, 0, T)
    k_features(pk01, 0, 1, True, (never0, spots(pk10, PPC)))
    pk11 = proj(1, 1, T)
    k_features(pk02, 0, 2, True, (never0, spots(pk10, 2 * PPC)[PPC:]))
    k_features(pk10, 1, 0, False)
    pk12 = proj(1, 2, T)
    k_features(pk11, 1, 1, False)

    w_copy(1, 3).wait()
    for c in range(3):
        w_copy(2, c).wait()
    fold(1, 3)
    pk03 = proj(1, 3, 0)
    k_features(pk12, 1, 2, False)
    pk13 = proj(1, 3, T)
    k_features(pk03, 0, 3, True)
    for c in range(3):
        fold(2, c)
    vt00 = proj(2, 0, 0)
    k_features(pk13, 1, 3, False)
    vt10 = proj(2, 0, T)
    kv_update(vt00, 0, 0, True)
    vt01 = proj(2, 1, 0)
    kv_update(vt10, 1, 0, False)
    vt11 = proj(2, 1, T)
    kv_update(vt01, 0, 1, True)

    w_copy(2, 3).wait()
    x_copy(2).wait()
    w_copy(0, 0).wait()
    side = _Side(never0)
    side.add(LN1_PLAN, lambda k, a: ln_rows(2 * T + k * LNC, LNC, never0, a))
    fold(0, 0, side, -1)
    fold(2, 3)
    kv_update(vt11, 1, 1, False)
    vt02 = proj_steps(side, 1, 2, 2, xn_tile(0))
    vt12 = proj_steps(side, 5, 2, 2, xn_tile(T))
    kv_update(vt02, 0, 2, True)
    vt03 = proj_steps(side, 9, 2, 3, xn_tile(0))
    kv_update(vt12, 1, 2, False)
    vt13 = proj_steps(side, 13, 2, 3, xn_tile(T))
    kv_update(vt03, 0, 3, True)
    kv_update(vt13, 1, 3, False)

    def phase1(u, carry):
        never = u < 0

        @pl.when(u == 0)
        def _():
            for c in range(1, NC):
                w_copy(0, c).wait()
            x_copy(3).wait()
            wo_copy.wait()
            wr_copy.wait()

        @pl.when(u == 1)
        def _():
            x_copy(4).wait()

        pending = None
        for i in range(2):
            t = 2 * u + 2 + i
            r0 = pl.multiple_of(t * T, T)
            rn = pl.multiple_of(jnp.minimum(t + 1, NT_ - 1) * T, T)
            side = _Side(never)
            xn = xn_tile(r0)
            for c in range(NC):
                pk = _dot(_unpack(wt_rows(1, c)), xn, NT)
                if c == 0 and pending is not None:
                    kv_update(*pending)
                k_features(pk, i, c, False)
            side.add(LN1_PLAN, lambda k, a: ln_rows(rn + k * LNC, LNC, never, a))
            if i == 0:
                def pack_wo(k, a):
                    rows = WO_ROWS // len(WO_PLAN)
                    w0 = pl.multiple_of(u * ((D - WO_ROWS) // 2) + k * rows, 16)
                    w = _pack(woraw_v[pl.ds(w0, rows), :])
                    d = jnp.concatenate([_lane_tile(pltpu.bitcast(a, U32), D // 128)] * (rows // 16), axis=0)
                    wo_v[pl.ds(pl.multiple_of(w0 // 2, 8), rows // 2), :] = jnp.where(never, d, w)
                side.add(WO_PLAN, pack_wo)
            else:
                def z_final(k, a):
                    z = _after(z_v[k], never, a)
                    zs = jnp.sum(z, axis=-1, keepdims=True)
                    zb_v[k] = jnp.broadcast_to(zs, (128, 128))
                    return zs[120:128, :]
                side.add(Z_PLAN, z_final)
            side.done(0, pk)
            vts = []
            for c in range(NC):
                vts.append(proj_steps(side, 4 * c + 1, 2, c, xn))
                if c > 0:
                    kv_update(vts[c - 1], i, c - 1, False, i == 1)
            pending = (vts[NC - 1], i, NC - 1, False, i == 1)
        fold(0, u + 1)
        kv_update(*pending)
        wr_v[...] = jnp.broadcast_to(wrraw_v[...].reshape(1, D).astype(F32), (8, D))
        return carry

    lax.fori_loop(0, (NT_ - 2) // 2, phase1, 0)

    def o_copy(r0, n, i):
        return pltpu.make_async_copy(o_v.at[pl.ds(r0, n), :], out_hbm.at[pl.ds(r0, n), :], sem.at[SO + i])

    def finish_rows(h_ref, k, r0, valid, st, never=None, anchor=None):
        best, besti = st["route"]
        wr = jnp.concatenate([wr_v[...]] * (LNC // 8), axis=0)
        sub = lax.broadcasted_iota(jnp.int32, (8, 1), 0)
        h = _after(h_ref[k * LNC:(k + 1) * LNC, :], never, anchor)
        m = _row_sum(h) * (1.0 / D)
        hc = h - m
        rstd = lax.rsqrt(_row_sum(hc * hc) * (1.0 / D) + LN_EPS)
        r = (_row_sum(hc * wr) * rstd).astype(BF16).astype(F32)
        hn = hc * rstd
        hn_v[pl.ds(half(r0), LNC // 2), :] = _pack(hn.astype(BF16))
        o_v[pl.ds(r0, LNC), :] = (hn + h).astype(BF16)
        if valid is not None:
            r = jnp.where(valid, r, -jnp.inf)
        for i in range(LNC // 8):
            ri = r[8 * i:8 * i + 8, :]
            better = ri > best
            best = jnp.where(better, ri, best)
            besti = jnp.where(better, sub + (r0 + 8 * i), besti)
        st["route"] = (best, besti)
        return best

    def q_features(pq, slot, c):
        for j in range(PPC):
            pr = c * PPC + j
            ep, en, sp, sn = _dual_exp(pq[64 * j:64 * j + 64, :])
            zz = [_lane_tile(zb_v[pr, 8 * i:8 * i + 8, :], pq.shape[1] // 128) for i in range(16)]
            ap = _pair_allreduce(_tree(jnp.add, [ep[i] * zz[i] for i in range(8)]), jnp.add)
            an = _pair_allreduce(_tree(jnp.add, [en[i] * zz[8 + i] for i in range(8)]), jnp.add)
            inv = _recip(ap * sn + (an + 1e-6 * sn) * sp)
            rp = sn * inv
            rn = sp * inv
            phi = jnp.concatenate([e * rp for e in ep] + [e * rn for e in en], axis=0)
            phi_v[slot][64 * pr:64 * pr + 64, :] = _pack(phi.astype(BF16))

    def attn_rows(slot, c, lo, hi):
        res = jnp.concatenate(
            [_dot(_unpack(kvbf_v[32 * pr:32 * pr + 32, :]), _unpack(phi_v[slot][64 * pr:64 * pr + 64, lo:hi]), NN)
             for pr in range(c * PPC, (c + 1) * PPC)], axis=0)
        return res.astype(BF16).T

    def out_proj(side, step0, o, k0, k1, n0=0, n1=D // 128):
        cols = []
        for n in range(n0, n1):
            w = side.gate(step0 + n, wo_v[k0 // 2:k1 // 2, n * 128:(n + 1) * 128])
            res = _dot(o, _unpack(w), NN)
            side.done(step0 + n, res)
            cols.append(res)
        return jnp.concatenate(cols, axis=1)

    def phase2(u, carry):
        for i in range(UNROLL2):
            carry = phase2_tile(u * UNROLL2 + i, i % 2, carry, u < 0)

        r0 = pl.multiple_of(u * (UNROLL2 * T), T)

        @pl.when(u == 0)
        def _():
            o_copy(0, UNROLL2 * T - TH, 0).start()

        @pl.when(u > 0)
        def _():
            o_copy(pl.multiple_of(jnp.maximum(r0 - TH, 0), TH), UNROLL2 * T, u).start()

        return carry

    def phase2_tile(t, slot, carry, never):
        r0 = pl.multiple_of(t * T, T)
        rb = pl.multiple_of(jnp.maximum(r0 - TH, 0), TH)
        side = _Side(never)
        st = {"route": carry}
        side.add(LN2B_PLAN, lambda k, a: finish_rows(hb_v, k, rb + k * LNC, t > 0, st, side.never, a))

        xn = xn_tile(r0)
        os_ = []
        for c in range(NC):
            pq = _dot(_unpack(wt_rows(0, c)), xn, NT)
            if c == 0:
                pq = side.gate(0, pq)
            q_features(pq, slot, c)
            if c > 0:
                os_.append(attn_rows(slot, c - 1, 0, T))
        oa = jnp.concatenate([o[0:TH, :] for o in os_[:2]], axis=1)
        ha0 = out_proj(side, 0, oa, 0, D // 2, 0, G3_AT)
        os_.append(attn_rows(slot, NC - 1, 0, T))
        ha1 = out_proj(side, 0, oa, 0, D // 2, G3_AT, D // 128)
        ha = jnp.concatenate([ha0, ha1], axis=1) + x_v[pl.ds(r0, TH), :].astype(F32)
        ha_v[...] = ha + out_proj(side, 8, jnp.concatenate([o[0:TH, :] for o in os_[2:]], axis=1), D // 2, D)
        side.add(LN2A_PLAN, lambda k, a: finish_rows(ha_v, k, r0 + k * LNC, None, st, side.never, a))
        ob = jnp.concatenate([o[TH:T, :] for o in os_], axis=1)
        hb_v[...] = x_v[pl.ds(r0 + TH, TH), :].astype(F32) + out_proj(side, 16, ob, 0, D)
        return st["route"]

    route = lax.fori_loop(
        0, NT_ // UNROLL2, phase2,
        (jnp.full((8, 1), -jnp.inf, F32), jnp.zeros((8, 1), jnp.int32)))
    wg_copy.wait()
    wu_copy.wait()
    wd_copy.wait()
    st = {"route": route}
    for k in range(TH // LNC):
        finish_rows(hb_v, k, S - TH + k * LNC, None, st)
    best, besti = st["route"]
    o_copy(S - TH, TH, NT_).start()

    rmax = jnp.max(best, axis=0, keepdims=True)
    idx = jnp.min(jnp.where(best == rmax, besti, S), axis=0, keepdims=True)
    idx_s = jnp.clip(idx[0, 0], 0, S - 1)
    blk = pl.multiple_of((idx_s >> 4) << 4, 16)
    xs = _unpack(hn_v[pl.ds(pl.multiple_of(blk >> 1, 8), 8), :])
    g = _dot(xs, wg_v[...], NN)
    u = _dot(xs, wu_v[...], NN)
    a = (g * jax.nn.sigmoid(g) * u).astype(BF16)
    y = _dot(a, wd_v[:, 0:D], NN) * jax.nn.sigmoid(rmax)
    sel = lax.broadcasted_iota(jnp.int32, (16, 1), 0) == (idx_s - blk)
    patch_v[...] = (o_v[pl.ds(blk, 16), :].astype(F32) + jnp.where(sel, y, 0.0)).astype(BF16)
    o_copy(0, UNROLL2 * T - TH, 0).wait()
    for u in range(1, NT_ // UNROLL2):
        o_copy(u * UNROLL2 * T - TH, UNROLL2 * T, u).wait()
    o_copy(S - TH, TH, NT_).wait()
    pc = pltpu.make_async_copy(patch_v, out_hbm.at[pl.ds(blk, 16), :], sem.at[SM + 3])
    pc.start()
    pc.wait()


@jax.jit
def pallas_sequential_preLN__linear_kernel_hedgehog__moe_arch_mod__prompt_kernel(
    A_x: jax.Array,
    A_wqkv: jax.Array,
    A_w_phi: jax.Array,
    A_wo: jax.Array,
    B_x: jax.Array,
    B_w_r: jax.Array,
    B_w_gate: jax.Array,
    B_w_up: jax.Array,
    B_w_down: jax.Array,
):
    del B_x
    hbm = pl.BlockSpec(memory_space=pl.ANY)
    out = pl.pallas_call(
        _kernel,
        out_shape=jax.ShapeDtypeStruct((S, D), BF16),
        in_specs=[hbm] * 8,
        out_specs=hbm,
        scratch_shapes=[
            pltpu.VMEM((S, D), BF16),
            pltpu.VMEM((S // 2, D), U32),
            pltpu.VMEM((3 * NC, D, RC), BF16),
            [pltpu.VMEM((D // 2, D), U32)] * 3,
            pltpu.VMEM((H, DH, DH), BF16),
            pltpu.VMEM((8 * 64, 128), U32),
            pltpu.VMEM((D, D), BF16),
            pltpu.VMEM((D // 2, D), U32),
            pltpu.VMEM((D,), BF16),
            pltpu.VMEM((8, D), F32),
            pltpu.VMEM((NPAIR, 64, 128), F32),
            pltpu.VMEM((NPAIR * 32, 128), U32),
            pltpu.VMEM((NPAIR, 128, 128), F32),
            pltpu.VMEM((NPAIR, 128, 128), F32),
            [pltpu.VMEM((NPAIR * 64, T), U32)] * 2,
            pltpu.VMEM((TH, D), F32),
            pltpu.VMEM((TH, D), F32),
            pltpu.VMEM((S // 2, D), U32),
            pltpu.VMEM((S, D), BF16),
            pltpu.VMEM((D, FF), BF16),
            pltpu.VMEM((D, FF), BF16),
            pltpu.VMEM((FF, D + WD_PAD), BF16),
            pltpu.VMEM((16, D), BF16),
            pltpu.SemaphoreType.DMA((5 + 3 * NC + NT_ + 8,)),
        ],
        compiler_params=pltpu.CompilerParams(vmem_limit_bytes=100 * 1024 * 1024,
                                             disable_semaphore_checks=True, disable_bounds_checks=True),
        name="hedgehog_mod",
    )(
        A_x.reshape(S, D),
        A_wqkv,
        A_w_phi,
        A_wo,
        B_w_r,
        B_w_gate,
        B_w_up,
        B_w_down,
    )
    return out.reshape(1, S, D)
```

```python
import jax
import jax.numpy as jnp
from jax import lax
import jax.experimental.pallas as pl
import jax.experimental.pallas.tpu as pltpu

F32 = jnp.float32
BF16 = jnp.bfloat16
U32 = jnp.uint32

S = 2048
D = 1024
H = 32
DH = 32
FF = 3584
NPAIR = H // 2
LOG2E = 1.4426950408889634
LN_EPS = 1e-5

T = 256
TH = T // 2
NT_ = S // T
RC = 256
NC = D // RC
PPC = RC // 64
LNC = 16
WD_PAD = 128

LN1_PLAN = tuple((k * 12 // 16, k * 12 // 16 + 3) for k in range(16))
LN2B_PLAN = ((None, 0), (None, 0), (None, 0), (1, 6), (3, 8), (5, 10), (7, 12), (9, 14))
LN2A_PLAN = ((None, 18), (None, 18), (16, 19), (17, 20), (18, 21), (19, 22), (20, 23), (21, None))
PRO_LN1_PLAN = tuple((None, None) for k in range(16))
WO_ROWS = 352
WO_PLAN = tuple((k + 1, None) for k in range(11))
Z_PLAN = tuple((1 + k * 12 // 16, 1 + k * 12 // 16 + 3) for k in range(16))
UNROLL2 = 2
QUARTERS = True
G3_AT = 4

NN = (((1,), (0,)), ((), ()))
NT = (((1,), (1,)), ((), ()))


def _dot(a, b, dims):
    return lax.dot_general(a, b, dims, preferred_element_type=F32)


def _recip(x):
    return pl.reciprocal(x, approx=False, full_range=False)


def _pack(x):
    return pltpu.bitcast(x, U32)


def _unpack(x):
    return pltpu.bitcast(x, BF16)


def _pair_allreduce(a, op):
    a = op(a, pltpu.roll(a, 2, 0))
    return op(a, pltpu.roll(a, 4, 0))


def _tree(op, xs):
    xs = list(xs)
    while len(xs) > 1:
        nxt = [op(xs[i], xs[i + 1]) for i in range(0, len(xs) - 1, 2)]
        if len(xs) % 2:
            nxt.append(xs[-1])
        xs = nxt
    return xs[0]


def _dual_exp(p):
    sl = [p[8 * i:8 * i + 8, :] for i in range(8)]
    mx = _pair_allreduce(_tree(jnp.maximum, sl), jnp.maximum)
    mn = _pair_allreduce(_tree(jnp.minimum, sl), jnp.minimum)
    ep = [jnp.exp2(s - mx) for s in sl]
    en = [jnp.exp2(mn - s) for s in sl]
    sp = _pair_allreduce(_tree(jnp.add, ep), jnp.add)
    sn = _pair_allreduce(_tree(jnp.add, en), jnp.add)
    return ep, en, sp, sn


def _after(x, never, anchor):
    if anchor is None:
        return x
    d = jnp.concatenate([anchor] * (x.shape[0] // 8), axis=0)
    if x.shape[1] == 128:
        return jnp.where(never, d, x)
    return jnp.concatenate([jnp.where(never, d, x[:, :128]), x[:, 128:]], axis=1)


def _gate(x, never, deps):
    for i, dep in enumerate(deps):
        d = jnp.broadcast_to(dep, (8, 128))
        if x.dtype != F32:
            d = pltpu.bitcast(d, x.dtype)
        blk = jnp.where(never, d, x[8 * i:8 * i + 8, :128])
        if x.shape[1] > 128:
            blk = jnp.concatenate([blk, x[8 * i:8 * i + 8, 128:]], axis=1)
        parts = ([x[:8 * i, :]] if i else []) + [blk, x[8 * i + 8:, :]]
        x = jnp.concatenate(parts, axis=0)
    return x


def _lane_fold(a):
    return _tree(jnp.add, [a[:, 128 * i:128 * i + 128] for i in range(a.shape[1] // 128)])


def _row_sum(a):
    return jnp.sum(_lane_fold(a), axis=-1, keepdims=True)


def _lane_tile(a, n):
    return a if n == 1 else jnp.concatenate([a] * n, axis=1)


class _Side:
    def __init__(self, never):
        self.never = never
        self.jobs = []
        self.deps = {}

    def add(self, plan, fn):
        for k, (rel, due) in enumerate(plan):
            if rel is None:
                self._run(due, fn, k, None)
            else:
                self.jobs.append((rel, due, fn, k))

    def _run(self, due, fn, k, anchor):
        dep = fn(k, anchor)
        if due is not None:
            self.deps.setdefault(due, []).append(dep)

    def gate(self, step, x):
        return _gate(x, self.never, self.deps.pop(step, []))

    def done(self, step, res):
        anchor = res[res.shape[0] - 8:, res.shape[1] - 128:]
        for job in [j for j in self.jobs if j[0] == step]:
            self.jobs.remove(job)
            self._run(job[1], job[2], job[3], anchor)


def _kernel(x_hbm, wqkv_hbm, wphi_hbm, wo_hbm, wr_hbm, wg_hbm, wu_hbm, wd_hbm, out_hbm,
            x_v, xn_v, wraw_v, wt_v, wphi_v, a_v, woraw_v, wo_v, wrraw_v, wr_v, kvacc_v, kvbf_v,
            z_v, zb_v, phi_v, ha_v, hb_v, hn_v, o_v, wg_v, wu_v, wd_v, patch_v,
            sem):
    SX, SW, SO, SM = 0, 5, 5 + 3 * NC, 5 + 3 * NC + NT_ + 1

    def x_copy(i):
        t0, t1 = ((0, 1), (1, 2), (2, 3), (3, 5), (5, NT_))[i]
        rows = pl.ds(t0 * T, (t1 - t0) * T)
        return pltpu.make_async_copy(x_hbm.at[rows, :], x_v.at[rows, :], sem.at[SX + i])

    def w_copy(j, c):
        return pltpu.make_async_copy(wqkv_hbm.at[:, pl.ds(j * D + c * RC, RC)], wraw_v.at[j * NC + c],
                                     sem.at[SW + j * NC + c])

    wphi_copy = pltpu.make_async_copy(wphi_hbm, wphi_v, sem.at[SM + 4])
    wr_copy = pltpu.make_async_copy(wr_hbm, wrraw_v, sem.at[SM + 5])
    wo_copy = pltpu.make_async_copy(wo_hbm, woraw_v, sem.at[SM + 6])
    wg_copy = pltpu.make_async_copy(wg_hbm, wg_v, sem.at[SM + 0])
    wu_copy = pltpu.make_async_copy(wu_hbm, wu_v, sem.at[SM + 1])
    wd_copy = pltpu.make_async_copy(wd_hbm, wd_v.at[:, pl.ds(0, D)], sem.at[SM + 2])

    wphi_copy.start()
    x_copy(0).start()
    w_copy(1, 0).start()
    w_copy(1, 1).start()
    x_copy(1).start()
    w_copy(1, 2).start()

    def half(r):
        return r // 2 if isinstance(r, int) else pl.multiple_of(r // 2, LNC // 2)

    def ln_rows(r0, n, never=None, anchor=None):
        x = _after(x_v[pl.ds(r0, n), :].astype(F32), never, anchor)
        xc = x - _row_sum(x) * (1.0 / D)
        rstd = lax.rsqrt(_row_sum(xc * xc) * (1.0 / D) + LN_EPS)
        xn_v[pl.ds(half(r0), n // 2), :] = _pack((xc * rstd).astype(BF16))
        return _tree(jnp.add, [rstd[8 * i:8 * i + 8, :] for i in range(min(n, LNC) // 8)])

    def xn_tile(r0):
        return _unpack(xn_v[pl.ds(half(r0), T // 2), :])

    wphi_copy.wait()
    x_copy(0).wait()
    w_copy(1, 3).start()
    for c in range(NC):
        w_copy(2, c).start()
    x_copy(2).start()

    row = lax.broadcasted_iota(jnp.int32, (128, DH), 0)
    col = lax.broadcasted_iota(jnp.int32, (128, DH), 1)
    expand = jnp.where(((row & 63) >> 1) == col, 1.0, 0.0).astype(BF16)
    a_all = _dot(expand, wphi_v[...].reshape(H * DH, DH), NT)
    row = lax.broadcasted_iota(jnp.int32, (128, 128), 0)
    col = lax.broadcasted_iota(jnp.int32, (128, 128), 1)
    a_keep = (2 * (row >> 6) + (row & 1)) == (col >> 5)
    for g in range(8):
        a_v[64 * g:64 * g + 64, :] = _pack(jnp.where(a_keep, a_all[:, g * 128:(g + 1) * 128], 0.0).astype(BF16))
    never0 = ln_rows(0, T)[0, 0] < 0.0
    hb_v[...] = jnp.zeros((TH, D), F32)

    def fold(j, c, side=None, step0=None):
        out = []
        for s in range(RC // 128):
            g = c * (RC // 128) + s
            w = wraw_v[j * NC + c, :, s * 128:(s + 1) * 128]
            g0 = 64 * g if isinstance(g, int) else pl.multiple_of(64 * g, 64)
            if j == 2:
                wt = w.T
            else:
                res = _dot(_unpack(a_v[pl.ds(g0, 64), :]), w, NT)
                if side is not None:
                    side.done(step0 + s, res)
                wt = (res * LOG2E).astype(BF16)
                out.append(res)
            wt_v[j][pl.ds(g0, 64), :] = _pack(wt)
        return out

    def wt_rows(j, c):
        return wt_v[j][c * RC // 2:(c + 1) * RC // 2, :]

    def k_features(pk, slot, c, first, ties=None):
        for j in range(PPC):
            pr = c * PPC + j
            p = pk[64 * j:64 * j + 64, :]
            if ties is not None:
                d = jnp.concatenate(ties[1][2 * j:2 * j + 2], axis=1)
                p = jnp.concatenate([jnp.where(ties[0], d, p[0:8, :]), p[8:, :]], axis=0)
            ep, en, sp, sn = _dual_exp(p)
            inv = _recip(sp * sn)
            rp = sn * inv
            rn = sp * inv
            phi = jnp.concatenate([e * rp for e in ep] + [e * rn for e in en], axis=0)
            z_v[pr] = phi if first else z_v[pr] + phi
            phi_v[slot][64 * pr:64 * pr + 64, :] = _pack(phi.astype(BF16))

    row = lax.broadcasted_iota(jnp.int32, (64, 128), 0)
    col = lax.broadcasted_iota(jnp.int32, (64, 128), 1)
    kv_keep = (row >> 5) == (col & 1)

    def kv_update(vt, slot, c, first, publish=False):
        for j in range(PPC):
            pr = c * PPC + j
            upd = _dot(vt[64 * j:64 * j + 64, :].astype(BF16), _unpack(phi_v[slot][64 * pr:64 * pr + 64, :]), NT)
            acc = upd if first else kvacc_v[pr] + upd
            kvacc_v[pr] = acc
            if publish:
                kvbf_v[32 * pr:32 * pr + 32, :] = _pack(jnp.where(kv_keep, acc, 0.0).astype(BF16))

    def proj(j, c, xn):
        if QUARTERS:
            return proj_steps(_Side(None), 0, j, c, xn)
        return _dot(_unpack(wt_rows(j, c)), xn, NT)

    def proj_steps(side, step0, j, c, xn):
        w = wt_rows(j, c)
        quarters = []
        for n in range(2):
            for m in range(2):
                step = step0 + 2 * n + m
                wq = side.gate(step, w[m * (RC // 4):(m + 1) * (RC // 4), :])
                res = _dot(_unpack(wq), xn[n * TH:(n + 1) * TH, :], NT)
                side.done(step, res)
                quarters.append(res)
        return jnp.concatenate(
            [jnp.concatenate([quarters[0], quarters[2]], axis=1),
             jnp.concatenate([quarters[1], quarters[3]], axis=1)], axis=0)

    def spots(res, n):
        m, w = res.shape
        allp = [res[r:r + 8, c:c + 128] for c in range(0, w, 128) for r in range(56, m, 64)]
        return [allp[(i * len(allp)) // n] for i in range(n)]

    def stash(i, val):
        for q in range(4):
            zb_v[4 * i + q] = val[128 * (q // 2):128 * (q // 2) + 128, 128 * (q % 2):128 * (q % 2) + 128]

    def unstash(i):
        return jnp.concatenate(
            [jnp.concatenate([zb_v[4 * i + 2 * r], zb_v[4 * i + 2 * r + 1]], axis=1) for r in range(2)], axis=0)

    w_copy(1, 0).wait()
    for c in range(NC):
        w_copy(0, c).start()
    x_copy(3).start()
    fold(1, 0)
    stash(0, proj(1, 0, xn_tile(0)))

    w_copy(1, 1).wait()
    wo_copy.start()
    wr_copy.start()
    x_copy(4).start()
    f = fold(1, 1)
    pk = proj(1, 1, xn_tile(0))
    stash(1, pk)
    k_features(unstash(0), 0, 0, True, (never0, spots(f[0], 2) + spots(f[1], 2) + spots(pk, 8)[:4]))

    x_copy(1).wait()
    w_copy(1, 2).wait()
    wg_copy.start()
    wu_copy.start()
    wd_copy.start()
    side = _Side(never0)
    side.add(PRO_LN1_PLAN, lambda k, a: ln_rows(T + k * LNC, LNC, never0, a))
    fold(1, 2, side, 0)
    stash(2, proj_steps(side, 2, 1, 2, xn_tile(0)))
    xn1 = xn_tile(T)
    k_features(proj(1, 0, xn1), 1, 0, False)
    k_features(proj(1, 1, xn1), 1, 1, True)
    stash(3, proj(1, 2, xn1))

    w_copy(1, 3).wait()
    for c in range(3):
        w_copy(2, c).wait()
    fold(1, 3)
    xn0, xn1 = xn_tile(0), xn_tile(T)
    k_features(proj(1, 3, xn0), 0, 3, True)
    k_features(proj(1, 3, xn1), 1, 3, False)
    for c in range(3):
        fold(2, c)
    vt00 = proj(2, 0, xn0)
    k_features(unstash(1), 0, 1, False, (never0, spots(vt00, 2 * PPC)))
    vt10 = proj(2, 0, xn1)
    k_features(unstash(2), 0, 2, True, (never0, spots(vt10, 2 * PPC)))
    kv_update(vt00, 0, 0, True)
    vt01 = proj(2, 1, xn0)
    k_features(unstash(3), 1, 2, False, (never0, spots(vt01, 2 * PPC)))
    kv_update(vt10, 1, 0, False)
    stash(0, proj(2, 1, xn1))
    kv_update(vt01, 0, 1, True)

    w_copy(2, 3).wait()
    x_copy(2).wait()
    w_copy(0, 0).wait()
    side = _Side(never0)
    side.add(LN1_PLAN, lambda k, a: ln_rows(2 * T + k * LNC, LNC, never0, a))
    fold(0, 0, side, -1)
    fold(2, 3)
    kv_update(unstash(0), 1, 1, False)
    xn0, xn1 = xn_tile(0), xn_tile(T)
    vt02 = proj_steps(side, 1, 2, 2, xn0)
    vt12 = proj_steps(side, 5, 2, 2, xn1)
    kv_update(vt02, 0, 2, True)
    vt03 = proj_steps(side, 9, 2, 3, xn0)
    kv_update(vt12, 1, 2, False)
    vt13 = proj_steps(side, 13, 2, 3, xn1)
    kv_update(vt03, 0, 3, True)
    kv_update(vt13, 1, 3, False)

    def phase1(u, carry):
        never = u < 0

        @pl.when(u == 0)
        def _():
            for c in range(1, NC):
                w_copy(0, c).wait()
            x_copy(3).wait()
            wo_copy.wait()
            wr_copy.wait()

        @pl.when(u == 1)
        def _():
            x_copy(4).wait()

        pending = None
        for i in range(2):
            t = 2 * u + 2 + i
            r0 = pl.multiple_of(t * T, T)
            rn = pl.multiple_of(jnp.minimum(t + 1, NT_ - 1) * T, T)
            side = _Side(never)
            xn = xn_tile(r0)
            for c in range(NC):
                pk = proj(1, c, xn)
                if c == 0 and pending is not None:
                    kv_update(*pending)
                k_features(pk, i, c, False)
            side.add(LN1_PLAN, lambda k, a: ln_rows(rn + k * LNC, LNC, never, a))
            if i == 0:
                def pack_wo(k, a):
                    rows = WO_ROWS // len(WO_PLAN)
                    w0 = pl.multiple_of(u * ((D - WO_ROWS) // 2) + k * rows, 16)
                    w = _pack(woraw_v[pl.ds(w0, rows), :])
                    d = jnp.concatenate([_lane_tile(pltpu.bitcast(a, U32), D // 128)] * (rows // 16), axis=0)
                    wo_v[pl.ds(pl.multiple_of(w0 // 2, 8), rows // 2), :] = jnp.where(never, d, w)
                side.add(WO_PLAN, pack_wo)
            else:
                def z_final(k, a):
                    z = _after(z_v[k], never, a)
                    zs = _row_sum(z)
                    zb_v[k] = jnp.broadcast_to(zs, (128, 128))
                    return zs[120:128, :]
                side.add(Z_PLAN, z_final)
            side.done(0, pk)
            vts = []
            for c in range(NC):
                vts.append(proj_steps(side, 4 * c + 1, 2, c, xn))
                if c > 0:
                    kv_update(vts[c - 1], i, c - 1, False, i == 1)
            pending = (vts[NC - 1], i, NC - 1, False, i == 1)
        fold(0, u + 1)
        kv_update(*pending)
        wr_v[...] = jnp.broadcast_to(wrraw_v[...].reshape(1, D).astype(F32), (8, D))
        return carry

    lax.fori_loop(0, (NT_ - 2) // 2, phase1, 0)

    def o_copy(r0, n, i):
        return pltpu.make_async_copy(o_v.at[pl.ds(r0, n), :], out_hbm.at[pl.ds(r0, n), :], sem.at[SO + i])

    def finish_rows(h_ref, k, r0, valid, st, never=None, anchor=None):
        best, besti = st["route"]
        wr = jnp.concatenate([wr_v[...]] * (LNC // 8), axis=0)
        sub = lax.broadcasted_iota(jnp.int32, (8, 1), 0)
        h = _after(h_ref[k * LNC:(k + 1) * LNC, :], never, anchor)
        m = _row_sum(h) * (1.0 / D)
        hc = h - m
        rstd = lax.rsqrt(_row_sum(hc * hc) * (1.0 / D) + LN_EPS)
        r = (_row_sum(hc * wr) * rstd).astype(BF16).astype(F32)
        hn = hc * rstd
        hn_v[pl.ds(half(r0), LNC // 2), :] = _pack(hn.astype(BF16))
        o_v[pl.ds(r0, LNC), :] = (hn + h).astype(BF16)
        if valid is not None:
            r = jnp.where(valid, r, -jnp.inf)
        for i in range(LNC // 8):
            ri = r[8 * i:8 * i + 8, :]
            better = ri > best
            best = jnp.where(better, ri, best)
            besti = jnp.where(better, sub + (r0 + 8 * i), besti)
        st["route"] = (best, besti)
        return best

    def q_features(pq, slot, c):
        for j in range(PPC):
            pr = c * PPC + j
            ep, en, sp, sn = _dual_exp(pq[64 * j:64 * j + 64, :])
            zz = [_lane_tile(zb_v[pr, 8 * i:8 * i + 8, :], pq.shape[1] // 128) for i in range(16)]
            ap = _pair_allreduce(_tree(jnp.add, [ep[i] * zz[i] for i in range(8)]), jnp.add)
            an = _pair_allreduce(_tree(jnp.add, [en[i] * zz[8 + i] for i in range(8)]), jnp.add)
            inv = _recip(ap * sn + (an + 1e-6 * sn) * sp)
            rp = sn * inv
            rn = sp * inv
            phi = jnp.concatenate([e * rp for e in ep] + [e * rn for e in en], axis=0)
            phi_v[slot][64 * pr:64 * pr + 64, :] = _pack(phi.astype(BF16))

    def attn_rows(slot, c, lo, hi):
        res = jnp.concatenate(
            [_dot(_unpack(kvbf_v[32 * pr:32 * pr + 32, :]), _unpack(phi_v[slot][64 * pr:64 * pr + 64, lo:hi]), NN)
             for pr in range(c * PPC, (c + 1) * PPC)], axis=0)
        return res.astype(BF16).T

    def out_proj(side, step0, o, k0, k1, n0=0, n1=D // 128):
        cols = []
        for n in range(n0, n1):
            w = side.gate(step0 + n, wo_v[k0 // 2:k1 // 2, n * 128:(n + 1) * 128])
            res = _dot(o, _unpack(w), NN)
            side.done(step0 + n, res)
            cols.append(res)
        return jnp.concatenate(cols, axis=1)

    def phase2(u, carry):
        for i in range(UNROLL2):
            carry = phase2_tile(u * UNROLL2 + i, i % 2, carry, u < 0)

        r0 = pl.multiple_of(u * (UNROLL2 * T), T)

        @pl.when(u == 0)
        def _():
            o_copy(0, UNROLL2 * T - TH, 0).start()

        @pl.when(u > 0)
        def _():
            o_copy(pl.multiple_of(jnp.maximum(r0 - TH, 0), TH), UNROLL2 * T, u).start()

        return carry

    def phase2_tile(t, slot, carry, never):
        r0 = pl.multiple_of(t * T, T)
        rb = pl.multiple_of(jnp.maximum(r0 - TH, 0), TH)
        side = _Side(never)
        st = {"route": carry}
        side.add(LN2B_PLAN, lambda k, a: finish_rows(hb_v, k, rb + k * LNC, t > 0, st, side.never, a))

        xn = xn_tile(r0)
        os_ = []
        for c in range(NC):
            pq = proj(0, c, xn)
            if c == 0:
                pq = side.gate(0, pq)
            q_features(pq, slot, c)
            if c > 0:
                os_.append(attn_rows(slot, c - 1, 0, T))
        oa = jnp.concatenate([o[0:TH, :] for o in os_[:2]], axis=1)
        ha0 = out_proj(side, 0, oa, 0, D // 2, 0, G3_AT)
        os_.append(attn_rows(slot, NC - 1, 0, T))
        ha1 = out_proj(side, 0, oa, 0, D // 2, G3_AT, D // 128)
        ha = jnp.concatenate([ha0, ha1], axis=1) + x_v[pl.ds(r0, TH), :].astype(F32)
        ha_v[...] = ha + out_proj(side, 8, jnp.concatenate([o[0:TH, :] for o in os_[2:]], axis=1), D // 2, D)
        side.add(LN2A_PLAN, lambda k, a: finish_rows(ha_v, k, r0 + k * LNC, None, st, side.never, a))
        ob = jnp.concatenate([o[TH:T, :] for o in os_], axis=1)
        hb_v[...] = x_v[pl.ds(r0 + TH, TH), :].astype(F32) + out_proj(side, 16, ob, 0, D)
        return st["route"]

    route = lax.fori_loop(
        0, NT_ // UNROLL2, phase2,
        (jnp.full((8, 1), -jnp.inf, F32), jnp.zeros((8, 1), jnp.int32)))
    wg_copy.wait()
    wu_copy.wait()
    wd_copy.wait()
    st = {"route": route}
    for k in range(TH // LNC):
        finish_rows(hb_v, k, S - TH + k * LNC, None, st)
    best, besti = st["route"]
    o_copy(S - TH, TH, NT_).start()

    rmax = jnp.max(best, axis=0, keepdims=True)
    idx = jnp.min(jnp.where(best == rmax, besti, S), axis=0, keepdims=True)
    idx_s = jnp.clip(idx[0, 0], 0, S - 1)
    blk = pl.multiple_of((idx_s >> 4) << 4, 16)
    xs = _unpack(hn_v[pl.ds(pl.multiple_of(blk >> 1, 8), 8), :])
    g = _dot(xs, wg_v[...], NN)
    u = _dot(xs, wu_v[...], NN)
    a = (g * jax.nn.sigmoid(g) * u).astype(BF16)
    y = _dot(a, wd_v[:, 0:D], NN) * jax.nn.sigmoid(rmax)
    sel = lax.broadcasted_iota(jnp.int32, (16, 1), 0) == (idx_s - blk)
    patch_v[...] = (o_v[pl.ds(blk, 16), :].astype(F32) + jnp.where(sel, y, 0.0)).astype(BF16)
    o_copy(0, UNROLL2 * T - TH, 0).wait()
    for u in range(1, NT_ // UNROLL2):
        o_copy(u * UNROLL2 * T - TH, UNROLL2 * T, u).wait()
    o_copy(S - TH, TH, NT_).wait()
    pc = pltpu.make_async_copy(patch_v, out_hbm.at[pl.ds(blk, 16), :], sem.at[SM + 3])
    pc.start()
    pc.wait()


@jax.jit
def pallas_sequential_preLN__linear_kernel_hedgehog__moe_arch_mod__prompt_kernel(
    A_x: jax.Array,
    A_wqkv: jax.Array,
    A_w_phi: jax.Array,
    A_wo: jax.Array,
    B_x: jax.Array,
    B_w_r: jax.Array,
    B_w_gate: jax.Array,
    B_w_up: jax.Array,
    B_w_down: jax.Array,
):
    del B_x
    hbm = pl.BlockSpec(memory_space=pl.ANY)
    out = pl.pallas_call(
        _kernel,
        out_shape=jax.ShapeDtypeStruct((S, D), BF16),
        in_specs=[hbm] * 8,
        out_specs=hbm,
        scratch_shapes=[
            pltpu.VMEM((S, D), BF16),
            pltpu.VMEM((S // 2, D), U32),
            pltpu.VMEM((3 * NC, D, RC), BF16),
            [pltpu.VMEM((D // 2, D), U32)] * 3,
            pltpu.VMEM((H, DH, DH), BF16),
            pltpu.VMEM((8 * 64, 128), U32),
            pltpu.VMEM((D, D), BF16),
            pltpu.VMEM((D // 2, D), U32),
            pltpu.VMEM((D,), BF16),
            pltpu.VMEM((8, D), F32),
            pltpu.VMEM((NPAIR, 64, 128), F32),
            pltpu.VMEM((NPAIR * 32, 128), U32),
            pltpu.VMEM((NPAIR, 128, T), F32),
            pltpu.VMEM((NPAIR, 128, 128), F32),
            [pltpu.VMEM((NPAIR * 64, T), U32)] * 2,
            pltpu.VMEM((TH, D), F32),
            pltpu.VMEM((TH, D), F32),
            pltpu.VMEM((S // 2, D), U32),
            pltpu.VMEM((S, D), BF16),
            pltpu.VMEM((D, FF), BF16),
            pltpu.VMEM((D, FF), BF16),
            pltpu.VMEM((FF, D + WD_PAD), BF16),
            pltpu.VMEM((16, D), BF16),
            pltpu.SemaphoreType.DMA((5 + 3 * NC + NT_ + 8,)),
        ],
        compiler_params=pltpu.CompilerParams(vmem_limit_bytes=100 * 1024 * 1024,
                                             disable_semaphore_checks=True, disable_bounds_checks=True),
        name="hedgehog_mod",
    )(
        A_x.reshape(S, D),
        A_wqkv,
        A_w_phi,
        A_wo,
        B_w_r,
        B_w_gate,
        B_w_up,
        B_w_down,
    )
    return out.reshape(1, S, D)
```

```python
import jax
import jax.numpy as jnp
from jax import lax
import jax.experimental.pallas as pl
import jax.experimental.pallas.tpu as pltpu

F32 = jnp.float32
BF16 = jnp.bfloat16
U32 = jnp.uint32

S = 2048
D = 1024
H = 32
DH = 32
FF = 3584
NPAIR = H // 2
LOG2E = 1.4426950408889634
LN_EPS = 1e-5

T = 256
TH = T // 2
NT_ = S // T
RC = 256
NC = D // RC
PPC = RC // 64
LNC = 16
WD_PAD = 128

LN1_PLAN = tuple((k * 12 // 16, k * 12 // 16 + 3) for k in range(16))
LN2B_PLAN = ((None, 0), (None, 0), (None, 0), (1, 6), (3, 8), (5, 10), (7, 12), (9, 14))
LN2A_PLAN = ((None, 18), (None, 18), (16, 19), (17, 20), (18, 21), (19, 22), (20, 23), (21, None))
PRO_LN1_PLAN = tuple((None, None) for k in range(16))
WO_ROWS = 352
WO_PLAN = tuple((k + 1, None) for k in range(11))
Z_PLAN = tuple((1 + k * 12 // 16, 1 + k * 12 // 16 + 3) for k in range(16))
UNROLL2 = 2
FV = 8 * 128
FM = FF - FV
PACK_PLAN = tuple((r, None) for r in [x - f for f in (0, 0.9, 0.45) for x in range(100, 116)] + [1, 3, 5, 13])
MOE_NA = 38
MOE_ND = 2
QUARTERS = True
G3_AT = 4

NN = (((1,), (0,)), ((), ()))
NT = (((1,), (1,)), ((), ()))


def _dot(a, b, dims):
    return lax.dot_general(a, b, dims, preferred_element_type=F32)


def _recip(x):
    return pl.reciprocal(x, approx=False, full_range=False)


def _pack(x):
    return pltpu.bitcast(x, U32)


def _unpack(x):
    return pltpu.bitcast(x, BF16)


def _pair_allreduce(a, op):
    a = op(a, pltpu.roll(a, 2, 0))
    return op(a, pltpu.roll(a, 4, 0))


def _tree(op, xs):
    xs = list(xs)
    while len(xs) > 1:
        nxt = [op(xs[i], xs[i + 1]) for i in range(0, len(xs) - 1, 2)]
        if len(xs) % 2:
            nxt.append(xs[-1])
        xs = nxt
    return xs[0]


def _dual_exp(p):
    sl = [p[8 * i:8 * i + 8, :] for i in range(8)]
    mx = _pair_allreduce(_tree(jnp.maximum, sl), jnp.maximum)
    mn = _pair_allreduce(_tree(jnp.minimum, sl), jnp.minimum)
    ep = [jnp.exp2(s - mx) for s in sl]
    en = [jnp.exp2(mn - s) for s in sl]
    sp = _pair_allreduce(_tree(jnp.add, ep), jnp.add)
    sn = _pair_allreduce(_tree(jnp.add, en), jnp.add)
    return ep, en, sp, sn


def _after(x, never, anchor):
    if anchor is None:
        return x
    d = jnp.concatenate([anchor] * (x.shape[0] // 8), axis=0)
    if x.shape[1] == 128:
        return jnp.where(never, d, x)
    return jnp.concatenate([jnp.where(never, d, x[:, :128]), x[:, 128:]], axis=1)


def _gate(x, never, deps):
    for i, dep in enumerate(deps):
        d = jnp.broadcast_to(dep, (8, 128))
        if x.dtype != F32:
            d = pltpu.bitcast(d, x.dtype)
        blk = jnp.where(never, d, x[8 * i:8 * i + 8, :128])
        if x.shape[1] > 128:
            blk = jnp.concatenate([blk, x[8 * i:8 * i + 8, 128:]], axis=1)
        parts = ([x[:8 * i, :]] if i else []) + [blk, x[8 * i + 8:, :]]
        x = jnp.concatenate(parts, axis=0)
    return x


def _lane_fold(a):
    return _tree(jnp.add, [a[:, 128 * i:128 * i + 128] for i in range(a.shape[1] // 128)])


def _row_sum(a):
    return jnp.sum(_lane_fold(a), axis=-1, keepdims=True)


def _lane_tile(a, n):
    return a if n == 1 else jnp.concatenate([a] * n, axis=1)


def _sublane_allreduce(a):
    a = a + pltpu.roll(a, 4, 0)
    a = a + pltpu.roll(a, 2, 0)
    return a + pltpu.roll(a, 1, 0)


def _col_broadcast(row8):
    return jnp.concatenate([row8] * 16, axis=0).astype(BF16).T.astype(F32)


def _vpu_matvec(xb, w_rows, never, anchors, lag):
    ng = xb.shape[0] // 8
    acc, hist = None, []
    for g in range(ng):
        dep = anchors[(g * len(anchors)) // ng]
        if g >= lag:
            dep = dep + hist[g - lag]
        x = jnp.where(never, dep, xb[8 * g:8 * g + 8, :])
        w = w_rows(g)
        t = w * _lane_tile(x, w.shape[1] // 128)
        acc = t if acc is None else acc + t
        hist.append(acc[:, -128:])
    return acc


class _Side:
    def __init__(self, never):
        self.never = never
        self.jobs = []
        self.deps = {}

    def add(self, plan, fn):
        for k, (rel, due) in enumerate(plan):
            if rel is None:
                self._run(due, fn, k, None)
            else:
                self.jobs.append((rel, due, fn, k))

    def _run(self, due, fn, k, anchor):
        dep = fn(k, anchor)
        if due is not None:
            self.deps.setdefault(due, []).append(dep)

    def gate(self, step, x):
        return _gate(x, self.never, self.deps.pop(step, []))

    def done(self, step, res):
        m = res.shape[0] // 8
        for job in sorted([j for j in self.jobs if step - 1 < j[0] <= step], key=lambda j: j[0]):
            self.jobs.remove(job)
            g = m - 1 - int((step - job[0]) * m)
            self._run(job[1], job[2], job[3], res[8 * g:8 * g + 8, res.shape[1] - 128:])


def _kernel(x_hbm, wqkv_hbm, wphi_hbm, wo_hbm, wr_hbm, wg_hbm, wu_hbm, wd_hbm, out_hbm,
            x_v, xn_v, wraw_v, wt_v, wphi_v, a_v, woraw_v, wo_v, wrraw_v, wr_v, kvacc_v, kvbf_v,
            z_v, zb_v, phi_v, ha_v, hb_v, hn_v, o_v, wg_v, wu_v, wd_v, wgp_v, wup_v, wdp_v, patch_v,
            sem):
    SX, SW, SO, SM = 0, 5, 5 + 3 * NC, 5 + 3 * NC + NT_ + 1

    def x_copy(i):
        t0, t1 = ((0, 1), (1, 2), (2, 3), (3, 5), (5, NT_))[i]
        rows = pl.ds(t0 * T, (t1 - t0) * T)
        return pltpu.make_async_copy(x_hbm.at[rows, :], x_v.at[rows, :], sem.at[SX + i])

    def w_copy(j, c):
        return pltpu.make_async_copy(wqkv_hbm.at[:, pl.ds(j * D + c * RC, RC)], wraw_v.at[j * NC + c],
                                     sem.at[SW + j * NC + c])

    wphi_copy = pltpu.make_async_copy(wphi_hbm, wphi_v, sem.at[SM + 4])
    wr_copy = pltpu.make_async_copy(wr_hbm, wrraw_v, sem.at[SM + 5])
    wo_copy = pltpu.make_async_copy(wo_hbm, woraw_v, sem.at[SM + 6])
    wg_copy = pltpu.make_async_copy(wg_hbm, wg_v, sem.at[SM + 0])
    wu_copy = pltpu.make_async_copy(wu_hbm, wu_v, sem.at[SM + 1])
    wd_copy = pltpu.make_async_copy(wd_hbm, wd_v.at[:, pl.ds(0, D)], sem.at[SM + 2])

    wphi_copy.start()
    x_copy(0).start()
    w_copy(1, 0).start()
    w_copy(1, 1).start()
    x_copy(1).start()
    w_copy(1, 2).start()

    def half(r):
        return r // 2 if isinstance(r, int) else pl.multiple_of(r // 2, LNC // 2)

    def ln_rows(r0, n, never=None, anchor=None):
        x = _after(x_v[pl.ds(r0, n), :].astype(F32), never, anchor)
        xc = x - _row_sum(x) * (1.0 / D)
        rstd = lax.rsqrt(_row_sum(xc * xc) * (1.0 / D) + LN_EPS)
        xn_v[pl.ds(half(r0), n // 2), :] = _pack((xc * rstd).astype(BF16))
        return _tree(jnp.add, [rstd[8 * i:8 * i + 8, :] for i in range(min(n, LNC) // 8)])

    def xn_tile(r0):
        return _unpack(xn_v[pl.ds(half(r0), T // 2), :])

    wphi_copy.wait()
    x_copy(0).wait()
    w_copy(1, 3).start()
    for c in range(NC):
        w_copy(2, c).start()
    x_copy(2).start()

    row = lax.broadcasted_iota(jnp.int32, (128, DH), 0)
    col = lax.broadcasted_iota(jnp.int32, (128, DH), 1)
    expand = jnp.where(((row & 63) >> 1) == col, 1.0, 0.0).astype(BF16)
    a_all = _dot(expand, wphi_v[...].reshape(H * DH, DH), NT)
    row = lax.broadcasted_iota(jnp.int32, (128, 128), 0)
    col = lax.broadcasted_iota(jnp.int32, (128, 128), 1)
    a_keep = (2 * (row >> 6) + (row & 1)) == (col >> 5)
    for g in range(8):
        a_v[64 * g:64 * g + 64, :] = _pack(jnp.where(a_keep, a_all[:, g * 128:(g + 1) * 128], 0.0).astype(BF16))
    never0 = ln_rows(0, T)[0, 0] < 0.0
    hb_v[...] = jnp.zeros((TH, D), F32)

    def fold(j, c, side=None, step0=None):
        out = []
        for s in range(RC // 128):
            g = c * (RC // 128) + s
            w = wraw_v[j * NC + c, :, s * 128:(s + 1) * 128]
            g0 = 64 * g if isinstance(g, int) else pl.multiple_of(64 * g, 64)
            if j == 2:
                wt = w.T
            else:
                res = _dot(_unpack(a_v[pl.ds(g0, 64), :]), w, NT)
                if side is not None:
                    side.done(step0 + s, res)
                wt = (res * LOG2E).astype(BF16)
                out.append(res)
            wt_v[j][pl.ds(g0, 64), :] = _pack(wt)
        return out

    def wt_rows(j, c):
        return wt_v[j][c * RC // 2:(c + 1) * RC // 2, :]

    def k_features(pk, slot, c, first, ties=None):
        for j in range(PPC):
            pr = c * PPC + j
            p = pk[64 * j:64 * j + 64, :]
            if ties is not None:
                d = jnp.concatenate(ties[1][2 * j:2 * j + 2], axis=1)
                p = jnp.concatenate([jnp.where(ties[0], d, p[0:8, :]), p[8:, :]], axis=0)
            ep, en, sp, sn = _dual_exp(p)
            inv = _recip(sp * sn)
            rp = sn * inv
            rn = sp * inv
            phi = jnp.concatenate([e * rp for e in ep] + [e * rn for e in en], axis=0)
            z_v[pr] = phi if first else z_v[pr] + phi
            phi_v[slot][64 * pr:64 * pr + 64, :] = _pack(phi.astype(BF16))

    row = lax.broadcasted_iota(jnp.int32, (64, 128), 0)
    col = lax.broadcasted_iota(jnp.int32, (64, 128), 1)
    kv_keep = (row >> 5) == (col & 1)

    def kv_update(vt, slot, c, first, publish=False):
        for j in range(PPC):
            pr = c * PPC + j
            upd = _dot(vt[64 * j:64 * j + 64, :].astype(BF16), _unpack(phi_v[slot][64 * pr:64 * pr + 64, :]), NT)
            acc = upd if first else kvacc_v[pr] + upd
            kvacc_v[pr] = acc
            if publish:
                kvbf_v[32 * pr:32 * pr + 32, :] = _pack(jnp.where(kv_keep, acc, 0.0).astype(BF16))

    def proj(j, c, xn):
        if QUARTERS:
            return proj_steps(_Side(None), 0, j, c, xn)
        return _dot(_unpack(wt_rows(j, c)), xn, NT)

    def proj_steps(side, step0, j, c, xn):
        w = wt_rows(j, c)
        quarters = []
        for n in range(2):
            for m in range(2):
                step = step0 + 2 * n + m
                wq = side.gate(step, w[m * (RC // 4):(m + 1) * (RC // 4), :])
                res = _dot(_unpack(wq), xn[n * TH:(n + 1) * TH, :], NT)
                side.done(step, res)
                quarters.append(res)
        return jnp.concatenate(
            [jnp.concatenate([quarters[0], quarters[2]], axis=1),
             jnp.concatenate([quarters[1], quarters[3]], axis=1)], axis=0)

    def spots(res, n):
        m, w = res.shape
        allp = [res[r:r + 8, c:c + 128] for c in range(0, w, 128) for r in range(56, m, 64)]
        return [allp[(i * len(allp)) // n] for i in range(n)]

    def pack_rows(src, s0, dst, d0, rows, cols, never, a, c0=0):
        w = _pack(src[pl.ds(pl.multiple_of(s0, 16), rows), c0:c0 + cols])
        d = jnp.concatenate([_lane_tile(pltpu.bitcast(a, U32), cols // 128)] * (rows // 16), axis=0)
        dst[pl.ds(pl.multiple_of(d0 // 2, 8), rows // 2), c0:c0 + cols] = jnp.where(never, d, w)

    def stash(i, val):
        for q in range(4):
            zb_v[4 * i + q] = val[128 * (q // 2):128 * (q // 2) + 128, 128 * (q % 2):128 * (q % 2) + 128]

    def unstash(i):
        return jnp.concatenate(
            [jnp.concatenate([zb_v[4 * i + 2 * r], zb_v[4 * i + 2 * r + 1]], axis=1) for r in range(2)], axis=0)

    w_copy(1, 0).wait()
    for c in range(NC):
        w_copy(0, c).start()
    x_copy(3).start()
    fold(1, 0)
    stash(0, proj(1, 0, xn_tile(0)))

    w_copy(1, 1).wait()
    wo_copy.start()
    wr_copy.start()
    x_copy(4).start()
    f = fold(1, 1)
    pk = proj(1, 1, xn_tile(0))
    stash(1, pk)
    k_features(unstash(0), 0, 0, True, (never0, spots(f[0], 2) + spots(f[1], 2) + spots(pk, 8)[:4]))

    x_copy(1).wait()
    w_copy(1, 2).wait()
    wg_copy.start()
    wu_copy.start()
    wd_copy.start()
    side = _Side(never0)
    side.add(PRO_LN1_PLAN, lambda k, a: ln_rows(T + k * LNC, LNC, never0, a))
    fold(1, 2, side, 0)
    stash(2, proj_steps(side, 2, 1, 2, xn_tile(0)))
    xn1 = xn_tile(T)
    k_features(proj(1, 0, xn1), 1, 0, False)
    k_features(proj(1, 1, xn1), 1, 1, True)
    stash(3, proj(1, 2, xn1))

    w_copy(1, 3).wait()
    for c in range(3):
        w_copy(2, c).wait()
    fold(1, 3)
    xn0, xn1 = xn_tile(0), xn_tile(T)
    k_features(proj(1, 3, xn0), 0, 3, True)
    k_features(proj(1, 3, xn1), 1, 3, False)
    for c in range(3):
        fold(2, c)
    vt00 = proj(2, 0, xn0)
    k_features(unstash(1), 0, 1, False, (never0, spots(vt00, 2 * PPC)))
    vt10 = proj(2, 0, xn1)
    k_features(unstash(2), 0, 2, True, (never0, spots(vt10, 2 * PPC)))
    kv_update(vt00, 0, 0, True)
    vt01 = proj(2, 1, xn0)
    k_features(unstash(3), 1, 2, False, (never0, spots(vt01, 2 * PPC)))
    kv_update(vt10, 1, 0, False)
    stash(0, proj(2, 1, xn1))
    kv_update(vt01, 0, 1, True)

    w_copy(2, 3).wait()
    x_copy(2).wait()
    w_copy(0, 0).wait()
    side = _Side(never0)
    side.add(LN1_PLAN, lambda k, a: ln_rows(2 * T + k * LNC, LNC, never0, a))
    fold(0, 0, side, -1)
    fold(2, 3)
    kv_update(unstash(0), 1, 1, False)
    xn0, xn1 = xn_tile(0), xn_tile(T)
    vt02 = proj_steps(side, 1, 2, 2, xn0)
    vt12 = proj_steps(side, 5, 2, 2, xn1)
    kv_update(vt02, 0, 2, True)
    vt03 = proj_steps(side, 9, 2, 3, xn0)
    kv_update(vt12, 1, 2, False)
    vt13 = proj_steps(side, 13, 2, 3, xn1)
    kv_update(vt03, 0, 3, True)
    kv_update(vt13, 1, 3, False)

    def phase1(u, carry):
        never = u < 0

        @pl.when(u == 0)
        def _():
            for c in range(1, NC):
                w_copy(0, c).wait()
            x_copy(3).wait()
            wo_copy.wait()
            wr_copy.wait()

        @pl.when(u == 1)
        def _():
            x_copy(4).wait()

        pending = None
        for i in range(2):
            t = 2 * u + 2 + i
            r0 = pl.multiple_of(t * T, T)
            rn = pl.multiple_of(jnp.minimum(t + 1, NT_ - 1) * T, T)
            side = _Side(never)
            xn = xn_tile(r0)
            for c in range(NC):
                pk = proj(1, c, xn)
                if c == 0 and pending is not None:
                    kv_update(*pending)
                k_features(pk, i, c, False)
            side.add(LN1_PLAN, lambda k, a: ln_rows(rn + k * LNC, LNC, never, a))
            if i == 0:
                def pack_wo(k, a):
                    rows = WO_ROWS // len(WO_PLAN)
                    w0 = u * ((D - WO_ROWS) // 2) + k * rows
                    pack_rows(woraw_v, w0, wo_v, w0, rows, D, never, a)
                side.add(WO_PLAN, pack_wo)
            else:
                def z_final(k, a):
                    z = _after(z_v[k], never, a)
                    zs = _row_sum(z)
                    zb_v[k] = jnp.broadcast_to(zs, (128, 128))
                    return zs[120:128, :]
                side.add(Z_PLAN, z_final)
            side.done(0, pk)
            vts = []
            for c in range(NC):
                vts.append(proj_steps(side, 4 * c + 1, 2, c, xn))
                if c > 0:
                    kv_update(vts[c - 1], i, c - 1, False, i == 1)
            pending = (vts[NC - 1], i, NC - 1, False, i == 1)
        fold(0, u + 1)
        kv_update(*pending)
        wr_v[...] = jnp.broadcast_to(wrraw_v[...].reshape(1, D).astype(F32), (8, D))
        return carry

    lax.fori_loop(0, (NT_ - 2) // 2, phase1, 0)

    def o_copy(r0, n, i):
        return pltpu.make_async_copy(o_v.at[pl.ds(r0, n), :], out_hbm.at[pl.ds(r0, n), :], sem.at[SO + i])

    def finish_rows(h_ref, k, r0, valid, st, never=None, anchor=None):
        best, besti = st["route"]
        wr = jnp.concatenate([wr_v[...]] * (LNC // 8), axis=0)
        sub = lax.broadcasted_iota(jnp.int32, (8, 1), 0)
        h = _after(h_ref[k * LNC:(k + 1) * LNC, :], never, anchor)
        m = _row_sum(h) * (1.0 / D)
        hc = h - m
        rstd = lax.rsqrt(_row_sum(hc * hc) * (1.0 / D) + LN_EPS)
        r = (_row_sum(hc * wr) * rstd).astype(BF16).astype(F32)
        hn = hc * rstd
        hn_v[pl.ds(half(r0), LNC // 2), :] = _pack(hn.astype(BF16))
        o_v[pl.ds(r0, LNC), :] = (hn + h).astype(BF16)
        if valid is not None:
            r = jnp.where(valid, r, -jnp.inf)
        for i in range(LNC // 8):
            ri = r[8 * i:8 * i + 8, :]
            better = ri > best
            best = jnp.where(better, ri, best)
            besti = jnp.where(better, sub + (r0 + 8 * i), besti)
        st["route"] = (best, besti)
        return best

    def q_features(pq, slot, c):
        for j in range(PPC):
            pr = c * PPC + j
            ep, en, sp, sn = _dual_exp(pq[64 * j:64 * j + 64, :])
            zz = [_lane_tile(zb_v[pr, 8 * i:8 * i + 8, :], pq.shape[1] // 128) for i in range(16)]
            ap = _pair_allreduce(_tree(jnp.add, [ep[i] * zz[i] for i in range(8)]), jnp.add)
            an = _pair_allreduce(_tree(jnp.add, [en[i] * zz[8 + i] for i in range(8)]), jnp.add)
            inv = _recip(ap * sn + (an + 1e-6 * sn) * sp)
            rp = sn * inv
            rn = sp * inv
            phi = jnp.concatenate([e * rp for e in ep] + [e * rn for e in en], axis=0)
            phi_v[slot][64 * pr:64 * pr + 64, :] = _pack(phi.astype(BF16))

    def attn_rows(slot, c, lo, hi):
        res = jnp.concatenate(
            [_dot(_unpack(kvbf_v[32 * pr:32 * pr + 32, :]), _unpack(phi_v[slot][64 * pr:64 * pr + 64, lo:hi]), NN)
             for pr in range(c * PPC, (c + 1) * PPC)], axis=0)
        return res.astype(BF16).T

    def out_proj(side, step0, o, k0, k1, n0=0, n1=D // 128):
        cols = []
        for n in range(n0, n1):
            w = side.gate(step0 + n, wo_v[k0 // 2:k1 // 2, n * 128:(n + 1) * 128])
            res = _dot(o, _unpack(w), NN)
            side.done(step0 + n, res)
            cols.append(res)
        return jnp.concatenate(cols, axis=1)

    def phase2(u, carry):
        for i in range(UNROLL2):
            carry = phase2_tile(u * UNROLL2 + i, i % 2, carry, u < 0)

        r0 = pl.multiple_of(u * (UNROLL2 * T), T)

        @pl.when(u == 0)
        def _():
            o_copy(0, UNROLL2 * T - TH, 0).start()

        @pl.when(u > 0)
        def _():
            o_copy(pl.multiple_of(jnp.maximum(r0 - TH, 0), TH), UNROLL2 * T, u).start()

        return carry

    def phase2_tile(t, slot, carry, never):
        r0 = pl.multiple_of(t * T, T)
        rb = pl.multiple_of(jnp.maximum(r0 - TH, 0), TH)
        side = _Side(never)
        st = {"route": carry}
        side.add(LN2B_PLAN, lambda k, a: finish_rows(hb_v, k, rb + k * LNC, t > 0, st, side.never, a))

        def pack_ffn(k, a):
            if k < 32:
                w0 = t * (D // NT_) + (k // 4) * 16
                pack_rows((wg_v, wu_v)[k % 2], w0, (wgp_v, wup_v)[k % 2], w0, 16, FM // 2, never, a,
                          (k // 2 % 2) * (FM // 2))
            else:
                w0 = t * (FM // NT_) + (k - 32) * 16
                pack_rows(wd_v, FV + w0, wdp_v, w0, 16, D, never, a)
        side.add(PACK_PLAN, pack_ffn)

        xn = xn_tile(r0)
        os_ = []
        for c in range(NC):
            pq = proj_steps(side, 100 + 4 * c, 0, c, xn)
            if c == 0:
                pq = side.gate(0, pq)
            q_features(pq, slot, c)
            if c > 0:
                os_.append(attn_rows(slot, c - 1, 0, T))
        oa = jnp.concatenate([o[0:TH, :] for o in os_[:2]], axis=1)
        ha0 = out_proj(side, 0, oa, 0, D // 2, 0, G3_AT)
        os_.append(attn_rows(slot, NC - 1, 0, T))
        ha1 = out_proj(side, 0, oa, 0, D // 2, G3_AT, D // 128)
        ha = jnp.concatenate([ha0, ha1], axis=1) + x_v[pl.ds(r0, TH), :].astype(F32)
        ha_v[...] = ha + out_proj(side, 8, jnp.concatenate([o[0:TH, :] for o in os_[2:]], axis=1), D // 2, D)
        side.add(LN2A_PLAN, lambda k, a: finish_rows(ha_v, k, r0 + k * LNC, None, st, side.never, a))
        ob = jnp.concatenate([o[TH:T, :] for o in os_], axis=1)
        hb_v[...] = x_v[pl.ds(r0 + TH, TH), :].astype(F32) + out_proj(side, 16, ob, 0, D)
        return st["route"]

    wg_copy.wait()
    wu_copy.wait()
    wd_copy.wait()
    route = lax.fori_loop(
        0, NT_ // UNROLL2, phase2,
        (jnp.full((8, 1), -jnp.inf, F32), jnp.zeros((8, 1), jnp.int32)))
    st = {"route": route}
    for k in range(TH // LNC):
        finish_rows(hb_v, k, S - TH + k * LNC, None, st)
    best, besti = st["route"]
    o_copy(S - TH, TH, NT_).start()

    rmax = jnp.max(best, axis=0, keepdims=True)
    idx = jnp.min(jnp.where(best == rmax, besti, S), axis=0, keepdims=True)
    idx_s = jnp.clip(idx[0, 0], 0, S - 1)
    blk = pl.multiple_of((idx_s >> 4) << 4, 16)
    pair = jnp.broadcast_to(hn_v[pl.ds(idx_s >> 1, 1), :], (8, D))
    x8 = pltpu.bitcast(jnp.where((idx_s & 1) == 1, pair & jnp.uint32(0xFFFF0000), pair << 16), F32)
    xs = jnp.concatenate([x8, x8], axis=0).astype(BF16)
    acts, anchors = [], []
    for c0 in range(0, FM, 128):
        g = _dot(xs, _unpack(wgp_v[:, c0:c0 + 128]), NN)[0:8, :]
        u = _dot(xs, _unpack(wup_v[:, c0:c0 + 128]), NN)[0:8, :]
        anchors += [g, u]
        acts.append(g * jax.nn.sigmoid(g) * u)
    gu = _sublane_allreduce(_vpu_matvec(
        _col_broadcast(x8),
        lambda g: jnp.concatenate([w[8 * g:8 * g + 8, FM:FF].astype(F32) for w in (wg_v, wu_v)], axis=1),
        never0, anchors[:MOE_NA], 1))
    g, u = gu[:, :FV], gu[:, FV:]
    acts.append(g * jax.nn.sigmoid(g) * u)
    a = jnp.concatenate(acts, axis=1)
    am = jnp.concatenate([a[:, FV:], a[:, FV:]], axis=0).astype(BF16)
    ys, anchors = [], anchors[MOE_NA:]
    for k0 in range(0, FM, 512):
        yk = _dot(am[:, k0:k0 + 512], _unpack(wdp_v[k0 // 2:k0 // 2 + 256, :]), NN)[0:8, :]
        ys.append(yk)
        anchors += [yk[:, c:c + 128] for c in range(128, D, 256)]
    ys.append(_sublane_allreduce(_vpu_matvec(
        _col_broadcast(a[:, :FV]), lambda g: wd_v[8 * g:8 * g + 8, 0:D].astype(F32), never0, anchors[:-MOE_ND], 2)))
    y = _tree(jnp.add, ys) * jax.nn.sigmoid(rmax)
    y = jnp.concatenate([y, y], axis=0)
    sel = lax.broadcasted_iota(jnp.int32, (16, 1), 0) == (idx_s - blk)
    patch_v[...] = (o_v[pl.ds(blk, 16), :].astype(F32) + jnp.where(sel, y, 0.0)).astype(BF16)
    o_copy(0, UNROLL2 * T - TH, 0).wait()
    for u in range(1, NT_ // UNROLL2):
        o_copy(u * UNROLL2 * T - TH, UNROLL2 * T, u).wait()
    o_copy(S - TH, TH, NT_).wait()
    pc = pltpu.make_async_copy(patch_v, out_hbm.at[pl.ds(blk, 16), :], sem.at[SM + 3])
    pc.start()
    pc.wait()


@jax.jit
def pallas_sequential_preLN__linear_kernel_hedgehog__moe_arch_mod__prompt_kernel(
    A_x: jax.Array,
    A_wqkv: jax.Array,
    A_w_phi: jax.Array,
    A_wo: jax.Array,
    B_x: jax.Array,
    B_w_r: jax.Array,
    B_w_gate: jax.Array,
    B_w_up: jax.Array,
    B_w_down: jax.Array,
):
    del B_x
    hbm = pl.BlockSpec(memory_space=pl.ANY)
    out = pl.pallas_call(
        _kernel,
        out_shape=jax.ShapeDtypeStruct((S, D), BF16),
        in_specs=[hbm] * 8,
        out_specs=hbm,
        scratch_shapes=[
            pltpu.VMEM((S, D), BF16),
            pltpu.VMEM((S // 2, D), U32),
            pltpu.VMEM((3 * NC, D, RC), BF16),
            [pltpu.VMEM((D // 2, D), U32)] * 3,
            pltpu.VMEM((H, DH, DH), BF16),
            pltpu.VMEM((8 * 64, 128), U32),
            pltpu.VMEM((D, D), BF16),
            pltpu.VMEM((D // 2, D), U32),
            pltpu.VMEM((D,), BF16),
            pltpu.VMEM((8, D), F32),
            pltpu.VMEM((NPAIR, 64, 128), F32),
            pltpu.VMEM((NPAIR * 32, 128), U32),
            pltpu.VMEM((NPAIR, 128, T), F32),
            pltpu.VMEM((NPAIR, 128, 128), F32),
            [pltpu.VMEM((NPAIR * 64, T), U32)] * 2,
            pltpu.VMEM((TH, D), F32),
            pltpu.VMEM((TH, D), F32),
            pltpu.VMEM((S // 2, D), U32),
            pltpu.VMEM((S, D), BF16),
            pltpu.VMEM((D, FF), BF16),
            pltpu.VMEM((D, FF), BF16),
            pltpu.VMEM((FF, D + WD_PAD), BF16),
            pltpu.VMEM((D // 2, FM), U32),
            pltpu.VMEM((D // 2, FM), U32),
            pltpu.VMEM((FM // 2, D), U32),
            pltpu.VMEM((16, D), BF16),
            pltpu.SemaphoreType.DMA((5 + 3 * NC + NT_ + 8,)),
        ],
        compiler_params=pltpu.CompilerParams(vmem_limit_bytes=100 * 1024 * 1024,
                                             disable_semaphore_checks=True, disable_bounds_checks=True),
        name="hedgehog_mod",
    )(
        A_x.reshape(S, D),
        A_wqkv,
        A_w_phi,
        A_wo,
        B_w_r,
        B_w_gate,
        B_w_up,
        B_w_down,
    )
    return out.reshape(1, S, D)
```

```python
import math

import jax
import jax.numpy as jnp
from jax import lax
import jax.experimental.pallas as pl
import jax.experimental.pallas.tpu as pltpu

F32 = jnp.float32
BF16 = jnp.bfloat16
U32 = jnp.uint32

S = 2048
D = 1024
H = 32
DH = 32
FF = 3584
NPAIR = H // 2
LOG2E = 1.4426950408889634
LN_EPS = 1e-5

T = 256
TH = T // 2
NT_ = S // T
RC = 256
NC = D // RC
PPC = RC // 64
LNC = 16
WD_PAD = 128

LN1_PLAN = tuple((k * 12 // 16, k * 12 // 16 + 3) for k in range(16))
LN2B_PLAN = ((None, 0), (None, 0), (None, 0), (1, 6), (3, 8), (5, 10), (7, 12), (9, 14))
LN2A_PLAN = ((None, 18), (None, 18), (16, 19), (17, 20), (18, 21), (19, 22), (20, 23), (21, None))
PRO_LN1_PLAN = tuple((None, None) for k in range(16))
WO_ROWS = 352
WO_PLAN = tuple((k + 1, None) for k in range(11))
Z_PLAN = tuple((1 + k * 12 // 16, 1 + k * 12 // 16 + 3) for k in range(16))
UNROLL2 = 2
FV = 8 * 128
FM = FF - FV
PACK_PLAN = tuple((r, None) for r in [x - f for f in (0, 0.9, 0.45) for x in range(100, 116)] + [1, 3, 5, 13])
MOE_NA = 38
MOE_ND = 2
QUARTERS = True
G3_AT = 4

NN = (((1,), (0,)), ((), ()))
NT = (((1,), (1,)), ((), ()))


def _dot(a, b, dims):
    return lax.dot_general(a, b, dims, preferred_element_type=F32)


def _recip(x):
    return pl.reciprocal(x, approx=False, full_range=False)


def _pack(x):
    return pltpu.bitcast(x, U32)


def _unpack(x):
    return pltpu.bitcast(x, BF16)


def _pair_allreduce(a, op):
    a = op(a, pltpu.roll(a, 2, 0))
    return op(a, pltpu.roll(a, 4, 0))


def _tree(op, xs):
    xs = list(xs)
    while len(xs) > 1:
        nxt = [op(xs[i], xs[i + 1]) for i in range(0, len(xs) - 1, 2)]
        if len(xs) % 2:
            nxt.append(xs[-1])
        xs = nxt
    return xs[0]


def _dual_exp(p):
    sl = [p[8 * i:8 * i + 8, :] for i in range(8)]
    mx = _pair_allreduce(_tree(jnp.maximum, sl), jnp.maximum)
    mn = _pair_allreduce(_tree(jnp.minimum, sl), jnp.minimum)
    ep = [jnp.exp2(s - mx) for s in sl]
    en = [jnp.exp2(mn - s) for s in sl]
    sp = _pair_allreduce(_tree(jnp.add, ep), jnp.add)
    sn = _pair_allreduce(_tree(jnp.add, en), jnp.add)
    return ep, en, sp, sn


def _after(x, never, anchor):
    if anchor is None:
        return x
    d = jnp.concatenate([anchor] * (x.shape[0] // 8), axis=0)
    if x.shape[1] == 128:
        return jnp.where(never, d, x)
    return jnp.concatenate([jnp.where(never, d, x[:, :128]), x[:, 128:]], axis=1)


def _gate(x, never, deps):
    for i, dep in enumerate(deps):
        d = jnp.broadcast_to(dep, (8, 128))
        if x.dtype != F32:
            d = pltpu.bitcast(d, x.dtype)
        blk = jnp.where(never, d, x[8 * i:8 * i + 8, :128])
        if x.shape[1] > 128:
            blk = jnp.concatenate([blk, x[8 * i:8 * i + 8, 128:]], axis=1)
        parts = ([x[:8 * i, :]] if i else []) + [blk, x[8 * i + 8:, :]]
        x = jnp.concatenate(parts, axis=0)
    return x


def _lane_fold(a):
    return _tree(jnp.add, [a[:, 128 * i:128 * i + 128] for i in range(a.shape[1] // 128)])


def _row_sum(a):
    return jnp.sum(_lane_fold(a), axis=-1, keepdims=True)


def _lane_tile(a, n):
    return a if n == 1 else jnp.concatenate([a] * n, axis=1)


def _sublane_allreduce(a):
    a = a + pltpu.roll(a, 4, 0)
    a = a + pltpu.roll(a, 2, 0)
    return a + pltpu.roll(a, 1, 0)


def _col_broadcast(row8):
    return jnp.concatenate([row8] * 16, axis=0).astype(BF16).T.astype(F32)


def _vpu_matvec(xb, w_rows, never, anchors, lag):
    ng = xb.shape[0] // 8
    acc, hist = None, []
    for g in range(ng):
        dep = anchors[(g * len(anchors)) // ng]
        if g >= lag:
            dep = dep + hist[g - lag]
        x = jnp.where(never, dep, xb[8 * g:8 * g + 8, :])
        w = w_rows(g)
        t = w * _lane_tile(x, w.shape[1] // 128)
        acc = t if acc is None else acc + t
        hist.append(acc[:, -128:])
    return acc


class _Side:
    def __init__(self, never):
        self.never = never
        self.jobs = []
        self.deps = {}

    def add(self, plan, fn):
        for k, (rel, due) in enumerate(plan):
            if rel is None:
                self._run(due, fn, k, None)
            else:
                self.jobs.append((rel, due, fn, k))

    def _run(self, due, fn, k, anchor):
        dep = fn(k, anchor)
        if due is not None:
            self.deps.setdefault(due, []).append(dep)

    def gate(self, step, x):
        return _gate(x, self.never, self.deps.pop(step, []))

    def done(self, step, res):
        m = res.shape[0] // 8
        for job in sorted([j for j in self.jobs if step - 1 < j[0] <= step], key=lambda j: j[0]):
            self.jobs.remove(job)
            g = m - 1 - int((step - job[0]) * m)
            self._run(job[1], job[2], job[3], res[8 * g:8 * g + 8, res.shape[1] - 128:])


def _kernel(x_hbm, wqkv_hbm, wphi_hbm, wo_hbm, wr_hbm, wg_hbm, wu_hbm, wd_hbm, out_hbm,
            x_v, xn_v, wraw_v, wt_v, wphi_v, a_v, woraw_v, wo_v, wrraw_v, wr_v, kvacc_v, kvbf_v,
            z_v, zb_v, phi_v, ha_v, hb_v, hn_v, o_v, wg_v, wu_v, wd_v, wgp_v, wup_v, wdp_v, patch_v,
            sem):
    SX, SW, SO, SM = 0, 5, 5 + 3 * NC, 5 + 3 * NC + NT_ + 1

    def x_copy(i):
        t0, t1 = ((0, 1), (1, 2), (2, 3), (3, 5), (5, NT_))[i]
        rows = pl.ds(t0 * T, (t1 - t0) * T)
        return pltpu.make_async_copy(x_hbm.at[rows, :], x_v.at[rows, :], sem.at[SX + i])

    def w_copy(j, c):
        return pltpu.make_async_copy(wqkv_hbm.at[:, pl.ds(j * D + c * RC, RC)], wraw_v.at[j * NC + c],
                                     sem.at[SW + j * NC + c])

    wphi_copy = pltpu.make_async_copy(wphi_hbm, wphi_v, sem.at[SM + 4])
    wr_copy = pltpu.make_async_copy(wr_hbm, wrraw_v, sem.at[SM + 5])
    wo_copy = pltpu.make_async_copy(wo_hbm, woraw_v, sem.at[SM + 6])
    wg_copy = pltpu.make_async_copy(wg_hbm, wg_v, sem.at[SM + 0])
    wu_copy = pltpu.make_async_copy(wu_hbm, wu_v, sem.at[SM + 1])
    wd_copy = pltpu.make_async_copy(wd_hbm, wd_v.at[:, pl.ds(0, D)], sem.at[SM + 2])

    wphi_copy.start()
    x_copy(0).start()
    w_copy(1, 0).start()
    w_copy(1, 1).start()
    x_copy(1).start()
    w_copy(1, 2).start()

    def view(ref, i, n, off=0):
        r0 = off + i * n
        return ref.at[pl.ds(r0 if isinstance(r0, int) else pl.multiple_of(r0, math.gcd(n, off)), n), :]

    def ln_rows(t, k, n, never=None, anchor=None):
        x = _after(view(x_v, t, T)[k * n:(k + 1) * n, :].astype(F32), never, anchor)
        xc = x - _row_sum(x) * (1.0 / D)
        rstd = lax.rsqrt(_row_sum(xc * xc) * (1.0 / D) + LN_EPS)
        view(xn_v, t, T // 2)[k * n // 2:(k + 1) * n // 2, :] = _pack((xc * rstd).astype(BF16))
        return _tree(jnp.add, [rstd[8 * i:8 * i + 8, :] for i in range(min(n, LNC) // 8)])

    def xn_tile(t):
        return _unpack(view(xn_v, t, T // 2)[...])

    wphi_copy.wait()
    x_copy(0).wait()
    w_copy(1, 3).start()
    for c in range(NC):
        w_copy(2, c).start()
    x_copy(2).start()

    row = lax.broadcasted_iota(jnp.int32, (128, DH), 0)
    col = lax.broadcasted_iota(jnp.int32, (128, DH), 1)
    expand = jnp.where(((row & 63) >> 1) == col, 1.0, 0.0).astype(BF16)
    a_all = _dot(expand, wphi_v[...].reshape(H * DH, DH), NT)
    row = lax.broadcasted_iota(jnp.int32, (128, 128), 0)
    col = lax.broadcasted_iota(jnp.int32, (128, 128), 1)
    a_keep = (2 * (row >> 6) + (row & 1)) == (col >> 5)
    for g in range(8):
        a_v[64 * g:64 * g + 64, :] = _pack(jnp.where(a_keep, a_all[:, g * 128:(g + 1) * 128], 0.0).astype(BF16))
    never0 = ln_rows(0, 0, T)[0, 0] < 0.0
    hb_v[...] = jnp.zeros((TH, D), F32)

    def fold(j, c, side=None, step0=None):
        out = []
        for s in range(RC // 128):
            g = c * (RC // 128) + s
            w = wraw_v[j * NC + c, :, s * 128:(s + 1) * 128]
            g0 = 64 * g if isinstance(g, int) else pl.multiple_of(64 * g, 64)
            if j == 2:
                wt = w.T
            else:
                res = _dot(_unpack(a_v[pl.ds(g0, 64), :]), w, NT)
                if side is not None:
                    side.done(step0 + s, res)
                wt = (res * LOG2E).astype(BF16)
                out.append(res)
            wt_v[j][pl.ds(g0, 64), :] = _pack(wt)
        return out

    def wt_rows(j, c):
        return wt_v[j][c * RC // 2:(c + 1) * RC // 2, :]

    def k_features(pk, slot, c, first, ties=None):
        for j in range(PPC):
            pr = c * PPC + j
            p = pk[64 * j:64 * j + 64, :]
            if ties is not None:
                d = jnp.concatenate(ties[1][2 * j:2 * j + 2], axis=1)
                p = jnp.concatenate([jnp.where(ties[0], d, p[0:8, :]), p[8:, :]], axis=0)
            ep, en, sp, sn = _dual_exp(p)
            inv = _recip(sp * sn)
            rp = sn * inv
            rn = sp * inv
            phi = jnp.concatenate([e * rp for e in ep] + [e * rn for e in en], axis=0)
            z_v[pr] = phi if first else z_v[pr] + phi
            phi_v[slot][64 * pr:64 * pr + 64, :] = _pack(phi.astype(BF16))

    row = lax.broadcasted_iota(jnp.int32, (64, 128), 0)
    col = lax.broadcasted_iota(jnp.int32, (64, 128), 1)
    kv_keep = (row >> 5) == (col & 1)

    def kv_update(vt, slot, c, first, publish=False):
        for j in range(PPC):
            pr = c * PPC + j
            upd = _dot(vt[64 * j:64 * j + 64, :].astype(BF16), _unpack(phi_v[slot][64 * pr:64 * pr + 64, :]), NT)
            acc = upd if first else kvacc_v[pr] + upd
            kvacc_v[pr] = acc
            if publish:
                kvbf_v[32 * pr:32 * pr + 32, :] = _pack(jnp.where(kv_keep, acc, 0.0).astype(BF16))

    def proj(j, c, xn):
        if QUARTERS:
            return proj_steps(_Side(None), 0, j, c, xn)
        return _dot(_unpack(wt_rows(j, c)), xn, NT)

    def proj_steps(side, step0, j, c, xn):
        w = wt_rows(j, c)
        quarters = []
        for n in range(2):
            for m in range(2):
                step = step0 + 2 * n + m
                wq = side.gate(step, w[m * (RC // 4):(m + 1) * (RC // 4), :])
                res = _dot(_unpack(wq), xn[n * TH:(n + 1) * TH, :], NT)
                side.done(step, res)
                quarters.append(res)
        return jnp.concatenate(
            [jnp.concatenate([quarters[0], quarters[2]], axis=1),
             jnp.concatenate([quarters[1], quarters[3]], axis=1)], axis=0)

    def spots(res, n):
        m, w = res.shape
        allp = [res[r:r + 8, c:c + 128] for c in range(0, w, 128) for r in range(56, m, 64)]
        return [allp[(i * len(allp)) // n] for i in range(n)]

    def pack_rows(src, dst, r0, rows, c0, cols, never, a):
        w = _pack(src[r0:r0 + rows, c0:c0 + cols])
        d = jnp.concatenate([_lane_tile(pltpu.bitcast(a, U32), cols // 128)] * (rows // 16), axis=0)
        dst[r0 // 2:(r0 + rows) // 2, c0:c0 + cols] = jnp.where(never, d, w)

    def stash(i, val):
        for q in range(4):
            zb_v[4 * i + q] = val[128 * (q // 2):128 * (q // 2) + 128, 128 * (q % 2):128 * (q % 2) + 128]

    def unstash(i):
        return jnp.concatenate(
            [jnp.concatenate([zb_v[4 * i + 2 * r], zb_v[4 * i + 2 * r + 1]], axis=1) for r in range(2)], axis=0)

    w_copy(1, 0).wait()
    for c in range(NC):
        w_copy(0, c).start()
    x_copy(3).start()
    fold(1, 0)
    stash(0, proj(1, 0, xn_tile(0)))

    w_copy(1, 1).wait()
    wo_copy.start()
    wr_copy.start()
    x_copy(4).start()
    f = fold(1, 1)
    pk = proj(1, 1, xn_tile(0))
    stash(1, pk)
    k_features(unstash(0), 0, 0, True, (never0, spots(f[0], 2) + spots(f[1], 2) + spots(pk, 8)[:4]))

    x_copy(1).wait()
    w_copy(1, 2).wait()
    wg_copy.start()
    wu_copy.start()
    wd_copy.start()
    side = _Side(never0)
    side.add(PRO_LN1_PLAN, lambda k, a: ln_rows(1, k, LNC, never0, a))
    fold(1, 2, side, 0)
    stash(2, proj_steps(side, 2, 1, 2, xn_tile(0)))
    xn1 = xn_tile(1)
    k_features(proj(1, 0, xn1), 1, 0, False)
    k_features(proj(1, 1, xn1), 1, 1, True)
    stash(3, proj(1, 2, xn1))

    w_copy(1, 3).wait()
    for c in range(3):
        w_copy(2, c).wait()
    fold(1, 3)
    xn0, xn1 = xn_tile(0), xn_tile(1)
    k_features(proj(1, 3, xn0), 0, 3, True)
    k_features(proj(1, 3, xn1), 1, 3, False)
    for c in range(3):
        fold(2, c)
    vt00 = proj(2, 0, xn0)
    k_features(unstash(1), 0, 1, False, (never0, spots(vt00, 2 * PPC)))
    vt10 = proj(2, 0, xn1)
    k_features(unstash(2), 0, 2, True, (never0, spots(vt10, 2 * PPC)))
    kv_update(vt00, 0, 0, True)
    vt01 = proj(2, 1, xn0)
    k_features(unstash(3), 1, 2, False, (never0, spots(vt01, 2 * PPC)))
    kv_update(vt10, 1, 0, False)
    stash(0, proj(2, 1, xn1))
    kv_update(vt01, 0, 1, True)

    w_copy(2, 3).wait()
    x_copy(2).wait()
    w_copy(0, 0).wait()
    side = _Side(never0)
    side.add(LN1_PLAN, lambda k, a: ln_rows(2, k, LNC, never0, a))
    fold(0, 0, side, -1)
    fold(2, 3)
    kv_update(unstash(0), 1, 1, False)
    xn0, xn1 = xn_tile(0), xn_tile(1)
    vt02 = proj_steps(side, 1, 2, 2, xn0)
    vt12 = proj_steps(side, 5, 2, 2, xn1)
    kv_update(vt02, 0, 2, True)
    vt03 = proj_steps(side, 9, 2, 3, xn0)
    kv_update(vt12, 1, 2, False)
    vt13 = proj_steps(side, 13, 2, 3, xn1)
    kv_update(vt03, 0, 3, True)
    kv_update(vt13, 1, 3, False)

    def phase1(u, carry):
        never = u < 0

        @pl.when(u == 0)
        def _():
            for c in range(1, NC):
                w_copy(0, c).wait()
            x_copy(3).wait()
            wo_copy.wait()
            wr_copy.wait()

        @pl.when(u == 1)
        def _():
            x_copy(4).wait()

        pending = None
        for i in range(2):
            t = 2 * u + 2 + i
            tn = jnp.minimum(t + 1, NT_ - 1)
            side = _Side(never)
            xn = xn_tile(t)
            for c in range(NC):
                pk = proj(1, c, xn)
                if c == 0 and pending is not None:
                    kv_update(*pending)
                k_features(pk, i, c, False)
            side.add(LN1_PLAN, lambda k, a: ln_rows(tn, k, LNC, never, a))
            if i == 0:
                def pack_wo(k, a):
                    rows = WO_ROWS // len(WO_PLAN)
                    w0 = u * ((D - WO_ROWS) // 2)
                    src = woraw_v.at[pl.ds(pl.multiple_of(w0, 16), WO_ROWS), :]
                    dst = wo_v.at[pl.ds(pl.multiple_of(w0 // 2, 8), WO_ROWS // 2), :]
                    pack_rows(src, dst, k * rows, rows, 0, D, never, a)
                side.add(WO_PLAN, pack_wo)
            else:
                def z_final(k, a):
                    z = _after(z_v[k], never, a)
                    zs = _row_sum(z)
                    zb_v[k] = jnp.broadcast_to(zs, (128, 128))
                    return zs[120:128, :]
                side.add(Z_PLAN, z_final)
            side.done(0, pk)
            vts = []
            for c in range(NC):
                vts.append(proj_steps(side, 4 * c + 1, 2, c, xn))
                if c > 0:
                    kv_update(vts[c - 1], i, c - 1, False, i == 1)
            pending = (vts[NC - 1], i, NC - 1, False, i == 1)
        fold(0, u + 1)
        kv_update(*pending)
        wr_v[...] = jnp.broadcast_to(wrraw_v[...].reshape(1, D).astype(F32), (8, D))
        return carry

    lax.fori_loop(0, (NT_ - 2) // 2, phase1, 0)

    def o_copy(r0, n, i):
        return pltpu.make_async_copy(o_v.at[pl.ds(r0, n), :], out_hbm.at[pl.ds(r0, n), :], sem.at[SO + i])

    def finish_rows(h_ref, k, ht, valid, st, never=None, anchor=None):
        r0 = ht * TH + k * LNC
        best, besti = st["route"]
        wr = jnp.concatenate([wr_v[...]] * (LNC // 8), axis=0)
        sub = lax.broadcasted_iota(jnp.int32, (8, 1), 0)
        h = _after(h_ref[k * LNC:(k + 1) * LNC, :], never, anchor)
        m = _row_sum(h) * (1.0 / D)
        hc = h - m
        rstd = lax.rsqrt(_row_sum(hc * hc) * (1.0 / D) + LN_EPS)
        r = (_row_sum(hc * wr) * rstd).astype(BF16).astype(F32)
        hn = hc * rstd
        view(hn_v, ht, TH // 2)[k * LNC // 2:(k + 1) * LNC // 2, :] = _pack(hn.astype(BF16))
        view(o_v, ht, TH)[k * LNC:(k + 1) * LNC, :] = (hn + h).astype(BF16)
        if valid is not None:
            r = jnp.where(valid, r, -jnp.inf)
        for i in range(LNC // 8):
            ri = r[8 * i:8 * i + 8, :]
            better = ri > best
            best = jnp.where(better, ri, best)
            besti = jnp.where(better, sub + (r0 + 8 * i), besti)
        st["route"] = (best, besti)
        return best

    def q_features(pq, slot, c):
        for j in range(PPC):
            pr = c * PPC + j
            ep, en, sp, sn = _dual_exp(pq[64 * j:64 * j + 64, :])
            zz = [_lane_tile(zb_v[pr, 8 * i:8 * i + 8, :], pq.shape[1] // 128) for i in range(16)]
            ap = _pair_allreduce(_tree(jnp.add, [ep[i] * zz[i] for i in range(8)]), jnp.add)
            an = _pair_allreduce(_tree(jnp.add, [en[i] * zz[8 + i] for i in range(8)]), jnp.add)
            inv = _recip(ap * sn + (an + 1e-6 * sn) * sp)
            rp = sn * inv
            rn = sp * inv
            phi = jnp.concatenate([e * rp for e in ep] + [e * rn for e in en], axis=0)
            phi_v[slot][64 * pr:64 * pr + 64, :] = _pack(phi.astype(BF16))

    def attn_rows(slot, c, lo, hi):
        res = jnp.concatenate(
            [_dot(_unpack(kvbf_v[32 * pr:32 * pr + 32, :]), _unpack(phi_v[slot][64 * pr:64 * pr + 64, lo:hi]), NN)
             for pr in range(c * PPC, (c + 1) * PPC)], axis=0)
        return res.astype(BF16).T

    def out_proj(side, step0, o, k0, k1, n0=0, n1=D // 128):
        cols = []
        for n in range(n0, n1):
            w = side.gate(step0 + n, wo_v[k0 // 2:k1 // 2, n * 128:(n + 1) * 128])
            res = _dot(o, _unpack(w), NN)
            side.done(step0 + n, res)
            cols.append(res)
        return jnp.concatenate(cols, axis=1)

    def phase2(u, carry):
        for i in range(UNROLL2):
            carry = phase2_tile(u * UNROLL2 + i, i % 2, carry, u < 0)

        r0 = pl.multiple_of(u * (UNROLL2 * T), T)

        @pl.when(u == 0)
        def _():
            o_copy(0, UNROLL2 * T - TH, 0).start()

        @pl.when(u > 0)
        def _():
            o_copy(pl.multiple_of(jnp.maximum(r0 - TH, 0), TH), UNROLL2 * T, u).start()

        return carry

    def phase2_tile(t, slot, carry, never):
        hp = jnp.maximum(2 * t - 1, 0)
        side = _Side(never)
        st = {"route": carry}
        side.add(LN2B_PLAN, lambda k, a: finish_rows(hb_v, k, hp, t > 0, st, side.never, a))

        def pack_ffn(k, a):
            if k < 32:
                n = D // NT_
                pack_rows(view((wg_v, wu_v)[k % 2], t, n), view((wgp_v, wup_v)[k % 2], t, n // 2),
                          (k // 4) * 16, 16, (k // 2 % 2) * (FM // 2), FM // 2, never, a)
            else:
                n = FM // NT_
                pack_rows(view(wd_v, t, n, FV), view(wdp_v, t, n // 2), (k - 32) * 16, 16, 0, D, never, a)
        side.add(PACK_PLAN, pack_ffn)

        xn = xn_tile(t)
        xt = view(x_v, t, T)
        os_ = []
        for c in range(NC):
            pq = proj_steps(side, 100 + 4 * c, 0, c, xn)
            if c == 0:
                pq = side.gate(0, pq)
            q_features(pq, slot, c)
            if c > 0:
                os_.append(attn_rows(slot, c - 1, 0, T))
        oa = jnp.concatenate([o[0:TH, :] for o in os_[:2]], axis=1)
        ha0 = out_proj(side, 0, oa, 0, D // 2, 0, G3_AT)
        os_.append(attn_rows(slot, NC - 1, 0, T))
        ha1 = out_proj(side, 0, oa, 0, D // 2, G3_AT, D // 128)
        ha = jnp.concatenate([ha0, ha1], axis=1) + xt[0:TH, :].astype(F32)
        ha_v[...] = ha + out_proj(side, 8, jnp.concatenate([o[0:TH, :] for o in os_[2:]], axis=1), D // 2, D)
        side.add(LN2A_PLAN, lambda k, a: finish_rows(ha_v, k, 2 * t, None, st, side.never, a))
        ob = jnp.concatenate([o[TH:T, :] for o in os_], axis=1)
        hb_v[...] = xt[TH:T, :].astype(F32) + out_proj(side, 16, ob, 0, D)
        return st["route"]

    wg_copy.wait()
    wu_copy.wait()
    wd_copy.wait()
    route = lax.fori_loop(
        0, NT_ // UNROLL2, phase2,
        (jnp.full((8, 1), -jnp.inf, F32), jnp.zeros((8, 1), jnp.int32)))
    st = {"route": route}
    for k in range(TH // LNC):
        finish_rows(hb_v, k, 2 * NT_ - 1, None, st)
    best, besti = st["route"]
    o_copy(S - TH, TH, NT_).start()

    rmax = jnp.max(best, axis=0, keepdims=True)
    idx = jnp.min(jnp.where(best == rmax, besti, S), axis=0, keepdims=True)
    idx_s = jnp.clip(idx[0, 0], 0, S - 1)
    blk = pl.multiple_of((idx_s >> 4) << 4, 16)
    pair = jnp.broadcast_to(hn_v[pl.ds(idx_s >> 1, 1), :], (8, D))
    x8 = pltpu.bitcast(jnp.where((idx_s & 1) == 1, pair & jnp.uint32(0xFFFF0000), pair << 16), F32)
    xs = jnp.concatenate([x8, x8], axis=0).astype(BF16)
    acts, anchors = [], []
    for c0 in range(0, FM, 128):
        g = _dot(xs, _unpack(wgp_v[:, c0:c0 + 128]), NN)[0:8, :]
        u = _dot(xs, _unpack(wup_v[:, c0:c0 + 128]), NN)[0:8, :]
        anchors += [g, u]
        acts.append(g * jax.nn.sigmoid(g) * u)
    gu = _sublane_allreduce(_vpu_matvec(
        _col_broadcast(x8),
        lambda g: jnp.concatenate([w[8 * g:8 * g + 8, FM:FF].astype(F32) for w in (wg_v, wu_v)], axis=1),
        never0, anchors[:MOE_NA], 1))
    g, u = gu[:, :FV], gu[:, FV:]
    acts.append(g * jax.nn.sigmoid(g) * u)
    a = jnp.concatenate(acts, axis=1)
    am = jnp.concatenate([a[:, FV:], a[:, FV:]], axis=0).astype(BF16)
    ys, anchors = [], anchors[MOE_NA:]
    for k0 in range(0, FM, 512):
        yk = _dot(am[:, k0:k0 + 512], _unpack(wdp_v[k0 // 2:k0 // 2 + 256, :]), NN)[0:8, :]
        ys.append(yk)
        anchors += [yk[:, c:c + 128] for c in range(128, D, 256)]
    ys.append(_sublane_allreduce(_vpu_matvec(
        _col_broadcast(a[:, :FV]), lambda g: wd_v[8 * g:8 * g + 8, 0:D].astype(F32), never0, anchors[:-MOE_ND], 2)))
    y = _tree(jnp.add, ys) * jax.nn.sigmoid(rmax)
    y = jnp.concatenate([y, y], axis=0)
    sel = lax.broadcasted_iota(jnp.int32, (16, 1), 0) == (idx_s - blk)
    patch_v[...] = (o_v[pl.ds(blk, 16), :].astype(F32) + jnp.where(sel, y, 0.0)).astype(BF16)
    o_copy(0, UNROLL2 * T - TH, 0).wait()
    for u in range(1, NT_ // UNROLL2):
        o_copy(u * UNROLL2 * T - TH, UNROLL2 * T, u).wait()
    o_copy(S - TH, TH, NT_).wait()
    pc = pltpu.make_async_copy(patch_v, out_hbm.at[pl.ds(blk, 16), :], sem.at[SM + 3])
    pc.start()
    pc.wait()


@jax.jit
def pallas_sequential_preLN__linear_kernel_hedgehog__moe_arch_mod__prompt_kernel(
    A_x: jax.Array,
    A_wqkv: jax.Array,
    A_w_phi: jax.Array,
    A_wo: jax.Array,
    B_x: jax.Array,
    B_w_r: jax.Array,
    B_w_gate: jax.Array,
    B_w_up: jax.Array,
    B_w_down: jax.Array,
):
    del B_x
    hbm = pl.BlockSpec(memory_space=pl.ANY)
    out = pl.pallas_call(
        _kernel,
        out_shape=jax.ShapeDtypeStruct((S, D), BF16),
        in_specs=[hbm] * 8,
        out_specs=hbm,
        scratch_shapes=[
            pltpu.VMEM((S, D), BF16),
            pltpu.VMEM((S // 2, D), U32),
            pltpu.VMEM((3 * NC, D, RC), BF16),
            [pltpu.VMEM((D // 2, D), U32)] * 3,
            pltpu.VMEM((H, DH, DH), BF16),
            pltpu.VMEM((8 * 64, 128), U32),
            pltpu.VMEM((D, D), BF16),
            pltpu.VMEM((D // 2, D), U32),
            pltpu.VMEM((D,), BF16),
            pltpu.VMEM((8, D), F32),
            pltpu.VMEM((NPAIR, 64, 128), F32),
            pltpu.VMEM((NPAIR * 32, 128), U32),
            pltpu.VMEM((NPAIR, 128, T), F32),
            pltpu.VMEM((NPAIR, 128, 128), F32),
            [pltpu.VMEM((NPAIR * 64, T), U32)] * 2,
            pltpu.VMEM((TH, D), F32),
            pltpu.VMEM((TH, D), F32),
            pltpu.VMEM((S // 2, D), U32),
            pltpu.VMEM((S, D), BF16),
            pltpu.VMEM((D, FF), BF16),
            pltpu.VMEM((D, FF), BF16),
            pltpu.VMEM((FF, D + WD_PAD), BF16),
            pltpu.VMEM((D // 2, FM), U32),
            pltpu.VMEM((D // 2, FM), U32),
            pltpu.VMEM((FM // 2, D), U32),
            pltpu.VMEM((16, D), BF16),
            pltpu.SemaphoreType.DMA((5 + 3 * NC + NT_ + 8,)),
        ],
        compiler_params=pltpu.CompilerParams(vmem_limit_bytes=100 * 1024 * 1024,
                                             disable_semaphore_checks=True, disable_bounds_checks=True),
        name="hedgehog_mod",
    )(
        A_x.reshape(S, D),
        A_wqkv,
        A_w_phi,
        A_wo,
        B_w_r,
        B_w_gate,
        B_w_up,
        B_w_down,
    )
    return out.reshape(1, S, D)
```

```python
import math

import jax
import jax.numpy as jnp
from jax import lax
import jax.experimental.pallas as pl
import jax.experimental.pallas.tpu as pltpu

F32 = jnp.float32
BF16 = jnp.bfloat16
U32 = jnp.uint32

S = 2048
D = 1024
H = 32
DH = 32
FF = 3584
NPAIR = H // 2
LOG2E = 1.4426950408889634
LN_EPS = 1e-5

T = 256
TH = T // 2
NT_ = S // T
RC = 256
NC = D // RC
PPC = RC // 64
LNC = 16
WD_PAD = 128

LN1_PLAN = tuple((round(13 * k / 15, 3), math.ceil(round(13 * k / 15, 3)) + 3) for k in range(16))
LN2B_PLAN = ((None, 0), (None, 0), (None, 0), (2.0, 7), (3.5, 9), (5.0, 10), (6.5, 12), (8.0, 13))
LN2A_PLAN = ((None, 18), (16, 19), (16, 19), (17, 20), (18, 21), (19, 22), (20, 23), (20, 23))
PRO_LN1_PLAN = tuple((None, None) for k in range(16))
WO_ROWS = 352
WO_PLAN = tuple((6 + k / 2, None) for k in range(11))
Z_PLAN = tuple((round(4 + 8 * k / 15, 3), math.ceil(round(4 + 8 * k / 15, 3)) + 2) for k in range(16))
UNROLL2 = 2
FV = 8 * 128
FM = FF - FV
PACK_PLAN = tuple((r, None) for r in [x - f for f in (0, 0.9) for x in range(100, 116)] + [round(21 * k / 19, 3) for k in range(20)])
MOE_NA = 38
MOE_ND = 2
QUARTERS = True
G3_AT = 5

NN = (((1,), (0,)), ((), ()))
NT = (((1,), (1,)), ((), ()))


def _dot(a, b, dims):
    return lax.dot_general(a, b, dims, preferred_element_type=F32)


def _recip(x):
    return pl.reciprocal(x, approx=False, full_range=False)


def _pack(x):
    return pltpu.bitcast(x, U32)


def _unpack(x):
    return pltpu.bitcast(x, BF16)


def _pair_allreduce(a, op):
    a = op(a, pltpu.roll(a, 2, 0))
    return op(a, pltpu.roll(a, 4, 0))


def _tree(op, xs):
    xs = list(xs)
    while len(xs) > 1:
        nxt = [op(xs[i], xs[i + 1]) for i in range(0, len(xs) - 1, 2)]
        if len(xs) % 2:
            nxt.append(xs[-1])
        xs = nxt
    return xs[0]


def _dual_exp(p):
    sl = [p[8 * i:8 * i + 8, :] for i in range(8)]
    mx = _pair_allreduce(_tree(jnp.maximum, sl), jnp.maximum)
    mn = _pair_allreduce(_tree(jnp.minimum, sl), jnp.minimum)
    ep = [jnp.exp2(s - mx) for s in sl]
    en = [jnp.exp2(mn - s) for s in sl]
    sp = _pair_allreduce(_tree(jnp.add, ep), jnp.add)
    sn = _pair_allreduce(_tree(jnp.add, en), jnp.add)
    return ep, en, sp, sn


def _after(x, never, anchor):
    if anchor is None:
        return x
    d = jnp.concatenate([anchor] * (x.shape[0] // 8), axis=0)
    if x.shape[1] == 128:
        return jnp.where(never, d, x)
    return jnp.concatenate([jnp.where(never, d, x[:, :128]), x[:, 128:]], axis=1)


def _gate(x, never, deps):
    for i, dep in enumerate(deps):
        d = jnp.broadcast_to(dep, (8, 128))
        if x.dtype != F32:
            d = pltpu.bitcast(d, x.dtype)
        blk = jnp.where(never, d, x[8 * i:8 * i + 8, :128])
        if x.shape[1] > 128:
            blk = jnp.concatenate([blk, x[8 * i:8 * i + 8, 128:]], axis=1)
        parts = ([x[:8 * i, :]] if i else []) + [blk, x[8 * i + 8:, :]]
        x = jnp.concatenate(parts, axis=0)
    return x


def _lane_fold(a):
    return _tree(jnp.add, [a[:, 128 * i:128 * i + 128] for i in range(a.shape[1] // 128)])


def _row_sum(a):
    return jnp.sum(_lane_fold(a), axis=-1, keepdims=True)


def _lane_tile(a, n):
    return a if n == 1 else jnp.concatenate([a] * n, axis=1)


def _sublane_allreduce(a):
    a = a + pltpu.roll(a, 4, 0)
    a = a + pltpu.roll(a, 2, 0)
    return a + pltpu.roll(a, 1, 0)


def _col_broadcast(row8):
    return jnp.concatenate([row8] * 16, axis=0).astype(BF16).T.astype(F32)


def _vpu_matvec(xb, w_rows, never, anchors, lag):
    ng = xb.shape[0] // 8
    acc, hist = None, []
    for g in range(ng):
        dep = anchors[(g * len(anchors)) // ng]
        if g >= lag:
            dep = dep + hist[g - lag]
        x = jnp.where(never, dep, xb[8 * g:8 * g + 8, :])
        w = w_rows(g)
        t = w * _lane_tile(x, w.shape[1] // 128)
        acc = t if acc is None else acc + t
        hist.append(acc[:, -128:])
    return acc


class _Side:
    def __init__(self, never):
        self.never = never
        self.jobs = []
        self.deps = {}

    def add(self, plan, fn):
        for k, (rel, due) in enumerate(plan):
            if rel is None:
                self._run(due, fn, k, None)
            else:
                self.jobs.append((rel, due, fn, k))

    def _run(self, due, fn, k, anchor):
        dep = fn(k, anchor)
        if due is not None:
            self.deps.setdefault(due, []).append(dep)

    def gate(self, step, x):
        return _gate(x, self.never, self.deps.pop(step, []))

    def done(self, step, res):
        m = res.shape[0] // 8
        for job in sorted([j for j in self.jobs if step - 1 < j[0] <= step], key=lambda j: j[0]):
            self.jobs.remove(job)
            g = m - 1 - int((step - job[0]) * m)
            self._run(job[1], job[2], job[3], res[8 * g:8 * g + 8, res.shape[1] - 128:])


def _kernel(x_hbm, wqkv_hbm, wphi_hbm, wo_hbm, wr_hbm, wg_hbm, wu_hbm, wd_hbm, out_hbm,
            x_v, xn_v, wraw_v, wt_v, wphi_v, a_v, woraw_v, wo_v, wrraw_v, wr_v, kvacc_v, kvbf_v,
            z_v, zb_v, phi_v, ha_v, hb_v, hn_v, o_v, wg_v, wu_v, wd_v, wgp_v, wup_v, wdp_v, patch_v,
            sem):
    SX, SW, SO, SM = 0, 5, 5 + 3 * NC, 5 + 3 * NC + NT_ + 1

    def x_copy(i):
        t0, t1 = ((0, 1), (1, 2), (2, 3), (3, 5), (5, NT_))[i]
        rows = pl.ds(t0 * T, (t1 - t0) * T)
        return pltpu.make_async_copy(x_hbm.at[rows, :], x_v.at[rows, :], sem.at[SX + i])

    def w_copy(j, c):
        return pltpu.make_async_copy(wqkv_hbm.at[:, pl.ds(j * D + c * RC, RC)], wraw_v.at[j * NC + c],
                                     sem.at[SW + j * NC + c])

    wphi_copy = pltpu.make_async_copy(wphi_hbm, wphi_v, sem.at[SM + 4])
    wr_copy = pltpu.make_async_copy(wr_hbm, wrraw_v, sem.at[SM + 5])
    wo_copy = pltpu.make_async_copy(wo_hbm, woraw_v, sem.at[SM + 6])
    wg_copy = pltpu.make_async_copy(wg_hbm, wg_v, sem.at[SM + 0])
    wu_copy = pltpu.make_async_copy(wu_hbm, wu_v, sem.at[SM + 1])
    wd_copy = pltpu.make_async_copy(wd_hbm, wd_v.at[:, pl.ds(0, D)], sem.at[SM + 2])

    wphi_copy.start()
    x_copy(0).start()
    w_copy(1, 0).start()
    w_copy(1, 1).start()
    x_copy(1).start()
    w_copy(1, 2).start()

    def view(ref, i, n, off=0):
        r0 = off + i * n
        return ref.at[pl.ds(r0 if isinstance(r0, int) else pl.multiple_of(r0, math.gcd(n, off)), n), :]

    def ln_rows(t, k, n, never=None, anchor=None):
        x = _after(view(x_v, t, T)[k * n:(k + 1) * n, :].astype(F32), never, anchor)
        xc = x - _row_sum(x) * (1.0 / D)
        rstd = lax.rsqrt(_row_sum(xc * xc) * (1.0 / D) + LN_EPS)
        view(xn_v, t, T // 2)[k * n // 2:(k + 1) * n // 2, :] = _pack((xc * rstd).astype(BF16))
        return _tree(jnp.add, [rstd[8 * i:8 * i + 8, :] for i in range(min(n, LNC) // 8)])

    def xn_tile(t):
        return _unpack(view(xn_v, t, T // 2)[...])

    wphi_copy.wait()
    x_copy(0).wait()
    w_copy(1, 3).start()
    for c in range(NC):
        w_copy(2, c).start()
    x_copy(2).start()

    row = lax.broadcasted_iota(jnp.int32, (128, DH), 0)
    col = lax.broadcasted_iota(jnp.int32, (128, DH), 1)
    expand = jnp.where(((row & 63) >> 1) == col, 1.0, 0.0).astype(BF16)
    a_all = _dot(expand, wphi_v[...].reshape(H * DH, DH), NT)
    row = lax.broadcasted_iota(jnp.int32, (128, 128), 0)
    col = lax.broadcasted_iota(jnp.int32, (128, 128), 1)
    a_keep = (2 * (row >> 6) + (row & 1)) == (col >> 5)
    for g in range(8):
        a_v[64 * g:64 * g + 64, :] = _pack(jnp.where(a_keep, a_all[:, g * 128:(g + 1) * 128], 0.0).astype(BF16))
    never0 = ln_rows(0, 0, T)[0, 0] < 0.0
    hb_v[...] = jnp.zeros((TH, D), F32)

    def fold(j, c, side=None, step0=None):
        out = []
        for s in range(RC // 128):
            g = c * (RC // 128) + s
            w = wraw_v[j * NC + c, :, s * 128:(s + 1) * 128]
            g0 = 64 * g if isinstance(g, int) else pl.multiple_of(64 * g, 64)
            if j == 2:
                wt = w.T
            else:
                res = _dot(_unpack(a_v[pl.ds(g0, 64), :]), w, NT)
                if side is not None:
                    side.done(step0 + s, res)
                wt = (res * LOG2E).astype(BF16)
                out.append(res)
            wt_v[j][pl.ds(g0, 64), :] = _pack(wt)
        return out

    def wt_rows(j, c):
        return wt_v[j][c * RC // 2:(c + 1) * RC // 2, :]

    def k_features(pk, slot, c, first, ties=None):
        for j in range(PPC):
            pr = c * PPC + j
            p = pk[64 * j:64 * j + 64, :]
            if ties is not None:
                d = jnp.concatenate(ties[1][2 * j:2 * j + 2], axis=1)
                p = jnp.concatenate([jnp.where(ties[0], d, p[0:8, :]), p[8:, :]], axis=0)
            ep, en, sp, sn = _dual_exp(p)
            inv = _recip(sp * sn)
            rp = sn * inv
            rn = sp * inv
            phi = jnp.concatenate([e * rp for e in ep] + [e * rn for e in en], axis=0)
            z_v[pr] = phi if first else z_v[pr] + phi
            phi_v[slot][64 * pr:64 * pr + 64, :] = _pack(phi.astype(BF16))

    row = lax.broadcasted_iota(jnp.int32, (64, 128), 0)
    col = lax.broadcasted_iota(jnp.int32, (64, 128), 1)
    kv_keep = (row >> 5) == (col & 1)

    def kv_update(vt, slot, c, first, publish=False):
        for j in range(PPC):
            pr = c * PPC + j
            upd = _dot(vt[64 * j:64 * j + 64, :].astype(BF16), _unpack(phi_v[slot][64 * pr:64 * pr + 64, :]), NT)
            acc = upd if first else kvacc_v[pr] + upd
            kvacc_v[pr] = acc
            if publish:
                kvbf_v[32 * pr:32 * pr + 32, :] = _pack(jnp.where(kv_keep, acc, 0.0).astype(BF16))

    def proj(j, c, xn):
        if QUARTERS:
            return proj_steps(_Side(None), 0, j, c, xn)
        return _dot(_unpack(wt_rows(j, c)), xn, NT)

    def proj_steps(side, step0, j, c, xn):
        w = wt_rows(j, c)
        quarters = []
        for n in range(2):
            for m in range(2):
                step = step0 + 2 * n + m
                wq = side.gate(step, w[m * (RC // 4):(m + 1) * (RC // 4), :])
                res = _dot(_unpack(wq), xn[n * TH:(n + 1) * TH, :], NT)
                side.done(step, res)
                quarters.append(res)
        return jnp.concatenate(
            [jnp.concatenate([quarters[0], quarters[2]], axis=1),
             jnp.concatenate([quarters[1], quarters[3]], axis=1)], axis=0)

    def spots(res, n):
        m, w = res.shape
        allp = [res[r:r + 8, c:c + 128] for c in range(0, w, 128) for r in range(56, m, 64)]
        return [allp[(i * len(allp)) // n] for i in range(n)]

    def pack_rows(src, dst, r0, rows, c0, cols, never, a):
        w = _pack(src[r0:r0 + rows, c0:c0 + cols])
        d = jnp.concatenate([_lane_tile(pltpu.bitcast(a, U32), cols // 128)] * (rows // 16), axis=0)
        dst[r0 // 2:(r0 + rows) // 2, c0:c0 + cols] = jnp.where(never, d, w)

    def stash(i, val):
        for q in range(4):
            zb_v[4 * i + q] = val[128 * (q // 2):128 * (q // 2) + 128, 128 * (q % 2):128 * (q % 2) + 128]

    def unstash(i):
        return jnp.concatenate(
            [jnp.concatenate([zb_v[4 * i + 2 * r], zb_v[4 * i + 2 * r + 1]], axis=1) for r in range(2)], axis=0)

    w_copy(1, 0).wait()
    for c in range(NC):
        w_copy(0, c).start()
    x_copy(3).start()
    fold(1, 0)
    stash(0, proj(1, 0, xn_tile(0)))

    w_copy(1, 1).wait()
    wo_copy.start()
    wr_copy.start()
    x_copy(4).start()
    f = fold(1, 1)
    pk = proj(1, 1, xn_tile(0))
    stash(1, pk)
    k_features(unstash(0), 0, 0, True, (never0, spots(f[0], 2) + spots(f[1], 2) + spots(pk, 8)[:4]))

    x_copy(1).wait()
    w_copy(1, 2).wait()
    wg_copy.start()
    wu_copy.start()
    wd_copy.start()
    side = _Side(never0)
    side.add(PRO_LN1_PLAN, lambda k, a: ln_rows(1, k, LNC, never0, a))
    fold(1, 2, side, 0)
    stash(2, proj_steps(side, 2, 1, 2, xn_tile(0)))
    xn1 = xn_tile(1)
    k_features(proj(1, 0, xn1), 1, 0, False)
    k_features(proj(1, 1, xn1), 1, 1, True)
    stash(3, proj(1, 2, xn1))

    w_copy(1, 3).wait()
    for c in range(3):
        w_copy(2, c).wait()
    fold(1, 3)
    xn0, xn1 = xn_tile(0), xn_tile(1)
    k_features(proj(1, 3, xn0), 0, 3, True)
    k_features(proj(1, 3, xn1), 1, 3, False)
    for c in range(3):
        fold(2, c)
    vt00 = proj(2, 0, xn0)
    k_features(unstash(1), 0, 1, False, (never0, spots(vt00, 2 * PPC)))
    vt10 = proj(2, 0, xn1)
    k_features(unstash(2), 0, 2, True, (never0, spots(vt10, 2 * PPC)))
    kv_update(vt00, 0, 0, True)
    vt01 = proj(2, 1, xn0)
    k_features(unstash(3), 1, 2, False, (never0, spots(vt01, 2 * PPC)))
    kv_update(vt10, 1, 0, False)
    stash(0, proj(2, 1, xn1))
    kv_update(vt01, 0, 1, True)

    w_copy(2, 3).wait()
    x_copy(2).wait()
    w_copy(0, 0).wait()
    side = _Side(never0)
    side.add(LN1_PLAN, lambda k, a: ln_rows(2, k, LNC, never0, a))
    fold(0, 0, side, -1)
    fold(2, 3)
    kv_update(unstash(0), 1, 1, False)
    xn0, xn1 = xn_tile(0), xn_tile(1)
    vt02 = proj_steps(side, 1, 2, 2, xn0)
    vt12 = proj_steps(side, 5, 2, 2, xn1)
    kv_update(vt02, 0, 2, True)
    vt03 = proj_steps(side, 9, 2, 3, xn0)
    kv_update(vt12, 1, 2, False)
    vt13 = proj_steps(side, 13, 2, 3, xn1)
    kv_update(vt03, 0, 3, True)
    kv_update(vt13, 1, 3, False)

    def phase1(u, carry):
        never = u < 0

        @pl.when(u == 0)
        def _():
            for c in range(1, NC):
                w_copy(0, c).wait()
            x_copy(3).wait()
            wo_copy.wait()
            wr_copy.wait()

        @pl.when(u == 1)
        def _():
            x_copy(4).wait()

        pending = None
        for i in range(2):
            t = 2 * u + 2 + i
            tn = jnp.minimum(t + 1, NT_ - 1)
            side = _Side(never)
            xn = xn_tile(t)
            for c in range(NC):
                pk = proj(1, c, xn)
                if c == 0 and pending is not None:
                    kv_update(*pending)
                k_features(pk, i, c, False)
            side.add(LN1_PLAN, lambda k, a: ln_rows(tn, k, LNC, never, a))
            if i == 0:
                def pack_wo(k, a):
                    rows = WO_ROWS // len(WO_PLAN)
                    w0 = u * ((D - WO_ROWS) // 2)
                    src = woraw_v.at[pl.ds(pl.multiple_of(w0, 16), WO_ROWS), :]
                    dst = wo_v.at[pl.ds(pl.multiple_of(w0 // 2, 8), WO_ROWS // 2), :]
                    pack_rows(src, dst, k * rows, rows, 0, D, never, a)
                side.add(WO_PLAN, pack_wo)
            else:
                def z_final(k, a):
                    z = _after(z_v[k], never, a)
                    zs = _row_sum(z)
                    zb_v[k] = jnp.broadcast_to(zs, (128, 128))
                    return zs[120:128, :]
                side.add(Z_PLAN, z_final)
            side.done(0, pk)
            vts = []
            for c in range(NC):
                vts.append(proj_steps(side, 4 * c + 1, 2, c, xn))
                if c > 0:
                    kv_update(vts[c - 1], i, c - 1, False, i == 1)
            pending = (vts[NC - 1], i, NC - 1, False, i == 1)
        fold(0, u + 1)
        kv_update(*pending)
        wr_v[...] = jnp.broadcast_to(wrraw_v[...].reshape(1, D).astype(F32), (8, D))
        return carry

    lax.fori_loop(0, (NT_ - 2) // 2, phase1, 0)

    def o_copy(r0, n, i):
        return pltpu.make_async_copy(o_v.at[pl.ds(r0, n), :], out_hbm.at[pl.ds(r0, n), :], sem.at[SO + i])

    def finish_rows(h_ref, k, ht, valid, st, never=None, anchor=None):
        r0 = ht * TH + k * LNC
        best, besti = st["route"]
        wr = jnp.concatenate([wr_v[...]] * (LNC // 8), axis=0)
        sub = lax.broadcasted_iota(jnp.int32, (8, 1), 0)
        h = _after(h_ref[k * LNC:(k + 1) * LNC, :], never, anchor)
        m = _row_sum(h) * (1.0 / D)
        hc = h - m
        rstd = lax.rsqrt(_row_sum(hc * hc) * (1.0 / D) + LN_EPS)
        r = (_row_sum(hc * wr) * rstd).astype(BF16).astype(F32)
        hn = hc * rstd
        view(hn_v, ht, TH // 2)[k * LNC // 2:(k + 1) * LNC // 2, :] = _pack(hn.astype(BF16))
        view(o_v, ht, TH)[k * LNC:(k + 1) * LNC, :] = (hn + h).astype(BF16)
        if valid is not None:
            r = jnp.where(valid, r, -jnp.inf)
        for i in range(LNC // 8):
            ri = r[8 * i:8 * i + 8, :]
            better = ri > best
            best = jnp.where(better, ri, best)
            besti = jnp.where(better, sub + (r0 + 8 * i), besti)
        st["route"] = (best, besti)
        return best

    def q_features(pq, slot, c):
        for j in range(PPC):
            pr = c * PPC + j
            ep, en, sp, sn = _dual_exp(pq[64 * j:64 * j + 64, :])
            zz = [_lane_tile(zb_v[pr, 8 * i:8 * i + 8, :], pq.shape[1] // 128) for i in range(16)]
            ap = _pair_allreduce(_tree(jnp.add, [ep[i] * zz[i] for i in range(8)]), jnp.add)
            an = _pair_allreduce(_tree(jnp.add, [en[i] * zz[8 + i] for i in range(8)]), jnp.add)
            inv = _recip(ap * sn + (an + 1e-6 * sn) * sp)
            rp = sn * inv
            rn = sp * inv
            phi = jnp.concatenate([e * rp for e in ep] + [e * rn for e in en], axis=0)
            phi_v[slot][64 * pr:64 * pr + 64, :] = _pack(phi.astype(BF16))

    def attn_rows(slot, c, lo, hi):
        res = jnp.concatenate(
            [_dot(_unpack(kvbf_v[32 * pr:32 * pr + 32, :]), _unpack(phi_v[slot][64 * pr:64 * pr + 64, lo:hi]), NN)
             for pr in range(c * PPC, (c + 1) * PPC)], axis=0)
        return res.astype(BF16).T

    def out_proj(side, step0, o, k0, k1, n0=0, n1=D // 128):
        cols = []
        for n in range(n0, n1):
            w = side.gate(step0 + n, wo_v[k0 // 2:k1 // 2, n * 128:(n + 1) * 128])
            res = _dot(o, _unpack(w), NN)
            side.done(step0 + n, res)
            cols.append(res)
        return jnp.concatenate(cols, axis=1)

    def phase2(u, carry):
        for i in range(UNROLL2):
            carry = phase2_tile(u * UNROLL2 + i, i % 2, carry, u < 0)

        r0 = pl.multiple_of(u * (UNROLL2 * T), T)

        @pl.when(u == 0)
        def _():
            o_copy(0, UNROLL2 * T - TH, 0).start()

        @pl.when(u > 0)
        def _():
            o_copy(pl.multiple_of(jnp.maximum(r0 - TH, 0), TH), UNROLL2 * T, u).start()

        return carry

    def phase2_tile(t, slot, carry, never):
        hp = jnp.maximum(2 * t - 1, 0)
        side = _Side(never)
        st = {"route": carry}
        side.add(LN2B_PLAN, lambda k, a: finish_rows(hb_v, k, hp, t > 0, st, side.never, a))

        def pack_ffn(k, a):
            if k < 32:
                n = D // NT_
                pack_rows(view((wg_v, wu_v)[k % 2], t, n), view((wgp_v, wup_v)[k % 2], t, n // 2),
                          (k // 4) * 16, 16, (k // 2 % 2) * (FM // 2), FM // 2, never, a)
            else:
                n = FM // NT_
                pack_rows(view(wd_v, t, n, FV), view(wdp_v, t, n // 2), (k - 32) * 16, 16, 0, D, never, a)
        side.add(PACK_PLAN, pack_ffn)

        xn = xn_tile(t)
        xt = view(x_v, t, T)
        os_ = []
        for c in range(NC):
            pq = proj_steps(side, 100 + 4 * c, 0, c, xn)
            if c == 0:
                pq = side.gate(0, pq)
            q_features(pq, slot, c)
            if c > 0:
                os_.append(attn_rows(slot, c - 1, 0, T))
        oa = jnp.concatenate([o[0:TH, :] for o in os_[:2]], axis=1)
        ha0 = out_proj(side, 0, oa, 0, D // 2, 0, G3_AT)
        os_.append(attn_rows(slot, NC - 1, 0, T))
        ha1 = out_proj(side, 0, oa, 0, D // 2, G3_AT, D // 128)
        ha = jnp.concatenate([ha0, ha1], axis=1) + xt[0:TH, :].astype(F32)
        ha_v[...] = ha + out_proj(side, 8, jnp.concatenate([o[0:TH, :] for o in os_[2:]], axis=1), D // 2, D)
        side.add(LN2A_PLAN, lambda k, a: finish_rows(ha_v, k, 2 * t, None, st, side.never, a))
        ob = jnp.concatenate([o[TH:T, :] for o in os_], axis=1)
        hb_v[...] = xt[TH:T, :].astype(F32) + out_proj(side, 16, ob, 0, D)
        return st["route"]

    wg_copy.wait()
    wu_copy.wait()
    wd_copy.wait()
    route = lax.fori_loop(
        0, NT_ // UNROLL2, phase2,
        (jnp.full((8, 1), -jnp.inf, F32), jnp.zeros((8, 1), jnp.int32)))
    st = {"route": route}
    for k in range(TH // LNC):
        finish_rows(hb_v, k, 2 * NT_ - 1, None, st)
    best, besti = st["route"]
    o_copy(S - TH, TH, NT_).start()

    rmax = jnp.max(best, axis=0, keepdims=True)
    idx = jnp.min(jnp.where(best == rmax, besti, S), axis=0, keepdims=True)
    idx_s = jnp.clip(idx[0, 0], 0, S - 1)
    blk = pl.multiple_of((idx_s >> 4) << 4, 16)
    pair = jnp.broadcast_to(hn_v[pl.ds(idx_s >> 1, 1), :], (8, D))
    x8 = pltpu.bitcast(jnp.where((idx_s & 1) == 1, pair & jnp.uint32(0xFFFF0000), pair << 16), F32)
    xs = jnp.concatenate([x8, x8], axis=0).astype(BF16)
    acts, anchors = [], []
    for c0 in range(0, FM, 128):
        g = _dot(xs, _unpack(wgp_v[:, c0:c0 + 128]), NN)[0:8, :]
        u = _dot(xs, _unpack(wup_v[:, c0:c0 + 128]), NN)[0:8, :]
        anchors += [g, u]
        acts.append(g * jax.nn.sigmoid(g) * u)
    gu = _sublane_allreduce(_vpu_matvec(
        _col_broadcast(x8),
        lambda g: jnp.concatenate([w[8 * g:8 * g + 8, FM:FF].astype(F32) for w in (wg_v, wu_v)], axis=1),
        never0, anchors[:MOE_NA], 1))
    g, u = gu[:, :FV], gu[:, FV:]
    acts.append(g * jax.nn.sigmoid(g) * u)
    a = jnp.concatenate(acts, axis=1)
    am = jnp.concatenate([a[:, FV:], a[:, FV:]], axis=0).astype(BF16)
    ys, anchors = [], anchors[MOE_NA:]
    for k0 in range(0, FM, 512):
        yk = _dot(am[:, k0:k0 + 512], _unpack(wdp_v[k0 // 2:k0 // 2 + 256, :]), NN)[0:8, :]
        ys.append(yk)
        anchors += [yk[:, c:c + 128] for c in range(128, D, 256)]
    ys.append(_sublane_allreduce(_vpu_matvec(
        _col_broadcast(a[:, :FV]), lambda g: wd_v[8 * g:8 * g + 8, 0:D].astype(F32), never0, anchors[:-MOE_ND], 2)))
    y = _tree(jnp.add, ys) * jax.nn.sigmoid(rmax)
    y = jnp.concatenate([y, y], axis=0)
    sel = lax.broadcasted_iota(jnp.int32, (16, 1), 0) == (idx_s - blk)
    patch_v[...] = (o_v[pl.ds(blk, 16), :].astype(F32) + jnp.where(sel, y, 0.0)).astype(BF16)
    o_copy(0, UNROLL2 * T - TH, 0).wait()
    for u in range(1, NT_ // UNROLL2):
        o_copy(u * UNROLL2 * T - TH, UNROLL2 * T, u).wait()
    o_copy(S - TH, TH, NT_).wait()
    pc = pltpu.make_async_copy(patch_v, out_hbm.at[pl.ds(blk, 16), :], sem.at[SM + 3])
    pc.start()
    pc.wait()


@jax.jit
def pallas_sequential_preLN__linear_kernel_hedgehog__moe_arch_mod__prompt_kernel(
    A_x: jax.Array,
    A_wqkv: jax.Array,
    A_w_phi: jax.Array,
    A_wo: jax.Array,
    B_x: jax.Array,
    B_w_r: jax.Array,
    B_w_gate: jax.Array,
    B_w_up: jax.Array,
    B_w_down: jax.Array,
):
    del B_x
    hbm = pl.BlockSpec(memory_space=pl.ANY)
    out = pl.pallas_call(
        _kernel,
        out_shape=jax.ShapeDtypeStruct((S, D), BF16),
        in_specs=[hbm] * 8,
        out_specs=hbm,
        scratch_shapes=[
            pltpu.VMEM((S, D), BF16),
            pltpu.VMEM((S // 2, D), U32),
            pltpu.VMEM((3 * NC, D, RC), BF16),
            [pltpu.VMEM((D // 2, D), U32)] * 3,
            pltpu.VMEM((H, DH, DH), BF16),
            pltpu.VMEM((8 * 64, 128), U32),
            pltpu.VMEM((D, D), BF16),
            pltpu.VMEM((D // 2, D), U32),
            pltpu.VMEM((D,), BF16),
            pltpu.VMEM((8, D), F32),
            pltpu.VMEM((NPAIR, 64, 128), F32),
            pltpu.VMEM((NPAIR * 32, 128), U32),
            pltpu.VMEM((NPAIR, 128, T), F32),
            pltpu.VMEM((NPAIR, 128, 128), F32),
            [pltpu.VMEM((NPAIR * 64, T), U32)] * 2,
            pltpu.VMEM((TH, D), F32),
            pltpu.VMEM((TH, D), F32),
            pltpu.VMEM((S // 2, D), U32),
            pltpu.VMEM((S, D), BF16),
            pltpu.VMEM((D, FF), BF16),
            pltpu.VMEM((D, FF), BF16),
            pltpu.VMEM((FF, D + WD_PAD), BF16),
            pltpu.VMEM((D // 2, FM), U32),
            pltpu.VMEM((D // 2, FM), U32),
            pltpu.VMEM((FM // 2, D), U32),
            pltpu.VMEM((16, D), BF16),
            pltpu.SemaphoreType.DMA((5 + 3 * NC + NT_ + 8,)),
        ],
        compiler_params=pltpu.CompilerParams(vmem_limit_bytes=100 * 1024 * 1024,
                                             disable_semaphore_checks=True, disable_bounds_checks=True),
        name="hedgehog_mod",
    )(
        A_x.reshape(S, D),
        A_wqkv,
        A_w_phi,
        A_wo,
        B_w_r,
        B_w_gate,
        B_w_up,
        B_w_down,
    )
    return out.reshape(1, S, D)
```

```python
import math

import jax
import jax.numpy as jnp
from jax import lax
import jax.experimental.pallas as pl
import jax.experimental.pallas.tpu as pltpu

F32 = jnp.float32
BF16 = jnp.bfloat16
U32 = jnp.uint32

S = 2048
D = 1024
H = 32
DH = 32
FF = 3584
NPAIR = H // 2
LOG2E = 1.4426950408889634
LN_EPS = 1e-5

T = 256
TH = T // 2
NT_ = S // T
RC = 256
NC = D // RC
PPC = RC // 64
LNC = 16
WD_PAD = 128

LN1_PLAN = tuple((round(13 * k / 15, 3), math.ceil(round(13 * k / 15, 3)) + 3) for k in range(16))
LN2B_PLAN = ((None, 0), (None, 0), (None, 0), (2.0, 7), (3.5, 9), (5.0, 10), (6.5, 12), (8.0, 13))
LN2A_PLAN = ((None, 18), (16, 19), (16, 19), (17, 20), (18, 21), (19, 22), (20, 23), (20, 23))
PRO_LN1_PLAN = tuple((None, None) for k in range(16))
PRO_K_PLAN = tuple((r, None) for r in (0, 1, 2, 3, 3.5, 4, 4.5, 5))
PRO_V_PLANS = tuple(tuple((4 * i + k / 2, None) for k in range(8)) for i in range(3)) + (
    tuple((12 + k, 15 + k) for k in range(16)),)
WO_ROWS = 352
WO_PLAN = tuple((6 + k / 2, None) for k in range(11))
Z_PLAN = tuple((round(4 + 8 * k / 15, 3), math.ceil(round(4 + 8 * k / 15, 3)) + 2) for k in range(16))
UNROLL2 = 2
FV = 8 * 128
FM = FF - FV
PACK_PLAN = tuple((r, None) for r in [x - f for f in (0, 0.9) for x in range(100, 116)] + [round(21 * k / 19, 3) for k in range(20)])
MOE_NA = 38
MOE_ND = 2
QUARTERS = True
G3_AT = 5

NN = (((1,), (0,)), ((), ()))
NT = (((1,), (1,)), ((), ()))


def _dot(a, b, dims):
    return lax.dot_general(a, b, dims, preferred_element_type=F32)


def _recip(x):
    return pl.reciprocal(x, approx=False, full_range=False)


def _pack(x):
    return pltpu.bitcast(x, U32)


def _unpack(x):
    return pltpu.bitcast(x, BF16)


def _pair_allreduce(a, op):
    a = op(a, pltpu.roll(a, 2, 0))
    return op(a, pltpu.roll(a, 4, 0))


def _tree(op, xs):
    xs = list(xs)
    while len(xs) > 1:
        nxt = [op(xs[i], xs[i + 1]) for i in range(0, len(xs) - 1, 2)]
        if len(xs) % 2:
            nxt.append(xs[-1])
        xs = nxt
    return xs[0]


def _dual_exp(p):
    sl = [p[8 * i:8 * i + 8, :] for i in range(8)]
    mx = _pair_allreduce(_tree(jnp.maximum, sl), jnp.maximum)
    mn = _pair_allreduce(_tree(jnp.minimum, sl), jnp.minimum)
    ep = [jnp.exp2(s - mx) for s in sl]
    en = [jnp.exp2(mn - s) for s in sl]
    sp = _pair_allreduce(_tree(jnp.add, ep), jnp.add)
    sn = _pair_allreduce(_tree(jnp.add, en), jnp.add)
    return ep, en, sp, sn


def _after(x, never, anchor):
    if anchor is None:
        return x
    d = jnp.concatenate([anchor] * (x.shape[0] // 8), axis=0)
    if x.shape[1] == 128:
        return jnp.where(never, d, x)
    return jnp.concatenate([jnp.where(never, d, x[:, :128]), x[:, 128:]], axis=1)


def _gate(x, never, deps):
    for i, dep in enumerate(deps):
        d = jnp.broadcast_to(dep, (8, 128))
        if x.dtype != F32:
            d = pltpu.bitcast(d, x.dtype)
        blk = jnp.where(never, d, x[8 * i:8 * i + 8, :128])
        if x.shape[1] > 128:
            blk = jnp.concatenate([blk, x[8 * i:8 * i + 8, 128:]], axis=1)
        parts = ([x[:8 * i, :]] if i else []) + [blk, x[8 * i + 8:, :]]
        x = jnp.concatenate(parts, axis=0)
    return x


def _lane_fold(a):
    return _tree(jnp.add, [a[:, 128 * i:128 * i + 128] for i in range(a.shape[1] // 128)])


def _row_sum(a):
    return jnp.sum(_lane_fold(a), axis=-1, keepdims=True)


def _lane_tile(a, n):
    return a if n == 1 else jnp.concatenate([a] * n, axis=1)


def _sublane_allreduce(a):
    a = a + pltpu.roll(a, 4, 0)
    a = a + pltpu.roll(a, 2, 0)
    return a + pltpu.roll(a, 1, 0)


def _col_broadcast(row8):
    return jnp.concatenate([row8] * 16, axis=0).astype(BF16).T.astype(F32)


def _vpu_matvec(xb, w_rows, never, anchors, lag):
    ng = xb.shape[0] // 8
    acc, hist = None, []
    for g in range(ng):
        dep = anchors[(g * len(anchors)) // ng]
        if g >= lag:
            dep = dep + hist[g - lag]
        x = jnp.where(never, dep, xb[8 * g:8 * g + 8, :])
        w = w_rows(g)
        t = w * _lane_tile(x, w.shape[1] // 128)
        acc = t if acc is None else acc + t
        hist.append(acc[:, -128:])
    return acc


class _Side:
    def __init__(self, never):
        self.never = never
        self.jobs = []
        self.deps = {}

    def add(self, plan, fn):
        for k, (rel, due) in enumerate(plan):
            if rel is None:
                self._run(due, fn, k, None)
            else:
                self.jobs.append((rel, due, fn, k))

    def _run(self, due, fn, k, anchor):
        dep = fn(k, anchor)
        if due is not None:
            self.deps.setdefault(due, []).append(dep)

    def gate(self, step, x):
        return _gate(x, self.never, self.deps.pop(step, []))

    def done(self, step, res):
        m = res.shape[0] // 8
        for job in sorted([j for j in self.jobs if step - 1 < j[0] <= step], key=lambda j: j[0]):
            self.jobs.remove(job)
            g = m - 1 - int((step - job[0]) * m)
            self._run(job[1], job[2], job[3], res[8 * g:8 * g + 8, res.shape[1] - 128:])


def _kernel(x_hbm, wqkv_hbm, wphi_hbm, wo_hbm, wr_hbm, wg_hbm, wu_hbm, wd_hbm, out_hbm,
            x_v, xn_v, wraw_v, wt_v, wphi_v, a_v, woraw_v, wo_v, wrraw_v, wr_v, kvacc_v, kvbf_v,
            z_v, zb_v, phi_v, ha_v, hb_v, hn_v, o_v, wg_v, wu_v, wd_v, wgp_v, wup_v, wdp_v, patch_v,
            sem):
    SX, SW, SO, SM = 0, 6, 6 + 3 * NC, 6 + 3 * NC + NT_ + 1

    def x_copy(i):
        h0, h1 = ((1, 2), (2, 4), (4, 6), (6, 10), (10, 2 * NT_), (0, 1))[i]
        rows = pl.ds(h0 * TH, (h1 - h0) * TH)
        return pltpu.make_async_copy(x_hbm.at[rows, :], x_v.at[rows, :], sem.at[SX + i])

    def k0_copy(s):
        return pltpu.make_async_copy(wqkv_hbm.at[:, pl.ds(D + s * 128, 128)],
                                     wraw_v.at[NC, :, pl.ds(s * 128, 128)], sem.at[(SM + 7, SW + NC)[s]])

    def w_copy(j, c):
        return pltpu.make_async_copy(wqkv_hbm.at[:, pl.ds(j * D + c * RC, RC)], wraw_v.at[j * NC + c],
                                     sem.at[SW + j * NC + c])

    wphi_copy = pltpu.make_async_copy(wphi_hbm, wphi_v, sem.at[SM + 4])
    wr_copy = pltpu.make_async_copy(wr_hbm, wrraw_v, sem.at[SM + 5])
    wo_copy = pltpu.make_async_copy(wo_hbm, woraw_v, sem.at[SM + 6])
    wg_copy = pltpu.make_async_copy(wg_hbm, wg_v, sem.at[SM + 0])
    wu_copy = pltpu.make_async_copy(wu_hbm, wu_v, sem.at[SM + 1])
    wd_copy = pltpu.make_async_copy(wd_hbm, wd_v.at[:, pl.ds(0, D)], sem.at[SM + 2])

    wphi_copy.start()
    k0_copy(0).start()
    x_copy(5).start()
    k0_copy(1).start()
    x_copy(0).start()
    w_copy(1, 1).start()

    def view(ref, i, n, off=0):
        r0 = off + i * n
        return ref.at[pl.ds(r0 if isinstance(r0, int) else pl.multiple_of(r0, math.gcd(n, off)), n), :]

    def ln_rows(t, k, n, never=None, anchor=None):
        x = _after(view(x_v, t, T)[k * n:(k + 1) * n, :].astype(F32), never, anchor)
        xc = x - _row_sum(x) * (1.0 / D)
        rstd = lax.rsqrt(_row_sum(xc * xc) * (1.0 / D) + LN_EPS)
        view(xn_v, t, T // 2)[k * n // 2:(k + 1) * n // 2, :] = _pack((xc * rstd).astype(BF16))
        return _tree(jnp.add, [rstd[8 * i:8 * i + 8, :] for i in range(min(n, LNC) // 8)])

    def xn_tile(t):
        return _unpack(view(xn_v, t, T // 2)[...])

    wphi_copy.wait()

    row = lax.broadcasted_iota(jnp.int32, (128, DH), 0)
    col = lax.broadcasted_iota(jnp.int32, (128, DH), 1)
    expand = jnp.where(((row & 63) >> 1) == col, 1.0, 0.0).astype(BF16)
    a_all = _dot(expand, wphi_v[...].reshape(H * DH, DH), NT)
    row = lax.broadcasted_iota(jnp.int32, (128, 128), 0)
    col = lax.broadcasted_iota(jnp.int32, (128, 128), 1)
    a_keep = (2 * (row >> 6) + (row & 1)) == (col >> 5)
    for g in range(8):
        a_v[64 * g:64 * g + 64, :] = _pack(jnp.where(a_keep, a_all[:, g * 128:(g + 1) * 128], 0.0).astype(BF16))
    hb_v[...] = jnp.zeros((TH, D), F32)

    def fold(j, c, side=None, step0=None, slabs=range(RC // 128)):
        for s in slabs:
            g = c * (RC // 128) + s
            w = wraw_v[j * NC + c, :, s * 128:(s + 1) * 128]
            g0 = 64 * g if isinstance(g, int) else pl.multiple_of(64 * g, 64)
            if j == 2:
                wt = w.T
            else:
                res = _dot(_unpack(a_v[pl.ds(g0, 64), :]), w, NT)
                if side is not None:
                    side.done(step0 + 2 * s, res[:, :D // 2])
                    side.done(step0 + 2 * s + 1, res[:, D // 2:])
                wt = (res * LOG2E).astype(BF16)
            wt_v[j][pl.ds(g0, 64), :] = _pack(wt)

    def wt_rows(j, c):
        return wt_v[j][c * RC // 2:(c + 1) * RC // 2, :]

    def k_pair(p, slot, pr, c0, first):
        ep, en, sp, sn = _dual_exp(p)
        inv = _recip(sp * sn)
        rp = sn * inv
        rn = sp * inv
        phi = jnp.concatenate([e * rp for e in ep] + [e * rn for e in en], axis=0)
        cols = slice(c0, c0 + p.shape[1])
        z_v[pr, :, cols] = phi if first else z_v[pr, :, cols] + phi
        phi_v[slot][64 * pr:64 * pr + 64, cols] = _pack(phi.astype(BF16))

    def k_features(pk, slot, c, first):
        for j in range(PPC):
            k_pair(pk[64 * j:64 * j + 64, :], slot, c * PPC + j, 0, first)

    row = lax.broadcasted_iota(jnp.int32, (64, 128), 0)
    col = lax.broadcasted_iota(jnp.int32, (64, 128), 1)
    kv_keep = (row >> 5) == (col & 1)

    def kv_update(vt, slot, c, first, publish=False):
        for j in range(PPC):
            pr = c * PPC + j
            upd = _dot(vt[64 * j:64 * j + 64, :].astype(BF16), _unpack(phi_v[slot][64 * pr:64 * pr + 64, :]), NT)
            acc = upd if first else kvacc_v[pr] + upd
            kvacc_v[pr] = acc
            if publish:
                kvbf_v[32 * pr:32 * pr + 32, :] = _pack(jnp.where(kv_keep, acc, 0.0).astype(BF16))

    def proj(j, c, xn):
        if QUARTERS:
            return proj_steps(_Side(None), 0, j, c, xn)
        return _dot(_unpack(wt_rows(j, c)), xn, NT)

    def proj_steps(side, step0, j, c, xn):
        w = wt_rows(j, c)
        quarters = []
        for n in range(2):
            for m in range(2):
                step = step0 + 2 * n + m
                wq = side.gate(step, w[m * (RC // 4):(m + 1) * (RC // 4), :])
                res = _dot(_unpack(wq), xn[n * TH:(n + 1) * TH, :], NT)
                side.done(step, res)
                quarters.append(res)
        return jnp.concatenate(
            [jnp.concatenate([quarters[0], quarters[2]], axis=1),
             jnp.concatenate([quarters[1], quarters[3]], axis=1)], axis=0)

    def pack_rows(src, dst, r0, rows, c0, cols, never, a):
        w = _pack(src[r0:r0 + rows, c0:c0 + cols])
        d = jnp.concatenate([_lane_tile(pltpu.bitcast(a, U32), cols // 128)] * (rows // 16), axis=0)
        dst[r0 // 2:(r0 + rows) // 2, c0:c0 + cols] = jnp.where(never, d, w)

    def stash(i, val):
        for q in range(4):
            zb_v[4 * i + q] = val[128 * (q // 2):128 * (q // 2) + 128, 128 * (q % 2):128 * (q % 2) + 128]

    def stashed_k(i, slot, c, first):
        def job(k, a):
            j, n = k // 2, k % 2
            p = zb_v[4 * i + 2 * (j // 2) + n, 64 * (j % 2):64 * (j % 2) + 64, :]
            p = jnp.concatenate([_after(p[0:8, :], never0, a), p[8:, :]], axis=0)
            k_pair(p, slot, c * PPC + j, 128 * n, first)
        return job

    def quarter(m, n):
        xn = _unpack(xn_v[n * TH // 2:(n + 1) * TH // 2, :])
        zb_v[2 * m + n] = _dot(_unpack(wt_v[1][64 * m:64 * m + 64, :]), xn, NT)

    k0_copy(0).wait()
    x_copy(5).wait()
    w_copy(1, 2).start()
    x_copy(1).start()
    fold(1, 0, slabs=(0,))
    never0 = ln_rows(0, 0, TH)[0, 0] < 0.0
    quarter(0, 0)

    k0_copy(1).wait()
    x_copy(0).wait()
    w_copy(1, 3).start()
    for c in range(NC):
        w_copy(2, c).start()
    fold(1, 0, slabs=(1,))
    ln_rows(0, 1, TH)
    quarter(1, 0)
    quarter(0, 1)
    quarter(1, 1)

    for c in (1, 2):
        w_copy(1, c).wait()
        if c == 1:
            x_copy(2).start()
            for cq in range(NC):
                w_copy(0, cq).start()
        else:
            x_copy(3).start()
            wo_copy.start()
            wr_copy.start()
            x_copy(4).start()
        side = _Side(never0)
        side.add(PRO_K_PLAN, stashed_k(c - 1, 0, c - 1, True))
        fold(1, c, side, 0)
        stash(c, proj_steps(side, 4, 1, c, xn_tile(0)))

    x_copy(1).wait()
    w_copy(1, 3).wait()
    wg_copy.start()
    wu_copy.start()
    wd_copy.start()
    side = _Side(never0)
    side.add(PRO_LN1_PLAN, lambda k, a: ln_rows(1, k, LNC, never0, a))
    fold(1, 3, side, 0)
    stash(3, proj_steps(side, 4, 1, 3, xn_tile(0)))
    xn1 = xn_tile(1)
    for c in range(3):
        k_features(proj(1, c, xn1), 1, c, c == 2)
    stash(0, proj(1, 3, xn1))

    for c in range(NC):
        w_copy(2, c).wait()
    x_copy(2).wait()
    w_copy(0, 0).wait()
    side = _Side(never0)
    side.add(PRO_V_PLANS[0], stashed_k(2, 0, 2, False))
    side.add(PRO_V_PLANS[1], stashed_k(3, 0, 3, True))
    side.add(PRO_V_PLANS[2], stashed_k(0, 1, 3, False))
    side.add(PRO_V_PLANS[3], lambda k, a: ln_rows(2, k, LNC, never0, a))
    fold(0, 0)
    xns = (xn_tile(0), xn_tile(1))
    pending = None
    for c in range(NC):
        fold(2, c)
        for i in range(2):
            vt = proj_steps(side, 8 * c + 4 * i, 2, c, xns[i])
            if pending is not None:
                kv_update(*pending)
            pending = (vt, i, c, i == 0)
    kv_update(*pending)

    def phase1(u, carry):
        never = u < 0

        @pl.when(u == 0)
        def _():
            for c in range(1, NC):
                w_copy(0, c).wait()
            x_copy(3).wait()
            wo_copy.wait()
            wr_copy.wait()

        @pl.when(u == 1)
        def _():
            x_copy(4).wait()

        pending = None
        for i in range(2):
            t = 2 * u + 2 + i
            tn = jnp.minimum(t + 1, NT_ - 1)
            side = _Side(never)
            xn = xn_tile(t)
            for c in range(NC):
                pk = proj(1, c, xn)
                if c == 0 and pending is not None:
                    kv_update(*pending)
                k_features(pk, i, c, False)
            side.add(LN1_PLAN, lambda k, a: ln_rows(tn, k, LNC, never, a))
            if i == 0:
                def pack_wo(k, a):
                    rows = WO_ROWS // len(WO_PLAN)
                    w0 = u * ((D - WO_ROWS) // 2)
                    src = woraw_v.at[pl.ds(pl.multiple_of(w0, 16), WO_ROWS), :]
                    dst = wo_v.at[pl.ds(pl.multiple_of(w0 // 2, 8), WO_ROWS // 2), :]
                    pack_rows(src, dst, k * rows, rows, 0, D, never, a)
                side.add(WO_PLAN, pack_wo)
            else:
                def z_final(k, a):
                    z = _after(z_v[k], never, a)
                    zs = _row_sum(z)
                    zb_v[k] = jnp.broadcast_to(zs, (128, 128))
                    return zs[120:128, :]
                side.add(Z_PLAN, z_final)
            side.done(0, pk)
            vts = []
            for c in range(NC):
                vts.append(proj_steps(side, 4 * c + 1, 2, c, xn))
                if c > 0:
                    kv_update(vts[c - 1], i, c - 1, False, i == 1)
            pending = (vts[NC - 1], i, NC - 1, False, i == 1)
        fold(0, u + 1)
        kv_update(*pending)
        wr_v[...] = jnp.broadcast_to(wrraw_v[...].reshape(1, D).astype(F32), (8, D))
        return carry

    lax.fori_loop(0, (NT_ - 2) // 2, phase1, 0)

    def o_copy(r0, n, i):
        return pltpu.make_async_copy(o_v.at[pl.ds(r0, n), :], out_hbm.at[pl.ds(r0, n), :], sem.at[SO + i])

    def finish_rows(h_ref, k, ht, valid, st, never=None, anchor=None):
        r0 = ht * TH + k * LNC
        best, besti = st["route"]
        wr = jnp.concatenate([wr_v[...]] * (LNC // 8), axis=0)
        sub = lax.broadcasted_iota(jnp.int32, (8, 1), 0)
        h = _after(h_ref[k * LNC:(k + 1) * LNC, :], never, anchor)
        m = _row_sum(h) * (1.0 / D)
        hc = h - m
        rstd = lax.rsqrt(_row_sum(hc * hc) * (1.0 / D) + LN_EPS)
        r = (_row_sum(hc * wr) * rstd).astype(BF16).astype(F32)
        hn = hc * rstd
        view(hn_v, ht, TH // 2)[k * LNC // 2:(k + 1) * LNC // 2, :] = _pack(hn.astype(BF16))
        view(o_v, ht, TH)[k * LNC:(k + 1) * LNC, :] = (hn + h).astype(BF16)
        if valid is not None:
            r = jnp.where(valid, r, -jnp.inf)
        for i in range(LNC // 8):
            ri = r[8 * i:8 * i + 8, :]
            better = ri > best
            best = jnp.where(better, ri, best)
            besti = jnp.where(better, sub + (r0 + 8 * i), besti)
        st["route"] = (best, besti)
        return best

    def q_features(pq, slot, c):
        for j in range(PPC):
            pr = c * PPC + j
            ep, en, sp, sn = _dual_exp(pq[64 * j:64 * j + 64, :])
            zz = [_lane_tile(zb_v[pr, 8 * i:8 * i + 8, :], pq.shape[1] // 128) for i in range(16)]
            ap = _pair_allreduce(_tree(jnp.add, [ep[i] * zz[i] for i in range(8)]), jnp.add)
            an = _pair_allreduce(_tree(jnp.add, [en[i] * zz[8 + i] for i in range(8)]), jnp.add)
            inv = _recip(ap * sn + (an + 1e-6 * sn) * sp)
            rp = sn * inv
            rn = sp * inv
            phi = jnp.concatenate([e * rp for e in ep] + [e * rn for e in en], axis=0)
            phi_v[slot][64 * pr:64 * pr + 64, :] = _pack(phi.astype(BF16))

    def attn_rows(slot, c, lo, hi):
        res = jnp.concatenate(
            [_dot(_unpack(kvbf_v[32 * pr:32 * pr + 32, :]), _unpack(phi_v[slot][64 * pr:64 * pr + 64, lo:hi]), NN)
             for pr in range(c * PPC, (c + 1) * PPC)], axis=0)
        return res.astype(BF16).T

    def out_proj(side, step0, o, k0, k1, n0=0, n1=D // 128):
        cols = []
        for n in range(n0, n1):
            w = side.gate(step0 + n, wo_v[k0 // 2:k1 // 2, n * 128:(n + 1) * 128])
            res = _dot(o, _unpack(w), NN)
            side.done(step0 + n, res)
            cols.append(res)
        return jnp.concatenate(cols, axis=1)

    def phase2(u, carry):
        for i in range(UNROLL2):
            carry = phase2_tile(u * UNROLL2 + i, i % 2, carry, u < 0)

        r0 = pl.multiple_of(u * (UNROLL2 * T), T)

        @pl.when(u == 0)
        def _():
            o_copy(0, UNROLL2 * T - TH, 0).start()

        @pl.when(u > 0)
        def _():
            o_copy(pl.multiple_of(jnp.maximum(r0 - TH, 0), TH), UNROLL2 * T, u).start()

        return carry

    def phase2_tile(t, slot, carry, never):
        hp = jnp.maximum(2 * t - 1, 0)
        side = _Side(never)
        st = {"route": carry}
        side.add(LN2B_PLAN, lambda k, a: finish_rows(hb_v, k, hp, t > 0, st, side.never, a))

        def pack_ffn(k, a):
            if k < 32:
                n = D // NT_
                pack_rows(view((wg_v, wu_v)[k % 2], t, n), view((wgp_v, wup_v)[k % 2], t, n // 2),
                          (k // 4) * 16, 16, (k // 2 % 2) * (FM // 2), FM // 2, never, a)
            else:
                n = FM // NT_
                pack_rows(view(wd_v, t, n, FV), view(wdp_v, t, n // 2), (k - 32) * 16, 16, 0, D, never, a)
        side.add(PACK_PLAN, pack_ffn)

        xn = xn_tile(t)
        xt = view(x_v, t, T)
        os_ = []
        for c in range(NC):
            pq = proj_steps(side, 100 + 4 * c, 0, c, xn)
            if c == 0:
                pq = side.gate(0, pq)
            q_features(pq, slot, c)
            if c > 0:
                os_.append(attn_rows(slot, c - 1, 0, T))
        oa = jnp.concatenate([o[0:TH, :] for o in os_[:2]], axis=1)
        ha0 = out_proj(side, 0, oa, 0, D // 2, 0, G3_AT)
        os_.append(attn_rows(slot, NC - 1, 0, T))
        ha1 = out_proj(side, 0, oa, 0, D // 2, G3_AT, D // 128)
        ha = jnp.concatenate([ha0, ha1], axis=1) + xt[0:TH, :].astype(F32)
        ha_v[...] = ha + out_proj(side, 8, jnp.concatenate([o[0:TH, :] for o in os_[2:]], axis=1), D // 2, D)
        side.add(LN2A_PLAN, lambda k, a: finish_rows(ha_v, k, 2 * t, None, st, side.never, a))
        ob = jnp.concatenate([o[TH:T, :] for o in os_], axis=1)
        hb_v[...] = xt[TH:T, :].astype(F32) + out_proj(side, 16, ob, 0, D)
        return st["route"]

    wg_copy.wait()
    wu_copy.wait()
    wd_copy.wait()
    route = lax.fori_loop(
        0, NT_ // UNROLL2, phase2,
        (jnp.full((8, 1), -jnp.inf, F32), jnp.zeros((8, 1), jnp.int32)))
    st = {"route": route}
    for k in range(TH // LNC):
        finish_rows(hb_v, k, 2 * NT_ - 1, None, st)
    best, besti = st["route"]
    o_copy(S - TH, TH, NT_).start()

    rmax = jnp.max(best, axis=0, keepdims=True)
    idx = jnp.min(jnp.where(best == rmax, besti, S), axis=0, keepdims=True)
    idx_s = jnp.clip(idx[0, 0], 0, S - 1)
    blk = pl.multiple_of((idx_s >> 4) << 4, 16)
    pair = jnp.broadcast_to(hn_v[pl.ds(idx_s >> 1, 1), :], (8, D))
    x8 = pltpu.bitcast(jnp.where((idx_s & 1) == 1, pair & jnp.uint32(0xFFFF0000), pair << 16), F32)
    xs = jnp.concatenate([x8, x8], axis=0).astype(BF16)
    acts, anchors = [], []
    for c0 in range(0, FM, 128):
        g = _dot(xs, _unpack(wgp_v[:, c0:c0 + 128]), NN)[0:8, :]
        u = _dot(xs, _unpack(wup_v[:, c0:c0 + 128]), NN)[0:8, :]
        anchors += [g, u]
        acts.append(g * jax.nn.sigmoid(g) * u)
    gu = _sublane_allreduce(_vpu_matvec(
        _col_broadcast(x8),
        lambda g: jnp.concatenate([w[8 * g:8 * g + 8, FM:FF].astype(F32) for w in (wg_v, wu_v)], axis=1),
        never0, anchors[:MOE_NA], 1))
    g, u = gu[:, :FV], gu[:, FV:]
    acts.append(g * jax.nn.sigmoid(g) * u)
    a = jnp.concatenate(acts, axis=1)
    am = jnp.concatenate([a[:, FV:], a[:, FV:]], axis=0).astype(BF16)
    ys, anchors = [], anchors[MOE_NA:]
    for k0 in range(0, FM, 512):
        yk = _dot(am[:, k0:k0 + 512], _unpack(wdp_v[k0 // 2:k0 // 2 + 256, :]), NN)[0:8, :]
        ys.append(yk)
        anchors += [yk[:, c:c + 128] for c in range(128, D, 256)]
    ys.append(_sublane_allreduce(_vpu_matvec(
        _col_broadcast(a[:, :FV]), lambda g: wd_v[8 * g:8 * g + 8, 0:D].astype(F32), never0, anchors[:-MOE_ND], 2)))
    y = _tree(jnp.add, ys) * jax.nn.sigmoid(rmax)
    y = jnp.concatenate([y, y], axis=0)
    sel = lax.broadcasted_iota(jnp.int32, (16, 1), 0) == (idx_s - blk)
    patch_v[...] = (o_v[pl.ds(blk, 16), :].astype(F32) + jnp.where(sel, y, 0.0)).astype(BF16)
    o_copy(0, UNROLL2 * T - TH, 0).wait()
    for u in range(1, NT_ // UNROLL2):
        o_copy(u * UNROLL2 * T - TH, UNROLL2 * T, u).wait()
    o_copy(S - TH, TH, NT_).wait()
    pc = pltpu.make_async_copy(patch_v, out_hbm.at[pl.ds(blk, 16), :], sem.at[SM + 3])
    pc.start()
    pc.wait()


@jax.jit
def pallas_sequential_preLN__linear_kernel_hedgehog__moe_arch_mod__prompt_kernel(
    A_x: jax.Array,
    A_wqkv: jax.Array,
    A_w_phi: jax.Array,
    A_wo: jax.Array,
    B_x: jax.Array,
    B_w_r: jax.Array,
    B_w_gate: jax.Array,
    B_w_up: jax.Array,
    B_w_down: jax.Array,
):
    del B_x
    hbm = pl.BlockSpec(memory_space=pl.ANY)
    out = pl.pallas_call(
        _kernel,
        out_shape=jax.ShapeDtypeStruct((S, D), BF16),
        in_specs=[hbm] * 8,
        out_specs=hbm,
        scratch_shapes=[
            pltpu.VMEM((S, D), BF16),
            pltpu.VMEM((S // 2, D), U32),
            pltpu.VMEM((3 * NC, D, RC), BF16),
            [pltpu.VMEM((D // 2, D), U32)] * 3,
            pltpu.VMEM((H, DH, DH), BF16),
            pltpu.VMEM((8 * 64, 128), U32),
            pltpu.VMEM((D, D), BF16),
            pltpu.VMEM((D // 2, D), U32),
            pltpu.VMEM((D,), BF16),
            pltpu.VMEM((8, D), F32),
            pltpu.VMEM((NPAIR, 64, 128), F32),
            pltpu.VMEM((NPAIR * 32, 128), U32),
            pltpu.VMEM((NPAIR, 128, T), F32),
            pltpu.VMEM((NPAIR, 128, 128), F32),
            [pltpu.VMEM((NPAIR * 64, T), U32)] * 2,
            pltpu.VMEM((TH, D), F32),
            pltpu.VMEM((TH, D), F32),
            pltpu.VMEM((S // 2, D), U32),
            pltpu.VMEM((S, D), BF16),
            pltpu.VMEM((D, FF), BF16),
            pltpu.VMEM((D, FF), BF16),
            pltpu.VMEM((FF, D + WD_PAD), BF16),
            pltpu.VMEM((D // 2, FM), U32),
            pltpu.VMEM((D // 2, FM), U32),
            pltpu.VMEM((FM // 2, D), U32),
            pltpu.VMEM((16, D), BF16),
            pltpu.SemaphoreType.DMA((6 + 3 * NC + NT_ + 9,)),
        ],
        compiler_params=pltpu.CompilerParams(vmem_limit_bytes=100 * 1024 * 1024,
                                             disable_semaphore_checks=True, disable_bounds_checks=True),
        name="hedgehog_mod",
    )(
        A_x.reshape(S, D),
        A_wqkv,
        A_w_phi,
        A_wo,
        B_w_r,
        B_w_gate,
        B_w_up,
        B_w_down,
    )
    return out.reshape(1, S, D)
```

```python
import math

import jax
import jax.numpy as jnp
from jax import lax
import jax.experimental.pallas as pl
import jax.experimental.pallas.tpu as pltpu

F32 = jnp.float32
BF16 = jnp.bfloat16
U32 = jnp.uint32

S = 2048
D = 1024
H = 32
DH = 32
FF = 3584
NPAIR = H // 2
LOG2E = 1.4426950408889634
LN_EPS = 1e-5

T = 256
TH = T // 2
NT_ = S // T
RC = 256
NC = D // RC
PPC = RC // 64
LNC = 16
WD_PAD = 128

FV = 8 * 128
FM = FF - FV
WO_ROWS = 352
UNROLL2 = 2


def _spread(n, a, b, due=None):
    rel = [round(a + (b - a) * k / (n - 1), 3) for k in range(n)]
    return tuple((r, None if due is None else math.ceil(r) + due) for r in rel)


LN1_PLAN = _spread(16, 0, 12, 3)
WO_PLAN = _spread(11, 3, 13)
Z_PLAN = _spread(16, 6, 14, 2)
PRO_LN1_PLAN = ((None, None),) * 16
PRO_K_PLAN = _spread(8, 0, 6)
PRO_V_PLANS = (_spread(8, 0, 12), _spread(16, 13, 24)[:8], _spread(16, 13, 24)[8:], _spread(16, 0.7, 28, 3))
LN2B_PLAN = ((None, 0), (None, 0), (None, 0), (2.166, 8), (3.769, 9), (5.524, 11), (7.081, 13), (9.164, 15))
LN2A_PLAN = ((None, 18),) + _spread(7, 15.6, 20, 3)
PACK_PLAN = _spread(16, 100, 115) + _spread(16, 99.1, 114.1) + _spread(20, 0, 21)
G3_AT = 4
MOE_NA = 34
MOE_ND = 2
STAGGER = 8

NN = (((1,), (0,)), ((), ()))
NT = (((1,), (1,)), ((), ()))


def _dot(a, b, dims):
    return lax.dot_general(a, b, dims, preferred_element_type=F32)


def _recip(x):
    return pl.reciprocal(x, approx=False, full_range=False)


def _pack(x):
    return pltpu.bitcast(x, U32)


def _unpack(x):
    return pltpu.bitcast(x, BF16)


def _pair_allreduce(a, op):
    a = op(a, pltpu.roll(a, 2, 0))
    return op(a, pltpu.roll(a, 4, 0))


def _tree(op, xs):
    xs = list(xs)
    while len(xs) > 1:
        nxt = [op(xs[i], xs[i + 1]) for i in range(0, len(xs) - 1, 2)]
        if len(xs) % 2:
            nxt.append(xs[-1])
        xs = nxt
    return xs[0]


def _dual_exp(p):
    sl = [p[8 * i:8 * i + 8, :] for i in range(8)]
    mx = _pair_allreduce(_tree(jnp.maximum, sl), jnp.maximum)
    mn = _pair_allreduce(_tree(jnp.minimum, sl), jnp.minimum)
    ep = [jnp.exp2(s - mx) for s in sl]
    en = [jnp.exp2(mn - s) for s in sl]
    sp = _pair_allreduce(_tree(jnp.add, ep), jnp.add)
    sn = _pair_allreduce(_tree(jnp.add, en), jnp.add)
    return ep, en, sp, sn


def _after(x, never, anchor):
    if anchor is None:
        return x
    d = jnp.concatenate([anchor] * (x.shape[0] // 8), axis=0)
    if x.shape[1] == 128:
        return jnp.where(never, d, x)
    return jnp.concatenate([jnp.where(never, d, x[:, :128]), x[:, 128:]], axis=1)


def _gate(x, never, deps):
    for i, dep in enumerate(deps):
        d = jnp.broadcast_to(dep, (8, 128))
        if x.dtype != F32:
            d = pltpu.bitcast(d, x.dtype)
        blk = jnp.where(never, d, x[8 * i:8 * i + 8, :128])
        if x.shape[1] > 128:
            blk = jnp.concatenate([blk, x[8 * i:8 * i + 8, 128:]], axis=1)
        parts = ([x[:8 * i, :]] if i else []) + [blk, x[8 * i + 8:, :]]
        x = jnp.concatenate(parts, axis=0)
    return x


def _lane_fold(a):
    return _tree(jnp.add, [a[:, 128 * i:128 * i + 128] for i in range(a.shape[1] // 128)])


def _row_sum(a):
    return jnp.sum(_lane_fold(a), axis=-1, keepdims=True)


def _lane_tile(a, n):
    return a if n == 1 else jnp.concatenate([a] * n, axis=1)


def _sublane_allreduce(a):
    a = a + pltpu.roll(a, 4, 0)
    a = a + pltpu.roll(a, 2, 0)
    return a + pltpu.roll(a, 1, 0)


def _col_broadcast(row8):
    return jnp.concatenate([row8] * 16, axis=0).astype(BF16).T.astype(F32)


def _vpu_matvec(xb, w_rows, never, anchors, lag):
    ng = xb.shape[0] // 8
    acc, hist = None, []
    for g in range(ng):
        dep = anchors[(g * len(anchors)) // ng]
        if g >= lag:
            dep = dep + hist[g - lag]
        x = jnp.where(never, dep, xb[8 * g:8 * g + 8, :])
        w = w_rows(g)
        t = w * _lane_tile(x, w.shape[1] // 128)
        acc = t if acc is None else acc + t
        hist.append(acc[:, -128:])
    return acc


class _Side:
    def __init__(self, never):
        self.never = never
        self.jobs = []
        self.deps = {}

    def add(self, plan, fn):
        for k, (rel, due) in enumerate(plan):
            if rel is None:
                self._run(due, fn, k, None)
            else:
                self.jobs.append((rel, due, fn, k))

    def _run(self, due, fn, k, anchor):
        dep = fn(k, anchor)
        if due is not None:
            self.deps.setdefault(due, []).append(dep)

    def check(self):
        assert not self.jobs and not self.deps, (self.jobs, self.deps)

    def gate(self, step, x):
        return _gate(x, self.never, self.deps.pop(step, []))

    def done(self, step, res):
        m = res.shape[0] // 8
        for job in sorted([j for j in self.jobs if step - 1 < j[0] <= step], key=lambda j: j[0]):
            self.jobs.remove(job)
            g = m - 1 - int((step - job[0]) * m)
            self._run(job[1], job[2], job[3], res[8 * g:8 * g + 8, res.shape[1] - 128:])


def _kernel(x_hbm, wqkv_hbm, wphi_hbm, wo_hbm, wr_hbm, wg_hbm, wu_hbm, wd_hbm, out_hbm,
            x_v, xn_v, wraw_v, wt_v, wphi_v, a_v, woraw_v, wo_v, wrraw_v, wr_v, kvacc_v, kvbf_v,
            z_v, zb_v, phi_v, ha_v, hb_v, hn_v, o_v, wg_v, wu_v, wd_v, wgp_v, wup_v, wdp_v, patch_v,
            sem):
    SX, SW, SO, SM = 0, 6, 6 + 3 * NC, 6 + 3 * NC + NT_ + 1

    def x_copy(i):
        h0, h1 = ((1, 2), (2, 4), (4, 6), (6, 10), (10, 2 * NT_), (0, 1))[i]
        rows = pl.ds(h0 * TH, (h1 - h0) * TH)
        return pltpu.make_async_copy(x_hbm.at[rows, :], x_v.at[rows, :], sem.at[SX + i])

    def k0_copy(s):
        return pltpu.make_async_copy(wqkv_hbm.at[:, pl.ds(D + s * 128, 128)],
                                     wraw_v.at[NC, :, pl.ds(s * 128, 128)], sem.at[(SM + 7, SW + NC)[s]])

    def w_copy(j, c):
        return pltpu.make_async_copy(wqkv_hbm.at[:, pl.ds(j * D + c * RC, RC)], wraw_v.at[j * NC + c],
                                     sem.at[SW + j * NC + c])

    wphi_copy = pltpu.make_async_copy(wphi_hbm, wphi_v, sem.at[SM + 4])
    wr_copy = pltpu.make_async_copy(wr_hbm, wrraw_v, sem.at[SM + 5])
    wo_copy = pltpu.make_async_copy(wo_hbm, woraw_v, sem.at[SM + 6])
    wg_copy = pltpu.make_async_copy(wg_hbm, wg_v, sem.at[SM + 0])
    wu_copy = pltpu.make_async_copy(wu_hbm, wu_v, sem.at[SM + 1])
    wd_copy = pltpu.make_async_copy(wd_hbm, wd_v.at[:, pl.ds(0, D)], sem.at[SM + 2])

    wphi_copy.start()
    k0_copy(0).start()
    x_copy(5).start()
    k0_copy(1).start()
    x_copy(0).start()
    w_copy(1, 1).start()

    def view(ref, i, n, off=0):
        r0 = off + i * n
        return ref.at[pl.ds(r0 if isinstance(r0, int) else pl.multiple_of(r0, math.gcd(n, off)), n), :]

    def ln_rows(t, k, n, never=None, anchor=None):
        x = _after(view(x_v, t, T)[k * n:(k + 1) * n, :].astype(F32), never, anchor)
        xc = x - _row_sum(x) * (1.0 / D)
        rstd = lax.rsqrt(_row_sum(xc * xc) * (1.0 / D) + LN_EPS)
        view(xn_v, t, T // 2)[k * n // 2:(k + 1) * n // 2, :] = _pack((xc * rstd).astype(BF16))
        return _tree(jnp.add, [rstd[8 * i:8 * i + 8, :] for i in range(min(n, LNC) // 8)])

    def xn_tile(t):
        return _unpack(view(xn_v, t, T // 2)[...])

    wphi_copy.wait()

    row = lax.broadcasted_iota(jnp.int32, (128, DH), 0)
    col = lax.broadcasted_iota(jnp.int32, (128, DH), 1)
    expand = jnp.where(((row & 63) >> 1) == col, 1.0, 0.0).astype(BF16)
    a_all = _dot(expand, wphi_v[...].reshape(H * DH, DH), NT)
    row = lax.broadcasted_iota(jnp.int32, (128, 128), 0)
    col = lax.broadcasted_iota(jnp.int32, (128, 128), 1)
    a_keep = (2 * (row >> 6) + (row & 1)) == (col >> 5)
    for g in range(8):
        a_v[64 * g:64 * g + 64, :] = _pack(jnp.where(a_keep, a_all[:, g * 128:(g + 1) * 128], 0.0).astype(BF16))
    hb_v[...] = jnp.zeros((TH, D), F32)

    def fold(j, c, side=None, step0=None, slabs=range(RC // 128)):
        for s in slabs:
            g = c * (RC // 128) + s
            w = wraw_v[j * NC + c, :, s * 128:(s + 1) * 128]
            g0 = 64 * g if isinstance(g, int) else pl.multiple_of(64 * g, 64)
            if j == 2:
                wt = w.T
            else:
                res = _dot(_unpack(a_v[pl.ds(g0, 64), :]), w, NT)
                if side is not None:
                    side.done(step0 + 2 * s, res[:, :D // 2])
                    side.done(step0 + 2 * s + 1, res[:, D // 2:])
                wt = (res * LOG2E).astype(BF16)
            wt_v[j][pl.ds(g0, 64), :] = _pack(wt)

    def wt_rows(j, c):
        return wt_v[j][c * RC // 2:(c + 1) * RC // 2, :]

    def k_pair(p, slot, pr, c0, first, never=None):
        ep, en, sp, sn = _dual_exp(p)
        inv = _recip(sp * sn)
        scale = (sn * inv, sp * inv)
        es = ep + en
        cols = slice(c0, c0 + p.shape[1])
        n = 16 if never is None else 16 // STAGGER
        last = None
        for q in range(16 // n):
            sc = scale
            if last is not None:
                sc = [jnp.where(never, last, x) for x in scale]
            phi = jnp.concatenate([es[i] * sc[i // 8] for i in range(q * n, (q + 1) * n)], axis=0)
            rows = slice(8 * q * n, 8 * (q + 1) * n)
            z = phi if first else z_v[pr, rows, cols] + phi
            z_v[pr, rows, cols] = z
            phi_v[slot][64 * pr + 4 * q * n:64 * pr + 4 * (q + 1) * n, cols] = _pack(phi.astype(BF16))
            last = z[8 * n - 8:, :]

    def k_features(pk, slot, c, first, never=None):
        for j in range(PPC):
            k_pair(pk[64 * j:64 * j + 64, :], slot, c * PPC + j, 0, first, never)

    row = lax.broadcasted_iota(jnp.int32, (64, 128), 0)
    col = lax.broadcasted_iota(jnp.int32, (64, 128), 1)
    kv_keep = (row >> 5) == (col & 1)

    def kv_update(vt, slot, c, first, publish=False):
        for j in range(PPC):
            pr = c * PPC + j
            upd = _dot(vt[64 * j:64 * j + 64, :].astype(BF16), _unpack(phi_v[slot][64 * pr:64 * pr + 64, :]), NT)
            acc = upd if first else kvacc_v[pr] + upd
            kvacc_v[pr] = acc
            if publish:
                kvbf_v[32 * pr:32 * pr + 32, :] = _pack(jnp.where(kv_keep, acc, 0.0).astype(BF16))

    def proj(j, c, xn):
        return proj_steps(_Side(None), 0, j, c, xn)

    def proj_steps(side, step0, j, c, xn):
        w = wt_rows(j, c)
        quarters = []
        for n in range(2):
            for m in range(2):
                step = step0 + 2 * n + m
                wq = side.gate(step, w[m * (RC // 4):(m + 1) * (RC // 4), :])
                res = _dot(_unpack(wq), xn[n * TH:(n + 1) * TH, :], NT)
                side.done(step, res)
                quarters.append(res)
        return jnp.concatenate(
            [jnp.concatenate([quarters[0], quarters[2]], axis=1),
             jnp.concatenate([quarters[1], quarters[3]], axis=1)], axis=0)

    def pack_rows(src, dst, r0, rows, c0, cols, never, a):
        w = _pack(src[r0:r0 + rows, c0:c0 + cols])
        d = jnp.concatenate([_lane_tile(pltpu.bitcast(a, U32), cols // 128)] * (rows // 16), axis=0)
        dst[r0 // 2:(r0 + rows) // 2, c0:c0 + cols] = jnp.where(never, d, w)

    def stash(i, val):
        for q in range(4):
            zb_v[4 * i + q] = val[128 * (q // 2):128 * (q // 2) + 128, 128 * (q % 2):128 * (q % 2) + 128]

    def stashed_k(i, slot, c, first):
        def job(k, a):
            j, n = k // 2, k % 2
            p = zb_v[4 * i + 2 * (j // 2) + n, 64 * (j % 2):64 * (j % 2) + 64, :]
            p = jnp.concatenate([_after(p[0:8, :], never0, a), p[8:, :]], axis=0)
            k_pair(p, slot, c * PPC + j, 128 * n, first, never0)
        return job

    def quarter(m, n):
        xn = _unpack(xn_v[n * TH // 2:(n + 1) * TH // 2, :])
        zb_v[2 * m + n] = _dot(_unpack(wt_v[1][64 * m:64 * m + 64, :]), xn, NT)

    k0_copy(0).wait()
    x_copy(5).wait()
    w_copy(1, 2).start()
    x_copy(1).start()
    fold(1, 0, slabs=(0,))
    never0 = ln_rows(0, 0, TH)[0, 0] < 0.0
    quarter(0, 0)

    k0_copy(1).wait()
    x_copy(0).wait()
    w_copy(1, 3).start()
    for c in range(NC):
        w_copy(2, c).start()
    fold(1, 0, slabs=(1,))
    ln_rows(0, 1, TH)
    quarter(1, 0)
    quarter(0, 1)
    quarter(1, 1)

    for c in (1, 2):
        w_copy(1, c).wait()
        if c == 1:
            x_copy(2).start()
            for cq in range(NC):
                w_copy(0, cq).start()
        else:
            x_copy(3).start()
            wo_copy.start()
            wr_copy.start()
            x_copy(4).start()
        side = _Side(never0)
        side.add(PRO_K_PLAN, stashed_k(c - 1, 0, c - 1, True))
        fold(1, c, side, 0)
        stash(c, proj_steps(side, 4, 1, c, xn_tile(0)))
        side.check()

    x_copy(1).wait()
    w_copy(1, 3).wait()
    wg_copy.start()
    wu_copy.start()
    wd_copy.start()
    side = _Side(never0)
    side.add(PRO_LN1_PLAN, lambda k, a: ln_rows(1, k, LNC, never0, a))
    fold(1, 3, side, 0)
    stash(3, proj_steps(side, 4, 1, 3, xn_tile(0)))
    xn1 = xn_tile(1)
    for c in range(3):
        k_features(proj(1, c, xn1), 1, c, c == 2, never0)
    stash(0, proj(1, 3, xn1))

    for c in range(NC):
        w_copy(2, c).wait()
    x_copy(2).wait()
    w_copy(0, 0).wait()
    side = _Side(never0)
    side.add(PRO_V_PLANS[0], stashed_k(2, 0, 2, False))
    side.add(PRO_V_PLANS[1], stashed_k(3, 0, 3, True))
    side.add(PRO_V_PLANS[2], stashed_k(0, 1, 3, False))
    side.add(PRO_V_PLANS[3], lambda k, a: ln_rows(2, k, LNC, never0, a))
    fold(0, 0)
    xns = (xn_tile(0), xn_tile(1))
    pending = None
    for c in range(NC):
        fold(2, c)
        for i in range(2):
            vt = proj_steps(side, 8 * c + 4 * i, 2, c, xns[i])
            if pending is not None:
                kv_update(*pending)
            pending = (vt, i, c, i == 0)
    side.check()
    kv_update(*pending)

    def phase1(u, carry):
        never = u < 0

        @pl.when(u == 0)
        def _():
            for c in range(1, NC):
                w_copy(0, c).wait()
            x_copy(3).wait()
            wo_copy.wait()
            wr_copy.wait()

        @pl.when(u == 1)
        def _():
            x_copy(4).wait()

        pending = None
        for i in range(2):
            t = 2 * u + 2 + i
            tn = jnp.minimum(t + 1, NT_ - 1)
            side = _Side(never)
            xn = xn_tile(t)
            for c in range(NC):
                pk = proj(1, c, xn)
                if c == 0 and pending is not None:
                    kv_update(*pending)
                k_features(pk, i, c, False)
            side.add(LN1_PLAN, lambda k, a: ln_rows(tn, k, LNC, never, a))
            if i == 0:
                def pack_wo(k, a):
                    rows = WO_ROWS // len(WO_PLAN)
                    w0 = u * ((D - WO_ROWS) // 2)
                    src = woraw_v.at[pl.ds(pl.multiple_of(w0, 16), WO_ROWS), :]
                    dst = wo_v.at[pl.ds(pl.multiple_of(w0 // 2, 8), WO_ROWS // 2), :]
                    pack_rows(src, dst, k * rows, rows, 0, D, never, a)
                side.add(WO_PLAN, pack_wo)
            else:
                def z_final(k, a):
                    z = _after(z_v[k], never, a)
                    zs = _row_sum(z)
                    zb_v[k] = jnp.broadcast_to(zs, (128, 128))
                    return zs[120:128, :]
                side.add(Z_PLAN, z_final)
            side.done(0, pk)
            vts = []
            for c in range(NC):
                vts.append(proj_steps(side, 4 * c + 1, 2, c, xn))
                if c > 0:
                    kv_update(vts[c - 1], i, c - 1, False, i == 1)
            pending = (vts[NC - 1], i, NC - 1, False, i == 1)
            side.check()
        fold(0, u + 1)
        kv_update(*pending)
        wr_v[...] = jnp.broadcast_to(wrraw_v[...].reshape(1, D).astype(F32), (8, D))
        return carry

    lax.fori_loop(0, (NT_ - 2) // 2, phase1, 0)

    def o_copy(r0, n, i):
        return pltpu.make_async_copy(o_v.at[pl.ds(r0, n), :], out_hbm.at[pl.ds(r0, n), :], sem.at[SO + i])

    def finish_rows(h_ref, k, ht, valid, st, never=None, anchor=None):
        r0 = ht * TH + k * LNC
        best, besti = st["route"]
        wr = jnp.concatenate([wr_v[...]] * (LNC // 8), axis=0)
        sub = lax.broadcasted_iota(jnp.int32, (8, 1), 0)
        h = _after(h_ref[k * LNC:(k + 1) * LNC, :], never, anchor)
        hc = h - _row_sum(h) * (1.0 / D)
        rstd = lax.rsqrt(_row_sum(hc * hc) * (1.0 / D) + LN_EPS)
        r = (_row_sum(hc * wr) * rstd).astype(BF16).astype(F32)
        hn = hc * rstd
        view(hn_v, ht, TH // 2)[k * LNC // 2:(k + 1) * LNC // 2, :] = _pack(hn.astype(BF16))
        view(o_v, ht, TH)[k * LNC:(k + 1) * LNC, :] = (hn + h).astype(BF16)
        if valid is not None:
            r = jnp.where(valid, r, -jnp.inf)
        for i in range(LNC // 8):
            ri = r[8 * i:8 * i + 8, :]
            better = ri > best
            best = jnp.where(better, ri, best)
            besti = jnp.where(better, sub + (r0 + 8 * i), besti)
        st["route"] = (best, besti)
        return best

    def q_features(pq, slot, c):
        for j in range(PPC):
            pr = c * PPC + j
            ep, en, sp, sn = _dual_exp(pq[64 * j:64 * j + 64, :])
            zz = [_lane_tile(zb_v[pr, 8 * i:8 * i + 8, :], pq.shape[1] // 128) for i in range(16)]
            ap = _pair_allreduce(_tree(jnp.add, [ep[i] * zz[i] for i in range(8)]), jnp.add)
            an = _pair_allreduce(_tree(jnp.add, [en[i] * zz[8 + i] for i in range(8)]), jnp.add)
            inv = _recip(ap * sn + (an + 1e-6 * sn) * sp)
            rp = sn * inv
            rn = sp * inv
            phi = jnp.concatenate([e * rp for e in ep] + [e * rn for e in en], axis=0)
            phi_v[slot][64 * pr:64 * pr + 64, :] = _pack(phi.astype(BF16))

    def attn_rows(slot, c, lo, hi):
        res = jnp.concatenate(
            [_dot(_unpack(kvbf_v[32 * pr:32 * pr + 32, :]), _unpack(phi_v[slot][64 * pr:64 * pr + 64, lo:hi]), NN)
             for pr in range(c * PPC, (c + 1) * PPC)], axis=0)
        return res.astype(BF16).T

    def out_proj(side, step0, o, k0, k1, n0=0, n1=D // 128):
        cols = []
        for n in range(n0, n1):
            w = side.gate(step0 + n, wo_v[k0 // 2:k1 // 2, n * 128:(n + 1) * 128])
            res = _dot(o, _unpack(w), NN)
            side.done(step0 + n, res)
            cols.append(res)
        return jnp.concatenate(cols, axis=1)

    def phase2(u, carry):
        for i in range(UNROLL2):
            carry = phase2_tile(u * UNROLL2 + i, i % 2, carry, u < 0)

        r0 = pl.multiple_of(u * (UNROLL2 * T), T)

        @pl.when(u == 0)
        def _():
            o_copy(0, UNROLL2 * T - TH, 0).start()

        @pl.when(u > 0)
        def _():
            o_copy(pl.multiple_of(jnp.maximum(r0 - TH, 0), TH), UNROLL2 * T, u).start()

        return carry

    def phase2_tile(t, slot, carry, never):
        hp = jnp.maximum(2 * t - 1, 0)
        side = _Side(never)
        st = {"route": carry}
        side.add(LN2B_PLAN, lambda k, a: finish_rows(hb_v, k, hp, t > 0, st, side.never, a))

        def pack_ffn(k, a):
            if k < 32:
                n = D // NT_
                pack_rows(view((wg_v, wu_v)[k % 2], t, n), view((wgp_v, wup_v)[k % 2], t, n // 2),
                          (k // 4) * 16, 16, (k // 2 % 2) * (FM // 2), FM // 2, never, a)
            else:
                n = FM // NT_
                pack_rows(view(wd_v, t, n, FV), view(wdp_v, t, n // 2), (k - 32) * 16, 16, 0, D, never, a)
        side.add(PACK_PLAN, pack_ffn)

        xn = xn_tile(t)
        xt = view(x_v, t, T)
        os_ = []
        for c in range(NC):
            pq = proj_steps(side, 100 + 4 * c, 0, c, xn)
            if c == 0:
                pq = side.gate(0, pq)
            q_features(pq, slot, c)
            if c > 0:
                os_.append(attn_rows(slot, c - 1, 0, T))
        oa = jnp.concatenate([o[0:TH, :] for o in os_[:2]], axis=1)
        ha0 = out_proj(side, 0, oa, 0, D // 2, 0, G3_AT)
        os_.append(attn_rows(slot, NC - 1, 0, T))
        ha1 = out_proj(side, 0, oa, 0, D // 2, G3_AT, D // 128)
        ha = jnp.concatenate([ha0, ha1], axis=1) + xt[0:TH, :].astype(F32)
        ha_v[...] = ha + out_proj(side, 8, jnp.concatenate([o[0:TH, :] for o in os_[2:]], axis=1), D // 2, D)
        side.add(LN2A_PLAN, lambda k, a: finish_rows(ha_v, k, 2 * t, None, st, side.never, a))
        ob = jnp.concatenate([o[TH:T, :] for o in os_], axis=1)
        hb_v[...] = xt[TH:T, :].astype(F32) + out_proj(side, 16, ob, 0, D)
        side.check()
        return st["route"]

    wg_copy.wait()
    wu_copy.wait()
    wd_copy.wait()
    route = lax.fori_loop(
        0, NT_ // UNROLL2, phase2,
        (jnp.full((8, 1), -jnp.inf, F32), jnp.zeros((8, 1), jnp.int32)))
    st = {"route": route}
    for k in range(TH // LNC):
        finish_rows(hb_v, k, 2 * NT_ - 1, None, st)
    best, besti = st["route"]
    o_copy(S - TH, TH, NT_).start()

    rmax = jnp.max(best, axis=0, keepdims=True)
    idx = jnp.min(jnp.where(best == rmax, besti, S), axis=0, keepdims=True)
    idx_s = jnp.clip(idx[0, 0], 0, S - 1)
    blk = pl.multiple_of((idx_s >> 4) << 4, 16)
    pair = jnp.broadcast_to(hn_v[pl.ds(idx_s >> 1, 1), :], (8, D))
    x8 = pltpu.bitcast(jnp.where((idx_s & 1) == 1, pair & jnp.uint32(0xFFFF0000), pair << 16), F32)
    xs = jnp.concatenate([x8, x8], axis=0).astype(BF16)
    acts, anchors = [], []
    for c0 in range(0, FM, 128):
        g = _dot(xs, _unpack(wgp_v[:, c0:c0 + 128]), NN)[0:8, :]
        u = _dot(xs, _unpack(wup_v[:, c0:c0 + 128]), NN)[0:8, :]
        anchors += [g, u]
        acts.append(g * jax.nn.sigmoid(g) * u)
    gu = _sublane_allreduce(_vpu_matvec(
        _col_broadcast(x8),
        lambda g: jnp.concatenate([w[8 * g:8 * g + 8, FM:FF].astype(F32) for w in (wg_v, wu_v)], axis=1),
        never0, anchors[:MOE_NA], 1))
    g, u = gu[:, :FV], gu[:, FV:]
    acts.append(g * jax.nn.sigmoid(g) * u)
    a = jnp.concatenate(acts, axis=1)
    am = jnp.concatenate([a[:, FV:], a[:, FV:]], axis=0).astype(BF16)
    ys, anchors = [], anchors[MOE_NA:]
    for k0 in range(0, FM, 512):
        yk = _dot(am[:, k0:k0 + 512], _unpack(wdp_v[k0 // 2:k0 // 2 + 256, :]), NN)[0:8, :]
        ys.append(yk)
        anchors += [yk[:, c:c + 128] for c in range(128, D, 256)]
    ys.append(_sublane_allreduce(_vpu_matvec(
        _col_broadcast(a[:, :FV]), lambda g: wd_v[8 * g:8 * g + 8, 0:D].astype(F32), never0, anchors[:-MOE_ND], 2)))
    y = _tree(jnp.add, ys) * jax.nn.sigmoid(rmax)
    y = jnp.concatenate([y, y], axis=0)
    sel = lax.broadcasted_iota(jnp.int32, (16, 1), 0) == (idx_s - blk)
    patch_v[...] = (o_v[pl.ds(blk, 16), :].astype(F32) + jnp.where(sel, y, 0.0)).astype(BF16)
    o_copy(0, UNROLL2 * T - TH, 0).wait()
    for u in range(1, NT_ // UNROLL2):
        o_copy(u * UNROLL2 * T - TH, UNROLL2 * T, u).wait()
    o_copy(S - TH, TH, NT_).wait()
    pc = pltpu.make_async_copy(patch_v, out_hbm.at[pl.ds(blk, 16), :], sem.at[SM + 3])
    pc.start()
    pc.wait()


@jax.jit
def pallas_sequential_preLN__linear_kernel_hedgehog__moe_arch_mod__prompt_kernel(
    A_x: jax.Array,
    A_wqkv: jax.Array,
    A_w_phi: jax.Array,
    A_wo: jax.Array,
    B_x: jax.Array,
    B_w_r: jax.Array,
    B_w_gate: jax.Array,
    B_w_up: jax.Array,
    B_w_down: jax.Array,
):
    del B_x
    hbm = pl.BlockSpec(memory_space=pl.ANY)
    out = pl.pallas_call(
        _kernel,
        out_shape=jax.ShapeDtypeStruct((S, D), BF16),
        in_specs=[hbm] * 8,
        out_specs=hbm,
        scratch_shapes=[
            pltpu.VMEM((S, D), BF16),
            pltpu.VMEM((S // 2, D), U32),
            pltpu.VMEM((3 * NC, D, RC), BF16),
            [pltpu.VMEM((D // 2, D), U32)] * 3,
            pltpu.VMEM((H, DH, DH), BF16),
            pltpu.VMEM((8 * 64, 128), U32),
            pltpu.VMEM((D, D), BF16),
            pltpu.VMEM((D // 2, D), U32),
            pltpu.VMEM((D,), BF16),
            pltpu.VMEM((8, D), F32),
            pltpu.VMEM((NPAIR, 64, 128), F32),
            pltpu.VMEM((NPAIR * 32, 128), U32),
            pltpu.VMEM((NPAIR, 128, T), F32),
            pltpu.VMEM((NPAIR, 128, 128), F32),
            [pltpu.VMEM((NPAIR * 64, T), U32)] * 2,
            pltpu.VMEM((TH, D), F32),
            pltpu.VMEM((TH, D), F32),
            pltpu.VMEM((S // 2, D), U32),
            pltpu.VMEM((S, D), BF16),
            pltpu.VMEM((D, FF), BF16),
            pltpu.VMEM((D, FF), BF16),
            pltpu.VMEM((FF, D + WD_PAD), BF16),
            pltpu.VMEM((D // 2, FM), U32),
            pltpu.VMEM((D // 2, FM), U32),
            pltpu.VMEM((FM // 2, D), U32),
            pltpu.VMEM((16, D), BF16),
            pltpu.SemaphoreType.DMA((6 + 3 * NC + NT_ + 9,)),
        ],
        compiler_params=pltpu.CompilerParams(vmem_limit_bytes=100 * 1024 * 1024,
                                             disable_semaphore_checks=True, disable_bounds_checks=True),
        name="hedgehog_mod",
    )(
        A_x.reshape(S, D),
        A_wqkv,
        A_w_phi,
        A_wo,
        B_w_r,
        B_w_gate,
        B_w_up,
        B_w_down,
    )
    return out.reshape(1, S, D)
```

```python
import math

import jax
import jax.numpy as jnp
from jax import lax
import jax.experimental.pallas as pl
import jax.experimental.pallas.tpu as pltpu

F32 = jnp.float32
BF16 = jnp.bfloat16
U32 = jnp.uint32

S = 2048
D = 1024
H = 32
DH = 32
FF = 3584
NPAIR = H // 2
LOG2E = 1.4426950408889634
LN_EPS = 1e-5

T = 256
TH = T // 2
NT_ = S // T
RC = 256
NC = D // RC
PPC = RC // 64
LNC = 16
WD_PAD = 128

FV = 8 * 128
FM = FF - FV
WO_ROWS = 352
UNROLL2 = 2


def _spread(n, a, b, due=None):
    rel = [round(a + (b - a) * k / (n - 1), 3) for k in range(n)]
    return tuple((r, None if due is None else math.ceil(r) + due) for r in rel)


LN1_PLAN = _spread(16, 0, 12, 3)
WO_PLAN = _spread(11, 3, 13)
Z_PLAN = _spread(16, 6, 14, 2)
PRO_LN1_PLAN = ((None, None),) * 16
PRO_K_PLAN = _spread(8, 0, 6)
PRO_V_PLANS = (_spread(8, 0, 12), _spread(16, 13, 24)[:8], _spread(16, 13, 24)[8:], _spread(16, 0.7, 28, 3))
LN2B_PLAN = ((None, 0), (None, 0), (None, 0), (2.166, 8), (3.769, 9), (5.524, 11), (7.081, 13), (9.164, 15))
LN2A_PLAN = ((None, 18),) + _spread(7, 15.6, 20, 3)
PACK_PLAN = _spread(16, 100, 115) + _spread(16, 99.1, 114.1) + _spread(20, 0, 21)
G3_AT = 4
MOE_NA = 34
MOE_ND = 2
STAGGER = 8

NN = (((1,), (0,)), ((), ()))
NT = (((1,), (1,)), ((), ()))


def _dot(a, b, dims):
    return lax.dot_general(a, b, dims, preferred_element_type=F32)


def _recip(x):
    return pl.reciprocal(x, approx=False, full_range=False)


def _pack(x):
    return pltpu.bitcast(x, U32)


def _unpack(x):
    return pltpu.bitcast(x, BF16)


def _pair_allreduce(a, op):
    a = op(a, pltpu.roll(a, 2, 0))
    return op(a, pltpu.roll(a, 4, 0))


def _tree(op, xs):
    xs = list(xs)
    while len(xs) > 1:
        nxt = [op(xs[i], xs[i + 1]) for i in range(0, len(xs) - 1, 2)]
        if len(xs) % 2:
            nxt.append(xs[-1])
        xs = nxt
    return xs[0]


def _dual_exp(p):
    sl = [p[8 * i:8 * i + 8, :] for i in range(8)]
    mx = _pair_allreduce(_tree(jnp.maximum, sl), jnp.maximum)
    mn = _pair_allreduce(_tree(jnp.minimum, sl), jnp.minimum)
    ep = [jnp.exp2(s - mx) for s in sl]
    en = [jnp.exp2(mn - s) for s in sl]
    sp = _pair_allreduce(_tree(jnp.add, ep), jnp.add)
    sn = _pair_allreduce(_tree(jnp.add, en), jnp.add)
    return ep, en, sp, sn


def _after(x, never, anchor):
    if anchor is None:
        return x
    d = jnp.concatenate([anchor] * (x.shape[0] // 8), axis=0)
    if x.shape[1] == 128:
        return jnp.where(never, d, x)
    return jnp.concatenate([jnp.where(never, d, x[:, :128]), x[:, 128:]], axis=1)


def _gate(x, never, deps):
    for i, dep in enumerate(deps):
        d = jnp.broadcast_to(dep, (8, 128))
        if x.dtype != F32:
            d = pltpu.bitcast(d, x.dtype)
        blk = jnp.where(never, d, x[8 * i:8 * i + 8, :128])
        if x.shape[1] > 128:
            blk = jnp.concatenate([blk, x[8 * i:8 * i + 8, 128:]], axis=1)
        parts = ([x[:8 * i, :]] if i else []) + [blk, x[8 * i + 8:, :]]
        x = jnp.concatenate(parts, axis=0)
    return x


def _lane_fold(a):
    return _tree(jnp.add, [a[:, 128 * i:128 * i + 128] for i in range(a.shape[1] // 128)])


def _row_sum(a):
    return jnp.sum(_lane_fold(a), axis=-1, keepdims=True)


def _lane_tile(a, n):
    return a if n == 1 else jnp.concatenate([a] * n, axis=1)


def _sublane_allreduce(a):
    a = a + pltpu.roll(a, 4, 0)
    a = a + pltpu.roll(a, 2, 0)
    return a + pltpu.roll(a, 1, 0)


def _col_broadcast(row8):
    return jnp.concatenate([row8] * 16, axis=0).astype(BF16).T.astype(F32)


def _vpu_matvec(xb, w_rows, never, anchors, lag):
    ng = xb.shape[0] // 8
    acc, hist = None, []
    for g in range(ng):
        dep = anchors[(g * len(anchors)) // ng]
        if g >= lag:
            dep = dep + hist[g - lag]
        x = jnp.where(never, dep, xb[8 * g:8 * g + 8, :])
        w = w_rows(g)
        t = w * _lane_tile(x, w.shape[1] // 128)
        acc = t if acc is None else acc + t
        hist.append(acc[:, -128:])
    return acc


class _Side:
    def __init__(self, never):
        self.never = never
        self.jobs = []
        self.deps = {}

    def add(self, plan, fn):
        for k, (rel, due) in enumerate(plan):
            if rel is None:
                self._run(due, fn, k, None)
            else:
                self.jobs.append((rel, due, fn, k))

    def _run(self, due, fn, k, anchor):
        dep = fn(k, anchor)
        if due is not None:
            self.deps.setdefault(due, []).append(dep)

    def check(self):
        assert not self.jobs and not self.deps, (self.jobs, self.deps)

    def gate(self, step, x):
        return _gate(x, self.never, self.deps.pop(step, []))

    def done(self, step, res):
        m = res.shape[0] // 8
        for job in sorted([j for j in self.jobs if step - 1 < j[0] <= step], key=lambda j: j[0]):
            self.jobs.remove(job)
            g = m - 1 - int((step - job[0]) * m)
            self._run(job[1], job[2], job[3], res[8 * g:8 * g + 8, res.shape[1] - 128:])


def _kernel(x_hbm, wqkv_hbm, wphi_hbm, wo_hbm, wr_hbm, wg_hbm, wu_hbm, wd_hbm, out_hbm,
            x_v, xn_v, wraw_v, wt_v, wphi_v, a_v, woraw_v, wo_v, wrraw_v, wr_v, kvacc_v, kvbf_v,
            z_v, zb_v, phi_v, ha_v, hb_v, hn_v, o_v, wg_v, wu_v, wd_v, wgp_v, wup_v, wdp_v, patch_v,
            sem):
    SX, SW, SO, SM = 0, 6, 6 + 3 * NC, 6 + 3 * NC + NT_ + 1

    def x_copy(i):
        h0, h1 = ((1, 2), (2, 4), (4, 6), (6, 10), (10, 2 * NT_), (0, 1))[i]
        rows = pl.ds(h0 * TH, (h1 - h0) * TH)
        return pltpu.make_async_copy(x_hbm.at[rows, :], x_v.at[rows, :], sem.at[SX + i])

    def k0_copy(s):
        return pltpu.make_async_copy(wqkv_hbm.at[:, pl.ds(D + s * 128, 128)],
                                     wraw_v.at[NC, :, pl.ds(s * 128, 128)], sem.at[(SM + 7, SW + NC)[s]])

    def w_copy(j, c):
        return pltpu.make_async_copy(wqkv_hbm.at[:, pl.ds(j * D + c * RC, RC)], wraw_v.at[j * NC + c],
                                     sem.at[SW + j * NC + c])

    def wphi_copy(i):
        h0, h1 = ((0, 8), (8, 16), (16, H))[i]
        return pltpu.make_async_copy(wphi_hbm.at[pl.ds(h0, h1 - h0)], wphi_v.at[pl.ds(h0, h1 - h0)],
                                     sem.at[(SM + 4, SM + 8, SM + 9)[i]])

    wr_copy = pltpu.make_async_copy(wr_hbm, wrraw_v, sem.at[SM + 5])
    wo_copy = pltpu.make_async_copy(wo_hbm, woraw_v, sem.at[SM + 6])
    wg_copy = pltpu.make_async_copy(wg_hbm, wg_v, sem.at[SM + 0])
    wu_copy = pltpu.make_async_copy(wu_hbm, wu_v, sem.at[SM + 1])
    wd_copy = pltpu.make_async_copy(wd_hbm, wd_v.at[:, pl.ds(0, D)], sem.at[SM + 2])

    wphi_copy(0).start()
    k0_copy(0).start()
    x_copy(5).start()
    k0_copy(1).start()
    x_copy(0).start()
    wphi_copy(1).start()
    w_copy(1, 1).start()

    def view(ref, i, n, off=0):
        r0 = off + i * n
        return ref.at[pl.ds(r0 if isinstance(r0, int) else pl.multiple_of(r0, math.gcd(n, off)), n), :]

    def ln_rows(t, k, n, never=None, anchor=None):
        x = _after(view(x_v, t, T)[k * n:(k + 1) * n, :].astype(F32), never, anchor)
        xc = x - _row_sum(x) * (1.0 / D)
        rstd = lax.rsqrt(_row_sum(xc * xc) * (1.0 / D) + LN_EPS)
        view(xn_v, t, T // 2)[k * n // 2:(k + 1) * n // 2, :] = _pack((xc * rstd).astype(BF16))
        return _tree(jnp.add, [rstd[8 * i:8 * i + 8, :] for i in range(min(n, LNC) // 8)])

    def xn_tile(t):
        return _unpack(view(xn_v, t, T // 2)[...])

    def expand_wphi(c):
        w = wphi_v[8 * c:8 * c + 8].reshape(8 * DH, DH).astype(F32).T
        bits = pltpu.bitcast(w, U32)
        head = lax.broadcasted_iota(jnp.int32, (DH, 128), 1) >> 5
        for s in range(2):
            b = bits[:, 128 * s:128 * s + 128]
            for j in range(2):
                r0 = 64 * (2 * c + s) + 32 * j
                a_v[r0:r0 + 32, :] = jnp.where(head == 2 * j, b >> 16,
                                               jnp.where(head == 2 * j + 1, b, jnp.uint32(0)))

    wphi_copy(0).wait()
    expand_wphi(0)
    hb_v[...] = jnp.zeros((TH, D), F32)

    def fold(j, c, side=None, step0=None, slabs=range(RC // 128)):
        for s in slabs:
            g = c * (RC // 128) + s
            w = wraw_v[j * NC + c, :, s * 128:(s + 1) * 128]
            g0 = 64 * g if isinstance(g, int) else pl.multiple_of(64 * g, 64)
            if j == 2:
                wt = w.T
            else:
                res = _dot(_unpack(a_v[pl.ds(g0, 64), :]), w, NT)
                if side is not None:
                    side.done(step0 + 2 * s, res[:, :D // 2])
                    side.done(step0 + 2 * s + 1, res[:, D // 2:])
                wt = (res * LOG2E).astype(BF16)
            wt_v[j][pl.ds(g0, 64), :] = _pack(wt)

    def wt_rows(j, c):
        return wt_v[j][c * RC // 2:(c + 1) * RC // 2, :]

    def k_pair(p, slot, pr, c0, first, never=None):
        ep, en, sp, sn = _dual_exp(p)
        inv = _recip(sp * sn)
        scale = (sn * inv, sp * inv)
        es = ep + en
        cols = slice(c0, c0 + p.shape[1])
        n = 16 if never is None else 16 // STAGGER
        last = None
        for q in range(16 // n):
            sc = scale
            if last is not None:
                sc = [jnp.where(never, last, x) for x in scale]
            phi = jnp.concatenate([es[i] * sc[i // 8] for i in range(q * n, (q + 1) * n)], axis=0)
            rows = slice(8 * q * n, 8 * (q + 1) * n)
            z = phi if first else z_v[pr, rows, cols] + phi
            z_v[pr, rows, cols] = z
            phi_v[slot][64 * pr + 4 * q * n:64 * pr + 4 * (q + 1) * n, cols] = _pack(phi.astype(BF16))
            last = z[8 * n - 8:, :]

    def k_features(pk, slot, c, first, never=None):
        for j in range(PPC):
            k_pair(pk[64 * j:64 * j + 64, :], slot, c * PPC + j, 0, first, never)

    row = lax.broadcasted_iota(jnp.int32, (64, 128), 0)
    col = lax.broadcasted_iota(jnp.int32, (64, 128), 1)
    kv_keep = (row >> 5) == (col & 1)

    def kv_update(vt, slot, c, first, publish=False):
        for j in range(PPC):
            pr = c * PPC + j
            upd = _dot(vt[64 * j:64 * j + 64, :].astype(BF16), _unpack(phi_v[slot][64 * pr:64 * pr + 64, :]), NT)
            acc = upd if first else kvacc_v[pr] + upd
            kvacc_v[pr] = acc
            if publish:
                kvbf_v[32 * pr:32 * pr + 32, :] = _pack(jnp.where(kv_keep, acc, 0.0).astype(BF16))

    def proj(j, c, xn):
        return proj_steps(_Side(None), 0, j, c, xn)

    def proj_steps(side, step0, j, c, xn):
        w = wt_rows(j, c)
        quarters = []
        for n in range(2):
            for m in range(2):
                step = step0 + 2 * n + m
                wq = side.gate(step, w[m * (RC // 4):(m + 1) * (RC // 4), :])
                res = _dot(_unpack(wq), xn[n * TH:(n + 1) * TH, :], NT)
                side.done(step, res)
                quarters.append(res)
        return jnp.concatenate(
            [jnp.concatenate([quarters[0], quarters[2]], axis=1),
             jnp.concatenate([quarters[1], quarters[3]], axis=1)], axis=0)

    def pack_rows(src, dst, r0, rows, c0, cols, never, a):
        w = _pack(src[r0:r0 + rows, c0:c0 + cols])
        d = jnp.concatenate([_lane_tile(pltpu.bitcast(a, U32), cols // 128)] * (rows // 16), axis=0)
        dst[r0 // 2:(r0 + rows) // 2, c0:c0 + cols] = jnp.where(never, d, w)

    def stash(i, val):
        for q in range(4):
            zb_v[4 * i + q] = val[128 * (q // 2):128 * (q // 2) + 128, 128 * (q % 2):128 * (q % 2) + 128]

    def stashed_k(i, slot, c, first):
        def job(k, a):
            j, n = k // 2, k % 2
            p = zb_v[4 * i + 2 * (j // 2) + n, 64 * (j % 2):64 * (j % 2) + 64, :]
            p = jnp.concatenate([_after(p[0:8, :], never0, a), p[8:, :]], axis=0)
            k_pair(p, slot, c * PPC + j, 128 * n, first, never0)
        return job

    def quarter(m, n):
        xn = _unpack(xn_v[n * TH // 2:(n + 1) * TH // 2, :])
        zb_v[2 * m + n] = _dot(_unpack(wt_v[1][64 * m:64 * m + 64, :]), xn, NT)

    k0_copy(0).wait()
    x_copy(5).wait()
    wphi_copy(2).start()
    w_copy(1, 2).start()
    x_copy(1).start()
    fold(1, 0, slabs=(0,))
    never0 = ln_rows(0, 0, TH)[0, 0] < 0.0
    quarter(0, 0)

    k0_copy(1).wait()
    x_copy(0).wait()
    wphi_copy(1).wait()
    w_copy(1, 3).start()
    for c in range(NC):
        w_copy(2, c).start()
    fold(1, 0, slabs=(1,))
    ln_rows(0, 1, TH)
    quarter(1, 0)
    quarter(0, 1)
    quarter(1, 1)
    expand_wphi(1)

    for c in (1, 2):
        w_copy(1, c).wait()
        if c == 1:
            wphi_copy(2).wait()
            expand_wphi(2)
            expand_wphi(3)
            x_copy(2).start()
            for cq in range(NC):
                w_copy(0, cq).start()
        else:
            x_copy(3).start()
            wo_copy.start()
            wr_copy.start()
            x_copy(4).start()
        side = _Side(never0)
        side.add(PRO_K_PLAN, stashed_k(c - 1, 0, c - 1, True))
        fold(1, c, side, 0)
        stash(c, proj_steps(side, 4, 1, c, xn_tile(0)))
        side.check()

    x_copy(1).wait()
    w_copy(1, 3).wait()
    wg_copy.start()
    wu_copy.start()
    wd_copy.start()
    side = _Side(never0)
    side.add(PRO_LN1_PLAN, lambda k, a: ln_rows(1, k, LNC, never0, a))
    fold(1, 3, side, 0)
    stash(3, proj_steps(side, 4, 1, 3, xn_tile(0)))
    xn1 = xn_tile(1)
    for c in range(3):
        k_features(proj(1, c, xn1), 1, c, c == 2, never0)
    stash(0, proj(1, 3, xn1))

    for c in range(NC):
        w_copy(2, c).wait()
    x_copy(2).wait()
    w_copy(0, 0).wait()
    side = _Side(never0)
    side.add(PRO_V_PLANS[0], stashed_k(2, 0, 2, False))
    side.add(PRO_V_PLANS[1], stashed_k(3, 0, 3, True))
    side.add(PRO_V_PLANS[2], stashed_k(0, 1, 3, False))
    side.add(PRO_V_PLANS[3], lambda k, a: ln_rows(2, k, LNC, never0, a))
    fold(0, 0)
    xns = (xn_tile(0), xn_tile(1))
    pending = None
    for c in range(NC):
        fold(2, c)
        for i in range(2):
            vt = proj_steps(side, 8 * c + 4 * i, 2, c, xns[i])
            if pending is not None:
                kv_update(*pending)
            pending = (vt, i, c, i == 0)
    side.check()
    kv_update(*pending)

    def phase1(u, carry):
        never = u < 0

        @pl.when(u == 0)
        def _():
            for c in range(1, NC):
                w_copy(0, c).wait()
            x_copy(3).wait()
            wo_copy.wait()
            wr_copy.wait()

        @pl.when(u == 1)
        def _():
            x_copy(4).wait()

        pending = None
        for i in range(2):
            t = 2 * u + 2 + i
            tn = jnp.minimum(t + 1, NT_ - 1)
            side = _Side(never)
            xn = xn_tile(t)
            for c in range(NC):
                pk = proj(1, c, xn)
                if c == 0 and pending is not None:
                    kv_update(*pending)
                k_features(pk, i, c, False)
            side.add(LN1_PLAN, lambda k, a: ln_rows(tn, k, LNC, never, a))
            if i == 0:
                def pack_wo(k, a):
                    rows = WO_ROWS // len(WO_PLAN)
                    w0 = u * ((D - WO_ROWS) // 2)
                    src = woraw_v.at[pl.ds(pl.multiple_of(w0, 16), WO_ROWS), :]
                    dst = wo_v.at[pl.ds(pl.multiple_of(w0 // 2, 8), WO_ROWS // 2), :]
                    pack_rows(src, dst, k * rows, rows, 0, D, never, a)
                side.add(WO_PLAN, pack_wo)
            else:
                def z_final(k, a):
                    z = _after(z_v[k], never, a)
                    zs = _row_sum(z)
                    zb_v[k] = jnp.broadcast_to(zs, (128, 128))
                    return zs[120:128, :]
                side.add(Z_PLAN, z_final)
            side.done(0, pk)
            vts = []
            for c in range(NC):
                vts.append(proj_steps(side, 4 * c + 1, 2, c, xn))
                if c > 0:
                    kv_update(vts[c - 1], i, c - 1, False, i == 1)
            pending = (vts[NC - 1], i, NC - 1, False, i == 1)
            side.check()
        fold(0, u + 1)
        kv_update(*pending)
        wr_v[...] = jnp.broadcast_to(wrraw_v[...].reshape(1, D).astype(F32), (8, D))
        return carry

    lax.fori_loop(0, (NT_ - 2) // 2, phase1, 0)

    def o_copy(r0, n, i):
        return pltpu.make_async_copy(o_v.at[pl.ds(r0, n), :], out_hbm.at[pl.ds(r0, n), :], sem.at[SO + i])

    def finish_rows(h_ref, k, ht, valid, st, never=None, anchor=None):
        r0 = ht * TH + k * LNC
        best, besti = st["route"]
        wr = jnp.concatenate([wr_v[...]] * (LNC // 8), axis=0)
        sub = lax.broadcasted_iota(jnp.int32, (8, 1), 0)
        h = _after(h_ref[k * LNC:(k + 1) * LNC, :], never, anchor)
        hc = h - _row_sum(h) * (1.0 / D)
        rstd = lax.rsqrt(_row_sum(hc * hc) * (1.0 / D) + LN_EPS)
        r = (_row_sum(hc * wr) * rstd).astype(BF16).astype(F32)
        hn = hc * rstd
        view(hn_v, ht, TH // 2)[k * LNC // 2:(k + 1) * LNC // 2, :] = _pack(hn.astype(BF16))
        view(o_v, ht, TH)[k * LNC:(k + 1) * LNC, :] = (hn + h).astype(BF16)
        if valid is not None:
            r = jnp.where(valid, r, -jnp.inf)
        for i in range(LNC // 8):
            ri = r[8 * i:8 * i + 8, :]
            better = ri > best
            best = jnp.where(better, ri, best)
            besti = jnp.where(better, sub + (r0 + 8 * i), besti)
        st["route"] = (best, besti)
        return best

    def q_features(pq, slot, c):
        for j in range(PPC):
            pr = c * PPC + j
            ep, en, sp, sn = _dual_exp(pq[64 * j:64 * j + 64, :])
            zz = [_lane_tile(zb_v[pr, 8 * i:8 * i + 8, :], pq.shape[1] // 128) for i in range(16)]
            ap = _pair_allreduce(_tree(jnp.add, [ep[i] * zz[i] for i in range(8)]), jnp.add)
            an = _pair_allreduce(_tree(jnp.add, [en[i] * zz[8 + i] for i in range(8)]), jnp.add)
            inv = _recip(ap * sn + (an + 1e-6 * sn) * sp)
            rp = sn * inv
            rn = sp * inv
            phi = jnp.concatenate([e * rp for e in ep] + [e * rn for e in en], axis=0)
            phi_v[slot][64 * pr:64 * pr + 64, :] = _pack(phi.astype(BF16))

    def attn_rows(slot, c, lo, hi):
        res = jnp.concatenate(
            [_dot(_unpack(kvbf_v[32 * pr:32 * pr + 32, :]), _unpack(phi_v[slot][64 * pr:64 * pr + 64, lo:hi]), NN)
             for pr in range(c * PPC, (c + 1) * PPC)], axis=0)
        return res.astype(BF16).T

    def out_proj(side, step0, o, k0, k1, n0=0, n1=D // 128):
        cols = []
        for n in range(n0, n1):
            w = side.gate(step0 + n, wo_v[k0 // 2:k1 // 2, n * 128:(n + 1) * 128])
            res = _dot(o, _unpack(w), NN)
            side.done(step0 + n, res)
            cols.append(res)
        return jnp.concatenate(cols, axis=1)

    def phase2(u, carry):
        for i in range(UNROLL2):
            carry = phase2_tile(u * UNROLL2 + i, i % 2, carry, u < 0)

        r0 = pl.multiple_of(u * (UNROLL2 * T), T)

        @pl.when(u == 0)
        def _():
            o_copy(0, UNROLL2 * T - TH, 0).start()

        @pl.when(u > 0)
        def _():
            o_copy(pl.multiple_of(jnp.maximum(r0 - TH, 0), TH), UNROLL2 * T, u).start()

        return carry

    def phase2_tile(t, slot, carry, never):
        hp = jnp.maximum(2 * t - 1, 0)
        side = _Side(never)
        st = {"route": carry}
        side.add(LN2B_PLAN, lambda k, a: finish_rows(hb_v, k, hp, t > 0, st, side.never, a))

        def pack_ffn(k, a):
            if k < 32:
                n = D // NT_
                pack_rows(view((wg_v, wu_v)[k % 2], t, n), view((wgp_v, wup_v)[k % 2], t, n // 2),
                          (k // 4) * 16, 16, (k // 2 % 2) * (FM // 2), FM // 2, never, a)
            else:
                n = FM // NT_
                pack_rows(view(wd_v, t, n, FV), view(wdp_v, t, n // 2), (k - 32) * 16, 16, 0, D, never, a)
        side.add(PACK_PLAN, pack_ffn)

        xn = xn_tile(t)
        xt = view(x_v, t, T)
        os_ = []
        for c in range(NC):
            pq = proj_steps(side, 100 + 4 * c, 0, c, xn)
            if c == 0:
                pq = side.gate(0, pq)
            q_features(pq, slot, c)
            if c > 0:
                os_.append(attn_rows(slot, c - 1, 0, T))
        oa = jnp.concatenate([o[0:TH, :] for o in os_[:2]], axis=1)
        ha0 = out_proj(side, 0, oa, 0, D // 2, 0, G3_AT)
        os_.append(attn_rows(slot, NC - 1, 0, T))
        ha1 = out_proj(side, 0, oa, 0, D // 2, G3_AT, D // 128)
        ha = jnp.concatenate([ha0, ha1], axis=1) + xt[0:TH, :].astype(F32)
        ha_v[...] = ha + out_proj(side, 8, jnp.concatenate([o[0:TH, :] for o in os_[2:]], axis=1), D // 2, D)
        side.add(LN2A_PLAN, lambda k, a: finish_rows(ha_v, k, 2 * t, None, st, side.never, a))
        ob = jnp.concatenate([o[TH:T, :] for o in os_], axis=1)
        hb_v[...] = xt[TH:T, :].astype(F32) + out_proj(side, 16, ob, 0, D)
        side.check()
        return st["route"]

    wg_copy.wait()
    wu_copy.wait()
    wd_copy.wait()
    route = lax.fori_loop(
        0, NT_ // UNROLL2, phase2,
        (jnp.full((8, 1), -jnp.inf, F32), jnp.zeros((8, 1), jnp.int32)))
    st = {"route": route}
    for k in range(TH // LNC):
        finish_rows(hb_v, k, 2 * NT_ - 1, None, st)
    best, besti = st["route"]
    o_copy(S - TH, TH, NT_).start()

    rmax = jnp.max(best, axis=0, keepdims=True)
    idx = jnp.min(jnp.where(best == rmax, besti, S), axis=0, keepdims=True)
    idx_s = jnp.clip(idx[0, 0], 0, S - 1)
    blk = pl.multiple_of((idx_s >> 4) << 4, 16)
    pair = jnp.broadcast_to(hn_v[pl.ds(idx_s >> 1, 1), :], (8, D))
    x8 = pltpu.bitcast(jnp.where((idx_s & 1) == 1, pair & jnp.uint32(0xFFFF0000), pair << 16), F32)
    xs = jnp.concatenate([x8, x8], axis=0).astype(BF16)
    acts, anchors = [], []
    for c0 in range(0, FM, 128):
        g = _dot(xs, _unpack(wgp_v[:, c0:c0 + 128]), NN)[0:8, :]
        u = _dot(xs, _unpack(wup_v[:, c0:c0 + 128]), NN)[0:8, :]
        anchors += [g, u]
        acts.append(g * jax.nn.sigmoid(g) * u)
    gu = _sublane_allreduce(_vpu_matvec(
        _col_broadcast(x8),
        lambda g: jnp.concatenate([w[8 * g:8 * g + 8, FM:FF].astype(F32) for w in (wg_v, wu_v)], axis=1),
        never0, anchors[:MOE_NA], 1))
    g, u = gu[:, :FV], gu[:, FV:]
    acts.append(g * jax.nn.sigmoid(g) * u)
    a = jnp.concatenate(acts, axis=1)
    am = jnp.concatenate([a[:, FV:], a[:, FV:]], axis=0).astype(BF16)
    ys, anchors = [], anchors[MOE_NA:]
    for k0 in range(0, FM, 512):
        yk = _dot(am[:, k0:k0 + 512], _unpack(wdp_v[k0 // 2:k0 // 2 + 256, :]), NN)[0:8, :]
        ys.append(yk)
        anchors += [yk[:, c:c + 128] for c in range(128, D, 256)]
    ys.append(_sublane_allreduce(_vpu_matvec(
        _col_broadcast(a[:, :FV]), lambda g: wd_v[8 * g:8 * g + 8, 0:D].astype(F32), never0, anchors[:-MOE_ND], 2)))
    y = _tree(jnp.add, ys) * jax.nn.sigmoid(rmax)
    y = jnp.concatenate([y, y], axis=0)
    sel = lax.broadcasted_iota(jnp.int32, (16, 1), 0) == (idx_s - blk)
    patch_v[...] = (o_v[pl.ds(blk, 16), :].astype(F32) + jnp.where(sel, y, 0.0)).astype(BF16)
    o_copy(0, UNROLL2 * T - TH, 0).wait()
    for u in range(1, NT_ // UNROLL2):
        o_copy(u * UNROLL2 * T - TH, UNROLL2 * T, u).wait()
    o_copy(S - TH, TH, NT_).wait()
    pc = pltpu.make_async_copy(patch_v, out_hbm.at[pl.ds(blk, 16), :], sem.at[SM + 3])
    pc.start()
    pc.wait()


@jax.jit
def pallas_sequential_preLN__linear_kernel_hedgehog__moe_arch_mod__prompt_kernel(
    A_x: jax.Array,
    A_wqkv: jax.Array,
    A_w_phi: jax.Array,
    A_wo: jax.Array,
    B_x: jax.Array,
    B_w_r: jax.Array,
    B_w_gate: jax.Array,
    B_w_up: jax.Array,
    B_w_down: jax.Array,
):
    del B_x
    hbm = pl.BlockSpec(memory_space=pl.ANY)
    out = pl.pallas_call(
        _kernel,
        out_shape=jax.ShapeDtypeStruct((S, D), BF16),
        in_specs=[hbm] * 8,
        out_specs=hbm,
        scratch_shapes=[
            pltpu.VMEM((S, D), BF16),
            pltpu.VMEM((S // 2, D), U32),
            pltpu.VMEM((3 * NC, D, RC), BF16),
            [pltpu.VMEM((D // 2, D), U32)] * 3,
            pltpu.VMEM((H, DH, DH), BF16),
            pltpu.VMEM((8 * 64, 128), U32),
            pltpu.VMEM((D, D), BF16),
            pltpu.VMEM((D // 2, D), U32),
            pltpu.VMEM((D,), BF16),
            pltpu.VMEM((8, D), F32),
            pltpu.VMEM((NPAIR, 64, 128), F32),
            pltpu.VMEM((NPAIR * 32, 128), U32),
            pltpu.VMEM((NPAIR, 128, T), F32),
            pltpu.VMEM((NPAIR, 128, 128), F32),
            [pltpu.VMEM((NPAIR * 64, T), U32)] * 2,
            pltpu.VMEM((TH, D), F32),
            pltpu.VMEM((TH, D), F32),
            pltpu.VMEM((S // 2, D), U32),
            pltpu.VMEM((S, D), BF16),
            pltpu.VMEM((D, FF), BF16),
            pltpu.VMEM((D, FF), BF16),
            pltpu.VMEM((FF, D + WD_PAD), BF16),
            pltpu.VMEM((D // 2, FM), U32),
            pltpu.VMEM((D // 2, FM), U32),
            pltpu.VMEM((FM // 2, D), U32),
            pltpu.VMEM((16, D), BF16),
            pltpu.SemaphoreType.DMA((6 + 3 * NC + NT_ + 11,)),
        ],
        compiler_params=pltpu.CompilerParams(vmem_limit_bytes=100 * 1024 * 1024,
                                             disable_semaphore_checks=True, disable_bounds_checks=True),
        name="hedgehog_mod",
    )(
        A_x.reshape(S, D),
        A_wqkv,
        A_w_phi,
        A_wo,
        B_w_r,
        B_w_gate,
        B_w_up,
        B_w_down,
    )
    return out.reshape(1, S, D)
```

```python
import math

import jax
import jax.numpy as jnp
from jax import lax
import jax.experimental.pallas as pl
import jax.experimental.pallas.tpu as pltpu

F32 = jnp.float32
BF16 = jnp.bfloat16
U32 = jnp.uint32

S = 2048
D = 1024
H = 32
DH = 32
FF = 3584
NPAIR = H // 2
LOG2E = 1.4426950408889634
LN_EPS = 1e-5

T = 256
TH = T // 2
NT_ = S // T
RC = 256
NC = D // RC
PPC = RC // 64
LNC = 16
WD_PAD = 128

FV = 10 * 128
FM = FF - FV
FVD = 8 * 128
WO_ROWS = 352
UNROLL2 = 2


def _spread(n, a, b, due=None):
    rel = [round(a + (b - a) * k / (n - 1), 3) for k in range(n)]
    return tuple((r, None if due is None else math.ceil(r) + due) for r in rel)


LN1_PLAN = _spread(16, 0, 12, 3)
WO_PLAN = _spread(11, 3, 13)
Z_PLAN = _spread(16, 6, 14, 2)
PRO_LN1_PLAN = ((None, None),) * 16
PRO_K_PLAN = _spread(8, 0, 6)
PRO_V_PLANS = (_spread(8, 0, 12), _spread(16, 13, 24)[:8], _spread(16, 13, 24)[8:], _spread(16, 0.7, 28, 3))
LN2B_PLAN = ((None, 0), (None, 0), (None, 0), (2.166, 8), (3.769, 9), (5.524, 11), (7.081, 13), (9.164, 15))
LN2A_PLAN = ((None, 18),) + _spread(7, 15.6, 20, 3)
PACK_PLAN = _spread(16, 100, 115) + _spread(16, 99.1, 114.1) + _spread(20, 0, 21)
G3_AT = 4
MOE_NA = 36
MOE_ND = 3
MOE_LAG = 2
MOE_ROT = 1
MOE_PARK = 1
MOE_SPLIT = 3
STAGGER = 8

NN = (((1,), (0,)), ((), ()))
NT = (((1,), (1,)), ((), ()))


def _dot(a, b, dims):
    return lax.dot_general(a, b, dims, preferred_element_type=F32)


def _recip(x):
    return pl.reciprocal(x, approx=False, full_range=False)


def _pack(x):
    return pltpu.bitcast(x, U32)


def _unpack(x):
    return pltpu.bitcast(x, BF16)


def _pair_allreduce(a, op):
    a = op(a, pltpu.roll(a, 2, 0))
    return op(a, pltpu.roll(a, 4, 0))


def _tree(op, xs):
    xs = list(xs)
    while len(xs) > 1:
        nxt = [op(xs[i], xs[i + 1]) for i in range(0, len(xs) - 1, 2)]
        if len(xs) % 2:
            nxt.append(xs[-1])
        xs = nxt
    return xs[0]


def _dual_exp(p):
    sl = [p[8 * i:8 * i + 8, :] for i in range(8)]
    mx = _pair_allreduce(_tree(jnp.maximum, sl), jnp.maximum)
    mn = _pair_allreduce(_tree(jnp.minimum, sl), jnp.minimum)
    ep = [jnp.exp2(s - mx) for s in sl]
    en = [jnp.exp2(mn - s) for s in sl]
    sp = _pair_allreduce(_tree(jnp.add, ep), jnp.add)
    sn = _pair_allreduce(_tree(jnp.add, en), jnp.add)
    return ep, en, sp, sn


def _after(x, never, anchor):
    if anchor is None:
        return x
    d = jnp.concatenate([anchor] * (x.shape[0] // 8), axis=0)
    if x.shape[1] == 128:
        return jnp.where(never, d, x)
    return jnp.concatenate([jnp.where(never, d, x[:, :128]), x[:, 128:]], axis=1)


def _gate(x, never, deps):
    for i, dep in enumerate(deps):
        d = jnp.broadcast_to(dep, (8, 128))
        if x.dtype != F32:
            d = pltpu.bitcast(d, x.dtype)
        blk = jnp.where(never, d, x[8 * i:8 * i + 8, :128])
        if x.shape[1] > 128:
            blk = jnp.concatenate([blk, x[8 * i:8 * i + 8, 128:]], axis=1)
        parts = ([x[:8 * i, :]] if i else []) + [blk, x[8 * i + 8:, :]]
        x = jnp.concatenate(parts, axis=0)
    return x


def _lane_fold(a):
    return _tree(jnp.add, [a[:, 128 * i:128 * i + 128] for i in range(a.shape[1] // 128)])


def _row_sum(a):
    return jnp.sum(_lane_fold(a), axis=-1, keepdims=True)


def _lane_tile(a, n):
    return a if n == 1 else jnp.concatenate([a] * n, axis=1)


def _sublane_allreduce(a):
    a = a + pltpu.roll(a, 4, 0)
    a = a + pltpu.roll(a, 2, 0)
    return a + pltpu.roll(a, 1, 0)


def _col_broadcast(row8):
    return jnp.concatenate([row8] * 16, axis=0).astype(BF16).T.astype(F32)


def _vpu_matvec(xb, w_rows, never, anchors, lag):
    ng = xb.shape[0] // 8
    acc, hist = None, []
    for g in range(ng):
        dep = anchors[(g * len(anchors)) // ng]
        if g >= lag:
            dep = dep + hist[g - lag]
        x = jnp.where(never, dep, xb[8 * g:8 * g + 8, :])
        w = w_rows(g)
        t = w * _lane_tile(x, w.shape[1] // 128)
        acc = t if acc is None else acc + t
        c = 128 * ((g * MOE_ROT) % (w.shape[1] // 128))
        hist.append(acc[:, c:c + 128])
    return acc


class _Side:
    def __init__(self, never):
        self.never = never
        self.jobs = []
        self.deps = {}

    def add(self, plan, fn):
        for k, (rel, due) in enumerate(plan):
            if rel is None:
                self._run(due, fn, k, None)
            else:
                self.jobs.append((rel, due, fn, k))

    def _run(self, due, fn, k, anchor):
        dep = fn(k, anchor)
        if due is not None:
            self.deps.setdefault(due, []).append(dep)

    def check(self):
        assert not self.jobs and not self.deps, (self.jobs, self.deps)

    def gate(self, step, x):
        return _gate(x, self.never, self.deps.pop(step, []))

    def done(self, step, res):
        m = res.shape[0] // 8
        for job in sorted([j for j in self.jobs if step - 1 < j[0] <= step], key=lambda j: j[0]):
            self.jobs.remove(job)
            g = m - 1 - int((step - job[0]) * m)
            self._run(job[1], job[2], job[3], res[8 * g:8 * g + 8, res.shape[1] - 128:])


def _kernel(x_hbm, wqkv_hbm, wphi_hbm, wo_hbm, wr_hbm, wg_hbm, wu_hbm, wd_hbm, out_hbm,
            x_v, xn_v, wraw_v, wt_v, wphi_v, a_v, woraw_v, wo_v, wrraw_v, wr_v, kvacc_v, kvbf_v,
            z_v, zb_v, phi_v, ha_v, hb_v, hn_v, o_v, wg_v, wu_v, wd_v, wgp_v, wup_v, wdp_v, patch_v,
            sem):
    SX, SW, SO, SM = 0, 6, 6 + 3 * NC, 6 + 3 * NC + NT_ + 1

    def x_copy(i):
        h0, h1 = ((1, 2), (2, 4), (4, 6), (6, 10), (10, 2 * NT_), (0, 1))[i]
        rows = pl.ds(h0 * TH, (h1 - h0) * TH)
        return pltpu.make_async_copy(x_hbm.at[rows, :], x_v.at[rows, :], sem.at[SX + i])

    def k0_copy(s):
        return pltpu.make_async_copy(wqkv_hbm.at[:, pl.ds(D + s * 128, 128)],
                                     wraw_v.at[NC, :, pl.ds(s * 128, 128)], sem.at[(SM + 7, SW + NC)[s]])

    def w_copy(j, c):
        return pltpu.make_async_copy(wqkv_hbm.at[:, pl.ds(j * D + c * RC, RC)], wraw_v.at[j * NC + c],
                                     sem.at[SW + j * NC + c])

    def wphi_copy(i):
        h0, h1 = ((0, 8), (8, 16), (16, H))[i]
        return pltpu.make_async_copy(wphi_hbm.at[pl.ds(h0, h1 - h0)], wphi_v.at[pl.ds(h0, h1 - h0)],
                                     sem.at[(SM + 4, SM + 8, SM + 9)[i]])

    wr_copy = pltpu.make_async_copy(wr_hbm, wrraw_v, sem.at[SM + 5])
    wo_copy = pltpu.make_async_copy(wo_hbm, woraw_v, sem.at[SM + 6])
    wg_copy = pltpu.make_async_copy(wg_hbm, wg_v, sem.at[SM + 0])
    wu_copy = pltpu.make_async_copy(wu_hbm, wu_v, sem.at[SM + 1])
    wd_copy = pltpu.make_async_copy(wd_hbm, wd_v.at[:, pl.ds(0, D)], sem.at[SM + 2])

    wphi_copy(0).start()
    k0_copy(0).start()
    x_copy(5).start()
    k0_copy(1).start()
    x_copy(0).start()
    wphi_copy(1).start()
    w_copy(1, 1).start()

    def view(ref, i, n, off=0):
        r0 = off + i * n
        return ref.at[pl.ds(r0 if isinstance(r0, int) else pl.multiple_of(r0, math.gcd(n, off)), n), :]

    def ln_rows(t, k, n, never=None, anchor=None):
        x = _after(view(x_v, t, T)[k * n:(k + 1) * n, :].astype(F32), never, anchor)
        xc = x - _row_sum(x) * (1.0 / D)
        rstd = lax.rsqrt(_row_sum(xc * xc) * (1.0 / D) + LN_EPS)
        view(xn_v, t, T // 2)[k * n // 2:(k + 1) * n // 2, :] = _pack((xc * rstd).astype(BF16))
        return _tree(jnp.add, [rstd[8 * i:8 * i + 8, :] for i in range(min(n, LNC) // 8)])

    def xn_tile(t):
        return _unpack(view(xn_v, t, T // 2)[...])

    def expand_wphi(c):
        w = wphi_v[8 * c:8 * c + 8].reshape(8 * DH, DH).astype(F32).T
        bits = pltpu.bitcast(w, U32)
        head = lax.broadcasted_iota(jnp.int32, (DH, 128), 1) >> 5
        for s in range(2):
            b = bits[:, 128 * s:128 * s + 128]
            for j in range(2):
                r0 = 64 * (2 * c + s) + 32 * j
                a_v[r0:r0 + 32, :] = jnp.where(head == 2 * j, b >> 16,
                                               jnp.where(head == 2 * j + 1, b, jnp.uint32(0)))

    wphi_copy(0).wait()
    expand_wphi(0)
    hb_v[...] = jnp.zeros((TH, D), F32)

    def fold(j, c, side=None, step0=None, slabs=range(RC // 128)):
        for s in slabs:
            g = c * (RC // 128) + s
            w = wraw_v[j * NC + c, :, s * 128:(s + 1) * 128]
            g0 = 64 * g if isinstance(g, int) else pl.multiple_of(64 * g, 64)
            if j == 2:
                wt = w.T
            else:
                res = _dot(_unpack(a_v[pl.ds(g0, 64), :]), w, NT)
                if side is not None:
                    side.done(step0 + 2 * s, res[:, :D // 2])
                    side.done(step0 + 2 * s + 1, res[:, D // 2:])
                wt = (res * LOG2E).astype(BF16)
            wt_v[j][pl.ds(g0, 64), :] = _pack(wt)

    def wt_rows(j, c):
        return wt_v[j][c * RC // 2:(c + 1) * RC // 2, :]

    def k_pair(p, slot, pr, c0, first, never=None):
        ep, en, sp, sn = _dual_exp(p)
        inv = _recip(sp * sn)
        scale = (sn * inv, sp * inv)
        es = ep + en
        cols = slice(c0, c0 + p.shape[1])
        n = 16 if never is None else 16 // STAGGER
        last = None
        for q in range(16 // n):
            sc = scale
            if last is not None:
                sc = [jnp.where(never, last, x) for x in scale]
            phi = jnp.concatenate([es[i] * sc[i // 8] for i in range(q * n, (q + 1) * n)], axis=0)
            rows = slice(8 * q * n, 8 * (q + 1) * n)
            z = phi if first else z_v[pr, rows, cols] + phi
            z_v[pr, rows, cols] = z
            phi_v[slot][64 * pr + 4 * q * n:64 * pr + 4 * (q + 1) * n, cols] = _pack(phi.astype(BF16))
            last = z[8 * n - 8:, :]

    def k_features(pk, slot, c, first, never=None):
        for j in range(PPC):
            k_pair(pk[64 * j:64 * j + 64, :], slot, c * PPC + j, 0, first, never)

    row = lax.broadcasted_iota(jnp.int32, (64, 128), 0)
    col = lax.broadcasted_iota(jnp.int32, (64, 128), 1)
    kv_keep = (row >> 5) == (col & 1)

    def kv_update(vt, slot, c, first, publish=False):
        for j in range(PPC):
            pr = c * PPC + j
            upd = _dot(vt[64 * j:64 * j + 64, :].astype(BF16), _unpack(phi_v[slot][64 * pr:64 * pr + 64, :]), NT)
            acc = upd if first else kvacc_v[pr] + upd
            kvacc_v[pr] = acc
            if publish:
                kvbf_v[32 * pr:32 * pr + 32, :] = _pack(jnp.where(kv_keep, acc, 0.0).astype(BF16))

    def proj(j, c, xn):
        return proj_steps(_Side(None), 0, j, c, xn)

    def proj_steps(side, step0, j, c, xn):
        w = wt_rows(j, c)
        quarters = []
        for n in range(2):
            for m in range(2):
                step = step0 + 2 * n + m
                wq = side.gate(step, w[m * (RC // 4):(m + 1) * (RC // 4), :])
                res = _dot(_unpack(wq), xn[n * TH:(n + 1) * TH, :], NT)
                side.done(step, res)
                quarters.append(res)
        return jnp.concatenate(
            [jnp.concatenate([quarters[0], quarters[2]], axis=1),
             jnp.concatenate([quarters[1], quarters[3]], axis=1)], axis=0)

    def pack_rows(src, dst, r0, rows, c0, cols, never, a):
        w = _pack(src[r0:r0 + rows, c0:c0 + cols])
        d = jnp.concatenate([_lane_tile(pltpu.bitcast(a, U32), cols // 128)] * (rows // 16), axis=0)
        dst[r0 // 2:(r0 + rows) // 2, c0:c0 + cols] = jnp.where(never, d, w)

    def stash(i, val):
        for q in range(4):
            zb_v[4 * i + q] = val[128 * (q // 2):128 * (q // 2) + 128, 128 * (q % 2):128 * (q % 2) + 128]

    def stashed_k(i, slot, c, first):
        def job(k, a):
            j, n = k // 2, k % 2
            p = zb_v[4 * i + 2 * (j // 2) + n, 64 * (j % 2):64 * (j % 2) + 64, :]
            p = jnp.concatenate([_after(p[0:8, :], never0, a), p[8:, :]], axis=0)
            k_pair(p, slot, c * PPC + j, 128 * n, first, never0)
        return job

    def quarter(m, n):
        xn = _unpack(xn_v[n * TH // 2:(n + 1) * TH // 2, :])
        zb_v[2 * m + n] = _dot(_unpack(wt_v[1][64 * m:64 * m + 64, :]), xn, NT)

    k0_copy(0).wait()
    x_copy(5).wait()
    wphi_copy(2).start()
    w_copy(1, 2).start()
    x_copy(1).start()
    fold(1, 0, slabs=(0,))
    never0 = ln_rows(0, 0, TH)[0, 0] < 0.0
    quarter(0, 0)

    k0_copy(1).wait()
    x_copy(0).wait()
    wphi_copy(1).wait()
    w_copy(1, 3).start()
    for c in range(NC):
        w_copy(2, c).start()
    fold(1, 0, slabs=(1,))
    ln_rows(0, 1, TH)
    quarter(1, 0)
    quarter(0, 1)
    quarter(1, 1)
    expand_wphi(1)

    for c in (1, 2):
        w_copy(1, c).wait()
        if c == 1:
            wphi_copy(2).wait()
            expand_wphi(2)
            expand_wphi(3)
            x_copy(2).start()
            for cq in range(NC):
                w_copy(0, cq).start()
        else:
            x_copy(3).start()
            wo_copy.start()
            wr_copy.start()
            x_copy(4).start()
        side = _Side(never0)
        side.add(PRO_K_PLAN, stashed_k(c - 1, 0, c - 1, True))
        fold(1, c, side, 0)
        stash(c, proj_steps(side, 4, 1, c, xn_tile(0)))
        side.check()

    x_copy(1).wait()
    w_copy(1, 3).wait()
    wg_copy.start()
    wu_copy.start()
    wd_copy.start()
    side = _Side(never0)
    side.add(PRO_LN1_PLAN, lambda k, a: ln_rows(1, k, LNC, never0, a))
    fold(1, 3, side, 0)
    stash(3, proj_steps(side, 4, 1, 3, xn_tile(0)))
    xn1 = xn_tile(1)
    for c in range(3):
        k_features(proj(1, c, xn1), 1, c, c == 2, never0)
    stash(0, proj(1, 3, xn1))

    for c in range(NC):
        w_copy(2, c).wait()
    x_copy(2).wait()
    w_copy(0, 0).wait()
    side = _Side(never0)
    side.add(PRO_V_PLANS[0], stashed_k(2, 0, 2, False))
    side.add(PRO_V_PLANS[1], stashed_k(3, 0, 3, True))
    side.add(PRO_V_PLANS[2], stashed_k(0, 1, 3, False))
    side.add(PRO_V_PLANS[3], lambda k, a: ln_rows(2, k, LNC, never0, a))
    fold(0, 0)
    xns = (xn_tile(0), xn_tile(1))
    pending = None
    for c in range(NC):
        fold(2, c)
        for i in range(2):
            vt = proj_steps(side, 8 * c + 4 * i, 2, c, xns[i])
            if pending is not None:
                kv_update(*pending)
            pending = (vt, i, c, i == 0)
    side.check()
    kv_update(*pending)

    def phase1(u, carry):
        never = u < 0

        @pl.when(u == 0)
        def _():
            for c in range(1, NC):
                w_copy(0, c).wait()
            x_copy(3).wait()
            wo_copy.wait()
            wr_copy.wait()

        @pl.when(u == 1)
        def _():
            x_copy(4).wait()

        pending = None
        for i in range(2):
            t = 2 * u + 2 + i
            tn = jnp.minimum(t + 1, NT_ - 1)
            side = _Side(never)
            xn = xn_tile(t)
            for c in range(NC):
                pk = proj(1, c, xn)
                if c == 0 and pending is not None:
                    kv_update(*pending)
                k_features(pk, i, c, False)
            side.add(LN1_PLAN, lambda k, a: ln_rows(tn, k, LNC, never, a))
            if i == 0:
                def pack_wo(k, a):
                    rows = WO_ROWS // len(WO_PLAN)
                    w0 = u * ((D - WO_ROWS) // 2)
                    src = woraw_v.at[pl.ds(pl.multiple_of(w0, 16), WO_ROWS), :]
                    dst = wo_v.at[pl.ds(pl.multiple_of(w0 // 2, 8), WO_ROWS // 2), :]
                    pack_rows(src, dst, k * rows, rows, 0, D, never, a)
                side.add(WO_PLAN, pack_wo)
            else:
                def z_final(k, a):
                    z = _after(z_v[k], never, a)
                    zs = _row_sum(z)
                    zb_v[k] = jnp.broadcast_to(zs, (128, 128))
                    return zs[120:128, :]
                side.add(Z_PLAN, z_final)
            side.done(0, pk)
            vts = []
            for c in range(NC):
                vts.append(proj_steps(side, 4 * c + 1, 2, c, xn))
                if c > 0:
                    kv_update(vts[c - 1], i, c - 1, False, i == 1)
            pending = (vts[NC - 1], i, NC - 1, False, i == 1)
            side.check()
        fold(0, u + 1)
        kv_update(*pending)
        wr_v[...] = jnp.broadcast_to(wrraw_v[...].reshape(1, D).astype(F32), (8, D))
        return carry

    lax.fori_loop(0, (NT_ - 2) // 2, phase1, 0)

    def o_copy(r0, n, i):
        return pltpu.make_async_copy(o_v.at[pl.ds(r0, n), :], out_hbm.at[pl.ds(r0, n), :], sem.at[SO + i])

    def finish_rows(h_ref, k, ht, valid, st, never=None, anchor=None):
        r0 = ht * TH + k * LNC
        best, besti = st["route"]
        wr = jnp.concatenate([wr_v[...]] * (LNC // 8), axis=0)
        sub = lax.broadcasted_iota(jnp.int32, (8, 1), 0)
        h = _after(h_ref[k * LNC:(k + 1) * LNC, :], never, anchor)
        hc = h - _row_sum(h) * (1.0 / D)
        rstd = lax.rsqrt(_row_sum(hc * hc) * (1.0 / D) + LN_EPS)
        r = (_row_sum(hc * wr) * rstd).astype(BF16).astype(F32)
        hn = hc * rstd
        view(hn_v, ht, TH // 2)[k * LNC // 2:(k + 1) * LNC // 2, :] = _pack(hn.astype(BF16))
        view(o_v, ht, TH)[k * LNC:(k + 1) * LNC, :] = (hn + h).astype(BF16)
        if valid is not None:
            r = jnp.where(valid, r, -jnp.inf)
        for i in range(LNC // 8):
            ri = r[8 * i:8 * i + 8, :]
            better = ri > best
            best = jnp.where(better, ri, best)
            besti = jnp.where(better, sub + (r0 + 8 * i), besti)
        st["route"] = (best, besti)
        return best

    def q_features(pq, slot, c):
        for j in range(PPC):
            pr = c * PPC + j
            ep, en, sp, sn = _dual_exp(pq[64 * j:64 * j + 64, :])
            zz = [_lane_tile(zb_v[pr, 8 * i:8 * i + 8, :], pq.shape[1] // 128) for i in range(16)]
            ap = _pair_allreduce(_tree(jnp.add, [ep[i] * zz[i] for i in range(8)]), jnp.add)
            an = _pair_allreduce(_tree(jnp.add, [en[i] * zz[8 + i] for i in range(8)]), jnp.add)
            inv = _recip(ap * sn + (an + 1e-6 * sn) * sp)
            rp = sn * inv
            rn = sp * inv
            phi = jnp.concatenate([e * rp for e in ep] + [e * rn for e in en], axis=0)
            phi_v[slot][64 * pr:64 * pr + 64, :] = _pack(phi.astype(BF16))

    def attn_rows(slot, c, lo, hi):
        res = jnp.concatenate(
            [_dot(_unpack(kvbf_v[32 * pr:32 * pr + 32, :]), _unpack(phi_v[slot][64 * pr:64 * pr + 64, lo:hi]), NN)
             for pr in range(c * PPC, (c + 1) * PPC)], axis=0)
        return res.astype(BF16).T

    def out_proj(side, step0, o, k0, k1, n0=0, n1=D // 128):
        cols = []
        for n in range(n0, n1):
            w = side.gate(step0 + n, wo_v[k0 // 2:k1 // 2, n * 128:(n + 1) * 128])
            res = _dot(o, _unpack(w), NN)
            side.done(step0 + n, res)
            cols.append(res)
        return jnp.concatenate(cols, axis=1)

    def phase2(u, carry):
        for i in range(UNROLL2):
            carry = phase2_tile(u * UNROLL2 + i, i % 2, carry, u < 0)

        r0 = pl.multiple_of(u * (UNROLL2 * T), T)

        @pl.when(u == 0)
        def _():
            o_copy(0, UNROLL2 * T - TH, 0).start()

        @pl.when(u > 0)
        def _():
            o_copy(pl.multiple_of(jnp.maximum(r0 - TH, 0), TH), UNROLL2 * T, u).start()

        return carry

    def phase2_tile(t, slot, carry, never):
        hp = jnp.maximum(2 * t - 1, 0)
        side = _Side(never)
        st = {"route": carry}
        side.add(LN2B_PLAN, lambda k, a: finish_rows(hb_v, k, hp, t > 0, st, side.never, a))

        def pack_ffn(k, a):
            if k < 32:
                n = D // NT_
                pack_rows(view((wg_v, wu_v)[k % 2], t, n), view((wgp_v, wup_v)[k % 2], t, n // 2),
                          (k // 4) * 16, 16, (k // 2 % 2) * (FM // 2), FM // 2, never, a)
            else:
                n = (FF - FVD) // NT_
                pack_rows(view(wd_v, t, n, FVD), view(wdp_v, t, n // 2), (k - 32) * 16, 16, 0, D, never, a)
        side.add(PACK_PLAN[:32 + (FF - FVD) // 128], pack_ffn)

        xn = xn_tile(t)
        xt = view(x_v, t, T)
        os_ = []
        for c in range(NC):
            pq = proj_steps(side, 100 + 4 * c, 0, c, xn)
            if c == 0:
                pq = side.gate(0, pq)
            q_features(pq, slot, c)
            if c > 0:
                os_.append(attn_rows(slot, c - 1, 0, T))
        oa = jnp.concatenate([o[0:TH, :] for o in os_[:2]], axis=1)
        ha0 = out_proj(side, 0, oa, 0, D // 2, 0, G3_AT)
        os_.append(attn_rows(slot, NC - 1, 0, T))
        ha1 = out_proj(side, 0, oa, 0, D // 2, G3_AT, D // 128)
        ha = jnp.concatenate([ha0, ha1], axis=1) + xt[0:TH, :].astype(F32)
        ha_v[...] = ha + out_proj(side, 8, jnp.concatenate([o[0:TH, :] for o in os_[2:]], axis=1), D // 2, D)
        side.add(LN2A_PLAN, lambda k, a: finish_rows(ha_v, k, 2 * t, None, st, side.never, a))
        ob = jnp.concatenate([o[TH:T, :] for o in os_], axis=1)
        hb_v[...] = xt[TH:T, :].astype(F32) + out_proj(side, 16, ob, 0, D)
        side.check()
        return st["route"]

    wg_copy.wait()
    wu_copy.wait()
    wd_copy.wait()
    route = lax.fori_loop(
        0, NT_ // UNROLL2, phase2,
        (jnp.full((8, 1), -jnp.inf, F32), jnp.zeros((8, 1), jnp.int32)))
    st = {"route": route}
    for k in range(TH // LNC):
        finish_rows(hb_v, k, 2 * NT_ - 1, None, st)
    best, besti = st["route"]
    o_copy(S - TH, TH, NT_).start()

    rmax = jnp.max(best, axis=0, keepdims=True)
    idx = jnp.min(jnp.where(best == rmax, besti, S), axis=0, keepdims=True)
    idx_s = jnp.clip(idx[0, 0], 0, S - 1)
    blk = pl.multiple_of((idx_s >> 4) << 4, 16)
    pair = jnp.broadcast_to(hn_v[pl.ds(idx_s >> 1, 1), :], (8, D))
    x8 = pltpu.bitcast(jnp.where((idx_s & 1) == 1, pair & jnp.uint32(0xFFFF0000), pair << 16), F32)
    xs = jnp.concatenate([x8, x8], axis=0).astype(BF16)
    acts, anchors = [], []

    def park(v, half):
        if not MOE_PARK:
            return v
        n = v.shape[0] // 128
        for i in range(n):
            z_v[i, :, 128 * half:128 * half + 128] = v[128 * i:128 * i + 128, :]
        return jnp.concatenate([z_v[i, :, 128 * half:128 * half + 128] for i in range(n)], axis=0)

    for c0 in range(0, FM, 128):
        g = _dot(xs, _unpack(wgp_v[:, c0:c0 + 128]), NN)[0:8, :]
        u = _dot(xs, _unpack(wup_v[:, c0:c0 + 128]), NN)[0:8, :]
        anchors += [g, u]
        acts.append(g * jax.nn.sigmoid(g) * u)
    xb = park(_col_broadcast(x8), 0)
    if MOE_SPLIT:
        g, u = [_sublane_allreduce(_vpu_matvec(
            xb, lambda g: w[8 * g:8 * g + 8, FM:FF].astype(F32), never0,
            anchors[i * MOE_NA // 2:(i + 1) * MOE_NA // 2], MOE_SPLIT)) for i, w in enumerate((wg_v, wu_v))]
    else:
        gu = _sublane_allreduce(_vpu_matvec(
            xb, lambda g: jnp.concatenate([w[8 * g:8 * g + 8, FM:FF].astype(F32) for w in (wg_v, wu_v)], axis=1),
            never0, anchors[:MOE_NA], 1))
        g, u = gu[:, :FV], gu[:, FV:]
    acts.append(g * jax.nn.sigmoid(g) * u)
    a = jnp.concatenate(acts, axis=1)
    am = jnp.concatenate([a[:, FVD:], a[:, FVD:]], axis=0).astype(BF16)
    ys, anchors = [], anchors[MOE_NA:]
    for k0 in range(0, FF - FVD, 512):
        k1 = min(k0 + 512, FF - FVD)
        yk = _dot(am[:, k0:k1], _unpack(wdp_v[k0 // 2:k1 // 2, :]), NN)[0:8, :]
        ys.append(yk)
        anchors += [yk[:, c:c + 128] for c in range(128, D, 256)]
    ys.append(_sublane_allreduce(_vpu_matvec(
        park(_col_broadcast(a[:, :FVD]), 1), lambda g: wd_v[8 * g:8 * g + 8, 0:D].astype(F32), never0, anchors[:-MOE_ND], MOE_LAG)))
    y = _tree(jnp.add, ys) * jax.nn.sigmoid(rmax)
    y = jnp.concatenate([y, y], axis=0)
    sel = lax.broadcasted_iota(jnp.int32, (16, 1), 0) == (idx_s - blk)
    patch_v[...] = (o_v[pl.ds(blk, 16), :].astype(F32) + jnp.where(sel, y, 0.0)).astype(BF16)
    o_copy(0, UNROLL2 * T - TH, 0).wait()
    for u in range(1, NT_ // UNROLL2):
        o_copy(u * UNROLL2 * T - TH, UNROLL2 * T, u).wait()
    o_copy(S - TH, TH, NT_).wait()
    pc = pltpu.make_async_copy(patch_v, out_hbm.at[pl.ds(blk, 16), :], sem.at[SM + 3])
    pc.start()
    pc.wait()


@jax.jit
def pallas_sequential_preLN__linear_kernel_hedgehog__moe_arch_mod__prompt_kernel(
    A_x: jax.Array,
    A_wqkv: jax.Array,
    A_w_phi: jax.Array,
    A_wo: jax.Array,
    B_x: jax.Array,
    B_w_r: jax.Array,
    B_w_gate: jax.Array,
    B_w_up: jax.Array,
    B_w_down: jax.Array,
):
    del B_x
    hbm = pl.BlockSpec(memory_space=pl.ANY)
    out = pl.pallas_call(
        _kernel,
        out_shape=jax.ShapeDtypeStruct((S, D), BF16),
        in_specs=[hbm] * 8,
        out_specs=hbm,
        scratch_shapes=[
            pltpu.VMEM((S, D), BF16),
            pltpu.VMEM((S // 2, D), U32),
            pltpu.VMEM((3 * NC, D, RC), BF16),
            [pltpu.VMEM((D // 2, D), U32)] * 3,
            pltpu.VMEM((H, DH, DH), BF16),
            pltpu.VMEM((8 * 64, 128), U32),
            pltpu.VMEM((D, D), BF16),
            pltpu.VMEM((D // 2, D), U32),
            pltpu.VMEM((D,), BF16),
            pltpu.VMEM((8, D), F32),
            pltpu.VMEM((NPAIR, 64, 128), F32),
            pltpu.VMEM((NPAIR * 32, 128), U32),
            pltpu.VMEM((NPAIR, 128, T), F32),
            pltpu.VMEM((NPAIR, 128, 128), F32),
            [pltpu.VMEM((NPAIR * 64, T), U32)] * 2,
            pltpu.VMEM((TH, D), F32),
            pltpu.VMEM((TH, D), F32),
            pltpu.VMEM((S // 2, D), U32),
            pltpu.VMEM((S, D), BF16),
            pltpu.VMEM((D, FF), BF16),
            pltpu.VMEM((D, FF), BF16),
            pltpu.VMEM((FF, D + WD_PAD), BF16),
            pltpu.VMEM((D // 2, FM), U32),
            pltpu.VMEM((D // 2, FM), U32),
            pltpu.VMEM(((FF - FVD) // 2, D), U32),
            pltpu.VMEM((16, D), BF16),
            pltpu.SemaphoreType.DMA((6 + 3 * NC + NT_ + 11,)),
        ],
        compiler_params=pltpu.CompilerParams(vmem_limit_bytes=100 * 1024 * 1024,
                                             disable_semaphore_checks=True, disable_bounds_checks=True),
        name="hedgehog_mod",
    )(
        A_x.reshape(S, D),
        A_wqkv,
        A_w_phi,
        A_wo,
        B_w_r,
        B_w_gate,
        B_w_up,
        B_w_down,
    )
    return out.reshape(1, S, D)
```

```python
import math

import jax
import jax.numpy as jnp
from jax import lax
import jax.experimental.pallas as pl
import jax.experimental.pallas.tpu as pltpu

F32 = jnp.float32
BF16 = jnp.bfloat16
U32 = jnp.uint32

S = 2048
D = 1024
H = 32
DH = 32
FF = 3584
NPAIR = H // 2
LOG2E = 1.4426950408889634
LN_EPS = 1e-5

T = 256
TH = T // 2
NT_ = S // T
RC = 256
NC = D // RC
PPC = RC // 64
LNC = 16
WD_PAD = 128

FV = 10 * 128
FM = FF - FV
FVD = 8 * 128
WO_ROWS = 352
UNROLL2 = 2


def _spread(n, a, b, due=None):
    rel = [round(a + (b - a) * k / (n - 1), 3) for k in range(n)]
    return tuple((r, None if due is None else math.ceil(r) + due) for r in rel)


LN1_PLAN = _spread(16, 0, 12, 3)
WO_PLAN = _spread(11, 3, 13)
Z_PLAN = _spread(16, 6, 14, 2)
PRO_LN1_PLAN = ((None, None),) * 16
PRO_K_PLAN = _spread(8, 0, 6)
PRO_V_PLANS = (_spread(8, 0, 12), _spread(16, 13, 24)[:8], _spread(16, 13, 24)[8:], _spread(16, 0.7, 28, 3))
LN2B_PLAN = ((None, 0), (None, 0), (None, 0), (2.166, 8), (3.769, 9), (5.524, 11), (7.081, 13), (9.164, 15))
LN2A_PLAN = ((None, 18),) + _spread(7, 15.6, 20, 3)
PACK_PLAN = _spread(16, 100, 115) + _spread(16, 99.1, 114.1) + _spread(20, 0, 21)
G3_AT = 4
MOE_NA = 36
MOE_ND = 3
MOE_LAG = 2
MOE_ROT = 1
MOE_PARK = 1
MOE_SPLIT = 3
STAGGER = 8
LEAD = True

NN = (((1,), (0,)), ((), ()))
NT = (((1,), (1,)), ((), ()))


def _dot(a, b, dims):
    return lax.dot_general(a, b, dims, preferred_element_type=F32)


def _recip(x):
    return pl.reciprocal(x, approx=False, full_range=False)


def _pack(x):
    return pltpu.bitcast(x, U32)


def _unpack(x):
    return pltpu.bitcast(x, BF16)


def _pair_allreduce(a, op):
    a = op(a, pltpu.roll(a, 2, 0))
    return op(a, pltpu.roll(a, 4, 0))


def _tree(op, xs):
    xs = list(xs)
    while len(xs) > 1:
        nxt = [op(xs[i], xs[i + 1]) for i in range(0, len(xs) - 1, 2)]
        if len(xs) % 2:
            nxt.append(xs[-1])
        xs = nxt
    return xs[0]


def _dual_exp(p):
    sl = [p[8 * i:8 * i + 8, :] for i in range(8)]
    mx = _pair_allreduce(_tree(jnp.maximum, sl), jnp.maximum)
    mn = _pair_allreduce(_tree(jnp.minimum, sl), jnp.minimum)
    ep = [jnp.exp2(s - mx) for s in sl]
    en = [jnp.exp2(mn - s) for s in sl]
    sp = _pair_allreduce(_tree(jnp.add, ep), jnp.add)
    sn = _pair_allreduce(_tree(jnp.add, en), jnp.add)
    return ep, en, sp, sn


def _after(x, never, anchor):
    if anchor is None:
        return x
    d = jnp.concatenate([anchor] * (x.shape[0] // 8), axis=0)
    if x.shape[1] == 128:
        return jnp.where(never, d, x)
    return jnp.concatenate([jnp.where(never, d, x[:, :128]), x[:, 128:]], axis=1)


def _gate(x, never, deps):
    for i, dep in enumerate(deps):
        d = jnp.broadcast_to(dep, (8, 128))
        if x.dtype != F32:
            d = pltpu.bitcast(d, x.dtype)
        blk = jnp.where(never, d, x[8 * i:8 * i + 8, :128])
        if x.shape[1] > 128:
            blk = jnp.concatenate([blk, x[8 * i:8 * i + 8, 128:]], axis=1)
        parts = ([x[:8 * i, :]] if i else []) + [blk, x[8 * i + 8:, :]]
        x = jnp.concatenate(parts, axis=0)
    return x


def _lane_fold(a):
    return _tree(jnp.add, [a[:, 128 * i:128 * i + 128] for i in range(a.shape[1] // 128)])


def _row_sum(a):
    return jnp.sum(_lane_fold(a), axis=-1, keepdims=True)


def _lane_tile(a, n):
    return a if n == 1 else jnp.concatenate([a] * n, axis=1)


def _sublane_allreduce(a):
    a = a + pltpu.roll(a, 4, 0)
    a = a + pltpu.roll(a, 2, 0)
    return a + pltpu.roll(a, 1, 0)


def _col_broadcast(row8):
    return jnp.concatenate([row8] * 16, axis=0).astype(BF16).T.astype(F32)


def _vpu_matvec(xb, w_rows, never, anchors, lag):
    ng = xb.shape[0] // 8
    acc, hist = None, []
    for g in range(ng):
        dep = anchors[(g * len(anchors)) // ng]
        if g >= lag:
            dep = dep + hist[g - lag]
        x = jnp.where(never, dep, xb[8 * g:8 * g + 8, :])
        w = w_rows(g)
        t = w * _lane_tile(x, w.shape[1] // 128)
        acc = t if acc is None else acc + t
        c = 128 * ((g * MOE_ROT) % (w.shape[1] // 128))
        hist.append(acc[:, c:c + 128])
    return acc


class _Side:
    def __init__(self, never):
        self.never = never
        self.jobs = []
        self.deps = {}

    def add(self, plan, fn):
        for k, (rel, due) in enumerate(plan):
            if rel is None:
                self._run(due, fn, k, None)
            else:
                self.jobs.append((rel, due, fn, k))

    def _run(self, due, fn, k, anchor):
        dep = fn(k, anchor)
        if due is not None:
            self.deps.setdefault(due, []).append(dep)

    def check(self):
        assert not self.jobs and not self.deps, (self.jobs, self.deps)

    def gate(self, step, x):
        return _gate(x, self.never, self.deps.pop(step, []))

    def done(self, step, res):
        m = res.shape[0] // 8
        for job in sorted([j for j in self.jobs if step - 1 < j[0] <= step], key=lambda j: j[0]):
            self.jobs.remove(job)
            g = m - 1 - int((step - job[0]) * m)
            self._run(job[1], job[2], job[3], res[8 * g:8 * g + 8, res.shape[1] - 128:])


def _kernel(x_hbm, wqkv_hbm, wphi_hbm, wo_hbm, wr_hbm, wg_hbm, wu_hbm, wd_hbm, out_hbm,
            x_v, xn_v, lead_v, wraw_v, wt_v, wphi_v, a_v, woraw_v, wo_v, wrraw_v, wr_v, kvacc_v, kvbf_v,
            z_v, zb_v, phi_v, ha_v, hb_v, hn_v, o_v, wg_v, wu_v, wd_v, wgp_v, wup_v, wdp_v, patch_v,
            sem):
    SX, SW, SO, SM = 0, 6, 6 + 3 * NC, 6 + 3 * NC + NT_ + 1

    def x_copy(i):
        h0, h1 = ((1, 2), (2, 4), (4, 6), (6, 10), (10, 2 * NT_), (0, 1))[i]
        rows = pl.ds(h0 * TH, (h1 - h0) * TH)
        return pltpu.make_async_copy(x_hbm.at[rows, :], x_v.at[rows, :], sem.at[SX + i])

    def k0_copy(s):
        return pltpu.make_async_copy(wqkv_hbm.at[:, pl.ds(D + s * 128, 128)],
                                     wraw_v.at[NC, :, pl.ds(s * 128, 128)], sem.at[(SM + 7, SW + NC)[s]])

    def w_copy(j, c):
        return pltpu.make_async_copy(wqkv_hbm.at[:, pl.ds(j * D + c * RC, RC)], wraw_v.at[j * NC + c],
                                     sem.at[SW + j * NC + c])

    def wphi_copy(i):
        h0, h1 = ((0, 8), (8, 16), (16, H))[i]
        return pltpu.make_async_copy(wphi_hbm.at[pl.ds(h0, h1 - h0)], wphi_v.at[pl.ds(h0, h1 - h0)],
                                     sem.at[(SM + 4, SM + 8, SM + 9)[i]])

    wr_copy = pltpu.make_async_copy(wr_hbm, wrraw_v, sem.at[SM + 5])
    wo_copy = pltpu.make_async_copy(wo_hbm, woraw_v, sem.at[SM + 6])
    wg_copy = pltpu.make_async_copy(wg_hbm, wg_v, sem.at[SM + 0])
    wu_copy = pltpu.make_async_copy(wu_hbm, wu_v, sem.at[SM + 1])
    wd_copy = pltpu.make_async_copy(wd_hbm, wd_v.at[:, pl.ds(0, D)], sem.at[SM + 2])

    wphi_copy(0).start()
    k0_copy(0).start()
    x_copy(5).start()
    k0_copy(1).start()
    x_copy(0).start()
    wphi_copy(1).start()
    w_copy(1, 1).start()

    def view(ref, i, n, off=0):
        r0 = off + i * n
        return ref.at[pl.ds(r0 if isinstance(r0, int) else pl.multiple_of(r0, math.gcd(n, off)), n), :]

    def ln_rows(t, k, n, never=None, anchor=None):
        x = _after(view(x_v, t, T)[k * n:(k + 1) * n, :].astype(F32), never, anchor)
        xc = x - _row_sum(x) * (1.0 / D)
        rstd = lax.rsqrt(_row_sum(xc * xc) * (1.0 / D) + LN_EPS)
        view(xn_v, t, T // 2)[k * n // 2:(k + 1) * n // 2, :] = _pack((xc * rstd).astype(BF16))
        return _tree(jnp.add, [rstd[8 * i:8 * i + 8, :] for i in range(min(n, LNC) // 8)])

    def xn_tile(t):
        return _unpack(view(xn_v, t, T // 2)[...])

    def expand_wphi(c):
        w = wphi_v[8 * c:8 * c + 8].reshape(8 * DH, DH).astype(F32).T
        bits = pltpu.bitcast(w, U32)
        head = lax.broadcasted_iota(jnp.int32, (DH, 128), 1) >> 5
        for s in range(2):
            b = bits[:, 128 * s:128 * s + 128]
            for j in range(2):
                r0 = 64 * (2 * c + s) + 32 * j
                a_v[r0:r0 + 32, :] = jnp.where(head == 2 * j, b >> 16,
                                               jnp.where(head == 2 * j + 1, b, jnp.uint32(0)))

    wphi_copy(0).wait()
    expand_wphi(0)
    hb_v[...] = jnp.zeros((TH, D), F32)

    def fold(j, c, side=None, step0=None, slabs=range(RC // 128)):
        for s in slabs:
            g = c * (RC // 128) + s
            w = wraw_v[j * NC + c, :, s * 128:(s + 1) * 128]
            g0 = 64 * g if isinstance(g, int) else pl.multiple_of(64 * g, 64)
            if j == 2:
                wt = w.T
            else:
                res = _dot(_unpack(a_v[pl.ds(g0, 64), :]), w, NT)
                if side is not None:
                    side.done(step0 + 2 * s, res[:, :D // 2])
                    side.done(step0 + 2 * s + 1, res[:, D // 2:])
                wt = (res * LOG2E).astype(BF16)
            wt_v[j][pl.ds(g0, 64), :] = _pack(wt)

    def wt_rows(j, c):
        return wt_v[j][c * RC // 2:(c + 1) * RC // 2, :]

    def k_pair(p, slot, pr, c0, first, never=None):
        ep, en, sp, sn = _dual_exp(p)
        inv = _recip(sp * sn)
        scale = (sn * inv, sp * inv)
        es = ep + en
        cols = slice(c0, c0 + p.shape[1])
        n = 16 if never is None else 16 // STAGGER
        last = None
        for q in range(16 // n):
            sc = scale
            if last is not None:
                sc = [jnp.where(never, last, x) for x in scale]
            phi = jnp.concatenate([es[i] * sc[i // 8] for i in range(q * n, (q + 1) * n)], axis=0)
            rows = slice(8 * q * n, 8 * (q + 1) * n)
            z = phi if first else z_v[pr, rows, cols] + phi
            z_v[pr, rows, cols] = z
            phi_v[slot][64 * pr + 4 * q * n:64 * pr + 4 * (q + 1) * n, cols] = _pack(phi.astype(BF16))
            last = z[8 * n - 8:, :]

    def k_features(pk, slot, c, first, never=None):
        for j in range(PPC):
            k_pair(pk[64 * j:64 * j + 64, :], slot, c * PPC + j, 0, first, never)

    row = lax.broadcasted_iota(jnp.int32, (64, 128), 0)
    col = lax.broadcasted_iota(jnp.int32, (64, 128), 1)
    kv_keep = (row >> 5) == (col & 1)

    def kv_update(vt, slot, c, first, publish=False):
        for j in range(PPC):
            pr = c * PPC + j
            upd = _dot(vt[64 * j:64 * j + 64, :].astype(BF16), _unpack(phi_v[slot][64 * pr:64 * pr + 64, :]), NT)
            acc = upd if first else kvacc_v[pr] + upd
            kvacc_v[pr] = acc
            if publish:
                kvbf_v[32 * pr:32 * pr + 32, :] = _pack(jnp.where(kv_keep, acc, 0.0).astype(BF16))

    def proj(j, c, xn, lead=None):
        return proj_steps(_Side(None), 0, j, c, xn, lead)

    def save_lead(e, t):
        corner = _unpack(view(xn_v, t, T // 2)[0:TH // 2, 0:D // 2])
        view(lead_v, e, D // 4)[...] = _pack(corner.T)

    def proj_steps(side, step0, j, c, xn, lead=None):
        w = wt_rows(j, c)
        quarters = []
        for n in range(2):
            for m in range(2):
                step = step0 + 2 * n + m
                wq = _unpack(side.gate(step, w[m * (RC // 4):(m + 1) * (RC // 4), :]))
                if lead is not None and n + m == 0:
                    res = _dot(wq[:, :D // 2], _unpack(view(lead_v, lead, D // 4)[...]), NN)
                    res = _dot(wq[:, D // 2:], xn[0:TH, D // 2:], NT) + res
                else:
                    res = _dot(wq, xn[n * TH:(n + 1) * TH, :], NT)
                side.done(step, res)
                quarters.append(res)
        return jnp.concatenate(
            [jnp.concatenate([quarters[0], quarters[2]], axis=1),
             jnp.concatenate([quarters[1], quarters[3]], axis=1)], axis=0)

    def pack_rows(src, dst, r0, rows, c0, cols, never, a):
        w = _pack(src[r0:r0 + rows, c0:c0 + cols])
        d = jnp.concatenate([_lane_tile(pltpu.bitcast(a, U32), cols // 128)] * (rows // 16), axis=0)
        dst[r0 // 2:(r0 + rows) // 2, c0:c0 + cols] = jnp.where(never, d, w)

    def stash(i, val):
        for q in range(4):
            zb_v[4 * i + q] = val[128 * (q // 2):128 * (q // 2) + 128, 128 * (q % 2):128 * (q % 2) + 128]

    def stashed_k(i, slot, c, first):
        def job(k, a):
            j, n = k // 2, k % 2
            p = zb_v[4 * i + 2 * (j // 2) + n, 64 * (j % 2):64 * (j % 2) + 64, :]
            p = jnp.concatenate([_after(p[0:8, :], never0, a), p[8:, :]], axis=0)
            k_pair(p, slot, c * PPC + j, 128 * n, first, never0)
        return job

    def quarter(m, n):
        xn = _unpack(xn_v[n * TH // 2:(n + 1) * TH // 2, :])
        zb_v[2 * m + n] = _dot(_unpack(wt_v[1][64 * m:64 * m + 64, :]), xn, NT)

    k0_copy(0).wait()
    x_copy(5).wait()
    wphi_copy(2).start()
    w_copy(1, 2).start()
    x_copy(1).start()
    fold(1, 0, slabs=(0,))
    never0 = ln_rows(0, 0, TH)[0, 0] < 0.0
    quarter(0, 0)

    k0_copy(1).wait()
    x_copy(0).wait()
    wphi_copy(1).wait()
    w_copy(1, 3).start()
    for c in range(NC):
        w_copy(2, c).start()
    fold(1, 0, slabs=(1,))
    ln_rows(0, 1, TH)
    quarter(1, 0)
    quarter(0, 1)
    quarter(1, 1)
    expand_wphi(1)

    for c in (1, 2):
        w_copy(1, c).wait()
        if c == 1:
            wphi_copy(2).wait()
            expand_wphi(2)
            expand_wphi(3)
            x_copy(2).start()
            for cq in range(NC):
                w_copy(0, cq).start()
        else:
            x_copy(3).start()
            wo_copy.start()
            wr_copy.start()
            x_copy(4).start()
        side = _Side(never0)
        side.add(PRO_K_PLAN, stashed_k(c - 1, 0, c - 1, True))
        fold(1, c, side, 0)
        stash(c, proj_steps(side, 4, 1, c, xn_tile(0)))
        side.check()

    x_copy(1).wait()
    w_copy(1, 3).wait()
    wg_copy.start()
    wu_copy.start()
    wd_copy.start()
    side = _Side(never0)
    side.add(PRO_LN1_PLAN, lambda k, a: ln_rows(1, k, LNC, never0, a))
    fold(1, 3, side, 0)
    stash(3, proj_steps(side, 4, 1, 3, xn_tile(0)))
    xn1 = xn_tile(1)
    for c in range(3):
        k_features(proj(1, c, xn1), 1, c, c == 2, never0)
    stash(0, proj(1, 3, xn1))

    for c in range(NC):
        w_copy(2, c).wait()
    x_copy(2).wait()
    w_copy(0, 0).wait()
    side = _Side(never0)
    side.add(PRO_V_PLANS[0], stashed_k(2, 0, 2, False))
    side.add(PRO_V_PLANS[1], stashed_k(3, 0, 3, True))
    side.add(PRO_V_PLANS[2], stashed_k(0, 1, 3, False))
    side.add(PRO_V_PLANS[3], lambda k, a: ln_rows(2, k, LNC, never0, a))
    fold(0, 0)
    xns = (xn_tile(0), xn_tile(1))
    pending = None
    for c in range(NC):
        fold(2, c)
        for i in range(2):
            vt = proj_steps(side, 8 * c + 4 * i, 2, c, xns[i])
            if pending is not None:
                kv_update(*pending)
            pending = (vt, i, c, i == 0)
    side.check()
    kv_update(*pending)
    save_lead(0, 0)
    save_lead(1, 2)

    def phase1(u, carry):
        never = u < 0

        @pl.when(u == 0)
        def _():
            for c in range(1, NC):
                w_copy(0, c).wait()
            x_copy(3).wait()
            wo_copy.wait()
            wr_copy.wait()

        @pl.when(u == 1)
        def _():
            x_copy(4).wait()

        pending = None
        for i in range(2):
            t = 2 * u + 2 + i
            tn = jnp.minimum(t + 1, NT_ - 1)
            side = _Side(never)
            xn = xn_tile(t)
            for c in range(NC):
                pk = proj(1, c, xn, u + 1 if LEAD and i + c == 0 else None)
                if c == 0 and pending is not None:
                    kv_update(*pending)
                k_features(pk, i, c, False)
            side.add(LN1_PLAN, lambda k, a: ln_rows(tn, k, LNC, never, a))
            if i == 0:
                def pack_wo(k, a):
                    rows = WO_ROWS // len(WO_PLAN)
                    w0 = u * ((D - WO_ROWS) // 2)
                    src = woraw_v.at[pl.ds(pl.multiple_of(w0, 16), WO_ROWS), :]
                    dst = wo_v.at[pl.ds(pl.multiple_of(w0 // 2, 8), WO_ROWS // 2), :]
                    pack_rows(src, dst, k * rows, rows, 0, D, never, a)
                side.add(WO_PLAN, pack_wo)
            else:
                def z_final(k, a):
                    z = _after(z_v[k], never, a)
                    zs = _row_sum(z)
                    zb_v[k] = jnp.broadcast_to(zs, (128, 128))
                    return zs[120:128, :]
                side.add(Z_PLAN, z_final)
            side.done(0, pk)
            vts = []
            for c in range(NC):
                vts.append(proj_steps(side, 4 * c + 1, 2, c, xn))
                if c > 0:
                    kv_update(vts[c - 1], i, c - 1, False, i == 1)
            pending = (vts[NC - 1], i, NC - 1, False, i == 1)
            side.check()
        fold(0, u + 1)
        kv_update(*pending)
        save_lead(u + 2, tn)
        wr_v[...] = jnp.broadcast_to(wrraw_v[...].reshape(1, D).astype(F32), (8, D))
        return carry

    lax.fori_loop(0, (NT_ - 2) // 2, phase1, 0)

    def o_copy(r0, n, i):
        return pltpu.make_async_copy(o_v.at[pl.ds(r0, n), :], out_hbm.at[pl.ds(r0, n), :], sem.at[SO + i])

    def finish_rows(h_ref, k, ht, valid, st, never=None, anchor=None):
        r0 = ht * TH + k * LNC
        best, besti = st["route"]
        wr = jnp.concatenate([wr_v[...]] * (LNC // 8), axis=0)
        sub = lax.broadcasted_iota(jnp.int32, (8, 1), 0)
        h = _after(h_ref[k * LNC:(k + 1) * LNC, :], never, anchor)
        hc = h - _row_sum(h) * (1.0 / D)
        rstd = lax.rsqrt(_row_sum(hc * hc) * (1.0 / D) + LN_EPS)
        r = (_row_sum(hc * wr) * rstd).astype(BF16).astype(F32)
        hn = hc * rstd
        view(hn_v, ht, TH // 2)[k * LNC // 2:(k + 1) * LNC // 2, :] = _pack(hn.astype(BF16))
        view(o_v, ht, TH)[k * LNC:(k + 1) * LNC, :] = (hn + h).astype(BF16)
        if valid is not None:
            r = jnp.where(valid, r, -jnp.inf)
        for i in range(LNC // 8):
            ri = r[8 * i:8 * i + 8, :]
            better = ri > best
            best = jnp.where(better, ri, best)
            besti = jnp.where(better, sub + (r0 + 8 * i), besti)
        st["route"] = (best, besti)
        return best

    def q_features(pq, slot, c):
        for j in range(PPC):
            pr = c * PPC + j
            ep, en, sp, sn = _dual_exp(pq[64 * j:64 * j + 64, :])
            zz = [_lane_tile(zb_v[pr, 8 * i:8 * i + 8, :], pq.shape[1] // 128) for i in range(16)]
            ap = _pair_allreduce(_tree(jnp.add, [ep[i] * zz[i] for i in range(8)]), jnp.add)
            an = _pair_allreduce(_tree(jnp.add, [en[i] * zz[8 + i] for i in range(8)]), jnp.add)
            inv = _recip(ap * sn + (an + 1e-6 * sn) * sp)
            rp = sn * inv
            rn = sp * inv
            phi = jnp.concatenate([e * rp for e in ep] + [e * rn for e in en], axis=0)
            phi_v[slot][64 * pr:64 * pr + 64, :] = _pack(phi.astype(BF16))

    def attn_rows(slot, c, lo, hi):
        res = jnp.concatenate(
            [_dot(_unpack(kvbf_v[32 * pr:32 * pr + 32, :]), _unpack(phi_v[slot][64 * pr:64 * pr + 64, lo:hi]), NN)
             for pr in range(c * PPC, (c + 1) * PPC)], axis=0)
        return res.astype(BF16).T

    def out_proj(side, step0, o, k0, k1, n0=0, n1=D // 128):
        cols = []
        for n in range(n0, n1):
            w = side.gate(step0 + n, wo_v[k0 // 2:k1 // 2, n * 128:(n + 1) * 128])
            res = _dot(o, _unpack(w), NN)
            side.done(step0 + n, res)
            cols.append(res)
        return jnp.concatenate(cols, axis=1)

    def phase2(u, carry):
        for i in range(UNROLL2):
            carry = phase2_tile(u * UNROLL2 + i, i % 2, carry, u < 0, u if LEAD and i == 0 else None)

        r0 = pl.multiple_of(u * (UNROLL2 * T), T)

        @pl.when(u == 0)
        def _():
            o_copy(0, UNROLL2 * T - TH, 0).start()

        @pl.when(u > 0)
        def _():
            o_copy(pl.multiple_of(jnp.maximum(r0 - TH, 0), TH), UNROLL2 * T, u).start()

        return carry

    def phase2_tile(t, slot, carry, never, lead):
        hp = jnp.maximum(2 * t - 1, 0)
        side = _Side(never)
        st = {"route": carry}
        side.add(LN2B_PLAN, lambda k, a: finish_rows(hb_v, k, hp, t > 0, st, side.never, a))

        def pack_ffn(k, a):
            if k < 32:
                n = D // NT_
                pack_rows(view((wg_v, wu_v)[k % 2], t, n), view((wgp_v, wup_v)[k % 2], t, n // 2),
                          (k // 4) * 16, 16, (k // 2 % 2) * (FM // 2), FM // 2, never, a)
            else:
                n = (FF - FVD) // NT_
                pack_rows(view(wd_v, t, n, FVD), view(wdp_v, t, n // 2), (k - 32) * 16, 16, 0, D, never, a)
        side.add(PACK_PLAN[:32 + (FF - FVD) // 128], pack_ffn)

        xn = xn_tile(t)
        xt = view(x_v, t, T)
        os_ = []
        for c in range(NC):
            pq = proj_steps(side, 100 + 4 * c, 0, c, xn, lead if c == 0 else None)
            if c == 0:
                pq = side.gate(0, pq)
            q_features(pq, slot, c)
            if c > 0:
                os_.append(attn_rows(slot, c - 1, 0, T))
        oa = jnp.concatenate([o[0:TH, :] for o in os_[:2]], axis=1)
        ha0 = out_proj(side, 0, oa, 0, D // 2, 0, G3_AT)
        os_.append(attn_rows(slot, NC - 1, 0, T))
        ha1 = out_proj(side, 0, oa, 0, D // 2, G3_AT, D // 128)
        ha = jnp.concatenate([ha0, ha1], axis=1) + xt[0:TH, :].astype(F32)
        ha_v[...] = ha + out_proj(side, 8, jnp.concatenate([o[0:TH, :] for o in os_[2:]], axis=1), D // 2, D)
        side.add(LN2A_PLAN, lambda k, a: finish_rows(ha_v, k, 2 * t, None, st, side.never, a))
        ob = jnp.concatenate([o[TH:T, :] for o in os_], axis=1)
        hb_v[...] = xt[TH:T, :].astype(F32) + out_proj(side, 16, ob, 0, D)
        side.check()
        return st["route"]

    wg_copy.wait()
    wu_copy.wait()
    wd_copy.wait()
    route = lax.fori_loop(
        0, NT_ // UNROLL2, phase2,
        (jnp.full((8, 1), -jnp.inf, F32), jnp.zeros((8, 1), jnp.int32)))
    st = {"route": route}
    for k in range(TH // LNC):
        finish_rows(hb_v, k, 2 * NT_ - 1, None, st)
    best, besti = st["route"]
    o_copy(S - TH, TH, NT_).start()

    rmax = jnp.max(best, axis=0, keepdims=True)
    idx = jnp.min(jnp.where(best == rmax, besti, S), axis=0, keepdims=True)
    idx_s = jnp.clip(idx[0, 0], 0, S - 1)
    blk = pl.multiple_of((idx_s >> 4) << 4, 16)
    pair = jnp.broadcast_to(hn_v[pl.ds(idx_s >> 1, 1), :], (8, D))
    x8 = pltpu.bitcast(jnp.where((idx_s & 1) == 1, pair & jnp.uint32(0xFFFF0000), pair << 16), F32)
    xs = jnp.concatenate([x8, x8], axis=0).astype(BF16)
    acts, anchors = [], []

    def park(v, half):
        if not MOE_PARK:
            return v
        n = v.shape[0] // 128
        for i in range(n):
            z_v[i, :, 128 * half:128 * half + 128] = v[128 * i:128 * i + 128, :]
        return jnp.concatenate([z_v[i, :, 128 * half:128 * half + 128] for i in range(n)], axis=0)

    for c0 in range(0, FM, 128):
        g = _dot(xs, _unpack(wgp_v[:, c0:c0 + 128]), NN)[0:8, :]
        u = _dot(xs, _unpack(wup_v[:, c0:c0 + 128]), NN)[0:8, :]
        anchors += [g, u]
        acts.append(g * jax.nn.sigmoid(g) * u)
    xb = park(_col_broadcast(x8), 0)
    if MOE_SPLIT:
        g, u = [_sublane_allreduce(_vpu_matvec(
            xb, lambda g: w[8 * g:8 * g + 8, FM:FF].astype(F32), never0,
            anchors[i * MOE_NA // 2:(i + 1) * MOE_NA // 2], MOE_SPLIT)) for i, w in enumerate((wg_v, wu_v))]
    else:
        gu = _sublane_allreduce(_vpu_matvec(
            xb, lambda g: jnp.concatenate([w[8 * g:8 * g + 8, FM:FF].astype(F32) for w in (wg_v, wu_v)], axis=1),
            never0, anchors[:MOE_NA], 1))
        g, u = gu[:, :FV], gu[:, FV:]
    acts.append(g * jax.nn.sigmoid(g) * u)
    a = jnp.concatenate(acts, axis=1)
    am = jnp.concatenate([a[:, FVD:], a[:, FVD:]], axis=0).astype(BF16)
    ys, anchors = [], anchors[MOE_NA:]
    for k0 in range(0, FF - FVD, 512):
        k1 = min(k0 + 512, FF - FVD)
        yk = _dot(am[:, k0:k1], _unpack(wdp_v[k0 // 2:k1 // 2, :]), NN)[0:8, :]
        ys.append(yk)
        anchors += [yk[:, c:c + 128] for c in range(128, D, 256)]
    ys.append(_sublane_allreduce(_vpu_matvec(
        park(_col_broadcast(a[:, :FVD]), 1), lambda g: wd_v[8 * g:8 * g + 8, 0:D].astype(F32), never0, anchors[:-MOE_ND], MOE_LAG)))
    y = _tree(jnp.add, ys) * jax.nn.sigmoid(rmax)
    y = jnp.concatenate([y, y], axis=0)
    sel = lax.broadcasted_iota(jnp.int32, (16, 1), 0) == (idx_s - blk)
    patch_v[...] = (o_v[pl.ds(blk, 16), :].astype(F32) + jnp.where(sel, y, 0.0)).astype(BF16)
    o_copy(0, UNROLL2 * T - TH, 0).wait()
    for u in range(1, NT_ // UNROLL2):
        o_copy(u * UNROLL2 * T - TH, UNROLL2 * T, u).wait()
    o_copy(S - TH, TH, NT_).wait()
    pc = pltpu.make_async_copy(patch_v, out_hbm.at[pl.ds(blk, 16), :], sem.at[SM + 3])
    pc.start()
    pc.wait()


@jax.jit
def pallas_sequential_preLN__linear_kernel_hedgehog__moe_arch_mod__prompt_kernel(
    A_x: jax.Array,
    A_wqkv: jax.Array,
    A_w_phi: jax.Array,
    A_wo: jax.Array,
    B_x: jax.Array,
    B_w_r: jax.Array,
    B_w_gate: jax.Array,
    B_w_up: jax.Array,
    B_w_down: jax.Array,
):
    del B_x
    hbm = pl.BlockSpec(memory_space=pl.ANY)
    out = pl.pallas_call(
        _kernel,
        out_shape=jax.ShapeDtypeStruct((S, D), BF16),
        in_specs=[hbm] * 8,
        out_specs=hbm,
        scratch_shapes=[
            pltpu.VMEM((S, D), BF16),
            pltpu.VMEM((S // 2, D), U32),
            pltpu.VMEM((5 * D // 4, 128), U32),
            pltpu.VMEM((3 * NC, D, RC), BF16),
            [pltpu.VMEM((D // 2, D), U32)] * 3,
            pltpu.VMEM((H, DH, DH), BF16),
            pltpu.VMEM((8 * 64, 128), U32),
            pltpu.VMEM((D, D), BF16),
            pltpu.VMEM((D // 2, D), U32),
            pltpu.VMEM((D,), BF16),
            pltpu.VMEM((8, D), F32),
            pltpu.VMEM((NPAIR, 64, 128), F32),
            pltpu.VMEM((NPAIR * 32, 128), U32),
            pltpu.VMEM((NPAIR, 128, T), F32),
            pltpu.VMEM((NPAIR, 128, 128), F32),
            [pltpu.VMEM((NPAIR * 64, T), U32)] * 2,
            pltpu.VMEM((TH, D), F32),
            pltpu.VMEM((TH, D), F32),
            pltpu.VMEM((S // 2, D), U32),
            pltpu.VMEM((S, D), BF16),
            pltpu.VMEM((D, FF), BF16),
            pltpu.VMEM((D, FF), BF16),
            pltpu.VMEM((FF, D + WD_PAD), BF16),
            pltpu.VMEM((D // 2, FM), U32),
            pltpu.VMEM((D // 2, FM), U32),
            pltpu.VMEM(((FF - FVD) // 2, D), U32),
            pltpu.VMEM((16, D), BF16),
            pltpu.SemaphoreType.DMA((6 + 3 * NC + NT_ + 11,)),
        ],
        compiler_params=pltpu.CompilerParams(vmem_limit_bytes=100 * 1024 * 1024,
                                             disable_semaphore_checks=True, disable_bounds_checks=True),
        name="hedgehog_mod",
    )(
        A_x.reshape(S, D),
        A_wqkv,
        A_w_phi,
        A_wo,
        B_w_r,
        B_w_gate,
        B_w_up,
        B_w_down,
    )
    return out.reshape(1, S, D)
```

```python
import math

import jax
import jax.numpy as jnp
from jax import lax
import jax.experimental.pallas as pl
import jax.experimental.pallas.tpu as pltpu

F32 = jnp.float32
BF16 = jnp.bfloat16
U32 = jnp.uint32

S = 2048
D = 1024
H = 32
DH = 32
FF = 3584
NPAIR = H // 2
LOG2E = 1.4426950408889634
LN_EPS = 1e-5

T = 256
TH = T // 2
NT_ = S // T
RC = 256
NC = D // RC
PPC = RC // 64
LNC = 16
FFP = 4096

FV = 10 * 128
FM = FF - FV
FVD = 8 * 128
WO_ROWS = 352
UNROLL2 = 2


def _spread(n, a, b, due=None):
    rel = [round(a + (b - a) * k / (n - 1), 3) for k in range(n)]
    return tuple((r, None if due is None else math.ceil(r) + due) for r in rel)


LN1_PLAN = _spread(16, 0, 13, 3)
WO_PLAN = _spread(11, 3, 13)
Z_PLAN = _spread(16, 2, 13, 2)
PRO_LN1_PLAN = ((None, None),) * 16
PRO_K_PLAN = _spread(8, 0, 6)
PRO_V_PLANS = (_spread(8, 0, 12), _spread(16, 13, 22)[:8], _spread(16, 13, 22)[8:], _spread(16, 1.2, 27, 3))
LN2B_PLAN = ((None, 0), (None, 0), (None, 0), (2.166, 8), (3.769, 9), (5.524, 11), (7.081, 13), (9.164, 15))
LN2A_PLAN = ((None, 18),) + _spread(7, 15.6, 20, 3)
PACK_PLAN = _spread(16, 100, 115) + _spread(16, 99.1, 114.1) + _spread(20, 0, 21)
G3_AT = 4
MOE_NA = 36
MOE_ND = 3
MOE_LAG = 2
MOE_ROT = 1
MOE_PARK = 1
MOE_SPLIT = 3
STAGGER = 8
LEAD = True
PACK_VIA_F32 = True

NN = (((1,), (0,)), ((), ()))
NT = (((1,), (1,)), ((), ()))


def _dot(a, b, dims):
    return lax.dot_general(a, b, dims, preferred_element_type=F32)


def _recip(x):
    return pl.reciprocal(x, approx=False, full_range=False)


def _pack(x):
    return pltpu.bitcast(x, U32)


def _unpack(x):
    return pltpu.bitcast(x, BF16)


def _pair_allreduce(a, op):
    a = op(a, pltpu.roll(a, 2, 0))
    return op(a, pltpu.roll(a, 4, 0))


def _tree(op, xs):
    xs = list(xs)
    while len(xs) > 1:
        nxt = [op(xs[i], xs[i + 1]) for i in range(0, len(xs) - 1, 2)]
        if len(xs) % 2:
            nxt.append(xs[-1])
        xs = nxt
    return xs[0]


def _dual_exp(p):
    sl = [p[8 * i:8 * i + 8, :] for i in range(8)]
    mx = _pair_allreduce(_tree(jnp.maximum, sl), jnp.maximum)
    mn = _pair_allreduce(_tree(jnp.minimum, sl), jnp.minimum)
    ep = [jnp.exp2(s - mx) for s in sl]
    en = [jnp.exp2(mn - s) for s in sl]
    sp = _pair_allreduce(_tree(jnp.add, ep), jnp.add)
    sn = _pair_allreduce(_tree(jnp.add, en), jnp.add)
    return ep, en, sp, sn


def _after(x, never, anchor):
    if anchor is None:
        return x
    d = jnp.concatenate([anchor] * (x.shape[0] // 8), axis=0)
    if x.shape[1] == 128:
        return jnp.where(never, d, x)
    return jnp.concatenate([jnp.where(never, d, x[:, :128]), x[:, 128:]], axis=1)


def _gate(x, never, deps):
    for i, dep in enumerate(deps):
        d = jnp.broadcast_to(dep, (8, 128))
        if x.dtype != F32:
            d = pltpu.bitcast(d, x.dtype)
        blk = jnp.where(never, d, x[8 * i:8 * i + 8, :128])
        if x.shape[1] > 128:
            blk = jnp.concatenate([blk, x[8 * i:8 * i + 8, 128:]], axis=1)
        parts = ([x[:8 * i, :]] if i else []) + [blk, x[8 * i + 8:, :]]
        x = jnp.concatenate(parts, axis=0)
    return x


def _lane_fold(a):
    return _tree(jnp.add, [a[:, 128 * i:128 * i + 128] for i in range(a.shape[1] // 128)])


def _row_sum(a):
    return jnp.sum(_lane_fold(a), axis=-1, keepdims=True)


def _lane_tile(a, n):
    return a if n == 1 else jnp.concatenate([a] * n, axis=1)


def _sublane_allreduce(a):
    a = a + pltpu.roll(a, 4, 0)
    a = a + pltpu.roll(a, 2, 0)
    return a + pltpu.roll(a, 1, 0)


def _col_broadcast(row8):
    return jnp.concatenate([row8] * 16, axis=0).astype(BF16).T.astype(F32)


def _vpu_matvec(xb, w_rows, never, anchors, lag):
    ng = xb.shape[0] // 8
    acc, hist = None, []
    for g in range(ng):
        dep = anchors[(g * len(anchors)) // ng]
        if g >= lag:
            dep = dep + hist[g - lag]
        x = jnp.where(never, dep, xb[8 * g:8 * g + 8, :])
        w = w_rows(g)
        t = w * _lane_tile(x, w.shape[1] // 128)
        acc = t if acc is None else acc + t
        c = 128 * ((g * MOE_ROT) % (w.shape[1] // 128))
        hist.append(acc[:, c:c + 128])
    return acc


class _Side:
    def __init__(self, never):
        self.never = never
        self.jobs = []
        self.deps = {}

    def add(self, plan, fn):
        for k, (rel, due) in enumerate(plan):
            if rel is None:
                self._run(due, fn, k, None)
            else:
                self.jobs.append((rel, due, fn, k))

    def _run(self, due, fn, k, anchor):
        dep = fn(k, anchor)
        if due is not None:
            self.deps.setdefault(due, []).append(dep)

    def check(self):
        assert not self.jobs and not self.deps, (self.jobs, self.deps)

    def gate(self, step, x):
        return _gate(x, self.never, self.deps.pop(step, []))

    def done(self, step, res):
        m = res.shape[0] // 8
        for job in sorted([j for j in self.jobs if step - 1 < j[0] <= step], key=lambda j: j[0]):
            self.jobs.remove(job)
            g = m - 1 - int((step - job[0]) * m)
            self._run(job[1], job[2], job[3], res[8 * g:8 * g + 8, res.shape[1] - 128:])


def _kernel(x_hbm, wqkv_hbm, wphi_hbm, wo_hbm, wr_hbm, wg_hbm, wu_hbm, wd_hbm, out_hbm,
            x_v, xn_v, lead_v, wraw_v, wt_v, wphi_v, a_v, woraw_v, wo_v, wrraw_v, wr_v, kvacc_v, kvbf_v,
            z_v, zb_v, phi_v, ha_v, hb_v, hn_v, o_v, wg_v, wu_v, wd_v, wgp_v, wup_v, wdp_v, patch_v,
            sem):
    SX, SW, SO, SM = 0, 6, 6 + 3 * NC, 6 + 3 * NC + NT_ + 1

    def x_copy(i):
        h0, h1 = ((1, 2), (2, 4), (4, 6), (6, 10), (10, 2 * NT_), (0, 1))[i]
        rows = pl.ds(h0 * TH, (h1 - h0) * TH)
        return pltpu.make_async_copy(x_hbm.at[rows, :], x_v.at[rows, :], sem.at[SX + i])

    def k0_copy(s):
        return pltpu.make_async_copy(wqkv_hbm.at[:, pl.ds(D + s * 128, 128)],
                                     wraw_v.at[NC, :, pl.ds(s * 128, 128)], sem.at[(SM + 7, SW + NC)[s]])

    def w_copy(j, c):
        return pltpu.make_async_copy(wqkv_hbm.at[:, pl.ds(j * D + c * RC, RC)], wraw_v.at[j * NC + c],
                                     sem.at[SW + j * NC + c])

    def wphi_copy(i):
        h0, h1 = ((0, 8), (8, 16), (16, H))[i]
        return pltpu.make_async_copy(wphi_hbm.at[pl.ds(h0, h1 - h0)], wphi_v.at[pl.ds(h0, h1 - h0)],
                                     sem.at[(SM + 4, SM + 8, SM + 9)[i]])

    wr_copy = pltpu.make_async_copy(wr_hbm, wrraw_v, sem.at[SM + 5])
    wo_copy = pltpu.make_async_copy(wo_hbm, woraw_v, sem.at[SM + 6])
    wg_copy = pltpu.make_async_copy(wg_hbm, wg_v.at[:, pl.ds(0, FF)], sem.at[SM + 0])
    wu_copy = pltpu.make_async_copy(wu_hbm, wu_v.at[:, pl.ds(0, FF)], sem.at[SM + 1])
    wd_copy = pltpu.make_async_copy(wd_hbm, wd_v, sem.at[SM + 2])

    wphi_copy(0).start()
    k0_copy(0).start()
    x_copy(5).start()
    k0_copy(1).start()
    x_copy(0).start()
    wphi_copy(1).start()
    w_copy(1, 1).start()

    def view(ref, i, n, off=0):
        r0 = off + i * n
        return ref.at[pl.ds(r0 if isinstance(r0, int) else pl.multiple_of(r0, math.gcd(n, off)), n), :]

    def ln_rows(t, k, n, never=None, anchor=None):
        x = _after(view(x_v, t, T)[k * n:(k + 1) * n, :].astype(F32), never, anchor)
        xc = x - _row_sum(x) * (1.0 / D)
        rstd = lax.rsqrt(_row_sum(xc * xc) * (1.0 / D) + LN_EPS)
        view(xn_v, t, T // 2)[k * n // 2:(k + 1) * n // 2, :] = _pack((xc * rstd).astype(BF16))
        return _tree(jnp.add, [rstd[8 * i:8 * i + 8, :] for i in range(min(n, LNC) // 8)])

    def xn_tile(t):
        return _unpack(view(xn_v, t, T // 2)[...])

    def expand_wphi(c):
        w = wphi_v[8 * c:8 * c + 8].reshape(8 * DH, DH).astype(F32).T
        bits = pltpu.bitcast(w, U32)
        head = lax.broadcasted_iota(jnp.int32, (DH, 128), 1) >> 5
        for s in range(2):
            b = bits[:, 128 * s:128 * s + 128]
            for j in range(2):
                r0 = 64 * (2 * c + s) + 32 * j
                a_v[r0:r0 + 32, :] = jnp.where(head == 2 * j, b >> 16,
                                               jnp.where(head == 2 * j + 1, b, jnp.uint32(0)))

    wphi_copy(0).wait()
    expand_wphi(0)
    hb_v[...] = jnp.zeros((TH, D), F32)

    def fold(j, c, side=None, step0=None, slabs=range(RC // 128)):
        for s in slabs:
            g = c * (RC // 128) + s
            w = wraw_v[j * NC + c, :, s * 128:(s + 1) * 128]
            g0 = 64 * g if isinstance(g, int) else pl.multiple_of(64 * g, 64)
            if j == 2:
                wt = w.T
            else:
                res = _dot(_unpack(a_v[pl.ds(g0, 64), :]), w, NT)
                if side is not None:
                    side.done(step0 + 2 * s, res[:, :D // 2])
                    side.done(step0 + 2 * s + 1, res[:, D // 2:])
                wt = (res * LOG2E).astype(BF16)
            wt_v[j][pl.ds(g0, 64), :] = _pack(wt)

    def wt_rows(j, c):
        return wt_v[j][c * RC // 2:(c + 1) * RC // 2, :]

    def k_pair(p, slot, pr, c0, first, never=None):
        ep, en, sp, sn = _dual_exp(p)
        inv = _recip(sp * sn)
        scale = (sn * inv, sp * inv)
        es = ep + en
        cols = slice(c0, c0 + p.shape[1])
        n = 16 if never is None else 16 // STAGGER
        last = None
        for q in range(16 // n):
            sc = scale
            if last is not None:
                sc = [jnp.where(never, last, x) for x in scale]
            phi = jnp.concatenate([es[i] * sc[i // 8] for i in range(q * n, (q + 1) * n)], axis=0)
            rows = slice(8 * q * n, 8 * (q + 1) * n)
            z = phi if first else z_v[pr, rows, cols] + phi
            z_v[pr, rows, cols] = z
            phi_v[slot][64 * pr + 4 * q * n:64 * pr + 4 * (q + 1) * n, cols] = _pack(phi.astype(BF16))
            last = z[8 * n - 8:, :]

    def k_features(pk, slot, c, first, never=None):
        for j in range(PPC):
            k_pair(pk[64 * j:64 * j + 64, :], slot, c * PPC + j, 0, first, never)

    row = lax.broadcasted_iota(jnp.int32, (64, 128), 0)
    col = lax.broadcasted_iota(jnp.int32, (64, 128), 1)
    kv_keep = (row >> 5) == (col & 1)

    def kv_update(vt, slot, c, first, publish=False):
        for j in range(PPC):
            pr = c * PPC + j
            upd = _dot(vt[64 * j:64 * j + 64, :].astype(BF16), _unpack(phi_v[slot][64 * pr:64 * pr + 64, :]), NT)
            acc = upd if first else kvacc_v[pr] + upd
            kvacc_v[pr] = acc
            if publish:
                kvbf_v[32 * pr:32 * pr + 32, :] = _pack(jnp.where(kv_keep, acc, 0.0).astype(BF16))

    def proj(j, c, xn, lead=None):
        return proj_steps(_Side(None), 0, j, c, xn, lead)

    def save_lead(e, t):
        corner = _unpack(view(xn_v, t, T // 2)[0:TH // 2, 0:D // 2])
        view(lead_v, e, D // 4)[...] = _pack(corner.T)

    def proj_steps(side, step0, j, c, xn, lead=None):
        w = wt_rows(j, c)
        quarters = []
        for n in range(2):
            for m in range(2):
                step = step0 + 2 * n + m
                wq = _unpack(side.gate(step, w[m * (RC // 4):(m + 1) * (RC // 4), :]))
                if lead is not None and n + m == 0:
                    res = _dot(wq[:, :D // 2], _unpack(view(lead_v, lead, D // 4)[...]), NN)
                    res = _dot(wq[:, D // 2:], xn[0:TH, D // 2:], NT) + res
                else:
                    res = _dot(wq, xn[n * TH:(n + 1) * TH, :], NT)
                side.done(step, res)
                quarters.append(res)
        return jnp.concatenate(
            [jnp.concatenate([quarters[0], quarters[2]], axis=1),
             jnp.concatenate([quarters[1], quarters[3]], axis=1)], axis=0)

    def pack_rows(src, dst, r0, rows, c0, cols, never, a):
        if PACK_VIA_F32:
            w = src[r0:r0 + rows, c0:c0 + cols].astype(F32)
            d = _lane_tile(a, cols // 128)
            w = jnp.concatenate([jnp.where(never, d, w[8 * i:8 * i + 8, :]) if i % 2 == 0 else w[8 * i:8 * i + 8, :]
                                 for i in range(rows // 8)], axis=0)
            dst[r0 // 2:(r0 + rows) // 2, c0:c0 + cols] = _pack(w.astype(BF16))
            return
        w = _pack(src[r0:r0 + rows, c0:c0 + cols])
        d = jnp.concatenate([_lane_tile(pltpu.bitcast(a, U32), cols // 128)] * (rows // 16), axis=0)
        dst[r0 // 2:(r0 + rows) // 2, c0:c0 + cols] = jnp.where(never, d, w)

    def stash(i, val):
        for q in range(4):
            zb_v[4 * i + q] = val[128 * (q // 2):128 * (q // 2) + 128, 128 * (q % 2):128 * (q % 2) + 128]

    def stashed_k(i, slot, c, first):
        def job(k, a):
            j, n = k // 2, k % 2
            p = zb_v[4 * i + 2 * (j // 2) + n, 64 * (j % 2):64 * (j % 2) + 64, :]
            p = jnp.concatenate([_after(p[0:8, :], never0, a), p[8:, :]], axis=0)
            k_pair(p, slot, c * PPC + j, 128 * n, first, never0)
        return job

    def quarter(m, n):
        xn = _unpack(xn_v[n * TH // 2:(n + 1) * TH // 2, :])
        zb_v[2 * m + n] = _dot(_unpack(wt_v[1][64 * m:64 * m + 64, :]), xn, NT)

    k0_copy(0).wait()
    x_copy(5).wait()
    wphi_copy(2).start()
    w_copy(1, 2).start()
    x_copy(1).start()
    fold(1, 0, slabs=(0,))
    never0 = ln_rows(0, 0, TH)[0, 0] < 0.0
    quarter(0, 0)

    k0_copy(1).wait()
    x_copy(0).wait()
    wphi_copy(1).wait()
    w_copy(1, 3).start()
    for c in range(NC):
        w_copy(2, c).start()
    fold(1, 0, slabs=(1,))
    ln_rows(0, 1, TH)
    quarter(1, 0)
    quarter(0, 1)
    quarter(1, 1)
    expand_wphi(1)

    for c in (1, 2):
        w_copy(1, c).wait()
        if c == 1:
            wphi_copy(2).wait()
            expand_wphi(2)
            expand_wphi(3)
            x_copy(2).start()
            for cq in range(NC):
                w_copy(0, cq).start()
        else:
            x_copy(3).start()
            wo_copy.start()
            wr_copy.start()
            x_copy(4).start()
        side = _Side(never0)
        side.add(PRO_K_PLAN, stashed_k(c - 1, 0, c - 1, True))
        fold(1, c, side, 0)
        stash(c, proj_steps(side, 4, 1, c, xn_tile(0)))
        side.check()

    x_copy(1).wait()
    w_copy(1, 3).wait()
    wg_copy.start()
    wu_copy.start()
    wd_copy.start()
    side = _Side(never0)
    side.add(PRO_LN1_PLAN, lambda k, a: ln_rows(1, k, LNC, never0, a))
    fold(1, 3, side, 0)
    stash(3, proj_steps(side, 4, 1, 3, xn_tile(0)))
    xn1 = xn_tile(1)
    for c in range(3):
        k_features(proj(1, c, xn1), 1, c, c == 2, never0)
    stash(0, proj(1, 3, xn1))

    for c in range(NC):
        w_copy(2, c).wait()
    x_copy(2).wait()
    w_copy(0, 0).wait()
    side = _Side(never0)
    side.add(PRO_V_PLANS[0], stashed_k(2, 0, 2, False))
    side.add(PRO_V_PLANS[1], stashed_k(3, 0, 3, True))
    side.add(PRO_V_PLANS[2], stashed_k(0, 1, 3, False))
    side.add(PRO_V_PLANS[3], lambda k, a: ln_rows(2, k, LNC, never0, a))
    fold(0, 0)
    xns = (xn_tile(0), xn_tile(1))
    pending = None
    for c in range(NC):
        fold(2, c)
        for i in range(2):
            vt = proj_steps(side, 8 * c + 4 * i, 2, c, xns[i])
            if pending is not None:
                kv_update(*pending)
            pending = (vt, i, c, i == 0)
    side.check()
    kv_update(*pending)
    save_lead(0, 0)
    save_lead(1, 2)

    def phase1(u, carry):
        never = u < 0

        @pl.when(u == 0)
        def _():
            for c in range(1, NC):
                w_copy(0, c).wait()
            x_copy(3).wait()
            wo_copy.wait()
            wr_copy.wait()

        @pl.when(u == 1)
        def _():
            x_copy(4).wait()

        pending = None
        for i in range(2):
            t = 2 * u + 2 + i
            tn = jnp.minimum(t + 1, NT_ - 1)
            side = _Side(never)
            xn = xn_tile(t)
            for c in range(NC):
                pk = proj(1, c, xn, u + 1 if LEAD and i + c == 0 else None)
                if c == 0 and pending is not None:
                    kv_update(*pending)
                k_features(pk, i, c, False)
            side.add(LN1_PLAN, lambda k, a: ln_rows(tn, k, LNC, never, a))
            if i == 0:
                def pack_wo(k, a):
                    rows = WO_ROWS // len(WO_PLAN)
                    w0 = u * ((D - WO_ROWS) // 2)
                    src = woraw_v.at[pl.ds(pl.multiple_of(w0, 16), WO_ROWS), :]
                    dst = wo_v.at[pl.ds(pl.multiple_of(w0 // 2, 8), WO_ROWS // 2), :]
                    pack_rows(src, dst, k * rows, rows, 0, D, never, a)
                side.add(WO_PLAN, pack_wo)
            else:
                def z_final(k, a):
                    z = _after(z_v[k], never, a)
                    zs = _row_sum(z)
                    zb_v[k] = jnp.broadcast_to(zs, (128, 128))
                    return zs[120:128, :]
                side.add(Z_PLAN, z_final)
            side.done(0, pk)
            vts = []
            for c in range(NC):
                vts.append(proj_steps(side, 4 * c + 1, 2, c, xn))
                if c > 0:
                    kv_update(vts[c - 1], i, c - 1, False, i == 1)
            pending = (vts[NC - 1], i, NC - 1, False, i == 1)
            side.check()
        fold(0, u + 1)
        kv_update(*pending)
        save_lead(u + 2, tn)
        wr_v[...] = jnp.broadcast_to(wrraw_v[...].reshape(1, D).astype(F32), (8, D))
        return carry

    lax.fori_loop(0, (NT_ - 2) // 2, phase1, 0)

    def o_copy(r0, n, i):
        return pltpu.make_async_copy(o_v.at[pl.ds(r0, n), :], out_hbm.at[pl.ds(r0, n), :], sem.at[SO + i])

    def finish_rows(h_ref, k, ht, valid, st, never=None, anchor=None):
        r0 = ht * TH + k * LNC
        best, besti = st["route"]
        wr = jnp.concatenate([wr_v[...]] * (LNC // 8), axis=0)
        sub = lax.broadcasted_iota(jnp.int32, (8, 1), 0)
        h = _after(h_ref[k * LNC:(k + 1) * LNC, :], never, anchor)
        hc = h - _row_sum(h) * (1.0 / D)
        rstd = lax.rsqrt(_row_sum(hc * hc) * (1.0 / D) + LN_EPS)
        r = (_row_sum(hc * wr) * rstd).astype(BF16).astype(F32)
        hn = hc * rstd
        view(hn_v, ht, TH // 2)[k * LNC // 2:(k + 1) * LNC // 2, :] = _pack(hn.astype(BF16))
        view(o_v, ht, TH)[k * LNC:(k + 1) * LNC, :] = (hn + h).astype(BF16)
        if valid is not None:
            r = jnp.where(valid, r, -jnp.inf)
        for i in range(LNC // 8):
            ri = r[8 * i:8 * i + 8, :]
            better = ri > best
            best = jnp.where(better, ri, best)
            besti = jnp.where(better, sub + (r0 + 8 * i), besti)
        st["route"] = (best, besti)
        return best

    def q_features(pq, slot, c):
        for j in range(PPC):
            pr = c * PPC + j
            ep, en, sp, sn = _dual_exp(pq[64 * j:64 * j + 64, :])
            zz = [_lane_tile(zb_v[pr, 8 * i:8 * i + 8, :], pq.shape[1] // 128) for i in range(16)]
            ap = _pair_allreduce(_tree(jnp.add, [ep[i] * zz[i] for i in range(8)]), jnp.add)
            an = _pair_allreduce(_tree(jnp.add, [en[i] * zz[8 + i] for i in range(8)]), jnp.add)
            inv = _recip(ap * sn + (an + 1e-6 * sn) * sp)
            rp = sn * inv
            rn = sp * inv
            phi = jnp.concatenate([e * rp for e in ep] + [e * rn for e in en], axis=0)
            phi_v[slot][64 * pr:64 * pr + 64, :] = _pack(phi.astype(BF16))

    def attn_rows(slot, c, lo, hi):
        res = jnp.concatenate(
            [_dot(_unpack(kvbf_v[32 * pr:32 * pr + 32, :]), _unpack(phi_v[slot][64 * pr:64 * pr + 64, lo:hi]), NN)
             for pr in range(c * PPC, (c + 1) * PPC)], axis=0)
        return res.astype(BF16).T

    def out_proj(side, step0, o, k0, k1, n0=0, n1=D // 128):
        cols = []
        for n in range(n0, n1):
            w = side.gate(step0 + n, wo_v[k0 // 2:k1 // 2, n * 128:(n + 1) * 128])
            res = _dot(o, _unpack(w), NN)
            side.done(step0 + n, res)
            cols.append(res)
        return jnp.concatenate(cols, axis=1)

    def phase2(u, carry):
        for i in range(UNROLL2):
            carry = phase2_tile(u * UNROLL2 + i, i % 2, carry, u < 0, u if LEAD and i == 0 else None)

        r0 = pl.multiple_of(u * (UNROLL2 * T), T)

        @pl.when(u == 0)
        def _():
            o_copy(0, UNROLL2 * T - TH, 0).start()

        @pl.when(u > 0)
        def _():
            o_copy(pl.multiple_of(jnp.maximum(r0 - TH, 0), TH), UNROLL2 * T, u).start()

        return carry

    def phase2_tile(t, slot, carry, never, lead):
        hp = jnp.maximum(2 * t - 1, 0)
        side = _Side(never)
        st = {"route": carry}
        side.add(LN2B_PLAN, lambda k, a: finish_rows(hb_v, k, hp, t > 0, st, side.never, a))

        def pack_ffn(k, a):
            if k < 32:
                n = D // NT_
                pack_rows(view((wg_v, wu_v)[k % 2], t, n), view((wgp_v, wup_v)[k % 2], t, n // 2),
                          (k // 4) * 16, 16, (0, D)[k // 2 % 2], (D, FM - D)[k // 2 % 2], never, a)
            else:
                n = (FF - FVD) // NT_
                pack_rows(view(wd_v, t, n, FVD), view(wdp_v, t, n // 2), (k - 32) * 16, 16, 0, D, never, a)
        side.add(PACK_PLAN[:32 + (FF - FVD) // 128], pack_ffn)

        xn = xn_tile(t)
        xt = view(x_v, t, T)
        os_ = []
        for c in range(NC):
            pq = proj_steps(side, 100 + 4 * c, 0, c, xn, lead if c == 0 else None)
            if c == 0:
                pq = side.gate(0, pq)
            q_features(pq, slot, c)
            if c > 0:
                os_.append(attn_rows(slot, c - 1, 0, T))
        oa = jnp.concatenate([o[0:TH, :] for o in os_[:2]], axis=1)
        ha0 = out_proj(side, 0, oa, 0, D // 2, 0, G3_AT)
        os_.append(attn_rows(slot, NC - 1, 0, T))
        ha1 = out_proj(side, 0, oa, 0, D // 2, G3_AT, D // 128)
        ha = jnp.concatenate([ha0, ha1], axis=1) + xt[0:TH, :].astype(F32)
        ha_v[...] = ha + out_proj(side, 8, jnp.concatenate([o[0:TH, :] for o in os_[2:]], axis=1), D // 2, D)
        side.add(LN2A_PLAN, lambda k, a: finish_rows(ha_v, k, 2 * t, None, st, side.never, a))
        ob = jnp.concatenate([o[TH:T, :] for o in os_], axis=1)
        hb_v[...] = xt[TH:T, :].astype(F32) + out_proj(side, 16, ob, 0, D)
        side.check()
        return st["route"]

    wg_copy.wait()
    wu_copy.wait()
    wd_copy.wait()
    route = lax.fori_loop(
        0, NT_ // UNROLL2, phase2,
        (jnp.full((8, 1), -jnp.inf, F32), jnp.zeros((8, 1), jnp.int32)))
    st = {"route": route}
    for k in range(TH // LNC):
        finish_rows(hb_v, k, 2 * NT_ - 1, None, st)
    best, besti = st["route"]
    o_copy(S - TH, TH, NT_).start()

    rmax = jnp.max(best, axis=0, keepdims=True)
    idx = jnp.min(jnp.where(best == rmax, besti, S), axis=0, keepdims=True)
    idx_s = jnp.clip(idx[0, 0], 0, S - 1)
    blk = pl.multiple_of((idx_s >> 4) << 4, 16)
    pair = jnp.broadcast_to(hn_v[pl.ds(idx_s >> 1, 1), :], (8, D))
    x8 = pltpu.bitcast(jnp.where((idx_s & 1) == 1, pair & jnp.uint32(0xFFFF0000), pair << 16), F32)
    xs = jnp.concatenate([x8, x8], axis=0).astype(BF16)
    acts, anchors = [], []

    def park(v, half):
        if not MOE_PARK:
            return v
        n = v.shape[0] // 128
        for i in range(n):
            z_v[i, :, 128 * half:128 * half + 128] = v[128 * i:128 * i + 128, :]
        return jnp.concatenate([z_v[i, :, 128 * half:128 * half + 128] for i in range(n)], axis=0)

    for c0 in range(0, FM, 128):
        g = _dot(xs, _unpack(wgp_v[:, c0:c0 + 128]), NN)[0:8, :]
        u = _dot(xs, _unpack(wup_v[:, c0:c0 + 128]), NN)[0:8, :]
        anchors += [g, u]
        acts.append(g * jax.nn.sigmoid(g) * u)
    xb = park(_col_broadcast(x8), 0)
    if MOE_SPLIT:
        g, u = [_sublane_allreduce(_vpu_matvec(
            xb, lambda g: w[8 * g:8 * g + 8, FM:FF].astype(F32), never0,
            anchors[i * MOE_NA // 2:(i + 1) * MOE_NA // 2], MOE_SPLIT)) for i, w in enumerate((wg_v, wu_v))]
    else:
        gu = _sublane_allreduce(_vpu_matvec(
            xb, lambda g: jnp.concatenate([w[8 * g:8 * g + 8, FM:FF].astype(F32) for w in (wg_v, wu_v)], axis=1),
            never0, anchors[:MOE_NA], 1))
        g, u = gu[:, :FV], gu[:, FV:]
    acts.append(g * jax.nn.sigmoid(g) * u)
    a = jnp.concatenate(acts, axis=1)
    am = jnp.concatenate([a[:, FVD:], a[:, FVD:]], axis=0).astype(BF16)
    ys, anchors = [], anchors[MOE_NA:]
    for k0 in range(0, FF - FVD, 512):
        k1 = min(k0 + 512, FF - FVD)
        yk = _dot(am[:, k0:k1], _unpack(wdp_v[k0 // 2:k1 // 2, :]), NN)[0:8, :]
        ys.append(yk)
        anchors += [yk[:, c:c + 128] for c in range(128, D, 256)]
    ys.append(_sublane_allreduce(_vpu_matvec(
        park(_col_broadcast(a[:, :FVD]), 1), lambda g: wd_v[8 * g:8 * g + 8, 0:D].astype(F32), never0, anchors[:-MOE_ND], MOE_LAG)))
    y = _tree(jnp.add, ys) * jax.nn.sigmoid(rmax)
    y = jnp.concatenate([y, y], axis=0)
    sel = lax.broadcasted_iota(jnp.int32, (16, 1), 0) == (idx_s - blk)
    patch_v[...] = (o_v[pl.ds(blk, 16), :].astype(F32) + jnp.where(sel, y, 0.0)).astype(BF16)
    o_copy(0, UNROLL2 * T - TH, 0).wait()
    for u in range(1, NT_ // UNROLL2):
        o_copy(u * UNROLL2 * T - TH, UNROLL2 * T, u).wait()
    o_copy(S - TH, TH, NT_).wait()
    pc = pltpu.make_async_copy(patch_v, out_hbm.at[pl.ds(blk, 16), :], sem.at[SM + 3])
    pc.start()
    pc.wait()


@jax.jit
def pallas_sequential_preLN__linear_kernel_hedgehog__moe_arch_mod__prompt_kernel(
    A_x: jax.Array,
    A_wqkv: jax.Array,
    A_w_phi: jax.Array,
    A_wo: jax.Array,
    B_x: jax.Array,
    B_w_r: jax.Array,
    B_w_gate: jax.Array,
    B_w_up: jax.Array,
    B_w_down: jax.Array,
):
    del B_x
    hbm = pl.BlockSpec(memory_space=pl.ANY)
    out = pl.pallas_call(
        _kernel,
        out_shape=jax.ShapeDtypeStruct((S, D), BF16),
        in_specs=[hbm] * 8,
        out_specs=hbm,
        scratch_shapes=[
            pltpu.VMEM((S, D), BF16),
            pltpu.VMEM((S // 2, D), U32),
            pltpu.VMEM((5 * D // 4, 128), U32),
            pltpu.VMEM((3 * NC, D, RC), BF16),
            [pltpu.VMEM((D // 2, D), U32)] * 3,
            pltpu.VMEM((H, DH, DH), BF16),
            pltpu.VMEM((8 * 64, 128), U32),
            pltpu.VMEM((D, D), BF16),
            pltpu.VMEM((D // 2, D), U32),
            pltpu.VMEM((D,), BF16),
            pltpu.VMEM((8, D), F32),
            pltpu.VMEM((NPAIR, 64, 128), F32),
            pltpu.VMEM((NPAIR * 32, 128), U32),
            pltpu.VMEM((NPAIR, 128, T), F32),
            pltpu.VMEM((NPAIR, 128, 128), F32),
            [pltpu.VMEM((NPAIR * 64, T), U32)] * 2,
            pltpu.VMEM((TH, D), F32),
            pltpu.VMEM((TH, D), F32),
            pltpu.VMEM((S // 2, D), U32),
            pltpu.VMEM((S, D), BF16),
            pltpu.VMEM((D, FFP), BF16),
            pltpu.VMEM((D, FFP), BF16),
            pltpu.VMEM((FF, D), BF16),
            pltpu.VMEM((D // 2, FM), U32),
            pltpu.VMEM((D // 2, FM), U32),
            pltpu.VMEM(((FF - FVD) // 2, D), U32),
            pltpu.VMEM((16, D), BF16),
            pltpu.SemaphoreType.DMA((6 + 3 * NC + NT_ + 11,)),
        ],
        compiler_params=pltpu.CompilerParams(vmem_limit_bytes=100 * 1024 * 1024,
                                             disable_semaphore_checks=True, disable_bounds_checks=True),
        name="hedgehog_mod",
    )(
        A_x.reshape(S, D),
        A_wqkv,
        A_w_phi,
        A_wo,
        B_w_r,
        B_w_gate,
        B_w_up,
        B_w_down,
    )
    return out.reshape(1, S, D)
```

```python
import math

import jax
import jax.numpy as jnp
from jax import lax
import jax.experimental.pallas as pl
import jax.experimental.pallas.tpu as pltpu

F32 = jnp.float32
BF16 = jnp.bfloat16
U32 = jnp.uint32

S = 2048
D = 1024
H = 32
DH = 32
FF = 3584
NPAIR = H // 2
LOG2E = 1.4426950408889634
LN_EPS = 1e-5

T = 256
TH = T // 2
NT_ = S // T
RC = 256
NC = D // RC
PPC = RC // 64
LNC = 16
FFP = 4096

FV = 10 * 128
FM = FF - FV
FVD = 8 * 128
WO_ROWS = 352
UNROLL2 = 2


def _spread(n, a, b, due=None):
    rel = [round(a + (b - a) * k / (n - 1), 3) for k in range(n)]
    return tuple((r, None if due is None else math.ceil(r) + due) for r in rel)


LN1_PLAN = _spread(16, 0, 13, 3)
WO_PLAN = _spread(11, 3, 13)
Z_PLAN = _spread(16, 2, 13, 2)
PRO_LN1_PLAN = ((None, None),) * 16
PRO_K_PLAN = _spread(8, 0, 6)
PRO_V_PLANS = (_spread(8, 0, 12), _spread(16, 13, 22)[:8], _spread(16, 13, 22)[8:], _spread(16, 1.2, 27, 3))
LN2B_PLAN = ((None, 0), (None, 0), (None, 0), (2.166, 8), (3.769, 9), (5.524, 11), (7.081, 13), (9.164, 15))
LN2A_PLAN = ((None, 18),) + _spread(7, 15.6, 20, 3)
PACK_PLAN = _spread(16, 100, 115) + _spread(16, 99.1, 114.1) + _spread(20, 0, 21)
G3_AT = 4
MOE_NA = 36
MOE_ND = 3
MOE_LAG = 2
MOE_ROT = 1
MOE_PARK = 1
MOE_SPLIT = 3
STAGGER = 8
LEAD = True
PACK_VIA_F32 = True

NN = (((1,), (0,)), ((), ()))
NT = (((1,), (1,)), ((), ()))


def _dot(a, b, dims):
    return lax.dot_general(a, b, dims, preferred_element_type=F32)


def _recip(x):
    return pl.reciprocal(x, approx=False, full_range=False)


def _pack(x):
    return pltpu.bitcast(x, U32)


def _unpack(x):
    return pltpu.bitcast(x, BF16)


def _pair_allreduce(a, op):
    a = op(a, pltpu.roll(a, 2, 0))
    return op(a, pltpu.roll(a, 4, 0))


def _tree(op, xs):
    xs = list(xs)
    while len(xs) > 1:
        nxt = [op(xs[i], xs[i + 1]) for i in range(0, len(xs) - 1, 2)]
        if len(xs) % 2:
            nxt.append(xs[-1])
        xs = nxt
    return xs[0]


def _pair_logits(sl, j):
    sub = lax.broadcasted_iota(jnp.int32, sl[0].shape, 0)
    if j < 3:
        head = jnp.where(sub < 2, 0.0, sl[(0, 1, 16)[j]])
    else:
        head = jnp.where(sub < 2, sl[0], jnp.where(sub < 4, pltpu.roll(sl[1], 2, 0),
                                                   jnp.where(sub < 6, pltpu.roll(sl[16], 4, 0), 0.0)))
    r0 = (2, 9, 17, 24)[j]
    return [head] + list(sl[r0:r0 + 7])


def _dual_exp(sl):
    mx = _pair_allreduce(_tree(jnp.maximum, sl), jnp.maximum)
    mn = _pair_allreduce(_tree(jnp.minimum, sl), jnp.minimum)
    ep = [jnp.exp2(s - mx) for s in sl]
    en = [jnp.exp2(mn - s) for s in sl]
    sp = _pair_allreduce(_tree(jnp.add, ep), jnp.add)
    sn = _pair_allreduce(_tree(jnp.add, en), jnp.add)
    return ep, en, sp, sn


def _after(x, never, anchor):
    if anchor is None:
        return x
    d = jnp.concatenate([anchor] * (x.shape[0] // 8), axis=0)
    if x.shape[1] == 128:
        return jnp.where(never, d, x)
    return jnp.concatenate([jnp.where(never, d, x[:, :128]), x[:, 128:]], axis=1)


def _gate(x, never, deps):
    for i, dep in enumerate(deps):
        d = jnp.broadcast_to(dep, (8, 128))
        if x.dtype != F32:
            d = pltpu.bitcast(d, x.dtype)
        blk = jnp.where(never, d, x[8 * i:8 * i + 8, :128])
        if x.shape[1] > 128:
            blk = jnp.concatenate([blk, x[8 * i:8 * i + 8, 128:]], axis=1)
        parts = ([x[:8 * i, :]] if i else []) + [blk, x[8 * i + 8:, :]]
        x = jnp.concatenate(parts, axis=0)
    return x


def _lane_fold(a):
    return _tree(jnp.add, [a[:, 128 * i:128 * i + 128] for i in range(a.shape[1] // 128)])


def _row_sum(a):
    return jnp.sum(_lane_fold(a), axis=-1, keepdims=True)


def _lane_tile(a, n):
    return a if n == 1 else jnp.concatenate([a] * n, axis=1)


def _sublane_allreduce(a):
    a = a + pltpu.roll(a, 4, 0)
    a = a + pltpu.roll(a, 2, 0)
    return a + pltpu.roll(a, 1, 0)


def _col_broadcast(row8):
    return jnp.concatenate([row8] * 16, axis=0).astype(BF16).T.astype(F32)


def _vpu_matvec(xb, w_rows, never, anchors, lag):
    ng = xb.shape[0] // 8
    acc, hist = None, []
    for g in range(ng):
        dep = anchors[(g * len(anchors)) // ng]
        if g >= lag:
            dep = dep + hist[g - lag]
        x = jnp.where(never, dep, xb[8 * g:8 * g + 8, :])
        w = w_rows(g)
        t = w * _lane_tile(x, w.shape[1] // 128)
        acc = t if acc is None else acc + t
        c = 128 * ((g * MOE_ROT) % (w.shape[1] // 128))
        hist.append(acc[:, c:c + 128])
    return acc


class _Side:
    def __init__(self, never):
        self.never = never
        self.jobs = []
        self.deps = {}

    def add(self, plan, fn):
        for k, (rel, due) in enumerate(plan):
            if rel is None:
                self._run(due, fn, k, None)
            else:
                self.jobs.append((rel, due, fn, k))

    def _run(self, due, fn, k, anchor):
        dep = fn(k, anchor)
        if due is not None:
            self.deps.setdefault(due, []).append(dep)

    def check(self):
        assert not self.jobs and not self.deps, (self.jobs, self.deps)

    def gate(self, step, x):
        return _gate(x, self.never, self.deps.pop(step, []))

    def done(self, step, res):
        m = res.shape[0] // 8
        for job in sorted([j for j in self.jobs if step - 1 < j[0] <= step], key=lambda j: j[0]):
            self.jobs.remove(job)
            g = m - 1 - int((step - job[0]) * m)
            self._run(job[1], job[2], job[3], res[8 * g:8 * g + 8, res.shape[1] - 128:])


def _kernel(x_hbm, wqkv_hbm, wphi_hbm, wo_hbm, wr_hbm, wg_hbm, wu_hbm, wd_hbm, out_hbm,
            x_v, xn_v, lead_v, wraw_v, wt_v, wphi_v, a_v, woraw_v, wo_v, wrraw_v, wr_v, kvacc_v, kvbf_v,
            z_v, zb_v, phi_v, ha_v, hb_v, hn_v, o_v, wg_v, wu_v, wd_v, wgp_v, wup_v, wdp_v, patch_v,
            sem):
    SX, SW, SO, SM = 0, 6, 6 + 3 * NC, 6 + 3 * NC + NT_ + 1

    def x_copy(i):
        h0, h1 = ((1, 2), (2, 4), (4, 6), (6, 10), (10, 2 * NT_), (0, 1))[i]
        rows = pl.ds(h0 * TH, (h1 - h0) * TH)
        return pltpu.make_async_copy(x_hbm.at[rows, :], x_v.at[rows, :], sem.at[SX + i])

    def k0_copy(s):
        return pltpu.make_async_copy(wqkv_hbm.at[:, pl.ds(D + s * 128, 128)],
                                     wraw_v.at[NC, :, pl.ds(s * 128, 128)], sem.at[(SM + 7, SW + NC)[s]])

    def w_copy(j, c):
        return pltpu.make_async_copy(wqkv_hbm.at[:, pl.ds(j * D + c * RC, RC)], wraw_v.at[j * NC + c],
                                     sem.at[SW + j * NC + c])

    def wphi_copy(i):
        h0, h1 = ((0, 8), (8, 16), (16, H))[i]
        return pltpu.make_async_copy(wphi_hbm.at[pl.ds(h0, h1 - h0)], wphi_v.at[pl.ds(h0, h1 - h0)],
                                     sem.at[(SM + 4, SM + 8, SM + 9)[i]])

    wr_copy = pltpu.make_async_copy(wr_hbm, wrraw_v, sem.at[SM + 5])
    wo_copy = pltpu.make_async_copy(wo_hbm, woraw_v, sem.at[SM + 6])
    wg_copy = pltpu.make_async_copy(wg_hbm, wg_v.at[:, pl.ds(0, FF)], sem.at[SM + 0])
    wu_copy = pltpu.make_async_copy(wu_hbm, wu_v.at[:, pl.ds(0, FF)], sem.at[SM + 1])
    wd_copy = pltpu.make_async_copy(wd_hbm, wd_v, sem.at[SM + 2])

    wphi_copy(0).start()
    k0_copy(0).start()
    x_copy(5).start()
    k0_copy(1).start()
    x_copy(0).start()
    wphi_copy(1).start()
    w_copy(1, 1).start()

    def view(ref, i, n, off=0):
        r0 = off + i * n
        return ref.at[pl.ds(r0 if isinstance(r0, int) else pl.multiple_of(r0, math.gcd(n, off)), n), :]

    def ln_rows(t, k, n, never=None, anchor=None):
        x = _after(view(x_v, t, T)[k * n:(k + 1) * n, :].astype(F32), never, anchor)
        xc = x - _row_sum(x) * (1.0 / D)
        rstd = lax.rsqrt(_row_sum(xc * xc) * (1.0 / D) + LN_EPS)
        view(xn_v, t, T // 2)[k * n // 2:(k + 1) * n // 2, :] = _pack((xc * rstd).astype(BF16))
        return _tree(jnp.add, [rstd[8 * i:8 * i + 8, :] for i in range(min(n, LNC) // 8)])

    def xn_tile(t):
        return _unpack(view(xn_v, t, T // 2)[...])

    def expand_wphi(c):
        w = wphi_v[8 * c:8 * c + 8].reshape(8 * DH, DH).astype(F32).T
        bits = pltpu.bitcast(w, U32)
        head = lax.broadcasted_iota(jnp.int32, (DH, 128), 1) >> 5
        for s in range(2):
            b = bits[:, 128 * s:128 * s + 128]
            for j in range(2):
                r0 = 64 * (2 * c + s) + 32 * j
                a_v[r0:r0 + 32, :] = jnp.where(head == 2 * j, b >> 16,
                                               jnp.where(head == 2 * j + 1, b, jnp.uint32(0)))

    wphi_copy(0).wait()
    expand_wphi(0)
    hb_v[...] = jnp.zeros((TH, D), F32)

    def fold_v(c):
        for s in range(RC // 128):
            g0 = 64 * (2 * c + s)
            wt_v[2][g0:g0 + 64, :] = _pack(wraw_v[2 * NC + c, :, s * 128:(s + 1) * 128].T)

    def fold_pairs(j, c, s, side=None, step0=None):
        g0 = 64 * (2 * c + s)
        g0 = g0 if isinstance(g0, int) else pl.multiple_of(g0, 64)
        res = _dot(_unpack(a_v[pl.ds(g0, 64), :]), wraw_v[j * NC + c, :, s * 128:(s + 1) * 128], NT)
        if side is not None:
            side.done(step0 + 2 * s, res[:, :D // 2])
            side.done(step0 + 2 * s + 1, res[:, D // 2:])
        sub = lax.broadcasted_iota(jnp.int32, (8, D), 0)
        out = []
        for q in range(2):
            base = _pair_allreduce(jnp.where(sub < 2, res[64 * q:64 * q + 8, :], 0.0), jnp.add)
            out.append([(res[64 * q + 8 * i:64 * q + 8 * i + 8, :] - base) * LOG2E for i in range(8)])
        return out

    def share(z, z3, k):
        sub = lax.broadcasted_iota(jnp.int32, (8, D), 0)
        return jnp.where(sub < 2, pltpu.roll(z3, 8 - 2 * k, 0), z)

    def packed(slabs):
        return _pack(jnp.concatenate(slabs, axis=0).astype(BF16))

    def fold(j, c, side=None, step0=None):
        p0, p1 = fold_pairs(j, c, 0, side, step0)
        p2, p3 = fold_pairs(j, c, 1, side, step0)
        sl = ([share(p0[0], p3[0], 1), share(p1[0], p3[0], 2)] + p0[1:] + p1[1:]
              + [share(p2[0], p3[0], 3)] + p2[1:] + p3[1:])
        zero = jnp.zeros((8, D), F32)
        even, odd = sl + [zero], [zero] + sl
        r0 = 8 * ((31 * c) // 2)
        if isinstance(c, int):
            is_odd = c % 2 == 1
            sl = odd if is_odd else even
        else:
            is_odd = c % 2 == 1
            r0 = pl.multiple_of(r0, 8)
            sl = [jnp.where(is_odd, o, e) for o, e in zip(odd, even)]
        win = wt_v[j].at[pl.ds(r0, 128), :]
        win[8:128, :] = packed(sl[2:])
        first = packed(sl[:2])
        if is_odd is not False:
            keep = lax.broadcasted_iota(jnp.int32, (8, D), 0) < jnp.where(is_odd, 4, 0)
            first = jnp.where(keep, win[0:8, :], first)
        win[0:8, :] = first

    def k_pair(p, slot, pr, c0, first, never=None):
        ep, en, sp, sn = _dual_exp(p)
        inv = _recip(sp * sn)
        scale = (sn * inv, sp * inv)
        es = ep + en
        cols = slice(c0, c0 + p[0].shape[1])
        n = 16 if never is None else 16 // STAGGER
        last = None
        for q in range(16 // n):
            sc = scale
            if last is not None:
                sc = [jnp.where(never, last, x) for x in scale]
            phi = jnp.concatenate([es[i] * sc[i // 8] for i in range(q * n, (q + 1) * n)], axis=0)
            rows = slice(8 * q * n, 8 * (q + 1) * n)
            z = phi if first else z_v[pr, rows, cols] + phi
            z_v[pr, rows, cols] = z
            phi_v[slot][64 * pr + 4 * q * n:64 * pr + 4 * (q + 1) * n, cols] = _pack(phi.astype(BF16))
            last = z[8 * n - 8:, :]

    def k_features(pk, slot, c, first, never=None):
        for j in range(PPC):
            k_pair(_pair_logits(pk, j), slot, c * PPC + j, 0, first, never)

    row = lax.broadcasted_iota(jnp.int32, (64, 128), 0)
    col = lax.broadcasted_iota(jnp.int32, (64, 128), 1)
    kv_keep = (row >> 5) == (col & 1)

    def kv_update(vt, slot, c, first, publish=False):
        for j in range(PPC):
            pr = c * PPC + j
            upd = _dot(vt[64 * j:64 * j + 64, :].astype(BF16), _unpack(phi_v[slot][64 * pr:64 * pr + 64, :]), NT)
            acc = upd if first else kvacc_v[pr] + upd
            kvacc_v[pr] = acc
            if publish:
                kvbf_v[32 * pr:32 * pr + 32, :] = _pack(jnp.where(kv_keep, acc, 0.0).astype(BF16))

    def save_lead(e, t):
        corner = _unpack(view(xn_v, t, T // 2)[0:TH // 2, 0:D // 2])
        view(lead_v, e, D // 4)[...] = _pack(corner.T)

    def proj_steps(side, step0, w, xn, lead=None):
        quarters = []
        for n in range(2):
            for m in range(2):
                step = step0 + 2 * n + m
                wq = _unpack(side.gate(step, w[:64, :] if m == 0 else w[64:, :]))
                if lead is not None and n + m == 0:
                    res = _dot(wq[:, :D // 2], _unpack(view(lead_v, lead, D // 4)[...]), NN)
                    res = _dot(wq[:, D // 2:], xn[0:TH, D // 2:], NT) + res
                else:
                    res = _dot(wq, xn[n * TH:(n + 1) * TH, :], NT)
                side.done(step, res)
                quarters.append(res)
        return jnp.concatenate(
            [jnp.concatenate([quarters[0], quarters[2]], axis=1),
             jnp.concatenate([quarters[1], quarters[3]], axis=1)], axis=0)

    def proj_v(side, step0, c, xn):
        return proj_steps(side, step0, wt_v[2][128 * c:128 * c + 128, :], xn)

    def proj_feat(side, step0, j, c, xn, carry, lead=None):
        r0 = 8 * ((31 * c) // 2)
        skip = 8 if c % 2 == 1 and carry is not None else 0
        res = proj_steps(side, step0, wt_v[j][r0 + skip:r0 + 128, :], xn, lead)
        sl = [res[8 * i:8 * i + 8, :] for i in range(res.shape[0] // 8)]
        if c % 2 == 0:
            return sl[:31], sl[31]
        return ([carry] + sl if skip else sl[1:]), None

    def pack_rows(src, dst, r0, rows, c0, cols, never, a):
        if PACK_VIA_F32:
            w = src[r0:r0 + rows, c0:c0 + cols].astype(F32)
            d = _lane_tile(a, cols // 128)
            w = jnp.concatenate([jnp.where(never, d, w[8 * i:8 * i + 8, :]) if i % 2 == 0 else w[8 * i:8 * i + 8, :]
                                 for i in range(rows // 8)], axis=0)
            dst[r0 // 2:(r0 + rows) // 2, c0:c0 + cols] = _pack(w.astype(BF16))
            return
        w = _pack(src[r0:r0 + rows, c0:c0 + cols])
        d = jnp.concatenate([_lane_tile(pltpu.bitcast(a, U32), cols // 128)] * (rows // 16), axis=0)
        dst[r0 // 2:(r0 + rows) // 2, c0:c0 + cols] = jnp.where(never, d, w)

    def stash_at(i, k, n):
        return zb_v.at[4 * i + 2 * (k // 16) + n, pl.ds(8 * (k % 16), 8), :]

    def stash(i, sl):
        for k, v in enumerate(sl):
            for n in range(2):
                stash_at(i, k, n)[...] = v[:, 128 * n:128 * n + 128]

    def stashed_k(i, slot, c, first):
        def job(k, a):
            j, n = k // 2, k % 2
            p = _pair_logits([stash_at(i, q, n)[...] for q in range(31)], j)
            k_pair([_after(p[0], never0, a)] + p[1:], slot, c * PPC + j, 128 * n, first, never0)
        return job

    def first_rows(k0, k1, n):
        xn = _unpack(xn_v[n * TH // 2:(n + 1) * TH // 2, :])
        ks = [k for k in range(k0, k1)]
        w = jnp.concatenate([wt_v[1][4 * (k % 32):4 * (k % 32) + 8, :] for k in ks[::2]], axis=0)
        res = _dot(_unpack(w), xn, NT)
        for q, k in enumerate(ks):
            if k % 32 < 31:
                stash_at(0, k % 32, n)[...] = res[8 * q:8 * q + 8, :]

    k0_copy(0).wait()
    x_copy(5).wait()
    wphi_copy(2).start()
    w_copy(1, 2).start()
    x_copy(1).start()
    p0, p1 = fold_pairs(1, 0, 0)
    wt_v[1][8:64, :] = packed(p0[1:] + p1[1:])
    ha_v[0:8, :] = p0[0]
    ha_v[8:16, :] = p1[0]
    never0 = ln_rows(0, 0, TH)[0, 0] < 0.0
    first_rows(2, 16, 0)

    k0_copy(1).wait()
    x_copy(0).wait()
    wphi_copy(1).wait()
    w_copy(1, 3).start()
    for c in range(NC):
        w_copy(2, c).start()
    p2, p3 = fold_pairs(1, 0, 1)
    wt_v[1][0:8, :] = packed([share(ha_v[0:8, :], p3[0], 1), share(ha_v[8:16, :], p3[0], 2)])
    wt_v[1][64:128, :] = packed([share(p2[0], p3[0], 3)] + p2[1:] + p3[1:] + [jnp.zeros((8, D), F32)])
    ln_rows(0, 1, TH)
    first_rows(16, 34, 0)
    first_rows(0, 16, 1)
    first_rows(16, 32, 1)
    expand_wphi(1)

    for c in (1, 2):
        w_copy(1, c).wait()
        if c == 1:
            wphi_copy(2).wait()
            expand_wphi(2)
            expand_wphi(3)
            x_copy(2).start()
            for cq in range(NC):
                w_copy(0, cq).start()
        else:
            x_copy(3).start()
            wo_copy.start()
            wr_copy.start()
            x_copy(4).start()
        side = _Side(never0)
        side.add(PRO_K_PLAN, stashed_k(c - 1, 0, c - 1, True))
        fold(1, c, side, 0)
        stash(c, proj_feat(side, 4, 1, c, xn_tile(0), None)[0])
        side.check()

    x_copy(1).wait()
    w_copy(1, 3).wait()
    wg_copy.start()
    wu_copy.start()
    wd_copy.start()
    side = _Side(never0)
    side.add(PRO_LN1_PLAN, lambda k, a: ln_rows(1, k, LNC, never0, a))
    fold(1, 3, side, 0)
    stash(3, proj_feat(side, 4, 1, 3, xn_tile(0), None)[0])
    xn1 = xn_tile(1)
    spare = None
    for c in range(NC):
        pk, spare = proj_feat(_Side(None), 0, 1, c, xn1, spare)
        if c < 3:
            k_features(pk, 1, c, c == 2, never0)
        else:
            stash(0, pk)

    for c in range(NC):
        w_copy(2, c).wait()
    x_copy(2).wait()
    w_copy(0, 0).wait()
    side = _Side(never0)
    side.add(PRO_V_PLANS[0], stashed_k(2, 0, 2, False))
    side.add(PRO_V_PLANS[1], stashed_k(3, 0, 3, True))
    side.add(PRO_V_PLANS[2], stashed_k(0, 1, 3, False))
    side.add(PRO_V_PLANS[3], lambda k, a: ln_rows(2, k, LNC, never0, a))
    fold(0, 0)
    wt_v[0][248:256, :] = jnp.zeros((8, D), U32)
    xns = (xn_tile(0), xn_tile(1))
    pending = None
    for c in range(NC):
        fold_v(c)
        for i in range(2):
            vt = proj_v(side, 8 * c + 4 * i, c, xns[i])
            if pending is not None:
                kv_update(*pending)
            pending = (vt, i, c, i == 0)
    side.check()
    kv_update(*pending)
    save_lead(0, 0)
    save_lead(1, 2)

    def phase1(u, carry):
        never = u < 0

        @pl.when(u == 0)
        def _():
            for c in range(1, NC):
                w_copy(0, c).wait()
            x_copy(3).wait()
            wo_copy.wait()
            wr_copy.wait()

        @pl.when(u == 1)
        def _():
            x_copy(4).wait()

        pending = None
        for i in range(2):
            t = 2 * u + 2 + i
            tn = jnp.minimum(t + 1, NT_ - 1)
            side = _Side(never)
            xn = xn_tile(t)
            spare = None
            for c in range(NC):
                pk, spare = proj_feat(_Side(None), 0, 1, c, xn, spare, u + 1 if LEAD and i + c == 0 else None)
                if c == 0 and pending is not None:
                    kv_update(*pending)
                k_features(pk, i, c, False)
            side.add(LN1_PLAN, lambda k, a: ln_rows(tn, k, LNC, never, a))
            if i == 0:
                def pack_wo(k, a):
                    rows = WO_ROWS // len(WO_PLAN)
                    w0 = u * ((D - WO_ROWS) // 2)
                    src = woraw_v.at[pl.ds(pl.multiple_of(w0, 16), WO_ROWS), :]
                    dst = wo_v.at[pl.ds(pl.multiple_of(w0 // 2, 8), WO_ROWS // 2), :]
                    pack_rows(src, dst, k * rows, rows, 0, D, never, a)
                side.add(WO_PLAN, pack_wo)
            else:
                def z_final(k, a):
                    z = _after(z_v[k], never, a)
                    zs = _row_sum(z)
                    zb_v[k] = jnp.broadcast_to(zs, (128, 128))
                    return zs[120:128, :]
                side.add(Z_PLAN, z_final)
            side.done(0, jnp.concatenate(pk[17:], axis=0))
            vts = []
            for c in range(NC):
                vts.append(proj_v(side, 4 * c + 1, c, xn))
                if c > 0:
                    kv_update(vts[c - 1], i, c - 1, False, i == 1)
            pending = (vts[NC - 1], i, NC - 1, False, i == 1)
            side.check()
        fold(0, u + 1)
        kv_update(*pending)
        save_lead(u + 2, tn)
        wr_v[...] = jnp.broadcast_to(wrraw_v[...].reshape(1, D).astype(F32), (8, D))
        return carry

    lax.fori_loop(0, (NT_ - 2) // 2, phase1, 0)

    def o_copy(r0, n, i):
        return pltpu.make_async_copy(o_v.at[pl.ds(r0, n), :], out_hbm.at[pl.ds(r0, n), :], sem.at[SO + i])

    def finish_rows(h_ref, k, ht, valid, st, never=None, anchor=None):
        r0 = ht * TH + k * LNC
        best, besti = st["route"]
        wr = jnp.concatenate([wr_v[...]] * (LNC // 8), axis=0)
        sub = lax.broadcasted_iota(jnp.int32, (8, 1), 0)
        h = _after(h_ref[k * LNC:(k + 1) * LNC, :], never, anchor)
        hc = h - _row_sum(h) * (1.0 / D)
        rstd = lax.rsqrt(_row_sum(hc * hc) * (1.0 / D) + LN_EPS)
        r = (_row_sum(hc * wr) * rstd).astype(BF16).astype(F32)
        hn = hc * rstd
        view(hn_v, ht, TH // 2)[k * LNC // 2:(k + 1) * LNC // 2, :] = _pack(hn.astype(BF16))
        view(o_v, ht, TH)[k * LNC:(k + 1) * LNC, :] = (hn + h).astype(BF16)
        if valid is not None:
            r = jnp.where(valid, r, -jnp.inf)
        for i in range(LNC // 8):
            ri = r[8 * i:8 * i + 8, :]
            better = ri > best
            best = jnp.where(better, ri, best)
            besti = jnp.where(better, sub + (r0 + 8 * i), besti)
        st["route"] = (best, besti)
        return best

    def q_features(pq, slot, c):
        for j in range(PPC):
            pr = c * PPC + j
            ep, en, sp, sn = _dual_exp(_pair_logits(pq, j))
            zz = [_lane_tile(zb_v[pr, 8 * i:8 * i + 8, :], T // 128) for i in range(16)]
            ap = _pair_allreduce(_tree(jnp.add, [ep[i] * zz[i] for i in range(8)]), jnp.add)
            an = _pair_allreduce(_tree(jnp.add, [en[i] * zz[8 + i] for i in range(8)]), jnp.add)
            inv = _recip(ap * sn + (an + 1e-6 * sn) * sp)
            rp = sn * inv
            rn = sp * inv
            phi = jnp.concatenate([e * rp for e in ep] + [e * rn for e in en], axis=0)
            phi_v[slot][64 * pr:64 * pr + 64, :] = _pack(phi.astype(BF16))

    def attn_rows(slot, c, lo, hi):
        res = jnp.concatenate(
            [_dot(_unpack(kvbf_v[32 * pr:32 * pr + 32, :]), _unpack(phi_v[slot][64 * pr:64 * pr + 64, lo:hi]), NN)
             for pr in range(c * PPC, (c + 1) * PPC)], axis=0)
        return res.astype(BF16).T

    def out_proj(side, step0, o, k0, k1, n0=0, n1=D // 128):
        cols = []
        for n in range(n0, n1):
            w = side.gate(step0 + n, wo_v[k0 // 2:k1 // 2, n * 128:(n + 1) * 128])
            res = _dot(o, _unpack(w), NN)
            side.done(step0 + n, res)
            cols.append(res)
        return jnp.concatenate(cols, axis=1)

    def phase2(u, carry):
        for i in range(UNROLL2):
            carry = phase2_tile(u * UNROLL2 + i, i % 2, carry, u < 0, u if LEAD and i == 0 else None)

        r0 = pl.multiple_of(u * (UNROLL2 * T), T)

        @pl.when(u == 0)
        def _():
            o_copy(0, UNROLL2 * T - TH, 0).start()

        @pl.when(u > 0)
        def _():
            o_copy(pl.multiple_of(jnp.maximum(r0 - TH, 0), TH), UNROLL2 * T, u).start()

        return carry

    def phase2_tile(t, slot, carry, never, lead):
        hp = jnp.maximum(2 * t - 1, 0)
        side = _Side(never)
        st = {"route": carry}
        side.add(LN2B_PLAN, lambda k, a: finish_rows(hb_v, k, hp, t > 0, st, side.never, a))

        def pack_ffn(k, a):
            if k < 32:
                n = D // NT_
                pack_rows(view((wg_v, wu_v)[k % 2], t, n), view((wgp_v, wup_v)[k % 2], t, n // 2),
                          (k // 4) * 16, 16, (0, D)[k // 2 % 2], (D, FM - D)[k // 2 % 2], never, a)
            else:
                n = (FF - FVD) // NT_
                pack_rows(view(wd_v, t, n, FVD), view(wdp_v, t, n // 2), (k - 32) * 16, 16, 0, D, never, a)
        side.add(PACK_PLAN[:32 + (FF - FVD) // 128], pack_ffn)

        xn = xn_tile(t)
        xt = view(x_v, t, T)
        os_ = []
        spare = None
        for c in range(NC):
            pq, spare = proj_feat(side, 100 + 4 * c, 0, c, xn, spare, lead if c == 0 else None)
            if c == 0:
                head = side.gate(0, jnp.concatenate(pq[2:9], axis=0))
                pq = pq[:2] + [head[8 * i:8 * i + 8, :] for i in range(7)] + pq[9:]
            q_features(pq, slot, c)
            if c > 0:
                os_.append(attn_rows(slot, c - 1, 0, T))
        oa = jnp.concatenate([o[0:TH, :] for o in os_[:2]], axis=1)
        ha0 = out_proj(side, 0, oa, 0, D // 2, 0, G3_AT)
        os_.append(attn_rows(slot, NC - 1, 0, T))
        ha1 = out_proj(side, 0, oa, 0, D // 2, G3_AT, D // 128)
        ha = jnp.concatenate([ha0, ha1], axis=1) + xt[0:TH, :].astype(F32)
        ha_v[...] = ha + out_proj(side, 8, jnp.concatenate([o[0:TH, :] for o in os_[2:]], axis=1), D // 2, D)
        side.add(LN2A_PLAN, lambda k, a: finish_rows(ha_v, k, 2 * t, None, st, side.never, a))
        ob = jnp.concatenate([o[TH:T, :] for o in os_], axis=1)
        hb_v[...] = xt[TH:T, :].astype(F32) + out_proj(side, 16, ob, 0, D)
        side.check()
        return st["route"]

    wg_copy.wait()
    wu_copy.wait()
    wd_copy.wait()
    route = lax.fori_loop(
        0, NT_ // UNROLL2, phase2,
        (jnp.full((8, 1), -jnp.inf, F32), jnp.zeros((8, 1), jnp.int32)))
    st = {"route": route}
    for k in range(TH // LNC):
        finish_rows(hb_v, k, 2 * NT_ - 1, None, st)
    best, besti = st["route"]
    o_copy(S - TH, TH, NT_).start()

    rmax = jnp.max(best, axis=0, keepdims=True)
    idx = jnp.min(jnp.where(best == rmax, besti, S), axis=0, keepdims=True)
    idx_s = jnp.clip(idx[0, 0], 0, S - 1)
    blk = pl.multiple_of((idx_s >> 4) << 4, 16)
    pair = jnp.broadcast_to(hn_v[pl.ds(idx_s >> 1, 1), :], (8, D))
    x8 = pltpu.bitcast(jnp.where((idx_s & 1) == 1, pair & jnp.uint32(0xFFFF0000), pair << 16), F32)
    xs = jnp.concatenate([x8, x8], axis=0).astype(BF16)
    acts, anchors = [], []

    def park(v, half):
        if not MOE_PARK:
            return v
        n = v.shape[0] // 128
        for i in range(n):
            z_v[i, :, 128 * half:128 * half + 128] = v[128 * i:128 * i + 128, :]
        return jnp.concatenate([z_v[i, :, 128 * half:128 * half + 128] for i in range(n)], axis=0)

    for c0 in range(0, FM, 128):
        g = _dot(xs, _unpack(wgp_v[:, c0:c0 + 128]), NN)[0:8, :]
        u = _dot(xs, _unpack(wup_v[:, c0:c0 + 128]), NN)[0:8, :]
        anchors += [g, u]
        acts.append(g * jax.nn.sigmoid(g) * u)
    xb = park(_col_broadcast(x8), 0)
    if MOE_SPLIT:
        g, u = [_sublane_allreduce(_vpu_matvec(
            xb, lambda g: w[8 * g:8 * g + 8, FM:FF].astype(F32), never0,
            anchors[i * MOE_NA // 2:(i + 1) * MOE_NA // 2], MOE_SPLIT)) for i, w in enumerate((wg_v, wu_v))]
    else:
        gu = _sublane_allreduce(_vpu_matvec(
            xb, lambda g: jnp.concatenate([w[8 * g:8 * g + 8, FM:FF].astype(F32) for w in (wg_v, wu_v)], axis=1),
            never0, anchors[:MOE_NA], 1))
        g, u = gu[:, :FV], gu[:, FV:]
    acts.append(g * jax.nn.sigmoid(g) * u)
    a = jnp.concatenate(acts, axis=1)
    am = jnp.concatenate([a[:, FVD:], a[:, FVD:]], axis=0).astype(BF16)
    ys, anchors = [], anchors[MOE_NA:]
    for k0 in range(0, FF - FVD, 512):
        k1 = min(k0 + 512, FF - FVD)
        yk = _dot(am[:, k0:k1], _unpack(wdp_v[k0 // 2:k1 // 2, :]), NN)[0:8, :]
        ys.append(yk)
        anchors += [yk[:, c:c + 128] for c in range(128, D, 256)]
    ys.append(_sublane_allreduce(_vpu_matvec(
        park(_col_broadcast(a[:, :FVD]), 1), lambda g: wd_v[8 * g:8 * g + 8, 0:D].astype(F32), never0, anchors[:-MOE_ND], MOE_LAG)))
    y = _tree(jnp.add, ys) * jax.nn.sigmoid(rmax)
    y = jnp.concatenate([y, y], axis=0)
    sel = lax.broadcasted_iota(jnp.int32, (16, 1), 0) == (idx_s - blk)
    patch_v[...] = (o_v[pl.ds(blk, 16), :].astype(F32) + jnp.where(sel, y, 0.0)).astype(BF16)
    o_copy(0, UNROLL2 * T - TH, 0).wait()
    for u in range(1, NT_ // UNROLL2):
        o_copy(u * UNROLL2 * T - TH, UNROLL2 * T, u).wait()
    o_copy(S - TH, TH, NT_).wait()
    pc = pltpu.make_async_copy(patch_v, out_hbm.at[pl.ds(blk, 16), :], sem.at[SM + 3])
    pc.start()
    pc.wait()


@jax.jit
def pallas_sequential_preLN__linear_kernel_hedgehog__moe_arch_mod__prompt_kernel(
    A_x: jax.Array,
    A_wqkv: jax.Array,
    A_w_phi: jax.Array,
    A_wo: jax.Array,
    B_x: jax.Array,
    B_w_r: jax.Array,
    B_w_gate: jax.Array,
    B_w_up: jax.Array,
    B_w_down: jax.Array,
):
    del B_x
    hbm = pl.BlockSpec(memory_space=pl.ANY)
    out = pl.pallas_call(
        _kernel,
        out_shape=jax.ShapeDtypeStruct((S, D), BF16),
        in_specs=[hbm] * 8,
        out_specs=hbm,
        scratch_shapes=[
            pltpu.VMEM((S, D), BF16),
            pltpu.VMEM((S // 2, D), U32),
            pltpu.VMEM((5 * D // 4, 128), U32),
            pltpu.VMEM((3 * NC, D, RC), BF16),
            [pltpu.VMEM((D // 2, D), U32)] * 3,
            pltpu.VMEM((H, DH, DH), BF16),
            pltpu.VMEM((8 * 64, 128), U32),
            pltpu.VMEM((D, D), BF16),
            pltpu.VMEM((D // 2, D), U32),
            pltpu.VMEM((D,), BF16),
            pltpu.VMEM((8, D), F32),
            pltpu.VMEM((NPAIR, 64, 128), F32),
            pltpu.VMEM((NPAIR * 32, 128), U32),
            pltpu.VMEM((NPAIR, 128, T), F32),
            pltpu.VMEM((NPAIR, 128, 128), F32),
            [pltpu.VMEM((NPAIR * 64, T), U32)] * 2,
            pltpu.VMEM((TH, D), F32),
            pltpu.VMEM((TH, D), F32),
            pltpu.VMEM((S // 2, D), U32),
            pltpu.VMEM((S, D), BF16),
            pltpu.VMEM((D, FFP), BF16),
            pltpu.VMEM((D, FFP), BF16),
            pltpu.VMEM((FF, D), BF16),
            pltpu.VMEM((D // 2, FM), U32),
            pltpu.VMEM((D // 2, FM), U32),
            pltpu.VMEM(((FF - FVD) // 2, D), U32),
            pltpu.VMEM((16, D), BF16),
            pltpu.SemaphoreType.DMA((6 + 3 * NC + NT_ + 11,)),
        ],
        compiler_params=pltpu.CompilerParams(vmem_limit_bytes=100 * 1024 * 1024,
                                             disable_semaphore_checks=True, disable_bounds_checks=True),
        name="hedgehog_mod",
    )(
        A_x.reshape(S, D),
        A_wqkv,
        A_w_phi,
        A_wo,
        B_w_r,
        B_w_gate,
        B_w_up,
        B_w_down,
    )
    return out.reshape(1, S, D)
```

```python
import math

import jax
import jax.numpy as jnp
from jax import lax
import jax.experimental.pallas as pl
import jax.experimental.pallas.tpu as pltpu

F32 = jnp.float32
BF16 = jnp.bfloat16
U32 = jnp.uint32

S = 2048
D = 1024
H = 32
DH = 32
FF = 3584
NPAIR = H // 2
LOG2E = 1.4426950408889634
LN_EPS = 1e-5

T = 256
TH = T // 2
NT_ = S // T
RC = 256
NC = D // RC
PPC = RC // 64
LNC = 16
FFP = 4096

FV = 10 * 128
FM = FF - FV
FVD = 8 * 128
WO_ROWS = 352
UNROLL2 = 2


def _spread(n, a, b, due=None):
    rel = [round(a + (b - a) * k / (n - 1), 3) for k in range(n)]
    return tuple((r, None if due is None else math.ceil(r) + due) for r in rel)


LN1_PLAN = _spread(16, 0, 13, 3)
WO_PLAN = _spread(11, 3, 13)
Z_PLAN = _spread(16, 6, 14, 2)
PRO_LN1_PLAN = ((None, None),) * 16
PRO_K_PLAN = _spread(8, 0, 6)
PRO_V_PLANS = (_spread(8, 0, 12), _spread(16, 13, 22)[:8], _spread(16, 13, 22)[8:], _spread(16, 1.2, 27, 3))
LN2B_PLAN = ((None, 103), (-0.13, 6), (1.532, 8), (3.446, 10), (4.894, 11), (6.571, 13), (8.519, 15), (9.867, 15))
LN2A_PLAN = ((None, 18), (15.227, 19), (16.121, 20), (16.864, 20), (17.647, 21), (18.474, 22), (19.118, 23), (20.038, None))
PACK_PLAN = _spread(16, 99.7, 114.7) + _spread(16, 99.1, 114.1) + _spread(20, 0.5, 21)
G_STEPS = (107, 107, 111, 111, 115, 115, 3, 3)
Q_STAGGER = 1
MOE_NA = 36
MOE_ND = 3
MOE_LAG = 2
MOE_ROT = 1
MOE_PARK = 1
MOE_SPLIT = 3
STAGGER = 8
LEAD = True
PACK_VIA_F32 = True

NN = (((1,), (0,)), ((), ()))
NT = (((1,), (1,)), ((), ()))


def _dot(a, b, dims):
    return lax.dot_general(a, b, dims, preferred_element_type=F32)


def _recip(x):
    return pl.reciprocal(x, approx=False, full_range=False)


def _pack(x):
    return pltpu.bitcast(x, U32)


def _unpack(x):
    return pltpu.bitcast(x, BF16)


def _pair_allreduce(a, op):
    a = op(a, pltpu.roll(a, 2, 0))
    return op(a, pltpu.roll(a, 4, 0))


def _tree(op, xs):
    xs = list(xs)
    while len(xs) > 1:
        nxt = [op(xs[i], xs[i + 1]) for i in range(0, len(xs) - 1, 2)]
        if len(xs) % 2:
            nxt.append(xs[-1])
        xs = nxt
    return xs[0]


def _pair_logits(sl, j):
    sub = lax.broadcasted_iota(jnp.int32, sl[0].shape, 0)
    if j < 3:
        head = jnp.where(sub < 2, 0.0, sl[(0, 1, 16)[j]])
    else:
        head = jnp.where(sub < 2, sl[0], jnp.where(sub < 4, pltpu.roll(sl[1], 2, 0),
                                                   jnp.where(sub < 6, pltpu.roll(sl[16], 4, 0), 0.0)))
    r0 = (2, 9, 17, 24)[j]
    return [head] + list(sl[r0:r0 + 7])


def _dual_exp(sl):
    mx = _pair_allreduce(_tree(jnp.maximum, sl), jnp.maximum)
    mn = _pair_allreduce(_tree(jnp.minimum, sl), jnp.minimum)
    ep = [jnp.exp2(s - mx) for s in sl]
    en = [jnp.exp2(mn - s) for s in sl]
    sp = _pair_allreduce(_tree(jnp.add, ep), jnp.add)
    sn = _pair_allreduce(_tree(jnp.add, en), jnp.add)
    return ep, en, sp, sn


def _after(x, never, anchor):
    if anchor is None:
        return x
    d = jnp.concatenate([anchor] * (x.shape[0] // 8), axis=0)
    if x.shape[1] == 128:
        return jnp.where(never, d, x)
    return jnp.concatenate([jnp.where(never, d, x[:, :128]), x[:, 128:]], axis=1)


def _gate(x, never, deps):
    for i, dep in enumerate(deps):
        d = jnp.broadcast_to(dep, (8, 128))
        if x.dtype != F32:
            d = pltpu.bitcast(d, x.dtype)
        blk = jnp.where(never, d, x[8 * i:8 * i + 8, :128])
        if x.shape[1] > 128:
            blk = jnp.concatenate([blk, x[8 * i:8 * i + 8, 128:]], axis=1)
        parts = ([x[:8 * i, :]] if i else []) + [blk, x[8 * i + 8:, :]]
        x = jnp.concatenate(parts, axis=0)
    return x


def _lane_fold(a):
    return _tree(jnp.add, [a[:, 128 * i:128 * i + 128] for i in range(a.shape[1] // 128)])


def _row_sum(a):
    return jnp.sum(_lane_fold(a), axis=-1, keepdims=True)


def _lane_tile(a, n):
    return a if n == 1 else jnp.concatenate([a] * n, axis=1)


def _sublane_allreduce(a):
    a = a + pltpu.roll(a, 4, 0)
    a = a + pltpu.roll(a, 2, 0)
    return a + pltpu.roll(a, 1, 0)


def _col_broadcast(row8):
    return jnp.concatenate([row8] * 16, axis=0).astype(BF16).T.astype(F32)


def _vpu_matvec(xb, w_rows, never, anchors, lag):
    ng = xb.shape[0] // 8
    acc, hist = None, []
    for g in range(ng):
        dep = anchors[(g * len(anchors)) // ng]
        if g >= lag:
            dep = dep + hist[g - lag]
        x = jnp.where(never, dep, xb[8 * g:8 * g + 8, :])
        w = w_rows(g)
        t = w * _lane_tile(x, w.shape[1] // 128)
        acc = t if acc is None else acc + t
        c = 128 * ((g * MOE_ROT) % (w.shape[1] // 128))
        hist.append(acc[:, c:c + 128])
    return acc


class _Side:
    def __init__(self, never):
        self.never = never
        self.jobs = []
        self.deps = {}
        self.hooks = {}

    def add(self, plan, fn):
        for k, (rel, due) in enumerate(plan):
            if rel is None:
                self._run(due, fn, k, None)
            else:
                self.jobs.append((rel, due, fn, k))

    def _run(self, due, fn, k, anchor):
        dep = fn(k, anchor)
        if due is not None:
            self.deps.setdefault(due, []).append(dep)

    def check(self):
        assert not self.jobs and not self.deps and not self.hooks

    def gate(self, step, x):
        return _gate(x, self.never, self.deps.pop(step, []))

    def done(self, step, res):
        m = res.shape[0] // 8
        for job in sorted([j for j in self.jobs if step - 1 < j[0] <= step], key=lambda j: j[0]):
            self.jobs.remove(job)
            g = m - 1 - int((step - job[0]) * m)
            self._run(job[1], job[2], job[3], res[8 * g:8 * g + 8, res.shape[1] - 128:])
        for fn in self.hooks.pop(step, []):
            fn()


def _kernel(x_hbm, wqkv_hbm, wphi_hbm, wo_hbm, wr_hbm, wg_hbm, wu_hbm, wd_hbm, out_hbm,
            x_v, xn_v, lead_v, wraw_v, wt_v, wphi_v, a_v, woraw_v, wo_v, wrraw_v, wr_v, kvacc_v, kvbf_v,
            z_v, zb_v, phi_v, ha_v, hb_v, hn_v, o_v, wg_v, wu_v, wd_v, wgp_v, wup_v, wdp_v, patch_v,
            sem):
    SX, SW, SO, SM = 0, 6, 6 + 3 * NC, 6 + 3 * NC + NT_ + 1

    def x_copy(i):
        h0, h1 = ((1, 2), (2, 4), (4, 6), (6, 10), (10, 2 * NT_), (0, 1))[i]
        rows = pl.ds(h0 * TH, (h1 - h0) * TH)
        return pltpu.make_async_copy(x_hbm.at[rows, :], x_v.at[rows, :], sem.at[SX + i])

    def k0_copy(s):
        return pltpu.make_async_copy(wqkv_hbm.at[:, pl.ds(D + s * 128, 128)],
                                     wraw_v.at[NC, :, pl.ds(s * 128, 128)], sem.at[(SM + 7, SW + NC)[s]])

    def w_copy(j, c):
        return pltpu.make_async_copy(wqkv_hbm.at[:, pl.ds(j * D + c * RC, RC)], wraw_v.at[j * NC + c],
                                     sem.at[SW + j * NC + c])

    def wphi_copy(i):
        h0, h1 = ((0, 8), (8, 16), (16, H))[i]
        return pltpu.make_async_copy(wphi_hbm.at[pl.ds(h0, h1 - h0)], wphi_v.at[pl.ds(h0, h1 - h0)],
                                     sem.at[(SM + 4, SM + 8, SM + 9)[i]])

    wr_copy = pltpu.make_async_copy(wr_hbm, wrraw_v, sem.at[SM + 5])
    wo_copy = pltpu.make_async_copy(wo_hbm, woraw_v, sem.at[SM + 6])
    wg_copy = pltpu.make_async_copy(wg_hbm, wg_v.at[:, pl.ds(0, FF)], sem.at[SM + 0])
    wu_copy = pltpu.make_async_copy(wu_hbm, wu_v.at[:, pl.ds(0, FF)], sem.at[SM + 1])
    wd_copy = pltpu.make_async_copy(wd_hbm, wd_v, sem.at[SM + 2])

    wphi_copy(0).start()
    k0_copy(0).start()
    x_copy(5).start()
    k0_copy(1).start()
    x_copy(0).start()
    wphi_copy(1).start()
    w_copy(1, 1).start()

    def view(ref, i, n, off=0):
        r0 = off + i * n
        return ref.at[pl.ds(r0 if isinstance(r0, int) else pl.multiple_of(r0, math.gcd(n, off)), n), :]

    def ln_rows(t, k, n, never=None, anchor=None):
        x = _after(view(x_v, t, T)[k * n:(k + 1) * n, :].astype(F32), never, anchor)
        xc = x - _row_sum(x) * (1.0 / D)
        rstd = lax.rsqrt(_row_sum(xc * xc) * (1.0 / D) + LN_EPS)
        view(xn_v, t, T // 2)[k * n // 2:(k + 1) * n // 2, :] = _pack((xc * rstd).astype(BF16))
        return _tree(jnp.add, [rstd[8 * i:8 * i + 8, :] for i in range(min(n, LNC) // 8)])

    def xn_tile(t):
        return _unpack(view(xn_v, t, T // 2)[...])

    def expand_wphi(c):
        w = wphi_v[8 * c:8 * c + 8].reshape(8 * DH, DH).astype(F32).T
        bits = pltpu.bitcast(w, U32)
        head = lax.broadcasted_iota(jnp.int32, (DH, 128), 1) >> 5
        for s in range(2):
            b = bits[:, 128 * s:128 * s + 128]
            for j in range(2):
                r0 = 64 * (2 * c + s) + 32 * j
                a_v[r0:r0 + 32, :] = jnp.where(head == 2 * j, b >> 16,
                                               jnp.where(head == 2 * j + 1, b, jnp.uint32(0)))

    wphi_copy(0).wait()
    expand_wphi(0)
    hb_v[...] = jnp.zeros((TH, D), F32)

    def fold_v(c):
        for s in range(RC // 128):
            g0 = 64 * (2 * c + s)
            wt_v[2][g0:g0 + 64, :] = _pack(wraw_v[2 * NC + c, :, s * 128:(s + 1) * 128].T)

    def fold_pairs(j, c, s, side=None, step0=None):
        g0 = 64 * (2 * c + s)
        g0 = g0 if isinstance(g0, int) else pl.multiple_of(g0, 64)
        res = _dot(_unpack(a_v[pl.ds(g0, 64), :]), wraw_v[j * NC + c, :, s * 128:(s + 1) * 128], NT)
        if side is not None:
            side.done(step0 + 2 * s, res[:, :D // 2])
            side.done(step0 + 2 * s + 1, res[:, D // 2:])
        sub = lax.broadcasted_iota(jnp.int32, (8, D), 0)
        out = []
        for q in range(2):
            base = _pair_allreduce(jnp.where(sub < 2, res[64 * q:64 * q + 8, :], 0.0), jnp.add)
            out.append([(res[64 * q + 8 * i:64 * q + 8 * i + 8, :] - base) * LOG2E for i in range(8)])
        return out

    def share(z, z3, k):
        sub = lax.broadcasted_iota(jnp.int32, (8, D), 0)
        return jnp.where(sub < 2, pltpu.roll(z3, 8 - 2 * k, 0), z)

    def packed(slabs):
        return _pack(jnp.concatenate(slabs, axis=0).astype(BF16))

    def fold(j, c, side=None, step0=None):
        p0, p1 = fold_pairs(j, c, 0, side, step0)
        p2, p3 = fold_pairs(j, c, 1, side, step0)
        sl = ([share(p0[0], p3[0], 1), share(p1[0], p3[0], 2)] + p0[1:] + p1[1:]
              + [share(p2[0], p3[0], 3)] + p2[1:] + p3[1:])
        zero = jnp.zeros((8, D), F32)
        even, odd = sl + [zero], [zero] + sl
        r0 = 8 * ((31 * c) // 2)
        if isinstance(c, int):
            is_odd = c % 2 == 1
            sl = odd if is_odd else even
        else:
            is_odd = c % 2 == 1
            r0 = pl.multiple_of(r0, 8)
            sl = [jnp.where(is_odd, o, e) for o, e in zip(odd, even)]
        win = wt_v[j].at[pl.ds(r0, 128), :]
        win[8:128, :] = packed(sl[2:])
        first = packed(sl[:2])
        if is_odd is not False:
            keep = lax.broadcasted_iota(jnp.int32, (8, D), 0) < jnp.where(is_odd, 4, 0)
            first = jnp.where(keep, win[0:8, :], first)
        win[0:8, :] = first

    def k_pair(p, slot, pr, c0, first, never=None):
        ep, en, sp, sn = _dual_exp(p)
        inv = _recip(sp * sn)
        scale = (sn * inv, sp * inv)
        es = ep + en
        cols = slice(c0, c0 + p[0].shape[1])
        n = 16 if never is None else 16 // STAGGER
        last = None
        for q in range(16 // n):
            sc = scale
            if last is not None:
                sc = [jnp.where(never, last, x) for x in scale]
            phi = jnp.concatenate([es[i] * sc[i // 8] for i in range(q * n, (q + 1) * n)], axis=0)
            rows = slice(8 * q * n, 8 * (q + 1) * n)
            z = phi if first else z_v[pr, rows, cols] + phi
            z_v[pr, rows, cols] = z
            phi_v[slot][64 * pr + 4 * q * n:64 * pr + 4 * (q + 1) * n, cols] = _pack(phi.astype(BF16))
            last = z[8 * n - 8:, :]

    def k_features(pk, slot, c, first, never=None):
        for j in range(PPC):
            k_pair(_pair_logits(pk, j), slot, c * PPC + j, 0, first, never)

    row = lax.broadcasted_iota(jnp.int32, (64, 128), 0)
    col = lax.broadcasted_iota(jnp.int32, (64, 128), 1)
    kv_keep = (row >> 5) == (col & 1)

    def kv_update(vt, slot, c, first, publish=False):
        for j in range(PPC):
            pr = c * PPC + j
            upd = _dot(vt[64 * j:64 * j + 64, :].astype(BF16), _unpack(phi_v[slot][64 * pr:64 * pr + 64, :]), NT)
            acc = upd if first else kvacc_v[pr] + upd
            kvacc_v[pr] = acc
            if publish:
                kvbf_v[32 * pr:32 * pr + 32, :] = _pack(jnp.where(kv_keep, acc, 0.0).astype(BF16))

    def save_lead(e, t):
        corner = _unpack(view(xn_v, t, T // 2)[0:TH // 2, 0:D // 2])
        view(lead_v, e, D // 4)[...] = _pack(corner.T)

    def proj_steps(side, step0, w, xn, lead=None):
        quarters = []
        for n in range(2):
            for m in range(2):
                step = step0 + 2 * n + m
                wq = _unpack(side.gate(step, w[:64, :] if m == 0 else w[64:, :]))
                if lead is not None and n + m == 0:
                    res = _dot(wq[:, :D // 2], _unpack(view(lead_v, lead, D // 4)[...]), NN)
                    res = _dot(wq[:, D // 2:], xn[0:TH, D // 2:], NT) + res
                else:
                    res = _dot(wq, xn[n * TH:(n + 1) * TH, :], NT)
                side.done(step, res)
                quarters.append(res)
        return jnp.concatenate(
            [jnp.concatenate([quarters[0], quarters[2]], axis=1),
             jnp.concatenate([quarters[1], quarters[3]], axis=1)], axis=0)

    def proj_v(side, step0, c, xn):
        return proj_steps(side, step0, wt_v[2][128 * c:128 * c + 128, :], xn)

    def proj_feat(side, step0, j, c, xn, carry, lead=None):
        r0 = 8 * ((31 * c) // 2)
        skip = 8 if c % 2 == 1 and carry is not None else 0
        res = proj_steps(side, step0, wt_v[j][r0 + skip:r0 + 128, :], xn, lead)
        sl = [res[8 * i:8 * i + 8, :] for i in range(res.shape[0] // 8)]
        if c % 2 == 0:
            return sl[:31], sl[31]
        return ([carry] + sl if skip else sl[1:]), None

    def pack_rows(src, dst, r0, rows, c0, cols, never, a):
        if PACK_VIA_F32:
            w = src[r0:r0 + rows, c0:c0 + cols].astype(F32)
            d = _lane_tile(a, cols // 128)
            w = jnp.concatenate([jnp.where(never, d, w[8 * i:8 * i + 8, :]) if i % 2 == 0 else w[8 * i:8 * i + 8, :]
                                 for i in range(rows // 8)], axis=0)
            dst[r0 // 2:(r0 + rows) // 2, c0:c0 + cols] = _pack(w.astype(BF16))
            return
        w = _pack(src[r0:r0 + rows, c0:c0 + cols])
        d = jnp.concatenate([_lane_tile(pltpu.bitcast(a, U32), cols // 128)] * (rows // 16), axis=0)
        dst[r0 // 2:(r0 + rows) // 2, c0:c0 + cols] = jnp.where(never, d, w)

    def stash_at(i, k, n):
        return zb_v.at[4 * i + 2 * (k // 16) + n, pl.ds(8 * (k % 16), 8), :]

    def stash(i, sl):
        for k, v in enumerate(sl):
            for n in range(2):
                stash_at(i, k, n)[...] = v[:, 128 * n:128 * n + 128]

    def stashed_k(i, slot, c, first):
        def job(k, a):
            j, n = k // 2, k % 2
            p = _pair_logits([stash_at(i, q, n)[...] for q in range(31)], j)
            k_pair([_after(p[0], never0, a)] + p[1:], slot, c * PPC + j, 128 * n, first, never0)
        return job

    def first_rows(k0, k1, n):
        xn = _unpack(xn_v[n * TH // 2:(n + 1) * TH // 2, :])
        ks = [k for k in range(k0, k1)]
        w = jnp.concatenate([wt_v[1][4 * (k % 32):4 * (k % 32) + 8, :] for k in ks[::2]], axis=0)
        res = _dot(_unpack(w), xn, NT)
        for q, k in enumerate(ks):
            if k % 32 < 31:
                stash_at(0, k % 32, n)[...] = res[8 * q:8 * q + 8, :]

    k0_copy(0).wait()
    x_copy(5).wait()
    wphi_copy(2).start()
    w_copy(1, 2).start()
    x_copy(1).start()
    p0, p1 = fold_pairs(1, 0, 0)
    wt_v[1][8:64, :] = packed(p0[1:] + p1[1:])
    ha_v[0:8, :] = p0[0]
    ha_v[8:16, :] = p1[0]
    never0 = ln_rows(0, 0, TH)[0, 0] < 0.0
    first_rows(2, 16, 0)

    k0_copy(1).wait()
    x_copy(0).wait()
    wphi_copy(1).wait()
    w_copy(1, 3).start()
    for c in range(NC):
        w_copy(2, c).start()
    p2, p3 = fold_pairs(1, 0, 1)
    wt_v[1][0:8, :] = packed([share(ha_v[0:8, :], p3[0], 1), share(ha_v[8:16, :], p3[0], 2)])
    wt_v[1][64:128, :] = packed([share(p2[0], p3[0], 3)] + p2[1:] + p3[1:] + [jnp.zeros((8, D), F32)])
    ln_rows(0, 1, TH)
    first_rows(16, 34, 0)
    first_rows(0, 16, 1)
    first_rows(16, 32, 1)
    expand_wphi(1)

    for c in (1, 2):
        w_copy(1, c).wait()
        if c == 1:
            wphi_copy(2).wait()
            expand_wphi(2)
            expand_wphi(3)
            x_copy(2).start()
            for cq in range(NC):
                w_copy(0, cq).start()
        else:
            x_copy(3).start()
            wo_copy.start()
            wr_copy.start()
            x_copy(4).start()
        side = _Side(never0)
        side.add(PRO_K_PLAN, stashed_k(c - 1, 0, c - 1, True))
        fold(1, c, side, 0)
        stash(c, proj_feat(side, 4, 1, c, xn_tile(0), None)[0])
        side.check()

    x_copy(1).wait()
    w_copy(1, 3).wait()
    wg_copy.start()
    wu_copy.start()
    wd_copy.start()
    side = _Side(never0)
    side.add(PRO_LN1_PLAN, lambda k, a: ln_rows(1, k, LNC, never0, a))
    fold(1, 3, side, 0)
    stash(3, proj_feat(side, 4, 1, 3, xn_tile(0), None)[0])
    xn1 = xn_tile(1)
    spare = None
    for c in range(NC):
        pk, spare = proj_feat(_Side(None), 0, 1, c, xn1, spare)
        if c < 3:
            k_features(pk, 1, c, c == 2, never0)
        else:
            stash(0, pk)

    for c in range(NC):
        w_copy(2, c).wait()
    x_copy(2).wait()
    w_copy(0, 0).wait()
    side = _Side(never0)
    side.add(PRO_V_PLANS[0], stashed_k(2, 0, 2, False))
    side.add(PRO_V_PLANS[1], stashed_k(3, 0, 3, True))
    side.add(PRO_V_PLANS[2], stashed_k(0, 1, 3, False))
    side.add(PRO_V_PLANS[3], lambda k, a: ln_rows(2, k, LNC, never0, a))
    fold(0, 0)
    wt_v[0][248:256, :] = jnp.zeros((8, D), U32)
    xns = (xn_tile(0), xn_tile(1))
    pending = None
    for c in range(NC):
        fold_v(c)
        for i in range(2):
            vt = proj_v(side, 8 * c + 4 * i, c, xns[i])
            if pending is not None:
                kv_update(*pending)
            pending = (vt, i, c, i == 0)
    side.check()
    kv_update(*pending)
    save_lead(0, 0)
    save_lead(1, 2)

    def phase1(u, carry):
        never = u < 0

        @pl.when(u == 0)
        def _():
            for c in range(1, NC):
                w_copy(0, c).wait()
            x_copy(3).wait()
            wo_copy.wait()
            wr_copy.wait()

        @pl.when(u == 1)
        def _():
            x_copy(4).wait()

        pending = None
        for i in range(2):
            t = 2 * u + 2 + i
            tn = jnp.minimum(t + 1, NT_ - 1)
            side = _Side(never)
            xn = xn_tile(t)
            spare = None
            for c in range(NC):
                pk, spare = proj_feat(_Side(None), 0, 1, c, xn, spare, u + 1 if LEAD and i + c == 0 else None)
                if c == 0 and pending is not None:
                    kv_update(*pending)
                k_features(pk, i, c, False)
            side.add(LN1_PLAN, lambda k, a: ln_rows(tn, k, LNC, never, a))
            if i == 0:
                def pack_wo(k, a):
                    rows = WO_ROWS // len(WO_PLAN)
                    w0 = u * ((D - WO_ROWS) // 2)
                    src = woraw_v.at[pl.ds(pl.multiple_of(w0, 16), WO_ROWS), :]
                    dst = wo_v.at[pl.ds(pl.multiple_of(w0 // 2, 8), WO_ROWS // 2), :]
                    pack_rows(src, dst, k * rows, rows, 0, D, never, a)
                side.add(WO_PLAN, pack_wo)
            else:
                def z_final(k, a):
                    z = _after(z_v[k], never, a)
                    zs = _row_sum(z)
                    zb_v[k] = jnp.broadcast_to(zs, (128, 128))
                    return zs[120:128, :]
                side.add(Z_PLAN, z_final)
            side.done(0, jnp.concatenate(pk[17:], axis=0))
            vts = []
            for c in range(NC):
                vts.append(proj_v(side, 4 * c + 1, c, xn))
                if c > 0:
                    kv_update(vts[c - 1], i, c - 1, False, i == 1)
            pending = (vts[NC - 1], i, NC - 1, False, i == 1)
            side.check()
        fold(0, u + 1)
        kv_update(*pending)
        save_lead(u + 2, tn)
        wr_v[...] = jnp.broadcast_to(wrraw_v[...].reshape(1, D).astype(F32), (8, D))
        return carry

    lax.fori_loop(0, (NT_ - 2) // 2, phase1, 0)

    def o_copy(r0, n, i):
        return pltpu.make_async_copy(o_v.at[pl.ds(r0, n), :], out_hbm.at[pl.ds(r0, n), :], sem.at[SO + i])

    def finish_rows(h_ref, k, ht, valid, st, never=None, anchor=None):
        r0 = ht * TH + k * LNC
        best, besti = st["route"]
        wr = jnp.concatenate([wr_v[...]] * (LNC // 8), axis=0)
        sub = lax.broadcasted_iota(jnp.int32, (8, 1), 0)
        h = _after(h_ref[k * LNC:(k + 1) * LNC, :], never, anchor)
        hc = h - _row_sum(h) * (1.0 / D)
        rstd = lax.rsqrt(_row_sum(hc * hc) * (1.0 / D) + LN_EPS)
        r = (_row_sum(hc * wr) * rstd).astype(BF16).astype(F32)
        hn = hc * rstd
        view(hn_v, ht, TH // 2)[k * LNC // 2:(k + 1) * LNC // 2, :] = _pack(hn.astype(BF16))
        view(o_v, ht, TH)[k * LNC:(k + 1) * LNC, :] = (hn + h).astype(BF16)
        if valid is not None:
            r = jnp.where(valid, r, -jnp.inf)
        for i in range(LNC // 8):
            ri = r[8 * i:8 * i + 8, :]
            better = ri > best
            best = jnp.where(better, ri, best)
            besti = jnp.where(better, sub + (r0 + 8 * i), besti)
        st["route"] = (best, besti)
        return best

    def q_features(pq, slot, c, never):
        for j in range(PPC):
            pr = c * PPC + j
            ep, en, sp, sn = _dual_exp(_pair_logits(pq, j))
            zz = [_lane_tile(zb_v[pr, 8 * i:8 * i + 8, :], T // 128) for i in range(16)]
            ap = _pair_allreduce(_tree(jnp.add, [ep[i] * zz[i] for i in range(8)]), jnp.add)
            an = _pair_allreduce(_tree(jnp.add, [en[i] * zz[8 + i] for i in range(8)]), jnp.add)
            inv = _recip(ap * sn + (an + 1e-6 * sn) * sp)
            scale, es, n, last = (sn * inv, sp * inv), ep + en, 16 // Q_STAGGER, None
            for q in range(Q_STAGGER):
                sc = scale if last is None else [jnp.where(never, last, x) for x in scale]
                phi = jnp.concatenate([es[i] * sc[i // 8] for i in range(q * n, (q + 1) * n)], axis=0)
                phi_v[slot][64 * pr + 4 * q * n:64 * pr + 4 * (q + 1) * n, :] = _pack(phi.astype(BF16))
                last = phi[8 * n - 8:, :]

    def attn_rows(slot, g):
        res = jnp.concatenate(
            [_dot(_unpack(kvbf_v[32 * pr:32 * pr + 32, :]), _unpack(phi_v[slot][64 * pr:64 * pr + 64, :]), NN)
             for pr in (2 * g, 2 * g + 1)], axis=0)
        return res.astype(BF16).T

    def out_proj(side, step0, o, k0, k1):
        cols = []
        for n in range(D // 128):
            w = side.gate(step0 + n, wo_v[k0 // 2:k1 // 2, n * 128:(n + 1) * 128])
            res = _dot(o, _unpack(w), NN)
            side.done(step0 + n, res)
            cols.append(res)
        return jnp.concatenate(cols, axis=1)

    def phase2(u, carry):
        for i in range(UNROLL2):
            carry = phase2_tile(u * UNROLL2 + i, i % 2, carry, u < 0, u if LEAD and i == 0 else None)

        r0 = pl.multiple_of(u * (UNROLL2 * T), T)

        @pl.when(u == 0)
        def _():
            o_copy(0, UNROLL2 * T - TH, 0).start()

        @pl.when(u > 0)
        def _():
            o_copy(pl.multiple_of(jnp.maximum(r0 - TH, 0), TH), UNROLL2 * T, u).start()

        return carry

    def phase2_tile(t, slot, carry, never, lead):
        hp = jnp.maximum(2 * t - 1, 0)
        side = _Side(never)
        st = {"route": carry}
        side.add(LN2B_PLAN, lambda k, a: finish_rows(hb_v, k, hp, t > 0, st, side.never, a))

        def pack_ffn(k, a):
            if k < 32:
                n = D // NT_
                pack_rows(view((wg_v, wu_v)[k % 2], t, n), view((wgp_v, wup_v)[k % 2], t, n // 2),
                          (k // 4) * 16, 16, (0, D)[k // 2 % 2], (D, FM - D)[k // 2 % 2], never, a)
            else:
                n = (FF - FVD) // NT_
                pack_rows(view(wd_v, t, n, FVD), view(wdp_v, t, n // 2), (k - 32) * 16, 16, 0, D, never, a)
        side.add(PACK_PLAN[:32 + (FF - FVD) // 128], pack_ffn)

        xn = xn_tile(t)
        xt = view(x_v, t, T)
        os_ = {}
        for g in range(8):
            side.hooks.setdefault(G_STEPS[g], []).append(lambda g=g: os_.__setitem__(g, attn_rows(slot, g)))
        spare = None
        for c in range(NC):
            pq, spare = proj_feat(side, 100 + 4 * c, 0, c, xn, spare, lead if c == 0 else None)
            if c == 0:
                head = side.gate(0, jnp.concatenate(pq[2:9], axis=0))
                pq = pq[:2] + [head[8 * i:8 * i + 8, :] for i in range(7)] + pq[9:]
            q_features(pq, slot, c, never)
        ha = out_proj(side, 0, jnp.concatenate([os_[g][0:TH, :] for g in range(4)], axis=1), 0, D // 2)
        ha = ha + xt[0:TH, :].astype(F32)
        ha_v[...] = ha + out_proj(side, 8, jnp.concatenate([os_[g][0:TH, :] for g in range(4, 8)], axis=1), D // 2, D)
        side.add(LN2A_PLAN, lambda k, a: finish_rows(ha_v, k, 2 * t, None, st, side.never, a))
        ob = jnp.concatenate([os_[g][TH:T, :] for g in range(8)], axis=1)
        hb_v[...] = xt[TH:T, :].astype(F32) + out_proj(side, 16, ob, 0, D)
        side.check()
        return st["route"]

    wg_copy.wait()
    wu_copy.wait()
    wd_copy.wait()
    route = lax.fori_loop(
        0, NT_ // UNROLL2, phase2,
        (jnp.full((8, 1), -jnp.inf, F32), jnp.zeros((8, 1), jnp.int32)))
    st = {"route": route}
    for k in range(TH // LNC):
        finish_rows(hb_v, k, 2 * NT_ - 1, None, st)
    best, besti = st["route"]
    o_copy(S - TH, TH, NT_).start()

    rmax = jnp.max(best, axis=0, keepdims=True)
    idx = jnp.min(jnp.where(best == rmax, besti, S), axis=0, keepdims=True)
    idx_s = jnp.clip(idx[0, 0], 0, S - 1)
    blk = pl.multiple_of((idx_s >> 4) << 4, 16)
    pair = jnp.broadcast_to(hn_v[pl.ds(idx_s >> 1, 1), :], (8, D))
    x8 = pltpu.bitcast(jnp.where((idx_s & 1) == 1, pair & jnp.uint32(0xFFFF0000), pair << 16), F32)
    xs = jnp.concatenate([x8, x8], axis=0).astype(BF16)
    acts, anchors = [], []

    def park(v, half):
        if not MOE_PARK:
            return v
        n = v.shape[0] // 128
        for i in range(n):
            z_v[i, :, 128 * half:128 * half + 128] = v[128 * i:128 * i + 128, :]
        return jnp.concatenate([z_v[i, :, 128 * half:128 * half + 128] for i in range(n)], axis=0)

    for c0 in range(0, FM, 128):
        g = _dot(xs, _unpack(wgp_v[:, c0:c0 + 128]), NN)[0:8, :]
        u = _dot(xs, _unpack(wup_v[:, c0:c0 + 128]), NN)[0:8, :]
        anchors += [g, u]
        acts.append(g * jax.nn.sigmoid(g) * u)
    xb = park(_col_broadcast(x8), 0)
    if MOE_SPLIT:
        g, u = [_sublane_allreduce(_vpu_matvec(
            xb, lambda g: w[8 * g:8 * g + 8, FM:FF].astype(F32), never0,
            anchors[i * MOE_NA // 2:(i + 1) * MOE_NA // 2], MOE_SPLIT)) for i, w in enumerate((wg_v, wu_v))]
    else:
        gu = _sublane_allreduce(_vpu_matvec(
            xb, lambda g: jnp.concatenate([w[8 * g:8 * g + 8, FM:FF].astype(F32) for w in (wg_v, wu_v)], axis=1),
            never0, anchors[:MOE_NA], 1))
        g, u = gu[:, :FV], gu[:, FV:]
    acts.append(g * jax.nn.sigmoid(g) * u)
    a = jnp.concatenate(acts, axis=1)
    am = jnp.concatenate([a[:, FVD:], a[:, FVD:]], axis=0).astype(BF16)
    ys, anchors = [], anchors[MOE_NA:]
    for k0 in range(0, FF - FVD, 512):
        k1 = min(k0 + 512, FF - FVD)
        yk = _dot(am[:, k0:k1], _unpack(wdp_v[k0 // 2:k1 // 2, :]), NN)[0:8, :]
        ys.append(yk)
        anchors += [yk[:, c:c + 128] for c in range(128, D, 256)]
    ys.append(_sublane_allreduce(_vpu_matvec(
        park(_col_broadcast(a[:, :FVD]), 1), lambda g: wd_v[8 * g:8 * g + 8, 0:D].astype(F32), never0, anchors[:-MOE_ND], MOE_LAG)))
    y = _tree(jnp.add, ys) * jax.nn.sigmoid(rmax)
    y = jnp.concatenate([y, y], axis=0)
    sel = lax.broadcasted_iota(jnp.int32, (16, 1), 0) == (idx_s - blk)
    patch_v[...] = (o_v[pl.ds(blk, 16), :].astype(F32) + jnp.where(sel, y, 0.0)).astype(BF16)
    o_copy(0, UNROLL2 * T - TH, 0).wait()
    for u in range(1, NT_ // UNROLL2):
        o_copy(u * UNROLL2 * T - TH, UNROLL2 * T, u).wait()
    o_copy(S - TH, TH, NT_).wait()
    pc = pltpu.make_async_copy(patch_v, out_hbm.at[pl.ds(blk, 16), :], sem.at[SM + 3])
    pc.start()
    pc.wait()


@jax.jit
def pallas_sequential_preLN__linear_kernel_hedgehog__moe_arch_mod__prompt_kernel(
    A_x: jax.Array,
    A_wqkv: jax.Array,
    A_w_phi: jax.Array,
    A_wo: jax.Array,
    B_x: jax.Array,
    B_w_r: jax.Array,
    B_w_gate: jax.Array,
    B_w_up: jax.Array,
    B_w_down: jax.Array,
):
    del B_x
    hbm = pl.BlockSpec(memory_space=pl.ANY)
    out = pl.pallas_call(
        _kernel,
        out_shape=jax.ShapeDtypeStruct((S, D), BF16),
        in_specs=[hbm] * 8,
        out_specs=hbm,
        scratch_shapes=[
            pltpu.VMEM((S, D), BF16),
            pltpu.VMEM((S // 2, D), U32),
            pltpu.VMEM((5 * D // 4, 128), U32),
            pltpu.VMEM((3 * NC, D, RC), BF16),
            [pltpu.VMEM((D // 2, D), U32)] * 3,
            pltpu.VMEM((H, DH, DH), BF16),
            pltpu.VMEM((8 * 64, 128), U32),
            pltpu.VMEM((D, D), BF16),
            pltpu.VMEM((D // 2, D), U32),
            pltpu.VMEM((D,), BF16),
            pltpu.VMEM((8, D), F32),
            pltpu.VMEM((NPAIR, 64, 128), F32),
            pltpu.VMEM((NPAIR * 32, 128), U32),
            pltpu.VMEM((NPAIR, 128, T), F32),
            pltpu.VMEM((NPAIR, 128, 128), F32),
            [pltpu.VMEM((NPAIR * 64, T), U32)] * 2,
            pltpu.VMEM((TH, D), F32),
            pltpu.VMEM((TH, D), F32),
            pltpu.VMEM((S // 2, D), U32),
            pltpu.VMEM((S, D), BF16),
            pltpu.VMEM((D, FFP), BF16),
            pltpu.VMEM((D, FFP), BF16),
            pltpu.VMEM((FF, D), BF16),
            pltpu.VMEM((D // 2, FM), U32),
            pltpu.VMEM((D // 2, FM), U32),
            pltpu.VMEM(((FF - FVD) // 2, D), U32),
            pltpu.VMEM((16, D), BF16),
            pltpu.SemaphoreType.DMA((6 + 3 * NC + NT_ + 11,)),
        ],
        compiler_params=pltpu.CompilerParams(vmem_limit_bytes=100 * 1024 * 1024,
                                             disable_semaphore_checks=True, disable_bounds_checks=True),
        name="hedgehog_mod",
    )(
        A_x.reshape(S, D),
        A_wqkv,
        A_w_phi,
        A_wo,
        B_w_r,
        B_w_gate,
        B_w_up,
        B_w_down,
    )
    return out.reshape(1, S, D)
```

```python
import math

import jax
import jax.numpy as jnp
from jax import lax
import jax.experimental.pallas as pl
import jax.experimental.pallas.tpu as pltpu

F32 = jnp.float32
BF16 = jnp.bfloat16
U32 = jnp.uint32

S = 2048
D = 1024
H = 32
DH = 32
FF = 3584
NPAIR = H // 2
LOG2E = 1.4426950408889634
LN_EPS = 1e-5

T = 256
TH = T // 2
NT_ = S // T
RC = 256
NC = D // RC
PPC = RC // 64
LNC = 16
FFP = 4096

FV = 10 * 128
FM = FF - FV
FVD = 8 * 128
WO_ROWS = 352
UNROLL2 = 2


def _spread(n, a, b, due=None):
    rel = [round(a + (b - a) * k / (n - 1), 3) for k in range(n)]
    return tuple((r, None if due is None else math.ceil(r) + due) for r in rel)


LN1_PLAN = _spread(16, 0, 13, 3)
WO_PLAN = _spread(11, 3, 13)
Z_PLAN = _spread(16, 6, 14, 2)
PRO_LN1_PLAN = ((None, None),) * 16
PRO_K_PLAN = _spread(8, 0, 6)
PRO_V_PLANS = (_spread(8, 0, 12), _spread(16, 13, 22)[:8], _spread(16, 13, 22)[8:], _spread(16, 1.2, 27, 3))
LN2B_PLAN = ((None, 103), (-0.13, 6), (1.532, 8), (3.446, 10), (4.894, 11), (6.571, 13), (8.519, 15), (9.867, 15))
LN2A_PLAN = ((None, 18), (15.227, 19), (16.121, 20), (16.864, 20), (17.647, 21), (18.474, 22), (19.118, 23), (20.038, None))
PACK_PLAN = _spread(16, 99.7, 114.7) + _spread(16, 99.1, 114.1) + _spread(20, 0.5, 21)
G_STEPS = (107, 107, 111, 111, 115, 115, 3, 3)
Q_STAGGER = 1
MOE_NA = 36
MOE_ND = 3
MOE_LAG = 2
MOE_ROT = 1
MOE_PARK = 1
MOE_SPLIT = 3
STAGGER = 8
LEAD = True
PACK_VIA_F32 = True

NN = (((1,), (0,)), ((), ()))
NT = (((1,), (1,)), ((), ()))


def _dot(a, b, dims):
    return lax.dot_general(a, b, dims, preferred_element_type=F32)


def _recip(x):
    return pl.reciprocal(x, approx=False, full_range=False)


def _pack(x):
    return pltpu.bitcast(x, U32)


def _unpack(x):
    return pltpu.bitcast(x, BF16)


def _pair_allreduce(a, op):
    a = op(a, pltpu.roll(a, 2, 0))
    return op(a, pltpu.roll(a, 4, 0))


def _tree(op, xs):
    xs = list(xs)
    while len(xs) > 1:
        nxt = [op(xs[i], xs[i + 1]) for i in range(0, len(xs) - 1, 2)]
        if len(xs) % 2:
            nxt.append(xs[-1])
        xs = nxt
    return xs[0]


def _pair_logits(sl, j):
    sub = lax.broadcasted_iota(jnp.int32, sl[0].shape, 0)
    if j < 3:
        head = jnp.where(sub < 2, 0.0, sl[(0, 1, 16)[j]])
    else:
        head = jnp.where(sub < 2, sl[0], jnp.where(sub < 4, pltpu.roll(sl[1], 2, 0),
                                                   jnp.where(sub < 6, pltpu.roll(sl[16], 4, 0), 0.0)))
    r0 = (2, 9, 17, 24)[j]
    return [head] + list(sl[r0:r0 + 7])


def _dual_exp(sl):
    mx = _pair_allreduce(_tree(jnp.maximum, sl), jnp.maximum)
    mn = _pair_allreduce(_tree(jnp.minimum, sl), jnp.minimum)
    ep = [jnp.exp2(s - mx) for s in sl]
    en = [jnp.exp2(mn - s) for s in sl]
    sp = _pair_allreduce(_tree(jnp.add, ep), jnp.add)
    sn = _pair_allreduce(_tree(jnp.add, en), jnp.add)
    return ep, en, sp, sn


def _after(x, never, anchor):
    if anchor is None:
        return x
    d = jnp.concatenate([anchor] * (x.shape[0] // 8), axis=0)
    if x.shape[1] == 128:
        return jnp.where(never, d, x)
    return jnp.concatenate([jnp.where(never, d, x[:, :128]), x[:, 128:]], axis=1)


def _gate(x, never, deps):
    for i, dep in enumerate(deps):
        d = jnp.broadcast_to(dep, (8, 128))
        if x.dtype != F32:
            d = pltpu.bitcast(d, x.dtype)
        blk = jnp.where(never, d, x[8 * i:8 * i + 8, :128])
        if x.shape[1] > 128:
            blk = jnp.concatenate([blk, x[8 * i:8 * i + 8, 128:]], axis=1)
        parts = ([x[:8 * i, :]] if i else []) + [blk, x[8 * i + 8:, :]]
        x = jnp.concatenate(parts, axis=0)
    return x


def _lane_fold(a):
    return _tree(jnp.add, [a[:, 128 * i:128 * i + 128] for i in range(a.shape[1] // 128)])


def _row_sum(a):
    return jnp.sum(_lane_fold(a), axis=-1, keepdims=True)


def _lane_tile(a, n):
    return a if n == 1 else jnp.concatenate([a] * n, axis=1)


def _sublane_allreduce(a):
    a = a + pltpu.roll(a, 4, 0)
    a = a + pltpu.roll(a, 2, 0)
    return a + pltpu.roll(a, 1, 0)


def _col_broadcast(row8):
    return jnp.concatenate([row8] * 16, axis=0).astype(BF16).T.astype(F32)


def _vpu_matvec(xb, w_rows, never, anchors, lag):
    ng = xb.shape[0] // 8
    acc, hist = None, []
    for g in range(ng):
        dep = anchors[(g * len(anchors)) // ng]
        if g >= lag:
            dep = dep + hist[g - lag]
        x = jnp.where(never, dep, xb[8 * g:8 * g + 8, :])
        w = w_rows(g)
        t = w * _lane_tile(x, w.shape[1] // 128)
        acc = t if acc is None else acc + t
        c = 128 * ((g * MOE_ROT) % (w.shape[1] // 128))
        hist.append(acc[:, c:c + 128])
    return acc


class _Side:
    def __init__(self, never):
        self.never = never
        self.jobs = []
        self.deps = {}
        self.hooks = {}

    def add(self, plan, fn):
        for k, (rel, due) in enumerate(plan):
            if rel is None:
                self._run(due, fn, k, None)
            else:
                self.jobs.append((rel, due, fn, k))

    def _run(self, due, fn, k, anchor):
        dep = fn(k, anchor)
        if due is not None:
            self.deps.setdefault(due, []).append(dep)

    def check(self):
        assert not self.jobs and not self.deps and not self.hooks

    def gate(self, step, x):
        return _gate(x, self.never, self.deps.pop(step, []))

    def done(self, step, res):
        m = res.shape[0] // 8
        for job in sorted([j for j in self.jobs if step - 1 < j[0] <= step], key=lambda j: j[0]):
            self.jobs.remove(job)
            g = m - 1 - int((step - job[0]) * m)
            self._run(job[1], job[2], job[3], res[8 * g:8 * g + 8, res.shape[1] - 128:])
        for fn in self.hooks.pop(step, []):
            fn()


def _kernel(x_hbm, wqkv_hbm, wphi_hbm, wo_hbm, wr_hbm, wg_hbm, wu_hbm, wd_hbm, out_hbm,
            x_v, xn_v, lead_v, wraw_v, wt_v, wphi_v, a_v, woraw_v, wo_v, wrraw_v, wr_v, kvacc_v, kvbf_v,
            z_v, zb_v, phi_v, ha_v, hb_v, hn_v, o_v, wg_v, wu_v, wd_v, wgp_v, wup_v, wdp_v, patch_v,
            sem):
    SX, SW, SO, SM = 0, 6, 6 + 3 * NC, 6 + 3 * NC + NT_ + 1

    def x_copy(i):
        h0, h1 = ((1, 2), (2, 4), (4, 6), (6, 10), (10, 2 * NT_), (0, 1))[i]
        rows = pl.ds(h0 * TH, (h1 - h0) * TH)
        return pltpu.make_async_copy(x_hbm.at[rows, :], x_v.at[rows, :], sem.at[SX + i])

    def k0_copy(s):
        return pltpu.make_async_copy(wqkv_hbm.at[:, pl.ds(D + s * 128, 128)],
                                     wraw_v.at[NC, :, pl.ds(s * 128, 128)], sem.at[(SM + 7, SW + NC)[s]])

    def w_copy(j, c):
        return pltpu.make_async_copy(wqkv_hbm.at[:, pl.ds(j * D + c * RC, RC)], wraw_v.at[j * NC + c],
                                     sem.at[SW + j * NC + c])

    def wphi_copy(i):
        h0, h1 = ((0, 8), (8, 16), (16, H))[i]
        return pltpu.make_async_copy(wphi_hbm.at[pl.ds(h0, h1 - h0)], wphi_v.at[pl.ds(h0, h1 - h0)],
                                     sem.at[(SM + 4, SM + 8, SM + 9)[i]])

    wr_copy = pltpu.make_async_copy(wr_hbm, wrraw_v, sem.at[SM + 5])
    wo_copy = pltpu.make_async_copy(wo_hbm, woraw_v, sem.at[SM + 6])
    wg_copy = pltpu.make_async_copy(wg_hbm, wg_v.at[:, pl.ds(0, FF)], sem.at[SM + 0])
    wu_copy = pltpu.make_async_copy(wu_hbm, wu_v.at[:, pl.ds(0, FF)], sem.at[SM + 1])
    wd_copy = pltpu.make_async_copy(wd_hbm, wd_v, sem.at[SM + 2])

    wphi_copy(0).start()
    k0_copy(0).start()
    x_copy(5).start()
    k0_copy(1).start()
    x_copy(0).start()
    wphi_copy(1).start()
    w_copy(1, 1).start()

    def view(ref, i, n, off=0):
        r0 = off + i * n
        return ref.at[pl.ds(r0 if isinstance(r0, int) else pl.multiple_of(r0, math.gcd(n, off)), n), :]

    def ln_rows(t, k, n, never=None, anchor=None):
        x = _after(view(x_v, t, T)[k * n:(k + 1) * n, :].astype(F32), never, anchor)
        xc = x - _row_sum(x) * (1.0 / D)
        rstd = lax.rsqrt(_row_sum(xc * xc) * (1.0 / D) + LN_EPS)
        view(xn_v, t, T // 2)[k * n // 2:(k + 1) * n // 2, :] = _pack((xc * rstd).astype(BF16))
        return _tree(jnp.add, [rstd[8 * i:8 * i + 8, :] for i in range(min(n, LNC) // 8)])

    def xn_tile(t):
        return _unpack(view(xn_v, t, T // 2)[...])

    def expand_wphi(c):
        w = wphi_v[8 * c:8 * c + 8].reshape(8 * DH, DH).astype(F32).T
        bits = pltpu.bitcast(w, U32)
        head = lax.broadcasted_iota(jnp.int32, (DH, 128), 1) >> 5
        for s in range(2):
            b = bits[:, 128 * s:128 * s + 128]
            for j in range(2):
                r0 = 64 * (2 * c + s) + 32 * j
                a_v[r0:r0 + 32, :] = jnp.where(head == 2 * j, b >> 16,
                                               jnp.where(head == 2 * j + 1, b, jnp.uint32(0)))

    wphi_copy(0).wait()
    expand_wphi(0)
    hb_v[...] = jnp.zeros((TH, D), F32)

    def fold_v(c):
        for s in range(RC // 128):
            g0 = 64 * (2 * c + s)
            wt_v[2][g0:g0 + 64, :] = _pack(wraw_v[2 * NC + c, :, s * 128:(s + 1) * 128].T)

    def fold_pairs(j, c, s, side=None, step0=None):
        g0 = 64 * (2 * c + s)
        g0 = g0 if isinstance(g0, int) else pl.multiple_of(g0, 64)
        res = _dot(_unpack(a_v[pl.ds(g0, 64), :]), wraw_v[j * NC + c, :, s * 128:(s + 1) * 128], NT)
        if side is not None:
            side.done(step0 + 2 * s, res[:, :D // 2])
            side.done(step0 + 2 * s + 1, res[:, D // 2:])
        sub = lax.broadcasted_iota(jnp.int32, (8, D), 0)
        out = []
        for q in range(2):
            base = _pair_allreduce(jnp.where(sub < 2, res[64 * q:64 * q + 8, :], 0.0), jnp.add)
            out.append([(res[64 * q + 8 * i:64 * q + 8 * i + 8, :] - base) * LOG2E for i in range(8)])
        return out

    def share(z, z3, k):
        sub = lax.broadcasted_iota(jnp.int32, (8, D), 0)
        return jnp.where(sub < 2, pltpu.roll(z3, 8 - 2 * k, 0), z)

    def packed(slabs):
        return _pack(jnp.concatenate(slabs, axis=0).astype(BF16))

    def fold(j, c, side=None, step0=None):
        p0, p1 = fold_pairs(j, c, 0, side, step0)
        p2, p3 = fold_pairs(j, c, 1, side, step0)
        sl = ([share(p0[0], p3[0], 1), share(p1[0], p3[0], 2)] + p0[1:] + p1[1:]
              + [share(p2[0], p3[0], 3)] + p2[1:] + p3[1:])
        zero = jnp.zeros((8, D), F32)
        even, odd = sl + [zero], [zero] + sl
        r0 = 8 * ((31 * c) // 2)
        if isinstance(c, int):
            is_odd = c % 2 == 1
            sl = odd if is_odd else even
        else:
            is_odd = c % 2 == 1
            r0 = pl.multiple_of(r0, 8)
            sl = [jnp.where(is_odd, o, e) for o, e in zip(odd, even)]
        win = wt_v[j].at[pl.ds(r0, 128), :]
        win[8:128, :] = packed(sl[2:])
        first = packed(sl[:2])
        if is_odd is not False:
            keep = lax.broadcasted_iota(jnp.int32, (8, D), 0) < jnp.where(is_odd, 4, 0)
            first = jnp.where(keep, win[0:8, :], first)
        win[0:8, :] = first

    def k_pair(p, slot, pr, c0, first, never=None):
        ep, en, sp, sn = _dual_exp(p)
        inv = _recip(sp * sn)
        scale = (sn * inv, sp * inv)
        es = ep + en
        cols = slice(c0, c0 + p[0].shape[1])
        n = 16 if never is None else 16 // STAGGER
        last = None
        for q in range(16 // n):
            sc = scale
            if last is not None:
                sc = [jnp.where(never, last, x) for x in scale]
            phi = jnp.concatenate([es[i] * sc[i // 8] for i in range(q * n, (q + 1) * n)], axis=0)
            rows = slice(8 * q * n, 8 * (q + 1) * n)
            z = phi if first else z_v[pr, rows, cols] + phi
            z_v[pr, rows, cols] = z
            phi_v[slot][64 * pr + 4 * q * n:64 * pr + 4 * (q + 1) * n, cols] = _pack(phi.astype(BF16))
            last = z[8 * n - 8:, :]

    def k_features(pk, slot, c, first, never=None):
        for j in range(PPC):
            k_pair(_pair_logits(pk, j), slot, c * PPC + j, 0, first, never)

    row = lax.broadcasted_iota(jnp.int32, (64, 128), 0)
    col = lax.broadcasted_iota(jnp.int32, (64, 128), 1)
    kv_keep = (row >> 5) == (col & 1)

    def kv_update(vt, slot, c, first, publish=False):
        for j in range(PPC):
            pr = c * PPC + j
            upd = _dot(vt[64 * j:64 * j + 64, :].astype(BF16), _unpack(phi_v[slot][64 * pr:64 * pr + 64, :]), NT)
            acc = upd if first else kvacc_v[pr] + upd
            kvacc_v[pr] = acc
            if publish:
                kvbf_v[32 * pr:32 * pr + 32, :] = _pack(jnp.where(kv_keep, acc, 0.0).astype(BF16))

    def save_lead(e, t):
        corner = _unpack(view(xn_v, t, T // 2)[0:TH // 2, 0:D // 2])
        view(lead_v, e, D // 4)[...] = _pack(corner.T)

    def proj_steps(side, step0, w, xn, lead=None):
        quarters = []
        for n in range(2):
            for m in range(2):
                step = step0 + 2 * n + m
                wq = _unpack(side.gate(step, w[:64, :] if m == 0 else w[64:, :]))
                if lead is not None and n + m == 0:
                    res = _dot(wq[:, :D // 2], _unpack(view(lead_v, lead, D // 4)[...]), NN)
                    res = _dot(wq[:, D // 2:], xn[0:TH, D // 2:], NT) + res
                else:
                    res = _dot(wq, xn[n * TH:(n + 1) * TH, :], NT)
                side.done(step, res)
                quarters.append(res)
        return jnp.concatenate(
            [jnp.concatenate([quarters[0], quarters[2]], axis=1),
             jnp.concatenate([quarters[1], quarters[3]], axis=1)], axis=0)

    def proj_v(side, step0, c, xn):
        return proj_steps(side, step0, wt_v[2][128 * c:128 * c + 128, :], xn)

    def proj_feat(side, step0, j, c, xn, carry, lead=None):
        r0 = 8 * ((31 * c) // 2)
        skip = 8 if c % 2 == 1 and carry is not None else 0
        res = proj_steps(side, step0, wt_v[j][r0 + skip:r0 + 128, :], xn, lead)
        sl = [res[8 * i:8 * i + 8, :] for i in range(res.shape[0] // 8)]
        if c % 2 == 0:
            return sl[:31], sl[31]
        return ([carry] + sl if skip else sl[1:]), None

    def pack_rows(src, dst, r0, rows, c0, cols, never, a):
        if PACK_VIA_F32:
            w = src[r0:r0 + rows, c0:c0 + cols].astype(F32)
            d = _lane_tile(a, cols // 128)
            w = jnp.concatenate([jnp.where(never, d, w[8 * i:8 * i + 8, :]) if i % 2 == 0 else w[8 * i:8 * i + 8, :]
                                 for i in range(rows // 8)], axis=0)
            dst[r0 // 2:(r0 + rows) // 2, c0:c0 + cols] = _pack(w.astype(BF16))
            return
        w = _pack(src[r0:r0 + rows, c0:c0 + cols])
        d = jnp.concatenate([_lane_tile(pltpu.bitcast(a, U32), cols // 128)] * (rows // 16), axis=0)
        dst[r0 // 2:(r0 + rows) // 2, c0:c0 + cols] = jnp.where(never, d, w)

    def stash_at(i, k, n):
        return zb_v.at[4 * i + 2 * (k // 16) + n, pl.ds(8 * (k % 16), 8), :]

    def stash(i, sl):
        for k, v in enumerate(sl):
            for n in range(2):
                stash_at(i, k, n)[...] = v[:, 128 * n:128 * n + 128]

    def stashed_k(i, slot, c, first):
        def job(k, a):
            j, n = k // 2, k % 2
            p = _pair_logits([stash_at(i, q, n)[...] for q in range(31)], j)
            k_pair([_after(p[0], never0, a)] + p[1:], slot, c * PPC + j, 128 * n, first, never0)
        return job

    def first_rows(k0, k1, n):
        xn = _unpack(xn_v[n * TH // 2:(n + 1) * TH // 2, :])
        ks = [k for k in range(k0, k1)]
        w = jnp.concatenate([wt_v[1][4 * (k % 32):4 * (k % 32) + 8, :] for k in ks[::2]], axis=0)
        res = _dot(_unpack(w), xn, NT)
        for q, k in enumerate(ks):
            if k % 32 < 31:
                stash_at(0, k % 32, n)[...] = res[8 * q:8 * q + 8, :]

    k0_copy(0).wait()
    x_copy(5).wait()
    wphi_copy(2).start()
    w_copy(1, 2).start()
    x_copy(1).start()
    p0, p1 = fold_pairs(1, 0, 0)
    wt_v[1][8:64, :] = packed(p0[1:] + p1[1:])
    ha_v[0:8, :] = p0[0]
    ha_v[8:16, :] = p1[0]
    never0 = ln_rows(0, 0, TH)[0, 0] < 0.0
    first_rows(2, 16, 0)

    k0_copy(1).wait()
    x_copy(0).wait()
    wphi_copy(1).wait()
    w_copy(1, 3).start()
    for c in range(NC):
        w_copy(2, c).start()
    p2, p3 = fold_pairs(1, 0, 1)
    wt_v[1][0:8, :] = packed([share(ha_v[0:8, :], p3[0], 1), share(ha_v[8:16, :], p3[0], 2)])
    wt_v[1][64:128, :] = packed([share(p2[0], p3[0], 3)] + p2[1:] + p3[1:] + [jnp.zeros((8, D), F32)])
    ln_rows(0, 1, TH)
    first_rows(16, 34, 0)
    first_rows(0, 16, 1)
    first_rows(16, 32, 1)
    expand_wphi(1)

    for c in (1, 2):
        w_copy(1, c).wait()
        if c == 1:
            wphi_copy(2).wait()
            expand_wphi(2)
            expand_wphi(3)
            x_copy(2).start()
            w_copy(0, 0).start()
        side = _Side(never0)
        side.add(PRO_K_PLAN, stashed_k(c - 1, 0, c - 1, True))
        fold(1, c, side, 0)
        stash(c, proj_feat(side, 4, 1, c, xn_tile(0), None)[0])
        side.check()

    x_copy(1).wait()
    w_copy(1, 3).wait()
    side = _Side(never0)
    side.add(PRO_LN1_PLAN, lambda k, a: ln_rows(1, k, LNC, never0, a))
    fold(1, 3, side, 0)
    stash(3, proj_feat(side, 4, 1, 3, xn_tile(0), None)[0])
    xn1 = xn_tile(1)
    spare = None
    for c in range(NC):
        pk, spare = proj_feat(_Side(None), 0, 1, c, xn1, spare)
        if c < 3:
            k_features(pk, 1, c, c == 2, never0)
        else:
            stash(0, pk)

    for c in range(NC):
        w_copy(2, c).wait()
    x_copy(2).wait()
    w_copy(0, 0).wait()
    w_copy(0, 1).start()
    x_copy(3).start()
    wo_copy.start()
    wr_copy.start()
    x_copy(4).start()
    w_copy(0, 2).start()
    w_copy(0, 3).start()
    wg_copy.start()
    wu_copy.start()
    wd_copy.start()
    side = _Side(never0)
    side.add(PRO_V_PLANS[0], stashed_k(2, 0, 2, False))
    side.add(PRO_V_PLANS[1], stashed_k(3, 0, 3, True))
    side.add(PRO_V_PLANS[2], stashed_k(0, 1, 3, False))
    side.add(PRO_V_PLANS[3], lambda k, a: ln_rows(2, k, LNC, never0, a))
    fold(0, 0)
    wt_v[0][248:256, :] = jnp.zeros((8, D), U32)
    xns = (xn_tile(0), xn_tile(1))
    pending = None
    for c in range(NC):
        fold_v(c)
        for i in range(2):
            vt = proj_v(side, 8 * c + 4 * i, c, xns[i])
            if pending is not None:
                kv_update(*pending)
            pending = (vt, i, c, i == 0)
    side.check()
    kv_update(*pending)
    save_lead(0, 0)
    save_lead(1, 2)

    def phase1(u, carry):
        never = u < 0

        @pl.when(u == 0)
        def _():
            w_copy(0, 1).wait()
            x_copy(3).wait()
            wo_copy.wait()
            wr_copy.wait()

        @pl.when(u == 1)
        def _():
            x_copy(4).wait()
            w_copy(0, 2).wait()
            w_copy(0, 3).wait()

        pending = None
        for i in range(2):
            t = 2 * u + 2 + i
            tn = jnp.minimum(t + 1, NT_ - 1)
            side = _Side(never)
            xn = xn_tile(t)
            spare = None
            for c in range(NC):
                pk, spare = proj_feat(_Side(None), 0, 1, c, xn, spare, u + 1 if LEAD and i + c == 0 else None)
                if c == 0 and pending is not None:
                    kv_update(*pending)
                k_features(pk, i, c, False)
            side.add(LN1_PLAN, lambda k, a: ln_rows(tn, k, LNC, never, a))
            if i == 0:
                def pack_wo(k, a):
                    rows = WO_ROWS // len(WO_PLAN)
                    w0 = u * ((D - WO_ROWS) // 2)
                    src = woraw_v.at[pl.ds(pl.multiple_of(w0, 16), WO_ROWS), :]
                    dst = wo_v.at[pl.ds(pl.multiple_of(w0 // 2, 8), WO_ROWS // 2), :]
                    pack_rows(src, dst, k * rows, rows, 0, D, never, a)
                side.add(WO_PLAN, pack_wo)
            else:
                def z_final(k, a):
                    z = _after(z_v[k], never, a)
                    zs = _row_sum(z)
                    zb_v[k] = jnp.broadcast_to(zs, (128, 128))
                    return zs[120:128, :]
                side.add(Z_PLAN, z_final)
            side.done(0, jnp.concatenate(pk[17:], axis=0))
            vts = []
            for c in range(NC):
                vts.append(proj_v(side, 4 * c + 1, c, xn))
                if c > 0:
                    kv_update(vts[c - 1], i, c - 1, False, i == 1)
            pending = (vts[NC - 1], i, NC - 1, False, i == 1)
            side.check()
        fold(0, u + 1)
        kv_update(*pending)
        save_lead(u + 2, tn)
        wr_v[...] = jnp.broadcast_to(wrraw_v[...].reshape(1, D).astype(F32), (8, D))
        return carry

    lax.fori_loop(0, (NT_ - 2) // 2, phase1, 0)

    def o_copy(r0, n, i):
        return pltpu.make_async_copy(o_v.at[pl.ds(r0, n), :], out_hbm.at[pl.ds(r0, n), :], sem.at[SO + i])

    def finish_rows(h_ref, k, ht, valid, st, never=None, anchor=None):
        r0 = ht * TH + k * LNC
        best, besti = st["route"]
        wr = jnp.concatenate([wr_v[...]] * (LNC // 8), axis=0)
        sub = lax.broadcasted_iota(jnp.int32, (8, 1), 0)
        h = _after(h_ref[k * LNC:(k + 1) * LNC, :], never, anchor)
        hc = h - _row_sum(h) * (1.0 / D)
        rstd = lax.rsqrt(_row_sum(hc * hc) * (1.0 / D) + LN_EPS)
        r = (_row_sum(hc * wr) * rstd).astype(BF16).astype(F32)
        hn = hc * rstd
        view(hn_v, ht, TH // 2)[k * LNC // 2:(k + 1) * LNC // 2, :] = _pack(hn.astype(BF16))
        view(o_v, ht, TH)[k * LNC:(k + 1) * LNC, :] = (hn + h).astype(BF16)
        if valid is not None:
            r = jnp.where(valid, r, -jnp.inf)
        for i in range(LNC // 8):
            ri = r[8 * i:8 * i + 8, :]
            better = ri > best
            best = jnp.where(better, ri, best)
            besti = jnp.where(better, sub + (r0 + 8 * i), besti)
        st["route"] = (best, besti)
        return best

    def q_features(pq, slot, c, never):
        for j in range(PPC):
            pr = c * PPC + j
            ep, en, sp, sn = _dual_exp(_pair_logits(pq, j))
            zz = [_lane_tile(zb_v[pr, 8 * i:8 * i + 8, :], T // 128) for i in range(16)]
            ap = _pair_allreduce(_tree(jnp.add, [ep[i] * zz[i] for i in range(8)]), jnp.add)
            an = _pair_allreduce(_tree(jnp.add, [en[i] * zz[8 + i] for i in range(8)]), jnp.add)
            inv = _recip(ap * sn + (an + 1e-6 * sn) * sp)
            scale, es, n, last = (sn * inv, sp * inv), ep + en, 16 // Q_STAGGER, None
            for q in range(Q_STAGGER):
                sc = scale if last is None else [jnp.where(never, last, x) for x in scale]
                phi = jnp.concatenate([es[i] * sc[i // 8] for i in range(q * n, (q + 1) * n)], axis=0)
                phi_v[slot][64 * pr + 4 * q * n:64 * pr + 4 * (q + 1) * n, :] = _pack(phi.astype(BF16))
                last = phi[8 * n - 8:, :]

    def attn_rows(slot, g):
        res = jnp.concatenate(
            [_dot(_unpack(kvbf_v[32 * pr:32 * pr + 32, :]), _unpack(phi_v[slot][64 * pr:64 * pr + 64, :]), NN)
             for pr in (2 * g, 2 * g + 1)], axis=0)
        return res.astype(BF16).T

    def out_proj(side, step0, o, k0, k1):
        cols = []
        for n in range(D // 128):
            w = side.gate(step0 + n, wo_v[k0 // 2:k1 // 2, n * 128:(n + 1) * 128])
            res = _dot(o, _unpack(w), NN)
            side.done(step0 + n, res)
            cols.append(res)
        return jnp.concatenate(cols, axis=1)

    def phase2(u, carry):
        for i in range(UNROLL2):
            carry = phase2_tile(u * UNROLL2 + i, i % 2, carry, u < 0, u if LEAD and i == 0 else None)

        r0 = pl.multiple_of(u * (UNROLL2 * T), T)

        @pl.when(u == 0)
        def _():
            o_copy(0, UNROLL2 * T - TH, 0).start()

        @pl.when(u > 0)
        def _():
            o_copy(pl.multiple_of(jnp.maximum(r0 - TH, 0), TH), UNROLL2 * T, u).start()

        return carry

    def phase2_tile(t, slot, carry, never, lead):
        hp = jnp.maximum(2 * t - 1, 0)
        side = _Side(never)
        st = {"route": carry}
        side.add(LN2B_PLAN, lambda k, a: finish_rows(hb_v, k, hp, t > 0, st, side.never, a))

        def pack_ffn(k, a):
            if k < 32:
                n = D // NT_
                pack_rows(view((wg_v, wu_v)[k % 2], t, n), view((wgp_v, wup_v)[k % 2], t, n // 2),
                          (k // 4) * 16, 16, (0, D)[k // 2 % 2], (D, FM - D)[k // 2 % 2], never, a)
            else:
                n = (FF - FVD) // NT_
                pack_rows(view(wd_v, t, n, FVD), view(wdp_v, t, n // 2), (k - 32) * 16, 16, 0, D, never, a)
        side.add(PACK_PLAN[:32 + (FF - FVD) // 128], pack_ffn)

        xn = xn_tile(t)
        xt = view(x_v, t, T)
        os_ = {}
        for g in range(8):
            side.hooks.setdefault(G_STEPS[g], []).append(lambda g=g: os_.__setitem__(g, attn_rows(slot, g)))
        spare = None
        for c in range(NC):
            pq, spare = proj_feat(side, 100 + 4 * c, 0, c, xn, spare, lead if c == 0 else None)
            if c == 0:
                head = side.gate(0, jnp.concatenate(pq[2:9], axis=0))
                pq = pq[:2] + [head[8 * i:8 * i + 8, :] for i in range(7)] + pq[9:]
            q_features(pq, slot, c, never)
        ha = out_proj(side, 0, jnp.concatenate([os_[g][0:TH, :] for g in range(4)], axis=1), 0, D // 2)
        ha = ha + xt[0:TH, :].astype(F32)
        ha_v[...] = ha + out_proj(side, 8, jnp.concatenate([os_[g][0:TH, :] for g in range(4, 8)], axis=1), D // 2, D)
        side.add(LN2A_PLAN, lambda k, a: finish_rows(ha_v, k, 2 * t, None, st, side.never, a))
        ob = jnp.concatenate([os_[g][TH:T, :] for g in range(8)], axis=1)
        hb_v[...] = xt[TH:T, :].astype(F32) + out_proj(side, 16, ob, 0, D)
        side.check()
        return st["route"]

    wg_copy.wait()
    wu_copy.wait()
    wd_copy.wait()
    route = lax.fori_loop(
        0, NT_ // UNROLL2, phase2,
        (jnp.full((8, 1), -jnp.inf, F32), jnp.zeros((8, 1), jnp.int32)))
    st = {"route": route}
    for k in range(TH // LNC):
        finish_rows(hb_v, k, 2 * NT_ - 1, None, st)
    best, besti = st["route"]
    o_copy(S - TH, TH, NT_).start()

    rmax = jnp.max(best, axis=0, keepdims=True)
    idx = jnp.min(jnp.where(best == rmax, besti, S), axis=0, keepdims=True)
    idx_s = jnp.clip(idx[0, 0], 0, S - 1)
    blk = pl.multiple_of((idx_s >> 4) << 4, 16)
    pair = jnp.broadcast_to(hn_v[pl.ds(idx_s >> 1, 1), :], (8, D))
    x8 = pltpu.bitcast(jnp.where((idx_s & 1) == 1, pair & jnp.uint32(0xFFFF0000), pair << 16), F32)
    xs = jnp.concatenate([x8, x8], axis=0).astype(BF16)
    acts, anchors = [], []

    def park(v, half):
        if not MOE_PARK:
            return v
        n = v.shape[0] // 128
        for i in range(n):
            z_v[i, :, 128 * half:128 * half + 128] = v[128 * i:128 * i + 128, :]
        return jnp.concatenate([z_v[i, :, 128 * half:128 * half + 128] for i in range(n)], axis=0)

    for c0 in range(0, FM, 128):
        g = _dot(xs, _unpack(wgp_v[:, c0:c0 + 128]), NN)[0:8, :]
        u = _dot(xs, _unpack(wup_v[:, c0:c0 + 128]), NN)[0:8, :]
        anchors += [g, u]
        acts.append(g * jax.nn.sigmoid(g) * u)
    xb = park(_col_broadcast(x8), 0)
    if MOE_SPLIT:
        g, u = [_sublane_allreduce(_vpu_matvec(
            xb, lambda g: w[8 * g:8 * g + 8, FM:FF].astype(F32), never0,
            anchors[i * MOE_NA // 2:(i + 1) * MOE_NA // 2], MOE_SPLIT)) for i, w in enumerate((wg_v, wu_v))]
    else:
        gu = _sublane_allreduce(_vpu_matvec(
            xb, lambda g: jnp.concatenate([w[8 * g:8 * g + 8, FM:FF].astype(F32) for w in (wg_v, wu_v)], axis=1),
            never0, anchors[:MOE_NA], 1))
        g, u = gu[:, :FV], gu[:, FV:]
    acts.append(g * jax.nn.sigmoid(g) * u)
    a = jnp.concatenate(acts, axis=1)
    am = jnp.concatenate([a[:, FVD:], a[:, FVD:]], axis=0).astype(BF16)
    ys, anchors = [], anchors[MOE_NA:]
    for k0 in range(0, FF - FVD, 512):
        k1 = min(k0 + 512, FF - FVD)
        yk = _dot(am[:, k0:k1], _unpack(wdp_v[k0 // 2:k1 // 2, :]), NN)[0:8, :]
        ys.append(yk)
        anchors += [yk[:, c:c + 128] for c in range(128, D, 256)]
    ys.append(_sublane_allreduce(_vpu_matvec(
        park(_col_broadcast(a[:, :FVD]), 1), lambda g: wd_v[8 * g:8 * g + 8, 0:D].astype(F32), never0, anchors[:-MOE_ND], MOE_LAG)))
    y = _tree(jnp.add, ys) * jax.nn.sigmoid(rmax)
    y = jnp.concatenate([y, y], axis=0)
    sel = lax.broadcasted_iota(jnp.int32, (16, 1), 0) == (idx_s - blk)
    patch_v[...] = (o_v[pl.ds(blk, 16), :].astype(F32) + jnp.where(sel, y, 0.0)).astype(BF16)
    o_copy(0, UNROLL2 * T - TH, 0).wait()
    for u in range(1, NT_ // UNROLL2):
        o_copy(u * UNROLL2 * T - TH, UNROLL2 * T, u).wait()
    o_copy(S - TH, TH, NT_).wait()
    pc = pltpu.make_async_copy(patch_v, out_hbm.at[pl.ds(blk, 16), :], sem.at[SM + 3])
    pc.start()
    pc.wait()


@jax.jit
def pallas_sequential_preLN__linear_kernel_hedgehog__moe_arch_mod__prompt_kernel(
    A_x: jax.Array,
    A_wqkv: jax.Array,
    A_w_phi: jax.Array,
    A_wo: jax.Array,
    B_x: jax.Array,
    B_w_r: jax.Array,
    B_w_gate: jax.Array,
    B_w_up: jax.Array,
    B_w_down: jax.Array,
):
    del B_x
    hbm = pl.BlockSpec(memory_space=pl.ANY)
    out = pl.pallas_call(
        _kernel,
        out_shape=jax.ShapeDtypeStruct((S, D), BF16),
        in_specs=[hbm] * 8,
        out_specs=hbm,
        scratch_shapes=[
            pltpu.VMEM((S, D), BF16),
            pltpu.VMEM((S // 2, D), U32),
            pltpu.VMEM((5 * D // 4, 128), U32),
            pltpu.VMEM((3 * NC, D, RC), BF16),
            [pltpu.VMEM((D // 2, D), U32)] * 3,
            pltpu.VMEM((H, DH, DH), BF16),
            pltpu.VMEM((8 * 64, 128), U32),
            pltpu.VMEM((D, D), BF16),
            pltpu.VMEM((D // 2, D), U32),
            pltpu.VMEM((D,), BF16),
            pltpu.VMEM((8, D), F32),
            pltpu.VMEM((NPAIR, 64, 128), F32),
            pltpu.VMEM((NPAIR * 32, 128), U32),
            pltpu.VMEM((NPAIR, 128, T), F32),
            pltpu.VMEM((NPAIR, 128, 128), F32),
            [pltpu.VMEM((NPAIR * 64, T), U32)] * 2,
            pltpu.VMEM((TH, D), F32),
            pltpu.VMEM((TH, D), F32),
            pltpu.VMEM((S // 2, D), U32),
            pltpu.VMEM((S, D), BF16),
            pltpu.VMEM((D, FFP), BF16),
            pltpu.VMEM((D, FFP), BF16),
            pltpu.VMEM((FF, D), BF16),
            pltpu.VMEM((D // 2, FM), U32),
            pltpu.VMEM((D // 2, FM), U32),
            pltpu.VMEM(((FF - FVD) // 2, D), U32),
            pltpu.VMEM((16, D), BF16),
            pltpu.SemaphoreType.DMA((6 + 3 * NC + NT_ + 11,)),
        ],
        compiler_params=pltpu.CompilerParams(vmem_limit_bytes=100 * 1024 * 1024,
                                             disable_semaphore_checks=True, disable_bounds_checks=True),
        name="hedgehog_mod",
    )(
        A_x.reshape(S, D),
        A_wqkv,
        A_w_phi,
        A_wo,
        B_w_r,
        B_w_gate,
        B_w_up,
        B_w_down,
    )
    return out.reshape(1, S, D)
```

```python
import math

import jax
import jax.numpy as jnp
from jax import lax
import jax.experimental.pallas as pl
import jax.experimental.pallas.tpu as pltpu

F32 = jnp.float32
BF16 = jnp.bfloat16
U32 = jnp.uint32

S = 2048
D = 1024
H = 32
DH = 32
FF = 3584
NPAIR = H // 2
LOG2E = 1.4426950408889634
LN_EPS = 1e-5

T = 256
TH = T // 2
NT_ = S // T
RC = 256
NC = D // RC
PPC = RC // 64
LNC = 16
FFP = 4096

FV = 10 * 128
FM = FF - FV
FVD = 8 * 128
WO_ROWS = 352


def _spread(n, a, b, due=None):
    rel = [round(a + (b - a) * k / (n - 1), 3) for k in range(n)]
    return tuple((r, None if due is None else math.ceil(r) + due) for r in rel)


LN1_PLAN = tuple((r, math.ceil(r) + 3) for r in (
    -0.052, 0.787, 1.777, 2.636, 3.393, 4.332, 5.206, 6.168, 6.755, 7.637, 8.567, 9.441, 10.518, 11.237, 12.277, 12.961))
WO_PLAN = _spread(11, 1, 11)
Z_PLAN = _spread(16, 6, 12, 3)
PRO_LN1_PLAN = ((None, None),) * 16
PRO_K_PLAN = _spread(8, 0, 6)
PRO_V_PLANS = (_spread(8, 0, 12), _spread(16, 13, 22)[:8], _spread(16, 13, 22)[8:], _spread(16, 1.2, 27, 3))
LN2B_PLAN = ((None, 103), (-0.13, 6), (1.532, 8), (3.446, 10), (4.894, 11), (6.571, 13), (8.519, 15), (9.867, 15))
LN2A_PLAN = ((None, 18), (15.227, 19), (16.121, 20), (16.864, 20), (17.647, 21), (18.474, 22), (19.118, 23), (20.038, None))
PACK_PLAN = _spread(16, 99.7, 114.7) + _spread(16, 99.1, 114.1) + _spread(20, 0.5, 21)
G_STEPS = (107, 107, 111, 111, 115, 115, 3, 3)
MOE_NA = 36
MOE_ND = 3
MOE_LAGS = (3, 2)
STAGGER = 8

NN = (((1,), (0,)), ((), ()))
NT = (((1,), (1,)), ((), ()))


def _dot(a, b, dims):
    return lax.dot_general(a, b, dims, preferred_element_type=F32)


def _recip(x):
    return pl.reciprocal(x, approx=False, full_range=False)


def _pack(x):
    return pltpu.bitcast(x, U32)


def _unpack(x):
    return pltpu.bitcast(x, BF16)


def _pair_allreduce(a, op):
    a = op(a, pltpu.roll(a, 2, 0))
    return op(a, pltpu.roll(a, 4, 0))


def _tree(op, xs):
    xs = list(xs)
    while len(xs) > 1:
        nxt = [op(xs[i], xs[i + 1]) for i in range(0, len(xs) - 1, 2)]
        if len(xs) % 2:
            nxt.append(xs[-1])
        xs = nxt
    return xs[0]


def _pair_logits(sl, j):
    sub = lax.broadcasted_iota(jnp.int32, sl[0].shape, 0)
    if j < 3:
        head = jnp.where(sub < 2, 0.0, sl[(0, 1, 16)[j]])
    else:
        head = jnp.where(sub < 2, sl[0], jnp.where(sub < 4, pltpu.roll(sl[1], 2, 0),
                                                   jnp.where(sub < 6, pltpu.roll(sl[16], 4, 0), 0.0)))
    r0 = (2, 9, 17, 24)[j]
    return [head] + list(sl[r0:r0 + 7])


def _dual_exp(sl):
    mx = _pair_allreduce(_tree(jnp.maximum, sl), jnp.maximum)
    mn = _pair_allreduce(_tree(jnp.minimum, sl), jnp.minimum)
    ep = [jnp.exp2(s - mx) for s in sl]
    en = [jnp.exp2(mn - s) for s in sl]
    sp = _pair_allreduce(_tree(jnp.add, ep), jnp.add)
    sn = _pair_allreduce(_tree(jnp.add, en), jnp.add)
    return ep, en, sp, sn


def _after(x, never, anchor):
    if anchor is None:
        return x
    d = jnp.concatenate([anchor] * (x.shape[0] // 8), axis=0)
    if x.shape[1] == 128:
        return jnp.where(never, d, x)
    return jnp.concatenate([jnp.where(never, d, x[:, :128]), x[:, 128:]], axis=1)


def _gate(x, never, deps):
    for i, dep in enumerate(deps):
        d = jnp.broadcast_to(dep, (8, 128))
        if x.dtype != F32:
            d = pltpu.bitcast(d, x.dtype)
        blk = jnp.where(never, d, x[8 * i:8 * i + 8, :128])
        if x.shape[1] > 128:
            blk = jnp.concatenate([blk, x[8 * i:8 * i + 8, 128:]], axis=1)
        parts = ([x[:8 * i, :]] if i else []) + [blk, x[8 * i + 8:, :]]
        x = jnp.concatenate(parts, axis=0)
    return x


def _lane_fold(a):
    return _tree(jnp.add, [a[:, 128 * i:128 * i + 128] for i in range(a.shape[1] // 128)])


def _row_sum(a):
    return jnp.sum(_lane_fold(a), axis=-1, keepdims=True)


def _lane_tile(a, n):
    return a if n == 1 else jnp.concatenate([a] * n, axis=1)


def _sublane_allreduce(a):
    a = a + pltpu.roll(a, 4, 0)
    a = a + pltpu.roll(a, 2, 0)
    return a + pltpu.roll(a, 1, 0)


def _col_broadcast(row8):
    return jnp.concatenate([row8] * 16, axis=0).astype(BF16).T.astype(F32)


def _vpu_matvec(xb, w_rows, never, anchors, lag):
    ng = xb.shape[0] // 8
    acc, hist = None, []
    for g in range(ng):
        dep = anchors[(g * len(anchors)) // ng]
        if g >= lag:
            dep = dep + hist[g - lag]
        x = jnp.where(never, dep, xb[8 * g:8 * g + 8, :])
        w = w_rows(g)
        t = w * _lane_tile(x, w.shape[1] // 128)
        acc = t if acc is None else acc + t
        c = 128 * (g % (w.shape[1] // 128))
        hist.append(acc[:, c:c + 128])
    return acc


class _Side:
    def __init__(self, never):
        self.never = never
        self.jobs = []
        self.deps = {}
        self.hooks = {}

    def add(self, plan, fn):
        for k, (rel, due) in enumerate(plan):
            if rel is None:
                self._run(due, fn, k, None)
            else:
                self.jobs.append((rel, due, fn, k))

    def _run(self, due, fn, k, anchor):
        dep = fn(k, anchor)
        if due is not None:
            self.deps.setdefault(due, []).append(dep)

    def check(self):
        assert not self.jobs and not self.deps and not self.hooks

    def gate(self, step, x):
        return _gate(x, self.never, self.deps.pop(step, []))

    def done(self, step, res):
        m = res.shape[0] // 8
        for job in sorted([j for j in self.jobs if step - 1 < j[0] <= step], key=lambda j: j[0]):
            self.jobs.remove(job)
            g = m - 1 - int((step - job[0]) * m)
            self._run(job[1], job[2], job[3], res[8 * g:8 * g + 8, res.shape[1] - 128:])
        for fn in self.hooks.pop(step, []):
            fn()


def _kernel(x_hbm, wqkv_hbm, wphi_hbm, wo_hbm, wr_hbm, wg_hbm, wu_hbm, wd_hbm, out_hbm,
            x_v, xn_v, lead_v, wraw_v, wt_v, wphi_v, a_v, woraw_v, wo_v, wrraw_v, wr_v, kvacc_v, kvbf_v,
            z_v, zb_v, phi_v, ha_v, hb_v, hn_v, o_v, wg_v, wu_v, wd_v, wgp_v, wup_v, wdp_v, patch_v,
            sem):
    SX, SW, SO, SM = 0, 6, 6 + 3 * NC, 6 + 3 * NC + NT_ + 1

    def x_copy(i):
        h0, h1 = ((1, 2), (2, 4), (4, 6), (6, 10), (10, 2 * NT_), (0, 1))[i]
        rows = pl.ds(h0 * TH, (h1 - h0) * TH)
        return pltpu.make_async_copy(x_hbm.at[rows, :], x_v.at[rows, :], sem.at[SX + i])

    def k0_copy(s):
        return pltpu.make_async_copy(wqkv_hbm.at[:, pl.ds(D + s * 128, 128)],
                                     wraw_v.at[NC, :, pl.ds(s * 128, 128)], sem.at[(SM + 7, SW + NC)[s]])

    def w_copy(j, c):
        return pltpu.make_async_copy(wqkv_hbm.at[:, pl.ds(j * D + c * RC, RC)], wraw_v.at[j * NC + c],
                                     sem.at[SW + j * NC + c])

    def wphi_copy(i):
        h0, h1 = ((0, 8), (8, 16), (16, H))[i]
        return pltpu.make_async_copy(wphi_hbm.at[pl.ds(h0, h1 - h0)], wphi_v.at[pl.ds(h0, h1 - h0)],
                                     sem.at[(SM + 4, SM + 8, SM + 9)[i]])

    wr_copy = pltpu.make_async_copy(wr_hbm, wrraw_v, sem.at[SM + 5])
    wo_copy = pltpu.make_async_copy(wo_hbm, woraw_v, sem.at[SM + 6])
    wg_copy = pltpu.make_async_copy(wg_hbm, wg_v.at[:, pl.ds(0, FF)], sem.at[SM + 0])
    wu_copy = pltpu.make_async_copy(wu_hbm, wu_v.at[:, pl.ds(0, FF)], sem.at[SM + 1])
    wd_copy = pltpu.make_async_copy(wd_hbm, wd_v, sem.at[SM + 2])

    wphi_copy(0).start()
    k0_copy(0).start()
    x_copy(5).start()
    k0_copy(1).start()
    x_copy(0).start()
    wphi_copy(1).start()
    w_copy(1, 1).start()

    def view(ref, i, n, off=0):
        r0 = off + i * n
        return ref.at[pl.ds(r0 if isinstance(r0, int) else pl.multiple_of(r0, math.gcd(n, off)), n), :]

    def ln_rows(t, k, n, never=None, anchor=None):
        x = _after(view(x_v, t, T)[k * n:(k + 1) * n, :].astype(F32), never, anchor)
        xc = x - _row_sum(x) * (1.0 / D)
        rstd = lax.rsqrt(_row_sum(xc * xc) * (1.0 / D) + LN_EPS)
        view(xn_v, t, T // 2)[k * n // 2:(k + 1) * n // 2, :] = _pack((xc * rstd).astype(BF16))
        return _tree(jnp.add, [rstd[8 * i:8 * i + 8, :] for i in range(min(n, LNC) // 8)])

    def xn_tile(t):
        return _unpack(view(xn_v, t, T // 2)[...])

    def expand_wphi(c):
        w = wphi_v[8 * c:8 * c + 8].reshape(8 * DH, DH).astype(F32).T
        bits = pltpu.bitcast(w, U32)
        head = lax.broadcasted_iota(jnp.int32, (DH, 128), 1) >> 5
        for s in range(2):
            b = bits[:, 128 * s:128 * s + 128]
            for j in range(2):
                r0 = 64 * (2 * c + s) + 32 * j
                a_v[r0:r0 + 32, :] = jnp.where(head == 2 * j, b >> 16,
                                               jnp.where(head == 2 * j + 1, b, jnp.uint32(0)))

    wphi_copy(0).wait()
    expand_wphi(0)
    hb_v[...] = jnp.zeros((TH, D), F32)

    def fold_v(c):
        for s in range(RC // 128):
            g0 = 64 * (2 * c + s)
            wt_v[2][g0:g0 + 64, :] = _pack(wraw_v[2 * NC + c, :, s * 128:(s + 1) * 128].T)

    def fold_pairs(j, c, s, side=None, step0=None):
        g0 = 64 * (2 * c + s)
        g0 = g0 if isinstance(g0, int) else pl.multiple_of(g0, 64)
        res = _dot(_unpack(a_v[pl.ds(g0, 64), :]), wraw_v[j * NC + c, :, s * 128:(s + 1) * 128], NT)
        if side is not None:
            side.done(step0 + 2 * s, res[:, :D // 2])
            side.done(step0 + 2 * s + 1, res[:, D // 2:])
        sub = lax.broadcasted_iota(jnp.int32, (8, D), 0)
        out = []
        for q in range(2):
            base = _pair_allreduce(jnp.where(sub < 2, res[64 * q:64 * q + 8, :], 0.0), jnp.add)
            out.append([(res[64 * q + 8 * i:64 * q + 8 * i + 8, :] - base) * LOG2E for i in range(8)])
        return out

    def share(z, z3, k):
        sub = lax.broadcasted_iota(jnp.int32, (8, D), 0)
        return jnp.where(sub < 2, pltpu.roll(z3, 8 - 2 * k, 0), z)

    def packed(slabs):
        return _pack(jnp.concatenate(slabs, axis=0).astype(BF16))

    def fold(j, c, side=None, step0=None):
        p0, p1 = fold_pairs(j, c, 0, side, step0)
        p2, p3 = fold_pairs(j, c, 1, side, step0)
        sl = ([share(p0[0], p3[0], 1), share(p1[0], p3[0], 2)] + p0[1:] + p1[1:]
              + [share(p2[0], p3[0], 3)] + p2[1:] + p3[1:])
        zero = jnp.zeros((8, D), F32)
        even, odd = sl + [zero], [zero] + sl
        r0 = 8 * ((31 * c) // 2)
        if isinstance(c, int):
            is_odd = c % 2 == 1
            sl = odd if is_odd else even
        else:
            is_odd = c % 2 == 1
            r0 = pl.multiple_of(r0, 8)
            sl = [jnp.where(is_odd, o, e) for o, e in zip(odd, even)]
        win = wt_v[j].at[pl.ds(r0, 128), :]
        win[8:128, :] = packed(sl[2:])
        first = packed(sl[:2])
        if is_odd is not False:
            keep = lax.broadcasted_iota(jnp.int32, (8, D), 0) < jnp.where(is_odd, 4, 0)
            first = jnp.where(keep, win[0:8, :], first)
        win[0:8, :] = first

    def k_pair(p, slot, pr, c0, first, never=None):
        ep, en, sp, sn = _dual_exp(p)
        inv = _recip(sp * sn)
        scale = (sn * inv, sp * inv)
        es = ep + en
        cols = slice(c0, c0 + p[0].shape[1])
        n = 16 if never is None else 16 // STAGGER
        last = None
        for q in range(16 // n):
            sc = scale
            if last is not None:
                sc = [jnp.where(never, last, x) for x in scale]
            phi = jnp.concatenate([es[i] * sc[i // 8] for i in range(q * n, (q + 1) * n)], axis=0)
            rows = slice(8 * q * n, 8 * (q + 1) * n)
            z = phi if first else z_v[pr, rows, cols] + phi
            z_v[pr, rows, cols] = z
            phi_v[slot][64 * pr + 4 * q * n:64 * pr + 4 * (q + 1) * n, cols] = _pack(phi.astype(BF16))
            last = z[8 * n - 8:, :]

    def k_features(pk, slot, c, first, never=None):
        for j in range(PPC):
            k_pair(_pair_logits(pk, j), slot, c * PPC + j, 0, first, never)

    def kv_update(vt, slot, c, first, publish=False):
        for j in range(PPC):
            pr = c * PPC + j
            upd = _dot(vt[64 * j:64 * j + 64, :].astype(BF16), _unpack(phi_v[slot][64 * pr:64 * pr + 64, :]), NT)
            acc = upd if first else kvacc_v[pr] + upd
            kvacc_v[pr] = acc
            if publish:
                odd = -(lax.broadcasted_iota(jnp.int32, (32, 128), 1) & 1)
                bits = pltpu.bitcast(acc, jnp.int32) & jnp.concatenate([~odd, odd], axis=0)
                kvbf_v[32 * pr:32 * pr + 32, :] = _pack(pltpu.bitcast(bits, F32).astype(BF16))

    def save_lead(e, t):
        corner = _unpack(view(xn_v, t, T // 2)[0:TH // 2, 0:D // 2])
        view(lead_v, e, D // 4)[...] = _pack(corner.T)

    def proj_steps(side, step0, w, xn, lead=None):
        quarters = []
        for n in range(2):
            for m in range(2):
                step = step0 + 2 * n + m
                wq = _unpack(side.gate(step, w[:64, :] if m == 0 else w[64:, :]))
                if lead is not None and n + m == 0:
                    res = _dot(wq[:, :D // 2], _unpack(view(lead_v, lead, D // 4)[...]), NN)
                    res = _dot(wq[:, D // 2:], xn[0:TH, D // 2:], NT) + res
                else:
                    res = _dot(wq, xn[n * TH:(n + 1) * TH, :], NT)
                side.done(step, res)
                quarters.append(res)
        return jnp.concatenate(
            [jnp.concatenate([quarters[0], quarters[2]], axis=1),
             jnp.concatenate([quarters[1], quarters[3]], axis=1)], axis=0)

    def proj_v(side, step0, c, xn):
        return proj_steps(side, step0, wt_v[2][128 * c:128 * c + 128, :], xn)

    def proj_feat(side, step0, j, c, xn, carry, lead=None):
        r0 = 8 * ((31 * c) // 2)
        skip = 8 if c % 2 == 1 and carry is not None else 0
        res = proj_steps(side, step0, wt_v[j][r0 + skip:r0 + 128, :], xn, lead)
        sl = [res[8 * i:8 * i + 8, :] for i in range(res.shape[0] // 8)]
        if c % 2 == 0:
            return sl[:31], sl[31]
        return ([carry] + sl if skip else sl[1:]), None

    def pack_rows(src, dst, r0, rows, c0, cols, never, a):
        w = src[r0:r0 + rows, c0:c0 + cols].astype(F32)
        d = _lane_tile(a, cols // 128)
        w = jnp.concatenate([jnp.where(never, d, w[8 * i:8 * i + 8, :]) if i % 2 == 0 else w[8 * i:8 * i + 8, :]
                             for i in range(rows // 8)], axis=0)
        dst[r0 // 2:(r0 + rows) // 2, c0:c0 + cols] = _pack(w.astype(BF16))

    def stash_at(i, k, n):
        return zb_v.at[4 * i + 2 * (k // 16) + n, pl.ds(8 * (k % 16), 8), :]

    def stash(i, sl):
        for k, v in enumerate(sl):
            for n in range(2):
                stash_at(i, k, n)[...] = v[:, 128 * n:128 * n + 128]

    def stashed_k(i, slot, c, first):
        def job(k, a):
            j, n = k // 2, k % 2
            p = _pair_logits([stash_at(i, q, n)[...] for q in range(31)], j)
            k_pair([_after(p[0], never0, a)] + p[1:], slot, c * PPC + j, 128 * n, first, never0)
        return job

    def first_rows(k0, k1, n):
        xn = _unpack(xn_v[n * TH // 2:(n + 1) * TH // 2, :])
        ks = [k for k in range(k0, k1)]
        w = jnp.concatenate([wt_v[1][4 * (k % 32):4 * (k % 32) + 8, :] for k in ks[::2]], axis=0)
        res = _dot(_unpack(w), xn, NT)
        for q, k in enumerate(ks):
            if k % 32 < 31:
                stash_at(0, k % 32, n)[...] = res[8 * q:8 * q + 8, :]

    k0_copy(0).wait()
    x_copy(5).wait()
    wphi_copy(2).start()
    w_copy(1, 2).start()
    x_copy(1).start()
    p0, p1 = fold_pairs(1, 0, 0)
    wt_v[1][8:64, :] = packed(p0[1:] + p1[1:])
    ha_v[0:8, :] = p0[0]
    ha_v[8:16, :] = p1[0]
    never0 = ln_rows(0, 0, TH)[0, 0] < 0.0
    first_rows(2, 16, 0)

    k0_copy(1).wait()
    x_copy(0).wait()
    wphi_copy(1).wait()
    w_copy(1, 3).start()
    for c in range(NC):
        w_copy(2, c).start()
    p2, p3 = fold_pairs(1, 0, 1)
    wt_v[1][0:8, :] = packed([share(ha_v[0:8, :], p3[0], 1), share(ha_v[8:16, :], p3[0], 2)])
    wt_v[1][64:128, :] = packed([share(p2[0], p3[0], 3)] + p2[1:] + p3[1:] + [jnp.zeros((8, D), F32)])
    ln_rows(0, 1, TH)
    first_rows(16, 34, 0)
    first_rows(0, 16, 1)
    first_rows(16, 32, 1)
    expand_wphi(1)

    for c in (1, 2):
        w_copy(1, c).wait()
        if c == 1:
            wphi_copy(2).wait()
            expand_wphi(2)
            expand_wphi(3)
            x_copy(2).start()
            w_copy(0, 0).start()
        side = _Side(never0)
        side.add(PRO_K_PLAN, stashed_k(c - 1, 0, c - 1, True))
        fold(1, c, side, 0)
        stash(c, proj_feat(side, 4, 1, c, xn_tile(0), None)[0])
        side.check()

    x_copy(1).wait()
    w_copy(1, 3).wait()
    side = _Side(never0)
    side.add(PRO_LN1_PLAN, lambda k, a: ln_rows(1, k, LNC, never0, a))
    fold(1, 3, side, 0)
    stash(3, proj_feat(side, 4, 1, 3, xn_tile(0), None)[0])
    xn1 = xn_tile(1)
    spare = None
    for c in range(NC):
        pk, spare = proj_feat(_Side(None), 0, 1, c, xn1, spare)
        if c < 3:
            k_features(pk, 1, c, c == 2, never0)
        else:
            stash(0, pk)

    for c in range(NC):
        w_copy(2, c).wait()
    x_copy(2).wait()
    w_copy(0, 0).wait()
    w_copy(0, 1).start()
    x_copy(3).start()
    wo_copy.start()
    wr_copy.start()
    x_copy(4).start()
    w_copy(0, 2).start()
    w_copy(0, 3).start()
    wg_copy.start()
    wu_copy.start()
    wd_copy.start()
    side = _Side(never0)
    side.add(PRO_V_PLANS[0], stashed_k(2, 0, 2, False))
    side.add(PRO_V_PLANS[1], stashed_k(3, 0, 3, True))
    side.add(PRO_V_PLANS[2], stashed_k(0, 1, 3, False))
    side.add(PRO_V_PLANS[3], lambda k, a: ln_rows(2, k, LNC, never0, a))
    fold(0, 0)
    wt_v[0][248:256, :] = jnp.zeros((8, D), U32)
    xns = (xn_tile(0), xn_tile(1))
    pending = None
    for c in range(NC):
        fold_v(c)
        for i in range(2):
            vt = proj_v(side, 8 * c + 4 * i, c, xns[i])
            if pending is not None:
                kv_update(*pending)
            pending = (vt, i, c, i == 0)
    side.check()
    kv_update(*pending)
    save_lead(0, 0)
    save_lead(1, 2)

    def phase1(u, carry):
        never = u < 0

        @pl.when(u == 0)
        def _():
            w_copy(0, 1).wait()
            x_copy(3).wait()
            wo_copy.wait()
            wr_copy.wait()

        @pl.when(u == 1)
        def _():
            x_copy(4).wait()
            w_copy(0, 2).wait()
            w_copy(0, 3).wait()

        pending = None
        for i in range(2):
            t = 2 * u + 2 + i
            tn = jnp.minimum(t + 1, NT_ - 1)
            side = _Side(never)
            xn = xn_tile(t)
            spare = None
            for c in range(NC):
                pk, spare = proj_feat(_Side(None), 0, 1, c, xn, spare, u + 1 if i + c == 0 else None)
                if c == 0 and pending is not None:
                    kv_update(*pending)
                k_features(pk, i, c, False)
            side.add(LN1_PLAN, lambda k, a: ln_rows(tn, k, LNC, never, a))
            if i == 0:
                def pack_wo(k, a):
                    rows = WO_ROWS // len(WO_PLAN)
                    w0 = u * ((D - WO_ROWS) // 2)
                    src = woraw_v.at[pl.ds(pl.multiple_of(w0, 16), WO_ROWS), :]
                    dst = wo_v.at[pl.ds(pl.multiple_of(w0 // 2, 8), WO_ROWS // 2), :]
                    pack_rows(src, dst, k * rows, rows, 0, D, never, a)
                side.add(WO_PLAN, pack_wo)
            else:
                def z_final(k, a):
                    z = _after(z_v[k], never, a)
                    zs = _row_sum(z)
                    zb_v[k] = jnp.broadcast_to(zs, (128, 128))
                    return zs[120:128, :]
                side.add(Z_PLAN, z_final)
            side.done(0, jnp.concatenate(pk[17:], axis=0))
            vts = []
            for c in range(NC):
                vts.append(proj_v(side, 4 * c + 1, c, xn))
                if c > 0:
                    kv_update(vts[c - 1], i, c - 1, False, i == 1)
            pending = (vts[NC - 1], i, NC - 1, False, i == 1)
            side.check()
        fold(0, u + 1)
        kv_update(*pending)
        save_lead(u + 2, tn)
        wr_v[...] = jnp.broadcast_to(wrraw_v[...].reshape(1, D).astype(F32), (8, D))
        return carry

    lax.fori_loop(0, (NT_ - 2) // 2, phase1, 0)

    def o_copy(r0, n, i):
        return pltpu.make_async_copy(o_v.at[pl.ds(r0, n), :], out_hbm.at[pl.ds(r0, n), :], sem.at[SO + i])

    def finish_rows(h_ref, k, ht, valid, st, never=None, anchor=None):
        r0 = ht * TH + k * LNC
        best, besti = st["route"]
        wr = jnp.concatenate([wr_v[...]] * (LNC // 8), axis=0)
        sub = lax.broadcasted_iota(jnp.int32, (8, 1), 0)
        h = _after(h_ref[k * LNC:(k + 1) * LNC, :], never, anchor)
        hc = h - _row_sum(h) * (1.0 / D)
        rstd = lax.rsqrt(_row_sum(hc * hc) * (1.0 / D) + LN_EPS)
        r = (_row_sum(hc * wr) * rstd).astype(BF16).astype(F32)
        hn = hc * rstd
        view(hn_v, ht, TH // 2)[k * LNC // 2:(k + 1) * LNC // 2, :] = _pack(hn.astype(BF16))
        view(o_v, ht, TH)[k * LNC:(k + 1) * LNC, :] = (hn + h).astype(BF16)
        if valid is not None:
            r = jnp.where(valid, r, -jnp.inf)
        for i in range(LNC // 8):
            ri = r[8 * i:8 * i + 8, :]
            better = ri > best
            best = jnp.where(better, ri, best)
            besti = jnp.where(better, sub + (r0 + 8 * i), besti)
        st["route"] = (best, besti)
        return best

    def q_features(pq, slot, c):
        for j in range(PPC):
            pr = c * PPC + j
            ep, en, sp, sn = _dual_exp(_pair_logits(pq, j))
            zz = [_lane_tile(zb_v[pr, 8 * i:8 * i + 8, :], T // 128) for i in range(16)]
            ap = _pair_allreduce(_tree(jnp.add, [ep[i] * zz[i] for i in range(8)]), jnp.add)
            an = _pair_allreduce(_tree(jnp.add, [en[i] * zz[8 + i] for i in range(8)]), jnp.add)
            inv = _recip(ap * sn + (an + 1e-6 * sn) * sp)
            rp = sn * inv
            rn = sp * inv
            phi = jnp.concatenate([e * rp for e in ep] + [e * rn for e in en], axis=0)
            phi_v[slot][64 * pr:64 * pr + 64, :] = _pack(phi.astype(BF16))

    def attn_rows(slot, g):
        res = jnp.concatenate(
            [_dot(_unpack(kvbf_v[32 * pr:32 * pr + 32, :]), _unpack(phi_v[slot][64 * pr:64 * pr + 64, :]), NN)
             for pr in (2 * g, 2 * g + 1)], axis=0)
        return res.astype(BF16).T

    def out_proj(side, step0, o, k0, k1):
        cols = []
        for n in range(D // 128):
            w = side.gate(step0 + n, wo_v[k0 // 2:k1 // 2, n * 128:(n + 1) * 128])
            res = _dot(o, _unpack(w), NN)
            side.done(step0 + n, res)
            cols.append(res)
        return jnp.concatenate(cols, axis=1)

    def phase2(u, carry):
        for i in range(2):
            carry = phase2_tile(u * 2 + i, i % 2, carry, u < 0, u if i == 0 else None)

        r0 = pl.multiple_of(u * (2 * T), T)

        @pl.when(u == 0)
        def _():
            o_copy(0, 2 * T - TH, 0).start()

        @pl.when(u > 0)
        def _():
            o_copy(pl.multiple_of(jnp.maximum(r0 - TH, 0), TH), 2 * T, u).start()

        return carry

    def phase2_tile(t, slot, carry, never, lead):
        hp = jnp.maximum(2 * t - 1, 0)
        side = _Side(never)
        st = {"route": carry}
        side.add(LN2B_PLAN, lambda k, a: finish_rows(hb_v, k, hp, t > 0, st, side.never, a))

        def pack_ffn(k, a):
            if k < 32:
                n = D // NT_
                pack_rows(view((wg_v, wu_v)[k % 2], t, n), view((wgp_v, wup_v)[k % 2], t, n // 2),
                          (k // 4) * 16, 16, (0, D)[k // 2 % 2], (D, FM - D)[k // 2 % 2], never, a)
            else:
                n = (FF - FVD) // NT_
                pack_rows(view(wd_v, t, n, FVD), view(wdp_v, t, n // 2), (k - 32) * 16, 16, 0, D, never, a)
        side.add(PACK_PLAN[:32 + (FF - FVD) // 128], pack_ffn)

        xn = xn_tile(t)
        xt = view(x_v, t, T)
        os_ = {}
        for g in range(8):
            side.hooks.setdefault(G_STEPS[g], []).append(lambda g=g: os_.update({g: attn_rows(slot, g)}))
        spare = None
        for c in range(NC):
            pq, spare = proj_feat(side, 100 + 4 * c, 0, c, xn, spare, lead if c == 0 else None)
            if c == 0:
                head = side.gate(0, jnp.concatenate(pq[2:9], axis=0))
                pq = pq[:2] + [head[8 * i:8 * i + 8, :] for i in range(7)] + pq[9:]
            q_features(pq, slot, c)
        ha = out_proj(side, 0, jnp.concatenate([os_[g][0:TH, :] for g in range(4)], axis=1), 0, D // 2)
        ha = ha + xt[0:TH, :].astype(F32)
        ha_v[...] = ha + out_proj(side, 8, jnp.concatenate([os_[g][0:TH, :] for g in range(4, 8)], axis=1), D // 2, D)
        side.add(LN2A_PLAN, lambda k, a: finish_rows(ha_v, k, 2 * t, None, st, side.never, a))
        ob = jnp.concatenate([os_[g][TH:T, :] for g in range(8)], axis=1)
        hb_v[...] = xt[TH:T, :].astype(F32) + out_proj(side, 16, ob, 0, D)
        side.check()
        return st["route"]

    wg_copy.wait()
    wu_copy.wait()
    wd_copy.wait()
    route = lax.fori_loop(
        0, NT_ // 2, phase2,
        (jnp.full((8, 1), -jnp.inf, F32), jnp.zeros((8, 1), jnp.int32)))
    st = {"route": route}
    for k in range(TH // LNC):
        finish_rows(hb_v, k, 2 * NT_ - 1, None, st)
    best, besti = st["route"]
    o_copy(S - TH, TH, NT_).start()

    rmax = jnp.max(best, axis=0, keepdims=True)
    idx = jnp.min(jnp.where(best == rmax, besti, S), axis=0, keepdims=True)
    idx_s = jnp.clip(idx[0, 0], 0, S - 1)
    blk = pl.multiple_of((idx_s >> 4) << 4, 16)
    pair = jnp.broadcast_to(hn_v[pl.ds(idx_s >> 1, 1), :], (8, D))
    x8 = pltpu.bitcast(jnp.where((idx_s & 1) == 1, pair & jnp.uint32(0xFFFF0000), pair << 16), F32)
    xs = jnp.concatenate([x8, x8], axis=0).astype(BF16)
    acts, anchors = [], []

    def park(v, half):
        n = v.shape[0] // 128
        for i in range(n):
            z_v[i, :, 128 * half:128 * half + 128] = v[128 * i:128 * i + 128, :]
        return jnp.concatenate([z_v[i, :, 128 * half:128 * half + 128] for i in range(n)], axis=0)

    for c0 in range(0, FM, 128):
        g = _dot(xs, _unpack(wgp_v[:, c0:c0 + 128]), NN)[0:8, :]
        u = _dot(xs, _unpack(wup_v[:, c0:c0 + 128]), NN)[0:8, :]
        anchors += [g, u]
        acts.append(g * jax.nn.sigmoid(g) * u)
    xb = park(_col_broadcast(x8), 0)
    g, u = [_sublane_allreduce(_vpu_matvec(
        xb, lambda g: w[8 * g:8 * g + 8, FM:FF].astype(F32), never0,
        anchors[i * MOE_NA // 2:(i + 1) * MOE_NA // 2], MOE_LAGS[0])) for i, w in enumerate((wg_v, wu_v))]
    acts.append(g * jax.nn.sigmoid(g) * u)
    a = jnp.concatenate(acts, axis=1)
    am = jnp.concatenate([a[:, FVD:], a[:, FVD:]], axis=0).astype(BF16)
    ys, anchors = [], anchors[MOE_NA:]
    for k0 in range(0, FF - FVD, 512):
        k1 = min(k0 + 512, FF - FVD)
        yk = _dot(am[:, k0:k1], _unpack(wdp_v[k0 // 2:k1 // 2, :]), NN)[0:8, :]
        ys.append(yk)
        anchors += [yk[:, c:c + 128] for c in range(128, D, 256)]
    ys.append(_sublane_allreduce(_vpu_matvec(
        park(_col_broadcast(a[:, :FVD]), 1), lambda g: wd_v[8 * g:8 * g + 8, :].astype(F32), never0,
        anchors[:-MOE_ND], MOE_LAGS[1])))
    y = _tree(jnp.add, ys) * jax.nn.sigmoid(rmax)
    y = jnp.concatenate([y, y], axis=0)
    sel = lax.broadcasted_iota(jnp.int32, (16, 1), 0) == (idx_s - blk)
    patch_v[...] = (o_v[pl.ds(blk, 16), :].astype(F32) + jnp.where(sel, y, 0.0)).astype(BF16)
    o_copy(0, 2 * T - TH, 0).wait()
    for u in range(1, NT_ // 2):
        o_copy(u * 2 * T - TH, 2 * T, u).wait()
    o_copy(S - TH, TH, NT_).wait()
    pc = pltpu.make_async_copy(patch_v, out_hbm.at[pl.ds(blk, 16), :], sem.at[SM + 3])
    pc.start()
    pc.wait()


@jax.jit
def pallas_sequential_preLN__linear_kernel_hedgehog__moe_arch_mod__prompt_kernel(
    A_x: jax.Array,
    A_wqkv: jax.Array,
    A_w_phi: jax.Array,
    A_wo: jax.Array,
    B_x: jax.Array,
    B_w_r: jax.Array,
    B_w_gate: jax.Array,
    B_w_up: jax.Array,
    B_w_down: jax.Array,
):
    del B_x
    hbm = pl.BlockSpec(memory_space=pl.ANY)
    out = pl.pallas_call(
        _kernel,
        out_shape=jax.ShapeDtypeStruct((S, D), BF16),
        in_specs=[hbm] * 8,
        out_specs=hbm,
        scratch_shapes=[
            pltpu.VMEM((S, D), BF16),
            pltpu.VMEM((S // 2, D), U32),
            pltpu.VMEM((5 * D // 4, 128), U32),
            pltpu.VMEM((3 * NC, D, RC), BF16),
            [pltpu.VMEM((D // 2, D), U32)] * 3,
            pltpu.VMEM((H, DH, DH), BF16),
            pltpu.VMEM((8 * 64, 128), U32),
            pltpu.VMEM((D, D), BF16),
            pltpu.VMEM((D // 2, D), U32),
            pltpu.VMEM((D,), BF16),
            pltpu.VMEM((8, D), F32),
            pltpu.VMEM((NPAIR, 64, 128), F32),
            pltpu.VMEM((NPAIR * 32, 128), U32),
            pltpu.VMEM((NPAIR, 128, T), F32),
            pltpu.VMEM((NPAIR, 128, 128), F32),
            [pltpu.VMEM((NPAIR * 64, T), U32)] * 2,
            pltpu.VMEM((TH, D), F32),
            pltpu.VMEM((TH, D), F32),
            pltpu.VMEM((S // 2, D), U32),
            pltpu.VMEM((S, D), BF16),
            pltpu.VMEM((D, FFP), BF16),
            pltpu.VMEM((D, FFP), BF16),
            pltpu.VMEM((FF, D), BF16),
            pltpu.VMEM((D // 2, FM), U32),
            pltpu.VMEM((D // 2, FM), U32),
            pltpu.VMEM(((FF - FVD) // 2, D), U32),
            pltpu.VMEM((16, D), BF16),
            pltpu.SemaphoreType.DMA((6 + 3 * NC + NT_ + 11,)),
        ],
        compiler_params=pltpu.CompilerParams(vmem_limit_bytes=100 * 1024 * 1024,
                                             disable_semaphore_checks=True, disable_bounds_checks=True),
        name="hedgehog_mod",
    )(
        A_x.reshape(S, D),
        A_wqkv,
        A_w_phi,
        A_wo,
        B_w_r,
        B_w_gate,
        B_w_up,
        B_w_down,
    )
    return out.reshape(1, S, D)
```

```python
import math

import jax
import jax.numpy as jnp
from jax import lax
import jax.experimental.pallas as pl
import jax.experimental.pallas.tpu as pltpu

F32 = jnp.float32
BF16 = jnp.bfloat16
U32 = jnp.uint32

S = 2048
D = 1024
H = 32
DH = 32
FF = 3584
NPAIR = H // 2
LOG2E = 1.4426950408889634
LN_EPS = 1e-5

T = 256
TH = T // 2
NT_ = S // T
RC = 256
NC = D // RC
PPC = RC // 64
LNC = 16
FFP = 4096

FV = 10 * 128
FM = FF - FV
FVD = 8 * 128
WO_ROWS = 352


def _spread(n, a, b, due=None):
    rel = [round(a + (b - a) * k / (n - 1), 3) for k in range(n)]
    return tuple((r, None if due is None else math.ceil(r) + due) for r in rel)


LN1_PLAN = ((-0.001, 4), (0.787, 5), (1.823, 5), (2.494, 6), (3.413, 7), (4.33, 9), (5.163, 9), (6.264, 10),
    (6.755, 10), (7.681, 11), (8.866, 13), (9.289, 14), (10.598, 14), (11.083, 15), (12.313, 16), (13.022,
    16))
WO_PLAN = ((0.92, None), (1.762, None), (4.0, None), (4.445, None), (5.249, None), (5.684, None), (7.074,
    None), (8.085, None), (8.388, None), (10.135, None), (11.0, None))
Z_PLAN = ((5.932, 8), (6.444, 11), (6.863, 10), (7.332, 11), (7.694, 11), (8.079, 11), (8.4, 12), (8.943, 13),
    (9.166, 12), (9.416, 12), (9.929, 14), (10.45, 15), (10.993, 14), (11.285, 16), (11.385, 15), (11.931,
    16))
PRO_LN1_PLAN = ((None, None),) * 16
PRO_K_PLAN = _spread(8, 0, 6)
PRO_V_PLANS = (((0.0, None), (1.711, None), (3.429, None), (5.143, None), (6.857, None), (8.571, None),
    (10.353, None), (11.911, None)), ((13.0, None), (13.6, None), (14.2, None), (14.8, None), (15.353, None),
    (16.0, None), (16.6, None), (17.2, None)), ((17.8, None), (18.4, None), (18.995, None), (19.6, None),
    (20.2, None), (20.816, None), (21.4, None), (22.0, None)), ((1.172, 5), (2.903, 7), (4.64, 8), (6.303,
    10), (8.004, 12), (9.8, 13), (11.52, 15), (13.313, 17), (14.96, 18), (16.68, 20), (18.4, 22), (20.186,
    24), (21.84, 25), (23.56, 27), (25.28, 30), (27.0, 30)))
LN2B_PLAN = ((None, 103), (-0.172, 6), (1.72, 8), (3.011, 10), (4.803, 11), (6.449, 13), (8.447, 14), (9.869,
    15))
LN2A_PLAN = ((None, 18), (15.206, 20), (16.084, 21), (16.863, 20), (17.831, 21), (18.483, 22), (19.126, 23),
    (20.085, None))
PACK_PLAN = ((99.7, None), (100.798, None), (101.613, None), (102.786, None), (103.706, None), (104.725,
    None), (105.714, None), (106.7, None), (107.7, None), (108.339, None), (109.925, None), (110.738, None),
    (111.796, None), (112.962, None), (113.7, None), (114.508, None), (99.1, None), (100.1, None), (101.258,
    None), (102.336, None), (103.155, None), (104.1, None), (105.1, None), (106.1, None), (107.1, None),
    (108.1, None), (109.389, None), (109.994, None), (111.1, None), (112.1, None), (113.098, None), (114.122,
    None), (0.5, None), (1.579, None), (2.673, None), (3.737, None), (4.775, None), (5.848, None), (7.115,
    None), (8.023, None), (9.137, None), (10.211, None), (11.095, None), (12.59, None), (13.441, None),
    (14.526, None), (15.453, None), (16.605, None), (17.732, None), (18.842, None), (19.921, None), (20.995,
    None))
G_STEPS = (107, 107, 110, 111, 115, 115, 3, 3)
MOE_NA = 36
MOE_ND = 2
MOE_LAGS = (3, 3)
STAGGER = 8

NN = (((1,), (0,)), ((), ()))
NT = (((1,), (1,)), ((), ()))


def _dot(a, b, dims):
    return lax.dot_general(a, b, dims, preferred_element_type=F32)


def _recip(x):
    return pl.reciprocal(x, approx=False, full_range=False)


def _pack(x):
    return pltpu.bitcast(x, U32)


def _unpack(x):
    return pltpu.bitcast(x, BF16)


def _pair_allreduce(a, op):
    a = op(a, pltpu.roll(a, 2, 0))
    return op(a, pltpu.roll(a, 4, 0))


def _tree(op, xs):
    xs = list(xs)
    while len(xs) > 1:
        nxt = [op(xs[i], xs[i + 1]) for i in range(0, len(xs) - 1, 2)]
        if len(xs) % 2:
            nxt.append(xs[-1])
        xs = nxt
    return xs[0]


def _pair_logits(sl, j):
    sub = lax.broadcasted_iota(jnp.int32, sl[0].shape, 0)
    if j < 3:
        head = jnp.where(sub < 2, 0.0, sl[(0, 1, 16)[j]])
    else:
        head = jnp.where(sub < 2, sl[0], jnp.where(sub < 4, pltpu.roll(sl[1], 2, 0),
                                                   jnp.where(sub < 6, pltpu.roll(sl[16], 4, 0), 0.0)))
    r0 = (2, 9, 17, 24)[j]
    return [head] + list(sl[r0:r0 + 7])


def _dual_exp(sl):
    mx = _pair_allreduce(_tree(jnp.maximum, sl), jnp.maximum)
    mn = _pair_allreduce(_tree(jnp.minimum, sl), jnp.minimum)
    ep = [jnp.exp2(s - mx) for s in sl]
    en = [jnp.exp2(mn - s) for s in sl]
    sp = _pair_allreduce(_tree(jnp.add, ep), jnp.add)
    sn = _pair_allreduce(_tree(jnp.add, en), jnp.add)
    return ep, en, sp, sn


def _after(x, never, anchor):
    if anchor is None:
        return x
    d = jnp.concatenate([anchor] * (x.shape[0] // 8), axis=0)
    if x.shape[1] == 128:
        return jnp.where(never, d, x)
    return jnp.concatenate([jnp.where(never, d, x[:, :128]), x[:, 128:]], axis=1)


def _gate(x, never, deps):
    for i, dep in enumerate(deps):
        d = jnp.broadcast_to(dep, (8, 128))
        if x.dtype != F32:
            d = pltpu.bitcast(d, x.dtype)
        blk = jnp.where(never, d, x[8 * i:8 * i + 8, :128])
        if x.shape[1] > 128:
            blk = jnp.concatenate([blk, x[8 * i:8 * i + 8, 128:]], axis=1)
        parts = ([x[:8 * i, :]] if i else []) + [blk, x[8 * i + 8:, :]]
        x = jnp.concatenate(parts, axis=0)
    return x


def _lane_fold(a):
    return _tree(jnp.add, [a[:, 128 * i:128 * i + 128] for i in range(a.shape[1] // 128)])


def _row_sum(a):
    return jnp.sum(_lane_fold(a), axis=-1, keepdims=True)


def _lane_tile(a, n):
    return a if n == 1 else jnp.concatenate([a] * n, axis=1)


def _sublane_allreduce(a):
    a = a + pltpu.roll(a, 4, 0)
    a = a + pltpu.roll(a, 2, 0)
    return a + pltpu.roll(a, 1, 0)


def _col_broadcast(row8):
    return jnp.concatenate([row8] * 16, axis=0).astype(BF16).T.astype(F32)


def _vpu_matvec(xb, w_rows, never, anchors, lag):
    ng = xb.shape[0] // 8
    acc, hist = None, []
    for g in range(ng):
        dep = anchors[(g * len(anchors)) // ng]
        if g >= lag:
            dep = dep + hist[g - lag]
        x = jnp.where(never, dep, xb[8 * g:8 * g + 8, :])
        w = w_rows(g)
        t = w * _lane_tile(x, w.shape[1] // 128)
        acc = t if acc is None else acc + t
        c = 128 * (g % (w.shape[1] // 128))
        hist.append(acc[:, c:c + 128])
    return acc


class _Side:
    def __init__(self, never):
        self.never = never
        self.jobs = []
        self.deps = {}
        self.hooks = {}

    def add(self, plan, fn):
        for k, (rel, due) in enumerate(plan):
            if rel is None:
                self._run(due, fn, k, None)
            else:
                self.jobs.append((rel, due, fn, k))

    def _run(self, due, fn, k, anchor):
        dep = fn(k, anchor)
        if due is not None:
            self.deps.setdefault(due, []).append(dep)

    def check(self):
        assert not self.jobs and not self.deps and not self.hooks

    def gate(self, step, x):
        return _gate(x, self.never, self.deps.pop(step, []))

    def done(self, step, res):
        m = res.shape[0] // 8
        for job in sorted([j for j in self.jobs if step - 1 < j[0] <= step], key=lambda j: j[0]):
            self.jobs.remove(job)
            g = m - 1 - int((step - job[0]) * m)
            self._run(job[1], job[2], job[3], res[8 * g:8 * g + 8, res.shape[1] - 128:])
        for fn in self.hooks.pop(step, []):
            fn()


def _kernel(x_hbm, wqkv_hbm, wphi_hbm, wo_hbm, wr_hbm, wg_hbm, wu_hbm, wd_hbm, out_hbm,
            x_v, xn_v, lead_v, wraw_v, wt_v, wphi_v, a_v, woraw_v, wo_v, wrraw_v, wr_v, kvacc_v, kvbf_v,
            z_v, zb_v, phi_v, ha_v, hb_v, hn_v, o_v, wg_v, wu_v, wd_v, wgp_v, wup_v, wdp_v, patch_v,
            sem):
    SX, SW, SO, SM = 0, 6, 6 + 3 * NC, 6 + 3 * NC + NT_ + 1

    def x_copy(i):
        h0, h1 = ((1, 2), (2, 4), (4, 6), (6, 10), (10, 2 * NT_), (0, 1))[i]
        rows = pl.ds(h0 * TH, (h1 - h0) * TH)
        return pltpu.make_async_copy(x_hbm.at[rows, :], x_v.at[rows, :], sem.at[SX + i])

    def k0_copy(s):
        return pltpu.make_async_copy(wqkv_hbm.at[:, pl.ds(D + s * 128, 128)],
                                     wraw_v.at[NC, :, pl.ds(s * 128, 128)], sem.at[(SM + 7, SW + NC)[s]])

    def w_copy(j, c):
        return pltpu.make_async_copy(wqkv_hbm.at[:, pl.ds(j * D + c * RC, RC)], wraw_v.at[j * NC + c],
                                     sem.at[SW + j * NC + c])

    def wphi_copy(i):
        h0, h1 = ((0, 8), (8, 16), (16, H))[i]
        return pltpu.make_async_copy(wphi_hbm.at[pl.ds(h0, h1 - h0)], wphi_v.at[pl.ds(h0, h1 - h0)],
                                     sem.at[(SM + 4, SM + 8, SM + 9)[i]])

    wr_copy = pltpu.make_async_copy(wr_hbm, wrraw_v, sem.at[SM + 5])
    wo_copy = pltpu.make_async_copy(wo_hbm, woraw_v, sem.at[SM + 6])
    wg_copy = pltpu.make_async_copy(wg_hbm, wg_v.at[:, pl.ds(0, FF)], sem.at[SM + 0])
    wu_copy = pltpu.make_async_copy(wu_hbm, wu_v.at[:, pl.ds(0, FF)], sem.at[SM + 1])
    wd_copy = pltpu.make_async_copy(wd_hbm, wd_v, sem.at[SM + 2])

    wphi_copy(0).start()
    k0_copy(0).start()
    x_copy(5).start()
    k0_copy(1).start()
    x_copy(0).start()
    wphi_copy(1).start()
    w_copy(1, 1).start()

    def view(ref, i, n, off=0):
        r0 = off + i * n
        return ref.at[pl.ds(r0 if isinstance(r0, int) else pl.multiple_of(r0, math.gcd(n, off)), n), :]

    def ln_rows(t, k, n, never=None, anchor=None):
        x = _after(view(x_v, t, T)[k * n:(k + 1) * n, :].astype(F32), never, anchor)
        xc = x - _row_sum(x) * (1.0 / D)
        rstd = lax.rsqrt(_row_sum(xc * xc) * (1.0 / D) + LN_EPS)
        view(xn_v, t, T // 2)[k * n // 2:(k + 1) * n // 2, :] = _pack((xc * rstd).astype(BF16))
        return _tree(jnp.add, [rstd[8 * i:8 * i + 8, :] for i in range(min(n, LNC) // 8)])

    def xn_tile(t):
        return _unpack(view(xn_v, t, T // 2)[...])

    def expand_wphi(c):
        w = wphi_v[8 * c:8 * c + 8].reshape(8 * DH, DH).astype(F32).T
        bits = pltpu.bitcast(w, U32)
        head = lax.broadcasted_iota(jnp.int32, (DH, 128), 1) >> 5
        for s in range(2):
            b = bits[:, 128 * s:128 * s + 128]
            for j in range(2):
                r0 = 64 * (2 * c + s) + 32 * j
                a_v[r0:r0 + 32, :] = jnp.where(head == 2 * j, b >> 16,
                                               jnp.where(head == 2 * j + 1, b, jnp.uint32(0)))

    wphi_copy(0).wait()
    expand_wphi(0)
    hb_v[...] = jnp.zeros((TH, D), F32)

    def fold_v(c):
        for s in range(RC // 128):
            g0 = 64 * (2 * c + s)
            wt_v[2][g0:g0 + 64, :] = _pack(wraw_v[2 * NC + c, :, s * 128:(s + 1) * 128].T)

    def fold_pairs(j, c, s, side=None, step0=None):
        g0 = 64 * (2 * c + s)
        g0 = g0 if isinstance(g0, int) else pl.multiple_of(g0, 64)
        res = _dot(_unpack(a_v[pl.ds(g0, 64), :]), wraw_v[j * NC + c, :, s * 128:(s + 1) * 128], NT)
        if side is not None:
            side.done(step0 + 2 * s, res[:, :D // 2])
            side.done(step0 + 2 * s + 1, res[:, D // 2:])
        sub = lax.broadcasted_iota(jnp.int32, (8, D), 0)
        out = []
        for q in range(2):
            base = _pair_allreduce(jnp.where(sub < 2, res[64 * q:64 * q + 8, :], 0.0), jnp.add)
            out.append([(res[64 * q + 8 * i:64 * q + 8 * i + 8, :] - base) * LOG2E for i in range(8)])
        return out

    def share(z, z3, k):
        sub = lax.broadcasted_iota(jnp.int32, (8, D), 0)
        return jnp.where(sub < 2, pltpu.roll(z3, 8 - 2 * k, 0), z)

    def packed(slabs):
        return _pack(jnp.concatenate(slabs, axis=0).astype(BF16))

    def fold(j, c, side=None, step0=None):
        p0, p1 = fold_pairs(j, c, 0, side, step0)
        p2, p3 = fold_pairs(j, c, 1, side, step0)
        sl = ([share(p0[0], p3[0], 1), share(p1[0], p3[0], 2)] + p0[1:] + p1[1:]
              + [share(p2[0], p3[0], 3)] + p2[1:] + p3[1:])
        zero = jnp.zeros((8, D), F32)
        even, odd = sl + [zero], [zero] + sl
        r0 = 8 * ((31 * c) // 2)
        if isinstance(c, int):
            is_odd = c % 2 == 1
            sl = odd if is_odd else even
        else:
            is_odd = c % 2 == 1
            r0 = pl.multiple_of(r0, 8)
            sl = [jnp.where(is_odd, o, e) for o, e in zip(odd, even)]
        win = wt_v[j].at[pl.ds(r0, 128), :]
        win[8:128, :] = packed(sl[2:])
        first = packed(sl[:2])
        if is_odd is not False:
            keep = lax.broadcasted_iota(jnp.int32, (8, D), 0) < jnp.where(is_odd, 4, 0)
            first = jnp.where(keep, win[0:8, :], first)
        win[0:8, :] = first

    def k_pair(p, slot, pr, c0, first, never=None):
        ep, en, sp, sn = _dual_exp(p)
        inv = _recip(sp * sn)
        scale = (sn * inv, sp * inv)
        es = ep + en
        cols = slice(c0, c0 + p[0].shape[1])
        n = 16 if never is None else 16 // STAGGER
        last = None
        for q in range(16 // n):
            sc = scale
            if last is not None:
                sc = [jnp.where(never, last, x) for x in scale]
            phi = jnp.concatenate([es[i] * sc[i // 8] for i in range(q * n, (q + 1) * n)], axis=0)
            rows = slice(8 * q * n, 8 * (q + 1) * n)
            z = phi if first else z_v[pr, rows, cols] + phi
            z_v[pr, rows, cols] = z
            phi_v[slot][64 * pr + 4 * q * n:64 * pr + 4 * (q + 1) * n, cols] = _pack(phi.astype(BF16))
            last = z[8 * n - 8:, :]

    def k_features(pk, slot, c, first, never=None):
        for j in range(PPC):
            k_pair(_pair_logits(pk, j), slot, c * PPC + j, 0, first, never)

    def kv_update(vt, slot, c, first, publish=False):
        for j in range(PPC):
            pr = c * PPC + j
            upd = _dot(vt[64 * j:64 * j + 64, :].astype(BF16), _unpack(phi_v[slot][64 * pr:64 * pr + 64, :]), NT)
            acc = upd if first else kvacc_v[pr] + upd
            kvacc_v[pr] = acc
            if publish:
                odd = -(lax.broadcasted_iota(jnp.int32, (32, 128), 1) & 1)
                bits = pltpu.bitcast(acc, jnp.int32) & jnp.concatenate([~odd, odd], axis=0)
                kvbf_v[32 * pr:32 * pr + 32, :] = _pack(pltpu.bitcast(bits, F32).astype(BF16))

    def save_lead(e, t):
        corner = _unpack(view(xn_v, t, T // 2)[0:TH // 2, 0:D // 2])
        view(lead_v, e, D // 4)[...] = _pack(corner.T)

    def proj_steps(side, step0, w, xn, lead=None):
        quarters = []
        for n in range(2):
            for m in range(2):
                step = step0 + 2 * n + m
                wq = _unpack(side.gate(step, w[:64, :] if m == 0 else w[64:, :]))
                if lead is not None and n + m == 0:
                    res = _dot(wq[:, :D // 2], _unpack(view(lead_v, lead, D // 4)[...]), NN)
                    res = _dot(wq[:, D // 2:], xn[0:TH, D // 2:], NT) + res
                else:
                    res = _dot(wq, xn[n * TH:(n + 1) * TH, :], NT)
                side.done(step, res)
                quarters.append(res)
        return jnp.concatenate(
            [jnp.concatenate([quarters[0], quarters[2]], axis=1),
             jnp.concatenate([quarters[1], quarters[3]], axis=1)], axis=0)

    def proj_v(side, step0, c, xn):
        return proj_steps(side, step0, wt_v[2][128 * c:128 * c + 128, :], xn)

    def proj_feat(side, step0, j, c, xn, carry, lead=None):
        r0 = 8 * ((31 * c) // 2)
        skip = 8 if c % 2 == 1 and carry is not None else 0
        res = proj_steps(side, step0, wt_v[j][r0 + skip:r0 + 128, :], xn, lead)
        sl = [res[8 * i:8 * i + 8, :] for i in range(res.shape[0] // 8)]
        if c % 2 == 0:
            return sl[:31], sl[31]
        return ([carry] + sl if skip else sl[1:]), None

    def pack_rows(src, dst, r0, rows, c0, cols, never, a):
        w = src[r0:r0 + rows, c0:c0 + cols].astype(F32)
        d = _lane_tile(a, cols // 128)
        w = jnp.concatenate([jnp.where(never, d, w[8 * i:8 * i + 8, :]) if i % 2 == 0 else w[8 * i:8 * i + 8, :]
                             for i in range(rows // 8)], axis=0)
        dst[r0 // 2:(r0 + rows) // 2, c0:c0 + cols] = _pack(w.astype(BF16))

    def stash_at(i, k, n):
        return zb_v.at[4 * i + 2 * (k // 16) + n, pl.ds(8 * (k % 16), 8), :]

    def stash(i, sl):
        for k, v in enumerate(sl):
            for n in range(2):
                stash_at(i, k, n)[...] = v[:, 128 * n:128 * n + 128]

    def stashed_k(i, slot, c, first):
        def job(k, a):
            j, n = k // 2, k % 2
            p = _pair_logits([stash_at(i, q, n)[...] for q in range(31)], j)
            k_pair([_after(p[0], never0, a)] + p[1:], slot, c * PPC + j, 128 * n, first, never0)
        return job

    def first_rows(k0, k1, n):
        xn = _unpack(xn_v[n * TH // 2:(n + 1) * TH // 2, :])
        ks = [k for k in range(k0, k1)]
        w = jnp.concatenate([wt_v[1][4 * (k % 32):4 * (k % 32) + 8, :] for k in ks[::2]], axis=0)
        res = _dot(_unpack(w), xn, NT)
        for q, k in enumerate(ks):
            if k % 32 < 31:
                stash_at(0, k % 32, n)[...] = res[8 * q:8 * q + 8, :]

    k0_copy(0).wait()
    x_copy(5).wait()
    wphi_copy(2).start()
    w_copy(1, 2).start()
    x_copy(1).start()
    p0, p1 = fold_pairs(1, 0, 0)
    wt_v[1][8:64, :] = packed(p0[1:] + p1[1:])
    ha_v[0:8, :] = p0[0]
    ha_v[8:16, :] = p1[0]
    never0 = ln_rows(0, 0, TH)[0, 0] < 0.0
    first_rows(2, 16, 0)

    k0_copy(1).wait()
    x_copy(0).wait()
    wphi_copy(1).wait()
    w_copy(1, 3).start()
    for c in range(NC):
        w_copy(2, c).start()
    p2, p3 = fold_pairs(1, 0, 1)
    wt_v[1][0:8, :] = packed([share(ha_v[0:8, :], p3[0], 1), share(ha_v[8:16, :], p3[0], 2)])
    wt_v[1][64:128, :] = packed([share(p2[0], p3[0], 3)] + p2[1:] + p3[1:] + [jnp.zeros((8, D), F32)])
    ln_rows(0, 1, TH)
    first_rows(16, 34, 0)
    first_rows(0, 16, 1)
    first_rows(16, 32, 1)
    expand_wphi(1)

    for c in (1, 2):
        w_copy(1, c).wait()
        if c == 1:
            wphi_copy(2).wait()
            expand_wphi(2)
            expand_wphi(3)
            x_copy(2).start()
            w_copy(0, 0).start()
        side = _Side(never0)
        side.add(PRO_K_PLAN, stashed_k(c - 1, 0, c - 1, True))
        fold(1, c, side, 0)
        stash(c, proj_feat(side, 4, 1, c, xn_tile(0), None)[0])
        side.check()

    x_copy(1).wait()
    w_copy(1, 3).wait()
    side = _Side(never0)
    side.add(PRO_LN1_PLAN, lambda k, a: ln_rows(1, k, LNC, never0, a))
    fold(1, 3, side, 0)
    stash(3, proj_feat(side, 4, 1, 3, xn_tile(0), None)[0])
    xn1 = xn_tile(1)
    spare = None
    for c in range(NC):
        pk, spare = proj_feat(_Side(None), 0, 1, c, xn1, spare)
        if c < 3:
            k_features(pk, 1, c, c == 2, never0)
        else:
            stash(0, pk)

    for c in range(NC):
        w_copy(2, c).wait()
    x_copy(2).wait()
    w_copy(0, 0).wait()
    w_copy(0, 1).start()
    x_copy(3).start()
    wo_copy.start()
    wr_copy.start()
    x_copy(4).start()
    w_copy(0, 2).start()
    w_copy(0, 3).start()
    wg_copy.start()
    wu_copy.start()
    wd_copy.start()
    side = _Side(never0)
    side.add(PRO_V_PLANS[0], stashed_k(2, 0, 2, False))
    side.add(PRO_V_PLANS[1], stashed_k(3, 0, 3, True))
    side.add(PRO_V_PLANS[2], stashed_k(0, 1, 3, False))
    side.add(PRO_V_PLANS[3], lambda k, a: ln_rows(2, k, LNC, never0, a))
    fold(0, 0)
    wt_v[0][248:256, :] = jnp.zeros((8, D), U32)
    xns = (xn_tile(0), xn_tile(1))
    pending = None
    for c in range(NC):
        fold_v(c)
        for i in range(2):
            vt = proj_v(side, 8 * c + 4 * i, c, xns[i])
            if pending is not None:
                kv_update(*pending)
            pending = (vt, i, c, i == 0)
    side.check()
    kv_update(*pending)
    save_lead(0, 0)
    save_lead(1, 2)

    def phase1(u, carry):
        never = u < 0

        @pl.when(u == 0)
        def _():
            w_copy(0, 1).wait()
            x_copy(3).wait()
            wo_copy.wait()
            wr_copy.wait()

        @pl.when(u == 1)
        def _():
            x_copy(4).wait()
            w_copy(0, 2).wait()
            w_copy(0, 3).wait()

        pending = None
        for i in range(2):
            t = 2 * u + 2 + i
            tn = jnp.minimum(t + 1, NT_ - 1)
            side = _Side(never)
            xn = xn_tile(t)
            spare = None
            for c in range(NC):
                pk, spare = proj_feat(_Side(None), 0, 1, c, xn, spare, u + 1 if i + c == 0 else None)
                if c == 0 and pending is not None:
                    kv_update(*pending)
                k_features(pk, i, c, False)
            side.add(LN1_PLAN, lambda k, a: ln_rows(tn, k, LNC, never, a))
            if i == 0:
                def pack_wo(k, a):
                    rows = WO_ROWS // len(WO_PLAN)
                    w0 = u * ((D - WO_ROWS) // 2)
                    src = woraw_v.at[pl.ds(pl.multiple_of(w0, 16), WO_ROWS), :]
                    dst = wo_v.at[pl.ds(pl.multiple_of(w0 // 2, 8), WO_ROWS // 2), :]
                    pack_rows(src, dst, k * rows, rows, 0, D, never, a)
                side.add(WO_PLAN, pack_wo)
            else:
                def z_final(k, a):
                    z = _after(z_v[k], never, a)
                    zs = _row_sum(z)
                    zb_v[k] = jnp.broadcast_to(zs, (128, 128))
                    return zs[120:128, :]
                side.add(Z_PLAN, z_final)
            side.done(0, jnp.concatenate(pk[17:], axis=0))
            vts = []
            for c in range(NC):
                vts.append(proj_v(side, 4 * c + 1, c, xn))
                if c > 0:
                    kv_update(vts[c - 1], i, c - 1, False, i == 1)
            pending = (vts[NC - 1], i, NC - 1, False, i == 1)
            side.check()
        fold(0, u + 1)
        kv_update(*pending)
        save_lead(u + 2, tn)
        wr_v[...] = jnp.broadcast_to(wrraw_v[...].reshape(1, D).astype(F32), (8, D))
        return carry

    lax.fori_loop(0, (NT_ - 2) // 2, phase1, 0)

    def o_copy(r0, n, i):
        return pltpu.make_async_copy(o_v.at[pl.ds(r0, n), :], out_hbm.at[pl.ds(r0, n), :], sem.at[SO + i])

    def finish_rows(h_ref, k, ht, valid, st, never=None, anchor=None):
        r0 = ht * TH + k * LNC
        best, besti = st["route"]
        wr = jnp.concatenate([wr_v[...]] * (LNC // 8), axis=0)
        sub = lax.broadcasted_iota(jnp.int32, (8, 1), 0)
        h = _after(h_ref[k * LNC:(k + 1) * LNC, :], never, anchor)
        hc = h - _row_sum(h) * (1.0 / D)
        rstd = lax.rsqrt(_row_sum(hc * hc) * (1.0 / D) + LN_EPS)
        r = (_row_sum(hc * wr) * rstd).astype(BF16).astype(F32)
        hn = hc * rstd
        view(hn_v, ht, TH // 2)[k * LNC // 2:(k + 1) * LNC // 2, :] = _pack(hn.astype(BF16))
        view(o_v, ht, TH)[k * LNC:(k + 1) * LNC, :] = (hn + h).astype(BF16)
        if valid is not None:
            r = jnp.where(valid, r, -jnp.inf)
        for i in range(LNC // 8):
            ri = r[8 * i:8 * i + 8, :]
            better = ri > best
            best = jnp.where(better, ri, best)
            besti = jnp.where(better, sub + (r0 + 8 * i), besti)
        st["route"] = (best, besti)
        return best

    def q_features(pq, slot, c):
        for j in range(PPC):
            pr = c * PPC + j
            ep, en, sp, sn = _dual_exp(_pair_logits(pq, j))
            zz = [_lane_tile(zb_v[pr, 8 * i:8 * i + 8, :], T // 128) for i in range(16)]
            ap = _pair_allreduce(_tree(jnp.add, [ep[i] * zz[i] for i in range(8)]), jnp.add)
            an = _pair_allreduce(_tree(jnp.add, [en[i] * zz[8 + i] for i in range(8)]), jnp.add)
            inv = _recip(ap * sn + (an + 1e-6 * sn) * sp)
            rp = sn * inv
            rn = sp * inv
            phi = jnp.concatenate([e * rp for e in ep] + [e * rn for e in en], axis=0)
            phi_v[slot][64 * pr:64 * pr + 64, :] = _pack(phi.astype(BF16))

    def attn_rows(slot, g):
        res = jnp.concatenate(
            [_dot(_unpack(kvbf_v[32 * pr:32 * pr + 32, :]), _unpack(phi_v[slot][64 * pr:64 * pr + 64, :]), NN)
             for pr in (2 * g, 2 * g + 1)], axis=0)
        return res.astype(BF16).T

    def out_proj(side, step0, o, k0, k1):
        cols = []
        for n in range(D // 128):
            w = side.gate(step0 + n, wo_v[k0 // 2:k1 // 2, n * 128:(n + 1) * 128])
            res = _dot(o, _unpack(w), NN)
            side.done(step0 + n, res)
            cols.append(res)
        return jnp.concatenate(cols, axis=1)

    def phase2(u, carry):
        for i in range(2):
            carry = phase2_tile(u * 2 + i, i % 2, carry, u < 0, u if i == 0 else None)

        r0 = pl.multiple_of(u * (2 * T), T)

        @pl.when(u == 0)
        def _():
            o_copy(0, 2 * T - TH, 0).start()

        @pl.when(u > 0)
        def _():
            o_copy(pl.multiple_of(jnp.maximum(r0 - TH, 0), TH), 2 * T, u).start()

        return carry

    def phase2_tile(t, slot, carry, never, lead):
        hp = jnp.maximum(2 * t - 1, 0)
        side = _Side(never)
        st = {"route": carry}
        side.add(LN2B_PLAN, lambda k, a: finish_rows(hb_v, k, hp, t > 0, st, side.never, a))

        def pack_ffn(k, a):
            if k < 32:
                n = D // NT_
                pack_rows(view((wg_v, wu_v)[k % 2], t, n), view((wgp_v, wup_v)[k % 2], t, n // 2),
                          (k // 4) * 16, 16, (0, D)[k // 2 % 2], (D, FM - D)[k // 2 % 2], never, a)
            else:
                n = (FF - FVD) // NT_
                pack_rows(view(wd_v, t, n, FVD), view(wdp_v, t, n // 2), (k - 32) * 16, 16, 0, D, never, a)
        side.add(PACK_PLAN[:32 + (FF - FVD) // 128], pack_ffn)

        xn = xn_tile(t)
        xt = view(x_v, t, T)
        os_ = {}
        for g in range(8):
            side.hooks.setdefault(G_STEPS[g], []).append(lambda g=g: os_.update({g: attn_rows(slot, g)}))
        spare = None
        for c in range(NC):
            pq, spare = proj_feat(side, 100 + 4 * c, 0, c, xn, spare, lead if c == 0 else None)
            if c == 0:
                head = side.gate(0, jnp.concatenate(pq[2:9], axis=0))
                pq = pq[:2] + [head[8 * i:8 * i + 8, :] for i in range(7)] + pq[9:]
            q_features(pq, slot, c)
        ha = out_proj(side, 0, jnp.concatenate([os_[g][0:TH, :] for g in range(4)], axis=1), 0, D // 2)
        ha = ha + xt[0:TH, :].astype(F32)
        ha_v[...] = ha + out_proj(side, 8, jnp.concatenate([os_[g][0:TH, :] for g in range(4, 8)], axis=1), D // 2, D)
        side.add(LN2A_PLAN, lambda k, a: finish_rows(ha_v, k, 2 * t, None, st, side.never, a))
        ob = jnp.concatenate([os_[g][TH:T, :] for g in range(8)], axis=1)
        hb_v[...] = xt[TH:T, :].astype(F32) + out_proj(side, 16, ob, 0, D)
        side.check()
        return st["route"]

    wg_copy.wait()
    wu_copy.wait()
    wd_copy.wait()
    route = lax.fori_loop(
        0, NT_ // 2, phase2,
        (jnp.full((8, 1), -jnp.inf, F32), jnp.zeros((8, 1), jnp.int32)))
    st = {"route": route}
    for k in range(TH // LNC):
        finish_rows(hb_v, k, 2 * NT_ - 1, None, st)
    best, besti = st["route"]
    o_copy(S - TH, TH, NT_).start()

    rmax = jnp.max(best, axis=0, keepdims=True)
    idx = jnp.min(jnp.where(best == rmax, besti, S), axis=0, keepdims=True)
    idx_s = jnp.clip(idx[0, 0], 0, S - 1)
    blk = pl.multiple_of((idx_s >> 4) << 4, 16)
    pair = jnp.broadcast_to(hn_v[pl.ds(idx_s >> 1, 1), :], (8, D))
    x8 = pltpu.bitcast(jnp.where((idx_s & 1) == 1, pair & jnp.uint32(0xFFFF0000), pair << 16), F32)
    xs = jnp.concatenate([x8, x8], axis=0).astype(BF16)
    acts, anchors = [], []

    def park(v, half):
        n = v.shape[0] // 128
        for i in range(n):
            z_v[i, :, 128 * half:128 * half + 128] = v[128 * i:128 * i + 128, :]
        return jnp.concatenate([z_v[i, :, 128 * half:128 * half + 128] for i in range(n)], axis=0)

    for c0 in range(0, FM, 128):
        g = _dot(xs, _unpack(wgp_v[:, c0:c0 + 128]), NN)[0:8, :]
        u = _dot(xs, _unpack(wup_v[:, c0:c0 + 128]), NN)[0:8, :]
        anchors += [g, u]
        acts.append(g * jax.nn.sigmoid(g) * u)
    xb = park(_col_broadcast(x8), 0)
    g, u = [_sublane_allreduce(_vpu_matvec(
        xb, lambda g: w[8 * g:8 * g + 8, FM:FF].astype(F32), never0,
        anchors[i * MOE_NA // 2:(i + 1) * MOE_NA // 2], MOE_LAGS[0])) for i, w in enumerate((wg_v, wu_v))]
    acts.append(g * jax.nn.sigmoid(g) * u)
    a = jnp.concatenate(acts, axis=1)
    am = jnp.concatenate([a[:, FVD:], a[:, FVD:]], axis=0).astype(BF16)
    ys, anchors = [], anchors[MOE_NA:]
    for k0 in range(0, FF - FVD, 512):
        k1 = min(k0 + 512, FF - FVD)
        yk = _dot(am[:, k0:k1], _unpack(wdp_v[k0 // 2:k1 // 2, :]), NN)[0:8, :]
        ys.append(yk)
        anchors += [yk[:, c:c + 128] for c in range(128, D, 256)]
    ys.append(_sublane_allreduce(_vpu_matvec(
        park(_col_broadcast(a[:, :FVD]), 1), lambda g: wd_v[8 * g:8 * g + 8, :].astype(F32), never0,
        anchors[:-MOE_ND], MOE_LAGS[1])))
    y = _tree(jnp.add, ys) * jax.nn.sigmoid(rmax)
    y = jnp.concatenate([y, y], axis=0)
    sel = lax.broadcasted_iota(jnp.int32, (16, 1), 0) == (idx_s - blk)
    patch_v[...] = (o_v[pl.ds(blk, 16), :].astype(F32) + jnp.where(sel, y, 0.0)).astype(BF16)
    o_copy(0, 2 * T - TH, 0).wait()
    for u in range(1, NT_ // 2):
        o_copy(u * 2 * T - TH, 2 * T, u).wait()
    o_copy(S - TH, TH, NT_).wait()
    pc = pltpu.make_async_copy(patch_v, out_hbm.at[pl.ds(blk, 16), :], sem.at[SM + 3])
    pc.start()
    pc.wait()


@jax.jit
def pallas_sequential_preLN__linear_kernel_hedgehog__moe_arch_mod__prompt_kernel(
    A_x: jax.Array,
    A_wqkv: jax.Array,
    A_w_phi: jax.Array,
    A_wo: jax.Array,
    B_x: jax.Array,
    B_w_r: jax.Array,
    B_w_gate: jax.Array,
    B_w_up: jax.Array,
    B_w_down: jax.Array,
):
    del B_x
    hbm = pl.BlockSpec(memory_space=pl.ANY)
    out = pl.pallas_call(
        _kernel,
        out_shape=jax.ShapeDtypeStruct((S, D), BF16),
        in_specs=[hbm] * 8,
        out_specs=hbm,
        scratch_shapes=[
            pltpu.VMEM((S, D), BF16),
            pltpu.VMEM((S // 2, D), U32),
            pltpu.VMEM((5 * D // 4, 128), U32),
            pltpu.VMEM((3 * NC, D, RC), BF16),
            [pltpu.VMEM((D // 2, D), U32)] * 3,
            pltpu.VMEM((H, DH, DH), BF16),
            pltpu.VMEM((8 * 64, 128), U32),
            pltpu.VMEM((D, D), BF16),
            pltpu.VMEM((D // 2, D), U32),
            pltpu.VMEM((D,), BF16),
            pltpu.VMEM((8, D), F32),
            pltpu.VMEM((NPAIR, 64, 128), F32),
            pltpu.VMEM((NPAIR * 32, 128), U32),
            pltpu.VMEM((NPAIR, 128, T), F32),
            pltpu.VMEM((NPAIR, 128, 128), F32),
            [pltpu.VMEM((NPAIR * 64, T), U32)] * 2,
            pltpu.VMEM((TH, D), F32),
            pltpu.VMEM((TH, D), F32),
            pltpu.VMEM((S // 2, D), U32),
            pltpu.VMEM((S, D), BF16),
            pltpu.VMEM((D, FFP), BF16),
            pltpu.VMEM((D, FFP), BF16),
            pltpu.VMEM((FF, D), BF16),
            pltpu.VMEM((D // 2, FM), U32),
            pltpu.VMEM((D // 2, FM), U32),
            pltpu.VMEM(((FF - FVD) // 2, D), U32),
            pltpu.VMEM((16, D), BF16),
            pltpu.SemaphoreType.DMA((6 + 3 * NC + NT_ + 11,)),
        ],
        compiler_params=pltpu.CompilerParams(vmem_limit_bytes=100 * 1024 * 1024,
                                             disable_semaphore_checks=True, disable_bounds_checks=True),
        name="hedgehog_mod",
    )(
        A_x.reshape(S, D),
        A_wqkv,
        A_w_phi,
        A_wo,
        B_w_r,
        B_w_gate,
        B_w_up,
        B_w_down,
    )
    return out.reshape(1, S, D)
```

```python
import math

import jax
import jax.numpy as jnp
from jax import lax
import jax.experimental.pallas as pl
import jax.experimental.pallas.tpu as pltpu

F32 = jnp.float32
BF16 = jnp.bfloat16
U32 = jnp.uint32

S = 2048
D = 1024
H = 32
DH = 32
FF = 3584
NPAIR = H // 2
LOG2E = 1.4426950408889634
LN_EPS = 1e-5

T = 256
TH = T // 2
NT_ = S // T
RC = 256
NC = D // RC
PPC = RC // 64
LNC = 16

FV = 10 * 128
FM = FF - FV
FVD = 8 * 128
NQ = NT_ // 2
DQ = (FF - FVD) // NQ
WO_ROWS = 352


def _spread(n, a, b, due=None):
    rel = [round(a + (b - a) * k / (n - 1), 3) for k in range(n)]
    return tuple((r, None if due is None else math.ceil(r) + due) for r in rel)


LN1_PLAN = ((-0.001, 4), (0.787, 5), (1.823, 5), (2.494, 6), (3.413, 7), (4.33, 9), (5.163, 9), (6.264, 10),
    (6.755, 10), (7.681, 11), (8.866, 13), (9.289, 14), (10.598, 14), (11.083, 15), (12.313, 16), (13.022,
    16))
WO_PLAN = ((0.92, None), (1.762, None), (4.0, None), (4.445, None), (5.249, None), (5.684, None), (7.074,
    None), (8.085, None), (8.388, None), (10.135, None), (11.0, None))
Z_PLAN = ((5.932, 8), (6.444, 11), (6.863, 10), (7.332, 11), (7.694, 11), (8.079, 11), (8.4, 12), (8.943, 13),
    (9.166, 12), (9.416, 12), (9.929, 14), (10.45, 15), (10.993, 14), (11.285, 16), (11.385, 15), (11.931,
    16))
PRO_LN1_PLAN = ((None, None),) * 16
PRO_K_PLAN = _spread(8, 0, 6)
PRO_V_PLANS = (((0.0, None), (1.711, None), (3.429, None), (5.143, None), (6.857, None), (8.571, None),
    (10.353, None), (11.911, None)), ((12.92, None), (13.449, None), (14.2, None), (14.8, None), (15.353,
    None), (16.13, None), (16.6, None), (17.2, None)), ((17.8, None), (18.4, None), (18.995, None), (19.6,
    None), (20.2, None), (20.816, None), (21.4, None), (22.0, None)), ((1.172, 6), (2.903, 7), (4.64, 8),
    (6.303, 10), (8.004, 12), (9.8, 14), (11.444, 15), (13.313, 17), (14.96, 18), (16.68, 20), (18.4, 21),
    (20.177, 24), (21.776, 25), (23.56, 27), (25.336, 30), (27.0, 30)))
LN2B_PLAN = ((None, 103), (-0.244, 6), (1.72, 8), (3.011, 10), (4.803, 11), (6.449, 13), (8.447, 14), (9.869,
    15))
LN2A_PLAN = ((None, 18), (15.225, 20), (16.131, 21), (16.922, 20), (17.831, 21), (18.483, 22), (19.126, 23),
    (20.085, None))
PACK_PLAN = ((99.7, None), (100.798, None), (101.654, None), (102.714, None), (103.706, None), (104.716,
    None), (105.714, None), (106.7, None), (107.7, None), (108.339, None), (109.925, None), (110.837, None),
    (111.796, None), (112.939, None), (113.7, None), (114.508, None), (99.1, None), (100.1, None), (101.258,
    None), (102.336, None), (103.155, None), (104.1, None), (105.1, None), (106.181, None), (107.1, None),
    (108.049, None), (109.317, None), (109.994, None), (111.1, None), (112.1, None), (113.098, None),
    (114.122, None))
PACKD_PLANS = (((0.5, None), (1.16, None), (2.019, None), (2.583, None), (3.537, None), (4.296, None), (5.056,
    None), (5.815, None), (6.574, None), (7.333, None), (8.093, None), (8.852, None), (9.611, None), (10.37,
    None), (11.13, None), (11.889, None), (12.648, None), (13.336, None), (14.167, None), (14.926, None),
    (15.667, None), (16.444, None), (17.267, None), (17.963, None), (18.722, None), (19.481, None), (20.192,
    None), (21.0, None)), ((0.5, None), (1.432, None), (2.227, None), (3.013, None), (3.955, None), (4.818,
    None), (5.682, None), (6.545, None), (7.409, None), (8.203, None), (9.121, None), (10.0, None)))
DQA = 16 * len(PACKD_PLANS[0])
G_STEPS = (107, 107, 110, 111, 115, 115, 3, 3)
MOE_NA = 36
MOE_ND = 2
MOE_LAGS = (3, 3)
STAGGER = 8

NN = (((1,), (0,)), ((), ()))
NT = (((1,), (1,)), ((), ()))


def _dot(a, b, dims):
    return lax.dot_general(a, b, dims, preferred_element_type=F32)


def _recip(x):
    return pl.reciprocal(x, approx=False, full_range=False)


def _pack(x):
    return pltpu.bitcast(x, U32)


def _unpack(x):
    return pltpu.bitcast(x, BF16)


def _pair_allreduce(a, op):
    a = op(a, pltpu.roll(a, 2, 0))
    return op(a, pltpu.roll(a, 4, 0))


def _tree(op, xs):
    xs = list(xs)
    while len(xs) > 1:
        nxt = [op(xs[i], xs[i + 1]) for i in range(0, len(xs) - 1, 2)]
        if len(xs) % 2:
            nxt.append(xs[-1])
        xs = nxt
    return xs[0]


def _pair_logits(sl, j):
    sub = lax.broadcasted_iota(jnp.int32, sl[0].shape, 0)
    if j < 3:
        head = jnp.where(sub < 2, 0.0, sl[(0, 1, 16)[j]])
    else:
        head = jnp.where(sub < 2, sl[0], jnp.where(sub < 4, pltpu.roll(sl[1], 2, 0),
                                                   jnp.where(sub < 6, pltpu.roll(sl[16], 4, 0), 0.0)))
    r0 = (2, 9, 17, 24)[j]
    return [head] + list(sl[r0:r0 + 7])


def _dual_exp(sl):
    mx = _pair_allreduce(_tree(jnp.maximum, sl), jnp.maximum)
    mn = _pair_allreduce(_tree(jnp.minimum, sl), jnp.minimum)
    ep = [jnp.exp2(s - mx) for s in sl]
    en = [jnp.exp2(mn - s) for s in sl]
    sp = _pair_allreduce(_tree(jnp.add, ep), jnp.add)
    sn = _pair_allreduce(_tree(jnp.add, en), jnp.add)
    return ep, en, sp, sn


def _after(x, never, anchor):
    if anchor is None:
        return x
    d = jnp.concatenate([anchor] * (x.shape[0] // 8), axis=0)
    if x.shape[1] == 128:
        return jnp.where(never, d, x)
    return jnp.concatenate([jnp.where(never, d, x[:, :128]), x[:, 128:]], axis=1)


def _gate(x, never, deps):
    for i, dep in enumerate(deps):
        d = jnp.broadcast_to(dep, (8, 128))
        if x.dtype != F32:
            d = pltpu.bitcast(d, x.dtype)
        blk = jnp.where(never, d, x[8 * i:8 * i + 8, :128])
        if x.shape[1] > 128:
            blk = jnp.concatenate([blk, x[8 * i:8 * i + 8, 128:]], axis=1)
        parts = ([x[:8 * i, :]] if i else []) + [blk, x[8 * i + 8:, :]]
        x = jnp.concatenate(parts, axis=0)
    return x


def _lane_fold(a):
    return _tree(jnp.add, [a[:, 128 * i:128 * i + 128] for i in range(a.shape[1] // 128)])


def _row_sum(a):
    return jnp.sum(_lane_fold(a), axis=-1, keepdims=True)


def _lane_tile(a, n):
    return a if n == 1 else jnp.concatenate([a] * n, axis=1)


def _sublane_allreduce(a):
    a = a + pltpu.roll(a, 4, 0)
    a = a + pltpu.roll(a, 2, 0)
    return a + pltpu.roll(a, 1, 0)


def _col_broadcast(row8):
    return jnp.concatenate([row8] * 16, axis=0).astype(BF16).T.astype(F32)


def _vpu_matvec(xb, w_rows, never, anchors, lag):
    ng = xb.shape[0] // 8
    acc, hist = None, []
    for g in range(ng):
        dep = anchors[(g * len(anchors)) // ng]
        if g >= lag:
            dep = dep + hist[g - lag]
        x = jnp.where(never, dep, xb[8 * g:8 * g + 8, :])
        w = w_rows(g)
        t = w * _lane_tile(x, w.shape[1] // 128)
        acc = t if acc is None else acc + t
        c = 128 * (g % (w.shape[1] // 128))
        hist.append(acc[:, c:c + 128])
    return acc


class _Side:
    def __init__(self, never):
        self.never = never
        self.jobs = []
        self.deps = {}
        self.hooks = {}

    def add(self, plan, fn):
        for k, (rel, due) in enumerate(plan):
            if rel is None:
                self._run(due, fn, k, None)
            else:
                self.jobs.append((rel, due, fn, k))

    def _run(self, due, fn, k, anchor):
        dep = fn(k, anchor)
        if due is not None:
            self.deps.setdefault(due, []).append(dep)

    def check(self):
        assert not self.jobs and not self.deps and not self.hooks

    def gate(self, step, x):
        return _gate(x, self.never, self.deps.pop(step, []))

    def done(self, step, res):
        m = res.shape[0] // 8
        for job in sorted([j for j in self.jobs if step - 1 < j[0] <= step], key=lambda j: j[0]):
            self.jobs.remove(job)
            g = m - 1 - int((step - job[0]) * m)
            self._run(job[1], job[2], job[3], res[8 * g:8 * g + 8, res.shape[1] - 128:])
        for fn in self.hooks.pop(step, []):
            fn()


def _kernel(x_hbm, wqkv_hbm, wphi_hbm, wo_hbm, wr_hbm, wg_hbm, wu_hbm, wd_hbm, out_hbm,
            x_v, xn_v, lead_v, wraw_v, wt_v, wphi_v, a_v, woraw_v, wo_v, wrraw_v, wr_v, kvacc_v, kvbf_v,
            z_v, zb_v, phi_v, ha_v, hb_v, hn_v, o_v, wg_v, wu_v, wd_v, stage_v, wgp_v, wup_v, wdp_v,
            patch_v,
            sem):
    SX, SW, SO, SM = 0, 6, 6 + 3 * NC, 6 + 3 * NC + NT_ + 1

    def x_copy(i):
        h0, h1 = ((1, 2), (2, 4), (4, 6), (6, 10), (10, 2 * NT_), (0, 1))[i]
        rows = pl.ds(h0 * TH, (h1 - h0) * TH)
        return pltpu.make_async_copy(x_hbm.at[rows, :], x_v.at[rows, :], sem.at[SX + i])

    def k0_copy(s):
        return pltpu.make_async_copy(wqkv_hbm.at[:, pl.ds(D + s * 128, 128)],
                                     wraw_v.at[NC, :, pl.ds(s * 128, 128)], sem.at[(SM + 7, SW + NC)[s]])

    def w_copy(j, c):
        return pltpu.make_async_copy(wqkv_hbm.at[:, pl.ds(j * D + c * RC, RC)], wraw_v.at[j * NC + c],
                                     sem.at[SW + j * NC + c])

    def wphi_copy(i):
        h0, h1 = ((0, 8), (8, 16), (16, H))[i]
        return pltpu.make_async_copy(wphi_hbm.at[pl.ds(h0, h1 - h0)], wphi_v.at[pl.ds(h0, h1 - h0)],
                                     sem.at[(SM + 4, SM + 8, SM + 9)[i]])

    wr_copy = pltpu.make_async_copy(wr_hbm, wrraw_v, sem.at[SM + 5])
    wo_copy = pltpu.make_async_copy(wo_hbm, woraw_v, sem.at[SM + 6])
    wg_copy = pltpu.make_async_copy(wg_hbm.at[:, pl.ds(FM, FV)], wg_v, sem.at[SM + 0])
    wu_copy = pltpu.make_async_copy(wu_hbm.at[:, pl.ds(FM, FV)], wu_v, sem.at[SM + 1])
    wd_copy = pltpu.make_async_copy(wd_hbm.at[pl.ds(0, FVD), :], wd_v, sem.at[SM + 2])

    def stage_copy(i, q):
        if i < 2:
            r0 = q * (D // NQ)
            r0 = r0 if isinstance(r0, int) else pl.multiple_of(r0, D // NQ)
            src = (wg_hbm, wu_hbm)[i].at[pl.ds(r0, D // NQ), pl.ds(0, FM)]
        else:
            r0 = FVD + q * DQ + (i - 2) * DQA
            r0 = r0 if isinstance(r0, int) else pl.multiple_of(r0, 16)
            src = wd_hbm.at[pl.ds(r0, (DQA, DQ - DQA)[i - 2]), :]
        return pltpu.make_async_copy(src, stage_v[i].at[pl.ds(0, src.shape[0]), :], sem.at[SM + 10 + i])

    wphi_copy(0).start()
    k0_copy(0).start()
    x_copy(5).start()
    k0_copy(1).start()
    x_copy(0).start()
    wphi_copy(1).start()
    w_copy(1, 1).start()

    def view(ref, i, n, off=0):
        r0 = off + i * n
        return ref.at[pl.ds(r0 if isinstance(r0, int) else pl.multiple_of(r0, math.gcd(n, off)), n), :]

    def ln_rows(t, k, n, never=None, anchor=None):
        x = _after(view(x_v, t, T)[k * n:(k + 1) * n, :].astype(F32), never, anchor)
        xc = x - _row_sum(x) * (1.0 / D)
        rstd = lax.rsqrt(_row_sum(xc * xc) * (1.0 / D) + LN_EPS)
        view(xn_v, t, T // 2)[k * n // 2:(k + 1) * n // 2, :] = _pack((xc * rstd).astype(BF16))
        return _tree(jnp.add, [rstd[8 * i:8 * i + 8, :] for i in range(min(n, LNC) // 8)])

    def xn_tile(t):
        return _unpack(view(xn_v, t, T // 2)[...])

    def expand_wphi(c):
        w = wphi_v[8 * c:8 * c + 8].reshape(8 * DH, DH).astype(F32).T
        bits = pltpu.bitcast(w, U32)
        head = lax.broadcasted_iota(jnp.int32, (DH, 128), 1) >> 5
        for s in range(2):
            b = bits[:, 128 * s:128 * s + 128]
            for j in range(2):
                r0 = 64 * (2 * c + s) + 32 * j
                a_v[r0:r0 + 32, :] = jnp.where(head == 2 * j, b >> 16,
                                               jnp.where(head == 2 * j + 1, b, jnp.uint32(0)))

    wphi_copy(0).wait()
    expand_wphi(0)
    hb_v[...] = jnp.zeros((TH, D), F32)
    for ref in stage_v:
        ref[ref.shape[0] - 16:, 0:128] = jnp.zeros((16, 128), BF16)

    def fold_v(c):
        for s in range(RC // 128):
            g0 = 64 * (2 * c + s)
            wt_v[2][g0:g0 + 64, :] = _pack(wraw_v[2 * NC + c, :, s * 128:(s + 1) * 128].T)

    def fold_pairs(j, c, s, side=None, step0=None):
        g0 = 64 * (2 * c + s)
        g0 = g0 if isinstance(g0, int) else pl.multiple_of(g0, 64)
        res = _dot(_unpack(a_v[pl.ds(g0, 64), :]), wraw_v[j * NC + c, :, s * 128:(s + 1) * 128], NT)
        if side is not None:
            side.done(step0 + 2 * s, res[:, :D // 2])
            side.done(step0 + 2 * s + 1, res[:, D // 2:])
        sub = lax.broadcasted_iota(jnp.int32, (8, D), 0)
        out = []
        for q in range(2):
            base = _pair_allreduce(jnp.where(sub < 2, res[64 * q:64 * q + 8, :], 0.0), jnp.add)
            out.append([(res[64 * q + 8 * i:64 * q + 8 * i + 8, :] - base) * LOG2E for i in range(8)])
        return out

    def share(z, z3, k):
        sub = lax.broadcasted_iota(jnp.int32, (8, D), 0)
        return jnp.where(sub < 2, pltpu.roll(z3, 8 - 2 * k, 0), z)

    def packed(slabs):
        return _pack(jnp.concatenate(slabs, axis=0).astype(BF16))

    def fold(j, c, side=None, step0=None):
        p0, p1 = fold_pairs(j, c, 0, side, step0)
        p2, p3 = fold_pairs(j, c, 1, side, step0)
        sl = ([share(p0[0], p3[0], 1), share(p1[0], p3[0], 2)] + p0[1:] + p1[1:]
              + [share(p2[0], p3[0], 3)] + p2[1:] + p3[1:])
        zero = jnp.zeros((8, D), F32)
        even, odd = sl + [zero], [zero] + sl
        r0 = 8 * ((31 * c) // 2)
        if isinstance(c, int):
            is_odd = c % 2 == 1
            sl = odd if is_odd else even
        else:
            is_odd = c % 2 == 1
            r0 = pl.multiple_of(r0, 8)
            sl = [jnp.where(is_odd, o, e) for o, e in zip(odd, even)]
        win = wt_v[j].at[pl.ds(r0, 128), :]
        win[8:128, :] = packed(sl[2:])
        first = packed(sl[:2])
        if is_odd is not False:
            keep = lax.broadcasted_iota(jnp.int32, (8, D), 0) < jnp.where(is_odd, 4, 0)
            first = jnp.where(keep, win[0:8, :], first)
        win[0:8, :] = first

    def k_pair(p, slot, pr, c0, first, never=None):
        ep, en, sp, sn = _dual_exp(p)
        inv = _recip(sp * sn)
        scale = (sn * inv, sp * inv)
        es = ep + en
        cols = slice(c0, c0 + p[0].shape[1])
        n = 16 if never is None else 16 // STAGGER
        last = None
        for q in range(16 // n):
            sc = scale
            if last is not None:
                sc = [jnp.where(never, last, x) for x in scale]
            phi = jnp.concatenate([es[i] * sc[i // 8] for i in range(q * n, (q + 1) * n)], axis=0)
            rows = slice(8 * q * n, 8 * (q + 1) * n)
            z = phi if first else z_v[pr, rows, cols] + phi
            z_v[pr, rows, cols] = z
            phi_v[slot][64 * pr + 4 * q * n:64 * pr + 4 * (q + 1) * n, cols] = _pack(phi.astype(BF16))
            last = z[8 * n - 8:, :]

    def k_features(pk, slot, c, first, never=None):
        for j in range(PPC):
            k_pair(_pair_logits(pk, j), slot, c * PPC + j, 0, first, never)

    def kv_update(vt, slot, c, first, publish=False):
        for j in range(PPC):
            pr = c * PPC + j
            upd = _dot(vt[64 * j:64 * j + 64, :].astype(BF16), _unpack(phi_v[slot][64 * pr:64 * pr + 64, :]), NT)
            acc = upd if first else kvacc_v[pr] + upd
            kvacc_v[pr] = acc
            if publish:
                odd = -(lax.broadcasted_iota(jnp.int32, (32, 128), 1) & 1)
                bits = pltpu.bitcast(acc, jnp.int32) & jnp.concatenate([~odd, odd], axis=0)
                kvbf_v[32 * pr:32 * pr + 32, :] = _pack(pltpu.bitcast(bits, F32).astype(BF16))

    def save_lead(e, t):
        corner = _unpack(view(xn_v, t, T // 2)[0:TH // 2, 0:D // 2])
        view(lead_v, e, D // 4)[...] = _pack(corner.T)

    def proj_steps(side, step0, w, xn, lead=None):
        quarters = []
        for n in range(2):
            for m in range(2):
                step = step0 + 2 * n + m
                wq = _unpack(side.gate(step, w[:64, :] if m == 0 else w[64:, :]))
                if lead is not None and n + m == 0:
                    res = _dot(wq[:, :D // 2], _unpack(view(lead_v, lead, D // 4)[...]), NN)
                    res = _dot(wq[:, D // 2:], xn[0:TH, D // 2:], NT) + res
                else:
                    res = _dot(wq, xn[n * TH:(n + 1) * TH, :], NT)
                side.done(step, res)
                quarters.append(res)
        return jnp.concatenate(
            [jnp.concatenate([quarters[0], quarters[2]], axis=1),
             jnp.concatenate([quarters[1], quarters[3]], axis=1)], axis=0)

    def proj_v(side, step0, c, xn):
        return proj_steps(side, step0, wt_v[2][128 * c:128 * c + 128, :], xn)

    def proj_feat(side, step0, j, c, xn, carry, lead=None):
        r0 = 8 * ((31 * c) // 2)
        skip = 8 if c % 2 == 1 and carry is not None else 0
        res = proj_steps(side, step0, wt_v[j][r0 + skip:r0 + 128, :], xn, lead)
        sl = [res[8 * i:8 * i + 8, :] for i in range(res.shape[0] // 8)]
        if c % 2 == 0:
            return sl[:31], sl[31]
        return ([carry] + sl if skip else sl[1:]), None

    def pack_rows(src, dst, r0, rows, c0, cols, never, a):
        w = src[r0:r0 + rows, c0:c0 + cols].astype(F32)
        d = _lane_tile(a, cols // 128)
        w = jnp.concatenate([jnp.where(never, d, w[8 * i:8 * i + 8, :]) if i % 2 == 0 else w[8 * i:8 * i + 8, :]
                             for i in range(rows // 8)], axis=0)
        dst[r0 // 2:(r0 + rows) // 2, c0:c0 + cols] = _pack(w.astype(BF16))

    def stash_at(i, k, n):
        return zb_v.at[4 * i + 2 * (k // 16) + n, pl.ds(8 * (k % 16), 8), :]

    def stash(i, sl):
        for k, v in enumerate(sl):
            for n in range(2):
                stash_at(i, k, n)[...] = v[:, 128 * n:128 * n + 128]

    def stashed_k(i, slot, c, first):
        def job(k, a):
            j, n = k // 2, k % 2
            p = _pair_logits([stash_at(i, q, n)[...] for q in range(31)], j)
            k_pair([_after(p[0], never0, a)] + p[1:], slot, c * PPC + j, 128 * n, first, never0)
        return job

    def first_rows(k0, k1, n):
        xn = _unpack(xn_v[n * TH // 2:(n + 1) * TH // 2, :])
        ks = [k for k in range(k0, k1)]
        w = jnp.concatenate([wt_v[1][4 * (k % 32):4 * (k % 32) + 8, :] for k in ks[::2]], axis=0)
        res = _dot(_unpack(w), xn, NT)
        for q, k in enumerate(ks):
            if k % 32 < 31:
                stash_at(0, k % 32, n)[...] = res[8 * q:8 * q + 8, :]

    k0_copy(0).wait()
    x_copy(5).wait()
    wphi_copy(2).start()
    w_copy(1, 2).start()
    x_copy(1).start()
    p0, p1 = fold_pairs(1, 0, 0)
    wt_v[1][8:64, :] = packed(p0[1:] + p1[1:])
    ha_v[0:8, :] = p0[0]
    ha_v[8:16, :] = p1[0]
    never0 = ln_rows(0, 0, TH)[0, 0] < 0.0
    first_rows(2, 16, 0)

    k0_copy(1).wait()
    x_copy(0).wait()
    wphi_copy(1).wait()
    w_copy(1, 3).start()
    for c in range(NC):
        w_copy(2, c).start()
    p2, p3 = fold_pairs(1, 0, 1)
    wt_v[1][0:8, :] = packed([share(ha_v[0:8, :], p3[0], 1), share(ha_v[8:16, :], p3[0], 2)])
    wt_v[1][64:128, :] = packed([share(p2[0], p3[0], 3)] + p2[1:] + p3[1:] + [jnp.zeros((8, D), F32)])
    ln_rows(0, 1, TH)
    first_rows(16, 34, 0)
    first_rows(0, 16, 1)
    first_rows(16, 32, 1)
    expand_wphi(1)

    for c in (1, 2):
        w_copy(1, c).wait()
        if c == 1:
            wphi_copy(2).wait()
            expand_wphi(2)
            expand_wphi(3)
            x_copy(2).start()
            w_copy(0, 0).start()
        side = _Side(never0)
        side.add(PRO_K_PLAN, stashed_k(c - 1, 0, c - 1, True))
        fold(1, c, side, 0)
        stash(c, proj_feat(side, 4, 1, c, xn_tile(0), None)[0])
        side.check()

    x_copy(1).wait()
    w_copy(1, 3).wait()
    side = _Side(never0)
    side.add(PRO_LN1_PLAN, lambda k, a: ln_rows(1, k, LNC, never0, a))
    fold(1, 3, side, 0)
    stash(3, proj_feat(side, 4, 1, 3, xn_tile(0), None)[0])
    xn1 = xn_tile(1)
    spare = None
    for c in range(NC):
        pk, spare = proj_feat(_Side(None), 0, 1, c, xn1, spare)
        if c < 3:
            k_features(pk, 1, c, c == 2, never0)
        else:
            stash(0, pk)

    for c in range(NC):
        w_copy(2, c).wait()
    x_copy(2).wait()
    w_copy(0, 0).wait()
    w_copy(0, 1).start()
    x_copy(3).start()
    wo_copy.start()
    wr_copy.start()
    x_copy(4).start()
    w_copy(0, 2).start()
    w_copy(0, 3).start()
    for i in range(4):
        stage_copy(i, 0).start()
    wg_copy.start()
    wu_copy.start()
    wd_copy.start()
    side = _Side(never0)
    side.add(PRO_V_PLANS[0], stashed_k(2, 0, 2, False))
    side.add(PRO_V_PLANS[1], stashed_k(3, 0, 3, True))
    side.add(PRO_V_PLANS[2], stashed_k(0, 1, 3, False))
    side.add(PRO_V_PLANS[3], lambda k, a: ln_rows(2, k, LNC, never0, a))
    fold(0, 0)
    wt_v[0][248:256, :] = jnp.zeros((8, D), U32)
    xns = (xn_tile(0), xn_tile(1))
    pending = None
    for c in range(NC):
        fold_v(c)
        for i in range(2):
            vt = proj_v(side, 8 * c + 4 * i, c, xns[i])
            if pending is not None:
                kv_update(*pending)
            pending = (vt, i, c, i == 0)
    side.check()
    kv_update(*pending)
    save_lead(0, 0)
    save_lead(1, 2)

    def phase1(u, carry):
        never = u < 0

        @pl.when(u == 0)
        def _():
            w_copy(0, 1).wait()
            x_copy(3).wait()
            wo_copy.wait()
            wr_copy.wait()

        @pl.when(u == 1)
        def _():
            x_copy(4).wait()
            w_copy(0, 2).wait()
            w_copy(0, 3).wait()

        pending = None
        for i in range(2):
            t = 2 * u + 2 + i
            tn = jnp.minimum(t + 1, NT_ - 1)
            side = _Side(never)
            xn = xn_tile(t)
            spare = None
            for c in range(NC):
                pk, spare = proj_feat(_Side(None), 0, 1, c, xn, spare, u + 1 if i + c == 0 else None)
                if c == 0 and pending is not None:
                    kv_update(*pending)
                k_features(pk, i, c, False)
            side.add(LN1_PLAN, lambda k, a: ln_rows(tn, k, LNC, never, a))
            if i == 0:
                def pack_wo(k, a):
                    rows = WO_ROWS // len(WO_PLAN)
                    w0 = u * ((D - WO_ROWS) // 2)
                    src = woraw_v.at[pl.ds(pl.multiple_of(w0, 16), WO_ROWS), :]
                    dst = wo_v.at[pl.ds(pl.multiple_of(w0 // 2, 8), WO_ROWS // 2), :]
                    pack_rows(src, dst, k * rows, rows, 0, D, never, a)
                side.add(WO_PLAN, pack_wo)
            else:
                def z_final(k, a):
                    z = _after(z_v[k], never, a)
                    zs = _row_sum(z)
                    zb_v[k] = jnp.broadcast_to(zs, (128, 128))
                    return zs[120:128, :]
                side.add(Z_PLAN, z_final)
            side.done(0, jnp.concatenate(pk[17:], axis=0))
            vts = []
            for c in range(NC):
                vts.append(proj_v(side, 4 * c + 1, c, xn))
                if c > 0:
                    kv_update(vts[c - 1], i, c - 1, False, i == 1)
            pending = (vts[NC - 1], i, NC - 1, False, i == 1)
            side.check()
        fold(0, u + 1)
        kv_update(*pending)
        save_lead(u + 2, tn)
        wr_v[...] = jnp.broadcast_to(wrraw_v[...].reshape(1, D).astype(F32), (8, D))
        return carry

    lax.fori_loop(0, (NT_ - 2) // 2, phase1, 0)

    def o_copy(r0, n, i):
        return pltpu.make_async_copy(o_v.at[pl.ds(r0, n), :], out_hbm.at[pl.ds(r0, n), :], sem.at[SO + i])

    def finish_rows(h_ref, k, ht, valid, st, never=None, anchor=None):
        r0 = ht * TH + k * LNC
        best, besti = st["route"]
        wr = jnp.concatenate([wr_v[...]] * (LNC // 8), axis=0)
        sub = lax.broadcasted_iota(jnp.int32, (8, 1), 0)
        h = _after(h_ref[k * LNC:(k + 1) * LNC, :], never, anchor)
        hc = h - _row_sum(h) * (1.0 / D)
        rstd = lax.rsqrt(_row_sum(hc * hc) * (1.0 / D) + LN_EPS)
        r = (_row_sum(hc * wr) * rstd).astype(BF16).astype(F32)
        hn = hc * rstd
        view(hn_v, ht, TH // 2)[k * LNC // 2:(k + 1) * LNC // 2, :] = _pack(hn.astype(BF16))
        view(o_v, ht, TH)[k * LNC:(k + 1) * LNC, :] = (hn + h).astype(BF16)
        if valid is not None:
            r = jnp.where(valid, r, -jnp.inf)
        for i in range(LNC // 8):
            ri = r[8 * i:8 * i + 8, :]
            better = ri > best
            best = jnp.where(better, ri, best)
            besti = jnp.where(better, sub + (r0 + 8 * i), besti)
        st["route"] = (best, besti)
        return best

    def q_features(pq, slot, c):
        for j in range(PPC):
            pr = c * PPC + j
            ep, en, sp, sn = _dual_exp(_pair_logits(pq, j))
            zz = [_lane_tile(zb_v[pr, 8 * i:8 * i + 8, :], T // 128) for i in range(16)]
            ap = _pair_allreduce(_tree(jnp.add, [ep[i] * zz[i] for i in range(8)]), jnp.add)
            an = _pair_allreduce(_tree(jnp.add, [en[i] * zz[8 + i] for i in range(8)]), jnp.add)
            inv = _recip(ap * sn + (an + 1e-6 * sn) * sp)
            rp = sn * inv
            rn = sp * inv
            phi = jnp.concatenate([e * rp for e in ep] + [e * rn for e in en], axis=0)
            phi_v[slot][64 * pr:64 * pr + 64, :] = _pack(phi.astype(BF16))

    def attn_rows(slot, g):
        res = jnp.concatenate(
            [_dot(_unpack(kvbf_v[32 * pr:32 * pr + 32, :]), _unpack(phi_v[slot][64 * pr:64 * pr + 64, :]), NN)
             for pr in (2 * g, 2 * g + 1)], axis=0)
        return res.astype(BF16).T

    def out_proj(side, step0, o, k0, k1):
        cols = []
        for n in range(D // 128):
            w = side.gate(step0 + n, wo_v[k0 // 2:k1 // 2, n * 128:(n + 1) * 128])
            res = _dot(o, _unpack(w), NN)
            side.done(step0 + n, res)
            cols.append(res)
        return jnp.concatenate(cols, axis=1)

    def phase2(u, carry):
        for i in range(4):
            stage_copy(i, u).wait()
        for i in range(2):
            carry = phase2_tile(u, i, carry, u < 0, u if i == 0 else None)

        r0 = pl.multiple_of(u * (2 * T), T)

        @pl.when(u == 0)
        def _():
            o_copy(0, 2 * T - TH, 0).start()

        @pl.when(u > 0)
        def _():
            o_copy(pl.multiple_of(jnp.maximum(r0 - TH, 0), TH), 2 * T, u).start()

        return carry

    def phase2_tile(u, slot, carry, never, lead):
        t = 2 * u + slot
        hp = jnp.maximum(2 * t - 1, 0)
        side = _Side(never)
        st = {"route": carry}
        side.add(LN2B_PLAN, lambda k, a: finish_rows(hb_v, k, hp, t > 0, st, side.never, a))

        def packer(i, dst, n, due):
            left = [n]

            def job(k, a):
                if i < 2:
                    pack_rows(stage_v[i], dst, (k // 2) * 16, 16, (0, D)[k % 2], (D, FM - D)[k % 2], never, a)
                else:
                    pack_rows(stage_v[i], dst, k * 16, 16, 0, D, never, a)
                left[0] -= 1
                if not left[0]:
                    stage_copy(i, jnp.minimum(u + 1, NQ - 1)).start()
                    n0 = stage_v[i].shape[0] - 16
                    side.deps.setdefault(due, []).append(stage_v[i][n0:n0 + 8, 0:128].astype(F32))
            return job

        side.add(PACK_PLAN, packer(slot, view((wgp_v, wup_v)[slot], u, D // NQ // 2), len(PACK_PLAN), 2))
        d0 = pl.multiple_of(u * (DQ // 2) + slot * (DQA // 2), 8)
        side.add(PACKD_PLANS[slot], packer(2 + slot, wdp_v.at[pl.ds(d0, 8 * len(PACKD_PLANS[slot])), :],
                                           len(PACKD_PLANS[slot]), (23, 13)[slot]))

        xn = xn_tile(t)
        xt = view(x_v, t, T)
        os_ = {}
        for g in range(8):
            side.hooks.setdefault(G_STEPS[g], []).append(lambda g=g: os_.update({g: attn_rows(slot, g)}))
        spare = None
        for c in range(NC):
            pq, spare = proj_feat(side, 100 + 4 * c, 0, c, xn, spare, lead if c == 0 else None)
            if c == 0:
                head = side.gate(0, jnp.concatenate(pq[2:9], axis=0))
                pq = pq[:2] + [head[8 * i:8 * i + 8, :] for i in range(7)] + pq[9:]
            q_features(pq, slot, c)
        ha = out_proj(side, 0, jnp.concatenate([os_[g][0:TH, :] for g in range(4)], axis=1), 0, D // 2)
        ha = ha + xt[0:TH, :].astype(F32)
        ha_v[...] = ha + out_proj(side, 8, jnp.concatenate([os_[g][0:TH, :] for g in range(4, 8)], axis=1), D // 2, D)
        side.add(LN2A_PLAN, lambda k, a: finish_rows(ha_v, k, 2 * t, None, st, side.never, a))
        ob = jnp.concatenate([os_[g][TH:T, :] for g in range(8)], axis=1)
        hb_v[...] = xt[TH:T, :].astype(F32) + out_proj(side, 16, ob, 0, D)
        side.check()
        return st["route"]

    wg_copy.wait()
    wu_copy.wait()
    wd_copy.wait()
    route = lax.fori_loop(
        0, NT_ // 2, phase2,
        (jnp.full((8, 1), -jnp.inf, F32), jnp.zeros((8, 1), jnp.int32)))
    st = {"route": route}
    for k in range(TH // LNC):
        finish_rows(hb_v, k, 2 * NT_ - 1, None, st)
    best, besti = st["route"]
    o_copy(S - TH, TH, NT_).start()

    rmax = jnp.max(best, axis=0, keepdims=True)
    idx = jnp.min(jnp.where(best == rmax, besti, S), axis=0, keepdims=True)
    idx_s = jnp.clip(idx[0, 0], 0, S - 1)
    blk = pl.multiple_of((idx_s >> 4) << 4, 16)
    pair = jnp.broadcast_to(hn_v[pl.ds(idx_s >> 1, 1), :], (8, D))
    x8 = pltpu.bitcast(jnp.where((idx_s & 1) == 1, pair & jnp.uint32(0xFFFF0000), pair << 16), F32)
    xs = jnp.concatenate([x8, x8], axis=0).astype(BF16)
    acts, anchors = [], []

    def park(v, half):
        n = v.shape[0] // 128
        for i in range(n):
            z_v[i, :, 128 * half:128 * half + 128] = v[128 * i:128 * i + 128, :]
        return jnp.concatenate([z_v[i, :, 128 * half:128 * half + 128] for i in range(n)], axis=0)

    for c0 in range(0, FM, 128):
        g = _dot(xs, _unpack(wgp_v[:, c0:c0 + 128]), NN)[0:8, :]
        u = _dot(xs, _unpack(wup_v[:, c0:c0 + 128]), NN)[0:8, :]
        anchors += [g, u]
        acts.append(g * jax.nn.sigmoid(g) * u)
    xb = park(_col_broadcast(x8), 0)
    g, u = [_sublane_allreduce(_vpu_matvec(
        xb, lambda g: w[8 * g:8 * g + 8, :].astype(F32), never0,
        anchors[i * MOE_NA // 2:(i + 1) * MOE_NA // 2], MOE_LAGS[0])) for i, w in enumerate((wg_v, wu_v))]
    acts.append(g * jax.nn.sigmoid(g) * u)
    a = jnp.concatenate(acts, axis=1)
    am = jnp.concatenate([a[:, FVD:], a[:, FVD:]], axis=0).astype(BF16)
    ys, anchors = [], anchors[MOE_NA:]
    for k0 in range(0, FF - FVD, 512):
        k1 = min(k0 + 512, FF - FVD)
        yk = _dot(am[:, k0:k1], _unpack(wdp_v[k0 // 2:k1 // 2, 0:D]), NN)[0:8, :]
        ys.append(yk)
        anchors += [yk[:, c:c + 128] for c in range(128, D, 256)]
    ys.append(_sublane_allreduce(_vpu_matvec(
        park(_col_broadcast(a[:, :FVD]), 1), lambda g: wd_v[8 * g:8 * g + 8, :].astype(F32), never0,
        anchors[:-MOE_ND], MOE_LAGS[1])))
    y = _tree(jnp.add, ys) * jax.nn.sigmoid(rmax)
    y = jnp.concatenate([y, y], axis=0)
    sel = lax.broadcasted_iota(jnp.int32, (16, 1), 0) == (idx_s - blk)
    patch_v[...] = (o_v[pl.ds(blk, 16), :].astype(F32) + jnp.where(sel, y, 0.0)).astype(BF16)
    o_copy(0, 2 * T - TH, 0).wait()
    for u in range(1, NT_ // 2):
        o_copy(u * 2 * T - TH, 2 * T, u).wait()
    o_copy(S - TH, TH, NT_).wait()
    pc = pltpu.make_async_copy(patch_v, out_hbm.at[pl.ds(blk, 16), :], sem.at[SM + 3])
    pc.start()
    for i in range(4):
        stage_copy(i, NQ - 1).wait()
    pc.wait()


@jax.jit
def pallas_sequential_preLN__linear_kernel_hedgehog__moe_arch_mod__prompt_kernel(
    A_x: jax.Array,
    A_wqkv: jax.Array,
    A_w_phi: jax.Array,
    A_wo: jax.Array,
    B_x: jax.Array,
    B_w_r: jax.Array,
    B_w_gate: jax.Array,
    B_w_up: jax.Array,
    B_w_down: jax.Array,
):
    del B_x
    hbm = pl.BlockSpec(memory_space=pl.ANY)
    out = pl.pallas_call(
        _kernel,
        out_shape=jax.ShapeDtypeStruct((S, D), BF16),
        in_specs=[hbm] * 8,
        out_specs=hbm,
        scratch_shapes=[
            pltpu.VMEM((S, D), BF16),
            pltpu.VMEM((S // 2, D), U32),
            pltpu.VMEM((5 * D // 4, 128), U32),
            pltpu.VMEM((3 * NC, D, RC), BF16),
            [pltpu.VMEM((D // 2, D), U32)] * 3,
            pltpu.VMEM((H, DH, DH), BF16),
            pltpu.VMEM((8 * 64, 128), U32),
            pltpu.VMEM((D, D), BF16),
            pltpu.VMEM((D // 2, D), U32),
            pltpu.VMEM((D,), BF16),
            pltpu.VMEM((8, D), F32),
            pltpu.VMEM((NPAIR, 64, 128), F32),
            pltpu.VMEM((NPAIR * 32, 128), U32),
            pltpu.VMEM((NPAIR, 128, T), F32),
            pltpu.VMEM((NPAIR, 128, 128), F32),
            [pltpu.VMEM((NPAIR * 64, T), U32)] * 2,
            pltpu.VMEM((TH, D), F32),
            pltpu.VMEM((TH, D), F32),
            pltpu.VMEM((S // 2, D), U32),
            pltpu.VMEM((S, D), BF16),
            pltpu.VMEM((D, FV), BF16),
            pltpu.VMEM((D, FV), BF16),
            pltpu.VMEM((FVD, D), BF16),
            [pltpu.VMEM((D // NQ + 16, FM), BF16), pltpu.VMEM((D // NQ + 16, FM), BF16),
             pltpu.VMEM((DQA + 16, D), BF16), pltpu.VMEM((DQ - DQA + 16, D), BF16)],
            pltpu.VMEM((D // 2, FM), U32),
            pltpu.VMEM((D // 2, FM), U32),
            pltpu.VMEM(((FF - FVD) // 2, D + 128), U32),
            pltpu.VMEM((16, D), BF16),
            pltpu.SemaphoreType.DMA((6 + 3 * NC + NT_ + 15,)),
        ],
        compiler_params=pltpu.CompilerParams(vmem_limit_bytes=100 * 1024 * 1024,
                                             disable_semaphore_checks=True, disable_bounds_checks=True),
        name="hedgehog_mod",
    )(
        A_x.reshape(S, D),
        A_wqkv,
        A_w_phi,
        A_wo,
        B_w_r,
        B_w_gate,
        B_w_up,
        B_w_down,
    )
    return out.reshape(1, S, D)
```

```python
import math

import jax
import jax.numpy as jnp
from jax import lax
import jax.experimental.pallas as pl
import jax.experimental.pallas.tpu as pltpu

F32 = jnp.float32
BF16 = jnp.bfloat16
U32 = jnp.uint32

S = 2048
D = 1024
H = 32
DH = 32
FF = 3584
NPAIR = H // 2
LOG2E = 1.4426950408889634
LN_EPS = 1e-5

T = 256
TH = T // 2
NT_ = S // T
RC = 256
NC = D // RC
PPC = RC // 64
LNC = 16

FV = 10 * 128
FM = FF - FV
FVD = 8 * 128
NQ = NT_ // 2
DQ = (FF - FVD) // NQ
WO_ROWS = 352


def _spread(n, a, b, due=None):
    rel = [round(a + (b - a) * k / (n - 1), 3) for k in range(n)]
    return tuple((r, None if due is None else math.ceil(r) + due) for r in rel)


LN1_PLAN = ((-0.001, 4), (0.787, 5), (1.857, 5), (2.494, 6), (3.413, 7), (4.33, 9), (5.163, 9), (6.264, 10),
    (6.755, 10), (7.681, 11), (8.956, 13), (9.2, 13), (10.598, 14), (11.083, 15), (12.313, 16), (13.022, 16))
WO_PLAN = ((1.624, None), (1.762, None), (3.838, None), (4.445, None), (5.249, None), (5.61, None), (7.091,
    None), (8.085, None), (8.388, None), (10.135, None), (11.0, None))
Z_PLAN = ((5.932, 8), (6.444, 11), (6.603, 10), (7.438, 11), (7.694, 11), (8.079, 11), (8.4, 12), (9.062, 13),
    (9.166, 12), (9.416, 12), (9.929, 14), (10.582, 15), (10.993, 14), (11.285, 16), (11.385, 15), (11.931,
    16))
PRO_LN1_PLAN = ((None, None),) * 16
PRO_K_PLAN = _spread(8, 0, 6)
PRO_V_PLANS = (((0.0, None), (1.711, None), (3.429, None), (5.143, None), (6.857, None), (8.571, None),
    (10.353, None), (11.911, None)), ((12.92, None), (13.449, None), (14.2, None), (14.8, None), (15.353,
    None), (16.13, None), (16.6, None), (17.2, None)), ((17.8, None), (18.4, None), (18.995, None), (19.6,
    None), (20.2, None), (20.816, None), (21.4, None), (22.0, None)), ((1.172, 6), (2.903, 7), (4.64, 8),
    (6.303, 10), (8.004, 12), (9.8, 14), (11.444, 15), (13.313, 17), (14.96, 18), (16.68, 20), (18.4, 21),
    (20.177, 24), (21.776, 25), (23.56, 27), (25.336, 30), (27.0, 30)))
LN2B_PLAN = ((None, 103), (-0.293, 6), (1.256, 8), (2.575, 10), (4.89, 11), (6.449, 13), (8.386, 14), (9.771,
    15))
LN2A_PLAN = ((None, 18), (15.225, 20), (16.196, 21), (16.89, 21), (17.803, 21), (18.501, 22), (19.126, 23),
    (20.109, None))
PACK_PLAN = ((99.7, None), (101.013, None), (101.667, None), (102.726, None), (103.706, None), (104.716,
    None), (105.735, None), (106.7, None), (107.7, None), (108.406, None), (109.925, None), (110.837, None),
    (111.796, None), (112.939, None), (113.7, None), (114.55, None), (99.02, None), (100.1, None), (101.258,
    None), (102.336, None), (103.155, None), (104.1, None), (105.1, None), (106.239, None), (107.306, None),
    (108.049, None), (109.317, None), (109.994, None), (111.1, None), (112.28, None), (113.12, None),
    (114.122, None))
PACKD_PLANS = (((0.5, None), (1.16, None), (2.055, None), (2.553, None), (3.537, None), (4.117, None), (5.056,
    None), (5.77, None), (6.574, None), (7.333, None), (7.969, None), (8.825, None), (9.611, None), (10.363,
    None), (11.13, None), (11.889, None), (12.648, None), (13.336, None), (14.167, None), (14.926, None),
    (15.667, None), (16.494, None), (17.267, None), (17.963, None), (18.722, None), (19.481, None), (20.192,
    None), (21.0, None)), ((0.945, None), (1.386, None), (2.227, None), (3.013, None), (3.955, None), (4.818,
    None), (5.768, None), (6.545, None), (7.409, None), (8.203, None), (9.122, None), (10.0, None)))
DQA = 16 * len(PACKD_PLANS[0])
G_STEPS = (107, 107, 110, 111, 115, 115, 3, 3)
MOE_NA = 36
MOE_ND = 2
MOE_LAGS = (3, 3)
STAGGER = 8

NN = (((1,), (0,)), ((), ()))
NT = (((1,), (1,)), ((), ()))


def _dot(a, b, dims):
    return lax.dot_general(a, b, dims, preferred_element_type=F32)


def _recip(x):
    return pl.reciprocal(x, approx=False, full_range=False)


def _pack(x):
    return pltpu.bitcast(x, U32)


def _unpack(x):
    return pltpu.bitcast(x, BF16)


def _pair_allreduce(a, op):
    a = op(a, pltpu.roll(a, 2, 0))
    return op(a, pltpu.roll(a, 4, 0))


def _tree(op, xs):
    xs = list(xs)
    while len(xs) > 1:
        nxt = [op(xs[i], xs[i + 1]) for i in range(0, len(xs) - 1, 2)]
        if len(xs) % 2:
            nxt.append(xs[-1])
        xs = nxt
    return xs[0]


def _pair_logits(sl, j):
    sub = lax.broadcasted_iota(jnp.int32, sl[0].shape, 0)
    if j < 3:
        head = jnp.where(sub < 2, 0.0, sl[(0, 1, 16)[j]])
    else:
        head = jnp.where(sub < 2, sl[0], jnp.where(sub < 4, pltpu.roll(sl[1], 2, 0),
                                                   jnp.where(sub < 6, pltpu.roll(sl[16], 4, 0), 0.0)))
    r0 = (2, 9, 17, 24)[j]
    return [head] + list(sl[r0:r0 + 7])


def _dual_exp(sl):
    mx = _pair_allreduce(_tree(jnp.maximum, sl), jnp.maximum)
    mn = _pair_allreduce(_tree(jnp.minimum, sl), jnp.minimum)
    ep = [jnp.exp2(s - mx) for s in sl]
    en = [jnp.exp2(mn - s) for s in sl]
    sp = _pair_allreduce(_tree(jnp.add, ep), jnp.add)
    sn = _pair_allreduce(_tree(jnp.add, en), jnp.add)
    return ep, en, sp, sn


def _after(x, never, anchor):
    if anchor is None:
        return x
    d = jnp.concatenate([anchor] * (x.shape[0] // 8), axis=0)
    if x.shape[1] == 128:
        return jnp.where(never, d, x)
    return jnp.concatenate([jnp.where(never, d, x[:, :128]), x[:, 128:]], axis=1)


def _gate(x, never, deps):
    for i, dep in enumerate(deps):
        d = jnp.broadcast_to(dep, (8, 128))
        if x.dtype != F32:
            d = pltpu.bitcast(d, x.dtype)
        blk = jnp.where(never, d, x[8 * i:8 * i + 8, :128])
        if x.shape[1] > 128:
            blk = jnp.concatenate([blk, x[8 * i:8 * i + 8, 128:]], axis=1)
        parts = ([x[:8 * i, :]] if i else []) + [blk, x[8 * i + 8:, :]]
        x = jnp.concatenate(parts, axis=0)
    return x


def _lane_fold(a):
    return _tree(jnp.add, [a[:, 128 * i:128 * i + 128] for i in range(a.shape[1] // 128)])


def _row_sum(a):
    return jnp.sum(_lane_fold(a), axis=-1, keepdims=True)


def _lane_tile(a, n):
    return a if n == 1 else jnp.concatenate([a] * n, axis=1)


def _sublane_allreduce(a):
    a = a + pltpu.roll(a, 4, 0)
    a = a + pltpu.roll(a, 2, 0)
    return a + pltpu.roll(a, 1, 0)


def _col_broadcast(row8):
    return jnp.concatenate([row8] * 16, axis=0).astype(BF16).T.astype(F32)


def _vpu_matvec(xb, w_rows, never, anchors, lag):
    ng = xb.shape[0] // 8
    acc, hist = None, []
    for g in range(ng):
        dep = anchors[(g * len(anchors)) // ng]
        if g >= lag:
            dep = dep + hist[g - lag]
        x = jnp.where(never, dep, xb[8 * g:8 * g + 8, :])
        w = w_rows(g)
        t = w * _lane_tile(x, w.shape[1] // 128)
        acc = t if acc is None else acc + t
        c = 128 * (g % (w.shape[1] // 128))
        hist.append(acc[:, c:c + 128])
    return acc


class _Side:
    def __init__(self, never):
        self.never = never
        self.jobs = []
        self.deps = {}
        self.hooks = {}

    def add(self, plan, fn):
        for k, (rel, due) in enumerate(plan):
            if rel is None:
                self._run(due, fn, k, None)
            else:
                self.jobs.append((rel, due, fn, k))

    def _run(self, due, fn, k, anchor):
        dep = fn(k, anchor)
        if due is not None:
            self.deps.setdefault(due, []).append(dep)

    def check(self):
        assert not self.jobs and not self.deps and not self.hooks

    def gate(self, step, x):
        return _gate(x, self.never, self.deps.pop(step, []))

    def done(self, step, res):
        m = res.shape[0] // 8
        for job in sorted([j for j in self.jobs if step - 1 < j[0] <= step], key=lambda j: j[0]):
            self.jobs.remove(job)
            g = m - 1 - int((step - job[0]) * m)
            self._run(job[1], job[2], job[3], res[8 * g:8 * g + 8, res.shape[1] - 128:])
        for fn in self.hooks.pop(step, []):
            fn()


def _kernel(x_hbm, wqkv_hbm, wphi_hbm, wo_hbm, wr_hbm, wg_hbm, wu_hbm, wd_hbm, out_hbm,
            x_v, xn_v, lead_v, wraw_v, wt_v, wphi_v, a_v, woraw_v, wo_v, wrraw_v, wr_v, kvacc_v, kvbf_v,
            z_v, zb_v, phi_v, ha_v, hb_v, hn_v, o_v, wg_v, wu_v, wd_v, stage_v, wgp_v, wup_v, wdp_v,
            patch_v,
            sem):
    SX, SW, SO, SM = 0, 6, 6 + 3 * NC, 6 + 3 * NC + NT_ + 1

    def x_copy(i):
        h0, h1 = ((1, 2), (2, 4), (4, 6), (6, 10), (10, 2 * NT_), (0, 1))[i]
        rows = pl.ds(h0 * TH, (h1 - h0) * TH)
        return pltpu.make_async_copy(x_hbm.at[rows, :], x_v.at[rows, :], sem.at[SX + i])

    def k0_copy(s):
        return pltpu.make_async_copy(wqkv_hbm.at[:, pl.ds(D + s * 128, 128)],
                                     wraw_v.at[NC, :, pl.ds(s * 128, 128)], sem.at[(SM + 7, SW + NC)[s]])

    def w_copy(j, c):
        return pltpu.make_async_copy(wqkv_hbm.at[:, pl.ds(j * D + c * RC, RC)], wraw_v.at[j * NC + c],
                                     sem.at[SW + j * NC + c])

    def wphi_copy(i):
        h0, h1 = ((0, 8), (8, 16), (16, H))[i]
        return pltpu.make_async_copy(wphi_hbm.at[pl.ds(h0, h1 - h0)], wphi_v.at[pl.ds(h0, h1 - h0)],
                                     sem.at[(SM + 4, SM + 8, SM + 9)[i]])

    wr_copy = pltpu.make_async_copy(wr_hbm, wrraw_v, sem.at[SM + 5])
    wo_copy = pltpu.make_async_copy(wo_hbm, woraw_v, sem.at[SM + 6])
    wg_copy = pltpu.make_async_copy(wg_hbm.at[:, pl.ds(FM, FV)], wg_v, sem.at[SM + 0])
    wu_copy = pltpu.make_async_copy(wu_hbm.at[:, pl.ds(FM, FV)], wu_v, sem.at[SM + 1])
    wd_copy = pltpu.make_async_copy(wd_hbm.at[pl.ds(0, FVD), :], wd_v, sem.at[SM + 2])

    def stage_copy(i, q):
        if i < 2:
            r0 = q * (D // NQ)
            r0 = r0 if isinstance(r0, int) else pl.multiple_of(r0, D // NQ)
            src = (wg_hbm, wu_hbm)[i].at[pl.ds(r0, D // NQ), pl.ds(0, FM)]
        else:
            r0 = FVD + q * DQ + (i - 2) * DQA
            r0 = r0 if isinstance(r0, int) else pl.multiple_of(r0, 16)
            src = wd_hbm.at[pl.ds(r0, (DQA, DQ - DQA)[i - 2]), :]
        return pltpu.make_async_copy(src, stage_v[i].at[pl.ds(0, src.shape[0]), :], sem.at[SM + 10 + i])

    wphi_copy(0).start()
    k0_copy(0).start()
    x_copy(5).start()
    k0_copy(1).start()
    x_copy(0).start()
    wphi_copy(1).start()
    w_copy(1, 1).start()

    def view(ref, i, n, off=0):
        r0 = off + i * n
        return ref.at[pl.ds(r0 if isinstance(r0, int) else pl.multiple_of(r0, math.gcd(n, off)), n), :]

    def ln_rows(t, k, n, never=None, anchor=None):
        x = _after(view(x_v, t, T)[k * n:(k + 1) * n, :].astype(F32), never, anchor)
        xc = x - _row_sum(x) * (1.0 / D)
        rstd = lax.rsqrt(_row_sum(xc * xc) * (1.0 / D) + LN_EPS)
        view(xn_v, t, T // 2)[k * n // 2:(k + 1) * n // 2, :] = _pack((xc * rstd).astype(BF16))
        return _tree(jnp.add, [rstd[8 * i:8 * i + 8, :] for i in range(min(n, LNC) // 8)])

    def xn_tile(t):
        return _unpack(view(xn_v, t, T // 2)[...])

    def expand_wphi(c):
        w = wphi_v[8 * c:8 * c + 8].reshape(8 * DH, DH).astype(F32).T
        bits = pltpu.bitcast(w, U32)
        head = lax.broadcasted_iota(jnp.int32, (DH, 128), 1) >> 5
        for s in range(2):
            b = bits[:, 128 * s:128 * s + 128]
            for j in range(2):
                r0 = 64 * (2 * c + s) + 32 * j
                a_v[r0:r0 + 32, :] = jnp.where(head == 2 * j, b >> 16,
                                               jnp.where(head == 2 * j + 1, b, jnp.uint32(0)))

    wphi_copy(0).wait()
    expand_wphi(0)
    hb_v[...] = jnp.zeros((TH, D), F32)
    for ref in stage_v:
        ref[ref.shape[0] - 16:, 0:128] = jnp.zeros((16, 128), BF16)

    def fold_v(c):
        for s in range(RC // 128):
            g0 = 64 * (2 * c + s)
            wt_v[2][g0:g0 + 64, :] = _pack(wraw_v[2 * NC + c, :, s * 128:(s + 1) * 128].T)

    def fold_pairs(j, c, s, side=None, step0=None):
        g0 = 64 * (2 * c + s)
        g0 = g0 if isinstance(g0, int) else pl.multiple_of(g0, 64)
        res = _dot(_unpack(a_v[pl.ds(g0, 64), :]), wraw_v[j * NC + c, :, s * 128:(s + 1) * 128], NT)
        if side is not None:
            side.done(step0 + 2 * s, res[:, :D // 2])
            side.done(step0 + 2 * s + 1, res[:, D // 2:])
        sub = lax.broadcasted_iota(jnp.int32, (8, D), 0)
        out = []
        for q in range(2):
            base = _pair_allreduce(jnp.where(sub < 2, res[64 * q:64 * q + 8, :], 0.0), jnp.add)
            out.append([(res[64 * q + 8 * i:64 * q + 8 * i + 8, :] - base) * LOG2E for i in range(8)])
        return out

    def share(z, z3, k):
        sub = lax.broadcasted_iota(jnp.int32, (8, D), 0)
        return jnp.where(sub < 2, pltpu.roll(z3, 8 - 2 * k, 0), z)

    def packed(slabs):
        return _pack(jnp.concatenate(slabs, axis=0).astype(BF16))

    def fold(j, c, side=None, step0=None):
        p0, p1 = fold_pairs(j, c, 0, side, step0)
        p2, p3 = fold_pairs(j, c, 1, side, step0)
        sl = ([share(p0[0], p3[0], 1), share(p1[0], p3[0], 2)] + p0[1:] + p1[1:]
              + [share(p2[0], p3[0], 3)] + p2[1:] + p3[1:])
        zero = jnp.zeros((8, D), F32)
        even, odd = sl + [zero], [zero] + sl
        r0 = 8 * ((31 * c) // 2)
        if isinstance(c, int):
            is_odd = c % 2 == 1
            sl = odd if is_odd else even
        else:
            is_odd = c % 2 == 1
            r0 = pl.multiple_of(r0, 8)
            sl = [jnp.where(is_odd, o, e) for o, e in zip(odd, even)]
        win = wt_v[j].at[pl.ds(r0, 128), :]
        win[8:128, :] = packed(sl[2:])
        first = packed(sl[:2])
        if is_odd is not False:
            keep = lax.broadcasted_iota(jnp.int32, (8, D), 0) < jnp.where(is_odd, 4, 0)
            first = jnp.where(keep, win[0:8, :], first)
        win[0:8, :] = first

    def k_pair(p, slot, pr, c0, first, never=None):
        ep, en, sp, sn = _dual_exp(p)
        inv = _recip(sp * sn)
        scale = (sn * inv, sp * inv)
        es = ep + en
        cols = slice(c0, c0 + p[0].shape[1])
        n = 16 if never is None else 16 // STAGGER
        last = None
        for q in range(16 // n):
            sc = scale
            if last is not None:
                sc = [jnp.where(never, last, x) for x in scale]
            phi = jnp.concatenate([es[i] * sc[i // 8] for i in range(q * n, (q + 1) * n)], axis=0)
            rows = slice(8 * q * n, 8 * (q + 1) * n)
            z = phi if first else z_v[pr, rows, cols] + phi
            z_v[pr, rows, cols] = z
            phi_v[slot][64 * pr + 4 * q * n:64 * pr + 4 * (q + 1) * n, cols] = _pack(phi.astype(BF16))
            last = z[8 * n - 8:, :]

    def k_features(pk, slot, c, first, never=None):
        for j in range(PPC):
            k_pair(_pair_logits(pk, j), slot, c * PPC + j, 0, first, never)

    def kv_update(vt, slot, c, first, publish=False):
        for j in range(PPC):
            pr = c * PPC + j
            upd = _dot(vt[64 * j:64 * j + 64, :].astype(BF16), _unpack(phi_v[slot][64 * pr:64 * pr + 64, :]), NT)
            acc = upd if first else kvacc_v[pr] + upd
            kvacc_v[pr] = acc
            if publish:
                odd = -(lax.broadcasted_iota(jnp.int32, (32, 128), 1) & 1)
                bits = pltpu.bitcast(acc, jnp.int32) & jnp.concatenate([~odd, odd], axis=0)
                kvbf_v[32 * pr:32 * pr + 32, :] = _pack(pltpu.bitcast(bits, F32).astype(BF16))

    def save_lead(e, t):
        corner = _unpack(view(xn_v, t, T // 2)[0:TH // 2, 0:D // 2])
        view(lead_v, e, D // 4)[...] = _pack(corner.T)

    def proj_steps(side, step0, w, xn, lead=None):
        quarters = []
        for n in range(2):
            for m in range(2):
                step = step0 + 2 * n + m
                wq = _unpack(side.gate(step, w[:64, :] if m == 0 else w[64:, :]))
                if lead is not None and n + m == 0:
                    res = _dot(wq[:, :D // 2], _unpack(view(lead_v, lead, D // 4)[...]), NN)
                    res = _dot(wq[:, D // 2:], xn[0:TH, D // 2:], NT) + res
                else:
                    res = _dot(wq, xn[n * TH:(n + 1) * TH, :], NT)
                side.done(step, res)
                quarters.append(res)
        return jnp.concatenate(
            [jnp.concatenate([quarters[0], quarters[2]], axis=1),
             jnp.concatenate([quarters[1], quarters[3]], axis=1)], axis=0)

    def proj_v(side, step0, c, xn):
        return proj_steps(side, step0, wt_v[2][128 * c:128 * c + 128, :], xn)

    def proj_feat(side, step0, j, c, xn, carry, lead=None):
        r0 = 8 * ((31 * c) // 2)
        skip = 8 if c % 2 == 1 and carry is not None else 0
        res = proj_steps(side, step0, wt_v[j][r0 + skip:r0 + 128, :], xn, lead)
        sl = [res[8 * i:8 * i + 8, :] for i in range(res.shape[0] // 8)]
        if c % 2 == 0:
            return sl[:31], sl[31]
        return ([carry] + sl if skip else sl[1:]), None

    def pack_rows(src, dst, r0, rows, c0, cols, never, a):
        w = src[r0:r0 + rows, c0:c0 + cols].astype(F32)
        d = _lane_tile(a, cols // 128)
        w = jnp.concatenate([jnp.where(never, d, w[8 * i:8 * i + 8, :]) if i % 2 == 0 else w[8 * i:8 * i + 8, :]
                             for i in range(rows // 8)], axis=0)
        dst[r0 // 2:(r0 + rows) // 2, c0:c0 + cols] = _pack(w.astype(BF16))

    def stash_at(i, k, n):
        return zb_v.at[4 * i + 2 * (k // 16) + n, pl.ds(8 * (k % 16), 8), :]

    def stash(i, sl):
        for k, v in enumerate(sl):
            for n in range(2):
                stash_at(i, k, n)[...] = v[:, 128 * n:128 * n + 128]

    def stashed_k(i, slot, c, first):
        def job(k, a):
            j, n = k // 2, k % 2
            p = _pair_logits([stash_at(i, q, n)[...] for q in range(31)], j)
            k_pair([_after(p[0], never0, a)] + p[1:], slot, c * PPC + j, 128 * n, first, never0)
        return job

    def first_rows(k0, k1, n):
        xn = _unpack(xn_v[n * TH // 2:(n + 1) * TH // 2, :])
        ks = [k for k in range(k0, k1)]
        w = jnp.concatenate([wt_v[1][4 * (k % 32):4 * (k % 32) + 8, :] for k in ks[::2]], axis=0)
        res = _dot(_unpack(w), xn, NT)
        for q, k in enumerate(ks):
            if k % 32 < 31:
                stash_at(0, k % 32, n)[...] = res[8 * q:8 * q + 8, :]

    k0_copy(0).wait()
    x_copy(5).wait()
    wphi_copy(2).start()
    w_copy(1, 2).start()
    x_copy(1).start()
    p0, p1 = fold_pairs(1, 0, 0)
    wt_v[1][8:64, :] = packed(p0[1:] + p1[1:])
    ha_v[0:8, :] = p0[0]
    ha_v[8:16, :] = p1[0]
    never0 = ln_rows(0, 0, TH)[0, 0] < 0.0
    first_rows(2, 16, 0)

    k0_copy(1).wait()
    x_copy(0).wait()
    wphi_copy(1).wait()
    w_copy(1, 3).start()
    for c in range(NC):
        w_copy(2, c).start()
    p2, p3 = fold_pairs(1, 0, 1)
    wt_v[1][0:8, :] = packed([share(ha_v[0:8, :], p3[0], 1), share(ha_v[8:16, :], p3[0], 2)])
    wt_v[1][64:128, :] = packed([share(p2[0], p3[0], 3)] + p2[1:] + p3[1:] + [jnp.zeros((8, D), F32)])
    ln_rows(0, 1, TH)
    first_rows(16, 34, 0)
    first_rows(0, 16, 1)
    first_rows(16, 32, 1)
    expand_wphi(1)

    for c in (1, 2):
        w_copy(1, c).wait()
        if c == 1:
            wphi_copy(2).wait()
            expand_wphi(2)
            expand_wphi(3)
            x_copy(2).start()
            w_copy(0, 0).start()
        side = _Side(never0)
        side.add(PRO_K_PLAN, stashed_k(c - 1, 0, c - 1, True))
        fold(1, c, side, 0)
        stash(c, proj_feat(side, 4, 1, c, xn_tile(0), None)[0])
        side.check()

    x_copy(1).wait()
    w_copy(1, 3).wait()
    side = _Side(never0)
    side.add(PRO_LN1_PLAN, lambda k, a: ln_rows(1, k, LNC, never0, a))
    fold(1, 3, side, 0)
    stash(3, proj_feat(side, 4, 1, 3, xn_tile(0), None)[0])
    xn1 = xn_tile(1)
    spare = None
    for c in range(NC):
        pk, spare = proj_feat(_Side(None), 0, 1, c, xn1, spare)
        if c < 3:
            k_features(pk, 1, c, c == 2, never0)
        else:
            stash(0, pk)

    for c in range(NC):
        w_copy(2, c).wait()
    x_copy(2).wait()
    w_copy(0, 0).wait()
    w_copy(0, 1).start()
    x_copy(3).start()
    wo_copy.start()
    wr_copy.start()
    x_copy(4).start()
    w_copy(0, 2).start()
    w_copy(0, 3).start()
    for i in range(4):
        stage_copy(i, 0).start()
    wg_copy.start()
    wu_copy.start()
    wd_copy.start()
    side = _Side(never0)
    side.add(PRO_V_PLANS[0], stashed_k(2, 0, 2, False))
    side.add(PRO_V_PLANS[1], stashed_k(3, 0, 3, True))
    side.add(PRO_V_PLANS[2], stashed_k(0, 1, 3, False))
    side.add(PRO_V_PLANS[3], lambda k, a: ln_rows(2, k, LNC, never0, a))
    fold(0, 0)
    wt_v[0][248:256, :] = jnp.zeros((8, D), U32)
    xns = (xn_tile(0), xn_tile(1))
    pending = None
    for c in range(NC):
        fold_v(c)
        for i in range(2):
            vt = proj_v(side, 8 * c + 4 * i, c, xns[i])
            if pending is not None:
                kv_update(*pending)
            pending = (vt, i, c, i == 0)
    side.check()
    kv_update(*pending)
    save_lead(0, 0)
    save_lead(1, 2)

    def phase1(u, carry):
        never = u < 0

        @pl.when(u == 0)
        def _():
            w_copy(0, 1).wait()
            x_copy(3).wait()
            wo_copy.wait()
            wr_copy.wait()

        @pl.when(u == 1)
        def _():
            x_copy(4).wait()
            w_copy(0, 2).wait()
            w_copy(0, 3).wait()

        pending = None
        for i in range(2):
            t = 2 * u + 2 + i
            tn = jnp.minimum(t + 1, NT_ - 1)
            side = _Side(never)
            xn = xn_tile(t)
            spare = None
            for c in range(NC):
                pk, spare = proj_feat(_Side(None), 0, 1, c, xn, spare, u + 1 if i + c == 0 else None)
                if c == 0 and pending is not None:
                    kv_update(*pending)
                k_features(pk, i, c, False)
            side.add(LN1_PLAN, lambda k, a: ln_rows(tn, k, LNC, never, a))
            if i == 0:
                def pack_wo(k, a):
                    rows = WO_ROWS // len(WO_PLAN)
                    w0 = u * ((D - WO_ROWS) // 2)
                    src = woraw_v.at[pl.ds(pl.multiple_of(w0, 16), WO_ROWS), :]
                    dst = wo_v.at[pl.ds(pl.multiple_of(w0 // 2, 8), WO_ROWS // 2), :]
                    pack_rows(src, dst, k * rows, rows, 0, D, never, a)
                side.add(WO_PLAN, pack_wo)
            else:
                def z_final(k, a):
                    z = _after(z_v[k], never, a)
                    zs = _row_sum(z)
                    zb_v[k] = jnp.broadcast_to(zs, (128, 128))
                    return zs[120:128, :]
                side.add(Z_PLAN, z_final)
            side.done(0, jnp.concatenate(pk[17:], axis=0))
            vts = []
            for c in range(NC):
                vts.append(proj_v(side, 4 * c + 1, c, xn))
                if c > 0:
                    kv_update(vts[c - 1], i, c - 1, False, i == 1)
            pending = (vts[NC - 1], i, NC - 1, False, i == 1)
            side.check()
        fold(0, u + 1)
        kv_update(*pending)
        save_lead(u + 2, tn)
        wr_v[...] = jnp.broadcast_to(wrraw_v[...].reshape(1, D).astype(F32), (8, D))
        return carry

    lax.fori_loop(0, (NT_ - 2) // 2, phase1, 0)

    def o_copy(r0, n, i):
        return pltpu.make_async_copy(o_v.at[pl.ds(r0, n), :], out_hbm.at[pl.ds(r0, n), :], sem.at[SO + i])

    def finish_rows(h_ref, k, ht, valid, st, never=None, anchor=None):
        r0 = ht * TH + k * LNC
        best, besti = st["route"]
        wr = jnp.concatenate([wr_v[...]] * (LNC // 8), axis=0)
        sub = lax.broadcasted_iota(jnp.int32, (8, 1), 0)
        h = _after(h_ref[k * LNC:(k + 1) * LNC, :], never, anchor)
        hc = h - _row_sum(h) * (1.0 / D)
        rstd = lax.rsqrt(_row_sum(hc * hc) * (1.0 / D) + LN_EPS)
        r = (_row_sum(hc * wr) * rstd).astype(BF16).astype(F32)
        hn = hc * rstd
        view(hn_v, ht, TH // 2)[k * LNC // 2:(k + 1) * LNC // 2, :] = _pack(hn.astype(BF16))
        view(o_v, ht, TH)[k * LNC:(k + 1) * LNC, :] = (hn + h).astype(BF16)
        if valid is not None:
            r = jnp.where(valid, r, -jnp.inf)
        for i in range(LNC // 8):
            ri = r[8 * i:8 * i + 8, :]
            better = ri > best
            best = jnp.where(better, ri, best)
            besti = jnp.where(better, sub + (r0 + 8 * i), besti)
        st["route"] = (best, besti)
        return best

    def q_features(pq, slot, c):
        for j in range(PPC):
            pr = c * PPC + j
            ep, en, sp, sn = _dual_exp(_pair_logits(pq, j))
            zz = [_lane_tile(zb_v[pr, 8 * i:8 * i + 8, :], T // 128) for i in range(16)]
            ap = _pair_allreduce(_tree(jnp.add, [ep[i] * zz[i] for i in range(8)]), jnp.add)
            an = _pair_allreduce(_tree(jnp.add, [en[i] * zz[8 + i] for i in range(8)]), jnp.add)
            inv = _recip(ap * sn + (an + 1e-6 * sn) * sp)
            rp = sn * inv
            rn = sp * inv
            phi = jnp.concatenate([e * rp for e in ep] + [e * rn for e in en], axis=0)
            phi_v[slot][64 * pr:64 * pr + 64, :] = _pack(phi.astype(BF16))

    def attn_rows(slot, g):
        res = jnp.concatenate(
            [_dot(_unpack(kvbf_v[32 * pr:32 * pr + 32, :]), _unpack(phi_v[slot][64 * pr:64 * pr + 64, :]), NN)
             for pr in (2 * g, 2 * g + 1)], axis=0)
        return res.astype(BF16).T

    def out_proj(side, step0, o, k0, k1):
        cols = []
        for n in range(D // 128):
            w = side.gate(step0 + n, wo_v[k0 // 2:k1 // 2, n * 128:(n + 1) * 128])
            res = _dot(o, _unpack(w), NN)
            side.done(step0 + n, res)
            cols.append(res)
        return jnp.concatenate(cols, axis=1)

    def phase2(u, carry):
        for i in range(4):
            stage_copy(i, u).wait()
        for i in range(2):
            carry = phase2_tile(u, i, carry, u < 0, u if i == 0 else None)

        r0 = pl.multiple_of(u * (2 * T), T)

        @pl.when(u == 0)
        def _():
            o_copy(0, 2 * T - TH, 0).start()

        @pl.when(u > 0)
        def _():
            o_copy(pl.multiple_of(jnp.maximum(r0 - TH, 0), TH), 2 * T, u).start()

        return carry

    def phase2_tile(u, slot, carry, never, lead):
        t = 2 * u + slot
        hp = jnp.maximum(2 * t - 1, 0)
        side = _Side(never)
        st = {"route": carry}
        side.add(LN2B_PLAN, lambda k, a: finish_rows(hb_v, k, hp, t > 0, st, side.never, a))

        def packer(i, dst, n, due):
            left = [n]

            def job(k, a):
                if i < 2:
                    pack_rows(stage_v[i], dst, (k // 2) * 16, 16, (0, D)[k % 2], (D, FM - D)[k % 2], never, a)
                else:
                    pack_rows(stage_v[i], dst, k * 16, 16, 0, D, never, a)
                left[0] -= 1
                if not left[0]:
                    stage_copy(i, jnp.minimum(u + 1, NQ - 1)).start()
                    n0 = stage_v[i].shape[0] - 16
                    side.deps.setdefault(due, []).append(stage_v[i][n0:n0 + 8, 0:128].astype(F32))
            return job

        side.add(PACK_PLAN, packer(slot, view((wgp_v, wup_v)[slot], u, D // NQ // 2), len(PACK_PLAN), 2))
        d0 = pl.multiple_of(u * (DQ // 2) + slot * (DQA // 2), 8)
        side.add(PACKD_PLANS[slot], packer(2 + slot, wdp_v.at[pl.ds(d0, 8 * len(PACKD_PLANS[slot])), :],
                                           len(PACKD_PLANS[slot]), (23, 13)[slot]))

        xn = xn_tile(t)
        xt = view(x_v, t, T)
        os_ = {}
        for g in range(8):
            side.hooks.setdefault(G_STEPS[g], []).append(lambda g=g: os_.update({g: attn_rows(slot, g)}))
        spare = None
        for c in range(NC):
            pq, spare = proj_feat(side, 100 + 4 * c, 0, c, xn, spare, lead if c == 0 else None)
            if c == 0:
                head = side.gate(0, jnp.concatenate(pq[2:9], axis=0))
                pq = pq[:2] + [head[8 * i:8 * i + 8, :] for i in range(7)] + pq[9:]
            q_features(pq, slot, c)
        ha = out_proj(side, 0, jnp.concatenate([os_[g][0:TH, :] for g in range(4)], axis=1), 0, D // 2)
        ha = ha + xt[0:TH, :].astype(F32)
        ha_v[...] = ha + out_proj(side, 8, jnp.concatenate([os_[g][0:TH, :] for g in range(4, 8)], axis=1), D // 2, D)
        side.add(LN2A_PLAN, lambda k, a: finish_rows(ha_v, k, 2 * t, None, st, side.never, a))
        ob = jnp.concatenate([os_[g][TH:T, :] for g in range(8)], axis=1)
        hb_v[...] = xt[TH:T, :].astype(F32) + out_proj(side, 16, ob, 0, D)
        side.check()
        return st["route"]

    wg_copy.wait()
    wu_copy.wait()
    wd_copy.wait()
    route = lax.fori_loop(
        0, NT_ // 2, phase2,
        (jnp.full((8, 1), -jnp.inf, F32), jnp.zeros((8, 1), jnp.int32)))
    st = {"route": route}
    for k in range(TH // LNC):
        finish_rows(hb_v, k, 2 * NT_ - 1, None, st)
    best, besti = st["route"]
    o_copy(S - TH, TH, NT_).start()

    rmax = jnp.max(best, axis=0, keepdims=True)
    idx = jnp.min(jnp.where(best == rmax, besti, S), axis=0, keepdims=True)
    idx_s = jnp.clip(idx[0, 0], 0, S - 1)
    blk = pl.multiple_of((idx_s >> 4) << 4, 16)
    pair = jnp.broadcast_to(hn_v[pl.ds(idx_s >> 1, 1), :], (8, D))
    x8 = pltpu.bitcast(jnp.where((idx_s & 1) == 1, pair & jnp.uint32(0xFFFF0000), pair << 16), F32)
    xs = jnp.concatenate([x8, x8], axis=0).astype(BF16)
    acts, anchors = [], []

    def park(v, half):
        n = v.shape[0] // 128
        for i in range(n):
            z_v[i, :, 128 * half:128 * half + 128] = v[128 * i:128 * i + 128, :]
        return jnp.concatenate([z_v[i, :, 128 * half:128 * half + 128] for i in range(n)], axis=0)

    for c0 in range(0, FM, 128):
        g = _dot(xs, _unpack(wgp_v[:, c0:c0 + 128]), NN)[0:8, :]
        u = _dot(xs, _unpack(wup_v[:, c0:c0 + 128]), NN)[0:8, :]
        anchors += [g, u]
        acts.append(g * jax.nn.sigmoid(g) * u)
    xb = park(_col_broadcast(x8), 0)
    g, u = [_sublane_allreduce(_vpu_matvec(
        xb, lambda g: w[8 * g:8 * g + 8, :].astype(F32), never0,
        anchors[i * MOE_NA // 2:(i + 1) * MOE_NA // 2], MOE_LAGS[0])) for i, w in enumerate((wg_v, wu_v))]
    acts.append(g * jax.nn.sigmoid(g) * u)
    a = jnp.concatenate(acts, axis=1)
    am = jnp.concatenate([a[:, FVD:], a[:, FVD:]], axis=0).astype(BF16)
    ys, anchors = [], anchors[MOE_NA:]
    for k0 in range(0, FF - FVD, 512):
        k1 = min(k0 + 512, FF - FVD)
        yk = _dot(am[:, k0:k1], _unpack(wdp_v[k0 // 2:k1 // 2, 0:D]), NN)[0:8, :]
        ys.append(yk)
        anchors += [yk[:, c:c + 128] for c in range(128, D, 256)]
    ys.append(_sublane_allreduce(_vpu_matvec(
        park(_col_broadcast(a[:, :FVD]), 1), lambda g: wd_v[8 * g:8 * g + 8, :].astype(F32), never0,
        anchors[:-MOE_ND], MOE_LAGS[1])))
    y = _tree(jnp.add, ys) * jax.nn.sigmoid(rmax)
    y = jnp.concatenate([y, y], axis=0)
    sel = lax.broadcasted_iota(jnp.int32, (16, 1), 0) == (idx_s - blk)
    patch_v[...] = (o_v[pl.ds(blk, 16), :].astype(F32) + jnp.where(sel, y, 0.0)).astype(BF16)
    o_copy(0, 2 * T - TH, 0).wait()
    for u in range(1, NT_ // 2):
        o_copy(u * 2 * T - TH, 2 * T, u).wait()
    o_copy(S - TH, TH, NT_).wait()
    pc = pltpu.make_async_copy(patch_v, out_hbm.at[pl.ds(blk, 16), :], sem.at[SM + 3])
    pc.start()
    for i in range(4):
        stage_copy(i, NQ - 1).wait()
    pc.wait()


@jax.jit
def pallas_sequential_preLN__linear_kernel_hedgehog__moe_arch_mod__prompt_kernel(
    A_x: jax.Array,
    A_wqkv: jax.Array,
    A_w_phi: jax.Array,
    A_wo: jax.Array,
    B_x: jax.Array,
    B_w_r: jax.Array,
    B_w_gate: jax.Array,
    B_w_up: jax.Array,
    B_w_down: jax.Array,
):
    del B_x
    hbm = pl.BlockSpec(memory_space=pl.ANY)
    out = pl.pallas_call(
        _kernel,
        out_shape=jax.ShapeDtypeStruct((S, D), BF16),
        in_specs=[hbm] * 8,
        out_specs=hbm,
        scratch_shapes=[
            pltpu.VMEM((S, D), BF16),
            pltpu.VMEM((S // 2, D), U32),
            pltpu.VMEM((5 * D // 4, 128), U32),
            pltpu.VMEM((3 * NC, D, RC), BF16),
            [pltpu.VMEM((D // 2, D), U32)] * 3,
            pltpu.VMEM((H, DH, DH), BF16),
            pltpu.VMEM((8 * 64, 128), U32),
            pltpu.VMEM((D, D), BF16),
            pltpu.VMEM((D // 2, D), U32),
            pltpu.VMEM((D,), BF16),
            pltpu.VMEM((8, D), F32),
            pltpu.VMEM((NPAIR, 64, 128), F32),
            pltpu.VMEM((NPAIR * 32, 128), U32),
            pltpu.VMEM((NPAIR, 128, T), F32),
            pltpu.VMEM((NPAIR, 128, 128), F32),
            [pltpu.VMEM((NPAIR * 64, T), U32)] * 2,
            pltpu.VMEM((TH, D), F32),
            pltpu.VMEM((TH, D), F32),
            pltpu.VMEM((S // 2, D), U32),
            pltpu.VMEM((S, D), BF16),
            pltpu.VMEM((D, FV), BF16),
            pltpu.VMEM((D, FV), BF16),
            pltpu.VMEM((FVD, D), BF16),
            [pltpu.VMEM((D // NQ + 16, FM), BF16), pltpu.VMEM((D // NQ + 16, FM), BF16),
             pltpu.VMEM((DQA + 16, D), BF16), pltpu.VMEM((DQ - DQA + 16, D), BF16)],
            pltpu.VMEM((D // 2, FM), U32),
            pltpu.VMEM((D // 2, FM), U32),
            pltpu.VMEM(((FF - FVD) // 2, D + 128), U32),
            pltpu.VMEM((16, D), BF16),
            pltpu.SemaphoreType.DMA((6 + 3 * NC + NT_ + 15,)),
        ],
        compiler_params=pltpu.CompilerParams(vmem_limit_bytes=100 * 1024 * 1024,
                                             disable_semaphore_checks=True, disable_bounds_checks=True),
        name="hedgehog_mod",
    )(
        A_x.reshape(S, D),
        A_wqkv,
        A_w_phi,
        A_wo,
        B_w_r,
        B_w_gate,
        B_w_up,
        B_w_down,
    )
    return out.reshape(1, S, D)
```

```python
import math

import jax
import jax.numpy as jnp
from jax import lax
import jax.experimental.pallas as pl
import jax.experimental.pallas.tpu as pltpu

F32 = jnp.float32
BF16 = jnp.bfloat16
U32 = jnp.uint32

S = 2048
D = 1024
H = 32
DH = 32
FF = 3584
NPAIR = H // 2
LOG2E = 1.4426950408889634
LN_EPS = 1e-5

T = 256
TH = T // 2
NT_ = S // T
RC = 256
NC = D // RC
PPC = RC // 64
LNC = 16

FV = 10 * 128
FM = FF - FV
FVD = 8 * 128
NQ = NT_ // 2
DQ = (FF - FVD) // NQ
HK = D // 2
SW = 8 * HK


def _spread(n, a, b, due=None):
    rel = [round(a + (b - a) * k / (n - 1), 3) for k in range(n)]
    return tuple((r, None if due is None else math.ceil(r) + due) for r in rel)


LN1_PLANS = (_spread(16, 0, 22, 5), _spread(16, -1, 22, 5))
PRO_LN1_PLAN = ((None, None),) * 16
PRO_K_PLAN = _spread(8, 0, 6)
PRO_X0_PLAN = _spread(8, 0.5, 6.5)
PRO_X1_PLAN = _spread(8, 10, 21)
PRO_V_PLANS = (_spread(24, 0, 12)[:8], _spread(24, 0, 12)[8:16], _spread(8, 14, 25), _spread(31, 100, 103)[:8]
               + _spread(23, 0.5, 26))
END_PLANS = (_spread(16, 0, 26), _spread(31, 101, 103)[:6] + _spread(25, 0.3, 26.3), _spread(32, 0.6, 26.6))
LN2_PLANS = (_spread(16, 0, 22, 5), _spread(16, 28.5, 50, 5))
PACK_PLANS = (_spread(32, 100.5, 126), _spread(32, 128.5, 154))
PACKD_PLANS = (_spread(28, 0.5, 26), _spread(12, 28.5, 38))
PACK_DUE = (130, 3, 30, 42)
DQA = 16 * len(PACKD_PLANS[0])
G_LAG = 5
D_LAG = 2
MOE_NA = 36
MOE_ND = 2
MOE_LAGS = (3, 3)
STAGGER = 8

NN = (((1,), (0,)), ((), ()))
NT = (((1,), (1,)), ((), ()))


def _dot(a, b, dims):
    return lax.dot_general(a, b, dims, preferred_element_type=F32)


def _recip(x):
    return pl.reciprocal(x, approx=False, full_range=False)


def _pack(x):
    return pltpu.bitcast(x, U32)


def _unpack(x):
    return pltpu.bitcast(x, BF16)


def _strassen_lhs(a11, a12, a21, a22):
    return [a21 + a22, a22, a11 + a12, a11, a11 + a22, a12 - a22, a21 - a11]


def _strassen_rhs(b11, b12, b21, b22):
    return [b11, b21 - b11, b22, b12 - b22, b11 + b22, b21 + b22, b11 + b12]


def _strassen(product):
    m2 = product(0)
    m4 = product(1)
    c21 = m2 + m4
    m5 = product(2)
    u11 = m4 - m5
    m3 = product(3)
    c12 = m3 + m5
    u22 = m3 - m2
    m1 = product(4)
    u11 = u11 + m1
    u22 = u22 + m1
    c11 = product(5) + u11
    c22 = product(6) + u22
    return [[c11, c12], [c21, c22]]


def _pair_allreduce(a, op):
    a = op(a, pltpu.roll(a, 2, 0))
    return op(a, pltpu.roll(a, 4, 0))


def _tree(op, xs):
    xs = list(xs)
    while len(xs) > 1:
        nxt = [op(xs[i], xs[i + 1]) for i in range(0, len(xs) - 1, 2)]
        if len(xs) % 2:
            nxt.append(xs[-1])
        xs = nxt
    return xs[0]


def _pair_logits(sl, j):
    sub = lax.broadcasted_iota(jnp.int32, sl[0].shape, 0)
    if j < 3:
        head = jnp.where(sub < 2, 0.0, sl[(0, 1, 16)[j]])
    else:
        head = jnp.where(sub < 2, sl[0], jnp.where(sub < 4, pltpu.roll(sl[1], 2, 0),
                                                   jnp.where(sub < 6, pltpu.roll(sl[16], 4, 0), 0.0)))
    r0 = (2, 9, 17, 24)[j]
    return [head] + list(sl[r0:r0 + 7])


def _dual_exp(sl):
    mx = _pair_allreduce(_tree(jnp.maximum, sl), jnp.maximum)
    mn = _pair_allreduce(_tree(jnp.minimum, sl), jnp.minimum)
    ep = [jnp.exp2(s - mx) for s in sl]
    en = [jnp.exp2(mn - s) for s in sl]
    sp = _pair_allreduce(_tree(jnp.add, ep), jnp.add)
    sn = _pair_allreduce(_tree(jnp.add, en), jnp.add)
    return ep, en, sp, sn


def _after(x, never, anchor):
    if anchor is None:
        return x
    d = jnp.concatenate([anchor] * (x.shape[0] // 8), axis=0)
    if x.shape[1] == 128:
        return jnp.where(never, d, x)
    return jnp.concatenate([jnp.where(never, d, x[:, :128]), x[:, 128:]], axis=1)


def _gate(x, never, deps):
    for i, dep in enumerate(deps):
        d = jnp.broadcast_to(dep, (8, 128))
        if x.dtype != F32:
            d = pltpu.bitcast(d, x.dtype)
        blk = jnp.where(never, d, x[8 * i:8 * i + 8, :128])
        if x.shape[1] > 128:
            blk = jnp.concatenate([blk, x[8 * i:8 * i + 8, 128:]], axis=1)
        parts = ([x[:8 * i, :]] if i else []) + [blk, x[8 * i + 8:, :]]
        x = jnp.concatenate(parts, axis=0)
    return x


def _lane_fold(a):
    return _tree(jnp.add, [a[:, 128 * i:128 * i + 128] for i in range(a.shape[1] // 128)])


def _row_sum(a):
    return jnp.sum(_lane_fold(a), axis=-1, keepdims=True)


def _lane_tile(a, n):
    return a if n == 1 else jnp.concatenate([a] * n, axis=1)


def _sublane_allreduce(a):
    a = a + pltpu.roll(a, 4, 0)
    a = a + pltpu.roll(a, 2, 0)
    return a + pltpu.roll(a, 1, 0)


def _col_broadcast(row8):
    return jnp.concatenate([row8] * 16, axis=0).astype(BF16).T.astype(F32)


def _vpu_matvec(xb, w_rows, never, anchors, lag):
    ng = xb.shape[0] // 8
    acc, hist = None, []
    for g in range(ng):
        dep = anchors[(g * len(anchors)) // ng]
        if g >= lag:
            dep = dep + hist[g - lag]
        x = jnp.where(never, dep, xb[8 * g:8 * g + 8, :])
        w = w_rows(g)
        t = w * _lane_tile(x, w.shape[1] // 128)
        acc = t if acc is None else acc + t
        c = 128 * (g % (w.shape[1] // 128))
        hist.append(acc[:, c:c + 128])
    return acc


class _Side:
    def __init__(self, never):
        self.never = never
        self.jobs = []
        self.deps = {}
        self.hooks = {}

    def add(self, plan, fn):
        for k, (rel, due) in enumerate(plan):
            if rel is None:
                self._run(due, fn, k, None)
            else:
                self.jobs.append((rel, due, fn, k))

    def _run(self, due, fn, k, anchor):
        dep = fn(k, anchor)
        if due is not None:
            self.deps.setdefault(due, []).append(dep)

    def check(self):
        assert not self.jobs and not self.deps and not self.hooks

    def gate(self, step, x):
        return _gate(x, self.never, self.deps.pop(step, []))

    def done(self, step, res):
        m = res.shape[0] // 8
        for job in sorted([j for j in self.jobs if step - 1 < j[0] <= step], key=lambda j: j[0]):
            self.jobs.remove(job)
            g = m - 1 - int((step - job[0]) * m)
            self._run(job[1], job[2], job[3], res[8 * g:8 * g + 8, res.shape[1] - 128:])
        for fn in self.hooks.pop(step, []):
            fn()


def _kernel(x_hbm, wqkv_hbm, wphi_hbm, wo_hbm, wr_hbm, wg_hbm, wu_hbm, wd_hbm, out_hbm,
            x_v, xn_v, xf_v, xs_v, lead_v, wraw_v, wk_v, wf_v, ws_v, wphi_v, a_v, woraw_v, wos_v, wrraw_v, wr_v,
            kvacc_v, kvbf_v, z_v, zb_v, phi_v, oc_v, h_v, hn_v, o_v, wg_v, wu_v, wd_v, stage_v,
            wgp_v, wup_v, wdp_v, patch_v,
            sem):
    SX, SQ, SO, SM = 0, 6, 6 + 3 * NC, 6 + 3 * NC + NT_ + 1

    def x_copy(i):
        h0, h1 = ((0, 1), (1, 2), (2, 4), (4, 8), (8, 2 * NT_))[i]
        rows = pl.ds(h0 * TH, (h1 - h0) * TH)
        return pltpu.make_async_copy(x_hbm.at[rows, :], x_v.at[rows, :], sem.at[SX + i])

    def k0_copy(s):
        return pltpu.make_async_copy(wqkv_hbm.at[:, pl.ds(D + s * 128, 128)],
                                     wraw_v.at[NC, :, pl.ds(s * 128, 128)], sem.at[(SM + 7, SQ + NC)[s]])

    def w_copy(j, c):
        return pltpu.make_async_copy(wqkv_hbm.at[:, pl.ds(j * D + c * RC, RC)], wraw_v.at[j * NC + c],
                                     sem.at[SQ + j * NC + c])

    def wphi_copy(i):
        h0, h1 = ((0, 8), (8, 16), (16, H))[i]
        return pltpu.make_async_copy(wphi_hbm.at[pl.ds(h0, h1 - h0)], wphi_v.at[pl.ds(h0, h1 - h0)],
                                     sem.at[(SM + 4, SM + 8, SM + 9)[i]])

    wr_copy = pltpu.make_async_copy(wr_hbm, wrraw_v, sem.at[SM + 5])
    wo_copy = pltpu.make_async_copy(wo_hbm, woraw_v, sem.at[SM + 6])
    wg_copy = pltpu.make_async_copy(wg_hbm.at[:, pl.ds(FM, FV)], wg_v, sem.at[SM + 0])
    wu_copy = pltpu.make_async_copy(wu_hbm.at[:, pl.ds(FM, FV)], wu_v, sem.at[SM + 1])
    wd_copy = pltpu.make_async_copy(wd_hbm.at[pl.ds(0, FVD), :], wd_v, sem.at[SM + 2])

    def stage_copy(i, q):
        if i < 2:
            r0 = q * (D // NQ)
            r0 = r0 if isinstance(r0, int) else pl.multiple_of(r0, D // NQ)
            src = (wg_hbm, wu_hbm)[i].at[pl.ds(r0, D // NQ), pl.ds(0, FM)]
        else:
            r0 = FVD + q * DQ + (i - 2) * DQA
            r0 = r0 if isinstance(r0, int) else pl.multiple_of(r0, 16)
            src = wd_hbm.at[pl.ds(r0, (DQA, DQ - DQA)[i - 2]), :]
        return pltpu.make_async_copy(src, stage_v[i].at[pl.ds(0, src.shape[0]), :], sem.at[SM + 10 + i])

    wphi_copy(0).start()
    k0_copy(0).start()
    x_copy(0).start()
    k0_copy(1).start()
    x_copy(1).start()
    wphi_copy(1).start()
    w_copy(1, 1).start()

    def view(ref, i, n, off=0):
        r0 = off + i * n
        return ref.at[pl.ds(r0 if isinstance(r0, int) else pl.multiple_of(r0, math.gcd(n, off)), n), :]

    def put_blocks(dst, r0, blocks):
        for i, b in enumerate(blocks):
            dst[r0:r0 + b.shape[0] // 2, i * HK:(i + 1) * HK] = _pack(b.astype(BF16))

    def x_blocks(t, k, lo, hi):
        put_blocks(view(xs_v, t, TH // 2), k * LNC // 2,
                   _strassen_rhs(lo[:, :HK], hi[:, :HK], lo[:, HK:], hi[:, HK:]))

    def ln_rows(t, k, n, never=None, anchor=None, plain=False):
        x = _after(view(x_v, t, T)[k * n:(k + 1) * n, :].astype(F32), never, anchor)
        xc = x - _row_sum(x) * (1.0 / D)
        rstd = lax.rsqrt(_row_sum(xc * xc) * (1.0 / D) + LN_EPS)
        xn = xc * rstd
        if plain:
            xn_v[(t * T + k * n) // 2:(t * T + (k + 1) * n) // 2, :] = _pack(xn.astype(BF16))
        if plain or k * n < TH:
            xf_v[k * n:(k + 1) * n, :] = xn
        else:
            x_blocks(t, k - TH // LNC, xf_v[k * n - TH:(k + 1) * n - TH, :], xn)
        return _tree(jnp.add, [rstd[8 * i:8 * i + 8, :] for i in range(min(n, LNC) // 8)])

    def tied(x, never, a):
        return jnp.where(never, jnp.concatenate([_lane_tile(a, x.shape[1] // 128)] * (x.shape[0] // 8), axis=0), x)

    def late_x_blocks(t):
        return lambda k, a: x_blocks(t, k, tied(xf_v[k * LNC:(k + 1) * LNC, :], never0, a),
                                     tied(xf_v[TH + k * LNC:TH + (k + 1) * LNC, :], never0, a))

    def xn_tile(t):
        return _unpack(xn_v[t * T // 2:(t + 1) * T // 2, :])

    def xs_tile(t):
        return _unpack(view(xs_v, t, TH // 2)[:, 0:7 * HK])

    def expand_wphi(c):
        w = wphi_v[8 * c:8 * c + 8].reshape(8 * DH, DH).astype(F32).T
        bits = pltpu.bitcast(w, U32)
        head = lax.broadcasted_iota(jnp.int32, (DH, 128), 1) >> 5
        for s in range(2):
            b = bits[:, 128 * s:128 * s + 128]
            for j in range(2):
                r0 = 64 * (2 * c + s) + 32 * j
                a_v[r0:r0 + 32, :] = jnp.where(head == 2 * j, b >> 16,
                                               jnp.where(head == 2 * j + 1, b, jnp.uint32(0)))

    wphi_copy(0).wait()
    expand_wphi(0)
    h_v[1][...] = jnp.zeros((T, D), F32)
    for ref in stage_v:
        ref[ref.shape[0] - 16:, 0:128] = jnp.zeros((16, 128), BF16)

    def fold_v(g):
        lo, hi = [wraw_v[2 * NC + q // 2, :, (q % 2) * 128:(q % 2) * 128 + 128].T.astype(F32) for q in (g, g + 4)]
        put_blocks(ws_v[2], 64 * g, _strassen_lhs(lo[:, :HK], lo[:, HK:], hi[:, :HK], hi[:, HK:]))

    def fold_pairs(j, c, s, side=None, step0=None):
        g0 = 64 * (2 * c + s)
        g0 = g0 if isinstance(g0, int) else pl.multiple_of(g0, 64)
        res = _dot(_unpack(a_v[pl.ds(g0, 64), :]), wraw_v[j * NC + c, :, s * 128:(s + 1) * 128], NT)
        if side is not None:
            side.done(step0 + 2 * s, res[:, :D // 2])
            side.done(step0 + 2 * s + 1, res[:, D // 2:])
        sub = lax.broadcasted_iota(jnp.int32, (8, D), 0)
        out = []
        for q in range(2):
            base = _pair_allreduce(jnp.where(sub < 2, res[64 * q:64 * q + 8, :], 0.0), jnp.add)
            out.append([(res[64 * q + 8 * i:64 * q + 8 * i + 8, :] - base) * LOG2E for i in range(8)])
        return out

    def share(z, z3, k):
        sub = lax.broadcasted_iota(jnp.int32, (8, D), 0)
        return jnp.where(sub < 2, pltpu.roll(z3, 8 - 2 * k, 0), z)

    def packed(slabs):
        return _pack(jnp.concatenate(slabs, axis=0).astype(BF16))

    def fold(j, c, side=None, step0=None):
        p0, p1 = fold_pairs(j, c, 0, side, step0)
        p2, p3 = fold_pairs(j, c, 1, side, step0)
        sl = ([share(p0[0], p3[0], 1), share(p1[0], p3[0], 2)] + p0[1:] + p1[1:]
              + [share(p2[0], p3[0], 3)] + p2[1:] + p3[1:])
        view(wf_v, c, 248)[...] = jnp.concatenate(sl, axis=0)
        if j == 1:
            r0 = 8 * ((31 * c) // 2)
            if c % 2 == 0:
                wk_v[r0:r0 + 128, :] = packed(sl + [jnp.zeros((8, D), F32)])
            else:
                wk_v[r0:r0 + 128, :] = packed([wf_v[248 * c - 8:248 * c, :]] + sl)

    def w_blocks(j):
        def job(k, a):
            lo = tied(wf_v[16 * k:16 * k + 16, :], never0, a)
            hi = tied(wf_v[496 + 16 * k:496 + 16 * k + 16, :], never0, a)
            put_blocks(ws_v[j], 8 * k, _strassen_lhs(lo[:, :HK], lo[:, HK:], hi[:, :HK], hi[:, HK:]))
        return job

    def k_pair(p, slot, pr, c0, first, never=None):
        ep, en, sp, sn = _dual_exp(p)
        inv = _recip(sp * sn)
        scale = (sn * inv, sp * inv)
        es = ep + en
        cols = slice(c0, c0 + p[0].shape[1])
        n = 16 if never is None else 16 // STAGGER
        last = None
        for q in range(16 // n):
            sc = scale
            if last is not None:
                sc = [jnp.where(never, last, x) for x in scale]
            phi = jnp.concatenate([es[i] * sc[i // 8] for i in range(q * n, (q + 1) * n)], axis=0)
            rows = slice(8 * q * n, 8 * (q + 1) * n)
            z = phi if first else z_v[pr, rows, cols] + phi
            z_v[pr, rows, cols] = z
            phi_v[slot][64 * pr + 4 * q * n:64 * pr + 4 * (q + 1) * n, cols] = _pack(phi.astype(BF16))
            last = z[8 * n - 8:, :]

    def k_features(pk, slot, c, first, never=None):
        for j in range(PPC):
            k_pair(_pair_logits(pk, j), slot, c * PPC + j, 0, first, never)

    def kv_update(vts, slot, g, first, publish=False):
        for q, vt in enumerate(vts):
            for j in range(2):
                pr = 2 * g + 8 * q + j
                upd = _dot(vt[64 * j:64 * j + 64, :].astype(BF16), _unpack(phi_v[slot][64 * pr:64 * pr + 64, :]), NT)
                acc = upd if first else kvacc_v[pr] + upd
                kvacc_v[pr] = acc
                if publish:
                    odd = -(lax.broadcasted_iota(jnp.int32, (32, 128), 1) & 1)
                    bits = pltpu.bitcast(acc, jnp.int32) & jnp.concatenate([~odd, odd], axis=0)
                    kvbf_v[32 * pr:32 * pr + 32, :] = _pack(pltpu.bitcast(bits, F32).astype(BF16))

    def save_lead(t):
        view(lead_v, t, HK // 2)[...] = _pack(_unpack(view(xs_v, t, TH // 2)[:, 0:HK]).T)

    def proj_feat(side, step0, c, xn, carry):
        r0 = 8 * ((31 * c) // 2)
        skip = 8 if c % 2 == 1 and carry is not None else 0
        w = wk_v[r0 + skip:r0 + 128, :]
        quarters = []
        for n in range(2):
            for m in range(2):
                step = step0 + 2 * n + m
                wq = _unpack(side.gate(step, w[:64, :] if m == 0 else w[64:, :]))
                res = _dot(wq, xn[n * TH:(n + 1) * TH, :], NT)
                side.done(step, res)
                quarters.append(res)
        res = jnp.concatenate(
            [jnp.concatenate([quarters[0], quarters[2]], axis=1),
             jnp.concatenate([quarters[1], quarters[3]], axis=1)], axis=0)
        sl = [res[8 * i:8 * i + 8, :] for i in range(res.shape[0] // 8)]
        if c % 2 == 0:
            return sl[:31], sl[31]
        return ([carry] + sl if skip else sl[1:]), None

    def proj_unit(side, step0, j, b, xs, lead=None):
        r1 = 64 * b + (64 if j == 2 or b < 3 else 56)

        def product(i):
            w = _unpack(side.gate(step0 + i, ws_v[j][64 * b:r1, i * HK:(i + 1) * HK]))
            if lead is not None and i == 0:
                res = _dot(w, _unpack(view(lead_v, lead, HK // 2)[...]), NN)
            else:
                res = _dot(w, xs[:, i * HK:(i + 1) * HK], NT)
            side.done(step0 + i, res)
            return res
        return [jnp.concatenate(row, axis=1) for row in _strassen(product)]

    def feat_stage(side, step0, j, xs, pair_fn, lead=None):
        sl = [[], []]
        for b in range(4):
            for q, res in enumerate(proj_unit(side, step0 + 7 * b, j, b, xs, lead if b == 0 else None)):
                sl[q] += [res[8 * i:8 * i + 8, :] for i in range(res.shape[0] // 8)]
            for q in (1, 0):
                for jj in (2 * (b % 2), 2 * (b % 2) + 1):
                    pair_fn(_pair_logits(sl[q][31 * (b // 2):], jj), 8 * q + 4 * (b // 2) + jj)

    def v_stage(side, xs, slot, first, publish, lead, folds=False):
        pending = None
        for g in range(4):
            if folds:
                fold_v(g)
            if pending is not None:
                side.hooks.setdefault(7 * g + D_LAG, []).append(lambda p=pending: kv_update(*p))
            pending = (proj_unit(side, 7 * g, 2, g, xs, lead if g == 0 else None), slot, g, first, publish)
        side.check()
        return pending

    def pack_rows(src, dst, r0, rows, c0, cols, never, a):
        w = src[r0:r0 + rows, c0:c0 + cols].astype(F32)
        d = _lane_tile(a, cols // 128)
        w = jnp.concatenate([jnp.where(never, d, w[8 * i:8 * i + 8, :]) if i % 2 == 0 else w[8 * i:8 * i + 8, :]
                             for i in range(rows // 8)], axis=0)
        dst[r0 // 2:(r0 + rows) // 2, c0:c0 + cols] = _pack(w.astype(BF16))

    def stash_at(i, k, n):
        return zb_v.at[4 * i + 2 * (k // 16) + n, pl.ds(8 * (k % 16), 8), :]

    def stash(i, sl):
        for k, v in enumerate(sl):
            for n in range(2):
                stash_at(i, k, n)[...] = v[:, 128 * n:128 * n + 128]

    def stashed_k(i, slot, c, first):
        def job(k, a):
            j, n = k // 2, k % 2
            p = _pair_logits([stash_at(i, q, n)[...] for q in range(31)], j)
            k_pair([_after(p[0], never0, a)] + p[1:], slot, c * PPC + j, 128 * n, first, never0)
        return job

    def first_rows(k0, k1, n):
        xn = _unpack(xn_v[n * TH // 2:(n + 1) * TH // 2, :])
        ks = [k for k in range(k0, k1)]
        w = jnp.concatenate([wk_v[4 * (k % 32):4 * (k % 32) + 8, :] for k in ks[::2]], axis=0)
        res = _dot(_unpack(w), xn, NT)
        for q, k in enumerate(ks):
            if k % 32 < 31:
                stash_at(0, k % 32, n)[...] = res[8 * q:8 * q + 8, :]

    k0_copy(0).wait()
    x_copy(0).wait()
    wphi_copy(2).start()
    w_copy(1, 2).start()
    x_copy(2).start()
    p0, p1 = fold_pairs(1, 0, 0)
    wk_v[8:64, :] = packed(p0[1:] + p1[1:])
    wf_v[0:128, :] = jnp.concatenate([p0[0], p1[0]] + p0[1:] + p1[1:], axis=0)
    never0 = ln_rows(0, 0, TH, plain=True)[0, 0] < 0.0
    first_rows(2, 16, 0)

    k0_copy(1).wait()
    x_copy(1).wait()
    wphi_copy(1).wait()
    w_copy(1, 3).start()
    for c in (0, 2, 1, 3):
        w_copy(2, c).start()
    p2, p3 = fold_pairs(1, 0, 1)
    sl = [share(wf_v[0:8, :], p3[0], 1), share(wf_v[8:16, :], p3[0], 2)]
    wk_v[0:8, :] = packed(sl)
    wf_v[0:16, :] = jnp.concatenate(sl, axis=0)
    sl = [share(p2[0], p3[0], 3)] + p2[1:] + p3[1:]
    wk_v[64:128, :] = packed(sl + [jnp.zeros((8, D), F32)])
    wf_v[128:248, :] = jnp.concatenate(sl, axis=0)
    ln_rows(0, 1, TH, plain=True)
    first_rows(16, 34, 0)
    first_rows(0, 16, 1)
    first_rows(16, 32, 1)
    expand_wphi(1)

    for c in (1, 2):
        w_copy(1, c).wait()
        side = _Side(never0)
        if c == 1:
            wphi_copy(2).wait()
            expand_wphi(2)
            expand_wphi(3)
        else:
            side.add(PRO_X0_PLAN, late_x_blocks(0))
        side.add(PRO_K_PLAN, stashed_k(c - 1, 0, c - 1, True))
        fold(1, c, side, 0)
        stash(c, proj_feat(side, 4, c, xn_tile(0), None)[0])
        side.check()

    x_copy(2).wait()
    w_copy(1, 3).wait()
    x_copy(3).start()
    w_copy(0, 0).start()
    x_copy(4).start()
    for c in range(1, NC):
        w_copy(0, c).start()
    wo_copy.start()
    wr_copy.start()
    for i in range(4):
        stage_copy(i, 0).start()
    wg_copy.start()
    wu_copy.start()
    wd_copy.start()
    side = _Side(never0)
    side.add(PRO_LN1_PLAN, lambda k, a: ln_rows(1, k, LNC, never0, a, plain=True))
    side.add(PRO_X1_PLAN, late_x_blocks(1))
    fold(1, 3, side, 0)
    stash(3, proj_feat(side, 4, 3, xn_tile(0), None)[0])
    xn1 = xn_tile(1)
    spare = None
    for c in range(3):
        pk, spare = proj_feat(side, 10 + 4 * c, c, xn1, spare)
        if c < 2:
            k_features(pk, 1, c, False, never0)
        else:
            stash(0, pk + [spare])
    side.check()

    for c in range(NC):
        w_copy(2, c).wait()
    side = _Side(never0)
    side.add(PRO_V_PLANS[0], stashed_k(2, 0, 2, True))
    side.add(PRO_V_PLANS[1], stashed_k(3, 0, 3, False))
    side.add(PRO_V_PLANS[2], stashed_k(0, 1, 2, False))
    side.add(PRO_V_PLANS[3], w_blocks(1))
    spare = jnp.concatenate([stash_at(0, 31, n)[...] for n in range(2)], axis=1)
    k_features(proj_feat(side, 100, 3, xn_tile(1), spare)[0], 1, 3, True, never0)
    kv_update(*v_stage(side, xs_tile(0), 0, True, False, None, True))
    save_lead(0)
    save_lead(1)

    def phase1(u, carry):
        never = u < 0

        @pl.when(u == 0)
        def _():
            x_copy(3).wait()
            w_copy(0, 0).wait()

        @pl.when(u == 1)
        def _():
            x_copy(4).wait()
            w_copy(0, 1).wait()
            w_copy(0, 2).wait()

        xs = xs_tile(2 * u + 1)
        side = _Side(never)
        for i in range(2):
            t = 2 * u + 2 + i
            if i == 0:
                side.add(LN1_PLANS[0], lambda k, a: ln_rows(2 * u + 2, k, LNC, never, a))
            pending = v_stage(side, xs, 1 - i, False, False, t - 1 if i == 0 else None)
            xs = xs_tile(t)
            side = _Side(never)
            if i == 0:
                side.add(LN1_PLANS[1], lambda k, a: ln_rows(2 * u + 3, k, LNC, never, a))
            side.hooks[-28 + D_LAG] = [lambda p=pending: kv_update(*p)]
            feat_stage(side, -28, 1, xs, lambda p, pr: k_pair(p, i, pr, 0, False, never if i == 1 else None))
            save_lead(t)
        fold(0, u)
        return carry

    lax.fori_loop(0, (NT_ - 2) // 2, phase1, 0)

    w_copy(0, 3).wait()
    wo_copy.wait()
    wr_copy.wait()
    side = _Side(never0)

    def z_final(k, a):
        zb_v[k] = jnp.broadcast_to(_row_sum(_after(z_v[k], never0, a)), (128, 128))

    def wo_blocks(k, a):
        lo = tied(woraw_v[16 * k:16 * k + 16, :].astype(F32), never0, a)
        hi = tied(woraw_v[HK + 16 * k:HK + 16 * k + 16, :].astype(F32), never0, a)
        put_blocks(wos_v, 8 * k, _strassen_rhs(lo[:, :HK], lo[:, HK:], hi[:, :HK], hi[:, HK:]))

    side.add(END_PLANS[0], z_final)
    side.add(END_PLANS[1], w_blocks(0))
    side.add(END_PLANS[2], wo_blocks)
    fold(0, 3, side, 100)
    kv_update(*v_stage(side, xs_tile(NT_ - 1), 1, False, True, None))
    wr_v[...] = jnp.broadcast_to(wrraw_v[...].reshape(1, D).astype(F32), (8, D))

    def o_copy(r0, n, i):
        return pltpu.make_async_copy(o_v.at[pl.ds(r0, n), :], out_hbm.at[pl.ds(r0, n), :], sem.at[SO + i])

    def finish_rows(h_ref, k, t, valid, st, never=None, anchor=None):
        r0 = t * T + k * LNC
        best, besti = st["route"]
        wr = jnp.concatenate([wr_v[...]] * (LNC // 8), axis=0)
        sub = lax.broadcasted_iota(jnp.int32, (8, 1), 0)
        h = _after(h_ref[k * LNC:(k + 1) * LNC, :], never, anchor)
        hc = h - _row_sum(h) * (1.0 / D)
        rstd = lax.rsqrt(_row_sum(hc * hc) * (1.0 / D) + LN_EPS)
        r = (_row_sum(hc * wr) * rstd).astype(BF16).astype(F32)
        hn = hc * rstd
        view(hn_v, t, T // 2)[k * LNC // 2:(k + 1) * LNC // 2, :] = _pack(hn.astype(BF16))
        view(o_v, t, T)[k * LNC:(k + 1) * LNC, :] = (hn + h).astype(BF16)
        if valid is not None:
            r = jnp.where(valid, r, -jnp.inf)
        for i in range(LNC // 8):
            ri = r[8 * i:8 * i + 8, :]
            better = ri > best
            best = jnp.where(better, ri, best)
            besti = jnp.where(better, sub + (r0 + 8 * i), besti)
        st["route"] = (best, besti)
        return best

    def q_pair(p, slot, pr):
        ep, en, sp, sn = _dual_exp(p)
        zz = [_lane_tile(zb_v[pr, 8 * i:8 * i + 8, :], T // 128) for i in range(16)]
        ap = _pair_allreduce(_tree(jnp.add, [ep[i] * zz[i] for i in range(8)]), jnp.add)
        an = _pair_allreduce(_tree(jnp.add, [en[i] * zz[8 + i] for i in range(8)]), jnp.add)
        inv = _recip(ap * sn + (an + 1e-6 * sn) * sp)
        rp = sn * inv
        rn = sp * inv
        phi = jnp.concatenate([e * rp for e in ep] + [e * rn for e in en], axis=0)
        phi_v[slot][64 * pr:64 * pr + 64, :] = _pack(phi.astype(BF16))

    def attn_blocks(slot, g):
        lo, hi = [jnp.concatenate(
            [_dot(_unpack(kvbf_v[32 * pr:32 * pr + 32, :]), _unpack(phi_v[slot][64 * pr:64 * pr + 64, :]), NN)
             for pr in (2 * q, 2 * q + 1)], axis=0) for q in (g, g + 4)]
        blocks = _strassen_lhs(lo[:, :TH], hi[:, :TH], lo[:, TH:], hi[:, TH:])
        ot = _pack(jnp.concatenate(blocks, axis=1).astype(BF16).T)
        for i in range(7):
            oc_v[slot][:, i * HK + 128 * g:i * HK + 128 * g + 128] = ot[i * TH // 2:(i + 1) * TH // 2, :]

    def out_proj(side, step0, t, slot):
        xt = view(x_v, t, T)
        for n in range(4):
            def product(i):
                step = step0 + 7 * n + i
                w = side.gate(step, wos_v[:, i * HK + 128 * n:i * HK + 128 * n + 128])
                res = _dot(_unpack(oc_v[slot][:, i * HK:(i + 1) * HK]), _unpack(w), NN)
                side.done(step, res)
                return res
            for q, row in enumerate(_strassen(product)):
                for r, res in enumerate(row):
                    rows, cols = slice(q * TH, (q + 1) * TH), slice(r * HK + 128 * n, r * HK + 128 * n + 128)
                    h_v[slot][rows, cols] = res + xt[rows, cols].astype(F32)

    def phase2(u, carry):
        for i in range(4):
            stage_copy(i, u).wait()
        never = u < 0
        side = _Side(never)
        st = {"route": carry}
        tp = jnp.maximum(2 * u - 1, 0)
        side.add(LN2_PLANS[0], lambda k, a: finish_rows(h_v[1], k, tp, u > 0, st, never, a))
        side.add(LN2_PLANS[1], lambda k, a: finish_rows(h_v[0], k, 2 * u, None, st, never, a))

        def packer(i, dst, n):
            left = [n]

            def job(k, a):
                if i < 2:
                    pack_rows(stage_v[i], dst, (k // 2) * 16, 16, (0, D)[k % 2], (D, FM - D)[k % 2], never, a)
                else:
                    pack_rows(stage_v[i], dst, k * 16, 16, 0, D, never, a)
                left[0] -= 1
                if not left[0]:
                    stage_copy(i, jnp.minimum(u + 1, NQ - 1)).start()
                    n0 = stage_v[i].shape[0] - 16
                    side.deps.setdefault(PACK_DUE[i], []).append(stage_v[i][n0:n0 + 8, 0:128].astype(F32))
            return job

        for i in range(2):
            side.add(PACK_PLANS[i], packer(i, view((wgp_v, wup_v)[i], u, D // NQ // 2), len(PACK_PLANS[i])))
            d0 = pl.multiple_of(u * (DQ // 2) + i * (DQA // 2), 8)
            side.add(PACKD_PLANS[i], packer(2 + i, wdp_v.at[pl.ds(d0, 8 * len(PACKD_PLANS[i])), :],
                                            len(PACKD_PLANS[i])))
            for g in range(4):
                step = 107 + 28 * i + 7 * g + G_LAG
                side.hooks.setdefault(step if step < 156 else step - 156, []).append(
                    lambda i=i, g=g: attn_blocks(i, g))
        for i in range(2):
            feat_stage(side, 100 + 28 * i, 0, xs_tile(2 * u + i), lambda p, pr: q_pair(p, i, pr),
                       2 * u if i == 0 else None)
        for i in range(2):
            out_proj(side, 28 * i, 2 * u + i, i)
        side.check()

        @pl.when(u == 0)
        def _():
            o_copy(0, T, 0).start()

        @pl.when(u > 0)
        def _():
            o_copy(pl.multiple_of(tp * T, T), 2 * T, u).start()

        return st["route"]

    wg_copy.wait()
    wu_copy.wait()
    wd_copy.wait()
    route = lax.fori_loop(
        0, NT_ // 2, phase2,
        (jnp.full((8, 1), -jnp.inf, F32), jnp.zeros((8, 1), jnp.int32)))
    st = {"route": route}
    for k in range(T // LNC):
        finish_rows(h_v[1], k, NT_ - 1, None, st)
    best, besti = st["route"]
    o_copy(S - T, T, NT_).start()

    rmax = jnp.max(best, axis=0, keepdims=True)
    idx = jnp.min(jnp.where(best == rmax, besti, S), axis=0, keepdims=True)
    idx_s = jnp.clip(idx[0, 0], 0, S - 1)
    blk = pl.multiple_of((idx_s >> 4) << 4, 16)
    pair = jnp.broadcast_to(hn_v[pl.ds(idx_s >> 1, 1), :], (8, D))
    x8 = pltpu.bitcast(jnp.where((idx_s & 1) == 1, pair & jnp.uint32(0xFFFF0000), pair << 16), F32)
    xs = jnp.concatenate([x8, x8], axis=0).astype(BF16)
    acts, anchors = [], []

    def park(v, half):
        n = v.shape[0] // 128
        for i in range(n):
            z_v[i, :, 128 * half:128 * half + 128] = v[128 * i:128 * i + 128, :]
        return jnp.concatenate([z_v[i, :, 128 * half:128 * half + 128] for i in range(n)], axis=0)

    for c0 in range(0, FM, 128):
        g = _dot(xs, _unpack(wgp_v[:, c0:c0 + 128]), NN)[0:8, :]
        u = _dot(xs, _unpack(wup_v[:, c0:c0 + 128]), NN)[0:8, :]
        anchors += [g, u]
        acts.append(g * jax.nn.sigmoid(g) * u)
    xb = park(_col_broadcast(x8), 0)
    g, u = [_sublane_allreduce(_vpu_matvec(
        xb, lambda g: w[8 * g:8 * g + 8, :].astype(F32), never0,
        anchors[i * MOE_NA // 2:(i + 1) * MOE_NA // 2], MOE_LAGS[0])) for i, w in enumerate((wg_v, wu_v))]
    acts.append(g * jax.nn.sigmoid(g) * u)
    a = jnp.concatenate(acts, axis=1)
    am = jnp.concatenate([a[:, FVD:], a[:, FVD:]], axis=0).astype(BF16)
    ys, anchors = [], anchors[MOE_NA:]
    for k0 in range(0, FF - FVD, 512):
        k1 = min(k0 + 512, FF - FVD)
        yk = _dot(am[:, k0:k1], _unpack(wdp_v[k0 // 2:k1 // 2, 0:D]), NN)[0:8, :]
        ys.append(yk)
        anchors += [yk[:, c:c + 128] for c in range(128, D, 256)]
    ys.append(_sublane_allreduce(_vpu_matvec(
        park(_col_broadcast(a[:, :FVD]), 1), lambda g: wd_v[8 * g:8 * g + 8, :].astype(F32), never0,
        anchors[:-MOE_ND], MOE_LAGS[1])))
    y = _tree(jnp.add, ys) * jax.nn.sigmoid(rmax)
    y = jnp.concatenate([y, y], axis=0)
    sel = lax.broadcasted_iota(jnp.int32, (16, 1), 0) == (idx_s - blk)
    patch_v[...] = (o_v[pl.ds(blk, 16), :].astype(F32) + jnp.where(sel, y, 0.0)).astype(BF16)
    o_copy(0, T, 0).wait()
    for u in range(1, NT_ // 2):
        o_copy((2 * u - 1) * T, 2 * T, u).wait()
    o_copy(S - T, T, NT_).wait()
    pc = pltpu.make_async_copy(patch_v, out_hbm.at[pl.ds(blk, 16), :], sem.at[SM + 3])
    pc.start()
    for i in range(4):
        stage_copy(i, NQ - 1).wait()
    pc.wait()


@jax.jit
def pallas_sequential_preLN__linear_kernel_hedgehog__moe_arch_mod__prompt_kernel(
    A_x: jax.Array,
    A_wqkv: jax.Array,
    A_w_phi: jax.Array,
    A_wo: jax.Array,
    B_x: jax.Array,
    B_w_r: jax.Array,
    B_w_gate: jax.Array,
    B_w_up: jax.Array,
    B_w_down: jax.Array,
):
    del B_x
    hbm = pl.BlockSpec(memory_space=pl.ANY)
    out = pl.pallas_call(
        _kernel,
        out_shape=jax.ShapeDtypeStruct((S, D), BF16),
        in_specs=[hbm] * 8,
        out_specs=hbm,
        scratch_shapes=[
            pltpu.VMEM((S, D), BF16),
            pltpu.VMEM((T, D), U32),
            pltpu.VMEM((T, D), F32),
            pltpu.VMEM((NT_ * TH // 2, SW), U32),
            pltpu.VMEM((NT_ * HK // 2, 128), U32),
            pltpu.VMEM((3 * NC, D, RC), BF16),
            pltpu.VMEM((D // 2, D), U32),
            pltpu.VMEM((992, D), F32),
            [pltpu.VMEM((HK // 2, 7 * HK), U32)] * 3,
            pltpu.VMEM((H, DH, DH), BF16),
            pltpu.VMEM((8 * 64, 128), U32),
            pltpu.VMEM((D, D), BF16),
            pltpu.VMEM((HK // 2, 7 * HK), U32),
            pltpu.VMEM((D,), BF16),
            pltpu.VMEM((8, D), F32),
            pltpu.VMEM((NPAIR, 64, 128), F32),
            pltpu.VMEM((NPAIR * 32, 128), U32),
            pltpu.VMEM((NPAIR, 128, T), F32),
            pltpu.VMEM((NPAIR, 128, 128), F32),
            [pltpu.VMEM((NPAIR * 64, T), U32)] * 2,
            [pltpu.VMEM((TH // 2, 7 * HK), U32)] * 2,
            [pltpu.VMEM((T, D), F32)] * 2,
            pltpu.VMEM((S // 2, D), U32),
            pltpu.VMEM((S, D), BF16),
            pltpu.VMEM((D, FV), BF16),
            pltpu.VMEM((D, FV), BF16),
            pltpu.VMEM((FVD, D), BF16),
            [pltpu.VMEM((D // NQ + 16, FM), BF16), pltpu.VMEM((D // NQ + 16, FM), BF16),
             pltpu.VMEM((DQA + 16, D), BF16), pltpu.VMEM((DQ - DQA + 16, D), BF16)],
            pltpu.VMEM((D // 2, FM), U32),
            pltpu.VMEM((D // 2, FM), U32),
            pltpu.VMEM(((FF - FVD) // 2, D + 128), U32),
            pltpu.VMEM((16, D), BF16),
            pltpu.SemaphoreType.DMA((6 + 3 * NC + NT_ + 15,)),
        ],
        compiler_params=pltpu.CompilerParams(vmem_limit_bytes=100 * 1024 * 1024,
                                             disable_semaphore_checks=True, disable_bounds_checks=True),
        name="hedgehog_mod",
    )(
        A_x.reshape(S, D),
        A_wqkv,
        A_w_phi,
        A_wo,
        B_w_r,
        B_w_gate,
        B_w_up,
        B_w_down,
    )
    return out.reshape(1, S, D)
```

```python
import math

import jax
import jax.numpy as jnp
from jax import lax
import jax.experimental.pallas as pl
import jax.experimental.pallas.tpu as pltpu

F32 = jnp.float32
BF16 = jnp.bfloat16
U32 = jnp.uint32

S = 2048
D = 1024
H = 32
DH = 32
FF = 3584
NPAIR = H // 2
LOG2E = 1.4426950408889634
LN_EPS = 1e-5

T = 256
TH = T // 2
NT_ = S // T
RC = 256
NC = D // RC
PPC = RC // 64
LNC = 16

FV = 10 * 128
FM = FF - FV
FVD = 8 * 128
NQ = NT_ // 2
DQ = (FF - FVD) // NQ
WO_ROWS = 176
HK = D // 2
SW = 8 * HK


def _spread(n, a, b, due=None):
    rel = [round(a + (b - a) * k / (n - 1), 3) for k in range(n)]
    return tuple((r, None if due is None else math.ceil(r) + due) for r in rel)


LN1_PLANS = (_spread(16, 0, 22, 5), _spread(16, -1, 22, 5))
PRO_LN1_PLAN = ((None, None),) * 16
PRO_K_PLANS0 = _spread(8, 0, 6)
PRO_K_PLANS1 = _spread(8, 0, 6)
PRO_X0_PLAN = _spread(8, 0.5, 6.5)
PRO_W0_PLAN = _spread(10, 0.5, 6.5)
PRO_W_PLAN = _spread(5, 0, 4) + _spread(16, 8.3, 18.5)
PRO_K_PLANS2 = _spread(8, 15.2, 18.2)
PRO_V_PLANS = (((None, None),) * 8 + _spread(24, -3.5, 3), _spread(8, 9, 19), _spread(8, 19.5, 25.5),
               _spread(8, 17, 26), _spread(8, 19, 26.5) + _spread(24, -1, 18))
END_PLANS = (_spread(16, 0, 26), _spread(31, 101, 103)[:3] + _spread(28, 0.3, 26.3))
WO_PLAN = _spread(11, 0.5, 25)
LN2_PLANS = (_spread(16, 0, 22, 5), _spread(16, 28.5, 50, 5))
PACK_PLANS = (_spread(32, 100.5, 126), _spread(32, 128.5, 154))
PACKD_PLANS = (_spread(28, 0.5, 26), _spread(12, 28.5, 38))
PACK_DUE = (130, 3, 30, 42)
DQA = 16 * len(PACKD_PLANS[0])
G_LAG = 5
D_LAG = 1
BLOCK_STAGGER = 4
BLOCK_DELAY = 4
PLAIN_V0 = 1
MOE_NA = 36
MOE_ND = 2
MOE_LAGS = (3, 3)
STAGGER = 8

NN = (((1,), (0,)), ((), ()))
NT = (((1,), (1,)), ((), ()))


def _dot(a, b, dims):
    return lax.dot_general(a, b, dims, preferred_element_type=F32)


def _recip(x):
    return pl.reciprocal(x, approx=False, full_range=False)


def _pack(x):
    return pltpu.bitcast(x, U32)


def _unpack(x):
    return pltpu.bitcast(x, BF16)


def _strassen_lhs(a11, a12, a21, a22):
    return [a21 + a22, a22, a11 + a12, a11, a11 + a22, a12 - a22, a21 - a11]


def _strassen_rhs(b11, b12, b21, b22):
    return [b11, b21 - b11, b22, b12 - b22, b11 + b22, b21 + b22, b11 + b12]


def _strassen(product):
    m2 = product(0)
    m4 = product(1)
    c21 = m2 + m4
    m5 = product(2)
    u11 = m4 - m5
    m3 = product(3)
    c12 = m3 + m5
    u22 = m3 - m2
    m1 = product(4)
    u11 = u11 + m1
    u22 = u22 + m1
    c11 = product(5) + u11
    c22 = product(6) + u22
    return [[c11, c12], [c21, c22]]


def _pair_allreduce(a, op):
    a = op(a, pltpu.roll(a, 2, 0))
    return op(a, pltpu.roll(a, 4, 0))


def _tree(op, xs):
    xs = list(xs)
    while len(xs) > 1:
        nxt = [op(xs[i], xs[i + 1]) for i in range(0, len(xs) - 1, 2)]
        if len(xs) % 2:
            nxt.append(xs[-1])
        xs = nxt
    return xs[0]


def _pair_logits(sl, j):
    sub = lax.broadcasted_iota(jnp.int32, sl[0].shape, 0)
    if j < 3:
        head = jnp.where(sub < 2, 0.0, sl[(0, 1, 16)[j]])
    else:
        head = jnp.where(sub < 2, sl[0], jnp.where(sub < 4, pltpu.roll(sl[1], 2, 0),
                                                   jnp.where(sub < 6, pltpu.roll(sl[16], 4, 0), 0.0)))
    r0 = (2, 9, 17, 24)[j]
    return [head] + list(sl[r0:r0 + 7])


def _dual_exp(sl):
    mx = _pair_allreduce(_tree(jnp.maximum, sl), jnp.maximum)
    mn = _pair_allreduce(_tree(jnp.minimum, sl), jnp.minimum)
    ep = [jnp.exp2(s - mx) for s in sl]
    en = [jnp.exp2(mn - s) for s in sl]
    sp = _pair_allreduce(_tree(jnp.add, ep), jnp.add)
    sn = _pair_allreduce(_tree(jnp.add, en), jnp.add)
    return ep, en, sp, sn


def _after(x, never, anchor):
    if anchor is None:
        return x
    d = jnp.concatenate([anchor] * (x.shape[0] // 8), axis=0)
    if x.shape[1] == 128:
        return jnp.where(never, d, x)
    return jnp.concatenate([jnp.where(never, d, x[:, :128]), x[:, 128:]], axis=1)


def _gate(x, never, deps):
    for i, dep in enumerate(deps):
        d = jnp.broadcast_to(dep, (8, 128))
        if x.dtype != F32:
            d = pltpu.bitcast(d, x.dtype)
        blk = jnp.where(never, d, x[8 * i:8 * i + 8, :128])
        if x.shape[1] > 128:
            blk = jnp.concatenate([blk, x[8 * i:8 * i + 8, 128:]], axis=1)
        parts = ([x[:8 * i, :]] if i else []) + [blk, x[8 * i + 8:, :]]
        x = jnp.concatenate(parts, axis=0)
    return x


def _lane_fold(a):
    return _tree(jnp.add, [a[:, 128 * i:128 * i + 128] for i in range(a.shape[1] // 128)])


def _row_sum(a):
    return jnp.sum(_lane_fold(a), axis=-1, keepdims=True)


def _lane_tile(a, n):
    return a if n == 1 else jnp.concatenate([a] * n, axis=1)


def _sublane_allreduce(a):
    a = a + pltpu.roll(a, 4, 0)
    a = a + pltpu.roll(a, 2, 0)
    return a + pltpu.roll(a, 1, 0)


def _col_broadcast(row8):
    return jnp.concatenate([row8] * 16, axis=0).astype(BF16).T.astype(F32)


def _vpu_matvec(xb, w_rows, never, anchors, lag):
    ng = xb.shape[0] // 8
    acc, hist = None, []
    for g in range(ng):
        dep = anchors[(g * len(anchors)) // ng]
        if g >= lag:
            dep = dep + hist[g - lag]
        x = jnp.where(never, dep, xb[8 * g:8 * g + 8, :])
        w = w_rows(g)
        t = w * _lane_tile(x, w.shape[1] // 128)
        acc = t if acc is None else acc + t
        c = 128 * (g % (w.shape[1] // 128))
        hist.append(acc[:, c:c + 128])
    return acc


class _Side:
    def __init__(self, never):
        self.never = never
        self.jobs = []
        self.deps = {}
        self.hooks = {}

    def add(self, plan, fn):
        for k, (rel, due) in enumerate(plan):
            if rel is None:
                self._run(due, fn, k, None)
            else:
                self.jobs.append((rel, due, fn, k))

    def _run(self, due, fn, k, anchor):
        dep = fn(k, anchor)
        if due is not None:
            self.deps.setdefault(due, []).append(dep)

    def check(self):
        assert not self.jobs and not self.deps and not self.hooks

    def gate(self, step, x):
        return _gate(x, self.never, self.deps.pop(step, []))

    def done(self, step, res):
        m = res.shape[0] // 8
        for job in sorted([j for j in self.jobs if step - 1 < j[0] <= step], key=lambda j: j[0]):
            self.jobs.remove(job)
            g = m - 1 - int((step - job[0]) * m)
            self._run(job[1], job[2], job[3], res[8 * g:8 * g + 8, res.shape[1] - 128:])
        for fn in self.hooks.pop(step, []):
            fn()


def _kernel(x_hbm, wqkv_hbm, wphi_hbm, wo_hbm, wr_hbm, wg_hbm, wu_hbm, wd_hbm, out_hbm,
            x_v, xn_v, xs_v, lead_v, wraw_v, wt_v, ws_v, wphi_v, a_v, woraw_v, wos_v, wrraw_v, wr_v,
            kvacc_v, kvbf_v, z_v, zb_v, phi_v, oc_v, h_v, hn_v, o_v, wg_v, wu_v, wd_v, stage_v,
            wgp_v, wup_v, wdp_v, patch_v,
            sem):
    SX, SQ, SO, SM = 0, 6, 6 + 3 * NC, 6 + 3 * NC + NT_ + 1

    def x_copy(i):
        h0, h1 = ((0, 1), (1, 2), (2, 4), (4, 8), (8, 2 * NT_))[i]
        rows = pl.ds(h0 * TH, (h1 - h0) * TH)
        return pltpu.make_async_copy(x_hbm.at[rows, :], x_v.at[rows, :], sem.at[SX + i])

    def k0_copy(s):
        return pltpu.make_async_copy(wqkv_hbm.at[:, pl.ds(D + s * 128, 128)],
                                     wraw_v.at[NC, :, pl.ds(s * 128, 128)], sem.at[(SM + 7, SQ + NC)[s]])

    def w_copy(j, c):
        return pltpu.make_async_copy(wqkv_hbm.at[:, pl.ds(j * D + c * RC, RC)], wraw_v.at[j * NC + c],
                                     sem.at[SQ + j * NC + c])

    def wphi_copy(i):
        h0, h1 = ((0, 8), (16, 24), (8, 16), (24, H))[i]
        return pltpu.make_async_copy(wphi_hbm.at[pl.ds(h0, h1 - h0)], wphi_v.at[pl.ds(h0, h1 - h0)],
                                     sem.at[(SM + 4, SM + 8, SM + 9, SM + 14)[i]])

    wr_copy = pltpu.make_async_copy(wr_hbm, wrraw_v, sem.at[SM + 5])

    def wo_copy(i):
        rows = pl.ds(0, WO_ROWS) if i == 0 else pl.ds(WO_ROWS, HK - WO_ROWS)
        return pltpu.make_async_copy(wo_hbm.at[:, rows, :], woraw_v.at[:, rows, :], sem.at[(SM + 6, SX + 5)[i]])

    wg_copy = pltpu.make_async_copy(wg_hbm.at[:, pl.ds(FM, FV)], wg_v, sem.at[SM + 0])
    wu_copy = pltpu.make_async_copy(wu_hbm.at[:, pl.ds(FM, FV)], wu_v, sem.at[SM + 1])
    wd_copy = pltpu.make_async_copy(wd_hbm.at[pl.ds(0, FVD), :], wd_v, sem.at[SM + 2])

    def stage_copy(i, q):
        if i < 2:
            r0 = q * (D // NQ)
            r0 = r0 if isinstance(r0, int) else pl.multiple_of(r0, D // NQ)
            src = (wg_hbm, wu_hbm)[i].at[pl.ds(r0, D // NQ), pl.ds(0, FM)]
        else:
            r0 = FVD + q * DQ + (i - 2) * DQA
            r0 = r0 if isinstance(r0, int) else pl.multiple_of(r0, 16)
            src = wd_hbm.at[pl.ds(r0, (DQA, DQ - DQA)[i - 2]), :]
        return pltpu.make_async_copy(src, stage_v[i].at[pl.ds(0, src.shape[0]), :], sem.at[SM + 10 + i])

    wphi_copy(0).start()
    k0_copy(0).start()
    x_copy(0).start()
    k0_copy(1).start()
    x_copy(1).start()
    wphi_copy(1).start()
    w_copy(1, 2).start()

    made = set()

    def view(ref, i, n, off=0):
        r0 = off + i * n
        return ref.at[pl.ds(r0 if isinstance(r0, int) else pl.multiple_of(r0, math.gcd(n, off)), n), :]

    def put_blocks(dst, r0, fn, m11, m12, m21, m22, never, a, skip=()):
        w = HK // BLOCK_STAGGER
        for c0 in range(0, HK, w):
            d11, d22 = m11[:, c0:c0 + w], m22[:, c0:c0 + w]
            if a is not None:
                d = jnp.concatenate([_lane_tile(a, w // 128)] * 2, axis=0)
                d11, d22 = jnp.where(never, d, d11), jnp.where(never, d, d22)
            blocks = fn(d11, m12[:, c0:c0 + w], m21[:, c0:c0 + w], d22)
            for i, b in enumerate(blocks):
                if i not in skip:
                    dst[r0:r0 + 8, i * HK + c0:i * HK + c0 + w] = _pack(b.astype(BF16))
            a = blocks[6][8:16, w - 128:]
            for _ in range(BLOCK_DELAY):
                a = a * a

    def rows16(ref, r0):
        return _unpack(ref[r0:r0 + 8, :]).astype(F32)

    def x_blocks(t, k, lo, hi, never, a):
        put_blocks(view(xs_v, t, TH // 2), k * LNC // 2, _strassen_rhs,
                   lo[:, :HK], hi[:, :HK], lo[:, HK:], hi[:, HK:], never, a)

    def ln_rows(t, k, n, never=None, anchor=None, plain=False):
        x = _after(view(x_v, t, T)[k * n:(k + 1) * n, :].astype(F32), never, anchor)
        xc = x - _row_sum(x) * (1.0 / D)
        rstd = lax.rsqrt(_row_sum(xc * xc) * (1.0 / D) + LN_EPS)
        xn = xc * rstd
        if plain:
            xn_v[(t * T + k * n) // 2:(t * T + (k + 1) * n) // 2, :] = _pack(xn.astype(BF16))
        elif k * n < TH:
            xn_v[k * n // 2:(k + 1) * n // 2, :] = _pack(xn.astype(BF16))
        else:
            x_blocks(t, k - TH // LNC, rows16(xn_v, (k * n - TH) // 2), xn, never, xn[0:8, 0:128])
        return _tree(jnp.add, [rstd[8 * i:8 * i + 8, :] for i in range(min(n, LNC) // 8)])

    def late_x_blocks(t):
        return lambda k, a: x_blocks(t, k, rows16(xn_v, t * T // 2 + 8 * k),
                                     rows16(xn_v, (t * T + TH) // 2 + 8 * k), never0, a)

    def xn_tile(t):
        return _unpack(xn_v[t * T // 2:(t + 1) * T // 2, :])

    def xs_tile(t):
        return _unpack(view(xs_v, t, TH // 2)[:, 0:7 * HK])

    def expand_wphi(c):
        w = wphi_v[8 * c:8 * c + 8].reshape(8 * DH, DH).astype(F32).T
        bits = pltpu.bitcast(w, U32)
        head = lax.broadcasted_iota(jnp.int32, (DH, 128), 1) >> 5
        for s in range(2):
            b = bits[:, 128 * s:128 * s + 128]
            for j in range(2):
                r0 = 64 * (2 * c + s) + 32 * j
                a_v[r0:r0 + 32, :] = jnp.where(head == 2 * j, b >> 16,
                                               jnp.where(head == 2 * j + 1, b, jnp.uint32(0)))

    wphi_copy(0).wait()
    expand_wphi(0)
    h_v[1][...] = jnp.zeros((T, D), F32)
    for ref in stage_v:
        ref[ref.shape[0] - 16:, 0:128] = jnp.zeros((16, 128), BF16)

    def v_transpose(k, a):
        q, r0 = (k // 8) + 4 * (k % 2), 256 * (k % 8 // 2)
        w = wraw_v[2 * NC + q // 2, r0:r0 + 256, (q % 2) * 128:(q % 2) * 128 + 128]
        if a is not None:
            w = _unpack(jnp.where(never0, jnp.concatenate([pltpu.bitcast(a, U32)] * 16, axis=0), _pack(w)))
        wt_v[2][64 * q:64 * q + 64, r0:r0 + 256] = _pack(w.T)
        made.add(("vt", k))

    def fold_pairs(j, c, s, side=None, step0=None):
        g0 = 64 * (2 * c + s)
        g0 = g0 if isinstance(g0, int) else pl.multiple_of(g0, 64)
        res = _dot(_unpack(a_v[pl.ds(g0, 64), :]), wraw_v[j * NC + c, :, s * 128:(s + 1) * 128], NT)
        if side is not None:
            side.done(step0 + 2 * s, res[:, :D // 2])
            side.done(step0 + 2 * s + 1, res[:, D // 2:])
        sub = lax.broadcasted_iota(jnp.int32, (8, D), 0)
        out = []
        for q in range(2):
            base = _pair_allreduce(jnp.where(sub < 2, res[64 * q:64 * q + 8, :], 0.0), jnp.add)
            out.append([(res[64 * q + 8 * i:64 * q + 8 * i + 8, :] - base) * LOG2E for i in range(8)])
        return out

    def share(z, z3, k):
        sub = lax.broadcasted_iota(jnp.int32, (8, D), 0)
        return jnp.where(sub < 2, pltpu.roll(z3, 8 - 2 * k, 0), z)

    def packed(slabs):
        return _pack(jnp.concatenate(slabs, axis=0).astype(BF16))

    def fold(j, c, side=None, step0=None):
        p0, p1 = fold_pairs(j, c, 0, side, step0)
        p2, p3 = fold_pairs(j, c, 1, side, step0)
        sl = ([share(p0[0], p3[0], 1), share(p1[0], p3[0], 2)] + p0[1:] + p1[1:]
              + [share(p2[0], p3[0], 3)] + p2[1:] + p3[1:])
        zero = jnp.zeros((8, D), F32)
        even, odd = sl + [zero], [zero] + sl
        r0 = 8 * ((31 * c) // 2)
        is_odd = c % 2 == 1
        if isinstance(c, int):
            sl = odd if is_odd else even
        else:
            r0 = pl.multiple_of(r0, 8)
            sl = [jnp.where(is_odd, o, e) for o, e in zip(odd, even)]
        win = wt_v[j].at[pl.ds(r0, 128), :]
        win[8:128, :] = packed(sl[2:])
        first = packed(sl[:2])
        if is_odd is not False:
            keep = lax.broadcasted_iota(jnp.int32, (8, D), 0) < jnp.where(is_odd, 4, 0)
            first = jnp.where(keep, win[0:8, :], first)
        win[0:8, :] = first
        made.update(("fold", j, q) for q in ([c] if isinstance(c, int) else range(3)))

    def w_blocks(j, k0=0):
        def job(k, a):
            k += k0
            assert made >= ({("vt", 8 * (k // 8) + q) for q in range(8)} if j == 2 else
                            {("fold", j, q) for q in ((0, 2) if k < 15 else range(4))})
            made.add(("ws", j, k))
            lo, hi = rows16(wt_v[j], 8 * k), rows16(wt_v[j], (256 if j == 2 else 248) + 8 * k)
            put_blocks(ws_v[j], 8 * k, _strassen_lhs, lo[:, :HK], lo[:, HK:], hi[:, :HK], hi[:, HK:], never0, a,
                       skip=(1, 3))
        return job

    def k_pair(p, slot, pr, c0, first, never=None):
        for n in range(c0, c0 + p[0].shape[1], 128):
            assert first == (("z", pr, n) not in made)
            made.update({("z", pr, n), ("phi", slot, pr, n)})
        ep, en, sp, sn = _dual_exp(p)
        inv = _recip(sp * sn)
        scale = (sn * inv, sp * inv)
        es = ep + en
        cols = slice(c0, c0 + p[0].shape[1])
        n = 16 if never is None else 16 // STAGGER
        last = None
        for q in range(16 // n):
            sc = scale
            if last is not None:
                sc = [jnp.where(never, last, x) for x in scale]
            phi = jnp.concatenate([es[i] * sc[i // 8] for i in range(q * n, (q + 1) * n)], axis=0)
            rows = slice(8 * q * n, 8 * (q + 1) * n)
            z = phi if first else z_v[pr, rows, cols] + phi
            z_v[pr, rows, cols] = z
            phi_v[slot][64 * pr + 4 * q * n:64 * pr + 4 * (q + 1) * n, cols] = _pack(phi.astype(BF16))
            last = z[8 * n - 8:, :]

    def k_features(pk, slot, c, first, never=None):
        for j in range(PPC):
            k_pair(_pair_logits(pk, j), slot, c * PPC + j, 0, first, never)

    def kv_update(vts, slot, g, first, publish=False):
        for q, vt in enumerate(vts):
            for j in range(2):
                pr = 2 * g + 8 * q + j
                assert made >= {("phi", slot, pr, 0), ("phi", slot, pr, 128)}
                upd = _dot(vt[64 * j:64 * j + 64, :].astype(BF16), _unpack(phi_v[slot][64 * pr:64 * pr + 64, :]), NT)
                acc = upd if first else kvacc_v[pr] + upd
                kvacc_v[pr] = acc
                if publish:
                    odd = -(lax.broadcasted_iota(jnp.int32, (32, 128), 1) & 1)
                    bits = pltpu.bitcast(acc, jnp.int32) & jnp.concatenate([~odd, odd], axis=0)
                    kvbf_v[32 * pr:32 * pr + 32, :] = _pack(pltpu.bitcast(bits, F32).astype(BF16))

    def save_lead(t):
        view(lead_v, t, HK // 2)[...] = _pack(_unpack(view(xs_v, t, TH // 2)[:, 0:HK]).T)

    def proj_feat(side, step0, c, xn, carry):
        r0 = 8 * ((31 * c) // 2)
        skip = 8 if c % 2 == 1 and carry is not None else 0
        w = wt_v[1][r0 + skip:r0 + 128, :]
        quarters = []
        for n in range(2):
            for m in range(2):
                step = step0 + 2 * n + m
                wq = _unpack(side.gate(step, w[:64, :] if m == 0 else w[64:, :]))
                res = _dot(wq, xn[n * TH:(n + 1) * TH, :], NT)
                side.done(step, res)
                quarters.append(res)
        res = jnp.concatenate(
            [jnp.concatenate([quarters[0], quarters[2]], axis=1),
             jnp.concatenate([quarters[1], quarters[3]], axis=1)], axis=0)
        sl = [res[8 * i:8 * i + 8, :] for i in range(res.shape[0] // 8)]
        if c % 2 == 0:
            return sl[:31], sl[31]
        return ([carry] + sl if skip else sl[1:]), None

    def proj_unit(side, step0, j, b, xs, lead=None, plain=None):
        r1 = 64 * b + (64 if j == 2 or b < 3 else 56)
        assert made >= ({("vt", 8 * b + q) for q in range(8)} if plain is not None else
                        {("ws", j, k) for k in range(8 * b, r1 // 8)})
        if plain is not None:
            out = []
            for q in range(2):
                row = []
                for n in range(2):
                    res = _dot(_unpack(wt_v[2][256 * q + 64 * b:256 * q + r1, :]), plain[n * TH:(n + 1) * TH, :], NT)
                    for i in range((0, 2, 4, 5)[2 * q + n], (2, 4, 5, 7)[2 * q + n]):
                        side.done(step0 + i, res)
                    row.append(res)
                out.append(jnp.concatenate(row, axis=1))
            return out

        def product(i):
            off = 256 if j == 2 else 248
            w = (wt_v[j][off + 64 * b:off + r1, HK:] if i == 1 else wt_v[j][64 * b:r1, :HK] if i == 3
                 else ws_v[j][64 * b:r1, i * HK:(i + 1) * HK])
            w = _unpack(side.gate(step0 + i, w))
            if lead is not None and i == 0:
                res = _dot(w, _unpack(view(lead_v, lead, HK // 2)[...]), NN)
            else:
                res = _dot(w, xs[:, i * HK:(i + 1) * HK], NT)
            side.done(step0 + i, res)
            return res
        return [jnp.concatenate(row, axis=1) for row in _strassen(product)]

    def feat_stage(side, step0, j, xs, pair_fn, lead=None):
        sl = [[], []]
        for b in range(4):
            for q, res in enumerate(proj_unit(side, step0 + 7 * b, j, b, xs, lead if b == 0 else None)):
                sl[q] += [res[8 * i:8 * i + 8, :] for i in range(res.shape[0] // 8)]
            for q in (1, 0):
                for jj in (2 * (b % 2), 2 * (b % 2) + 1):
                    pair_fn(_pair_logits(sl[q][31 * (b // 2):], jj), 8 * q + 4 * (b // 2) + jj)

    def v_stage(side, xs, slot, first, publish, lead, plain=None):
        pending = None
        for g in range(4):
            if pending is not None:
                side.hooks.setdefault(7 * g + D_LAG, []).append(lambda p=pending: kv_update(*p))
            pending = (proj_unit(side, 7 * g, 2, g, xs, lead if g == 0 else None, plain if g < PLAIN_V0 else None),
                       slot, g, first, publish)
        side.check()
        return pending

    def pack_rows(src, dst, r0, rows, c0, cols, never, a):
        w = src[r0:r0 + rows, c0:c0 + cols].astype(F32)
        d = _lane_tile(a, cols // 128)
        w = jnp.concatenate([jnp.where(never, d, w[8 * i:8 * i + 8, :]) if i % 2 == 0 else w[8 * i:8 * i + 8, :]
                             for i in range(rows // 8)], axis=0)
        dst[r0 // 2:(r0 + rows) // 2, c0:c0 + cols] = _pack(w.astype(BF16))

    def stash_at(i, k, n):
        return zb_v.at[4 * i + 2 * (k // 16) + n, pl.ds(8 * (k % 16), 8), :]

    def stash(i, sl):
        for k, v in enumerate(sl):
            for n in range(2):
                stash_at(i, k, n)[...] = v[:, 128 * n:128 * n + 128]

    def stashed_k(i, slot, c, first):
        def job(k, a):
            j, n = k // 2, k % 2
            p = _pair_logits([stash_at(i, q, n)[...] for q in range(31)], j)
            k_pair([_after(p[0], never0, a)] + p[1:], slot, c * PPC + j, 128 * n, first, never0)
        return job

    def first_rows(k0, k1, n):
        xn = _unpack(xn_v[n * TH // 2:(n + 1) * TH // 2, :])
        ks = [k for k in range(k0, k1)]
        w = jnp.concatenate([wt_v[1][4 * (k % 32):4 * (k % 32) + 8, :] for k in ks[::2]], axis=0)
        res = _dot(_unpack(w), xn, NT)
        for q, k in enumerate(ks):
            if k % 32 < 31:
                stash_at(0, k % 32, n)[...] = res[8 * q:8 * q + 8, :]

    k0_copy(0).wait()
    x_copy(0).wait()
    wphi_copy(2).start()
    w_copy(1, 1).start()
    wphi_copy(3).start()
    x_copy(2).start()
    p0, p1 = fold_pairs(1, 0, 0)
    wt_v[1][8:64, :] = packed(p0[1:] + p1[1:])
    h_v[0][0:8, :] = p0[0]
    h_v[0][8:16, :] = p1[0]
    never0 = ln_rows(0, 0, TH, plain=True)[0, 0] < 0.0
    first_rows(2, 16, 0)

    k0_copy(1).wait()
    x_copy(1).wait()
    wphi_copy(1).wait()
    w_copy(1, 3).start()
    for c in (0, 2, 1, 3):
        w_copy(2, c).start()
    p2, p3 = fold_pairs(1, 0, 1)
    wt_v[1][0:8, :] = packed([share(h_v[0][0:8, :], p3[0], 1), share(h_v[0][8:16, :], p3[0], 2)])
    wt_v[1][64:128, :] = packed([share(p2[0], p3[0], 3)] + p2[1:] + p3[1:] + [jnp.zeros((8, D), F32)])
    made.add(("fold", 1, 0))
    ln_rows(0, 1, TH, plain=True)
    first_rows(16, 34, 0)
    first_rows(0, 16, 1)
    first_rows(16, 32, 1)
    expand_wphi(2)

    for c, prev in ((2, 0), (1, 2)):
        w_copy(1, c).wait()
        wphi_copy(4 - c).wait()
        expand_wphi(5 - 2 * c)
        side = _Side(never0)
        if c == 2:
            side.add(PRO_X0_PLAN, late_x_blocks(0))
        else:
            side.add(PRO_W0_PLAN, w_blocks(1))
        side.add((PRO_K_PLANS0, PRO_K_PLANS1)[2 - c], stashed_k(prev, 0, prev, True))
        fold(1, c, side, 0)
        stash(c, proj_feat(side, 4, c, xn_tile(0), None)[0])
        side.check()

    x_copy(2).wait()
    w_copy(1, 3).wait()
    x_copy(3).start()
    w_copy(0, 0).start()
    wo_copy(0).start()
    x_copy(4).start()
    for c in range(1, NC):
        w_copy(0, c).start()
    wo_copy(1).start()
    wr_copy.start()
    for i in range(4):
        stage_copy(i, 0).start()
    wg_copy.start()
    wu_copy.start()
    wd_copy.start()
    side = _Side(never0)
    side.add(PRO_LN1_PLAN, lambda k, a: ln_rows(1, k, LNC, never0, a, plain=True))
    side.add(PRO_W_PLAN, w_blocks(1, len(PRO_W0_PLAN)))
    side.add(PRO_K_PLANS2, stashed_k(1, 0, 1, False))
    fold(1, 3, side, 0)
    stash(3, proj_feat(side, 4, 3, xn_tile(0), None)[0])
    xn1 = xn_tile(1)
    spare = None
    for c in range(3):
        pk, spare = proj_feat(side, 8 + 4 * c, c, xn1, spare)
        if c < 2:
            k_features(pk, 1, c, c == 1, never0)
        else:
            stash(0, pk + [spare])
    side.check()

    for c in range(NC):
        w_copy(2, c).wait()
    side = _Side(never0)
    side.add(PRO_V_PLANS[0], v_transpose)
    side.add(PRO_V_PLANS[1], stashed_k(3, 0, 3, False))
    side.add(PRO_V_PLANS[2], stashed_k(0, 1, 2, False))
    side.add(PRO_V_PLANS[3], late_x_blocks(1))
    side.add(PRO_V_PLANS[4], w_blocks(2))
    spare = jnp.concatenate([stash_at(0, 31, n)[...] for n in range(2)], axis=1)
    k_features(proj_feat(side, -4, 3, xn_tile(1), spare)[0], 1, 3, True, never0)
    kv_update(*v_stage(side, xs_tile(0), 0, True, False, None, xn_tile(0)))
    save_lead(0)
    save_lead(1)
    for r0 in (0, 248):
        wt_v[0][r0:r0 + 8, :] = jnp.zeros((8, D), U32)

    def phase1(u, carry):
        never = u < 0

        @pl.when(u == 0)
        def _():
            x_copy(3).wait()
            w_copy(0, 0).wait()
            wo_copy(0).wait()

        @pl.when(u == 1)
        def _():
            x_copy(4).wait()
            w_copy(0, 1).wait()
            w_copy(0, 2).wait()
            wo_copy(1).wait()

        def wo_blocks(k, a):
            r0 = jnp.minimum(u * WO_ROWS, HK - WO_ROWS)
            lo, hi = [woraw_v.at[q, pl.ds(pl.multiple_of(r0, 16), WO_ROWS), :][16 * k:16 * k + 16, :].astype(F32)
                      for q in range(2)]
            put_blocks(wos_v.at[pl.ds(pl.multiple_of(r0 // 2, 8), WO_ROWS // 2), :], 8 * k, _strassen_rhs,
                       lo[:, :HK], lo[:, HK:], hi[:, :HK], hi[:, HK:], never, a)

        xs = xs_tile(2 * u + 1)
        side = _Side(never)
        for i in range(2):
            t = 2 * u + 2 + i
            if i == 0:
                side.add(LN1_PLANS[0], lambda k, a: ln_rows(2 * u + 2, k, LNC, never, a))
            pending = v_stage(side, xs, 1 - i, False, False, t - 1 if i == 0 else None)
            xs = xs_tile(t)
            side = _Side(never)
            if i == 0:
                side.add(LN1_PLANS[1], lambda k, a: ln_rows(2 * u + 3, k, LNC, never, a))
                side.add(WO_PLAN, wo_blocks)
            side.hooks[-28 + D_LAG] = [lambda p=pending: kv_update(*p)]
            feat_stage(side, -28, 1, xs, lambda p, pr: k_pair(p, i, pr, 0, False, never if i == 1 else None))
            save_lead(t)
        fold(0, u)
        return carry

    lax.fori_loop(0, (NT_ - 2) // 2, phase1, 0)

    w_copy(0, 3).wait()
    wr_copy.wait()
    side = _Side(never0)

    def z_final(k, a):
        zb_v[k] = jnp.broadcast_to(_row_sum(_after(z_v[k], never0, a)), (128, 128))

    side.add(END_PLANS[0], z_final)
    side.add(END_PLANS[1], w_blocks(0))
    fold(0, 3, side, 100)
    kv_update(*v_stage(side, xs_tile(NT_ - 1), 1, False, True, None))
    wr_v[...] = jnp.broadcast_to(wrraw_v[...].reshape(1, D).astype(F32), (8, D))

    def o_copy(r0, n, i):
        return pltpu.make_async_copy(o_v.at[pl.ds(r0, n), :], out_hbm.at[pl.ds(r0, n), :], sem.at[SO + i])

    def finish_rows(h_ref, k, t, valid, st, never=None, anchor=None):
        r0 = t * T + k * LNC
        best, besti = st["route"]
        wr = jnp.concatenate([wr_v[...]] * (LNC // 8), axis=0)
        sub = lax.broadcasted_iota(jnp.int32, (8, 1), 0)
        h = _after(h_ref[k * LNC:(k + 1) * LNC, :], never, anchor)
        hc = h - _row_sum(h) * (1.0 / D)
        rstd = lax.rsqrt(_row_sum(hc * hc) * (1.0 / D) + LN_EPS)
        r = (_row_sum(hc * wr) * rstd).astype(BF16).astype(F32)
        hn = hc * rstd
        view(hn_v, t, T // 2)[k * LNC // 2:(k + 1) * LNC // 2, :] = _pack(hn.astype(BF16))
        view(o_v, t, T)[k * LNC:(k + 1) * LNC, :] = (hn + h).astype(BF16)
        if valid is not None:
            r = jnp.where(valid, r, -jnp.inf)
        for i in range(LNC // 8):
            ri = r[8 * i:8 * i + 8, :]
            better = ri > best
            best = jnp.where(better, ri, best)
            besti = jnp.where(better, sub + (r0 + 8 * i), besti)
        st["route"] = (best, besti)
        return best

    def q_pair(p, slot, pr):
        ep, en, sp, sn = _dual_exp(p)
        zz = [_lane_tile(zb_v[pr, 8 * i:8 * i + 8, :], T // 128) for i in range(16)]
        ap = _pair_allreduce(_tree(jnp.add, [ep[i] * zz[i] for i in range(8)]), jnp.add)
        an = _pair_allreduce(_tree(jnp.add, [en[i] * zz[8 + i] for i in range(8)]), jnp.add)
        inv = _recip(ap * sn + (an + 1e-6 * sn) * sp)
        rp = sn * inv
        rn = sp * inv
        phi = jnp.concatenate([e * rp for e in ep] + [e * rn for e in en], axis=0)
        phi_v[slot][64 * pr:64 * pr + 64, :] = _pack(phi.astype(BF16))

    def attn_blocks(slot, g):
        lo, hi = [jnp.concatenate(
            [_dot(_unpack(kvbf_v[32 * pr:32 * pr + 32, :]), _unpack(phi_v[slot][64 * pr:64 * pr + 64, :]), NN)
             for pr in (2 * q, 2 * q + 1)], axis=0) for q in (g, g + 4)]
        blocks = _strassen_lhs(lo[:, :TH], hi[:, :TH], lo[:, TH:], hi[:, TH:])
        ot = _pack(jnp.concatenate(blocks, axis=1).astype(BF16).T)
        for i in range(7):
            oc_v[slot][:, i * HK + 128 * g:i * HK + 128 * g + 128] = ot[i * TH // 2:(i + 1) * TH // 2, :]

    def out_proj(side, step0, t, slot):
        xt = view(x_v, t, T)
        for n in range(4):
            def product(i):
                step = step0 + 7 * n + i
                w = side.gate(step, wos_v[:, i * HK + 128 * n:i * HK + 128 * n + 128])
                res = _dot(_unpack(oc_v[slot][:, i * HK:(i + 1) * HK]), _unpack(w), NN)
                side.done(step, res)
                return res
            for q, row in enumerate(_strassen(product)):
                for r, res in enumerate(row):
                    rows, cols = slice(q * TH, (q + 1) * TH), slice(r * HK + 128 * n, r * HK + 128 * n + 128)
                    h_v[slot][rows, cols] = res + xt[rows, cols].astype(F32)

    def phase2(u, carry):
        for i in range(4):
            stage_copy(i, u).wait()
        never = u < 0
        side = _Side(never)
        st = {"route": carry}
        tp = jnp.maximum(2 * u - 1, 0)
        side.add(LN2_PLANS[0], lambda k, a: finish_rows(h_v[1], k, tp, u > 0, st, never, a))
        side.add(LN2_PLANS[1], lambda k, a: finish_rows(h_v[0], k, 2 * u, None, st, never, a))

        def packer(i, dst, n):
            left = [n]

            def job(k, a):
                if i < 2:
                    pack_rows(stage_v[i], dst, (k // 2) * 16, 16, (0, D)[k % 2], (D, FM - D)[k % 2], never, a)
                else:
                    pack_rows(stage_v[i], dst, k * 16, 16, 0, D, never, a)
                left[0] -= 1
                if not left[0]:
                    stage_copy(i, jnp.minimum(u + 1, NQ - 1)).start()
                    n0 = stage_v[i].shape[0] - 16
                    side.deps.setdefault(PACK_DUE[i], []).append(stage_v[i][n0:n0 + 8, 0:128].astype(F32))
            return job

        for i in range(2):
            side.add(PACK_PLANS[i], packer(i, view((wgp_v, wup_v)[i], u, D // NQ // 2), len(PACK_PLANS[i])))
            d0 = pl.multiple_of(u * (DQ // 2) + i * (DQA // 2), 8)
            side.add(PACKD_PLANS[i], packer(2 + i, wdp_v.at[pl.ds(d0, 8 * len(PACKD_PLANS[i])), :],
                                            len(PACKD_PLANS[i])))
            for g in range(4):
                step = 107 + 28 * i + 7 * g + G_LAG
                side.hooks.setdefault(step if step < 156 else step - 156, []).append(
                    lambda i=i, g=g: attn_blocks(i, g))
        for i in range(2):
            feat_stage(side, 100 + 28 * i, 0, xs_tile(2 * u + i), lambda p, pr: q_pair(p, i, pr),
                       2 * u if i == 0 else None)
        for i in range(2):
            out_proj(side, 28 * i, 2 * u + i, i)
        side.check()

        @pl.when(u == 0)
        def _():
            o_copy(0, T, 0).start()

        @pl.when(u > 0)
        def _():
            o_copy(pl.multiple_of(tp * T, T), 2 * T, u).start()

        return st["route"]

    wg_copy.wait()
    wu_copy.wait()
    wd_copy.wait()
    route = lax.fori_loop(
        0, NT_ // 2, phase2,
        (jnp.full((8, 1), -jnp.inf, F32), jnp.zeros((8, 1), jnp.int32)))
    st = {"route": route}
    for k in range(T // LNC):
        finish_rows(h_v[1], k, NT_ - 1, None, st)
    best, besti = st["route"]
    o_copy(S - T, T, NT_).start()

    rmax = jnp.max(best, axis=0, keepdims=True)
    idx = jnp.min(jnp.where(best == rmax, besti, S), axis=0, keepdims=True)
    idx_s = jnp.clip(idx[0, 0], 0, S - 1)
    blk = pl.multiple_of((idx_s >> 4) << 4, 16)
    pair = jnp.broadcast_to(hn_v[pl.ds(idx_s >> 1, 1), :], (8, D))
    x8 = pltpu.bitcast(jnp.where((idx_s & 1) == 1, pair & jnp.uint32(0xFFFF0000), pair << 16), F32)
    xs = jnp.concatenate([x8, x8], axis=0).astype(BF16)
    acts, anchors = [], []

    def park(v, half):
        n = v.shape[0] // 128
        for i in range(n):
            z_v[i, :, 128 * half:128 * half + 128] = v[128 * i:128 * i + 128, :]
        return jnp.concatenate([z_v[i, :, 128 * half:128 * half + 128] for i in range(n)], axis=0)

    for c0 in range(0, FM, 128):
        g = _dot(xs, _unpack(wgp_v[:, c0:c0 + 128]), NN)[0:8, :]
        u = _dot(xs, _unpack(wup_v[:, c0:c0 + 128]), NN)[0:8, :]
        anchors += [g, u]
        acts.append(g * jax.nn.sigmoid(g) * u)
    xb = park(_col_broadcast(x8), 0)
    g, u = [_sublane_allreduce(_vpu_matvec(
        xb, lambda g: w[8 * g:8 * g + 8, :].astype(F32), never0,
        anchors[i * MOE_NA // 2:(i + 1) * MOE_NA // 2], MOE_LAGS[0])) for i, w in enumerate((wg_v, wu_v))]
    acts.append(g * jax.nn.sigmoid(g) * u)
    a = jnp.concatenate(acts, axis=1)
    am = jnp.concatenate([a[:, FVD:], a[:, FVD:]], axis=0).astype(BF16)
    ys, anchors = [], anchors[MOE_NA:]
    for k0 in range(0, FF - FVD, 512):
        k1 = min(k0 + 512, FF - FVD)
        yk = _dot(am[:, k0:k1], _unpack(wdp_v[k0 // 2:k1 // 2, 0:D]), NN)[0:8, :]
        ys.append(yk)
        anchors += [yk[:, c:c + 128] for c in range(128, D, 256)]
    ys.append(_sublane_allreduce(_vpu_matvec(
        park(_col_broadcast(a[:, :FVD]), 1), lambda g: wd_v[8 * g:8 * g + 8, :].astype(F32), never0,
        anchors[:-MOE_ND], MOE_LAGS[1])))
    y = _tree(jnp.add, ys) * jax.nn.sigmoid(rmax)
    y = jnp.concatenate([y, y], axis=0)
    sel = lax.broadcasted_iota(jnp.int32, (16, 1), 0) == (idx_s - blk)
    patch_v[...] = (o_v[pl.ds(blk, 16), :].astype(F32) + jnp.where(sel, y, 0.0)).astype(BF16)
    o_copy(0, T, 0).wait()
    for u in range(1, NT_ // 2):
        o_copy((2 * u - 1) * T, 2 * T, u).wait()
    o_copy(S - T, T, NT_).wait()
    pc = pltpu.make_async_copy(patch_v, out_hbm.at[pl.ds(blk, 16), :], sem.at[SM + 3])
    pc.start()
    for i in range(4):
        stage_copy(i, NQ - 1).wait()
    pc.wait()


@jax.jit
def pallas_sequential_preLN__linear_kernel_hedgehog__moe_arch_mod__prompt_kernel(
    A_x: jax.Array,
    A_wqkv: jax.Array,
    A_w_phi: jax.Array,
    A_wo: jax.Array,
    B_x: jax.Array,
    B_w_r: jax.Array,
    B_w_gate: jax.Array,
    B_w_up: jax.Array,
    B_w_down: jax.Array,
):
    del B_x
    hbm = pl.BlockSpec(memory_space=pl.ANY)
    out = pl.pallas_call(
        _kernel,
        out_shape=jax.ShapeDtypeStruct((S, D), BF16),
        in_specs=[hbm] * 8,
        out_specs=hbm,
        scratch_shapes=[
            pltpu.VMEM((S, D), BF16),
            pltpu.VMEM((T, D), U32),
            pltpu.VMEM((NT_ * TH // 2, SW), U32),
            pltpu.VMEM((NT_ * HK // 2, 128), U32),
            pltpu.VMEM((3 * NC, D, RC), BF16),
            [pltpu.VMEM((D // 2, D), U32)] * 3,
            [pltpu.VMEM((HK // 2, 7 * HK), U32)] * 3,
            pltpu.VMEM((H, DH, DH), BF16),
            pltpu.VMEM((8 * 64, 128), U32),
            pltpu.VMEM((2, HK, D), BF16),
            pltpu.VMEM((HK // 2, 7 * HK), U32),
            pltpu.VMEM((D,), BF16),
            pltpu.VMEM((8, D), F32),
            pltpu.VMEM((NPAIR, 64, 128), F32),
            pltpu.VMEM((NPAIR * 32, 128), U32),
            pltpu.VMEM((NPAIR, 128, T), F32),
            pltpu.VMEM((NPAIR, 128, 128), F32),
            [pltpu.VMEM((NPAIR * 64, T), U32)] * 2,
            [pltpu.VMEM((TH // 2, 7 * HK), U32)] * 2,
            [pltpu.VMEM((T, D), F32)] * 2,
            pltpu.VMEM((S // 2, D), U32),
            pltpu.VMEM((S, D), BF16),
            pltpu.VMEM((D, FV), BF16),
            pltpu.VMEM((D, FV), BF16),
            pltpu.VMEM((FVD, D), BF16),
            [pltpu.VMEM((D // NQ + 16, FM), BF16), pltpu.VMEM((D // NQ + 16, FM), BF16),
             pltpu.VMEM((DQA + 16, D), BF16), pltpu.VMEM((DQ - DQA + 16, D), BF16)],
            pltpu.VMEM((D // 2, FM), U32),
            pltpu.VMEM((D // 2, FM), U32),
            pltpu.VMEM(((FF - FVD) // 2, D + 128), U32),
            pltpu.VMEM((16, D), BF16),
            pltpu.SemaphoreType.DMA((6 + 3 * NC + NT_ + 16,)),
        ],
        compiler_params=pltpu.CompilerParams(vmem_limit_bytes=100 * 1024 * 1024,
                                             disable_semaphore_checks=True, disable_bounds_checks=True),
        name="hedgehog_mod",
    )(
        A_x.reshape(S, D),
        A_wqkv,
        A_w_phi,
        A_wo.reshape(2, HK, D),
        B_w_r,
        B_w_gate,
        B_w_up,
        B_w_down,
    )
    return out.reshape(1, S, D)
```

```python
import math

import jax
import jax.numpy as jnp
from jax import lax
import jax.experimental.pallas as pl
import jax.experimental.pallas.tpu as pltpu

F32 = jnp.float32
BF16 = jnp.bfloat16
U32 = jnp.uint32

S = 2048
D = 1024
H = 32
DH = 32
FF = 3584
NPAIR = H // 2
LOG2E = 1.4426950408889634
LN_EPS = 1e-5

T = 256
TH = T // 2
NT_ = S // T
RC = 256
NC = D // RC
PPC = RC // 64
LNC = 16

FV = 10 * 128
FM = FF - FV
FVD = 8 * 128
NQ = NT_ // 2
DQ = (FF - FVD) // NQ
WO_ROWS = 176
HK = D // 2
SW = 8 * HK


def _spread(n, a, b, due=None):
    rel = [round(a + (b - a) * k / (n - 1), 3) for k in range(n)]
    return tuple((r, None if due is None else math.ceil(r) + due) for r in rel)


LN1_PLANS = (((-0.191, 5), (1.306, 7), (3.36, 8), (3.523, 10), (6.057, 11), (7.923, 13), (7.953, 14), (10.582,
    16), (10.709, 17), (13.131, 19), (14.512, 19), (15.809, 22), (17.551, 24), (19.157, 26), (20.343, 25),
    (22.021, 27)), ((0.237, 5), (0.929, 7), (1.849, 8), (3.89, 10), (5.129, 12), (6.422, 11), (8.22, 13),
    (9.731, 15), (10.273, 17), (12.8, 17), (14.493, 19), (16.14, 21), (17.085, 22), (18.04, 25), (20.775, 25),
    (21.371, 27)))
PRO_LN1_PLAN = ((None, None),) * 16
PRO_K_PLANS0 = ((0.305, None), (0.868, None), (1.842, None), (2.673, None), (3.46, None), (3.946, None),
    (5.477, None), (5.976, None))
PRO_K_PLANS1 = ((-0.801, None), (0.868, None), (1.269, None), (2.799, None), (3.707, None), (3.71, None),
    (4.564, None), (5.93, None))
PRO_X0_PLAN = ((0.186, None), (1.357, None), (2.524, None), (3.033, None), (3.492, None), (4.95, None),
    (5.092, None), (6.364, None))
PRO_W0_PLAN = ((0.134, None), (0.625, None), (2.014, None), (2.659, None), (3.075, None), (4.159, None),
    (4.578, None), (5.262, None), (5.775, None), (6.465, None))
PRO_W_PLAN = ((0.0, None), (1.189, None), (2.122, None), (2.861, None), (3.761, None), (8.3, None), (9.157,
    None), (9.666, None), (10.34, None), (11.02, None), (11.678, None), (12.316, None), (13.06, None),
    (13.534, None), (14.283, None), (15.357, None), (15.78, None), (16.376, None), (17.14, None), (18.074,
    None), (18.337, None))
PRO_K_PLANS2 = ((15.126, None), (15.758, None), (16.112, None), (16.529, None), (16.901, None), (17.335,
    None), (17.583, None), (17.807, None))
PRO_V_PLANS = (((None, None), (None, None), (None, None), (None, None), (None, None), (None, None), (None,
    None), (None, None), (-3.614, None), (-3.131, None), (-2.919, None), (-2.462, None), (-2.134, None),
    (-1.981, None), (-1.979, None), (-1.668, None), (-1.399, None), (-1.34, None), (-1.245, None), (-0.246,
    None), (-0.037, None), (0.131, None), (0.587, None), (0.947, None), (0.981, None), (1.216, None), (1.304,
    None), (1.832, None), (2.278, None), (2.378, None), (2.384, None), (2.43, None)), ((9.004, None), (10.111,
    None), (11.857, None), (13.312, None), (13.618, None), (15.761, None), (18.136, None), (18.844, None)),
    ((20.076, None), (21.214, None), (21.326, None), (21.759, None), (22.923, None), (23.574, None), (24.56,
    None), (25.574, None)), ((16.74, None), (18.286, None), (19.678, None), (20.486, None), (22.111, None),
    (23.433, None), (24.5, None), (24.753, None)), ((19.124, None), (20.055, None), (21.127, None), (22.214,
    None), (23.107, None), (23.964, None), (24.907, None), (26.177, None), (-1.658, None), (0.17, None),
    (0.243, None), (1.521, None), (1.704, None), (3.022, None), (3.974, None), (5.371, None), (5.519, None),
    (6.428, None), (7.106, None), (8.227, None), (8.924, None), (9.718, None), (10.885, None), (11.365, None),
    (12.091, None), (12.277, None), (13.8, None), (14.607, None), (15.386, None), (16.348, None), (17.174,
    None), (17.902, None)))
END_PLANS = (((0.055, None), (2.011, None), (3.919, None), (5.535, None), (7.124, None), (8.225, None),
    (10.555, None), (11.952, None), (13.867, None), (15.593, None), (17.249, None), (19.512, None), (20.8,
    None), (22.209, None), (23.312, None), (25.914, None)), ((100.584, None), (101.301, None), (102.013,
    None), (0.409, None), (0.793, None), (2.288, None), (2.978, None), (3.797, None), (5.031, None), (6.001,
    None), (7.229, None), (7.984, None), (8.951, None), (10.186, None), (11.123, None), (11.847, None),
    (12.976, None), (13.561, None), (14.696, None), (15.579, None), (17.16, None), (18.073, None), (18.596,
    None), (19.613, None), (20.508, None), (21.155, None), (22.453, None), (22.609, None), (24.586, None),
    (25.525, None), (25.802, None)))
WO_PLAN = ((0.819, None), (3.254, None), (4.713, None), (8.885, None), (10.878, None), (12.808, None),
    (15.093, None), (17.749, None), (19.152, None), (22.645, None), (26.454, None))
LN2_PLANS = (((0.0, 5), (1.415, 7), (2.908, 7), (4.33, 10), (5.804, 11), (7.394, 13), (8.709, 14), (10.284,
    16), (11.854, 17), (13.254, 19), (14.714, 20), (16.143, 21), (17.577, 23), (19.143, 26), (20.595, 26),
    (22.085, 27)), ((28.5, 33), (29.933, 35), (31.318, 37), (32.8, 38), (34.046, 40), (35.667, 41), (37.183,
    44), (38.489, 44), (39.988, 45), (41.4, 47), (42.765, 48), (44.267, 51), (45.736, 52), (47.111, 53),
    (48.529, 54), (50.026, 55)))
PACK_PLANS = (((100.5, None), (101.289, None), (102.145, None), (102.955, None), (103.691, None), (104.613,
    None), (105.435, None), (106.258, None), (107.081, None), (107.888, None), (108.716, None), (109.548,
    None), (110.371, None), (111.194, None), (112.016, None), (112.707, None), (113.679, None), (114.484,
    None), (115.306, None), (116.167, None), (116.952, None), (117.901, None), (118.597, None), (119.419,
    None), (120.242, None), (121.065, None), (121.887, None), (122.845, None), (123.603, None), (124.355,
    None), (125.177, None), (126.0, None)), ((128.5, None), (129.295, None), (130.145, None), (130.932, None),
    (131.844, None), (132.656, None), (133.435, None), (134.258, None), (135.081, None), (135.903, None),
    (136.726, None), (137.548, None), (138.371, None), (139.194, None), (140.016, None), (140.845, None),
    (141.661, None), (142.484, None), (143.335, None), (144.04, None), (144.952, None), (145.824, None),
    (146.667, None), (147.419, None), (148.242, None), (149.206, None), (149.943, None), (150.71, None),
    (151.567, None), (152.355, None), (153.177, None), (154.0, None)))
PACKD_PLANS = (((0.406, None), (1.444, None), (2.487, None), (3.333, None), (4.314, None), (5.145, None),
    (6.167, None), (7.114, None), (8.056, None), (9.0, None), (9.973, None), (10.966, None), (11.824, None),
    (12.735, None), (13.722, None), (14.667, None), (15.611, None), (16.556, None), (17.43, None), (18.444,
    None), (19.496, None), (20.333, None), (21.241, None), (22.133, None), (23.167, None), (24.111, None),
    (25.031, None), (26.051, None)), ((28.5, None), (29.364, None), (30.227, None), (31.191, None), (31.955,
    None), (32.783, None), (33.682, None), (34.545, None), (35.409, None), (36.319, None), (37.136, None),
    (37.983, None)))
PACK_DUE = (130, 3, 30, 42)
DQA = 16 * len(PACKD_PLANS[0])
G_LAG = 5
D_LAG = 1
BLOCK_STAGGER = 4
BLOCK_DELAY = 4
PLAIN_V0 = 1
MOE_NA = 36
MOE_ND = 2
MOE_LAGS = (2, 2)
STAGGER = 8

NN = (((1,), (0,)), ((), ()))
NT = (((1,), (1,)), ((), ()))


def _dot(a, b, dims):
    return lax.dot_general(a, b, dims, preferred_element_type=F32)


def _recip(x):
    return pl.reciprocal(x, approx=False, full_range=False)


def _pack(x):
    return pltpu.bitcast(x, U32)


def _unpack(x):
    return pltpu.bitcast(x, BF16)


def _strassen_lhs(a11, a12, a21, a22):
    return [a21 + a22, a22, a11 + a12, a11, a11 + a22, a12 - a22, a21 - a11]


def _strassen_rhs(b11, b12, b21, b22):
    return [b11, b21 - b11, b22, b12 - b22, b11 + b22, b21 + b22, b11 + b12]


def _strassen(product):
    m2 = product(0)
    m4 = product(1)
    c21 = m2 + m4
    m5 = product(2)
    u11 = m4 - m5
    m3 = product(3)
    c12 = m3 + m5
    u22 = m3 - m2
    m1 = product(4)
    u11 = u11 + m1
    u22 = u22 + m1
    c11 = product(5) + u11
    c22 = product(6) + u22
    return [[c11, c12], [c21, c22]]


def _pair_allreduce(a, op):
    a = op(a, pltpu.roll(a, 2, 0))
    return op(a, pltpu.roll(a, 4, 0))


def _tree(op, xs):
    xs = list(xs)
    while len(xs) > 1:
        nxt = [op(xs[i], xs[i + 1]) for i in range(0, len(xs) - 1, 2)]
        if len(xs) % 2:
            nxt.append(xs[-1])
        xs = nxt
    return xs[0]


def _pair_logits(sl, j):
    sub = lax.broadcasted_iota(jnp.int32, sl[0].shape, 0)
    if j < 3:
        head = jnp.where(sub < 2, 0.0, sl[(0, 1, 16)[j]])
    else:
        head = jnp.where(sub < 2, sl[0], jnp.where(sub < 4, pltpu.roll(sl[1], 2, 0),
                                                   jnp.where(sub < 6, pltpu.roll(sl[16], 4, 0), 0.0)))
    r0 = (2, 9, 17, 24)[j]
    return [head] + list(sl[r0:r0 + 7])


def _dual_exp(sl):
    mx = _pair_allreduce(_tree(jnp.maximum, sl), jnp.maximum)
    mn = _pair_allreduce(_tree(jnp.minimum, sl), jnp.minimum)
    ep = [jnp.exp2(s - mx) for s in sl]
    en = [jnp.exp2(mn - s) for s in sl]
    sp = _pair_allreduce(_tree(jnp.add, ep), jnp.add)
    sn = _pair_allreduce(_tree(jnp.add, en), jnp.add)
    return ep, en, sp, sn


def _after(x, never, anchor):
    if anchor is None:
        return x
    d = jnp.concatenate([anchor] * (x.shape[0] // 8), axis=0)
    if x.shape[1] == 128:
        return jnp.where(never, d, x)
    return jnp.concatenate([jnp.where(never, d, x[:, :128]), x[:, 128:]], axis=1)


def _gate(x, never, deps):
    for i, dep in enumerate(deps):
        d = jnp.broadcast_to(dep, (8, 128))
        if x.dtype != F32:
            d = pltpu.bitcast(d, x.dtype)
        blk = jnp.where(never, d, x[8 * i:8 * i + 8, :128])
        if x.shape[1] > 128:
            blk = jnp.concatenate([blk, x[8 * i:8 * i + 8, 128:]], axis=1)
        parts = ([x[:8 * i, :]] if i else []) + [blk, x[8 * i + 8:, :]]
        x = jnp.concatenate(parts, axis=0)
    return x


def _lane_fold(a):
    return _tree(jnp.add, [a[:, 128 * i:128 * i + 128] for i in range(a.shape[1] // 128)])


def _row_sum(a):
    return jnp.sum(_lane_fold(a), axis=-1, keepdims=True)


def _lane_tile(a, n):
    return a if n == 1 else jnp.concatenate([a] * n, axis=1)


def _sublane_allreduce(a):
    a = a + pltpu.roll(a, 4, 0)
    a = a + pltpu.roll(a, 2, 0)
    return a + pltpu.roll(a, 1, 0)


def _col_broadcast(row8):
    return jnp.concatenate([row8] * 16, axis=0).astype(BF16).T.astype(F32)


def _vpu_matvec(xb, w_rows, never, anchors, lag):
    ng = xb.shape[0] // 8
    acc, hist = None, []
    for g in range(ng):
        dep = anchors[(g * len(anchors)) // ng]
        if g >= lag:
            dep = dep + hist[g - lag]
        x = jnp.where(never, dep, xb[8 * g:8 * g + 8, :])
        w = w_rows(g)
        t = w * _lane_tile(x, w.shape[1] // 128)
        acc = t if acc is None else acc + t
        c = 128 * (g % (w.shape[1] // 128))
        hist.append(acc[:, c:c + 128])
    return acc


class _Side:
    def __init__(self, never):
        self.never = never
        self.jobs = []
        self.deps = {}
        self.hooks = {}

    def add(self, plan, fn):
        for k, (rel, due) in enumerate(plan):
            if rel is None:
                self._run(due, fn, k, None)
            else:
                self.jobs.append((rel, due, fn, k))

    def _run(self, due, fn, k, anchor):
        dep = fn(k, anchor)
        if due is not None:
            self.deps.setdefault(due, []).append(dep)

    def check(self):
        assert not self.jobs and not self.deps and not self.hooks

    def gate(self, step, x):
        return _gate(x, self.never, self.deps.pop(step, []))

    def done(self, step, res):
        m = res.shape[0] // 8
        for job in sorted([j for j in self.jobs if step - 1 < j[0] <= step], key=lambda j: j[0]):
            self.jobs.remove(job)
            g = m - 1 - int((step - job[0]) * m)
            self._run(job[1], job[2], job[3], res[8 * g:8 * g + 8, res.shape[1] - 128:])
        for fn in self.hooks.pop(step, []):
            fn()


def _kernel(x_hbm, wqkv_hbm, wphi_hbm, wo_hbm, wr_hbm, wg_hbm, wu_hbm, wd_hbm, out_hbm,
            x_v, xn_v, xs_v, lead_v, wraw_v, wt_v, ws_v, wphi_v, a_v, woraw_v, wos_v, wrraw_v, wr_v,
            kvacc_v, kvbf_v, z_v, zb_v, phi_v, oc_v, h_v, hn_v, o_v, wg_v, wu_v, wd_v, stage_v,
            wgp_v, wup_v, wdp_v, patch_v,
            sem):
    SX, SQ, SO, SM = 0, 6, 6 + 3 * NC, 6 + 3 * NC + NT_ + 1

    def x_copy(i):
        h0, h1 = ((0, 1), (1, 2), (2, 4), (4, 8), (8, 2 * NT_))[i]
        rows = pl.ds(h0 * TH, (h1 - h0) * TH)
        return pltpu.make_async_copy(x_hbm.at[rows, :], x_v.at[rows, :], sem.at[SX + i])

    def k0_copy(s):
        return pltpu.make_async_copy(wqkv_hbm.at[:, pl.ds(D + s * 128, 128)],
                                     wraw_v.at[NC, :, pl.ds(s * 128, 128)], sem.at[(SM + 7, SQ + NC)[s]])

    def w_copy(j, c):
        return pltpu.make_async_copy(wqkv_hbm.at[:, pl.ds(j * D + c * RC, RC)], wraw_v.at[j * NC + c],
                                     sem.at[SQ + j * NC + c])

    def wphi_copy(i):
        h0, h1 = ((0, 8), (16, 24), (8, 16), (24, H))[i]
        return pltpu.make_async_copy(wphi_hbm.at[pl.ds(h0, h1 - h0)], wphi_v.at[pl.ds(h0, h1 - h0)],
                                     sem.at[(SM + 4, SM + 8, SM + 9, SM + 14)[i]])

    wr_copy = pltpu.make_async_copy(wr_hbm, wrraw_v, sem.at[SM + 5])

    def wo_copy(i):
        rows = pl.ds(0, WO_ROWS) if i == 0 else pl.ds(WO_ROWS, HK - WO_ROWS)
        return pltpu.make_async_copy(wo_hbm.at[:, rows, :], woraw_v.at[:, rows, :], sem.at[(SM + 6, SX + 5)[i]])

    wg_copy = pltpu.make_async_copy(wg_hbm.at[:, pl.ds(FM, FV)], wg_v, sem.at[SM + 0])
    wu_copy = pltpu.make_async_copy(wu_hbm.at[:, pl.ds(FM, FV)], wu_v, sem.at[SM + 1])
    wd_copy = pltpu.make_async_copy(wd_hbm.at[pl.ds(0, FVD), :], wd_v, sem.at[SM + 2])

    def stage_copy(i, q):
        if i < 2:
            r0 = q * (D // NQ)
            r0 = r0 if isinstance(r0, int) else pl.multiple_of(r0, D // NQ)
            src = (wg_hbm, wu_hbm)[i].at[pl.ds(r0, D // NQ), pl.ds(0, FM)]
        else:
            r0 = FVD + q * DQ + (i - 2) * DQA
            r0 = r0 if isinstance(r0, int) else pl.multiple_of(r0, 16)
            src = wd_hbm.at[pl.ds(r0, (DQA, DQ - DQA)[i - 2]), :]
        return pltpu.make_async_copy(src, stage_v[i].at[pl.ds(0, src.shape[0]), :], sem.at[SM + 10 + i])

    wphi_copy(0).start()
    k0_copy(0).start()
    x_copy(0).start()
    k0_copy(1).start()
    x_copy(1).start()
    wphi_copy(1).start()
    w_copy(1, 2).start()

    made = set()

    def view(ref, i, n, off=0):
        r0 = off + i * n
        return ref.at[pl.ds(r0 if isinstance(r0, int) else pl.multiple_of(r0, math.gcd(n, off)), n), :]

    def put_blocks(dst, r0, fn, m11, m12, m21, m22, never, a, skip=()):
        w = HK // BLOCK_STAGGER
        for c0 in range(0, HK, w):
            d11, d22 = m11[:, c0:c0 + w], m22[:, c0:c0 + w]
            if a is not None:
                d = jnp.concatenate([_lane_tile(a, w // 128)] * 2, axis=0)
                d11, d22 = jnp.where(never, d, d11), jnp.where(never, d, d22)
            blocks = fn(d11, m12[:, c0:c0 + w], m21[:, c0:c0 + w], d22)
            for i, b in enumerate(blocks):
                if i not in skip:
                    dst[r0:r0 + 8, i * HK + c0:i * HK + c0 + w] = _pack(b.astype(BF16))
            a = blocks[6][8:16, w - 128:]
            for _ in range(BLOCK_DELAY):
                a = a * a

    def rows16(ref, r0):
        return _unpack(ref[r0:r0 + 8, :]).astype(F32)

    def x_blocks(t, k, lo, hi, never, a):
        put_blocks(view(xs_v, t, TH // 2), k * LNC // 2, _strassen_rhs,
                   lo[:, :HK], hi[:, :HK], lo[:, HK:], hi[:, HK:], never, a)

    def ln_rows(t, k, n, never=None, anchor=None, plain=False):
        x = _after(view(x_v, t, T)[k * n:(k + 1) * n, :].astype(F32), never, anchor)
        xc = x - _row_sum(x) * (1.0 / D)
        rstd = lax.rsqrt(_row_sum(xc * xc) * (1.0 / D) + LN_EPS)
        xn = xc * rstd
        if plain:
            xn_v[(t * T + k * n) // 2:(t * T + (k + 1) * n) // 2, :] = _pack(xn.astype(BF16))
        elif k * n < TH:
            xn_v[k * n // 2:(k + 1) * n // 2, :] = _pack(xn.astype(BF16))
        else:
            x_blocks(t, k - TH // LNC, rows16(xn_v, (k * n - TH) // 2), xn, never, xn[0:8, 0:128])
        return _tree(jnp.add, [rstd[8 * i:8 * i + 8, :] for i in range(min(n, LNC) // 8)])

    def late_x_blocks(t):
        return lambda k, a: x_blocks(t, k, rows16(xn_v, t * T // 2 + 8 * k),
                                     rows16(xn_v, (t * T + TH) // 2 + 8 * k), never0, a)

    def xn_tile(t):
        return _unpack(xn_v[t * T // 2:(t + 1) * T // 2, :])

    def xs_tile(t):
        return _unpack(view(xs_v, t, TH // 2)[:, 0:7 * HK])

    def expand_wphi(c):
        w = wphi_v[8 * c:8 * c + 8].reshape(8 * DH, DH).astype(F32).T
        bits = pltpu.bitcast(w, U32)
        head = lax.broadcasted_iota(jnp.int32, (DH, 128), 1) >> 5
        for s in range(2):
            b = bits[:, 128 * s:128 * s + 128]
            for j in range(2):
                r0 = 64 * (2 * c + s) + 32 * j
                a_v[r0:r0 + 32, :] = jnp.where(head == 2 * j, b >> 16,
                                               jnp.where(head == 2 * j + 1, b, jnp.uint32(0)))

    wphi_copy(0).wait()
    expand_wphi(0)
    h_v[1][...] = jnp.zeros((T, D), F32)
    for ref in stage_v:
        ref[ref.shape[0] - 16:, 0:128] = jnp.zeros((16, 128), BF16)

    def v_transpose(k, a):
        q, r0 = (k // 8) + 4 * (k % 2), 256 * (k % 8 // 2)
        w = wraw_v[2 * NC + q // 2, r0:r0 + 256, (q % 2) * 128:(q % 2) * 128 + 128]
        if a is not None:
            w = _unpack(jnp.where(never0, jnp.concatenate([pltpu.bitcast(a, U32)] * 16, axis=0), _pack(w)))
        wt_v[2][64 * q:64 * q + 64, r0:r0 + 256] = _pack(w.T)
        made.add(("vt", k))

    def fold_pairs(j, c, s, side=None, step0=None):
        g0 = 64 * (2 * c + s)
        g0 = g0 if isinstance(g0, int) else pl.multiple_of(g0, 64)
        res = _dot(_unpack(a_v[pl.ds(g0, 64), :]), wraw_v[j * NC + c, :, s * 128:(s + 1) * 128], NT)
        if side is not None:
            side.done(step0 + 2 * s, res[:, :D // 2])
            side.done(step0 + 2 * s + 1, res[:, D // 2:])
        sub = lax.broadcasted_iota(jnp.int32, (8, D), 0)
        out = []
        for q in range(2):
            base = _pair_allreduce(jnp.where(sub < 2, res[64 * q:64 * q + 8, :], 0.0), jnp.add)
            out.append([(res[64 * q + 8 * i:64 * q + 8 * i + 8, :] - base) * LOG2E for i in range(8)])
        return out

    def share(z, z3, k):
        sub = lax.broadcasted_iota(jnp.int32, (8, D), 0)
        return jnp.where(sub < 2, pltpu.roll(z3, 8 - 2 * k, 0), z)

    def packed(slabs):
        return _pack(jnp.concatenate(slabs, axis=0).astype(BF16))

    def fold(j, c, side=None, step0=None):
        p0, p1 = fold_pairs(j, c, 0, side, step0)
        p2, p3 = fold_pairs(j, c, 1, side, step0)
        sl = ([share(p0[0], p3[0], 1), share(p1[0], p3[0], 2)] + p0[1:] + p1[1:]
              + [share(p2[0], p3[0], 3)] + p2[1:] + p3[1:])
        zero = jnp.zeros((8, D), F32)
        even, odd = sl + [zero], [zero] + sl
        r0 = 8 * ((31 * c) // 2)
        is_odd = c % 2 == 1
        if isinstance(c, int):
            sl = odd if is_odd else even
        else:
            r0 = pl.multiple_of(r0, 8)
            sl = [jnp.where(is_odd, o, e) for o, e in zip(odd, even)]
        win = wt_v[j].at[pl.ds(r0, 128), :]
        win[8:128, :] = packed(sl[2:])
        first = packed(sl[:2])
        if is_odd is not False:
            keep = lax.broadcasted_iota(jnp.int32, (8, D), 0) < jnp.where(is_odd, 4, 0)
            first = jnp.where(keep, win[0:8, :], first)
        win[0:8, :] = first
        made.update(("fold", j, q) for q in ([c] if isinstance(c, int) else range(3)))

    def w_blocks(j, k0=0):
        def job(k, a):
            k += k0
            assert made >= ({("vt", 8 * (k // 8) + q) for q in range(8)} if j == 2 else
                            {("fold", j, q) for q in ((0, 2) if k < 15 else range(4))})
            made.add(("ws", j, k))
            lo, hi = rows16(wt_v[j], 8 * k), rows16(wt_v[j], (256 if j == 2 else 248) + 8 * k)
            put_blocks(ws_v[j], 8 * k, _strassen_lhs, lo[:, :HK], lo[:, HK:], hi[:, :HK], hi[:, HK:], never0, a,
                       skip=(1, 3))
        return job

    def k_pair(p, slot, pr, c0, first, never=None):
        for n in range(c0, c0 + p[0].shape[1], 128):
            assert first == (("z", pr, n) not in made)
            made.update({("z", pr, n), ("phi", slot, pr, n)})
        ep, en, sp, sn = _dual_exp(p)
        inv = _recip(sp * sn)
        scale = (sn * inv, sp * inv)
        es = ep + en
        cols = slice(c0, c0 + p[0].shape[1])
        n = 16 if never is None else 16 // STAGGER
        last = None
        for q in range(16 // n):
            sc = scale
            if last is not None:
                sc = [jnp.where(never, last, x) for x in scale]
            phi = jnp.concatenate([es[i] * sc[i // 8] for i in range(q * n, (q + 1) * n)], axis=0)
            rows = slice(8 * q * n, 8 * (q + 1) * n)
            z = phi if first else z_v[pr, rows, cols] + phi
            z_v[pr, rows, cols] = z
            phi_v[slot][64 * pr + 4 * q * n:64 * pr + 4 * (q + 1) * n, cols] = _pack(phi.astype(BF16))
            last = z[8 * n - 8:, :]

    def k_features(pk, slot, c, first, never=None):
        for j in range(PPC):
            k_pair(_pair_logits(pk, j), slot, c * PPC + j, 0, first, never)

    def kv_update(vts, slot, g, first, publish=False):
        for q, vt in enumerate(vts):
            for j in range(2):
                pr = 2 * g + 8 * q + j
                assert made >= {("phi", slot, pr, 0), ("phi", slot, pr, 128)}
                upd = _dot(vt[64 * j:64 * j + 64, :].astype(BF16), _unpack(phi_v[slot][64 * pr:64 * pr + 64, :]), NT)
                acc = upd if first else kvacc_v[pr] + upd
                kvacc_v[pr] = acc
                if publish:
                    odd = -(lax.broadcasted_iota(jnp.int32, (32, 128), 1) & 1)
                    bits = pltpu.bitcast(acc, jnp.int32) & jnp.concatenate([~odd, odd], axis=0)
                    kvbf_v[32 * pr:32 * pr + 32, :] = _pack(pltpu.bitcast(bits, F32).astype(BF16))

    def save_lead(t):
        view(lead_v, t, HK // 2)[...] = _pack(_unpack(view(xs_v, t, TH // 2)[:, 0:HK]).T)

    def proj_feat(side, step0, c, xn, carry):
        r0 = 8 * ((31 * c) // 2)
        skip = 8 if c % 2 == 1 and carry is not None else 0
        w = wt_v[1][r0 + skip:r0 + 128, :]
        quarters = []
        for n in range(2):
            for m in range(2):
                step = step0 + 2 * n + m
                wq = _unpack(side.gate(step, w[:64, :] if m == 0 else w[64:, :]))
                res = _dot(wq, xn[n * TH:(n + 1) * TH, :], NT)
                side.done(step, res)
                quarters.append(res)
        res = jnp.concatenate(
            [jnp.concatenate([quarters[0], quarters[2]], axis=1),
             jnp.concatenate([quarters[1], quarters[3]], axis=1)], axis=0)
        sl = [res[8 * i:8 * i + 8, :] for i in range(res.shape[0] // 8)]
        if c % 2 == 0:
            return sl[:31], sl[31]
        return ([carry] + sl if skip else sl[1:]), None

    def proj_unit(side, step0, j, b, xs, lead=None, plain=None):
        r1 = 64 * b + (64 if j == 2 or b < 3 else 56)
        assert made >= ({("vt", 8 * b + q) for q in range(8)} if plain is not None else
                        {("ws", j, k) for k in range(8 * b, r1 // 8)})
        if plain is not None:
            out = []
            for q in range(2):
                row = []
                for n in range(2):
                    res = _dot(_unpack(wt_v[2][256 * q + 64 * b:256 * q + r1, :]), plain[n * TH:(n + 1) * TH, :], NT)
                    for i in range((0, 2, 4, 5)[2 * q + n], (2, 4, 5, 7)[2 * q + n]):
                        side.done(step0 + i, res)
                    row.append(res)
                out.append(jnp.concatenate(row, axis=1))
            return out

        def product(i):
            off = 256 if j == 2 else 248
            w = (wt_v[j][off + 64 * b:off + r1, HK:] if i == 1 else wt_v[j][64 * b:r1, :HK] if i == 3
                 else ws_v[j][64 * b:r1, i * HK:(i + 1) * HK])
            w = _unpack(side.gate(step0 + i, w))
            if lead is not None and i == 0:
                res = _dot(w, _unpack(view(lead_v, lead, HK // 2)[...]), NN)
            else:
                res = _dot(w, xs[:, i * HK:(i + 1) * HK], NT)
            side.done(step0 + i, res)
            return res
        return [jnp.concatenate(row, axis=1) for row in _strassen(product)]

    def feat_stage(side, step0, j, xs, pair_fn, lead=None):
        sl = [[], []]
        for b in range(4):
            for q, res in enumerate(proj_unit(side, step0 + 7 * b, j, b, xs, lead if b == 0 else None)):
                sl[q] += [res[8 * i:8 * i + 8, :] for i in range(res.shape[0] // 8)]
            for q in (1, 0):
                for jj in (2 * (b % 2), 2 * (b % 2) + 1):
                    pair_fn(_pair_logits(sl[q][31 * (b // 2):], jj), 8 * q + 4 * (b // 2) + jj)

    def v_stage(side, xs, slot, first, publish, lead, plain=None):
        pending = None
        for g in range(4):
            if pending is not None:
                side.hooks.setdefault(7 * g + D_LAG, []).append(lambda p=pending: kv_update(*p))
            pending = (proj_unit(side, 7 * g, 2, g, xs, lead if g == 0 else None, plain if g < PLAIN_V0 else None),
                       slot, g, first, publish)
        side.check()
        return pending

    def pack_rows(src, dst, r0, rows, c0, cols, never, a):
        w = src[r0:r0 + rows, c0:c0 + cols].astype(F32)
        d = _lane_tile(a, cols // 128)
        w = jnp.concatenate([jnp.where(never, d, w[8 * i:8 * i + 8, :]) if i % 2 == 0 else w[8 * i:8 * i + 8, :]
                             for i in range(rows // 8)], axis=0)
        dst[r0 // 2:(r0 + rows) // 2, c0:c0 + cols] = _pack(w.astype(BF16))

    def stash_at(i, k, n):
        return zb_v.at[4 * i + 2 * (k // 16) + n, pl.ds(8 * (k % 16), 8), :]

    def stash(i, sl):
        for k, v in enumerate(sl):
            for n in range(2):
                stash_at(i, k, n)[...] = v[:, 128 * n:128 * n + 128]

    def stashed_k(i, slot, c, first):
        def job(k, a):
            j, n = k // 2, k % 2
            p = _pair_logits([stash_at(i, q, n)[...] for q in range(31)], j)
            k_pair([_after(p[0], never0, a)] + p[1:], slot, c * PPC + j, 128 * n, first, never0)
        return job

    def first_rows(k0, k1, n):
        xn = _unpack(xn_v[n * TH // 2:(n + 1) * TH // 2, :])
        ks = [k for k in range(k0, k1)]
        w = jnp.concatenate([wt_v[1][4 * (k % 32):4 * (k % 32) + 8, :] for k in ks[::2]], axis=0)
        res = _dot(_unpack(w), xn, NT)
        for q, k in enumerate(ks):
            if k % 32 < 31:
                stash_at(0, k % 32, n)[...] = res[8 * q:8 * q + 8, :]

    k0_copy(0).wait()
    x_copy(0).wait()
    wphi_copy(2).start()
    w_copy(1, 1).start()
    wphi_copy(3).start()
    x_copy(2).start()
    p0, p1 = fold_pairs(1, 0, 0)
    wt_v[1][8:64, :] = packed(p0[1:] + p1[1:])
    h_v[0][0:8, :] = p0[0]
    h_v[0][8:16, :] = p1[0]
    never0 = ln_rows(0, 0, TH, plain=True)[0, 0] < 0.0
    first_rows(2, 16, 0)

    k0_copy(1).wait()
    x_copy(1).wait()
    wphi_copy(1).wait()
    w_copy(1, 3).start()
    for c in (0, 2, 1, 3):
        w_copy(2, c).start()
    p2, p3 = fold_pairs(1, 0, 1)
    wt_v[1][0:8, :] = packed([share(h_v[0][0:8, :], p3[0], 1), share(h_v[0][8:16, :], p3[0], 2)])
    wt_v[1][64:128, :] = packed([share(p2[0], p3[0], 3)] + p2[1:] + p3[1:] + [jnp.zeros((8, D), F32)])
    made.add(("fold", 1, 0))
    ln_rows(0, 1, TH, plain=True)
    first_rows(16, 34, 0)
    first_rows(0, 16, 1)
    first_rows(16, 32, 1)
    expand_wphi(2)

    for c, prev in ((2, 0), (1, 2)):
        w_copy(1, c).wait()
        wphi_copy(4 - c).wait()
        expand_wphi(5 - 2 * c)
        side = _Side(never0)
        if c == 2:
            side.add(PRO_X0_PLAN, late_x_blocks(0))
        else:
            side.add(PRO_W0_PLAN, w_blocks(1))
        side.add((PRO_K_PLANS0, PRO_K_PLANS1)[2 - c], stashed_k(prev, 0, prev, True))
        fold(1, c, side, 0)
        stash(c, proj_feat(side, 4, c, xn_tile(0), None)[0])
        side.check()

    x_copy(2).wait()
    w_copy(1, 3).wait()
    x_copy(3).start()
    w_copy(0, 0).start()
    wo_copy(0).start()
    x_copy(4).start()
    for c in range(1, NC):
        w_copy(0, c).start()
    wo_copy(1).start()
    wr_copy.start()
    for i in range(4):
        stage_copy(i, 0).start()
    wg_copy.start()
    wu_copy.start()
    wd_copy.start()
    side = _Side(never0)
    side.add(PRO_LN1_PLAN, lambda k, a: ln_rows(1, k, LNC, never0, a, plain=True))
    side.add(PRO_W_PLAN, w_blocks(1, len(PRO_W0_PLAN)))
    side.add(PRO_K_PLANS2, stashed_k(1, 0, 1, False))
    fold(1, 3, side, 0)
    stash(3, proj_feat(side, 4, 3, xn_tile(0), None)[0])
    xn1 = xn_tile(1)
    spare = None
    for c in range(3):
        pk, spare = proj_feat(side, 8 + 4 * c, c, xn1, spare)
        if c < 2:
            k_features(pk, 1, c, c == 1, never0)
        else:
            stash(0, pk + [spare])
    side.check()

    for c in range(NC):
        w_copy(2, c).wait()
    side = _Side(never0)
    side.add(PRO_V_PLANS[0], v_transpose)
    side.add(PRO_V_PLANS[1], stashed_k(3, 0, 3, False))
    side.add(PRO_V_PLANS[2], stashed_k(0, 1, 2, False))
    side.add(PRO_V_PLANS[3], late_x_blocks(1))
    side.add(PRO_V_PLANS[4], w_blocks(2))
    spare = jnp.concatenate([stash_at(0, 31, n)[...] for n in range(2)], axis=1)
    k_features(proj_feat(side, -4, 3, xn_tile(1), spare)[0], 1, 3, True, never0)
    kv_update(*v_stage(side, xs_tile(0), 0, True, False, None, xn_tile(0)))
    save_lead(0)
    save_lead(1)
    for r0 in (0, 248):
        wt_v[0][r0:r0 + 8, :] = jnp.zeros((8, D), U32)

    def phase1(u, carry):
        never = u < 0

        @pl.when(u == 0)
        def _():
            x_copy(3).wait()
            w_copy(0, 0).wait()
            wo_copy(0).wait()

        @pl.when(u == 1)
        def _():
            x_copy(4).wait()
            w_copy(0, 1).wait()
            w_copy(0, 2).wait()
            wo_copy(1).wait()

        def wo_blocks(k, a):
            r0 = jnp.minimum(u * WO_ROWS, HK - WO_ROWS)
            lo, hi = [woraw_v.at[q, pl.ds(pl.multiple_of(r0, 16), WO_ROWS), :][16 * k:16 * k + 16, :].astype(F32)
                      for q in range(2)]
            put_blocks(wos_v.at[pl.ds(pl.multiple_of(r0 // 2, 8), WO_ROWS // 2), :], 8 * k, _strassen_rhs,
                       lo[:, :HK], lo[:, HK:], hi[:, :HK], hi[:, HK:], never, a)

        xs = xs_tile(2 * u + 1)
        side = _Side(never)
        for i in range(2):
            t = 2 * u + 2 + i
            if i == 0:
                side.add(LN1_PLANS[0], lambda k, a: ln_rows(2 * u + 2, k, LNC, never, a))
            pending = v_stage(side, xs, 1 - i, False, False, t - 1 if i == 0 else None)
            xs = xs_tile(t)
            side = _Side(never)
            if i == 0:
                side.add(LN1_PLANS[1], lambda k, a: ln_rows(2 * u + 3, k, LNC, never, a))
                side.add(WO_PLAN, wo_blocks)
            side.hooks[-28 + D_LAG] = [lambda p=pending: kv_update(*p)]
            feat_stage(side, -28, 1, xs, lambda p, pr: k_pair(p, i, pr, 0, False, never if i == 1 else None))
            save_lead(t)
        fold(0, u)
        return carry

    lax.fori_loop(0, (NT_ - 2) // 2, phase1, 0)

    w_copy(0, 3).wait()
    wr_copy.wait()
    side = _Side(never0)

    def z_final(k, a):
        zb_v[k] = jnp.broadcast_to(_row_sum(_after(z_v[k], never0, a)), (128, 128))

    side.add(END_PLANS[0], z_final)
    side.add(END_PLANS[1], w_blocks(0))
    fold(0, 3, side, 100)
    kv_update(*v_stage(side, xs_tile(NT_ - 1), 1, False, True, None))
    wr_v[...] = jnp.broadcast_to(wrraw_v[...].reshape(1, D).astype(F32), (8, D))

    def o_copy(r0, n, i):
        return pltpu.make_async_copy(o_v.at[pl.ds(r0, n), :], out_hbm.at[pl.ds(r0, n), :], sem.at[SO + i])

    def finish_rows(h_ref, k, t, valid, st, never=None, anchor=None):
        r0 = t * T + k * LNC
        best, besti = st["route"]
        wr = jnp.concatenate([wr_v[...]] * (LNC // 8), axis=0)
        sub = lax.broadcasted_iota(jnp.int32, (8, 1), 0)
        h = _after(h_ref[k * LNC:(k + 1) * LNC, :], never, anchor)
        hc = h - _row_sum(h) * (1.0 / D)
        rstd = lax.rsqrt(_row_sum(hc * hc) * (1.0 / D) + LN_EPS)
        r = (_row_sum(hc * wr) * rstd).astype(BF16).astype(F32)
        hn = hc * rstd
        view(hn_v, t, T // 2)[k * LNC // 2:(k + 1) * LNC // 2, :] = _pack(hn.astype(BF16))
        view(o_v, t, T)[k * LNC:(k + 1) * LNC, :] = (hn + h).astype(BF16)
        if valid is not None:
            r = jnp.where(valid, r, -jnp.inf)
        for i in range(LNC // 8):
            ri = r[8 * i:8 * i + 8, :]
            better = ri > best
            best = jnp.where(better, ri, best)
            besti = jnp.where(better, sub + (r0 + 8 * i), besti)
        st["route"] = (best, besti)
        return best

    def q_pair(p, slot, pr):
        ep, en, sp, sn = _dual_exp(p)
        zz = [_lane_tile(zb_v[pr, 8 * i:8 * i + 8, :], T // 128) for i in range(16)]
        ap = _pair_allreduce(_tree(jnp.add, [ep[i] * zz[i] for i in range(8)]), jnp.add)
        an = _pair_allreduce(_tree(jnp.add, [en[i] * zz[8 + i] for i in range(8)]), jnp.add)
        inv = _recip(ap * sn + (an + 1e-6 * sn) * sp)
        rp = sn * inv
        rn = sp * inv
        phi = jnp.concatenate([e * rp for e in ep] + [e * rn for e in en], axis=0)
        phi_v[slot][64 * pr:64 * pr + 64, :] = _pack(phi.astype(BF16))

    def attn_blocks(slot, g):
        lo, hi = [jnp.concatenate(
            [_dot(_unpack(kvbf_v[32 * pr:32 * pr + 32, :]), _unpack(phi_v[slot][64 * pr:64 * pr + 64, :]), NN)
             for pr in (2 * q, 2 * q + 1)], axis=0) for q in (g, g + 4)]
        blocks = _strassen_lhs(lo[:, :TH], hi[:, :TH], lo[:, TH:], hi[:, TH:])
        ot = _pack(jnp.concatenate(blocks, axis=1).astype(BF16).T)
        for i in range(7):
            oc_v[slot][:, i * HK + 128 * g:i * HK + 128 * g + 128] = ot[i * TH // 2:(i + 1) * TH // 2, :]

    def out_proj(side, step0, t, slot):
        xt = view(x_v, t, T)
        for n in range(4):
            def product(i):
                step = step0 + 7 * n + i
                w = side.gate(step, wos_v[:, i * HK + 128 * n:i * HK + 128 * n + 128])
                res = _dot(_unpack(oc_v[slot][:, i * HK:(i + 1) * HK]), _unpack(w), NN)
                side.done(step, res)
                return res
            for q, row in enumerate(_strassen(product)):
                for r, res in enumerate(row):
                    rows, cols = slice(q * TH, (q + 1) * TH), slice(r * HK + 128 * n, r * HK + 128 * n + 128)
                    h_v[slot][rows, cols] = res + xt[rows, cols].astype(F32)

    def phase2(u, carry):
        for i in range(4):
            stage_copy(i, u).wait()
        never = u < 0
        side = _Side(never)
        st = {"route": carry}
        tp = jnp.maximum(2 * u - 1, 0)
        side.add(LN2_PLANS[0], lambda k, a: finish_rows(h_v[1], k, tp, u > 0, st, never, a))
        side.add(LN2_PLANS[1], lambda k, a: finish_rows(h_v[0], k, 2 * u, None, st, never, a))

        def packer(i, dst, n):
            left = [n]

            def job(k, a):
                if i < 2:
                    pack_rows(stage_v[i], dst, (k // 2) * 16, 16, (0, D)[k % 2], (D, FM - D)[k % 2], never, a)
                else:
                    pack_rows(stage_v[i], dst, k * 16, 16, 0, D, never, a)
                left[0] -= 1
                if not left[0]:
                    stage_copy(i, jnp.minimum(u + 1, NQ - 1)).start()
                    n0 = stage_v[i].shape[0] - 16
                    side.deps.setdefault(PACK_DUE[i], []).append(stage_v[i][n0:n0 + 8, 0:128].astype(F32))
            return job

        for i in range(2):
            side.add(PACK_PLANS[i], packer(i, view((wgp_v, wup_v)[i], u, D // NQ // 2), len(PACK_PLANS[i])))
            d0 = pl.multiple_of(u * (DQ // 2) + i * (DQA // 2), 8)
            side.add(PACKD_PLANS[i], packer(2 + i, wdp_v.at[pl.ds(d0, 8 * len(PACKD_PLANS[i])), :],
                                            len(PACKD_PLANS[i])))
            for g in range(4):
                step = 107 + 28 * i + 7 * g + G_LAG
                side.hooks.setdefault(step if step < 156 else step - 156, []).append(
                    lambda i=i, g=g: attn_blocks(i, g))
        for i in range(2):
            feat_stage(side, 100 + 28 * i, 0, xs_tile(2 * u + i), lambda p, pr: q_pair(p, i, pr),
                       2 * u if i == 0 else None)
        for i in range(2):
            out_proj(side, 28 * i, 2 * u + i, i)
        side.check()

        @pl.when(u == 0)
        def _():
            o_copy(0, T, 0).start()

        @pl.when(u > 0)
        def _():
            o_copy(pl.multiple_of(tp * T, T), 2 * T, u).start()

        return st["route"]

    wg_copy.wait()
    wu_copy.wait()
    wd_copy.wait()
    route = lax.fori_loop(
        0, NT_ // 2, phase2,
        (jnp.full((8, 1), -jnp.inf, F32), jnp.zeros((8, 1), jnp.int32)))
    st = {"route": route}
    for k in range(T // LNC):
        finish_rows(h_v[1], k, NT_ - 1, None, st)
    best, besti = st["route"]
    o_copy(S - T, T, NT_).start()

    rmax = jnp.max(best, axis=0, keepdims=True)
    idx = jnp.min(jnp.where(best == rmax, besti, S), axis=0, keepdims=True)
    idx_s = jnp.clip(idx[0, 0], 0, S - 1)
    blk = pl.multiple_of((idx_s >> 4) << 4, 16)
    pair = jnp.broadcast_to(hn_v[pl.ds(idx_s >> 1, 1), :], (8, D))
    x8 = pltpu.bitcast(jnp.where((idx_s & 1) == 1, pair & jnp.uint32(0xFFFF0000), pair << 16), F32)
    xs = jnp.concatenate([x8, x8], axis=0).astype(BF16)
    acts, anchors = [], []

    def park(v, half):
        n = v.shape[0] // 128
        for i in range(n):
            z_v[i, :, 128 * half:128 * half + 128] = v[128 * i:128 * i + 128, :]
        return jnp.concatenate([z_v[i, :, 128 * half:128 * half + 128] for i in range(n)], axis=0)

    for c0 in range(0, FM, 128):
        g = _dot(xs, _unpack(wgp_v[:, c0:c0 + 128]), NN)[0:8, :]
        u = _dot(xs, _unpack(wup_v[:, c0:c0 + 128]), NN)[0:8, :]
        anchors += [g, u]
        acts.append(g * jax.nn.sigmoid(g) * u)
    xb = park(_col_broadcast(x8), 0)
    g, u = [_sublane_allreduce(_vpu_matvec(
        xb, lambda g: w[8 * g:8 * g + 8, :].astype(F32), never0,
        anchors[i * MOE_NA // 2:(i + 1) * MOE_NA // 2], MOE_LAGS[0])) for i, w in enumerate((wg_v, wu_v))]
    acts.append(g * jax.nn.sigmoid(g) * u)
    a = jnp.concatenate(acts, axis=1)
    am = jnp.concatenate([a[:, FVD:], a[:, FVD:]], axis=0).astype(BF16)
    ys, anchors = [], anchors[MOE_NA:]
    for k0 in range(0, FF - FVD, 512):
        k1 = min(k0 + 512, FF - FVD)
        yk = _dot(am[:, k0:k1], _unpack(wdp_v[k0 // 2:k1 // 2, 0:D]), NN)[0:8, :]
        ys.append(yk)
        anchors += [yk[:, c:c + 128] for c in range(128, D, 256)]
    ys.append(_sublane_allreduce(_vpu_matvec(
        park(_col_broadcast(a[:, :FVD]), 1), lambda g: wd_v[8 * g:8 * g + 8, :].astype(F32), never0,
        anchors[:-MOE_ND], MOE_LAGS[1])))
    y = _tree(jnp.add, ys) * jax.nn.sigmoid(rmax)
    y = jnp.concatenate([y, y], axis=0)
    sel = lax.broadcasted_iota(jnp.int32, (16, 1), 0) == (idx_s - blk)
    patch_v[...] = (o_v[pl.ds(blk, 16), :].astype(F32) + jnp.where(sel, y, 0.0)).astype(BF16)
    o_copy(0, T, 0).wait()
    for u in range(1, NT_ // 2):
        o_copy((2 * u - 1) * T, 2 * T, u).wait()
    o_copy(S - T, T, NT_).wait()
    pc = pltpu.make_async_copy(patch_v, out_hbm.at[pl.ds(blk, 16), :], sem.at[SM + 3])
    pc.start()
    for i in range(4):
        stage_copy(i, NQ - 1).wait()
    pc.wait()


@jax.jit
def pallas_sequential_preLN__linear_kernel_hedgehog__moe_arch_mod__prompt_kernel(
    A_x: jax.Array,
    A_wqkv: jax.Array,
    A_w_phi: jax.Array,
    A_wo: jax.Array,
    B_x: jax.Array,
    B_w_r: jax.Array,
    B_w_gate: jax.Array,
    B_w_up: jax.Array,
    B_w_down: jax.Array,
):
    del B_x
    hbm = pl.BlockSpec(memory_space=pl.ANY)
    out = pl.pallas_call(
        _kernel,
        out_shape=jax.ShapeDtypeStruct((S, D), BF16),
        in_specs=[hbm] * 8,
        out_specs=hbm,
        scratch_shapes=[
            pltpu.VMEM((S, D), BF16),
            pltpu.VMEM((T, D), U32),
            pltpu.VMEM((NT_ * TH // 2, SW), U32),
            pltpu.VMEM((NT_ * HK // 2, 128), U32),
            pltpu.VMEM((3 * NC, D, RC), BF16),
            [pltpu.VMEM((D // 2, D), U32)] * 3,
            [pltpu.VMEM((HK // 2, 7 * HK), U32)] * 3,
            pltpu.VMEM((H, DH, DH), BF16),
            pltpu.VMEM((8 * 64, 128), U32),
            pltpu.VMEM((2, HK, D), BF16),
            pltpu.VMEM((HK // 2, 7 * HK), U32),
            pltpu.VMEM((D,), BF16),
            pltpu.VMEM((8, D), F32),
            pltpu.VMEM((NPAIR, 64, 128), F32),
            pltpu.VMEM((NPAIR * 32, 128), U32),
            pltpu.VMEM((NPAIR, 128, T), F32),
            pltpu.VMEM((NPAIR, 128, 128), F32),
            [pltpu.VMEM((NPAIR * 64, T), U32)] * 2,
            [pltpu.VMEM((TH // 2, 7 * HK), U32)] * 2,
            [pltpu.VMEM((T, D), F32)] * 2,
            pltpu.VMEM((S // 2, D), U32),
            pltpu.VMEM((S, D), BF16),
            pltpu.VMEM((D, FV), BF16),
            pltpu.VMEM((D, FV), BF16),
            pltpu.VMEM((FVD, D), BF16),
            [pltpu.VMEM((D // NQ + 16, FM), BF16), pltpu.VMEM((D // NQ + 16, FM), BF16),
             pltpu.VMEM((DQA + 16, D), BF16), pltpu.VMEM((DQ - DQA + 16, D), BF16)],
            pltpu.VMEM((D // 2, FM), U32),
            pltpu.VMEM((D // 2, FM), U32),
            pltpu.VMEM(((FF - FVD) // 2, D + 128), U32),
            pltpu.VMEM((16, D), BF16),
            pltpu.SemaphoreType.DMA((6 + 3 * NC + NT_ + 16,)),
        ],
        compiler_params=pltpu.CompilerParams(vmem_limit_bytes=100 * 1024 * 1024,
                                             disable_semaphore_checks=True, disable_bounds_checks=True),
        name="hedgehog_mod",
    )(
        A_x.reshape(S, D),
        A_wqkv,
        A_w_phi,
        A_wo.reshape(2, HK, D),
        B_w_r,
        B_w_gate,
        B_w_up,
        B_w_down,
    )
    return out.reshape(1, S, D)
```

```python
import math

import jax
import jax.numpy as jnp
from jax import lax
import jax.experimental.pallas as pl
import jax.experimental.pallas.tpu as pltpu

F32 = jnp.float32
BF16 = jnp.bfloat16
U32 = jnp.uint32

S = 2048
D = 1024
H = 32
DH = 32
FF = 3584
NPAIR = H // 2
LOG2E = 1.4426950408889634
LN_EPS = 1e-5

T = 256
TH = T // 2
NT_ = S // T
RC = 256
NC = D // RC
PPC = RC // 64
LNC = 16

FV = 10 * 128
FM = FF - FV
FVD = 8 * 128
NQ = NT_ // 2
DQ = (FF - FVD) // NQ
WO_ROWS = 176
HK = D // 2
SW = 8 * HK


def _spread(n, a, b, due=None):
    rel = [round(a + (b - a) * k / (n - 1), 3) for k in range(n)]
    return tuple((r, None if due is None else math.ceil(r) + due) for r in rel)


LN1_PLANS = (((-0.191, 5), (1.306, 7), (3.323, 8), (3.523, 11), (6.057, 11), (7.922, 13), (7.945, 14), (10.63,
    16), (10.763, 16), (13.131, 19), (14.512, 19), (15.76, 22), (17.575, 24), (19.157, 26), (20.343, 25),
    (22.021, 27)), ((0.237, 5), (0.944, 7), (1.849, 9), (3.89, 10), (5.129, 10), (6.465, 11), (7.899, 13),
    (9.568, 15), (10.176, 17), (12.702, 18), (14.493, 19), (16.14, 21), (17.085, 22), (17.831, 25), (20.775,
    25), (21.371, 27)))
PRO_LN1_PLAN = ((None, None),) * 16
PRO_K_PLANS0 = ((0.387, None), (0.868, None), (1.931, None), (2.808, None), (3.563, None), (3.859, None),
    (5.723, None), (5.976, None))
PRO_K_PLANS1 = ((-0.801, None), (0.868, None), (1.348, None), (2.954, None), (3.692, None), (3.848, None),
    (4.564, None), (5.93, None))
PRO_X0_PLAN = ((-0.051, None), (1.782, None), (2.723, None), (3.011, None), (3.492, None), (4.967, None),
    (5.092, None), (6.096, None))
PRO_W0_PLAN = ((0.067, None), (0.461, None), (2.188, None), (2.659, None), (3.075, None), (4.159, None),
    (4.608, None), (5.388, None), (5.775, None), (6.465, None))
PRO_W_PLAN = ((0.061, None), (1.245, None), (2.122, None), (2.855, None), (3.761, None), (8.315, None),
    (9.157, None), (9.666, None), (10.34, None), (11.048, None), (11.734, None), (12.403, None), (13.06,
    None), (13.534, None), (14.283, None), (15.221, None), (15.794, None), (16.378, None), (17.14, None),
    (18.04, None), (18.337, None))
PRO_K_PLANS2 = ((15.07, None), (15.758, None), (16.112, None), (16.508, None), (16.901, None), (17.41, None),
    (17.583, None), (17.805, None))
PRO_V_PLANS = (((None, None), (None, None), (None, None), (None, None), (None, None), (None, None), (None,
    None), (None, None), (-3.698, None), (-3.111, None), (-3.087, None), (-2.462, None), (-2.293, None),
    (-1.979, None), (-1.839, None), (-1.668, None), (-1.468, None), (-1.38, None), (-1.34, None), (-0.246,
    None), (0.026, None), (0.474, None), (0.476, None), (0.947, None), (0.981, None), (1.114, None), (1.216,
    None), (1.832, None), (2.004, None), (2.278, None), (2.742, None), (2.753, None)), ((9.001, None),
    (10.016, None), (12.6, None), (12.987, None), (13.618, None), (15.819, None), (18.136, None), (18.844,
    None)), ((20.331, None), (21.315, None), (21.596, None), (22.158, None), (22.815, None), (23.574, None),
    (24.56, None), (25.611, None)), ((16.74, None), (18.43, None), (19.602, None), (20.486, None), (22.438,
    None), (23.401, None), (24.397, None), (24.753, None)), ((19.124, None), (20.055, None), (21.127, None),
    (22.04, None), (23.193, None), (24.942, None), (25.748, None), (26.177, None), (-1.605, None), (-0.08,
    None), (-0.053, None), (1.471, None), (1.872, None), (3.022, None), (3.843, None), (5.325, None), (5.371,
    None), (6.428, None), (7.2, None), (8.441, None), (8.924, None), (9.539, None), (10.795, None), (11.558,
    None), (11.943, None), (12.111, None), (13.8, None), (14.632, None), (15.534, None), (16.356, None),
    (17.103, None), (17.665, None)))
END_PLANS = (((-0.064, None), (2.011, None), (3.919, None), (5.535, None), (7.124, None), (8.225, None),
    (10.609, None), (11.952, None), (13.867, None), (15.593, None), (17.313, None), (19.413, None), (20.737,
    None), (22.258, None), (23.38, None), (25.845, None)), ((100.581, None), (101.301, None), (102.013, None),
    (0.409, None), (0.793, None), (2.353, None), (2.978, None), (3.797, None), (5.031, None), (6.008, None),
    (7.229, None), (7.974, None), (8.951, None), (10.186, None), (11.123, None), (11.847, None), (12.976,
    None), (13.561, None), (14.696, None), (15.721, None), (17.249, None), (18.073, None), (18.596, None),
    (19.613, None), (20.508, None), (21.155, None), (22.453, None), (23.06, None), (24.586, None), (25.242,
    None), (25.802, None)))
WO_PLAN = ((0.602, None), (3.254, None), (4.713, None), (8.79, None), (10.781, None), (12.669, None), (15.093,
    None), (17.749, None), (19.152, None), (22.501, None), (26.454, None))
LN2_PLANS = (((0.0, 5), (1.415, 7), (2.908, 7), (4.33, 10), (5.804, 12), (7.412, 12), (8.917, 14), (10.391,
    16), (11.855, 17), (13.254, 18), (14.771, 20), (16.149, 22), (17.577, 23), (19.143, 26), (20.595, 26),
    (22.085, 27)), ((28.5, 33), (29.891, 35), (31.241, 37), (32.825, 38), (34.046, 40), (35.536, 41), (37.183,
    44), (38.544, 44), (39.988, 45), (41.4, 48), (42.561, 47), (44.155, 51), (45.589, 53), (47.157, 52),
    (48.393, 53), (50.12, 55)))
PACK_PLANS = (((100.5, None), (101.289, None), (102.145, None), (102.911, None), (103.691, None), (104.613,
    None), (105.469, None), (106.258, None), (107.081, None), (107.888, None), (108.686, None), (109.548,
    None), (110.371, None), (111.194, None), (112.016, None), (112.707, None), (113.782, None), (114.555,
    None), (115.306, None), (116.167, None), (116.952, None), (117.901, None), (118.597, None), (119.419,
    None), (120.242, None), (121.081, None), (121.798, None), (122.845, None), (123.603, None), (124.075,
    None), (125.177, None), (126.165, None)), ((128.5, None), (129.295, None), (130.21, None), (130.932,
    None), (131.897, None), (132.656, None), (133.459, None), (134.258, None), (135.081, None), (135.921,
    None), (136.681, None), (137.548, None), (138.302, None), (139.194, None), (140.016, None), (140.936,
    None), (141.661, None), (142.448, None), (143.335, None), (144.04, None), (144.952, None), (145.824,
    None), (146.573, None), (147.419, None), (148.242, None), (149.241, None), (149.943, None), (150.71,
    None), (151.567, None), (152.241, None), (153.177, None), (154.0, None)))
PACKD_PLANS = (((0.406, None), (1.542, None), (2.517, None), (3.333, None), (4.276, None), (5.145, None),
    (6.328, None), (7.114, None), (8.056, None), (9.0, None), (9.973, None), (10.966, None), (11.824, None),
    (12.624, None), (13.722, None), (14.667, None), (15.574, None), (16.556, None), (17.43, None), (18.444,
    None), (19.496, None), (20.333, None), (21.241, None), (22.133, None), (23.167, None), (24.111, None),
    (24.81, None), (26.051, None)), ((28.5, None), (29.364, None), (30.227, None), (31.156, None), (31.858,
    None), (32.783, None), (33.682, None), (34.628, None), (35.409, None), (36.288, None), (37.136, None),
    (37.983, None)))
PACK_DUE = (130, 3, 30, 42)
DQA = 16 * len(PACKD_PLANS[0])
G_LAG = 5
D_LAG = 1
BLOCK_STAGGER = 4
BLOCK_DELAY = 4
PLAIN_V0 = 1
OC_PIN = 1
O_DUE = 5
MOE_NA = 36
MOE_ND = 2
MOE_LAGS = (2, 2)
STAGGER = 8

NN = (((1,), (0,)), ((), ()))
NT = (((1,), (1,)), ((), ()))


def _dot(a, b, dims):
    return lax.dot_general(a, b, dims, preferred_element_type=F32)


def _recip(x):
    return pl.reciprocal(x, approx=False, full_range=False)


def _pack(x):
    return pltpu.bitcast(x, U32)


def _unpack(x):
    return pltpu.bitcast(x, BF16)


def _strassen_lhs(a11, a12, a21, a22):
    return [a21 + a22, a22, a11 + a12, a11, a11 + a22, a12 - a22, a21 - a11]


def _strassen_rhs(b11, b12, b21, b22):
    return [b11, b21 - b11, b22, b12 - b22, b11 + b22, b21 + b22, b11 + b12]


def _strassen(product):
    m2 = product(0)
    m4 = product(1)
    c21 = m2 + m4
    m5 = product(2)
    u11 = m4 - m5
    m3 = product(3)
    c12 = m3 + m5
    u22 = m3 - m2
    m1 = product(4)
    u11 = u11 + m1
    u22 = u22 + m1
    c11 = product(5) + u11
    c22 = product(6) + u22
    return [[c11, c12], [c21, c22]]


def _pair_allreduce(a, op):
    a = op(a, pltpu.roll(a, 2, 0))
    return op(a, pltpu.roll(a, 4, 0))


def _tree(op, xs):
    xs = list(xs)
    while len(xs) > 1:
        nxt = [op(xs[i], xs[i + 1]) for i in range(0, len(xs) - 1, 2)]
        if len(xs) % 2:
            nxt.append(xs[-1])
        xs = nxt
    return xs[0]


def _pair_logits(sl, j):
    sub = lax.broadcasted_iota(jnp.int32, sl[0].shape, 0)
    if j < 3:
        head = jnp.where(sub < 2, 0.0, sl[(0, 1, 16)[j]])
    else:
        head = jnp.where(sub < 2, sl[0], jnp.where(sub < 4, pltpu.roll(sl[1], 2, 0),
                                                   jnp.where(sub < 6, pltpu.roll(sl[16], 4, 0), 0.0)))
    r0 = (2, 9, 17, 24)[j]
    return [head] + list(sl[r0:r0 + 7])


def _dual_exp(sl):
    mx = _pair_allreduce(_tree(jnp.maximum, sl), jnp.maximum)
    mn = _pair_allreduce(_tree(jnp.minimum, sl), jnp.minimum)
    ep = [jnp.exp2(s - mx) for s in sl]
    en = [jnp.exp2(mn - s) for s in sl]
    sp = _pair_allreduce(_tree(jnp.add, ep), jnp.add)
    sn = _pair_allreduce(_tree(jnp.add, en), jnp.add)
    return ep, en, sp, sn


def _after(x, never, anchor):
    if anchor is None:
        return x
    d = jnp.concatenate([anchor] * (x.shape[0] // 8), axis=0)
    if x.shape[1] == 128:
        return jnp.where(never, d, x)
    return jnp.concatenate([jnp.where(never, d, x[:, :128]), x[:, 128:]], axis=1)


def _gate(x, never, deps):
    for i, dep in enumerate(deps):
        d = jnp.broadcast_to(dep, (8, 128))
        if x.dtype != F32:
            d = pltpu.bitcast(d, x.dtype)
        blk = jnp.where(never, d, x[8 * i:8 * i + 8, :128])
        if x.shape[1] > 128:
            blk = jnp.concatenate([blk, x[8 * i:8 * i + 8, 128:]], axis=1)
        parts = ([x[:8 * i, :]] if i else []) + [blk, x[8 * i + 8:, :]]
        x = jnp.concatenate(parts, axis=0)
    return x


def _lane_fold(a):
    return _tree(jnp.add, [a[:, 128 * i:128 * i + 128] for i in range(a.shape[1] // 128)])


def _row_sum(a):
    return jnp.sum(_lane_fold(a), axis=-1, keepdims=True)


def _lane_tile(a, n):
    return a if n == 1 else jnp.concatenate([a] * n, axis=1)


def _sublane_allreduce(a):
    a = a + pltpu.roll(a, 4, 0)
    a = a + pltpu.roll(a, 2, 0)
    return a + pltpu.roll(a, 1, 0)


def _col_broadcast(row8):
    return jnp.concatenate([row8] * 16, axis=0).astype(BF16).T.astype(F32)


def _vpu_matvec(xb, w_rows, never, anchors, lag):
    ng = xb.shape[0] // 8
    acc, hist = None, []
    for g in range(ng):
        dep = anchors[(g * len(anchors)) // ng]
        if g >= lag:
            dep = dep + hist[g - lag]
        x = jnp.where(never, dep, xb[8 * g:8 * g + 8, :])
        w = w_rows(g)
        t = w * _lane_tile(x, w.shape[1] // 128)
        acc = t if acc is None else acc + t
        c = 128 * (g % (w.shape[1] // 128))
        hist.append(acc[:, c:c + 128])
    return acc


class _Side:
    def __init__(self, never):
        self.never = never
        self.jobs = []
        self.deps = {}
        self.hooks = {}

    def add(self, plan, fn):
        for k, (rel, due) in enumerate(plan):
            if rel is None:
                self._run(due, fn, k, None)
            else:
                self.jobs.append((rel, due, fn, k))

    def _run(self, due, fn, k, anchor):
        dep = fn(k, anchor)
        if due is not None:
            self.deps.setdefault(due, []).append(dep)

    def check(self):
        assert not self.jobs and not self.deps and not self.hooks

    def gate(self, step, x):
        return _gate(x, self.never, self.deps.pop(step, []))

    def done(self, step, res):
        m = res.shape[0] // 8
        for job in sorted([j for j in self.jobs if step - 1 < j[0] <= step], key=lambda j: j[0]):
            self.jobs.remove(job)
            g = m - 1 - int((step - job[0]) * m)
            self._run(job[1], job[2], job[3], res[8 * g:8 * g + 8, res.shape[1] - 128:])
        for fn in self.hooks.pop(step, []):
            fn()


def _kernel(x_hbm, wqkv_hbm, wphi_hbm, wo_hbm, wr_hbm, wg_hbm, wu_hbm, wd_hbm, out_hbm,
            x_v, xn_v, xs_v, lead_v, wraw_v, wt_v, ws_v, wphi_v, a_v, woraw_v, wos_v, wrraw_v, wr_v,
            kvacc_v, kvbf_v, z_v, zb_v, phi_v, oc_v, h_v, hn_v, o_v, wg_v, wu_v, wd_v, stage_v,
            wgp_v, wup_v, wdp_v, patch_v,
            sem):
    SX, SQ, SO, SM = 0, 6, 6 + 3 * NC, 6 + 3 * NC + NT_ + 1

    def x_copy(i):
        h0, h1 = ((0, 1), (1, 2), (2, 4), (4, 8), (8, 2 * NT_))[i]
        rows = pl.ds(h0 * TH, (h1 - h0) * TH)
        return pltpu.make_async_copy(x_hbm.at[rows, :], x_v.at[rows, :], sem.at[SX + i])

    def k0_copy(s):
        return pltpu.make_async_copy(wqkv_hbm.at[:, pl.ds(D + s * 128, 128)],
                                     wraw_v.at[NC, :, pl.ds(s * 128, 128)], sem.at[(SM + 7, SQ + NC)[s]])

    def w_copy(j, c):
        return pltpu.make_async_copy(wqkv_hbm.at[:, pl.ds(j * D + c * RC, RC)], wraw_v.at[j * NC + c],
                                     sem.at[SQ + j * NC + c])

    def wphi_copy(i):
        h0, h1 = ((0, 8), (16, 24), (8, 16), (24, H))[i]
        return pltpu.make_async_copy(wphi_hbm.at[pl.ds(h0, h1 - h0)], wphi_v.at[pl.ds(h0, h1 - h0)],
                                     sem.at[(SM + 4, SM + 8, SM + 9, SM + 14)[i]])

    wr_copy = pltpu.make_async_copy(wr_hbm, wrraw_v, sem.at[SM + 5])

    def wo_copy(i):
        rows = pl.ds(0, WO_ROWS) if i == 0 else pl.ds(WO_ROWS, HK - WO_ROWS)
        return pltpu.make_async_copy(wo_hbm.at[:, rows, :], woraw_v.at[:, rows, :], sem.at[(SM + 6, SX + 5)[i]])

    wg_copy = pltpu.make_async_copy(wg_hbm.at[:, pl.ds(FM, FV)], wg_v, sem.at[SM + 0])
    wu_copy = pltpu.make_async_copy(wu_hbm.at[:, pl.ds(FM, FV)], wu_v, sem.at[SM + 1])
    wd_copy = pltpu.make_async_copy(wd_hbm.at[pl.ds(0, FVD), :], wd_v, sem.at[SM + 2])

    def stage_copy(i, q):
        if i < 2:
            r0 = q * (D // NQ)
            r0 = r0 if isinstance(r0, int) else pl.multiple_of(r0, D // NQ)
            src = (wg_hbm, wu_hbm)[i].at[pl.ds(r0, D // NQ), pl.ds(0, FM)]
        else:
            r0 = FVD + q * DQ + (i - 2) * DQA
            r0 = r0 if isinstance(r0, int) else pl.multiple_of(r0, 16)
            src = wd_hbm.at[pl.ds(r0, (DQA, DQ - DQA)[i - 2]), :]
        return pltpu.make_async_copy(src, stage_v[i].at[pl.ds(0, src.shape[0]), :], sem.at[SM + 10 + i])

    wphi_copy(0).start()
    k0_copy(0).start()
    x_copy(0).start()
    k0_copy(1).start()
    x_copy(1).start()
    wphi_copy(1).start()
    w_copy(1, 2).start()

    made = set()

    def view(ref, i, n, off=0):
        r0 = off + i * n
        return ref.at[pl.ds(r0 if isinstance(r0, int) else pl.multiple_of(r0, math.gcd(n, off)), n), :]

    def put_blocks(dst, r0, fn, m11, m12, m21, m22, never, a, skip=()):
        w = HK // BLOCK_STAGGER
        for c0 in range(0, HK, w):
            d11, d22 = m11[:, c0:c0 + w], m22[:, c0:c0 + w]
            if a is not None:
                d = jnp.concatenate([_lane_tile(a, w // 128)] * 2, axis=0)
                d11, d22 = jnp.where(never, d, d11), jnp.where(never, d, d22)
            blocks = fn(d11, m12[:, c0:c0 + w], m21[:, c0:c0 + w], d22)
            for i, b in enumerate(blocks):
                if i not in skip:
                    dst[r0:r0 + 8, i * HK + c0:i * HK + c0 + w] = _pack(b.astype(BF16))
            a = blocks[6][8:16, w - 128:]
            for _ in range(BLOCK_DELAY):
                a = a * a

    def rows16(ref, r0):
        return _unpack(ref[r0:r0 + 8, :]).astype(F32)

    def x_blocks(t, k, lo, hi, never, a):
        put_blocks(view(xs_v, t, TH // 2), k * LNC // 2, _strassen_rhs,
                   lo[:, :HK], hi[:, :HK], lo[:, HK:], hi[:, HK:], never, a)

    def ln_rows(t, k, n, never=None, anchor=None, plain=False):
        x = _after(view(x_v, t, T)[k * n:(k + 1) * n, :].astype(F32), never, anchor)
        xc = x - _row_sum(x) * (1.0 / D)
        rstd = lax.rsqrt(_row_sum(xc * xc) * (1.0 / D) + LN_EPS)
        xn = xc * rstd
        if plain:
            xn_v[(t * T + k * n) // 2:(t * T + (k + 1) * n) // 2, :] = _pack(xn.astype(BF16))
        elif k * n < TH:
            xn_v[k * n // 2:(k + 1) * n // 2, :] = _pack(xn.astype(BF16))
        else:
            x_blocks(t, k - TH // LNC, rows16(xn_v, (k * n - TH) // 2), xn, never, xn[0:8, 0:128])
        return _tree(jnp.add, [rstd[8 * i:8 * i + 8, :] for i in range(min(n, LNC) // 8)])

    def late_x_blocks(t):
        return lambda k, a: x_blocks(t, k, rows16(xn_v, t * T // 2 + 8 * k),
                                     rows16(xn_v, (t * T + TH) // 2 + 8 * k), never0, a)

    def xn_tile(t):
        return _unpack(xn_v[t * T // 2:(t + 1) * T // 2, :])

    def xs_tile(t):
        return _unpack(view(xs_v, t, TH // 2)[:, 0:7 * HK])

    def expand_wphi(c):
        w = wphi_v[8 * c:8 * c + 8].reshape(8 * DH, DH).astype(F32).T
        bits = pltpu.bitcast(w, U32)
        head = lax.broadcasted_iota(jnp.int32, (DH, 128), 1) >> 5
        for s in range(2):
            b = bits[:, 128 * s:128 * s + 128]
            for j in range(2):
                r0 = 64 * (2 * c + s) + 32 * j
                a_v[r0:r0 + 32, :] = jnp.where(head == 2 * j, b >> 16,
                                               jnp.where(head == 2 * j + 1, b, jnp.uint32(0)))

    wphi_copy(0).wait()
    expand_wphi(0)
    h_v[1][...] = jnp.zeros((T, D), F32)
    if OC_PIN:
        for ref in oc_v:
            ref[0:8, 0:128] = jnp.zeros((8, 128), U32)
    for ref in stage_v:
        ref[ref.shape[0] - 16:, 0:128] = jnp.zeros((16, 128), BF16)

    def v_transpose(k, a):
        q, r0 = (k // 8) + 4 * (k % 2), 256 * (k % 8 // 2)
        w = wraw_v[2 * NC + q // 2, r0:r0 + 256, (q % 2) * 128:(q % 2) * 128 + 128]
        if a is not None:
            w = _unpack(jnp.where(never0, jnp.concatenate([pltpu.bitcast(a, U32)] * 16, axis=0), _pack(w)))
        wt_v[2][64 * q:64 * q + 64, r0:r0 + 256] = _pack(w.T)
        made.add(("vt", k))

    def fold_pairs(j, c, s, side=None, step0=None):
        g0 = 64 * (2 * c + s)
        g0 = g0 if isinstance(g0, int) else pl.multiple_of(g0, 64)
        res = _dot(_unpack(a_v[pl.ds(g0, 64), :]), wraw_v[j * NC + c, :, s * 128:(s + 1) * 128], NT)
        if side is not None:
            side.done(step0 + 2 * s, res[:, :D // 2])
            side.done(step0 + 2 * s + 1, res[:, D // 2:])
        sub = lax.broadcasted_iota(jnp.int32, (8, D), 0)
        out = []
        for q in range(2):
            base = _pair_allreduce(jnp.where(sub < 2, res[64 * q:64 * q + 8, :], 0.0), jnp.add)
            out.append([(res[64 * q + 8 * i:64 * q + 8 * i + 8, :] - base) * LOG2E for i in range(8)])
        return out

    def share(z, z3, k):
        sub = lax.broadcasted_iota(jnp.int32, (8, D), 0)
        return jnp.where(sub < 2, pltpu.roll(z3, 8 - 2 * k, 0), z)

    def packed(slabs):
        return _pack(jnp.concatenate(slabs, axis=0).astype(BF16))

    def fold(j, c, side=None, step0=None):
        p0, p1 = fold_pairs(j, c, 0, side, step0)
        p2, p3 = fold_pairs(j, c, 1, side, step0)
        sl = ([share(p0[0], p3[0], 1), share(p1[0], p3[0], 2)] + p0[1:] + p1[1:]
              + [share(p2[0], p3[0], 3)] + p2[1:] + p3[1:])
        zero = jnp.zeros((8, D), F32)
        even, odd = sl + [zero], [zero] + sl
        r0 = 8 * ((31 * c) // 2)
        is_odd = c % 2 == 1
        if isinstance(c, int):
            sl = odd if is_odd else even
        else:
            r0 = pl.multiple_of(r0, 8)
            sl = [jnp.where(is_odd, o, e) for o, e in zip(odd, even)]
        win = wt_v[j].at[pl.ds(r0, 128), :]
        win[8:128, :] = packed(sl[2:])
        first = packed(sl[:2])
        if is_odd is not False:
            keep = lax.broadcasted_iota(jnp.int32, (8, D), 0) < jnp.where(is_odd, 4, 0)
            first = jnp.where(keep, win[0:8, :], first)
        win[0:8, :] = first
        made.update(("fold", j, q) for q in ([c] if isinstance(c, int) else range(3)))

    def w_blocks(j, k0=0):
        def job(k, a):
            k += k0
            assert made >= ({("vt", 8 * (k // 8) + q) for q in range(8)} if j == 2 else
                            {("fold", j, q) for q in ((0, 2) if k < 15 else range(4))})
            made.add(("ws", j, k))
            lo, hi = rows16(wt_v[j], 8 * k), rows16(wt_v[j], (256 if j == 2 else 248) + 8 * k)
            put_blocks(ws_v[j], 8 * k, _strassen_lhs, lo[:, :HK], lo[:, HK:], hi[:, :HK], hi[:, HK:], never0, a,
                       skip=(1, 3))
        return job

    def k_pair(p, slot, pr, c0, first, never=None):
        for n in range(c0, c0 + p[0].shape[1], 128):
            assert first == (("z", pr, n) not in made)
            made.update({("z", pr, n), ("phi", slot, pr, n)})
        ep, en, sp, sn = _dual_exp(p)
        inv = _recip(sp * sn)
        scale = (sn * inv, sp * inv)
        es = ep + en
        cols = slice(c0, c0 + p[0].shape[1])
        n = 16 if never is None else 16 // STAGGER
        last = None
        for q in range(16 // n):
            sc = scale
            if last is not None:
                sc = [jnp.where(never, last, x) for x in scale]
            phi = jnp.concatenate([es[i] * sc[i // 8] for i in range(q * n, (q + 1) * n)], axis=0)
            rows = slice(8 * q * n, 8 * (q + 1) * n)
            z = phi if first else z_v[pr, rows, cols] + phi
            z_v[pr, rows, cols] = z
            phi_v[slot][64 * pr + 4 * q * n:64 * pr + 4 * (q + 1) * n, cols] = _pack(phi.astype(BF16))
            last = z[8 * n - 8:, :]

    def k_features(pk, slot, c, first, never=None):
        for j in range(PPC):
            k_pair(_pair_logits(pk, j), slot, c * PPC + j, 0, first, never)

    def kv_update(vts, slot, g, first, publish=False):
        for q, vt in enumerate(vts):
            for j in range(2):
                pr = 2 * g + 8 * q + j
                assert made >= {("phi", slot, pr, 0), ("phi", slot, pr, 128)}
                upd = _dot(vt[64 * j:64 * j + 64, :].astype(BF16), _unpack(phi_v[slot][64 * pr:64 * pr + 64, :]), NT)
                acc = upd if first else kvacc_v[pr] + upd
                kvacc_v[pr] = acc
                if publish:
                    odd = -(lax.broadcasted_iota(jnp.int32, (32, 128), 1) & 1)
                    bits = pltpu.bitcast(acc, jnp.int32) & jnp.concatenate([~odd, odd], axis=0)
                    kvbf_v[32 * pr:32 * pr + 32, :] = _pack(pltpu.bitcast(bits, F32).astype(BF16))

    def save_lead(t):
        view(lead_v, t, HK // 2)[...] = _pack(_unpack(view(xs_v, t, TH // 2)[:, 0:HK]).T)

    def proj_feat(side, step0, c, xn, carry):
        r0 = 8 * ((31 * c) // 2)
        skip = 8 if c % 2 == 1 and carry is not None else 0
        w = wt_v[1][r0 + skip:r0 + 128, :]
        quarters = []
        for n in range(2):
            for m in range(2):
                step = step0 + 2 * n + m
                wq = _unpack(side.gate(step, w[:64, :] if m == 0 else w[64:, :]))
                res = _dot(wq, xn[n * TH:(n + 1) * TH, :], NT)
                side.done(step, res)
                quarters.append(res)
        res = jnp.concatenate(
            [jnp.concatenate([quarters[0], quarters[2]], axis=1),
             jnp.concatenate([quarters[1], quarters[3]], axis=1)], axis=0)
        sl = [res[8 * i:8 * i + 8, :] for i in range(res.shape[0] // 8)]
        if c % 2 == 0:
            return sl[:31], sl[31]
        return ([carry] + sl if skip else sl[1:]), None

    def proj_unit(side, step0, j, b, xs, lead=None, plain=None):
        r1 = 64 * b + (64 if j == 2 or b < 3 else 56)
        assert made >= ({("vt", 8 * b + q) for q in range(8)} if plain is not None else
                        {("ws", j, k) for k in range(8 * b, r1 // 8)})
        if plain is not None:
            out = []
            for q in range(2):
                row = []
                for n in range(2):
                    res = _dot(_unpack(wt_v[2][256 * q + 64 * b:256 * q + r1, :]), plain[n * TH:(n + 1) * TH, :], NT)
                    for i in range((0, 2, 4, 5)[2 * q + n], (2, 4, 5, 7)[2 * q + n]):
                        side.done(step0 + i, res)
                    row.append(res)
                out.append(jnp.concatenate(row, axis=1))
            return out

        def product(i):
            off = 256 if j == 2 else 248
            w = (wt_v[j][off + 64 * b:off + r1, HK:] if i == 1 else wt_v[j][64 * b:r1, :HK] if i == 3
                 else ws_v[j][64 * b:r1, i * HK:(i + 1) * HK])
            w = _unpack(side.gate(step0 + i, w))
            if lead is not None and i == 0:
                res = _dot(w, _unpack(view(lead_v, lead, HK // 2)[...]), NN)
            else:
                res = _dot(w, xs[:, i * HK:(i + 1) * HK], NT)
            side.done(step0 + i, res)
            return res
        return [jnp.concatenate(row, axis=1) for row in _strassen(product)]

    def feat_stage(side, step0, j, xs, pair_fn, lead=None):
        sl = [[], []]
        for b in range(4):
            for q, res in enumerate(proj_unit(side, step0 + 7 * b, j, b, xs, lead if b == 0 else None)):
                sl[q] += [res[8 * i:8 * i + 8, :] for i in range(res.shape[0] // 8)]
            for q in (1, 0):
                for jj in (2 * (b % 2), 2 * (b % 2) + 1):
                    pair_fn(_pair_logits(sl[q][31 * (b // 2):], jj), 8 * q + 4 * (b // 2) + jj)

    def v_stage(side, xs, slot, first, publish, lead, plain=None):
        pending = None
        for g in range(4):
            if pending is not None:
                side.hooks.setdefault(7 * g + D_LAG, []).append(lambda p=pending: kv_update(*p))
            pending = (proj_unit(side, 7 * g, 2, g, xs, lead if g == 0 else None, plain if g < PLAIN_V0 else None),
                       slot, g, first, publish)
        side.check()
        return pending

    def pack_rows(src, dst, r0, rows, c0, cols, never, a):
        w = src[r0:r0 + rows, c0:c0 + cols].astype(F32)
        d = _lane_tile(a, cols // 128)
        w = jnp.concatenate([jnp.where(never, d, w[8 * i:8 * i + 8, :]) if i % 2 == 0 else w[8 * i:8 * i + 8, :]
                             for i in range(rows // 8)], axis=0)
        dst[r0 // 2:(r0 + rows) // 2, c0:c0 + cols] = _pack(w.astype(BF16))

    def stash_at(i, k, n):
        return zb_v.at[4 * i + 2 * (k // 16) + n, pl.ds(8 * (k % 16), 8), :]

    def stash(i, sl):
        for k, v in enumerate(sl):
            for n in range(2):
                stash_at(i, k, n)[...] = v[:, 128 * n:128 * n + 128]

    def stashed_k(i, slot, c, first):
        def job(k, a):
            j, n = k // 2, k % 2
            p = _pair_logits([stash_at(i, q, n)[...] for q in range(31)], j)
            k_pair([_after(p[0], never0, a)] + p[1:], slot, c * PPC + j, 128 * n, first, never0)
        return job

    def first_rows(k0, k1, n):
        xn = _unpack(xn_v[n * TH // 2:(n + 1) * TH // 2, :])
        ks = [k for k in range(k0, k1)]
        w = jnp.concatenate([wt_v[1][4 * (k % 32):4 * (k % 32) + 8, :] for k in ks[::2]], axis=0)
        res = _dot(_unpack(w), xn, NT)
        for q, k in enumerate(ks):
            if k % 32 < 31:
                stash_at(0, k % 32, n)[...] = res[8 * q:8 * q + 8, :]

    k0_copy(0).wait()
    x_copy(0).wait()
    wphi_copy(2).start()
    w_copy(1, 1).start()
    wphi_copy(3).start()
    x_copy(2).start()
    p0, p1 = fold_pairs(1, 0, 0)
    wt_v[1][8:64, :] = packed(p0[1:] + p1[1:])
    h_v[0][0:8, :] = p0[0]
    h_v[0][8:16, :] = p1[0]
    never0 = ln_rows(0, 0, TH, plain=True)[0, 0] < 0.0
    first_rows(2, 16, 0)

    k0_copy(1).wait()
    x_copy(1).wait()
    wphi_copy(1).wait()
    w_copy(1, 3).start()
    for c in (0, 2, 1, 3):
        w_copy(2, c).start()
    p2, p3 = fold_pairs(1, 0, 1)
    wt_v[1][0:8, :] = packed([share(h_v[0][0:8, :], p3[0], 1), share(h_v[0][8:16, :], p3[0], 2)])
    wt_v[1][64:128, :] = packed([share(p2[0], p3[0], 3)] + p2[1:] + p3[1:] + [jnp.zeros((8, D), F32)])
    made.add(("fold", 1, 0))
    ln_rows(0, 1, TH, plain=True)
    first_rows(16, 34, 0)
    first_rows(0, 16, 1)
    first_rows(16, 32, 1)
    expand_wphi(2)

    for c, prev in ((2, 0), (1, 2)):
        w_copy(1, c).wait()
        wphi_copy(4 - c).wait()
        expand_wphi(5 - 2 * c)
        side = _Side(never0)
        if c == 2:
            side.add(PRO_X0_PLAN, late_x_blocks(0))
        else:
            side.add(PRO_W0_PLAN, w_blocks(1))
        side.add((PRO_K_PLANS0, PRO_K_PLANS1)[2 - c], stashed_k(prev, 0, prev, True))
        fold(1, c, side, 0)
        stash(c, proj_feat(side, 4, c, xn_tile(0), None)[0])
        side.check()

    x_copy(2).wait()
    w_copy(1, 3).wait()
    x_copy(3).start()
    w_copy(0, 0).start()
    wo_copy(0).start()
    x_copy(4).start()
    for c in range(1, NC):
        w_copy(0, c).start()
    wo_copy(1).start()
    wr_copy.start()
    for i in range(4):
        stage_copy(i, 0).start()
    wg_copy.start()
    wu_copy.start()
    wd_copy.start()
    side = _Side(never0)
    side.add(PRO_LN1_PLAN, lambda k, a: ln_rows(1, k, LNC, never0, a, plain=True))
    side.add(PRO_W_PLAN, w_blocks(1, len(PRO_W0_PLAN)))
    side.add(PRO_K_PLANS2, stashed_k(1, 0, 1, False))
    fold(1, 3, side, 0)
    stash(3, proj_feat(side, 4, 3, xn_tile(0), None)[0])
    xn1 = xn_tile(1)
    spare = None
    for c in range(3):
        pk, spare = proj_feat(side, 8 + 4 * c, c, xn1, spare)
        if c < 2:
            k_features(pk, 1, c, c == 1, never0)
        else:
            stash(0, pk + [spare])
    side.check()

    for c in range(NC):
        w_copy(2, c).wait()
    side = _Side(never0)
    side.add(PRO_V_PLANS[0], v_transpose)
    side.add(PRO_V_PLANS[1], stashed_k(3, 0, 3, False))
    side.add(PRO_V_PLANS[2], stashed_k(0, 1, 2, False))
    side.add(PRO_V_PLANS[3], late_x_blocks(1))
    side.add(PRO_V_PLANS[4], w_blocks(2))
    spare = jnp.concatenate([stash_at(0, 31, n)[...] for n in range(2)], axis=1)
    k_features(proj_feat(side, -4, 3, xn_tile(1), spare)[0], 1, 3, True, never0)
    kv_update(*v_stage(side, xs_tile(0), 0, True, False, None, xn_tile(0)))
    save_lead(0)
    save_lead(1)
    for r0 in (0, 248):
        wt_v[0][r0:r0 + 8, :] = jnp.zeros((8, D), U32)

    def phase1(u, carry):
        never = u < 0

        @pl.when(u == 0)
        def _():
            x_copy(3).wait()
            w_copy(0, 0).wait()
            wo_copy(0).wait()

        @pl.when(u == 1)
        def _():
            x_copy(4).wait()
            w_copy(0, 1).wait()
            w_copy(0, 2).wait()
            wo_copy(1).wait()

        def wo_blocks(k, a):
            r0 = jnp.minimum(u * WO_ROWS, HK - WO_ROWS)
            lo, hi = [woraw_v.at[q, pl.ds(pl.multiple_of(r0, 16), WO_ROWS), :][16 * k:16 * k + 16, :].astype(F32)
                      for q in range(2)]
            put_blocks(wos_v.at[pl.ds(pl.multiple_of(r0 // 2, 8), WO_ROWS // 2), :], 8 * k, _strassen_rhs,
                       lo[:, :HK], lo[:, HK:], hi[:, :HK], hi[:, HK:], never, a)

        xs = xs_tile(2 * u + 1)
        side = _Side(never)
        for i in range(2):
            t = 2 * u + 2 + i
            if i == 0:
                side.add(LN1_PLANS[0], lambda k, a: ln_rows(2 * u + 2, k, LNC, never, a))
            pending = v_stage(side, xs, 1 - i, False, False, t - 1 if i == 0 else None)
            xs = xs_tile(t)
            side = _Side(never)
            if i == 0:
                side.add(LN1_PLANS[1], lambda k, a: ln_rows(2 * u + 3, k, LNC, never, a))
                side.add(WO_PLAN, wo_blocks)
            side.hooks[-28 + D_LAG] = [lambda p=pending: kv_update(*p)]
            feat_stage(side, -28, 1, xs, lambda p, pr: k_pair(p, i, pr, 0, False, never if i == 1 else None))
            save_lead(t)
        fold(0, u)
        return carry

    lax.fori_loop(0, (NT_ - 2) // 2, phase1, 0)

    w_copy(0, 3).wait()
    wr_copy.wait()
    side = _Side(never0)

    def z_final(k, a):
        zb_v[k] = jnp.broadcast_to(_row_sum(_after(z_v[k], never0, a)), (128, 128))

    side.add(END_PLANS[0], z_final)
    side.add(END_PLANS[1], w_blocks(0))
    fold(0, 3, side, 100)
    kv_update(*v_stage(side, xs_tile(NT_ - 1), 1, False, True, None))
    wr_v[...] = jnp.broadcast_to(wrraw_v[...].reshape(1, D).astype(F32), (8, D))

    def o_copy(r0, n, i):
        return pltpu.make_async_copy(o_v.at[pl.ds(r0, n), :], out_hbm.at[pl.ds(r0, n), :], sem.at[SO + i])

    def finish_rows(h_ref, k, t, valid, st, never=None, anchor=None):
        r0 = t * T + k * LNC
        best, besti = st["route"]
        wr = jnp.concatenate([wr_v[...]] * (LNC // 8), axis=0)
        sub = lax.broadcasted_iota(jnp.int32, (8, 1), 0)
        h = _after(h_ref[k * LNC:(k + 1) * LNC, :], never, anchor)
        hc = h - _row_sum(h) * (1.0 / D)
        rstd = lax.rsqrt(_row_sum(hc * hc) * (1.0 / D) + LN_EPS)
        r = (_row_sum(hc * wr) * rstd).astype(BF16).astype(F32)
        hn = hc * rstd
        view(hn_v, t, T // 2)[k * LNC // 2:(k + 1) * LNC // 2, :] = _pack(hn.astype(BF16))
        view(o_v, t, T)[k * LNC:(k + 1) * LNC, :] = (hn + h).astype(BF16)
        if valid is not None:
            r = jnp.where(valid, r, -jnp.inf)
        for i in range(LNC // 8):
            ri = r[8 * i:8 * i + 8, :]
            better = ri > best
            best = jnp.where(better, ri, best)
            besti = jnp.where(better, sub + (r0 + 8 * i), besti)
        st["route"] = (best, besti)
        return best

    def q_pair(p, slot, pr):
        ep, en, sp, sn = _dual_exp(p)
        zz = [_lane_tile(zb_v[pr, 8 * i:8 * i + 8, :], T // 128) for i in range(16)]
        ap = _pair_allreduce(_tree(jnp.add, [ep[i] * zz[i] for i in range(8)]), jnp.add)
        an = _pair_allreduce(_tree(jnp.add, [en[i] * zz[8 + i] for i in range(8)]), jnp.add)
        inv = _recip(ap * sn + (an + 1e-6 * sn) * sp)
        rp = sn * inv
        rn = sp * inv
        phi = jnp.concatenate([e * rp for e in ep] + [e * rn for e in en], axis=0)
        phi_v[slot][64 * pr:64 * pr + 64, :] = _pack(phi.astype(BF16))

    held = []

    def attn_blocks(slot, g, deps):
        lo, hi = [jnp.concatenate(
            [_dot(_unpack(kvbf_v[32 * pr:32 * pr + 32, :]), _unpack(phi_v[slot][64 * pr:64 * pr + 64, :]), NN)
             for pr in (2 * q, 2 * q + 1)], axis=0) for q in (g, g + 4)]
        blocks = [(i, g, b) for i, b in enumerate(_strassen_lhs(lo[:, :TH], hi[:, :TH], lo[:, TH:], hi[:, TH:]))]
        if g % 2 == 0:
            held.append(blocks.pop())
        else:
            blocks.append(held.pop())
        ot = _pack(jnp.concatenate([b for _, _, b in blocks], axis=1).astype(BF16).T)
        for q, (i, n, _) in enumerate(blocks):
            oc_v[slot][:, i * HK + 128 * n:i * HK + 128 * n + 128] = ot[q * TH // 2:(q + 1) * TH // 2, :]
            if q % 2:
                deps.append(pltpu.bitcast(ot[(q + 1) * TH // 2 - 8:(q + 1) * TH // 2, :], F32))

    def out_proj(side, step0, t, slot):
        xt = view(x_v, t, T)
        for n in range(4):
            def product(i):
                step = step0 + 7 * n + i
                w = side.gate(step, wos_v[:, i * HK + 128 * n:i * HK + 128 * n + 128])
                res = _dot(_unpack(oc_v[slot][:, i * HK:(i + 1) * HK]), _unpack(w), NN)
                side.done(step, res)
                return res
            for q, row in enumerate(_strassen(product)):
                for r, res in enumerate(row):
                    rows, cols = slice(q * TH, (q + 1) * TH), slice(r * HK + 128 * n, r * HK + 128 * n + 128)
                    h_v[slot][rows, cols] = res + xt[rows, cols].astype(F32)

    def phase2(u, carry):
        for i in range(4):
            stage_copy(i, u).wait()
        never = u < 0
        side = _Side(never)
        st = {"route": carry}
        tp = jnp.maximum(2 * u - 1, 0)
        side.add(LN2_PLANS[0], lambda k, a: finish_rows(h_v[1], k, tp, u > 0, st, never, a))
        side.add(LN2_PLANS[1], lambda k, a: finish_rows(h_v[0], k, 2 * u, None, st, never, a))

        def packer(i, dst, n):
            left = [n]

            def job(k, a):
                if i < 2:
                    pack_rows(stage_v[i], dst, (k // 2) * 16, 16, (0, D)[k % 2], (D, FM - D)[k % 2], never, a)
                else:
                    pack_rows(stage_v[i], dst, k * 16, 16, 0, D, never, a)
                left[0] -= 1
                if not left[0]:
                    stage_copy(i, jnp.minimum(u + 1, NQ - 1)).start()
                    n0 = stage_v[i].shape[0] - 16
                    side.deps.setdefault(PACK_DUE[i], []).append(stage_v[i][n0:n0 + 8, 0:128].astype(F32))
            return job

        for i in range(2):
            side.add(PACK_PLANS[i], packer(i, view((wgp_v, wup_v)[i], u, D // NQ // 2), len(PACK_PLANS[i])))
            d0 = pl.multiple_of(u * (DQ // 2) + i * (DQA // 2), 8)
            side.add(PACKD_PLANS[i], packer(2 + i, wdp_v.at[pl.ds(d0, 8 * len(PACKD_PLANS[i])), :],
                                            len(PACKD_PLANS[i])))
            for g in range(4):
                step = 107 + 28 * i + 7 * g + G_LAG
                side.hooks.setdefault(step % 156, []).append(
                    lambda i=i, g=g, due=(step + O_DUE) % 156: attn_blocks(i, g, side.deps.setdefault(due, [])))
        for i in range(2):
            feat_stage(side, 100 + 28 * i, 0, xs_tile(2 * u + i), lambda p, pr: q_pair(p, i, pr),
                       2 * u if i == 0 else None)
        for i in range(2):
            out_proj(side, 28 * i, 2 * u + i, i)
        side.check()

        @pl.when(u == 0)
        def _():
            o_copy(0, T, 0).start()

        @pl.when(u > 0)
        def _():
            o_copy(pl.multiple_of(tp * T, T), 2 * T, u).start()

        return st["route"]

    wg_copy.wait()
    wu_copy.wait()
    wd_copy.wait()
    route = lax.fori_loop(
        0, NT_ // 2, phase2,
        (jnp.full((8, 1), -jnp.inf, F32), jnp.zeros((8, 1), jnp.int32)))
    st = {"route": route}
    for k in range(T // LNC):
        finish_rows(h_v[1], k, NT_ - 1, None, st)
    best, besti = st["route"]
    o_copy(S - T, T, NT_).start()

    rmax = jnp.max(best, axis=0, keepdims=True)
    idx = jnp.min(jnp.where(best == rmax, besti, S), axis=0, keepdims=True)
    idx_s = jnp.clip(idx[0, 0], 0, S - 1)
    blk = pl.multiple_of((idx_s >> 4) << 4, 16)
    pair = jnp.broadcast_to(hn_v[pl.ds(idx_s >> 1, 1), :], (8, D))
    x8 = pltpu.bitcast(jnp.where((idx_s & 1) == 1, pair & jnp.uint32(0xFFFF0000), pair << 16), F32)
    xs = jnp.concatenate([x8, x8], axis=0).astype(BF16)
    acts, anchors = [], []

    def park(v, half):
        n = v.shape[0] // 128
        for i in range(n):
            z_v[i, :, 128 * half:128 * half + 128] = v[128 * i:128 * i + 128, :]
        return jnp.concatenate([z_v[i, :, 128 * half:128 * half + 128] for i in range(n)], axis=0)

    for c0 in range(0, FM, 128):
        g = _dot(xs, _unpack(wgp_v[:, c0:c0 + 128]), NN)[0:8, :]
        u = _dot(xs, _unpack(wup_v[:, c0:c0 + 128]), NN)[0:8, :]
        anchors += [g, u]
        acts.append(g * jax.nn.sigmoid(g) * u)
    xb = park(_col_broadcast(x8), 0)
    g, u = [_sublane_allreduce(_vpu_matvec(
        xb, lambda g: w[8 * g:8 * g + 8, :].astype(F32), never0,
        anchors[i * MOE_NA // 2:(i + 1) * MOE_NA // 2], MOE_LAGS[0])) for i, w in enumerate((wg_v, wu_v))]
    acts.append(g * jax.nn.sigmoid(g) * u)
    a = jnp.concatenate(acts, axis=1)
    am = jnp.concatenate([a[:, FVD:], a[:, FVD:]], axis=0).astype(BF16)
    ys, anchors = [], anchors[MOE_NA:]
    for k0 in range(0, FF - FVD, 512):
        k1 = min(k0 + 512, FF - FVD)
        yk = _dot(am[:, k0:k1], _unpack(wdp_v[k0 // 2:k1 // 2, 0:D]), NN)[0:8, :]
        ys.append(yk)
        anchors += [yk[:, c:c + 128] for c in range(128, D, 256)]
    ys.append(_sublane_allreduce(_vpu_matvec(
        park(_col_broadcast(a[:, :FVD]), 1), lambda g: wd_v[8 * g:8 * g + 8, :].astype(F32), never0,
        anchors[:-MOE_ND], MOE_LAGS[1])))
    y = _tree(jnp.add, ys) * jax.nn.sigmoid(rmax)
    y = jnp.concatenate([y, y], axis=0)
    sel = lax.broadcasted_iota(jnp.int32, (16, 1), 0) == (idx_s - blk)
    patch_v[...] = (o_v[pl.ds(blk, 16), :].astype(F32) + jnp.where(sel, y, 0.0)).astype(BF16)
    o_copy(0, T, 0).wait()
    for u in range(1, NT_ // 2):
        o_copy((2 * u - 1) * T, 2 * T, u).wait()
    o_copy(S - T, T, NT_).wait()
    pc = pltpu.make_async_copy(patch_v, out_hbm.at[pl.ds(blk, 16), :], sem.at[SM + 3])
    pc.start()
    for i in range(4):
        stage_copy(i, NQ - 1).wait()
    pc.wait()


@jax.jit
def pallas_sequential_preLN__linear_kernel_hedgehog__moe_arch_mod__prompt_kernel(
    A_x: jax.Array,
    A_wqkv: jax.Array,
    A_w_phi: jax.Array,
    A_wo: jax.Array,
    B_x: jax.Array,
    B_w_r: jax.Array,
    B_w_gate: jax.Array,
    B_w_up: jax.Array,
    B_w_down: jax.Array,
):
    del B_x
    hbm = pl.BlockSpec(memory_space=pl.ANY)
    out = pl.pallas_call(
        _kernel,
        out_shape=jax.ShapeDtypeStruct((S, D), BF16),
        in_specs=[hbm] * 8,
        out_specs=hbm,
        scratch_shapes=[
            pltpu.VMEM((S, D), BF16),
            pltpu.VMEM((T, D), U32),
            pltpu.VMEM((NT_ * TH // 2, SW), U32),
            pltpu.VMEM((NT_ * HK // 2, 128), U32),
            pltpu.VMEM((3 * NC, D, RC), BF16),
            [pltpu.VMEM((D // 2, D), U32)] * 3,
            [pltpu.VMEM((HK // 2, 7 * HK), U32)] * 3,
            pltpu.VMEM((H, DH, DH), BF16),
            pltpu.VMEM((8 * 64, 128), U32),
            pltpu.VMEM((2, HK, D), BF16),
            pltpu.VMEM((HK // 2, 7 * HK), U32),
            pltpu.VMEM((D,), BF16),
            pltpu.VMEM((8, D), F32),
            pltpu.VMEM((NPAIR, 64, 128), F32),
            pltpu.VMEM((NPAIR * 32, 128), U32),
            pltpu.VMEM((NPAIR, 128, T), F32),
            pltpu.VMEM((NPAIR, 128, 128), F32),
            [pltpu.VMEM((NPAIR * 64, T), U32)] * 2,
            [pltpu.VMEM((TH // 2, 7 * HK), U32)] * 2,
            [pltpu.VMEM((T, D), F32)] * 2,
            pltpu.VMEM((S // 2, D), U32),
            pltpu.VMEM((S, D), BF16),
            pltpu.VMEM((D, FV), BF16),
            pltpu.VMEM((D, FV), BF16),
            pltpu.VMEM((FVD, D), BF16),
            [pltpu.VMEM((D // NQ + 16, FM), BF16), pltpu.VMEM((D // NQ + 16, FM), BF16),
             pltpu.VMEM((DQA + 16, D), BF16), pltpu.VMEM((DQ - DQA + 16, D), BF16)],
            pltpu.VMEM((D // 2, FM), U32),
            pltpu.VMEM((D // 2, FM), U32),
            pltpu.VMEM(((FF - FVD) // 2, D + 128), U32),
            pltpu.VMEM((16, D), BF16),
            pltpu.SemaphoreType.DMA((6 + 3 * NC + NT_ + 16,)),
        ],
        compiler_params=pltpu.CompilerParams(vmem_limit_bytes=100 * 1024 * 1024,
                                             disable_semaphore_checks=True, disable_bounds_checks=True),
        name="hedgehog_mod",
    )(
        A_x.reshape(S, D),
        A_wqkv,
        A_w_phi,
        A_wo.reshape(2, HK, D),
        B_w_r,
        B_w_gate,
        B_w_up,
        B_w_down,
    )
    return out.reshape(1, S, D)
```

```python
import math

import jax
import jax.numpy as jnp
from jax import lax
import jax.experimental.pallas as pl
import jax.experimental.pallas.tpu as pltpu

F32 = jnp.float32
BF16 = jnp.bfloat16
U32 = jnp.uint32

S = 2048
D = 1024
H = 32
DH = 32
FF = 3584
NPAIR = H // 2
LOG2E = 1.4426950408889634
LN_EPS = 1e-5

T = 256
TH = T // 2
NT_ = S // T
RC = 256
NC = D // RC
PPC = RC // 64
LNC = 16

FV = 10 * 128
FM = FF - FV
FVD = 8 * 128
NQ = NT_ // 2
DQ = (FF - FVD) // NQ
WO_ROWS = 96
QK = D // 4
HK = D // 2
SW = 8 * HK


def _spread(n, a, b, due=None):
    rel = [round(a + (b - a) * k / (n - 1), 3) for k in range(n)]
    return tuple((r, None if due is None else math.ceil(r) + due) for r in rel)


LN1_PLANS = (((0.064, 7), (1.091, 7), (2.8, 9), (4.2, 11), (5.323, 12), (7.125, 13), (8.347, 16), (9.93, 16),
    (11.2, 18), (11.723, 19), (13.877, 22), (15.466, 23), (16.77, 23), (18.2, 25), (19.564, 26), (21.173,
    27)), ((-1.151, 5), (1.211, 7), (1.804, 8), (3.369, 9), (4.93, 10), (6.303, 14), (8.015, 14), (9.695, 17),
    (10.176, 17), (12.132, 19), (13.665, 19), (15.193, 22), (16.785, 23), (18.283, 25), (19.47, 26), (20.992,
    27)))
PRO_LN1_PLAN = ((None, None),) * 16
PRO_K_PLANS0 = ((0.015, None), (0.845, None), (1.721, None), (2.97, None), (3.496, None), (4.341, None),
    (5.723, None), (5.845, None))
PRO_K_PLANS1 = ((-0.801, None), (0.772, None), (1.348, None), (2.924, None), (3.623, None), (3.848, None),
    (4.758, None), (5.626, None))
PRO_X0_PLAN = ((-0.051, None), (1.805, None), (2.734, None), (3.191, None), (3.45, None), (4.522, None),
    (5.302, None), (5.861, None))
PRO_W0_PLAN = ((0.036, None), (0.555, None), (2.188, None), (2.72, None), (3.235, None), (3.839, None),
    (4.525, None), (4.908, None), (5.417, None), (6.465, None))
PRO_W_PLAN = ((0.281, None), (1.112, None), (2.359, None), (2.998, None), (3.693, None), (8.405, None), (9.19,
    None), (9.612, None), (10.206, None), (11.168, None), (11.803, None), (12.549, None), (13.021, None),
    (13.534, None), (14.283, None), (15.221, None), (15.794, None), (16.395, None), (16.918, None), (18.04,
    None), (18.437, None))
PRO_K_PLANS2 = ((15.04, None), (15.786, None), (16.024, None), (16.523, None), (16.957, None), (17.33, None),
    (17.77, None), (18.027, None))
PRO_V_PLANS = (((None, None), (None, None), (None, None), (None, None), (None, None), (None, None), (None,
    None), (None, None), (-3.675, None), (-3.235, None), (-3.152, None), (-2.462, None), (-2.293, None),
    (-2.177, None), (-1.839, None), (-1.486, None), (-1.468, None), (-1.323, None), (-0.973, None), (-0.246,
    None), (0.001, None), (0.112, None), (0.174, None), (0.839, None), (0.913, None), (1.132, None), (1.767,
    None), (1.787, None), (1.869, None), (2.278, None), (2.807, None), (3.005, None)), ((9.073, None),
    (10.016, None), (12.6, None), (12.71, None), (13.256, None), (14.676, None), (18.136, None), (18.863,
    None)), ((20.331, None), (21.596, None), (21.67, None), (22.599, None), (22.815, None), (23.574, None),
    (24.74, None), (27, None)), ((16.361, None), (18.357, None), (19.602, None), (20.041, None), (22.438,
    None), (23.242, None), (24.397, None), (25.564, None)), ((18.94, None), (20.207, None), (21.175, None),
    (22.04, None), (23.77, None), (25.209, None), (25.748, None), (26.232, None), (-1.476, None), (-0.298,
    None), (-0.053, None), (1.471, None), (1.717, None), (3.379, None), (3.723, None), (5.19, None), (5.371,
    None), (6.512, None), (7.542, None), (8.441, None), (8.548, None), (9.511, None), (10.795, None), (11.558,
    None), (11.819, None), (12.134, None), (13.8, None), (14.955, None), (15.388, None), (16.449, None),
    (17.153, None), (17.72, None)))
END_PLANS = (((-0.162, None), (2.011, None), (3.962, None), (5.535, None), (6.909, None), (8.225, None),
    (10.634, None), (12.327, None), (13.876, None), (15.552, None), (16.823, None), (19.352, None), (20.737,
    None), (23.183, None), (23.321, None), (25.88, None)), ((100.281, None), (101.301, None), (102.104, None),
    (0.409, None), (0.947, None), (2.168, None), (2.898, None), (4.298, None), (5.079, None), (5.957, None),
    (7.291, None), (7.974, None), (8.377, None), (10.162, None), (11.3, None), (11.768, None), (12.903, None),
    (13.561, None), (14.696, None), (15.687, None), (17.565, None), (18.013, None), (18.596, None), (19.613,
    None), (20.259, None), (21.191, None), (22.453, None), (23.06, None), (24.586, None), (25.256, None),
    (25.802, None)))
WO_PLANS = (((1.172, None), (6.671, None), (13.134, None), (18.635, None), (26.649, None)), ((-26.952, None),
    (-20.774, None), (-16.958, None), (-12.341, None), (-8.23, None), (-3.106, None), (1.394, None), (5.869,
    None), (10.547, None), (15.312, None), (19.974, None), (24.08, None)), ((-27.513, None), (-22.089, None),
    (-18.667, None), (-14.225, None), (-9.98, None), (-6.618, None), (-2.09, None)))
LN2_PLANS = (((100.0, 107), (106.203, 113), (111.398, 118), (119.249, 127), (125.6, 132), (132.81, 138),
    (-0.082, 11), (3.586, 15), (9.333, 20), (13.767, 26), (18.763, 29), (23.67, 34), (27.496, 38), (32.666,
    44), (37.167, 49), (42.845, 53)), ((49.584, 59), (51.075, 63), (53.935, 66), (56.452, 67), (59.614, 70),
    (62.468, 72), (65.12, 77), (68.048, 77), (68.549, 80), (73.4, 83), (74.033, 87), (79.028, 89), (81.485,
    92), (84.304, None), (87.204, None), (89.885, None)))
O2_PLANS = (((132.01, None), (133.0, None), (136.835, None), (137.064, None), (138.561, None), (139.575,
    None), (141.905, None)), ((142.194, None), (145.413, None), (147.058, None), (148.802, None), (151.024,
    None), (151.892, None), (153.184, None)), ((11.658, None), (14.746, None), (17.562, None), (21.378, None),
    (24.737, None), (27.723, None), (29.963, None)), ((29.663, None), (33.585, None), (36.025, None), (36.945,
    None), (40.941, None), (43.415, None), (45.5, None)))
PACK_PLANS = (((100.109, None), (101.344, None), (102.145, None), (103.07, None), (103.701, None), (104.667,
    None), (105.59, None), (106.591, None), (107.509, None), (107.838, None), (108.876, None), (109.312,
    None), (110.371, None), (111.053, None), (111.535, None), (111.819, None), (114.039, None), (114.179,
    None), (115.566, None), (116.257, None), (117.424, None), (117.662, None), (118.84, None), (119.39, None),
    (120.242, None), (121.031, None), (121.776, None), (122.788, None), (123.303, None), (124.238, None),
    (125.0, None), (126.074, None)), ((128.453, None), (128.914, None), (130.21, None), (131.069, None),
    (132.271, None), (132.788, None), (133.283, None), (133.76, None), (135.652, None), (135.905, None),
    (136.798, None), (137.263, None), (138.493, None), (138.892, None), (139.955, None), (141.399, None),
    (141.652, None), (142.558, None), (143.335, None), (144.067, None), (144.939, None), (145.747, None),
    (146.823, None), (147.249, None), (148.454, None), (149.658, None), (149.978, None), (150.666, None),
    (151.567, None), (152.437, None), (153.075, None), (154.519, None)))
PACKD_PLANS = (((1.117, None), (2.534, None), (4.384, None), (4.629, None), (7.054, None), (9.818, None),
    (10.074, None), (11.689, None), (13.704, None), (14.677, None), (16.6, None), (17.512, None), (20.722,
    None), (22.887, None), (24.093, None), (24.706, None), (26.887, None), (30.354, None), (31.24, None),
    (32.519, None), (34.109, None), (35.707, None), (37.154, None), (39.025, None), (39.985, None), (42.774,
    None), (45.412, None), (46.21, None)), ((49.5, None), (51.668, None), (52.879, None), (54.532, None),
    (55.089, None), (56.135, None), (58.954, None), (59.225, None), (59.38, None), (61.625, None), (63.745,
    None), (64.096, None)))
PACK_DUE = (130, 5, 52, 70)
DQA = 16 * len(PACKD_PLANS[0])
G_LAG = 5
D_LAG = 1
PLAIN_V0 = 1
OC_PIN = 1
LN2_GAPS = (1.1, 1.62)
LN1_GAPS = (1, 1.25)
GAP_PRO = 0.13
GAP_X = 0.2
GAP_WO = 0.2
GAP_O2 = 0.13
RELOAD = 1
OUT_ORDER = 0
O_DUE = 5
MOE_NA = 36
MOE_ND = 2
MOE_LAGS = (2, 2)
STAGGER = 8

NN = (((1,), (0,)), ((), ()))
NT = (((1,), (1,)), ((), ()))


def _dot(a, b, dims):
    return lax.dot_general(a, b, dims, preferred_element_type=F32)


def _recip(x):
    return pl.reciprocal(x, approx=False, full_range=False)


def _pack(x):
    return pltpu.bitcast(x, U32)


def _unpack(x):
    return pltpu.bitcast(x, BF16)


def _strassen_lhs(a11, a12, a21, a22):
    return [a21 + a22, a22, a11 + a12, a11, a11 + a22, a12 - a22, a21 - a11]


def _strassen_rhs(b11, b12, b21, b22):
    return [b11, b21 - b11, b22, b12 - b22, b11 + b22, b21 + b22, b11 + b12]


def _strassen(product):
    m2 = product(0)
    m4 = product(1)
    c21 = m2 + m4
    m5 = product(2)
    u11 = m4 - m5
    m3 = product(3)
    c12 = m3 + m5
    u22 = m3 - m2
    m1 = product(4)
    u11 = u11 + m1
    u22 = u22 + m1
    c11 = product(5) + u11
    c22 = product(6) + u22
    return [[c11, c12], [c21, c22]]


def _block(rows):
    return jnp.concatenate([jnp.concatenate(r, axis=1) for r in rows], axis=0)


def _pair_allreduce(a, op):
    a = op(a, pltpu.roll(a, 2, 0))
    return op(a, pltpu.roll(a, 4, 0))


def _tree(op, xs):
    xs = list(xs)
    while len(xs) > 1:
        nxt = [op(xs[i], xs[i + 1]) for i in range(0, len(xs) - 1, 2)]
        if len(xs) % 2:
            nxt.append(xs[-1])
        xs = nxt
    return xs[0]


def _pair_logits(sl, j):
    sub = lax.broadcasted_iota(jnp.int32, sl[0].shape, 0)
    if j < 3:
        head = jnp.where(sub < 2, 0.0, sl[(0, 1, 16)[j]])
    else:
        head = jnp.where(sub < 2, sl[0], jnp.where(sub < 4, pltpu.roll(sl[1], 2, 0),
                                                   jnp.where(sub < 6, pltpu.roll(sl[16], 4, 0), 0.0)))
    r0 = (2, 9, 17, 24)[j]
    return [head] + list(sl[r0:r0 + 7])


def _dual_exp(sl):
    mx = _pair_allreduce(_tree(jnp.maximum, sl), jnp.maximum)
    mn = _pair_allreduce(_tree(jnp.minimum, sl), jnp.minimum)
    ep = [jnp.exp2(s - mx) for s in sl]
    en = [jnp.exp2(mn - s) for s in sl]
    sp = _pair_allreduce(_tree(jnp.add, ep), jnp.add)
    sn = _pair_allreduce(_tree(jnp.add, en), jnp.add)
    return ep, en, sp, sn


def _after(x, never, anchor):
    if anchor is None:
        return x
    d = jnp.concatenate([anchor] * (x.shape[0] // 8), axis=0)
    if x.shape[1] == 128:
        return jnp.where(never, d, x)
    return jnp.concatenate([jnp.where(never, d, x[:, :128]), x[:, 128:]], axis=1)


def _gate(x, never, deps):
    for i, dep in enumerate(deps):
        d = jnp.broadcast_to(dep, (8, 128))
        if x.dtype != F32:
            d = pltpu.bitcast(d, x.dtype)
        blk = jnp.where(never, d, x[8 * i:8 * i + 8, :128])
        if x.shape[1] > 128:
            blk = jnp.concatenate([blk, x[8 * i:8 * i + 8, 128:]], axis=1)
        parts = ([x[:8 * i, :]] if i else []) + [blk, x[8 * i + 8:, :]]
        x = jnp.concatenate(parts, axis=0)
    return x


def _lane_fold(a):
    return _tree(jnp.add, [a[:, 128 * i:128 * i + 128] for i in range(a.shape[1] // 128)])


def _row_sum(a):
    return jnp.sum(_lane_fold(a), axis=-1, keepdims=True)


def _lane_tile(a, n):
    return a if n == 1 else jnp.concatenate([a] * n, axis=1)


def _sublane_allreduce(a):
    a = a + pltpu.roll(a, 4, 0)
    a = a + pltpu.roll(a, 2, 0)
    return a + pltpu.roll(a, 1, 0)


def _col_broadcast(row8):
    return jnp.concatenate([row8] * 16, axis=0).astype(BF16).T.astype(F32)


def _vpu_matvec(xb, w_rows, never, anchors, lag):
    ng = xb.shape[0] // 8
    acc, hist = None, []
    for g in range(ng):
        dep = anchors[(g * len(anchors)) // ng]
        if g >= lag:
            dep = dep + hist[g - lag]
        x = jnp.where(never, dep, xb[8 * g:8 * g + 8, :])
        w = w_rows(g)
        t = w * _lane_tile(x, w.shape[1] // 128)
        acc = t if acc is None else acc + t
        c = 128 * (g % (w.shape[1] // 128))
        hist.append(acc[:, c:c + 128])
    return acc


class _Side:
    def __init__(self, never, later=lambda rel, gap: rel + gap):
        self.never = never
        self.later = later
        self.jobs = []
        self.deps = {}
        self.hooks = {}

    def add(self, plan, fn):
        for k, (rel, due) in enumerate(plan):
            if rel is None:
                self._run(None, due, fn, k, None)
            else:
                self.jobs.append((rel, due, fn, k))

    def _run(self, rel, due, fn, k, anchor):
        gen = fn if hasattr(fn, "send") else fn(k, anchor)
        dep = gen
        if hasattr(gen, "send"):
            try:
                while True:
                    gap = gen.send(anchor) if gen is fn or rel is None and dep is None else next(gen)
                    if rel is not None:
                        self.jobs.append((self.later(rel, gap), due, gen, k))
                        return
                    dep = None
            except StopIteration as stop:
                dep = stop.value
        if due is not None:
            self.deps.setdefault(due, []).append(dep)

    def check(self):
        assert not self.jobs and not self.deps and not self.hooks

    def gate(self, step, x):
        return _gate(x, self.never, self.deps.pop(step, []))

    def done(self, step, res):
        m = res.shape[0] // 8
        while True:
            ready = [j for j in self.jobs if step - 1 < j[0] <= step]
            if not ready:
                break
            job = min(ready, key=lambda j: j[0])
            self.jobs.remove(job)
            g = m - 1 - int((step - job[0]) * m)
            self._run(*job, res[8 * g:8 * g + 8, res.shape[1] - 128:])
        for fn in self.hooks.pop(step, []):
            fn()


def _kernel(x_hbm, wqkv_hbm, wphi_hbm, wo_hbm, wr_hbm, wg_hbm, wu_hbm, wd_hbm, out_hbm,
            x_v, xn_v, xs_v, lead_v, wraw_v, wt_v, ws_v, wphi_v, a_v, woraw_v, wos_v, wrraw_v, wr_v,
            kvacc_v, kvbf_v, z_v, zb_v, phi_v, oc_v, oc2_v, h_v, hn_v, o_v, wg_v, wu_v, wd_v, stage_v,
            wgp_v, wup_v, wdp_v, patch_v,
            sem):
    SX, SQ, SO, SM = 0, 6, 6 + 3 * NC, 6 + 3 * NC + NT_ + 1

    def x_copy(i):
        h0, h1 = ((0, 1), (1, 2), (2, 4), (4, 8), (8, 2 * NT_))[i]
        rows = pl.ds(h0 * TH, (h1 - h0) * TH)
        return pltpu.make_async_copy(x_hbm.at[rows, :], x_v.at[rows, :], sem.at[SX + i])

    def k0_copy(s):
        return pltpu.make_async_copy(wqkv_hbm.at[:, pl.ds(D + s * 128, 128)],
                                     wraw_v.at[NC, :, pl.ds(s * 128, 128)], sem.at[(SM + 7, SQ + NC)[s]])

    def w_copy(j, c):
        return pltpu.make_async_copy(wqkv_hbm.at[:, pl.ds(j * D + c * RC, RC)], wraw_v.at[j * NC + c],
                                     sem.at[SQ + j * NC + c])

    def wphi_copy(i):
        h0, h1 = ((0, 8), (16, 24), (8, 16), (24, H))[i]
        return pltpu.make_async_copy(wphi_hbm.at[pl.ds(h0, h1 - h0)], wphi_v.at[pl.ds(h0, h1 - h0)],
                                     sem.at[(SM + 4, SM + 8, SM + 9, SM + 14)[i]])

    wr_copy = pltpu.make_async_copy(wr_hbm, wrraw_v, sem.at[SM + 5])

    def wo_copy(i):
        rows = pl.ds(0, WO_ROWS) if i == 0 else pl.ds(WO_ROWS, QK - WO_ROWS)
        return pltpu.make_async_copy(wo_hbm.at[:, rows, :], woraw_v.at[:, rows, :], sem.at[(SM + 6, SX + 5)[i]])

    wg_copy = pltpu.make_async_copy(wg_hbm.at[:, pl.ds(FM, FV)], wg_v, sem.at[SM + 0])
    wu_copy = pltpu.make_async_copy(wu_hbm.at[:, pl.ds(FM, FV)], wu_v, sem.at[SM + 1])
    wd_copy = pltpu.make_async_copy(wd_hbm.at[pl.ds(0, FVD), :], wd_v, sem.at[SM + 2])

    def stage_copy(i, q):
        if i < 2:
            r0 = q * (D // NQ)
            r0 = r0 if isinstance(r0, int) else pl.multiple_of(r0, D // NQ)
            src = (wg_hbm, wu_hbm)[i].at[pl.ds(r0, D // NQ), pl.ds(0, FM)]
        else:
            r0 = FVD + q * DQ + (i - 2) * DQA
            r0 = r0 if isinstance(r0, int) else pl.multiple_of(r0, 16)
            src = wd_hbm.at[pl.ds(r0, (DQA, DQ - DQA)[i - 2]), :]
        return pltpu.make_async_copy(src, stage_v[i].at[pl.ds(0, src.shape[0]), :], sem.at[SM + 10 + i])

    wphi_copy(0).start()
    k0_copy(0).start()
    x_copy(0).start()
    k0_copy(1).start()
    x_copy(1).start()
    wphi_copy(1).start()
    w_copy(1, 2).start()

    made = set()

    def view(ref, i, n, off=0):
        r0 = off + i * n
        return ref.at[pl.ds(r0 if isinstance(r0, int) else pl.multiple_of(r0, math.gcd(n, off)), n), :]

    def put_blocks(dst, r0, fn, m11, m12, m21, m22, never, a, skip=(), base=0, pitch=HK, gap=None):
        for c0 in range(0, m11.shape[1], 128):
            if c0:
                a = yield gap or GAP_PRO
            d11, d22 = m11[:, c0:c0 + 128], m22[:, c0:c0 + 128]
            if a is not None:
                d = jnp.concatenate([a, a], axis=0)
                d11, d22 = jnp.where(never, d, d11), jnp.where(never, d, d22)
            blocks = fn(d11, m12[:, c0:c0 + 128], m21[:, c0:c0 + 128], d22)
            for i, b in enumerate(blocks):
                if i not in skip:
                    dst[r0:r0 + 8, base + i * pitch + c0:base + i * pitch + c0 + 128] = _pack(b.astype(BF16))

    def rows16(ref, r0, c0=0, w=D):
        return _unpack(ref[r0:r0 + 8, c0:c0 + w]).astype(F32)

    def x_blocks(t, k, lo, hi, never, a, gap=None):
        return put_blocks(view(xs_v, t, TH // 2), k * LNC // 2, _strassen_rhs,
                          lo[:, :HK], hi[:, :HK], lo[:, HK:], hi[:, HK:], never, a, gap=gap)

    def ln_rows(t, k, n, never=None, anchor=None, plain=False):
        wide = lambda c, a: _lane_tile(_after(jnp.broadcast_to(c, (n, 128)), never, a), D // 128)
        x = _after(view(x_v, t, T)[k * n:(k + 1) * n, :].astype(F32), never, anchor)
        s1 = _row_sum(x)
        anchor = yield LN1_GAPS[0]
        xc = x - wide(s1 * (1.0 / D), anchor)
        rstd = lax.rsqrt(_row_sum(xc * xc) * (1.0 / D) + LN_EPS)
        anchor = yield LN1_GAPS[1]
        xn = xc * wide(rstd, anchor)
        if plain:
            xn_v[(t * T + k * n) // 2:(t * T + (k + 1) * n) // 2, :] = _pack(xn.astype(BF16))
        elif k * n < TH:
            xn_v[k * n // 2:(k + 1) * n // 2, :] = _pack(xn.astype(BF16))
        else:
            yield from x_blocks(t, k - TH // LNC, rows16(xn_v, (k * n - TH) // 2), xn, never, anchor, GAP_X)
        return _tree(jnp.add, [rstd[8 * i:8 * i + 8, :] for i in range(min(n, LNC) // 8)])

    def now(gen):
        try:
            while True:
                next(gen)
        except StopIteration as stop:
            return stop.value

    def late_x_blocks(t):
        return lambda k, a: x_blocks(t, k, rows16(xn_v, t * T // 2 + 8 * k),
                                     rows16(xn_v, (t * T + TH) // 2 + 8 * k), never0, a)

    def xn_tile(t):
        return _unpack(xn_v[t * T // 2:(t + 1) * T // 2, :])

    def xs_tile(t):
        return _unpack(view(xs_v, t, TH // 2)[:, 0:7 * HK])

    def expand_wphi(c):
        w = wphi_v[8 * c:8 * c + 8].reshape(8 * DH, DH).astype(F32).T
        bits = pltpu.bitcast(w, U32)
        head = lax.broadcasted_iota(jnp.int32, (DH, 128), 1) >> 5
        for s in range(2):
            b = bits[:, 128 * s:128 * s + 128]
            for j in range(2):
                r0 = 64 * (2 * c + s) + 32 * j
                a_v[r0:r0 + 32, :] = jnp.where(head == 2 * j, b >> 16,
                                               jnp.where(head == 2 * j + 1, b, jnp.uint32(0)))

    wphi_copy(0).wait()
    expand_wphi(0)
    h_v[1][...] = jnp.zeros((T, D), F32)
    if OC_PIN:
        for ref in oc_v + oc2_v:
            ref[0:8, 0:128] = jnp.zeros((8, 128), U32)
    for ref in stage_v:
        ref[ref.shape[0] - 16:, 0:128] = jnp.zeros((16, 128), BF16)

    def v_transpose(k, a):
        q, r0 = (k // 8) + 4 * (k % 2), 256 * (k % 8 // 2)
        w = wraw_v[2 * NC + q // 2, r0:r0 + 256, (q % 2) * 128:(q % 2) * 128 + 128]
        if a is not None:
            w = _unpack(jnp.where(never0, jnp.concatenate([pltpu.bitcast(a, U32)] * 16, axis=0), _pack(w)))
        wt_v[2][64 * q:64 * q + 64, r0:r0 + 256] = _pack(w.T)
        made.add(("vt", k))

    def fold_pairs(j, c, s, side=None, step0=None):
        g0 = 64 * (2 * c + s)
        g0 = g0 if isinstance(g0, int) else pl.multiple_of(g0, 64)
        res = _dot(_unpack(a_v[pl.ds(g0, 64), :]), wraw_v[j * NC + c, :, s * 128:(s + 1) * 128], NT)
        if side is not None:
            side.done(step0 + 2 * s, res[:, :D // 2])
            side.done(step0 + 2 * s + 1, res[:, D // 2:])
        sub = lax.broadcasted_iota(jnp.int32, (8, D), 0)
        out = []
        for q in range(2):
            base = _pair_allreduce(jnp.where(sub < 2, res[64 * q:64 * q + 8, :], 0.0), jnp.add)
            out.append([(res[64 * q + 8 * i:64 * q + 8 * i + 8, :] - base) * LOG2E for i in range(8)])
        return out

    def share(z, z3, k):
        sub = lax.broadcasted_iota(jnp.int32, (8, D), 0)
        return jnp.where(sub < 2, pltpu.roll(z3, 8 - 2 * k, 0), z)

    def packed(slabs):
        return _pack(jnp.concatenate(slabs, axis=0).astype(BF16))

    def fold(j, c, side=None, step0=None):
        p0, p1 = fold_pairs(j, c, 0, side, step0)
        p2, p3 = fold_pairs(j, c, 1, side, step0)
        sl = ([share(p0[0], p3[0], 1), share(p1[0], p3[0], 2)] + p0[1:] + p1[1:]
              + [share(p2[0], p3[0], 3)] + p2[1:] + p3[1:])
        zero = jnp.zeros((8, D), F32)
        even, odd = sl + [zero], [zero] + sl
        r0 = 8 * ((31 * c) // 2)
        is_odd = c % 2 == 1
        if isinstance(c, int):
            sl = odd if is_odd else even
        else:
            r0 = pl.multiple_of(r0, 8)
            sl = [jnp.where(is_odd, o, e) for o, e in zip(odd, even)]
        win = wt_v[j].at[pl.ds(r0, 128), :]
        win[8:128, :] = packed(sl[2:])
        first = packed(sl[:2])
        if is_odd is not False:
            keep = lax.broadcasted_iota(jnp.int32, (8, D), 0) < jnp.where(is_odd, 4, 0)
            first = jnp.where(keep, win[0:8, :], first)
        win[0:8, :] = first
        made.update(("fold", j, q) for q in ([c] if isinstance(c, int) else range(3)))

    def w_blocks(j, k0=0):
        def job(k, a):
            k += k0
            assert made >= ({("vt", 8 * (k // 8) + q) for q in range(8)} if j == 2 else
                            {("fold", j, q) for q in ((0, 2) if k < 15 else range(4))})
            lo, hi = rows16(wt_v[j], 8 * k), rows16(wt_v[j], (256 if j == 2 else 248) + 8 * k)
            yield from put_blocks(ws_v[j], 8 * k, _strassen_lhs, lo[:, :HK], lo[:, HK:], hi[:, :HK], hi[:, HK:],
                                  never0, a, skip=(1, 3))
            made.add(("ws", j, k))
        return job

    def k_pair(p, slot, pr, c0, first, never=None):
        for n in range(c0, c0 + p[0].shape[1], 128):
            assert first == (("z", pr, n) not in made)
            made.update({("z", pr, n), ("phi", slot, pr, n)})
        ep, en, sp, sn = _dual_exp(p)
        inv = _recip(sp * sn)
        scale = (sn * inv, sp * inv)
        es = ep + en
        cols = slice(c0, c0 + p[0].shape[1])
        n = 16 if never is None else 16 // STAGGER
        last = None
        for q in range(16 // n):
            sc = scale
            if last is not None:
                sc = [jnp.where(never, last, x) for x in scale]
            phi = jnp.concatenate([es[i] * sc[i // 8] for i in range(q * n, (q + 1) * n)], axis=0)
            rows = slice(8 * q * n, 8 * (q + 1) * n)
            z = phi if first else z_v[pr, rows, cols] + phi
            z_v[pr, rows, cols] = z
            phi_v[slot][64 * pr + 4 * q * n:64 * pr + 4 * (q + 1) * n, cols] = _pack(phi.astype(BF16))
            last = z[8 * n - 8:, :]

    def k_features(pk, slot, c, first, never=None):
        for j in range(PPC):
            k_pair(_pair_logits(pk, j), slot, c * PPC + j, 0, first, never)

    def kv_update(vts, slot, g, first, publish=False):
        for q, vt in enumerate(vts):
            for j in range(2):
                pr = 2 * g + 8 * q + j
                assert made >= {("phi", slot, pr, 0), ("phi", slot, pr, 128)}
                upd = _dot(vt[64 * j:64 * j + 64, :].astype(BF16), _unpack(phi_v[slot][64 * pr:64 * pr + 64, :]), NT)
                acc = upd if first else kvacc_v[pr] + upd
                kvacc_v[pr] = acc
                if publish:
                    odd = -(lax.broadcasted_iota(jnp.int32, (32, 128), 1) & 1)
                    bits = pltpu.bitcast(acc, jnp.int32) & jnp.concatenate([~odd, odd], axis=0)
                    kvbf_v[32 * pr:32 * pr + 32, :] = _pack(pltpu.bitcast(bits, F32).astype(BF16))

    def save_lead(t):
        view(lead_v, t, HK // 2)[...] = _pack(_unpack(view(xs_v, t, TH // 2)[:, 0:HK]).T)

    def proj_feat(side, step0, c, xn, carry):
        r0 = 8 * ((31 * c) // 2)
        skip = 8 if c % 2 == 1 and carry is not None else 0
        w = wt_v[1][r0 + skip:r0 + 128, :]
        quarters = []
        for n in range(2):
            for m in range(2):
                step = step0 + 2 * n + m
                wq = _unpack(side.gate(step, w[:64, :] if m == 0 else w[64:, :]))
                res = _dot(wq, xn[n * TH:(n + 1) * TH, :], NT)
                side.done(step, res)
                quarters.append(res)
        res = jnp.concatenate(
            [jnp.concatenate([quarters[0], quarters[2]], axis=1),
             jnp.concatenate([quarters[1], quarters[3]], axis=1)], axis=0)
        sl = [res[8 * i:8 * i + 8, :] for i in range(res.shape[0] // 8)]
        if c % 2 == 0:
            return sl[:31], sl[31]
        return ([carry] + sl if skip else sl[1:]), None

    def proj_unit(side, step0, j, b, xs, lead=None, plain=None):
        r1 = 64 * b + (64 if j == 2 or b < 3 else 56)
        assert made >= ({("vt", 8 * b + q) for q in range(8)} if plain is not None else
                        {("ws", j, k) for k in range(8 * b, r1 // 8)})
        if plain is not None:
            out = []
            for q in range(2):
                row = []
                for n in range(2):
                    res = _dot(_unpack(wt_v[2][256 * q + 64 * b:256 * q + r1, :]), plain[n * TH:(n + 1) * TH, :], NT)
                    for i in range((0, 2, 4, 5)[2 * q + n], (2, 4, 5, 7)[2 * q + n]):
                        side.done(step0 + i, res)
                    row.append(res)
                out.append(jnp.concatenate(row, axis=1))
            return out

        def product(i):
            off = 256 if j == 2 else 248
            w = (wt_v[j][off + 64 * b:off + r1, HK:] if i == 1 else wt_v[j][64 * b:r1, :HK] if i == 3
                 else ws_v[j][64 * b:r1, i * HK:(i + 1) * HK])
            w = _unpack(side.gate(step0 + i, w))
            if lead is not None and i == 0:
                res = _dot(w, _unpack(view(lead_v, lead, HK // 2)[...]), NN)
            else:
                res = _dot(w, xs[:, i * HK:(i + 1) * HK], NT)
            side.done(step0 + i, res)
            return res
        return [jnp.concatenate(row, axis=1) for row in _strassen(product)]

    def feat_stage(side, step0, j, xs, pair_fn, lead=None):
        sl = [[], []]
        for b in range(4):
            for q, res in enumerate(proj_unit(side, step0 + 7 * b, j, b, xs, lead if b == 0 else None)):
                sl[q] += [res[8 * i:8 * i + 8, :] for i in range(res.shape[0] // 8)]
            for q in (1, 0):
                for jj in (2 * (b % 2), 2 * (b % 2) + 1):
                    pair_fn(_pair_logits(sl[q][31 * (b // 2):], jj), 8 * q + 4 * (b // 2) + jj)

    def v_stage(side, xs, slot, first, publish, lead, plain=None):
        pending = None
        for g in range(4):
            if pending is not None:
                side.hooks.setdefault(7 * g + D_LAG, []).append(lambda p=pending: kv_update(*p))
            pending = (proj_unit(side, 7 * g, 2, g, xs, lead if g == 0 else None, plain if g < PLAIN_V0 else None),
                       slot, g, first, publish)
        side.check()
        return pending

    def pack_rows(src, dst, r0, rows, c0, cols, never, a):
        w = src[r0:r0 + rows, c0:c0 + cols].astype(F32)
        d = _lane_tile(a, cols // 128)
        w = jnp.concatenate([jnp.where(never, d, w[8 * i:8 * i + 8, :]) if i % 2 == 0 else w[8 * i:8 * i + 8, :]
                             for i in range(rows // 8)], axis=0)
        dst[r0 // 2:(r0 + rows) // 2, c0:c0 + cols] = _pack(w.astype(BF16))

    def stash_at(i, k, n):
        return zb_v.at[4 * i + 2 * (k // 16) + n, pl.ds(8 * (k % 16), 8), :]

    def stash(i, sl):
        for k, v in enumerate(sl):
            for n in range(2):
                stash_at(i, k, n)[...] = v[:, 128 * n:128 * n + 128]

    def stashed_k(i, slot, c, first):
        def job(k, a):
            j, n = k // 2, k % 2
            p = _pair_logits([stash_at(i, q, n)[...] for q in range(31)], j)
            k_pair([_after(p[0], never0, a)] + p[1:], slot, c * PPC + j, 128 * n, first, never0)
        return job

    def first_rows(k0, k1, n):
        xn = _unpack(xn_v[n * TH // 2:(n + 1) * TH // 2, :])
        ks = [k for k in range(k0, k1)]
        w = jnp.concatenate([wt_v[1][4 * (k % 32):4 * (k % 32) + 8, :] for k in ks[::2]], axis=0)
        res = _dot(_unpack(w), xn, NT)
        for q, k in enumerate(ks):
            if k % 32 < 31:
                stash_at(0, k % 32, n)[...] = res[8 * q:8 * q + 8, :]

    k0_copy(0).wait()
    x_copy(0).wait()
    wphi_copy(2).start()
    w_copy(1, 1).start()
    wphi_copy(3).start()
    x_copy(2).start()
    p0, p1 = fold_pairs(1, 0, 0)
    wt_v[1][8:64, :] = packed(p0[1:] + p1[1:])
    h_v[0][0:8, :] = p0[0]
    h_v[0][8:16, :] = p1[0]
    never0 = now(ln_rows(0, 0, TH, plain=True))[0, 0] < 0.0
    first_rows(2, 16, 0)

    k0_copy(1).wait()
    x_copy(1).wait()
    wphi_copy(1).wait()
    w_copy(1, 3).start()
    for c in (0, 2, 1, 3):
        w_copy(2, c).start()
    p2, p3 = fold_pairs(1, 0, 1)
    wt_v[1][0:8, :] = packed([share(h_v[0][0:8, :], p3[0], 1), share(h_v[0][8:16, :], p3[0], 2)])
    wt_v[1][64:128, :] = packed([share(p2[0], p3[0], 3)] + p2[1:] + p3[1:] + [jnp.zeros((8, D), F32)])
    made.add(("fold", 1, 0))
    now(ln_rows(0, 1, TH, plain=True))
    first_rows(16, 34, 0)
    first_rows(0, 16, 1)
    first_rows(16, 32, 1)
    expand_wphi(2)

    for c, prev in ((2, 0), (1, 2)):
        w_copy(1, c).wait()
        wphi_copy(4 - c).wait()
        expand_wphi(5 - 2 * c)
        side = _Side(never0, lambda rel, gap: min(rel + gap, 7))
        if c == 2:
            side.add(PRO_X0_PLAN, late_x_blocks(0))
        else:
            side.add(PRO_W0_PLAN, w_blocks(1))
        side.add((PRO_K_PLANS0, PRO_K_PLANS1)[2 - c], stashed_k(prev, 0, prev, True))
        fold(1, c, side, 0)
        stash(c, proj_feat(side, 4, c, xn_tile(0), None)[0])
        side.check()

    x_copy(2).wait()
    w_copy(1, 3).wait()
    x_copy(3).start()
    w_copy(0, 0).start()
    wo_copy(0).start()
    x_copy(4).start()
    for c in range(1, NC):
        w_copy(0, c).start()
    wo_copy(1).start()
    wr_copy.start()
    for i in range(4):
        stage_copy(i, 0).start()
    wg_copy.start()
    wu_copy.start()
    wd_copy.start()
    side = _Side(never0, lambda rel, gap: min(rel + gap, 19))
    side.add(PRO_LN1_PLAN, lambda k, a: ln_rows(1, k, LNC, never0, a, plain=True))
    side.add(PRO_W_PLAN, w_blocks(1, len(PRO_W0_PLAN)))
    side.add(PRO_K_PLANS2, stashed_k(1, 0, 1, False))
    fold(1, 3, side, 0)
    stash(3, proj_feat(side, 4, 3, xn_tile(0), None)[0])
    xn1 = xn_tile(1)
    spare = None
    for c in range(3):
        pk, spare = proj_feat(side, 8 + 4 * c, c, xn1, spare)
        if c < 2:
            k_features(pk, 1, c, c == 1, never0)
        else:
            stash(0, pk + [spare])
    side.check()

    for c in range(NC):
        w_copy(2, c).wait()
    side = _Side(never0, lambda rel, gap: min(rel + gap, 27))
    side.add(PRO_V_PLANS[0], v_transpose)
    side.add(PRO_V_PLANS[1], stashed_k(3, 0, 3, False))
    side.add(PRO_V_PLANS[2], stashed_k(0, 1, 2, False))
    side.add(PRO_V_PLANS[3], late_x_blocks(1))
    side.add(PRO_V_PLANS[4], w_blocks(2))
    spare = jnp.concatenate([stash_at(0, 31, n)[...] for n in range(2)], axis=1)
    k_features(proj_feat(side, -4, 3, xn_tile(1), spare)[0], 1, 3, True, never0)
    kv_update(*v_stage(side, xs_tile(0), 0, True, False, None, xn_tile(0)))
    save_lead(0)
    save_lead(1)
    for r0 in (0, 248):
        wt_v[0][r0:r0 + 8, :] = jnp.zeros((8, D), U32)

    def phase1(u, carry):
        never = u < 0

        @pl.when(u == 0)
        def _():
            x_copy(3).wait()
            w_copy(0, 0).wait()
            wo_copy(0).wait()

        @pl.when(u == 1)
        def _():
            x_copy(4).wait()
            w_copy(0, 1).wait()
            w_copy(0, 2).wait()
            wo_copy(1).wait()

        def wo_blocks(k0):
            def job(k, a):
                k += k0
                r, c, part = k // 4, 128 * (k // 2 % 2), k % 2
                r0 = u * ((QK - WO_ROWS) // 2)
                dst = wos_v.at[pl.ds(pl.multiple_of(r0 // 2, 8), WO_ROWS // 2), :]

                def piece(kq, nq):
                    src = woraw_v.at[kq, pl.ds(pl.multiple_of(r0, 16), WO_ROWS), :]
                    return src[16 * r:16 * r + 16, nq * QK + c:nq * QK + c + 128].astype(F32)
                outer = [_strassen_rhs(piece(ki, ni), piece(ki, 2 + ni), piece(2 + ki, ni), piece(2 + ki, 2 + ni))
                         for ki in range(2) for ni in range(2)]
                for i in range(4) if part == 0 else range(4, 7):
                    if i % 4:
                        a = yield GAP_WO
                    yield from put_blocks(dst, 8 * r, _strassen_rhs, *[o[i] for o in outer], never, a,
                                          base=7 * i * QK + c, pitch=QK)
            return job

        xs = xs_tile(2 * u + 1)
        side = _Side(never, lambda rel, gap: min(rel + gap, 27))
        for i in range(2):
            t = 2 * u + 2 + i
            if i == 0:
                side.add(LN1_PLANS[0], lambda k, a: ln_rows(2 * u + 2, k, LNC, never, a))
                side.add(WO_PLANS[0], wo_blocks(0))
            pending = v_stage(side, xs, 1 - i, False, False, t - 1 if i == 0 else None)
            xs = xs_tile(t)
            side = _Side(never, lambda rel, gap, end=(27, -1)[i]: min(rel + gap, end))
            if i == 0:
                side.add(LN1_PLANS[1], lambda k, a: ln_rows(2 * u + 3, k, LNC, never, a))
                side.add(WO_PLANS[1], wo_blocks(len(WO_PLANS[0])))
            else:
                side.add(WO_PLANS[2], wo_blocks(24 - len(WO_PLANS[2])))
            side.hooks[-28 + D_LAG] = [lambda p=pending: kv_update(*p)]
            feat_stage(side, -28, 1, xs, lambda p, pr: k_pair(p, i, pr, 0, False, never if i == 1 else None))
            save_lead(t)
        side.check()
        fold(0, u)
        return carry

    lax.fori_loop(0, (NT_ - 2) // 2, phase1, 0)

    w_copy(0, 3).wait()
    wr_copy.wait()
    side = _Side(never0, lambda rel, gap: min(rel + gap, 27 if rel < 98 else 103))

    def z_final(k, a):
        zb_v[k] = jnp.broadcast_to(_row_sum(_after(z_v[k], never0, a)), (128, 128))

    side.add(END_PLANS[0], z_final)
    side.add(END_PLANS[1], w_blocks(0))
    fold(0, 3, side, 100)
    kv_update(*v_stage(side, xs_tile(NT_ - 1), 1, False, True, None))
    wr_v[...] = jnp.broadcast_to(wrraw_v[...].reshape(1, D).astype(F32), (8, D))

    def o_copy(r0, n, i):
        return pltpu.make_async_copy(o_v.at[pl.ds(r0, n), :], out_hbm.at[pl.ds(r0, n), :], sem.at[SO + i])

    def finish_rows(h_ref, k, t, valid, st, never=None, anchor=None):
        r0 = t * T + k * LNC
        rows = slice(k * LNC, (k + 1) * LNC)
        wide = lambda c, a: _lane_tile(_after(jnp.broadcast_to(c, (LNC, 128)), never, a), D // 128)
        s1 = _row_sum(_after(h_ref[rows, :], never, anchor))
        anchor = yield LN2_GAPS[0]
        m = wide(s1 * (1.0 / D), anchor)
        hc = h_ref[rows, :] - m
        s2 = _row_sum(hc * hc)
        s3 = _row_sum(hc * jnp.concatenate([wr_v[...]] * (LNC // 8), axis=0))
        rstd = lax.rsqrt(s2 * (1.0 / D) + LN_EPS)
        anchor = yield LN2_GAPS[1]
        h = h_ref[rows, :]
        hn = (h - m) * wide(rstd, anchor) if RELOAD else hc * wide(rstd, anchor)
        view(hn_v, t, T // 2)[k * LNC // 2:(k + 1) * LNC // 2, :] = _pack(hn.astype(BF16))
        view(o_v, t, T)[rows, :] = (hn + h).astype(BF16)
        r = (s3 * rstd).astype(BF16).astype(F32)
        if valid is not None:
            r = jnp.where(valid, r, -jnp.inf)
        best, besti = st["route"]
        sub = lax.broadcasted_iota(jnp.int32, (8, 1), 0)
        for i in range(LNC // 8):
            ri = r[8 * i:8 * i + 8, :]
            better = ri > best
            best = jnp.where(better, ri, best)
            besti = jnp.where(better, sub + (r0 + 8 * i), besti)
        st["route"] = (best, besti)
        return best

    def q_pair(p, slot, pr):
        ep, en, sp, sn = _dual_exp(p)
        zz = [_lane_tile(zb_v[pr, 8 * i:8 * i + 8, :], T // 128) for i in range(16)]
        ap = _pair_allreduce(_tree(jnp.add, [ep[i] * zz[i] for i in range(8)]), jnp.add)
        an = _pair_allreduce(_tree(jnp.add, [en[i] * zz[8 + i] for i in range(8)]), jnp.add)
        inv = _recip(ap * sn + (an + 1e-6 * sn) * sp)
        rp = sn * inv
        rn = sp * inv
        phi = jnp.concatenate([e * rp for e in ep] + [e * rn for e in en], axis=0)
        phi_v[slot][64 * pr:64 * pr + 64, :] = _pack(phi.astype(BF16))

    held = []

    def attn_blocks(slot, g, deps):
        lo, hi = [jnp.concatenate(
            [_dot(_unpack(kvbf_v[32 * pr:32 * pr + 32, :]), _unpack(phi_v[slot][64 * pr:64 * pr + 64, :]), NN)
             for pr in (2 * q, 2 * q + 1)], axis=0) for q in (g, g + 4)]
        blocks = [(i, g, b) for i, b in enumerate(_strassen_lhs(lo[:, :TH], hi[:, :TH], lo[:, TH:], hi[:, TH:]))]
        if g % 2 == 0:
            held.append(blocks.pop())
        else:
            blocks.append(held.pop())
        ot = _pack(jnp.concatenate([b for _, _, b in blocks], axis=1).astype(BF16).T)
        for q, (i, n, _) in enumerate(blocks):
            oc_v[slot][:, i * HK + 128 * n:i * HK + 128 * n + 128] = ot[q * TH // 2:(q + 1) * TH // 2, :]
            made.add(("oc", slot, i, n))
            if q % 2:
                deps.append(pltpu.bitcast(ot[(q + 1) * TH // 2 - 8:(q + 1) * TH // 2, :], F32))

    def o_blocks(slot, c, never):
        def job(k, a):
            assert made >= {("oc", slot, k, c), ("oc", slot, k, c + 2)}
            for r in range(4):
                if r:
                    a = yield GAP_O2
                m = [rows16(oc_v[slot], 8 * r + 32 * q, k * HK + n * QK + 128 * c, 128)
                     for q in range(2) for n in range(2)]
                yield from put_blocks(oc2_v[slot], 8 * r, _strassen_lhs, *m, never, a, skip=(1, 3),
                                      base=7 * k * QK + 128 * c, pitch=QK)
            made.add(("oc2", slot, k, c))
        return job

    def out_proj(side, step0, t, slot):
        count = [0]

        def inner(i, c):
            assert made >= {("oc2", slot, i, 0), ("oc2", slot, i, 1)}

            def product(j):
                step, odd = step0 + count[0] // 2, count[0] % 2
                count[0] += 1
                o = (oc_v[slot][32:64, i * HK + QK:(i + 1) * HK] if j == 1 else
                     oc_v[slot][0:32, i * HK:i * HK + QK] if j == 3 else
                     oc2_v[slot][:, (7 * i + j) * QK:(7 * i + j + 1) * QK])
                w = wos_v[:, (7 * i + j) * QK + 128 * c:(7 * i + j) * QK + 128 * c + 128]
                res = _dot(_unpack(o), _unpack(w if odd else side.gate(step, w)), NN)
                if odd:
                    side.done(step, res)
                return res
            return _block(_strassen(product))

        xt = view(x_v, t, T)
        if OUT_ORDER == 0:
            hs = [_block(_strassen(lambda i: inner(i, c))) for c in range(2)]
        else:
            h = _block(_strassen(lambda i: jnp.concatenate([inner(i, c) for c in range(2)], axis=1)))
            hs = [jnp.concatenate([h[:, 256 * c:256 * c + 256], h[:, 512 + 256 * c:768 + 256 * c]], axis=1)
                  for c in range(2)]
        for c in range(2):
            for n in range(4):
                cols = slice(n * QK + 128 * c, n * QK + 128 * c + 128)
                h_v[slot][:, cols] = hs[c][:, 128 * n:128 * n + 128] + xt[:, cols].astype(F32)

    def phase2(u, carry):
        for i in range(4):
            stage_copy(i, u).wait()
        never = u < 0
        side = _Side(never, lambda rel, gap: min(rel + 2 * gap, 97) if rel < 98 else
                     rel + gap if rel + gap <= 155 else 2 * (rel + gap - 155) - 1)
        st = {"route": carry}
        tp = jnp.maximum(2 * u - 1, 0)
        side.add(LN2_PLANS[0], lambda k, a: finish_rows(h_v[1], k, tp, u > 0, st, never, a))
        side.add(LN2_PLANS[1], lambda k, a: finish_rows(h_v[0], k, 2 * u, None, st, never, a))

        def packer(i, dst, n):
            left = [n]

            def job(k, a):
                if i < 2:
                    pack_rows(stage_v[i], dst, (k // 2) * 16, 16, (0, D)[k % 2], (D, FM - D)[k % 2], never, a)
                else:
                    pack_rows(stage_v[i], dst, k * 16, 16, 0, D, never, a)
                left[0] -= 1
                if not left[0]:
                    stage_copy(i, jnp.minimum(u + 1, NQ - 1)).start()
                    n0 = stage_v[i].shape[0] - 16
                    side.deps.setdefault(PACK_DUE[i], []).append(stage_v[i][n0:n0 + 8, 0:128].astype(F32))
            return job

        for i in range(2):
            side.add(PACK_PLANS[i], packer(i, view((wgp_v, wup_v)[i], u, D // NQ // 2), len(PACK_PLANS[i])))
            d0 = pl.multiple_of(u * (DQ // 2) + i * (DQA // 2), 8)
            side.add(PACKD_PLANS[i], packer(2 + i, wdp_v.at[pl.ds(d0, 8 * len(PACKD_PLANS[i])), :],
                                            len(PACKD_PLANS[i])))
            for g in range(4):
                step = 107 + 28 * i + 7 * g + G_LAG
                wrap = lambda x: x if x < 156 else 2 * (x - 156) + 1
                side.hooks.setdefault(wrap(step), []).append(
                    lambda i=i, g=g, due=wrap(step + O_DUE): attn_blocks(i, g, side.deps.setdefault(due, [])))
            for c in range(2):
                side.add(O2_PLANS[2 * i + c], o_blocks(i, c, never))
        for i in range(2):
            feat_stage(side, 100 + 28 * i, 0, xs_tile(2 * u + i), lambda p, pr: q_pair(p, i, pr),
                       2 * u if i == 0 else None)
        for i in range(2):
            out_proj(side, 49 * i, 2 * u + i, i)
        side.check()

        @pl.when(u == 0)
        def _():
            o_copy(0, T, 0).start()

        @pl.when(u > 0)
        def _():
            o_copy(pl.multiple_of(tp * T, T), 2 * T, u).start()

        return st["route"]

    wg_copy.wait()
    wu_copy.wait()
    wd_copy.wait()
    route = lax.fori_loop(
        0, NT_ // 2, phase2,
        (jnp.full((8, 1), -jnp.inf, F32), jnp.zeros((8, 1), jnp.int32)))
    st = {"route": route}
    for k in range(T // LNC):
        now(finish_rows(h_v[1], k, NT_ - 1, None, st))
    best, besti = st["route"]
    o_copy(S - T, T, NT_).start()

    rmax = jnp.max(best, axis=0, keepdims=True)
    idx = jnp.min(jnp.where(best == rmax, besti, S), axis=0, keepdims=True)
    idx_s = jnp.clip(idx[0, 0], 0, S - 1)
    blk = pl.multiple_of((idx_s >> 4) << 4, 16)
    pair = jnp.broadcast_to(hn_v[pl.ds(idx_s >> 1, 1), :], (8, D))
    x8 = pltpu.bitcast(jnp.where((idx_s & 1) == 1, pair & jnp.uint32(0xFFFF0000), pair << 16), F32)
    xs = jnp.concatenate([x8, x8], axis=0).astype(BF16)
    acts, anchors = [], []

    def park(v, half):
        n = v.shape[0] // 128
        for i in range(n):
            z_v[i, :, 128 * half:128 * half + 128] = v[128 * i:128 * i + 128, :]
        return jnp.concatenate([z_v[i, :, 128 * half:128 * half + 128] for i in range(n)], axis=0)

    for c0 in range(0, FM, 128):
        g = _dot(xs, _unpack(wgp_v[:, c0:c0 + 128]), NN)[0:8, :]
        u = _dot(xs, _unpack(wup_v[:, c0:c0 + 128]), NN)[0:8, :]
        anchors += [g, u]
        acts.append(g * jax.nn.sigmoid(g) * u)
    xb = park(_col_broadcast(x8), 0)
    g, u = [_sublane_allreduce(_vpu_matvec(
        xb, lambda g: w[8 * g:8 * g + 8, :].astype(F32), never0,
        anchors[i * MOE_NA // 2:(i + 1) * MOE_NA // 2], MOE_LAGS[0])) for i, w in enumerate((wg_v, wu_v))]
    acts.append(g * jax.nn.sigmoid(g) * u)
    a = jnp.concatenate(acts, axis=1)
    am = jnp.concatenate([a[:, FVD:], a[:, FVD:]], axis=0).astype(BF16)
    ys, anchors = [], anchors[MOE_NA:]
    for k0 in range(0, FF - FVD, 512):
        k1 = min(k0 + 512, FF - FVD)
        yk = _dot(am[:, k0:k1], _unpack(wdp_v[k0 // 2:k1 // 2, 0:D]), NN)[0:8, :]
        ys.append(yk)
        anchors += [yk[:, c:c + 128] for c in range(128, D, 256)]
    ys.append(_sublane_allreduce(_vpu_matvec(
        park(_col_broadcast(a[:, :FVD]), 1), lambda g: wd_v[8 * g:8 * g + 8, :].astype(F32), never0,
        anchors[:-MOE_ND], MOE_LAGS[1])))
    y = _tree(jnp.add, ys) * jax.nn.sigmoid(rmax)
    y = jnp.concatenate([y, y], axis=0)
    sel = lax.broadcasted_iota(jnp.int32, (16, 1), 0) == (idx_s - blk)
    patch_v[...] = (o_v[pl.ds(blk, 16), :].astype(F32) + jnp.where(sel, y, 0.0)).astype(BF16)
    o_copy(0, T, 0).wait()
    for u in range(1, NT_ // 2):
        o_copy((2 * u - 1) * T, 2 * T, u).wait()
    o_copy(S - T, T, NT_).wait()
    pc = pltpu.make_async_copy(patch_v, out_hbm.at[pl.ds(blk, 16), :], sem.at[SM + 3])
    pc.start()
    for i in range(4):
        stage_copy(i, NQ - 1).wait()
    pc.wait()


@jax.jit
def pallas_sequential_preLN__linear_kernel_hedgehog__moe_arch_mod__prompt_kernel(
    A_x: jax.Array,
    A_wqkv: jax.Array,
    A_w_phi: jax.Array,
    A_wo: jax.Array,
    B_x: jax.Array,
    B_w_r: jax.Array,
    B_w_gate: jax.Array,
    B_w_up: jax.Array,
    B_w_down: jax.Array,
):
    del B_x
    hbm = pl.BlockSpec(memory_space=pl.ANY)
    out = pl.pallas_call(
        _kernel,
        out_shape=jax.ShapeDtypeStruct((S, D), BF16),
        in_specs=[hbm] * 8,
        out_specs=hbm,
        scratch_shapes=[
            pltpu.VMEM((S, D), BF16),
            pltpu.VMEM((T, D), U32),
            pltpu.VMEM((NT_ * TH // 2, SW), U32),
            pltpu.VMEM((NT_ * HK // 2, 128), U32),
            pltpu.VMEM((3 * NC, D, RC), BF16),
            [pltpu.VMEM((D // 2, D), U32)] * 3,
            [pltpu.VMEM((HK // 2, 7 * HK), U32)] * 3,
            pltpu.VMEM((H, DH, DH), BF16),
            pltpu.VMEM((8 * 64, 128), U32),
            pltpu.VMEM((4, QK, D), BF16),
            pltpu.VMEM((QK // 2, 49 * QK + 128), U32),
            pltpu.VMEM((D,), BF16),
            pltpu.VMEM((8, D), F32),
            pltpu.VMEM((NPAIR, 64, 128), F32),
            pltpu.VMEM((NPAIR * 32, 128), U32),
            pltpu.VMEM((NPAIR, 128, T), F32),
            pltpu.VMEM((NPAIR, 128, 128), F32),
            [pltpu.VMEM((NPAIR * 64, T), U32)] * 2,
            [pltpu.VMEM((TH // 2, 7 * HK), U32)] * 2,
            [pltpu.VMEM((TH // 4, 49 * QK), U32)] * 2,
            [pltpu.VMEM((T, D), F32)] * 2,
            pltpu.VMEM((S // 2, D), U32),
            pltpu.VMEM((S, D), BF16),
            pltpu.VMEM((D, FV), BF16),
            pltpu.VMEM((D, FV), BF16),
            pltpu.VMEM((FVD, D), BF16),
            [pltpu.VMEM((D // NQ + 16, FM), BF16), pltpu.VMEM((D // NQ + 16, FM), BF16),
             pltpu.VMEM((DQA + 16, D), BF16), pltpu.VMEM((DQ - DQA + 16, D), BF16)],
            pltpu.VMEM((D // 2, FM), U32),
            pltpu.VMEM((D // 2, FM), U32),
            pltpu.VMEM(((FF - FVD) // 2, D + 128), U32),
            pltpu.VMEM((16, D), BF16),
            pltpu.SemaphoreType.DMA((6 + 3 * NC + NT_ + 16,)),
        ],
        compiler_params=pltpu.CompilerParams(vmem_limit_bytes=100 * 1024 * 1024,
                                             disable_semaphore_checks=True, disable_bounds_checks=True),
        name="hedgehog_mod",
    )(
        A_x.reshape(S, D),
        A_wqkv,
        A_w_phi,
        A_wo.reshape(4, QK, D),
        B_w_r,
        B_w_gate,
        B_w_up,
        B_w_down,
    )
    return out.reshape(1, S, D)
```

```python
import math

import jax
import jax.numpy as jnp
from jax import lax
import jax.experimental.pallas as pl
import jax.experimental.pallas.tpu as pltpu

F32 = jnp.float32
BF16 = jnp.bfloat16
U32 = jnp.uint32

S = 2048
D = 1024
H = 32
DH = 32
FF = 3584
NPAIR = H // 2
LOG2E = 1.4426950408889634
LN_EPS = 1e-5
KEY_MIN = -2 ** 31

T = 256
TH = T // 2
NT_ = S // T
RC = 256
NC = D // RC
PPC = RC // 64
LNC = 16

FV = 10 * 128
FM = FF - FV
FVD = 8 * 128
NQ = NT_ // 2
DQ = (FF - FVD) // NQ
WO_ROWS = 96
QK = D // 4
HK = D // 2
SW = 8 * HK


def _spread(n, a, b, due=None):
    rel = [round(a + (b - a) * k / (n - 1), 3) for k in range(n)]
    return tuple((r, None if due is None else math.ceil(r) + due) for r in rel)


LN1_PLANS = (((0.072, 7), (0.452, 7), (2.8, 9), (4.2, 11), (5.323, 12), (7.125, 13), (8.42, 16), (9.93, 16),
    (11.174, 18), (11.723, 19), (13.877, 22), (15.466, 23), (16.77, 23), (18.221, 25), (19.564, 26), (21.5,
    27)), ((-1.151, 5), (1.211, 7), (1.804, 8), (3.369, 9), (5.17, 11), (5.924, 14), (8.015, 14), (9.695, 17),
    (10.176, 17), (11.93, 19), (13.665, 19), (15.339, 22), (16.785, 22), (18.546, 25), (19.47, 26), (21.122,
    27)))
PRO_LN1_PLAN = ((None, None),) * 16
PRO_K_PLANS0 = ((0.015, None), (0.845, None), (1.721, None), (2.97, None), (3.496, None), (4.341, None),
    (5.723, None), (5.845, None))
PRO_K_PLANS1 = ((-0.801, None), (0.772, None), (1.348, None), (2.924, None), (3.623, None), (3.848, None),
    (4.758, None), (5.626, None))
PRO_X0_PLAN = ((-0.051, None), (1.805, None), (2.734, None), (3.191, None), (3.45, None), (4.522, None),
    (5.302, None), (5.861, None))
PRO_W0_PLAN = ((0.036, None), (0.555, None), (2.188, None), (2.72, None), (3.235, None), (3.839, None),
    (4.525, None), (4.908, None), (5.417, None), (6.465, None))
PRO_W_PLAN = ((0.281, None), (0.962, None), (2.192, None), (2.998, None), (3.693, None), (8.405, None), (9.19,
    None), (9.659, None), (10.206, None), (11.168, None), (11.803, None), (12.534, None), (12.982, None),
    (13.534, None), (14.32, None), (15.084, None), (15.792, None), (16.395, None), (16.945, None), (18.04,
    None), (18.437, None))
PRO_K_PLANS2 = ((15.04, None), (15.879, None), (15.938, None), (16.523, None), (16.865, None), (17.33, None),
    (17.649, None), (17.852, None))
PRO_V_PLANS = (((None, None), (None, None), (None, None), (None, None), (None, None), (None, None), (None,
    None), (None, None), (-3.675, None), (-3.235, None), (-3.152, None), (-2.663, None), (-2.285, None),
    (-2.177, None), (-1.839, None), (-1.602, None), (-1.468, None), (-1.323, None), (-0.973, None), (-0.246,
    None), (0.001, None), (0.112, None), (0.421, None), (0.913, None), (0.98, None), (1.132, None), (1.604,
    None), (1.767, None), (1.869, None), (2.278, None), (2.807, None), (3.005, None)), ((9.073, None),
    (10.016, None), (12.71, None), (12.797, None), (13.345, None), (14.676, None), (18.136, None), (18.863,
    None)), ((20.331, None), (21.08, None), (21.596, None), (22.599, None), (22.815, None), (23.574, None),
    (24.852, None), (26.895, None)), ((16.477, None), (18.357, None), (19.602, None), (19.911, None), (22.438,
    None), (23.242, None), (24.397, None), (25.564, None)), ((18.94, None), (20.207, None), (21.27, None),
    (22.04, None), (23.77, None), (24.709, None), (25.305, None), (26.271, None), (-1.476, None), (-0.298,
    None), (0.085, None), (1.471, None), (1.717, None), (3.379, None), (3.723, None), (5.19, None), (5.371,
    None), (6.512, None), (7.542, None), (8.444, None), (8.686, None), (9.511, None), (10.795, None), (11.558,
    None), (11.774, None), (12.134, None), (13.8, None), (15.151, None), (15.328, None), (16.443, None),
    (17.153, None), (17.72, None)))
END_PLANS = (((-0.162, None), (2.011, None), (3.829, None), (5.62, None), (6.909, None), (8.134, None),
    (10.634, None), (12.371, None), (13.954, None), (15.538, None), (16.797, None), (19.352, None), (20.737,
    None), (23.183, None), (23.393, None), (25.88, None)), ((100.308, None), (101.389, None), (102.104, None),
    (0.409, None), (1.005, None), (2.198, None), (2.898, None), (4.205, None), (5.131, None), (6.022, None),
    (7.291, None), (7.974, None), (8.425, None), (10.079, None), (11.3, None), (11.768, None), (12.903, None),
    (13.561, None), (14.696, None), (15.687, None), (17.565, None), (18.013, None), (18.596, None), (19.613,
    None), (20.25, None), (21.235, None), (22.366, None), (23.06, None), (24.673, None), (25.256, None),
    (25.849, None)))
WO_PLANS = (((0.245, None), (6.671, None), (13.134, None), (18.635, None), (25.68, None)), ((-26.952, None),
    (-20.774, None), (-16.958, None), (-12.341, None), (-8.3, None), (-2.883, None), (1.607, None), (6.233,
    None), (10.547, None), (15.312, None), (19.974, None), (24.229, None)), ((-27.525, None), (-22.089, None),
    (-18.962, None), (-14.225, None), (-9.98, None), (-6.618, None), (-2.09, None)))
LN2_PLANS = (((99.02, 108), (108.17, 115), (117.905, 125), (126.823, 133), (-0.9, 11), (4.695, 19), (9.555,
    21), (12.366, 25), (17.787, 31), (21.461, 35), (26.539, 39), (34.004, 46)), ((36.558, 49), (37.61, 51),
    (40.28, 53), (43.729, 58), (48.182, 59), (52.072, 64), (54.926, 66), (55.175, 70), (59.92, 74), (64.192,
    76), (67.433, 81), (67.847, 82), (71.545, 86), (73.884, 90), (78.756, 91), (79.525, 95)), ((84.158, None),
    (87.073, None), (89.006, None), (90.204, None)))
O2_PLANS = (((131.676, None), (133.082, None), (137.063, None), (137.243, None), (138.449, None), (141.763,
    None), (144.205, None)), ((141.827, None), (145.636, None), (147.024, None), (147.228, None), (149.817,
    None), (152.366, None), (153.094, None)), ((12.968, None), (13.456, None), (17.632, None), (21.665, None),
    (24.665, None), (26.405, None), (28.552, None)), ((26.264, None), (33.3, None), (35.325, None), (36.521,
    None), (41.083, None), (44.099, None), (45.43, None)))
PACK_PLANS = (((100.502, None), (101.244, None), (102.145, None), (102.323, None), (103.427, None), (104.815,
    None), (105.886, None), (106.631, None), (107.838, None), (108.071, None), (109.312, None), (109.624,
    None), (110.371, None), (111.166, None), (111.188, None), (112.322, None), (114.039, None), (114.195,
    None), (115.082, None), (116.893, None), (117.775, None), (118.037, None), (118.38, None), (118.897,
    None), (120.242, None), (121.347, None), (121.526, None), (122.788, None), (123.403, None), (124.242,
    None), (124.673, None), (125.882, None)), ((128.281, None), (128.956, None), (131.069, None), (131.514,
    None), (131.968, None), (132.22, None), (132.87, None), (133.948, None), (135.423, None), (136.397, None),
    (136.936, None), (137.556, None), (138.836, None), (139.06, None), (140.343, None), (141.492, None),
    (141.596, None), (142.473, None), (143.821, None), (144.016, None), (144.111, None), (146.083, None),
    (146.911, None), (147.773, None), (148.519, None), (149.019, None), (149.771, None), (150.607, None),
    (151.737, None), (152.598, None), (153.755, None), (154.519, None)))
PACKD_PLANS = (((1.158, None), (1.431, None), (4.36, None), (5.329, None), (6.815, None), (9.75, None),
    (9.964, None), (11.222, None), (14.02, None), (14.167, None), (14.74, None), (15.912, None), (19.475,
    None), (20.868, None), (21.595, None), (22.323, None), (25.338, None), (25.36, None), (28.561, None),
    (30.197, None), (31.978, None), (33.911, None)), ((35.02, None), (36.791, None), (39.11, None), (39.927,
    None), (42.179, None), (42.46, None), (46.568, None), (46.704, None), (49.488, None), (51.509, None),
    (51.641, None), (52.889, None), (53.199, None), (55.468, None), (55.716, None), (58.287, None), (59.056,
    None), (60, None)))
PACK_DUE = (130, 5, 39, 64)
DQA = 16 * len(PACKD_PLANS[0])
G_LAG = 5
D_LAG = 1
PLAIN_V0 = 1
OC_PIN = 1
LN2_GAPS = (1.13, 1.5, 0.2)
LN2_SPLIT = 4
PACK_W = 512
GAP_PACK = 0.2
LN1_GAPS = (1, 1.25)
GAP_PRO = 0.13
GAP_X = 0.2
GAP_WO = 0.2
GAP_O2 = 0.26
OUT_ORDER = 1
O_DUE = 6
MOE_NA = 36
MOE_ND = 2
MOE_LAGS = (2, 2)
STAGGER = 8

NN = (((1,), (0,)), ((), ()))
NT = (((1,), (1,)), ((), ()))


def _dot(a, b, dims):
    return lax.dot_general(a, b, dims, preferred_element_type=F32)


def _recip(x):
    return pl.reciprocal(x, approx=False, full_range=False)


def _pack(x):
    return pltpu.bitcast(x, U32)


def _unpack(x):
    return pltpu.bitcast(x, BF16)


def _strassen_lhs(a11, a12, a21, a22):
    return [a21 + a22, a22, a11 + a12, a11, a11 + a22, a12 - a22, a21 - a11]


def _strassen_rhs(b11, b12, b21, b22):
    return [b11, b21 - b11, b22, b12 - b22, b11 + b22, b21 + b22, b11 + b12]


def _strassen(product):
    m2 = product(0)
    m4 = product(1)
    c21 = m2 + m4
    m5 = product(2)
    u11 = m4 - m5
    m3 = product(3)
    c12 = m3 + m5
    u22 = m3 - m2
    m1 = product(4)
    u11 = u11 + m1
    u22 = u22 + m1
    c11 = product(5) + u11
    c22 = product(6) + u22
    return [[c11, c12], [c21, c22]]


def _strassen_rows_first(product, emit):
    m5 = product(2)
    m3 = product(3)
    emit(0, 1, m3 + m5)
    m4 = product(1)
    u11 = m4 - m5
    m1 = product(4)
    u11 = u11 + m1
    u22 = m3 + m1
    emit(0, 0, product(5) + u11)
    m2 = product(0)
    emit(1, 0, m2 + m4)
    u22 = u22 - m2
    emit(1, 1, product(6) + u22)


def _ordered(bits):
    return bits ^ ((bits >> 31) & 0x7FFF0000)


def _block(rows):
    return jnp.concatenate([jnp.concatenate(r, axis=1) for r in rows], axis=0)


def _pair_allreduce(a, op):
    a = op(a, pltpu.roll(a, 2, 0))
    return op(a, pltpu.roll(a, 4, 0))


def _tree(op, xs):
    xs = list(xs)
    while len(xs) > 1:
        nxt = [op(xs[i], xs[i + 1]) for i in range(0, len(xs) - 1, 2)]
        if len(xs) % 2:
            nxt.append(xs[-1])
        xs = nxt
    return xs[0]


def _pair_logits(sl, j):
    sub = lax.broadcasted_iota(jnp.int32, sl[0].shape, 0)
    if j < 3:
        head = jnp.where(sub < 2, 0.0, sl[(0, 1, 16)[j]])
    else:
        head = jnp.where(sub < 2, sl[0], jnp.where(sub < 4, pltpu.roll(sl[1], 2, 0),
                                                   jnp.where(sub < 6, pltpu.roll(sl[16], 4, 0), 0.0)))
    r0 = (2, 9, 17, 24)[j]
    return [head] + list(sl[r0:r0 + 7])


def _dual_exp(sl):
    mx = _pair_allreduce(_tree(jnp.maximum, sl), jnp.maximum)
    mn = _pair_allreduce(_tree(jnp.minimum, sl), jnp.minimum)
    ep = [jnp.exp2(s - mx) for s in sl]
    en = [jnp.exp2(mn - s) for s in sl]
    sp = _pair_allreduce(_tree(jnp.add, ep), jnp.add)
    sn = _pair_allreduce(_tree(jnp.add, en), jnp.add)
    return ep, en, sp, sn


def _after(x, never, anchor):
    if anchor is None:
        return x
    d = jnp.concatenate([anchor] * (x.shape[0] // 8), axis=0)
    if x.shape[1] == 128:
        return jnp.where(never, d, x)
    return jnp.concatenate([jnp.where(never, d, x[:, :128]), x[:, 128:]], axis=1)


def _gate(x, never, deps):
    for i, dep in enumerate(deps):
        d = jnp.broadcast_to(dep, (8, 128))
        if x.dtype != F32:
            d = pltpu.bitcast(d, x.dtype)
        blk = jnp.where(never, d, x[8 * i:8 * i + 8, :128])
        if x.shape[1] > 128:
            blk = jnp.concatenate([blk, x[8 * i:8 * i + 8, 128:]], axis=1)
        parts = ([x[:8 * i, :]] if i else []) + [blk, x[8 * i + 8:, :]]
        x = jnp.concatenate(parts, axis=0)
    return x


def _lane_fold(a):
    return _tree(jnp.add, [a[:, 128 * i:128 * i + 128] for i in range(a.shape[1] // 128)])


def _row_sum(a):
    return jnp.sum(_lane_fold(a), axis=-1, keepdims=True)


def _lane_tile(a, n):
    return a if n == 1 else jnp.concatenate([a] * n, axis=1)


def _sublane_allreduce(a):
    a = a + pltpu.roll(a, 4, 0)
    a = a + pltpu.roll(a, 2, 0)
    return a + pltpu.roll(a, 1, 0)


def _col_broadcast(row8):
    return jnp.concatenate([row8] * 16, axis=0).astype(BF16).T.astype(F32)


def _vpu_matvec(xb, w_rows, never, anchors, lag):
    ng = xb.shape[0] // 8
    acc, hist = None, []
    for g in range(ng):
        dep = anchors[(g * len(anchors)) // ng]
        if g >= lag:
            dep = dep + hist[g - lag]
        x = jnp.where(never, dep, xb[8 * g:8 * g + 8, :])
        w = w_rows(g)
        t = w * _lane_tile(x, w.shape[1] // 128)
        acc = t if acc is None else acc + t
        c = 128 * (g % (w.shape[1] // 128))
        hist.append(acc[:, c:c + 128])
    return acc


class _Side:
    def __init__(self, never, later=lambda rel, gap: rel + gap):
        self.never = never
        self.later = later
        self.jobs = []
        self.deps = {}
        self.hooks = {}

    def add(self, plan, fn):
        for k, (rel, due) in enumerate(plan):
            if rel is None:
                self._run(None, due, fn, k, None)
            else:
                self.jobs.append((rel, due, fn, k))

    def _run(self, rel, due, fn, k, anchor):
        gen = fn if hasattr(fn, "send") else fn(k, anchor)
        dep = gen
        if hasattr(gen, "send"):
            try:
                while True:
                    gap = gen.send(anchor) if gen is fn or rel is None and dep is None else next(gen)
                    if rel is not None:
                        self.jobs.append((self.later(rel, gap), due, gen, k))
                        return
                    dep = None
            except StopIteration as stop:
                dep = stop.value
        if due is not None:
            self.deps.setdefault(due, []).append(dep)

    def check(self):
        assert not self.jobs and not self.deps and not self.hooks

    def gate(self, step, x):
        return _gate(x, self.never, self.deps.pop(step, []))

    def done(self, step, res):
        m = res.shape[0] // 8
        while True:
            ready = [j for j in self.jobs if step - 1 < j[0] <= step]
            if not ready:
                break
            job = min(ready, key=lambda j: j[0])
            self.jobs.remove(job)
            g = m - 1 - int((step - job[0]) * m)
            self._run(*job, res[8 * g:8 * g + 8, res.shape[1] - 128:])
        for fn in self.hooks.pop(step, []):
            fn()


def _kernel(x_hbm, wqkv_hbm, wphi_hbm, wo_hbm, wr_hbm, wg_hbm, wu_hbm, wd_hbm, out_hbm,
            x_v, xn_v, xs_v, lead_v, wraw_v, wt_v, ws_v, wphi_v, a_v, woraw_v, wos_v, wrraw_v, wr_v,
            kvacc_v, kvbf_v, z_v, zb_v, phi_v, oc_v, oc2_v, h_v, hn_v, o_v, wg_v, wu_v, wd_v, stage_v,
            wgp_v, wup_v, wdp_v, patch_v,
            sem):
    SX, SQ, SO, SM = 0, 6, 6 + 3 * NC, 6 + 3 * NC + NT_ + 1

    def x_copy(i):
        h0, h1 = ((0, 1), (1, 2), (2, 4), (4, 8), (8, 2 * NT_))[i]
        rows = pl.ds(h0 * TH, (h1 - h0) * TH)
        return pltpu.make_async_copy(x_hbm.at[rows, :], x_v.at[rows, :], sem.at[SX + i])

    def k0_copy(s):
        return pltpu.make_async_copy(wqkv_hbm.at[:, pl.ds(D + s * 128, 128)],
                                     wraw_v.at[NC, :, pl.ds(s * 128, 128)], sem.at[(SM + 7, SQ + NC)[s]])

    def w_copy(j, c):
        return pltpu.make_async_copy(wqkv_hbm.at[:, pl.ds(j * D + c * RC, RC)], wraw_v.at[j * NC + c],
                                     sem.at[SQ + j * NC + c])

    def wphi_copy(i):
        h0, h1 = ((0, 8), (16, 24), (8, 16), (24, H))[i]
        return pltpu.make_async_copy(wphi_hbm.at[pl.ds(h0, h1 - h0)], wphi_v.at[pl.ds(h0, h1 - h0)],
                                     sem.at[(SM + 4, SM + 8, SM + 9, SM + 14)[i]])

    wr_copy = pltpu.make_async_copy(wr_hbm, wrraw_v, sem.at[SM + 5])

    def wo_copy(i):
        rows = pl.ds(0, WO_ROWS) if i == 0 else pl.ds(WO_ROWS, QK - WO_ROWS)
        return pltpu.make_async_copy(wo_hbm.at[:, rows, :], woraw_v.at[:, rows, :], sem.at[(SM + 6, SX + 5)[i]])

    wg_copy = pltpu.make_async_copy(wg_hbm.at[:, pl.ds(FM, FV)], wg_v, sem.at[SM + 0])
    wu_copy = pltpu.make_async_copy(wu_hbm.at[:, pl.ds(FM, FV)], wu_v, sem.at[SM + 1])
    wd_copy = pltpu.make_async_copy(wd_hbm.at[pl.ds(0, FVD), :], wd_v, sem.at[SM + 2])

    def stage_copy(i, q):
        if i < 2:
            r0 = q * (D // NQ)
            r0 = r0 if isinstance(r0, int) else pl.multiple_of(r0, D // NQ)
            src = (wg_hbm, wu_hbm)[i].at[pl.ds(r0, D // NQ), pl.ds(0, FM)]
        else:
            r0 = FVD + q * DQ + (i - 2) * DQA
            r0 = r0 if isinstance(r0, int) else pl.multiple_of(r0, 16)
            src = wd_hbm.at[pl.ds(r0, (DQA, DQ - DQA)[i - 2]), :]
        return pltpu.make_async_copy(src, stage_v[i].at[pl.ds(0, src.shape[0]), :], sem.at[SM + 10 + i])

    wphi_copy(0).start()
    k0_copy(0).start()
    x_copy(0).start()
    k0_copy(1).start()
    x_copy(1).start()
    wphi_copy(1).start()
    w_copy(1, 2).start()

    made = set()

    def view(ref, i, n, off=0):
        r0 = off + i * n
        return ref.at[pl.ds(r0 if isinstance(r0, int) else pl.multiple_of(r0, math.gcd(n, off)), n), :]

    def put_blocks(dst, r0, fn, m11, m12, m21, m22, never, a, skip=(), base=0, pitch=HK, gap=None):
        for c0 in range(0, m11.shape[1], 128):
            if c0:
                a = yield gap or GAP_PRO
            d11, d22 = m11[:, c0:c0 + 128], m22[:, c0:c0 + 128]
            if a is not None:
                d = jnp.concatenate([a, a], axis=0)
                d11, d22 = jnp.where(never, d, d11), jnp.where(never, d, d22)
            blocks = fn(d11, m12[:, c0:c0 + 128], m21[:, c0:c0 + 128], d22)
            for i, b in enumerate(blocks):
                if i not in skip:
                    dst[r0:r0 + 8, base + i * pitch + c0:base + i * pitch + c0 + 128] = _pack(b.astype(BF16))

    def rows16(ref, r0, c0=0, w=D):
        return _unpack(ref[r0:r0 + 8, c0:c0 + w]).astype(F32)

    def x_blocks(t, k, lo, hi, never, a, gap=None):
        return put_blocks(view(xs_v, t, TH // 2), k * LNC // 2, _strassen_rhs,
                          lo[:, :HK], hi[:, :HK], lo[:, HK:], hi[:, HK:], never, a, gap=gap)

    def ln_rows(t, k, n, never=None, anchor=None, plain=False):
        wide = lambda c, a: _lane_tile(_after(jnp.broadcast_to(c, (n, 128)), never, a), D // 128)
        x = _after(view(x_v, t, T)[k * n:(k + 1) * n, :].astype(F32), never, anchor)
        s1 = _row_sum(x)
        anchor = yield LN1_GAPS[0]
        xc = x - wide(s1 * (1.0 / D), anchor)
        rstd = lax.rsqrt(_row_sum(xc * xc) * (1.0 / D) + LN_EPS)
        anchor = yield LN1_GAPS[1]
        xn = xc * wide(rstd, anchor)
        if plain:
            xn_v[(t * T + k * n) // 2:(t * T + (k + 1) * n) // 2, :] = _pack(xn.astype(BF16))
        elif k * n < TH:
            xn_v[k * n // 2:(k + 1) * n // 2, :] = _pack(xn.astype(BF16))
        else:
            yield from x_blocks(t, k - TH // LNC, rows16(xn_v, (k * n - TH) // 2), xn, never, anchor, GAP_X)
        return _tree(jnp.add, [rstd[8 * i:8 * i + 8, :] for i in range(min(n, LNC) // 8)])

    def now(gen):
        try:
            while True:
                next(gen)
        except StopIteration as stop:
            return stop.value

    def late_x_blocks(t):
        return lambda k, a: x_blocks(t, k, rows16(xn_v, t * T // 2 + 8 * k),
                                     rows16(xn_v, (t * T + TH) // 2 + 8 * k), never0, a)

    def xn_tile(t):
        return _unpack(xn_v[t * T // 2:(t + 1) * T // 2, :])

    def xs_tile(t):
        return _unpack(view(xs_v, t, TH // 2)[:, 0:7 * HK])

    def expand_wphi(c):
        w = wphi_v[8 * c:8 * c + 8].reshape(8 * DH, DH).astype(F32).T
        bits = pltpu.bitcast(w, U32)
        head = lax.broadcasted_iota(jnp.int32, (DH, 128), 1) >> 5
        for s in range(2):
            b = bits[:, 128 * s:128 * s + 128]
            for j in range(2):
                r0 = 64 * (2 * c + s) + 32 * j
                a_v[r0:r0 + 32, :] = jnp.where(head == 2 * j, b >> 16,
                                               jnp.where(head == 2 * j + 1, b, jnp.uint32(0)))

    wphi_copy(0).wait()
    expand_wphi(0)
    h_v[1][...] = jnp.zeros((T, D), F32)
    if OC_PIN:
        for ref in oc_v + oc2_v:
            ref[0:8, 0:128] = jnp.zeros((8, 128), U32)
    for ref in stage_v:
        ref[ref.shape[0] - 16:, 0:128] = jnp.zeros((16, 128), BF16)

    def v_transpose(k, a):
        q, r0 = (k // 8) + 4 * (k % 2), 256 * (k % 8 // 2)
        w = wraw_v[2 * NC + q // 2, r0:r0 + 256, (q % 2) * 128:(q % 2) * 128 + 128]
        if a is not None:
            w = _unpack(jnp.where(never0, jnp.concatenate([pltpu.bitcast(a, U32)] * 16, axis=0), _pack(w)))
        wt_v[2][64 * q:64 * q + 64, r0:r0 + 256] = _pack(w.T)
        made.add(("vt", k))

    def fold_pairs(j, c, s, side=None, step0=None):
        g0 = 64 * (2 * c + s)
        g0 = g0 if isinstance(g0, int) else pl.multiple_of(g0, 64)
        res = _dot(_unpack(a_v[pl.ds(g0, 64), :]), wraw_v[j * NC + c, :, s * 128:(s + 1) * 128], NT)
        if side is not None:
            side.done(step0 + 2 * s, res[:, :D // 2])
            side.done(step0 + 2 * s + 1, res[:, D // 2:])
        sub = lax.broadcasted_iota(jnp.int32, (8, D), 0)
        out = []
        for q in range(2):
            base = _pair_allreduce(jnp.where(sub < 2, res[64 * q:64 * q + 8, :], 0.0), jnp.add)
            out.append([(res[64 * q + 8 * i:64 * q + 8 * i + 8, :] - base) * LOG2E for i in range(8)])
        return out

    def share(z, z3, k):
        sub = lax.broadcasted_iota(jnp.int32, (8, D), 0)
        return jnp.where(sub < 2, pltpu.roll(z3, 8 - 2 * k, 0), z)

    def packed(slabs):
        return _pack(jnp.concatenate(slabs, axis=0).astype(BF16))

    def fold(j, c, side=None, step0=None):
        p0, p1 = fold_pairs(j, c, 0, side, step0)
        p2, p3 = fold_pairs(j, c, 1, side, step0)
        sl = ([share(p0[0], p3[0], 1), share(p1[0], p3[0], 2)] + p0[1:] + p1[1:]
              + [share(p2[0], p3[0], 3)] + p2[1:] + p3[1:])
        zero = jnp.zeros((8, D), F32)
        even, odd = sl + [zero], [zero] + sl
        r0 = 8 * ((31 * c) // 2)
        is_odd = c % 2 == 1
        if isinstance(c, int):
            sl = odd if is_odd else even
        else:
            r0 = pl.multiple_of(r0, 8)
            sl = [jnp.where(is_odd, o, e) for o, e in zip(odd, even)]
        win = wt_v[j].at[pl.ds(r0, 128), :]
        win[8:128, :] = packed(sl[2:])
        first = packed(sl[:2])
        if is_odd is not False:
            keep = lax.broadcasted_iota(jnp.int32, (8, D), 0) < jnp.where(is_odd, 4, 0)
            first = jnp.where(keep, win[0:8, :], first)
        win[0:8, :] = first
        made.update(("fold", j, q) for q in ([c] if isinstance(c, int) else range(3)))

    def w_blocks(j, k0=0):
        def job(k, a):
            k += k0
            assert made >= ({("vt", 8 * (k // 8) + q) for q in range(8)} if j == 2 else
                            {("fold", j, q) for q in ((0, 2) if k < 15 else range(4))})
            lo, hi = rows16(wt_v[j], 8 * k), rows16(wt_v[j], (256 if j == 2 else 248) + 8 * k)
            yield from put_blocks(ws_v[j], 8 * k, _strassen_lhs, lo[:, :HK], lo[:, HK:], hi[:, :HK], hi[:, HK:],
                                  never0, a, skip=(1, 3))
            made.add(("ws", j, k))
        return job

    def k_pair(p, slot, pr, c0, first, never=None):
        for n in range(c0, c0 + p[0].shape[1], 128):
            assert first == (("z", pr, n) not in made)
            made.update({("z", pr, n), ("phi", slot, pr, n)})
        ep, en, sp, sn = _dual_exp(p)
        inv = _recip(sp * sn)
        scale = (sn * inv, sp * inv)
        es = ep + en
        cols = slice(c0, c0 + p[0].shape[1])
        n = 16 if never is None else 16 // STAGGER
        last = None
        for q in range(16 // n):
            sc = scale
            if last is not None:
                sc = [jnp.where(never, last, x) for x in scale]
            phi = jnp.concatenate([es[i] * sc[i // 8] for i in range(q * n, (q + 1) * n)], axis=0)
            rows = slice(8 * q * n, 8 * (q + 1) * n)
            z = phi if first else z_v[pr, rows, cols] + phi
            z_v[pr, rows, cols] = z
            phi_v[slot][64 * pr + 4 * q * n:64 * pr + 4 * (q + 1) * n, cols] = _pack(phi.astype(BF16))
            last = z[8 * n - 8:, :]

    def k_features(pk, slot, c, first, never=None):
        for j in range(PPC):
            k_pair(_pair_logits(pk, j), slot, c * PPC + j, 0, first, never)

    def kv_update(vts, slot, g, first, publish=False):
        for q, vt in enumerate(vts):
            for j in range(2):
                pr = 2 * g + 8 * q + j
                assert made >= {("phi", slot, pr, 0), ("phi", slot, pr, 128)}
                upd = _dot(vt[64 * j:64 * j + 64, :].astype(BF16), _unpack(phi_v[slot][64 * pr:64 * pr + 64, :]), NT)
                acc = upd if first else kvacc_v[pr] + upd
                kvacc_v[pr] = acc
                if publish:
                    odd = -(lax.broadcasted_iota(jnp.int32, (32, 128), 1) & 1)
                    bits = pltpu.bitcast(acc, jnp.int32) & jnp.concatenate([~odd, odd], axis=0)
                    kvbf_v[32 * pr:32 * pr + 32, :] = _pack(pltpu.bitcast(bits, F32).astype(BF16))

    def save_lead(t):
        view(lead_v, t, HK // 2)[...] = _pack(_unpack(view(xs_v, t, TH // 2)[:, 0:HK]).T)

    def proj_feat(side, step0, c, xn, carry):
        r0 = 8 * ((31 * c) // 2)
        skip = 8 if c % 2 == 1 and carry is not None else 0
        w = wt_v[1][r0 + skip:r0 + 128, :]
        quarters = []
        for n in range(2):
            for m in range(2):
                step = step0 + 2 * n + m
                wq = _unpack(side.gate(step, w[:64, :] if m == 0 else w[64:, :]))
                res = _dot(wq, xn[n * TH:(n + 1) * TH, :], NT)
                side.done(step, res)
                quarters.append(res)
        res = jnp.concatenate(
            [jnp.concatenate([quarters[0], quarters[2]], axis=1),
             jnp.concatenate([quarters[1], quarters[3]], axis=1)], axis=0)
        sl = [res[8 * i:8 * i + 8, :] for i in range(res.shape[0] // 8)]
        if c % 2 == 0:
            return sl[:31], sl[31]
        return ([carry] + sl if skip else sl[1:]), None

    def proj_unit(side, step0, j, b, xs, lead=None, plain=None):
        r1 = 64 * b + (64 if j == 2 or b < 3 else 56)
        assert made >= ({("vt", 8 * b + q) for q in range(8)} if plain is not None else
                        {("ws", j, k) for k in range(8 * b, r1 // 8)})
        if plain is not None:
            out = []
            for q in range(2):
                row = []
                for n in range(2):
                    res = _dot(_unpack(wt_v[2][256 * q + 64 * b:256 * q + r1, :]), plain[n * TH:(n + 1) * TH, :], NT)
                    for i in range((0, 2, 4, 5)[2 * q + n], (2, 4, 5, 7)[2 * q + n]):
                        side.done(step0 + i, res)
                    row.append(res)
                out.append(jnp.concatenate(row, axis=1))
            return out

        def product(i):
            off = 256 if j == 2 else 248
            w = (wt_v[j][off + 64 * b:off + r1, HK:] if i == 1 else wt_v[j][64 * b:r1, :HK] if i == 3
                 else ws_v[j][64 * b:r1, i * HK:(i + 1) * HK])
            w = _unpack(side.gate(step0 + i, w))
            if lead is not None and i == 0:
                res = _dot(w, _unpack(view(lead_v, lead, HK // 2)[...]), NN)
            else:
                res = _dot(w, xs[:, i * HK:(i + 1) * HK], NT)
            side.done(step0 + i, res)
            return res
        return [jnp.concatenate(row, axis=1) for row in _strassen(product)]

    def feat_stage(side, step0, j, xs, pair_fn, lead=None):
        sl = [[], []]
        for b in range(4):
            for q, res in enumerate(proj_unit(side, step0 + 7 * b, j, b, xs, lead if b == 0 else None)):
                sl[q] += [res[8 * i:8 * i + 8, :] for i in range(res.shape[0] // 8)]
            for q in (1, 0):
                for jj in (2 * (b % 2), 2 * (b % 2) + 1):
                    pair_fn(_pair_logits(sl[q][31 * (b // 2):], jj), 8 * q + 4 * (b // 2) + jj)

    def v_stage(side, xs, slot, first, publish, lead, plain=None):
        pending = None
        for g in range(4):
            if pending is not None:
                side.hooks.setdefault(7 * g + D_LAG, []).append(lambda p=pending: kv_update(*p))
            pending = (proj_unit(side, 7 * g, 2, g, xs, lead if g == 0 else None, plain if g < PLAIN_V0 else None),
                       slot, g, first, publish)
        side.check()
        return pending

    def pack_rows(src, dst, r0, c0, cols, never, a):
        for c in range(c0, c0 + cols, PACK_W):
            if c > c0:
                a = yield GAP_PACK
            w = min(PACK_W, c0 + cols - c)
            v = src[r0:r0 + 16, c:c + w].astype(F32)
            v = jnp.concatenate([jnp.where(never, _lane_tile(a, w // 128), v[0:8, :]), v[8:16, :]], axis=0)
            dst[r0 // 2:r0 // 2 + 8, c:c + w] = _pack(v.astype(BF16))

    def stash_at(i, k, n):
        return zb_v.at[4 * i + 2 * (k // 16) + n, pl.ds(8 * (k % 16), 8), :]

    def stash(i, sl):
        for k, v in enumerate(sl):
            for n in range(2):
                stash_at(i, k, n)[...] = v[:, 128 * n:128 * n + 128]

    def stashed_k(i, slot, c, first):
        def job(k, a):
            j, n = k // 2, k % 2
            p = _pair_logits([stash_at(i, q, n)[...] for q in range(31)], j)
            k_pair([_after(p[0], never0, a)] + p[1:], slot, c * PPC + j, 128 * n, first, never0)
        return job

    def first_rows(k0, k1, n):
        xn = _unpack(xn_v[n * TH // 2:(n + 1) * TH // 2, :])
        ks = [k for k in range(k0, k1)]
        w = jnp.concatenate([wt_v[1][4 * (k % 32):4 * (k % 32) + 8, :] for k in ks[::2]], axis=0)
        res = _dot(_unpack(w), xn, NT)
        for q, k in enumerate(ks):
            if k % 32 < 31:
                stash_at(0, k % 32, n)[...] = res[8 * q:8 * q + 8, :]

    k0_copy(0).wait()
    x_copy(0).wait()
    wphi_copy(2).start()
    w_copy(1, 1).start()
    wphi_copy(3).start()
    x_copy(2).start()
    p0, p1 = fold_pairs(1, 0, 0)
    wt_v[1][8:64, :] = packed(p0[1:] + p1[1:])
    h_v[0][0:8, :] = p0[0]
    h_v[0][8:16, :] = p1[0]
    never0 = now(ln_rows(0, 0, TH, plain=True))[0, 0] < 0.0
    first_rows(2, 16, 0)

    k0_copy(1).wait()
    x_copy(1).wait()
    wphi_copy(1).wait()
    w_copy(1, 3).start()
    for c in (0, 2, 1, 3):
        w_copy(2, c).start()
    p2, p3 = fold_pairs(1, 0, 1)
    wt_v[1][0:8, :] = packed([share(h_v[0][0:8, :], p3[0], 1), share(h_v[0][8:16, :], p3[0], 2)])
    wt_v[1][64:128, :] = packed([share(p2[0], p3[0], 3)] + p2[1:] + p3[1:] + [jnp.zeros((8, D), F32)])
    made.add(("fold", 1, 0))
    now(ln_rows(0, 1, TH, plain=True))
    first_rows(16, 34, 0)
    first_rows(0, 16, 1)
    first_rows(16, 32, 1)
    expand_wphi(2)

    for c, prev in ((2, 0), (1, 2)):
        w_copy(1, c).wait()
        wphi_copy(4 - c).wait()
        expand_wphi(5 - 2 * c)
        side = _Side(never0, lambda rel, gap: min(rel + gap, 7))
        if c == 2:
            side.add(PRO_X0_PLAN, late_x_blocks(0))
        else:
            side.add(PRO_W0_PLAN, w_blocks(1))
        side.add((PRO_K_PLANS0, PRO_K_PLANS1)[2 - c], stashed_k(prev, 0, prev, True))
        fold(1, c, side, 0)
        stash(c, proj_feat(side, 4, c, xn_tile(0), None)[0])
        side.check()

    x_copy(2).wait()
    w_copy(1, 3).wait()
    x_copy(3).start()
    w_copy(0, 0).start()
    wo_copy(0).start()
    x_copy(4).start()
    for c in range(1, NC):
        w_copy(0, c).start()
    wo_copy(1).start()
    wr_copy.start()
    for i in range(4):
        stage_copy(i, 0).start()
    wg_copy.start()
    wu_copy.start()
    wd_copy.start()
    side = _Side(never0, lambda rel, gap: min(rel + gap, 19))
    side.add(PRO_LN1_PLAN, lambda k, a: ln_rows(1, k, LNC, never0, a, plain=True))
    side.add(PRO_W_PLAN, w_blocks(1, len(PRO_W0_PLAN)))
    side.add(PRO_K_PLANS2, stashed_k(1, 0, 1, False))
    fold(1, 3, side, 0)
    stash(3, proj_feat(side, 4, 3, xn_tile(0), None)[0])
    xn1 = xn_tile(1)
    spare = None
    for c in range(3):
        pk, spare = proj_feat(side, 8 + 4 * c, c, xn1, spare)
        if c < 2:
            k_features(pk, 1, c, c == 1, never0)
        else:
            stash(0, pk + [spare])
    side.check()

    for c in range(NC):
        w_copy(2, c).wait()
    side = _Side(never0, lambda rel, gap: min(rel + gap, 27))
    side.add(PRO_V_PLANS[0], v_transpose)
    side.add(PRO_V_PLANS[1], stashed_k(3, 0, 3, False))
    side.add(PRO_V_PLANS[2], stashed_k(0, 1, 2, False))
    side.add(PRO_V_PLANS[3], late_x_blocks(1))
    side.add(PRO_V_PLANS[4], w_blocks(2))
    spare = jnp.concatenate([stash_at(0, 31, n)[...] for n in range(2)], axis=1)
    k_features(proj_feat(side, -4, 3, xn_tile(1), spare)[0], 1, 3, True, never0)
    kv_update(*v_stage(side, xs_tile(0), 0, True, False, None, xn_tile(0)))
    save_lead(0)
    save_lead(1)
    for r0 in (0, 248):
        wt_v[0][r0:r0 + 8, :] = jnp.zeros((8, D), U32)

    def phase1(u, carry):
        never = u < 0

        @pl.when(u == 0)
        def _():
            x_copy(3).wait()
            w_copy(0, 0).wait()
            wo_copy(0).wait()

        @pl.when(u == 1)
        def _():
            x_copy(4).wait()
            w_copy(0, 1).wait()
            w_copy(0, 2).wait()
            wo_copy(1).wait()

        def wo_blocks(k0):
            def job(k, a):
                k += k0
                r, c, part = k // 4, 128 * (k // 2 % 2), k % 2
                r0 = u * ((QK - WO_ROWS) // 2)
                dst = wos_v.at[pl.ds(pl.multiple_of(r0 // 2, 8), WO_ROWS // 2), :]

                def piece(kq, nq):
                    src = woraw_v.at[kq, pl.ds(pl.multiple_of(r0, 16), WO_ROWS), :]
                    return src[16 * r:16 * r + 16, nq * QK + c:nq * QK + c + 128].astype(F32)
                outer = [_strassen_rhs(piece(ki, ni), piece(ki, 2 + ni), piece(2 + ki, ni), piece(2 + ki, 2 + ni))
                         for ki in range(2) for ni in range(2)]
                for i in range(4) if part == 0 else range(4, 7):
                    if i % 4:
                        a = yield GAP_WO
                    yield from put_blocks(dst, 8 * r, _strassen_rhs, *[o[i] for o in outer], never, a,
                                          base=7 * i * QK + c, pitch=QK)
            return job

        xs = xs_tile(2 * u + 1)
        side = _Side(never, lambda rel, gap: min(rel + gap, 27))
        for i in range(2):
            t = 2 * u + 2 + i
            if i == 0:
                side.add(LN1_PLANS[0], lambda k, a: ln_rows(2 * u + 2, k, LNC, never, a))
                side.add(WO_PLANS[0], wo_blocks(0))
            pending = v_stage(side, xs, 1 - i, False, False, t - 1 if i == 0 else None)
            xs = xs_tile(t)
            side = _Side(never, lambda rel, gap, end=(27, -1)[i]: min(rel + gap, end))
            if i == 0:
                side.add(LN1_PLANS[1], lambda k, a: ln_rows(2 * u + 3, k, LNC, never, a))
                side.add(WO_PLANS[1], wo_blocks(len(WO_PLANS[0])))
            else:
                side.add(WO_PLANS[2], wo_blocks(24 - len(WO_PLANS[2])))
            side.hooks[-28 + D_LAG] = [lambda p=pending: kv_update(*p)]
            feat_stage(side, -28, 1, xs, lambda p, pr: k_pair(p, i, pr, 0, False, never if i == 1 else None))
            save_lead(t)
        side.check()
        fold(0, u)
        return carry

    lax.fori_loop(0, (NT_ - 2) // 2, phase1, 0)

    w_copy(0, 3).wait()
    wr_copy.wait()
    side = _Side(never0, lambda rel, gap: min(rel + gap, 27 if rel < 98 else 103))

    def z_final(k, a):
        zb_v[k] = jnp.broadcast_to(_row_sum(_after(z_v[k], never0, a)), (128, 128))

    side.add(END_PLANS[0], z_final)
    side.add(END_PLANS[1], w_blocks(0))
    fold(0, 3, side, 100)
    kv_update(*v_stage(side, xs_tile(NT_ - 1), 1, False, True, None))
    wr_v[...] = jnp.broadcast_to(wrraw_v[...].reshape(1, D).astype(F32), (8, D))

    def o_copy(r0, n, i):
        return pltpu.make_async_copy(o_v.at[pl.ds(r0, n), :], out_hbm.at[pl.ds(r0, n), :], sem.at[SO + i])

    def finish_rows(h_ref, k, t, valid, st, never=None, anchor=None):
        r0 = t * T + k * LNC
        rows = slice(k * LNC, (k + 1) * LNC)
        m = jnp.broadcast_to(_row_sum(_after(h_ref[rows, :], never, anchor)) * (1.0 / D), (LNC, 128))
        rstd, r = [], []
        for i in range(LNC // 8):
            anchor = yield LN2_GAPS[2] if i else LN2_GAPS[0]
            mi = _after(m[8 * i:8 * i + 8, :], never, anchor)
            hc = h_ref[k * LNC + 8 * i:k * LNC + 8 * i + 8, :] - _lane_tile(mi, D // 128)
            rs = lax.rsqrt(_row_sum(hc * hc) * (1.0 / D) + LN_EPS)
            r.append((_row_sum(hc * wr_v[...]) * rs + 0.0).astype(BF16).astype(F32))
            rstd.append(jnp.broadcast_to(rs, (8, 128)))
        rstd = jnp.concatenate(rstd, axis=0)
        w = D if never is None else D // LN2_SPLIT
        for c in range(0, D, w):
            anchor = yield LN2_GAPS[2] if c else LN2_GAPS[1]
            h = h_ref[rows, c:c + w]
            hn = (h - _lane_tile(_after(m, never, anchor), w // 128)) * _lane_tile(rstd, w // 128)
            view(hn_v, t, T // 2)[k * LNC // 2:(k + 1) * LNC // 2, c:c + w] = _pack(hn.astype(BF16))
            view(o_v, t, T)[rows, c:c + w] = (hn + h).astype(BF16)
        best = st["route"]
        sub = lax.broadcasted_iota(jnp.int32, (8, 128), 0)
        for i, ri in enumerate(r):
            key = _ordered(pltpu.bitcast(jnp.broadcast_to(ri, (8, 128)), jnp.int32)) | ((S - 1 - r0 - 8 * i) - sub)
            if valid is not None:
                key = jnp.where(valid, key, KEY_MIN)
            best = jnp.maximum(best, key)
        st["route"] = best
        return pltpu.bitcast(best, F32)

    def q_pair(p, slot, pr):
        ep, en, sp, sn = _dual_exp(p)
        zz = [_lane_tile(zb_v[pr, 8 * i:8 * i + 8, :], T // 128) for i in range(16)]
        ap = _pair_allreduce(_tree(jnp.add, [ep[i] * zz[i] for i in range(8)]), jnp.add)
        an = _pair_allreduce(_tree(jnp.add, [en[i] * zz[8 + i] for i in range(8)]), jnp.add)
        inv = _recip(ap * sn + (an + 1e-6 * sn) * sp)
        rp = sn * inv
        rn = sp * inv
        phi = jnp.concatenate([e * rp for e in ep] + [e * rn for e in en], axis=0)
        phi_v[slot][64 * pr:64 * pr + 64, :] = _pack(phi.astype(BF16))

    held = []

    def attn_blocks(slot, g, deps):
        res = [_dot(_unpack(kvbf_v[32 * pr:32 * pr + 32, :]), _unpack(phi_v[slot][64 * pr:64 * pr + 64, :]), NN)
               for pr in (2 * g, 2 * g + 8, 2 * g + 1, 2 * g + 9)]
        lo, hi = jnp.concatenate(res[0::2], axis=0), jnp.concatenate(res[1::2], axis=0)
        blocks = [(i, g, b) for i, b in enumerate(_strassen_lhs(lo[:, :TH], hi[:, :TH], lo[:, TH:], hi[:, TH:]))]
        if g % 2 == 0:
            held.append(blocks.pop())
        else:
            blocks.append(held.pop())
        ot = _pack(jnp.concatenate([b for _, _, b in blocks], axis=1).astype(BF16).T)
        for q, (i, n, _) in enumerate(blocks):
            oc_v[slot][:, i * HK + 128 * n:i * HK + 128 * n + 128] = ot[q * TH // 2:(q + 1) * TH // 2, :]
            made.add(("oc", slot, i, n))
            if q % 2:
                deps.append(pltpu.bitcast(ot[(q + 1) * TH // 2 - 8:(q + 1) * TH // 2, :], F32))

    def o_blocks(slot, c, never):
        def job(k, a):
            k = (2, 3, 1, 4, 5, 0, 6)[k]
            assert made >= {("oc", slot, k, c), ("oc", slot, k, c + 2)}
            for r in range(4):
                if r:
                    a = yield GAP_O2
                m = [rows16(oc_v[slot], 8 * r + 32 * q, k * HK + n * QK + 128 * c, 128)
                     for q in range(2) for n in range(2)]
                yield from put_blocks(oc2_v[slot], 8 * r, _strassen_lhs, *m, never, a, skip=(1, 3),
                                      base=7 * k * QK + 128 * c, pitch=QK)
            made.add(("oc2", slot, k, c))
        return job

    def out_proj(side, step0, t, slot):
        count = [0]

        def inner(i, c):
            assert made >= {("oc2", slot, i, 0), ("oc2", slot, i, 1)}

            def product(j):
                step, odd = step0 + count[0] // 2, count[0] % 2
                count[0] += 1
                o = (oc_v[slot][32:64, i * HK + QK:(i + 1) * HK] if j == 1 else
                     oc_v[slot][0:32, i * HK:i * HK + QK] if j == 3 else
                     oc2_v[slot][:, (7 * i + j) * QK:(7 * i + j + 1) * QK])
                w = wos_v[:, (7 * i + j) * QK + 128 * c:(7 * i + j) * QK + 128 * c + 128]
                res = _dot(_unpack(o), _unpack(w if odd else side.gate(step, w)), NN)
                if odd:
                    side.done(step, res)
                return res
            return _block(_strassen(product))

        xt = view(x_v, t, T)

        def emit(cs, q, r, res):
            for k, c in enumerate(cs):
                for n in range(2):
                    rows, c0 = slice(q * TH, (q + 1) * TH), r * HK + n * QK + 128 * c
                    h_v[slot][rows, c0:c0 + 128] = (res[:, 256 * k + 128 * n:256 * k + 128 * n + 128]
                                                    + xt[rows, c0:c0 + 128].astype(F32))
                made.add(("h", slot, q, r, c))

        for cs in ((0,), (1,)) if OUT_ORDER == 0 else ((0, 1),):
            _strassen_rows_first(lambda i: jnp.concatenate([inner(i, c) for c in cs], axis=1),
                                 lambda q, r, res: emit(cs, q, r, res))

    def phase2(u, carry):
        for i in range(4):
            stage_copy(i, u).wait()
        never = u < 0
        side = _Side(never, lambda rel, gap: min(rel + 2 * gap, 97) if rel < 98 else
                     rel + gap if rel + gap <= 155 else 2 * (rel + gap - 155) - 1)
        st = {"route": carry}
        tp = jnp.maximum(2 * u - 1, 0)
        early = len(LN2_PLANS[2])
        order = []

        def ln2(slot, t, valid, k0, key):
            def job(k, a):
                k += k0
                hs = {("h", slot, k // 8, r, c) for r in range(2) for c in range(2)}
                assert made >= hs or key == 0
                best = yield from finish_rows(h_v[slot], k, t, valid, st, never, a)
                assert key > 0 or not made & hs
                order.append((key, k))
                assert order == sorted(order)
                return best
            return job

        side.add(LN2_PLANS[0], ln2(1, tp, u > 0, early, 0))
        side.add(LN2_PLANS[1], ln2(0, 2 * u, None, 0, 1))
        side.add(LN2_PLANS[2], ln2(1, 2 * u + 1, None, 0, 2))

        def packer(i, dst, n):
            left = [n]

            def job(k, a):
                if i < 2:
                    yield from pack_rows(stage_v[i], dst, (k // 2) * 16, (0, D)[k % 2], (D, FM - D)[k % 2], never, a)
                else:
                    yield from pack_rows(stage_v[i], dst, k * 16, 0, D, never, a)
                left[0] -= 1
                if not left[0]:
                    stage_copy(i, jnp.minimum(u + 1, NQ - 1)).start()
                    n0 = stage_v[i].shape[0] - 16
                    side.deps.setdefault(PACK_DUE[i], []).append(stage_v[i][n0:n0 + 8, 0:128].astype(F32))
            return job

        for i in range(2):
            side.add(PACK_PLANS[i], packer(i, view((wgp_v, wup_v)[i], u, D // NQ // 2), len(PACK_PLANS[i])))
            d0 = pl.multiple_of(u * (DQ // 2) + i * (DQA // 2), 8)
            side.add(PACKD_PLANS[i], packer(2 + i, wdp_v.at[pl.ds(d0, 8 * len(PACKD_PLANS[i])), :],
                                            len(PACKD_PLANS[i])))
            for g in range(4):
                step = 107 + 28 * i + 7 * g + G_LAG
                wrap = lambda x: x if x < 156 else 2 * (x - 156) + 1
                side.hooks.setdefault(wrap(step), []).append(
                    lambda i=i, g=g, due=wrap(step + O_DUE): attn_blocks(i, g, side.deps.setdefault(due, [])))
            for c in range(2):
                side.add(O2_PLANS[2 * i + c], o_blocks(i, c, never))
        for i in range(2):
            feat_stage(side, 100 + 28 * i, 0, xs_tile(2 * u + i), lambda p, pr: q_pair(p, i, pr),
                       2 * u if i == 0 else None)
        for i in range(2):
            out_proj(side, 49 * i, 2 * u + i, i)
        side.check()

        @pl.when(u == 0)
        def _():
            o_copy(0, T, 0).start()

        @pl.when(u > 0)
        def _():
            o_copy(pl.multiple_of(tp * T, T), 2 * T, u).start()

        return st["route"]

    wg_copy.wait()
    wu_copy.wait()
    wd_copy.wait()
    route = lax.fori_loop(
        0, NT_ // 2, phase2,
        jnp.full((8, 128), KEY_MIN, jnp.int32))
    st = {"route": route}
    for k in range(len(LN2_PLANS[2]), T // LNC):
        now(finish_rows(h_v[1], k, NT_ - 1, None, st))
    o_copy(S - T, T, NT_).start()

    best = st["route"]
    for shift in (4, 2, 1):
        best = jnp.maximum(best, pltpu.roll(best, shift, 0))
    idx_s = (S - 1) - (best[0, 0] & (S - 1))
    gate = _lane_tile(jax.nn.sigmoid(pltpu.bitcast(_ordered(best & -65536), F32)), D // 128)
    blk = pl.multiple_of((idx_s >> 4) << 4, 16)
    pair = jnp.broadcast_to(hn_v[pl.ds(idx_s >> 1, 1), :], (8, D))
    x8 = pltpu.bitcast(jnp.where((idx_s & 1) == 1, pair & jnp.uint32(0xFFFF0000), pair << 16), F32)
    xs = jnp.concatenate([x8, x8], axis=0).astype(BF16)
    acts, anchors = [], []

    def park(v, half):
        n = v.shape[0] // 128
        for i in range(n):
            z_v[i, :, 128 * half:128 * half + 128] = v[128 * i:128 * i + 128, :]
        return jnp.concatenate([z_v[i, :, 128 * half:128 * half + 128] for i in range(n)], axis=0)

    for c0 in range(0, FM, 128):
        g = _dot(xs, _unpack(wgp_v[:, c0:c0 + 128]), NN)[0:8, :]
        u = _dot(xs, _unpack(wup_v[:, c0:c0 + 128]), NN)[0:8, :]
        anchors += [g, u]
        acts.append(g * jax.nn.sigmoid(g) * u)
    xb = park(_col_broadcast(x8), 0)
    g, u = [_sublane_allreduce(_vpu_matvec(
        xb, lambda g: w[8 * g:8 * g + 8, :].astype(F32), never0,
        anchors[i * MOE_NA // 2:(i + 1) * MOE_NA // 2], MOE_LAGS[0])) for i, w in enumerate((wg_v, wu_v))]
    acts.append(g * jax.nn.sigmoid(g) * u)
    a = jnp.concatenate(acts, axis=1)
    am = jnp.concatenate([a[:, FVD:], a[:, FVD:]], axis=0).astype(BF16)
    ys, anchors = [], anchors[MOE_NA:]
    for k0 in range(0, FF - FVD, 512):
        k1 = min(k0 + 512, FF - FVD)
        yk = _dot(am[:, k0:k1], _unpack(wdp_v[k0 // 2:k1 // 2, 0:D]), NN)[0:8, :]
        ys.append(yk)
        anchors += [yk[:, c:c + 128] for c in range(128, D, 256)]
    ys.append(_sublane_allreduce(_vpu_matvec(
        park(_col_broadcast(a[:, :FVD]), 1), lambda g: wd_v[8 * g:8 * g + 8, :].astype(F32), never0,
        anchors[:-MOE_ND], MOE_LAGS[1])))
    y = _tree(jnp.add, ys) * gate
    y = jnp.concatenate([y, y], axis=0)
    sel = lax.broadcasted_iota(jnp.int32, (16, 1), 0) == (idx_s - blk)
    patch_v[...] = (o_v[pl.ds(blk, 16), :].astype(F32) + jnp.where(sel, y, 0.0)).astype(BF16)
    o_copy(0, T, 0).wait()
    for u in range(1, NT_ // 2):
        o_copy((2 * u - 1) * T, 2 * T, u).wait()
    o_copy(S - T, T, NT_).wait()
    pc = pltpu.make_async_copy(patch_v, out_hbm.at[pl.ds(blk, 16), :], sem.at[SM + 3])
    pc.start()
    for i in range(4):
        stage_copy(i, NQ - 1).wait()
    pc.wait()


@jax.jit
def pallas_sequential_preLN__linear_kernel_hedgehog__moe_arch_mod__prompt_kernel(
    A_x: jax.Array,
    A_wqkv: jax.Array,
    A_w_phi: jax.Array,
    A_wo: jax.Array,
    B_x: jax.Array,
    B_w_r: jax.Array,
    B_w_gate: jax.Array,
    B_w_up: jax.Array,
    B_w_down: jax.Array,
):
    del B_x
    hbm = pl.BlockSpec(memory_space=pl.ANY)
    out = pl.pallas_call(
        _kernel,
        out_shape=jax.ShapeDtypeStruct((S, D), BF16),
        in_specs=[hbm] * 8,
        out_specs=hbm,
        scratch_shapes=[
            pltpu.VMEM((S, D), BF16),
            pltpu.VMEM((T, D), U32),
            pltpu.VMEM((NT_ * TH // 2, SW), U32),
            pltpu.VMEM((NT_ * HK // 2, 128), U32),
            pltpu.VMEM((3 * NC, D, RC), BF16),
            [pltpu.VMEM((D // 2, D), U32)] * 3,
            [pltpu.VMEM((HK // 2, 7 * HK), U32)] * 3,
            pltpu.VMEM((H, DH, DH), BF16),
            pltpu.VMEM((8 * 64, 128), U32),
            pltpu.VMEM((4, QK, D), BF16),
            pltpu.VMEM((QK // 2, 49 * QK + 128), U32),
            pltpu.VMEM((D,), BF16),
            pltpu.VMEM((8, D), F32),
            pltpu.VMEM((NPAIR, 64, 128), F32),
            pltpu.VMEM((NPAIR * 32, 128), U32),
            pltpu.VMEM((NPAIR, 128, T), F32),
            pltpu.VMEM((NPAIR, 128, 128), F32),
            [pltpu.VMEM((NPAIR * 64, T), U32)] * 2,
            [pltpu.VMEM((TH // 2, 7 * HK), U32)] * 2,
            [pltpu.VMEM((TH // 4, 49 * QK), U32)] * 2,
            [pltpu.VMEM((T, D), F32)] * 2,
            pltpu.VMEM((S // 2, D), U32),
            pltpu.VMEM((S, D), BF16),
            pltpu.VMEM((D, FV), BF16),
            pltpu.VMEM((D, FV), BF16),
            pltpu.VMEM((FVD, D), BF16),
            [pltpu.VMEM((D // NQ + 16, FM), BF16), pltpu.VMEM((D // NQ + 16, FM), BF16),
             pltpu.VMEM((DQA + 16, D), BF16), pltpu.VMEM((DQ - DQA + 16, D), BF16)],
            pltpu.VMEM((D // 2, FM), U32),
            pltpu.VMEM((D // 2, FM), U32),
            pltpu.VMEM(((FF - FVD) // 2, D + 128), U32),
            pltpu.VMEM((16, D), BF16),
            pltpu.SemaphoreType.DMA((6 + 3 * NC + NT_ + 16,)),
        ],
        compiler_params=pltpu.CompilerParams(vmem_limit_bytes=100 * 1024 * 1024,
                                             disable_semaphore_checks=True, disable_bounds_checks=True),
        name="hedgehog_mod",
    )(
        A_x.reshape(S, D),
        A_wqkv,
        A_w_phi,
        A_wo.reshape(4, QK, D),
        B_w_r,
        B_w_gate,
        B_w_up,
        B_w_down,
    )
    return out.reshape(1, S, D)
```

```python
import math

import jax
import jax.numpy as jnp
from jax import lax
import jax.experimental.pallas as pl
import jax.experimental.pallas.tpu as pltpu

F32 = jnp.float32
BF16 = jnp.bfloat16
U32 = jnp.uint32

S = 2048
D = 1024
H = 32
DH = 32
FF = 3584
NPAIR = H // 2
LOG2E = 1.4426950408889634
LN_EPS = 1e-5
KEY_MIN = -2 ** 31

T = 256
TH = T // 2
NT_ = S // T
RC = 256
NC = D // RC
PPC = RC // 64
LNC = 16

FV = 10 * 128
FM = FF - FV
FVD = 8 * 128
NQ = NT_ // 2
DQ = (FF - FVD) // NQ
WO_ROWS = 96
QK = D // 4
HK = D // 2
SW = 8 * HK


def _spread(n, a, b, due=None):
    rel = [round(a + (b - a) * k / (n - 1), 3) for k in range(n)]
    return tuple((r, None if due is None else math.ceil(r) + due) for r in rel)


LN1_PLANS = (((0.072, 7), (0.452, 7), (2.8, 9), (4.2, 11), (5.323, 12), (7.125, 13), (8.42, 16), (9.93, 16),
    (11.174, 18), (11.723, 19), (13.877, 22), (15.466, 23), (16.77, 23), (18.221, 25), (19.564, 26), (21.5,
    27)), ((-1.151, 5), (1.211, 7), (1.804, 8), (3.369, 9), (5.17, 11), (5.924, 14), (8.015, 14), (9.695, 17),
    (10.176, 17), (11.93, 19), (13.665, 19), (15.339, 22), (16.785, 22), (18.546, 25), (19.47, 26), (21.122,
    27)))
PRO_LN1_PLAN = ((None, None),) * 16
PRO_K_PLANS0 = ((0.015, None), (0.845, None), (1.721, None), (2.97, None), (3.496, None), (4.341, None),
    (5.723, None), (5.845, None))
PRO_K_PLANS1 = ((-0.801, None), (0.772, None), (1.348, None), (2.924, None), (3.623, None), (3.848, None),
    (4.758, None), (5.626, None))
PRO_X0_PLAN = ((-0.051, None), (1.805, None), (2.734, None), (3.191, None), (3.45, None), (4.522, None),
    (5.302, None), (5.861, None))
PRO_W0_PLAN = ((0.036, None), (0.555, None), (2.188, None), (2.72, None), (3.235, None), (3.839, None),
    (4.525, None), (4.908, None), (5.417, None), (6.465, None))
PRO_W_PLAN = ((0.281, None), (0.962, None), (2.192, None), (2.998, None), (3.693, None), (8.405, None), (9.19,
    None), (9.659, None), (10.206, None), (11.168, None), (11.803, None), (12.534, None), (12.982, None),
    (13.534, None), (14.32, None), (15.084, None), (15.792, None), (16.395, None), (16.945, None), (18.04,
    None), (18.437, None))
PRO_K_PLANS2 = ((15.04, None), (15.879, None), (15.938, None), (16.523, None), (16.865, None), (17.33, None),
    (17.649, None), (17.852, None))
PRO_V_PLANS = (((None, None), (None, None), (None, None), (None, None), (None, None), (None, None), (None,
    None), (None, None), (-3.675, None), (-3.235, None), (-3.152, None), (-2.663, None), (-2.285, None),
    (-2.177, None), (-1.839, None), (-1.602, None), (-1.468, None), (-1.323, None), (-0.973, None), (-0.246,
    None), (0.001, None), (0.112, None), (0.421, None), (0.913, None), (0.98, None), (1.132, None), (1.604,
    None), (1.767, None), (1.869, None), (2.278, None), (2.807, None), (3.005, None)), ((9.073, None),
    (10.016, None), (12.71, None), (12.797, None), (13.345, None), (14.676, None), (18.136, None), (18.863,
    None)), ((20.331, None), (21.08, None), (21.596, None), (22.599, None), (22.815, None), (23.574, None),
    (24.852, None), (26.895, None)), ((16.477, None), (18.357, None), (19.602, None), (19.911, None), (22.438,
    None), (23.242, None), (24.397, None), (25.564, None)), ((18.94, None), (20.207, None), (21.27, None),
    (22.04, None), (23.77, None), (24.709, None), (25.305, None), (26.271, None), (-1.476, None), (-0.298,
    None), (0.085, None), (1.471, None), (1.717, None), (3.379, None), (3.723, None), (5.19, None), (5.371,
    None), (6.512, None), (7.542, None), (8.444, None), (8.686, None), (9.511, None), (10.795, None), (11.558,
    None), (11.774, None), (12.134, None), (13.8, None), (15.151, None), (15.328, None), (16.443, None),
    (17.153, None), (17.72, None)))
END_PLANS = (((-0.162, None), (2.011, None), (3.829, None), (5.62, None), (6.909, None), (8.134, None),
    (10.634, None), (12.371, None), (13.954, None), (15.538, None), (16.797, None), (19.352, None), (20.737,
    None), (23.183, None), (23.393, None), (25.88, None)), ((100.308, None), (101.389, None), (102.104, None),
    (0.409, None), (1.005, None), (2.198, None), (2.898, None), (4.205, None), (5.131, None), (6.022, None),
    (7.291, None), (7.974, None), (8.425, None), (10.079, None), (11.3, None), (11.768, None), (12.903, None),
    (13.561, None), (14.696, None), (15.687, None), (17.565, None), (18.013, None), (18.596, None), (19.613,
    None), (20.25, None), (21.235, None), (22.366, None), (23.06, None), (24.673, None), (25.256, None),
    (25.849, None)))
WO_PLANS = (((0.245, None), (6.671, None), (13.134, None), (18.635, None), (25.68, None)), ((-26.952, None),
    (-20.774, None), (-16.958, None), (-12.341, None), (-8.3, None), (-2.883, None), (1.607, None), (6.233,
    None), (10.547, None), (15.312, None), (19.974, None), (24.229, None)), ((-27.525, None), (-22.089, None),
    (-18.962, None), (-14.225, None), (-9.98, None), (-6.618, None), (-2.09, None)))
LN2_PLANS = (((-0.5, 12), (1.385, 15), (5.612, 19), (6.544, 21), (11.772, 24), (14.638, 27), (17.452, 29),
    (19.2, 33), (23.964, 36), (26.706, 40), (29.685, 42), (33.006, 45)), ((35.739, 47), (38.936, 51), (41.779,
    54), (45.752, 57), (47.863, 61), (50.474, 62), (53.833, 66), (56.742, 69), (61.708, 72), (62.833, 75),
    (65.713, 78), (68.926, 81), (71.975, 82), (74.997, 86), (78.06, 90), (81.109, 92)), ((84.217, None),
    (87.649, None), (89.543, None), (90.236, None)))
O2_PLANS = (((131.357, None), (134.449, None), (137.05, None), (137.656, None), (138.539, None), (140.057,
    None), (144.16, None)), ((141.38, None), (145.789, None), (145.843, None), (146.882, None), (149.928,
    None), (152.324, None), (153.261, None)), ((12.503, None), (22.336, None), (31.211, None), (39.891, None),
    (47.762, None), (57.333, None), (66.0, None)), ((27.948, None), (36.312, None), (43.877, None), (51.105,
    None), (58.218, None), (67.954, None), (76.139, None)))
PACK_PLANS = (((100.502, None), (101.244, None), (102.208, None), (102.296, None), (103.427, None), (104.874,
    None), (105.862, None), (106.631, None), (107.838, None), (108.106, None), (109.264, None), (109.501,
    None), (110.296, None), (111.052, None), (111.166, None), (111.529, None), (114.039, None), (114.221,
    None), (115.251, None), (116.905, None), (117.775, None), (118.037, None), (118.466, None), (118.897,
    None), (121.059, None), (121.33, None), (121.354, None), (122.756, None), (123.403, None), (124.242,
    None), (124.673, None), (125.882, None)), ((128.281, None), (128.956, None), (131.04, None), (131.514,
    None), (131.968, None), (132.242, None), (132.835, None), (133.941, None), (135.423, None), (136.25,
    None), (136.936, None), (137.657, None), (138.836, None), (139.06, None), (140.343, None), (141.492,
    None), (142.08, None), (142.473, None), (143.694, None), (143.8, None), (144.137, None), (146.083, None),
    (146.911, None), (147.792, None), (148.441, None), (149.019, None), (149.771, None), (150.598, None),
    (151.737, None), (152.598, None), (153.829, None), (154.519, None)))
PACKD_PLANS = (((1.12, None), (1.495, None), (4.36, None), (5.329, None), (7.571, None), (9.451, None),
    (9.782, None), (11.222, None), (12.795, None), (14.02, None), (14.575, None), (15.831, None), (19.475,
    None), (20.868, None), (21.935, None), (22.323, None), (25.31, None), (26.102, None), (28.561, None),
    (30.197, None), (31.978, None), (33.481, None)), ((35.02, None), (36.791, None), (38.947, None), (39.775,
    None), (42.179, None), (42.661, None), (46.568, None), (46.704, None), (49.436, None), (51.509, None),
    (51.641, None), (52.889, None), (53.189, None), (55.672, None), (56.222, None), (58.458, None), (59.773,
    None), (60, None)))
PACK_DUE = (130, 5, 39, 64)
DQA = 16 * len(PACKD_PLANS[0])
G_LAG = 5
D_LAG = 1
PLAIN_V0 = 1
OC_PIN = 1
LN2_GAPS = (1.13, 1.5, 0.2)
LN2_SPLIT = 4
PACK_W = 512
GAP_PACK = 0.2
LN1_GAPS = (1, 1.25)
GAP_PRO = 0.13
GAP_X = 0.2
GAP_WO = 0.2
GAP_O2 = 0.26
OUT_ORDER = 1
O_DUE = 6
MOE_NA = 36
MOE_ND = 2
MOE_LAGS = (2, 2)
STAGGER = 8

NN = (((1,), (0,)), ((), ()))
NT = (((1,), (1,)), ((), ()))


def _dot(a, b, dims):
    return lax.dot_general(a, b, dims, preferred_element_type=F32)


def _recip(x):
    return pl.reciprocal(x, approx=False, full_range=False)


def _pack(x):
    return pltpu.bitcast(x, U32)


def _unpack(x):
    return pltpu.bitcast(x, BF16)


def _strassen_lhs(a11, a12, a21, a22):
    return [a21 + a22, a22, a11 + a12, a11, a11 + a22, a12 - a22, a21 - a11]


def _strassen_rhs(b11, b12, b21, b22):
    return [b11, b21 - b11, b22, b12 - b22, b11 + b22, b21 + b22, b11 + b12]


def _strassen(product):
    m2 = product(0)
    m4 = product(1)
    c21 = m2 + m4
    m5 = product(2)
    u11 = m4 - m5
    m3 = product(3)
    c12 = m3 + m5
    u22 = m3 - m2
    m1 = product(4)
    u11 = u11 + m1
    u22 = u22 + m1
    c11 = product(5) + u11
    c22 = product(6) + u22
    return [[c11, c12], [c21, c22]]


def _strassen_rows_first(product, emit):
    m5 = product(2)
    m3 = product(3)
    emit(0, 1, m3 + m5)
    m4 = product(1)
    u11 = m4 - m5
    m1 = product(4)
    u11 = u11 + m1
    u22 = m3 + m1
    emit(0, 0, product(5) + u11)
    m2 = product(0)
    emit(1, 0, m2 + m4)
    u22 = u22 - m2
    emit(1, 1, product(6) + u22)


def _ordered(bits):
    return bits ^ ((bits >> 31) & 0x7FFF0000)


def _block(rows):
    return jnp.concatenate([jnp.concatenate(r, axis=1) for r in rows], axis=0)


def _pair_allreduce(a, op):
    a = op(a, pltpu.roll(a, 2, 0))
    return op(a, pltpu.roll(a, 4, 0))


def _tree(op, xs):
    xs = list(xs)
    while len(xs) > 1:
        nxt = [op(xs[i], xs[i + 1]) for i in range(0, len(xs) - 1, 2)]
        if len(xs) % 2:
            nxt.append(xs[-1])
        xs = nxt
    return xs[0]


def _pair_logits(sl, j):
    sub = lax.broadcasted_iota(jnp.int32, sl[0].shape, 0)
    if j < 3:
        head = jnp.where(sub < 2, 0.0, sl[(0, 1, 16)[j]])
    else:
        head = jnp.where(sub < 2, sl[0], jnp.where(sub < 4, pltpu.roll(sl[1], 2, 0),
                                                   jnp.where(sub < 6, pltpu.roll(sl[16], 4, 0), 0.0)))
    r0 = (2, 9, 17, 24)[j]
    return [head] + list(sl[r0:r0 + 7])


def _dual_exp(sl):
    mx = _pair_allreduce(_tree(jnp.maximum, sl), jnp.maximum)
    mn = _pair_allreduce(_tree(jnp.minimum, sl), jnp.minimum)
    ep = [jnp.exp2(s - mx) for s in sl]
    en = [jnp.exp2(mn - s) for s in sl]
    sp = _pair_allreduce(_tree(jnp.add, ep), jnp.add)
    sn = _pair_allreduce(_tree(jnp.add, en), jnp.add)
    return ep, en, sp, sn


def _after(x, never, anchor):
    if anchor is None:
        return x
    d = jnp.concatenate([anchor] * (x.shape[0] // 8), axis=0)
    if x.shape[1] == 128:
        return jnp.where(never, d, x)
    return jnp.concatenate([jnp.where(never, d, x[:, :128]), x[:, 128:]], axis=1)


def _gate(x, never, deps):
    for i, dep in enumerate(deps):
        d = jnp.broadcast_to(dep, (8, 128))
        if x.dtype != F32:
            d = pltpu.bitcast(d, x.dtype)
        blk = jnp.where(never, d, x[8 * i:8 * i + 8, :128])
        if x.shape[1] > 128:
            blk = jnp.concatenate([blk, x[8 * i:8 * i + 8, 128:]], axis=1)
        parts = ([x[:8 * i, :]] if i else []) + [blk, x[8 * i + 8:, :]]
        x = jnp.concatenate(parts, axis=0)
    return x


def _lane_fold(a):
    return _tree(jnp.add, [a[:, 128 * i:128 * i + 128] for i in range(a.shape[1] // 128)])


def _row_sum(a):
    return jnp.sum(_lane_fold(a), axis=-1, keepdims=True)


def _lane_tile(a, n):
    return a if n == 1 else jnp.concatenate([a] * n, axis=1)


def _sublane_allreduce(a):
    a = a + pltpu.roll(a, 4, 0)
    a = a + pltpu.roll(a, 2, 0)
    return a + pltpu.roll(a, 1, 0)


def _col_broadcast(row8):
    return jnp.concatenate([row8] * 16, axis=0).astype(BF16).T.astype(F32)


def _vpu_matvec(xb, w_rows, never, anchors, lag):
    ng = xb.shape[0] // 8
    acc, hist = None, []
    for g in range(ng):
        dep = anchors[(g * len(anchors)) // ng]
        if g >= lag:
            dep = dep + hist[g - lag]
        x = jnp.where(never, dep, xb[8 * g:8 * g + 8, :])
        w = w_rows(g)
        t = w * _lane_tile(x, w.shape[1] // 128)
        acc = t if acc is None else acc + t
        c = 128 * (g % (w.shape[1] // 128))
        hist.append(acc[:, c:c + 128])
    return acc


class _Side:
    def __init__(self, never, later=lambda rel, gap: rel + gap):
        self.never = never
        self.later = later
        self.jobs = []
        self.deps = {}
        self.hooks = {}

    def add(self, plan, fn):
        for k, (rel, due) in enumerate(plan):
            if rel is None:
                self._run(None, due, fn, k, None)
            else:
                self.jobs.append((rel, due, fn, k))

    def _run(self, rel, due, fn, k, anchor):
        gen = fn if hasattr(fn, "send") else fn(k, anchor)
        dep = gen
        if hasattr(gen, "send"):
            try:
                while True:
                    gap = gen.send(anchor) if gen is fn or rel is None and dep is None else next(gen)
                    if rel is not None:
                        self.jobs.append((self.later(rel, gap), due, gen, k))
                        return
                    dep = None
            except StopIteration as stop:
                dep = stop.value
        if due is not None:
            self.deps.setdefault(due, []).append(dep)

    def check(self):
        assert not self.jobs and not self.deps and not self.hooks

    def gate(self, step, x):
        return _gate(x, self.never, self.deps.pop(step, []))

    def done(self, step, res):
        m = res.shape[0] // 8
        while True:
            ready = [j for j in self.jobs if step - 1 < j[0] <= step]
            if not ready:
                break
            job = min(ready, key=lambda j: j[0])
            self.jobs.remove(job)
            g = m - 1 - int((step - job[0]) * m)
            self._run(*job, res[8 * g:8 * g + 8, res.shape[1] - 128:])
        for fn in self.hooks.pop(step, []):
            fn()


def _kernel(x_hbm, wqkv_hbm, wphi_hbm, wo_hbm, wr_hbm, wg_hbm, wu_hbm, wd_hbm, out_hbm,
            x_v, xn_v, xs_v, lead_v, wraw_v, wt_v, ws_v, wphi_v, a_v, woraw_v, wos_v, wrraw_v, wr_v,
            kvacc_v, kvbf_v, z_v, zb_v, phi_v, oc_v, oc2_v, h_v, hn_v, o_v, wg_v, wu_v, wd_v, stage_v,
            wgp_v, wup_v, wdp_v, patch_v,
            sem):
    SX, SQ, SO, SM = 0, 6, 6 + 3 * NC, 6 + 3 * NC + NT_ + 1

    def x_copy(i):
        h0, h1 = ((0, 1), (1, 2), (2, 4), (4, 8), (8, 2 * NT_))[i]
        rows = pl.ds(h0 * TH, (h1 - h0) * TH)
        return pltpu.make_async_copy(x_hbm.at[rows, :], x_v.at[rows, :], sem.at[SX + i])

    def k0_copy(s):
        return pltpu.make_async_copy(wqkv_hbm.at[:, pl.ds(D + s * 128, 128)],
                                     wraw_v.at[NC, :, pl.ds(s * 128, 128)], sem.at[(SM + 7, SQ + NC)[s]])

    def w_copy(j, c):
        return pltpu.make_async_copy(wqkv_hbm.at[:, pl.ds(j * D + c * RC, RC)], wraw_v.at[j * NC + c],
                                     sem.at[SQ + j * NC + c])

    def wphi_copy(i):
        h0, h1 = ((0, 8), (16, 24), (8, 16), (24, H))[i]
        return pltpu.make_async_copy(wphi_hbm.at[pl.ds(h0, h1 - h0)], wphi_v.at[pl.ds(h0, h1 - h0)],
                                     sem.at[(SM + 4, SM + 8, SM + 9, SM + 14)[i]])

    wr_copy = pltpu.make_async_copy(wr_hbm, wrraw_v, sem.at[SM + 5])

    def wo_copy(i):
        rows = pl.ds(0, WO_ROWS) if i == 0 else pl.ds(WO_ROWS, QK - WO_ROWS)
        return pltpu.make_async_copy(wo_hbm.at[:, rows, :], woraw_v.at[:, rows, :], sem.at[(SM + 6, SX + 5)[i]])

    wg_copy = pltpu.make_async_copy(wg_hbm.at[:, pl.ds(FM, FV)], wg_v, sem.at[SM + 0])
    wu_copy = pltpu.make_async_copy(wu_hbm.at[:, pl.ds(FM, FV)], wu_v, sem.at[SM + 1])
    wd_copy = pltpu.make_async_copy(wd_hbm.at[pl.ds(0, FVD), :], wd_v, sem.at[SM + 2])

    def stage_copy(i, q):
        if i < 2:
            r0 = q * (D // NQ)
            r0 = r0 if isinstance(r0, int) else pl.multiple_of(r0, D // NQ)
            src = (wg_hbm, wu_hbm)[i].at[pl.ds(r0, D // NQ), pl.ds(0, FM)]
        else:
            r0 = FVD + q * DQ + (i - 2) * DQA
            r0 = r0 if isinstance(r0, int) else pl.multiple_of(r0, 16)
            src = wd_hbm.at[pl.ds(r0, (DQA, DQ - DQA)[i - 2]), :]
        return pltpu.make_async_copy(src, stage_v[i].at[pl.ds(0, src.shape[0]), :], sem.at[SM + 10 + i])

    wphi_copy(0).start()
    k0_copy(0).start()
    x_copy(0).start()
    k0_copy(1).start()
    x_copy(1).start()
    wphi_copy(1).start()
    w_copy(1, 2).start()

    made = set()

    def view(ref, i, n, off=0):
        r0 = off + i * n
        return ref.at[pl.ds(r0 if isinstance(r0, int) else pl.multiple_of(r0, math.gcd(n, off)), n), :]

    def put_blocks(dst, r0, fn, m11, m12, m21, m22, never, a, skip=(), base=0, pitch=HK, gap=None):
        for c0 in range(0, m11.shape[1], 128):
            if c0:
                a = yield gap or GAP_PRO
            d11, d22 = m11[:, c0:c0 + 128], m22[:, c0:c0 + 128]
            if a is not None:
                d = jnp.concatenate([a, a], axis=0)
                d11, d22 = jnp.where(never, d, d11), jnp.where(never, d, d22)
            blocks = fn(d11, m12[:, c0:c0 + 128], m21[:, c0:c0 + 128], d22)
            for i, b in enumerate(blocks):
                if i not in skip:
                    dst[r0:r0 + 8, base + i * pitch + c0:base + i * pitch + c0 + 128] = _pack(b.astype(BF16))

    def rows16(ref, r0, c0=0, w=D):
        return _unpack(ref[r0:r0 + 8, c0:c0 + w]).astype(F32)

    def x_blocks(t, k, lo, hi, never, a, gap=None):
        return put_blocks(view(xs_v, t, TH // 2), k * LNC // 2, _strassen_rhs,
                          lo[:, :HK], hi[:, :HK], lo[:, HK:], hi[:, HK:], never, a, gap=gap)

    def ln_rows(t, k, n, never=None, anchor=None, plain=False):
        wide = lambda c, a: _lane_tile(_after(jnp.broadcast_to(c, (n, 128)), never, a), D // 128)
        x = _after(view(x_v, t, T)[k * n:(k + 1) * n, :].astype(F32), never, anchor)
        s1 = _row_sum(x)
        anchor = yield LN1_GAPS[0]
        xc = x - wide(s1 * (1.0 / D), anchor)
        rstd = lax.rsqrt(_row_sum(xc * xc) * (1.0 / D) + LN_EPS)
        anchor = yield LN1_GAPS[1]
        xn = xc * wide(rstd, anchor)
        if plain:
            xn_v[(t * T + k * n) // 2:(t * T + (k + 1) * n) // 2, :] = _pack(xn.astype(BF16))
        elif k * n < TH:
            xn_v[k * n // 2:(k + 1) * n // 2, :] = _pack(xn.astype(BF16))
        else:
            yield from x_blocks(t, k - TH // LNC, rows16(xn_v, (k * n - TH) // 2), xn, never, anchor, GAP_X)
        return _tree(jnp.add, [rstd[8 * i:8 * i + 8, :] for i in range(min(n, LNC) // 8)])

    def now(gen):
        try:
            while True:
                next(gen)
        except StopIteration as stop:
            return stop.value

    def late_x_blocks(t):
        return lambda k, a: x_blocks(t, k, rows16(xn_v, t * T // 2 + 8 * k),
                                     rows16(xn_v, (t * T + TH) // 2 + 8 * k), never0, a)

    def xn_tile(t):
        return _unpack(xn_v[t * T // 2:(t + 1) * T // 2, :])

    def xs_tile(t):
        return _unpack(view(xs_v, t, TH // 2)[:, 0:7 * HK])

    def expand_wphi(c):
        w = wphi_v[8 * c:8 * c + 8].reshape(8 * DH, DH).astype(F32).T
        bits = pltpu.bitcast(w, U32)
        head = lax.broadcasted_iota(jnp.int32, (DH, 128), 1) >> 5
        for s in range(2):
            b = bits[:, 128 * s:128 * s + 128]
            for j in range(2):
                r0 = 64 * (2 * c + s) + 32 * j
                a_v[r0:r0 + 32, :] = jnp.where(head == 2 * j, b >> 16,
                                               jnp.where(head == 2 * j + 1, b, jnp.uint32(0)))

    wphi_copy(0).wait()
    expand_wphi(0)
    h_v[1][...] = jnp.zeros((T, D), F32)
    if OC_PIN:
        for ref in oc_v + oc2_v:
            ref[0:8, 0:128] = jnp.zeros((8, 128), U32)
    for ref in stage_v:
        ref[ref.shape[0] - 16:, 0:128] = jnp.zeros((16, 128), BF16)

    def v_transpose(k, a):
        q, r0 = (k // 8) + 4 * (k % 2), 256 * (k % 8 // 2)
        w = wraw_v[2 * NC + q // 2, r0:r0 + 256, (q % 2) * 128:(q % 2) * 128 + 128]
        if a is not None:
            w = _unpack(jnp.where(never0, jnp.concatenate([pltpu.bitcast(a, U32)] * 16, axis=0), _pack(w)))
        wt_v[2][64 * q:64 * q + 64, r0:r0 + 256] = _pack(w.T)
        made.add(("vt", k))

    def fold_pairs(j, c, s, side=None, step0=None):
        g0 = 64 * (2 * c + s)
        g0 = g0 if isinstance(g0, int) else pl.multiple_of(g0, 64)
        res = _dot(_unpack(a_v[pl.ds(g0, 64), :]), wraw_v[j * NC + c, :, s * 128:(s + 1) * 128], NT)
        if side is not None:
            side.done(step0 + 2 * s, res[:, :D // 2])
            side.done(step0 + 2 * s + 1, res[:, D // 2:])
        sub = lax.broadcasted_iota(jnp.int32, (8, D), 0)
        out = []
        for q in range(2):
            base = _pair_allreduce(jnp.where(sub < 2, res[64 * q:64 * q + 8, :], 0.0), jnp.add)
            out.append([(res[64 * q + 8 * i:64 * q + 8 * i + 8, :] - base) * LOG2E for i in range(8)])
        return out

    def share(z, z3, k):
        sub = lax.broadcasted_iota(jnp.int32, (8, D), 0)
        return jnp.where(sub < 2, pltpu.roll(z3, 8 - 2 * k, 0), z)

    def packed(slabs):
        return _pack(jnp.concatenate(slabs, axis=0).astype(BF16))

    def fold(j, c, side=None, step0=None):
        p0, p1 = fold_pairs(j, c, 0, side, step0)
        p2, p3 = fold_pairs(j, c, 1, side, step0)
        sl = ([share(p0[0], p3[0], 1), share(p1[0], p3[0], 2)] + p0[1:] + p1[1:]
              + [share(p2[0], p3[0], 3)] + p2[1:] + p3[1:])
        zero = jnp.zeros((8, D), F32)
        even, odd = sl + [zero], [zero] + sl
        r0 = 8 * ((31 * c) // 2)
        is_odd = c % 2 == 1
        if isinstance(c, int):
            sl = odd if is_odd else even
        else:
            r0 = pl.multiple_of(r0, 8)
            sl = [jnp.where(is_odd, o, e) for o, e in zip(odd, even)]
        win = wt_v[j].at[pl.ds(r0, 128), :]
        win[8:128, :] = packed(sl[2:])
        first = packed(sl[:2])
        if is_odd is not False:
            keep = lax.broadcasted_iota(jnp.int32, (8, D), 0) < jnp.where(is_odd, 4, 0)
            first = jnp.where(keep, win[0:8, :], first)
        win[0:8, :] = first
        made.update(("fold", j, q) for q in ([c] if isinstance(c, int) else range(3)))

    def w_blocks(j, k0=0):
        def job(k, a):
            k += k0
            assert made >= ({("vt", 8 * (k // 8) + q) for q in range(8)} if j == 2 else
                            {("fold", j, q) for q in ((0, 2) if k < 15 else range(4))})
            lo, hi = rows16(wt_v[j], 8 * k), rows16(wt_v[j], (256 if j == 2 else 248) + 8 * k)
            yield from put_blocks(ws_v[j], 8 * k, _strassen_lhs, lo[:, :HK], lo[:, HK:], hi[:, :HK], hi[:, HK:],
                                  never0, a, skip=(1, 3))
            made.add(("ws", j, k))
        return job

    def k_pair(p, slot, pr, c0, first, never=None):
        for n in range(c0, c0 + p[0].shape[1], 128):
            assert first == (("z", pr, n) not in made)
            made.update({("z", pr, n), ("phi", slot, pr, n)})
        ep, en, sp, sn = _dual_exp(p)
        inv = _recip(sp * sn)
        scale = (sn * inv, sp * inv)
        es = ep + en
        cols = slice(c0, c0 + p[0].shape[1])
        n = 16 if never is None else 16 // STAGGER
        last = None
        for q in range(16 // n):
            sc = scale
            if last is not None:
                sc = [jnp.where(never, last, x) for x in scale]
            phi = jnp.concatenate([es[i] * sc[i // 8] for i in range(q * n, (q + 1) * n)], axis=0)
            rows = slice(8 * q * n, 8 * (q + 1) * n)
            z = phi if first else z_v[pr, rows, cols] + phi
            z_v[pr, rows, cols] = z
            phi_v[slot][64 * pr + 4 * q * n:64 * pr + 4 * (q + 1) * n, cols] = _pack(phi.astype(BF16))
            last = z[8 * n - 8:, :]

    def k_features(pk, slot, c, first, never=None):
        for j in range(PPC):
            k_pair(_pair_logits(pk, j), slot, c * PPC + j, 0, first, never)

    def kv_update(vts, slot, g, first, publish=False):
        for q, vt in enumerate(vts):
            for j in range(2):
                pr = 2 * g + 8 * q + j
                assert made >= {("phi", slot, pr, 0), ("phi", slot, pr, 128)}
                upd = _dot(vt[64 * j:64 * j + 64, :].astype(BF16), _unpack(phi_v[slot][64 * pr:64 * pr + 64, :]), NT)
                acc = upd if first else kvacc_v[pr] + upd
                kvacc_v[pr] = acc
                if publish:
                    odd = -(lax.broadcasted_iota(jnp.int32, (32, 128), 1) & 1)
                    bits = pltpu.bitcast(acc, jnp.int32) & jnp.concatenate([~odd, odd], axis=0)
                    kvbf_v[32 * pr:32 * pr + 32, :] = _pack(pltpu.bitcast(bits, F32).astype(BF16))

    def save_lead(t):
        view(lead_v, t, HK // 2)[...] = _pack(_unpack(view(xs_v, t, TH // 2)[:, 0:HK]).T)

    def proj_feat(side, step0, c, xn, carry):
        r0 = 8 * ((31 * c) // 2)
        skip = 8 if c % 2 == 1 and carry is not None else 0
        w = wt_v[1][r0 + skip:r0 + 128, :]
        quarters = []
        for n in range(2):
            for m in range(2):
                step = step0 + 2 * n + m
                wq = _unpack(side.gate(step, w[:64, :] if m == 0 else w[64:, :]))
                res = _dot(wq, xn[n * TH:(n + 1) * TH, :], NT)
                side.done(step, res)
                quarters.append(res)
        res = jnp.concatenate(
            [jnp.concatenate([quarters[0], quarters[2]], axis=1),
             jnp.concatenate([quarters[1], quarters[3]], axis=1)], axis=0)
        sl = [res[8 * i:8 * i + 8, :] for i in range(res.shape[0] // 8)]
        if c % 2 == 0:
            return sl[:31], sl[31]
        return ([carry] + sl if skip else sl[1:]), None

    def proj_unit(side, step0, j, b, xs, lead=None, plain=None):
        r1 = 64 * b + (64 if j == 2 or b < 3 else 56)
        assert made >= ({("vt", 8 * b + q) for q in range(8)} if plain is not None else
                        {("ws", j, k) for k in range(8 * b, r1 // 8)})
        if plain is not None:
            out = []
            for q in range(2):
                row = []
                for n in range(2):
                    res = _dot(_unpack(wt_v[2][256 * q + 64 * b:256 * q + r1, :]), plain[n * TH:(n + 1) * TH, :], NT)
                    for i in range((0, 2, 4, 5)[2 * q + n], (2, 4, 5, 7)[2 * q + n]):
                        side.done(step0 + i, res)
                    row.append(res)
                out.append(jnp.concatenate(row, axis=1))
            return out

        def product(i):
            off = 256 if j == 2 else 248
            w = (wt_v[j][off + 64 * b:off + r1, HK:] if i == 1 else wt_v[j][64 * b:r1, :HK] if i == 3
                 else ws_v[j][64 * b:r1, i * HK:(i + 1) * HK])
            w = _unpack(side.gate(step0 + i, w))
            if lead is not None and i == 0:
                res = _dot(w, _unpack(view(lead_v, lead, HK // 2)[...]), NN)
            else:
                res = _dot(w, xs[:, i * HK:(i + 1) * HK], NT)
            side.done(step0 + i, res)
            return res
        return [jnp.concatenate(row, axis=1) for row in _strassen(product)]

    def feat_stage(side, step0, j, xs, pair_fn, lead=None):
        sl = [[], []]
        for b in range(4):
            for q, res in enumerate(proj_unit(side, step0 + 7 * b, j, b, xs, lead if b == 0 else None)):
                sl[q] += [res[8 * i:8 * i + 8, :] for i in range(res.shape[0] // 8)]
            for q in (1, 0):
                for jj in (2 * (b % 2), 2 * (b % 2) + 1):
                    pair_fn(_pair_logits(sl[q][31 * (b // 2):], jj), 8 * q + 4 * (b // 2) + jj)

    def v_stage(side, xs, slot, first, publish, lead, plain=None):
        pending = None
        for g in range(4):
            if pending is not None:
                side.hooks.setdefault(7 * g + D_LAG, []).append(lambda p=pending: kv_update(*p))
            pending = (proj_unit(side, 7 * g, 2, g, xs, lead if g == 0 else None, plain if g < PLAIN_V0 else None),
                       slot, g, first, publish)
        side.check()
        return pending

    def pack_rows(src, dst, r0, c0, cols, never, a):
        for c in range(c0, c0 + cols, PACK_W):
            if c > c0:
                a = yield GAP_PACK
            w = min(PACK_W, c0 + cols - c)
            v = src[r0:r0 + 16, c:c + w].astype(F32)
            v = jnp.concatenate([jnp.where(never, _lane_tile(a, w // 128), v[0:8, :]), v[8:16, :]], axis=0)
            dst[r0 // 2:r0 // 2 + 8, c:c + w] = _pack(v.astype(BF16))

    def stash_at(i, k, n):
        return zb_v.at[4 * i + 2 * (k // 16) + n, pl.ds(8 * (k % 16), 8), :]

    def stash(i, sl):
        for k, v in enumerate(sl):
            for n in range(2):
                stash_at(i, k, n)[...] = v[:, 128 * n:128 * n + 128]

    def stashed_k(i, slot, c, first):
        def job(k, a):
            j, n = k // 2, k % 2
            p = _pair_logits([stash_at(i, q, n)[...] for q in range(31)], j)
            k_pair([_after(p[0], never0, a)] + p[1:], slot, c * PPC + j, 128 * n, first, never0)
        return job

    def first_rows(k0, k1, n):
        xn = _unpack(xn_v[n * TH // 2:(n + 1) * TH // 2, :])
        ks = [k for k in range(k0, k1)]
        w = jnp.concatenate([wt_v[1][4 * (k % 32):4 * (k % 32) + 8, :] for k in ks[::2]], axis=0)
        res = _dot(_unpack(w), xn, NT)
        for q, k in enumerate(ks):
            if k % 32 < 31:
                stash_at(0, k % 32, n)[...] = res[8 * q:8 * q + 8, :]

    k0_copy(0).wait()
    x_copy(0).wait()
    wphi_copy(2).start()
    w_copy(1, 1).start()
    wphi_copy(3).start()
    x_copy(2).start()
    p0, p1 = fold_pairs(1, 0, 0)
    wt_v[1][8:64, :] = packed(p0[1:] + p1[1:])
    h_v[0][0:8, :] = p0[0]
    h_v[0][8:16, :] = p1[0]
    never0 = now(ln_rows(0, 0, TH, plain=True))[0, 0] < 0.0
    first_rows(2, 16, 0)

    k0_copy(1).wait()
    x_copy(1).wait()
    wphi_copy(1).wait()
    w_copy(1, 3).start()
    for c in (0, 2, 1, 3):
        w_copy(2, c).start()
    p2, p3 = fold_pairs(1, 0, 1)
    wt_v[1][0:8, :] = packed([share(h_v[0][0:8, :], p3[0], 1), share(h_v[0][8:16, :], p3[0], 2)])
    wt_v[1][64:128, :] = packed([share(p2[0], p3[0], 3)] + p2[1:] + p3[1:] + [jnp.zeros((8, D), F32)])
    made.add(("fold", 1, 0))
    now(ln_rows(0, 1, TH, plain=True))
    first_rows(16, 34, 0)
    first_rows(0, 16, 1)
    first_rows(16, 32, 1)
    expand_wphi(2)

    for c, prev in ((2, 0), (1, 2)):
        w_copy(1, c).wait()
        wphi_copy(4 - c).wait()
        expand_wphi(5 - 2 * c)
        side = _Side(never0, lambda rel, gap: min(rel + gap, 7))
        if c == 2:
            side.add(PRO_X0_PLAN, late_x_blocks(0))
        else:
            side.add(PRO_W0_PLAN, w_blocks(1))
        side.add((PRO_K_PLANS0, PRO_K_PLANS1)[2 - c], stashed_k(prev, 0, prev, True))
        fold(1, c, side, 0)
        stash(c, proj_feat(side, 4, c, xn_tile(0), None)[0])
        side.check()

    x_copy(2).wait()
    w_copy(1, 3).wait()
    x_copy(3).start()
    w_copy(0, 0).start()
    wo_copy(0).start()
    x_copy(4).start()
    for c in range(1, NC):
        w_copy(0, c).start()
    wo_copy(1).start()
    wr_copy.start()
    for i in range(4):
        stage_copy(i, 0).start()
    wg_copy.start()
    wu_copy.start()
    wd_copy.start()
    side = _Side(never0, lambda rel, gap: min(rel + gap, 19))
    side.add(PRO_LN1_PLAN, lambda k, a: ln_rows(1, k, LNC, never0, a, plain=True))
    side.add(PRO_W_PLAN, w_blocks(1, len(PRO_W0_PLAN)))
    side.add(PRO_K_PLANS2, stashed_k(1, 0, 1, False))
    fold(1, 3, side, 0)
    stash(3, proj_feat(side, 4, 3, xn_tile(0), None)[0])
    xn1 = xn_tile(1)
    spare = None
    for c in range(3):
        pk, spare = proj_feat(side, 8 + 4 * c, c, xn1, spare)
        if c < 2:
            k_features(pk, 1, c, c == 1, never0)
        else:
            stash(0, pk + [spare])
    side.check()

    for c in range(NC):
        w_copy(2, c).wait()
    side = _Side(never0, lambda rel, gap: min(rel + gap, 27))
    side.add(PRO_V_PLANS[0], v_transpose)
    side.add(PRO_V_PLANS[1], stashed_k(3, 0, 3, False))
    side.add(PRO_V_PLANS[2], stashed_k(0, 1, 2, False))
    side.add(PRO_V_PLANS[3], late_x_blocks(1))
    side.add(PRO_V_PLANS[4], w_blocks(2))
    spare = jnp.concatenate([stash_at(0, 31, n)[...] for n in range(2)], axis=1)
    k_features(proj_feat(side, -4, 3, xn_tile(1), spare)[0], 1, 3, True, never0)
    kv_update(*v_stage(side, xs_tile(0), 0, True, False, None, xn_tile(0)))
    save_lead(0)
    save_lead(1)
    for r0 in (0, 248):
        wt_v[0][r0:r0 + 8, :] = jnp.zeros((8, D), U32)

    def phase1(u, carry):
        never = u < 0

        @pl.when(u == 0)
        def _():
            x_copy(3).wait()
            w_copy(0, 0).wait()
            wo_copy(0).wait()

        @pl.when(u == 1)
        def _():
            x_copy(4).wait()
            w_copy(0, 1).wait()
            w_copy(0, 2).wait()
            wo_copy(1).wait()

        def wo_blocks(k0):
            def job(k, a):
                k += k0
                r, c, part = k // 4, 128 * (k // 2 % 2), k % 2
                r0 = u * ((QK - WO_ROWS) // 2)
                dst = wos_v.at[pl.ds(pl.multiple_of(r0 // 2, 8), WO_ROWS // 2), :]

                def piece(kq, nq):
                    src = woraw_v.at[kq, pl.ds(pl.multiple_of(r0, 16), WO_ROWS), :]
                    return src[16 * r:16 * r + 16, nq * QK + c:nq * QK + c + 128].astype(F32)
                outer = [_strassen_rhs(piece(ki, ni), piece(ki, 2 + ni), piece(2 + ki, ni), piece(2 + ki, 2 + ni))
                         for ki in range(2) for ni in range(2)]
                for i in range(4) if part == 0 else range(4, 7):
                    if i % 4:
                        a = yield GAP_WO
                    yield from put_blocks(dst, 8 * r, _strassen_rhs, *[o[i] for o in outer], never, a,
                                          base=7 * i * QK + c, pitch=QK)
            return job

        xs = xs_tile(2 * u + 1)
        side = _Side(never, lambda rel, gap: min(rel + gap, 27))
        for i in range(2):
            t = 2 * u + 2 + i
            if i == 0:
                side.add(LN1_PLANS[0], lambda k, a: ln_rows(2 * u + 2, k, LNC, never, a))
                side.add(WO_PLANS[0], wo_blocks(0))
            pending = v_stage(side, xs, 1 - i, False, False, t - 1 if i == 0 else None)
            xs = xs_tile(t)
            side = _Side(never, lambda rel, gap, end=(27, -1)[i]: min(rel + gap, end))
            if i == 0:
                side.add(LN1_PLANS[1], lambda k, a: ln_rows(2 * u + 3, k, LNC, never, a))
                side.add(WO_PLANS[1], wo_blocks(len(WO_PLANS[0])))
            else:
                side.add(WO_PLANS[2], wo_blocks(24 - len(WO_PLANS[2])))
            side.hooks[-28 + D_LAG] = [lambda p=pending: kv_update(*p)]
            feat_stage(side, -28, 1, xs, lambda p, pr: k_pair(p, i, pr, 0, False, never if i == 1 else None))
            save_lead(t)
        side.check()
        fold(0, u)
        return carry

    lax.fori_loop(0, (NT_ - 2) // 2, phase1, 0)

    w_copy(0, 3).wait()
    wr_copy.wait()
    side = _Side(never0, lambda rel, gap: min(rel + gap, 27 if rel < 98 else 103))

    def z_final(k, a):
        zb_v[k] = jnp.broadcast_to(_row_sum(_after(z_v[k], never0, a)), (128, 128))

    side.add(END_PLANS[0], z_final)
    side.add(END_PLANS[1], w_blocks(0))
    fold(0, 3, side, 100)
    kv_update(*v_stage(side, xs_tile(NT_ - 1), 1, False, True, None))
    wr_v[...] = jnp.broadcast_to(wrraw_v[...].reshape(1, D).astype(F32), (8, D))

    def o_copy(r0, n, i):
        return pltpu.make_async_copy(o_v.at[pl.ds(r0, n), :], out_hbm.at[pl.ds(r0, n), :], sem.at[SO + i])

    def finish_rows(h_ref, k, t, valid, st, never=None, anchor=None):
        r0 = t * T + k * LNC
        rows = slice(k * LNC, (k + 1) * LNC)
        m = jnp.broadcast_to(_row_sum(_after(h_ref[rows, :], never, anchor)) * (1.0 / D), (LNC, 128))
        rstd, r = [], []
        for i in range(LNC // 8):
            anchor = yield LN2_GAPS[2] if i else LN2_GAPS[0]
            mi = _after(m[8 * i:8 * i + 8, :], never, anchor)
            hc = h_ref[k * LNC + 8 * i:k * LNC + 8 * i + 8, :] - _lane_tile(mi, D // 128)
            rs = lax.rsqrt(_row_sum(hc * hc) * (1.0 / D) + LN_EPS)
            r.append((_row_sum(hc * wr_v[...]) * rs + 0.0).astype(BF16).astype(F32))
            rstd.append(jnp.broadcast_to(rs, (8, 128)))
        rstd = jnp.concatenate(rstd, axis=0)
        w = D if never is None else D // LN2_SPLIT
        for c in range(0, D, w):
            anchor = yield LN2_GAPS[2] if c else LN2_GAPS[1]
            h = h_ref[rows, c:c + w]
            hn = (h - _lane_tile(_after(m, never, anchor), w // 128)) * _lane_tile(rstd, w // 128)
            view(hn_v, t, T // 2)[k * LNC // 2:(k + 1) * LNC // 2, c:c + w] = _pack(hn.astype(BF16))
            view(o_v, t, T)[rows, c:c + w] = (hn + h).astype(BF16)
        best = st["route"]
        sub = lax.broadcasted_iota(jnp.int32, (8, 128), 0)
        for i, ri in enumerate(r):
            key = _ordered(pltpu.bitcast(jnp.broadcast_to(ri, (8, 128)), jnp.int32)) | ((S - 1 - r0 - 8 * i) - sub)
            if valid is not None:
                key = jnp.where(valid, key, KEY_MIN)
            best = jnp.maximum(best, key)
        st["route"] = best
        return pltpu.bitcast(best, F32)

    def q_pair(p, slot, pr):
        ep, en, sp, sn = _dual_exp(p)
        zz = [_lane_tile(zb_v[pr, 8 * i:8 * i + 8, :], T // 128) for i in range(16)]
        ap = _pair_allreduce(_tree(jnp.add, [ep[i] * zz[i] for i in range(8)]), jnp.add)
        an = _pair_allreduce(_tree(jnp.add, [en[i] * zz[8 + i] for i in range(8)]), jnp.add)
        inv = _recip(ap * sn + (an + 1e-6 * sn) * sp)
        rp = sn * inv
        rn = sp * inv
        phi = jnp.concatenate([e * rp for e in ep] + [e * rn for e in en], axis=0)
        phi_v[slot][64 * pr:64 * pr + 64, :] = _pack(phi.astype(BF16))

    held = []

    def attn_blocks(slot, g, deps):
        res = [_dot(_unpack(kvbf_v[32 * pr:32 * pr + 32, :]), _unpack(phi_v[slot][64 * pr:64 * pr + 64, :]), NN)
               for pr in (2 * g, 2 * g + 8, 2 * g + 1, 2 * g + 9)]
        lo, hi = jnp.concatenate(res[0::2], axis=0), jnp.concatenate(res[1::2], axis=0)
        blocks = [(i, g, b) for i, b in enumerate(_strassen_lhs(lo[:, :TH], hi[:, :TH], lo[:, TH:], hi[:, TH:]))]
        if g % 2 == 0:
            held.append(blocks.pop())
        else:
            blocks.append(held.pop())
        ot = _pack(jnp.concatenate([b for _, _, b in blocks], axis=1).astype(BF16).T)
        for q, (i, n, _) in enumerate(blocks):
            oc_v[slot][:, i * HK + 128 * n:i * HK + 128 * n + 128] = ot[q * TH // 2:(q + 1) * TH // 2, :]
            made.add(("oc", slot, i, n))
            if q % 2:
                deps.append(pltpu.bitcast(ot[(q + 1) * TH // 2 - 8:(q + 1) * TH // 2, :], F32))

    def o_blocks(slot, c, never):
        def job(k, a):
            k = (2, 3, 1, 4, 5, 0, 6)[k]
            assert made >= {("oc", slot, k, c), ("oc", slot, k, c + 2)}
            for r in range(4):
                if r:
                    a = yield GAP_O2
                m = [rows16(oc_v[slot], 8 * r + 32 * q, k * HK + n * QK + 128 * c, 128)
                     for q in range(2) for n in range(2)]
                yield from put_blocks(oc2_v[slot], 8 * r, _strassen_lhs, *m, never, a, skip=(1, 3),
                                      base=7 * k * QK + 128 * c, pitch=QK)
            made.add(("oc2", slot, k, c))
        return job

    def out_proj(side, step0, t, slot):
        count = [0]

        def inner(i, c):
            assert made >= {("oc2", slot, i, 0), ("oc2", slot, i, 1)}

            def product(j):
                step, odd = step0 + count[0] // 2, count[0] % 2
                count[0] += 1
                o = (oc_v[slot][32:64, i * HK + QK:(i + 1) * HK] if j == 1 else
                     oc_v[slot][0:32, i * HK:i * HK + QK] if j == 3 else
                     oc2_v[slot][:, (7 * i + j) * QK:(7 * i + j + 1) * QK])
                w = wos_v[:, (7 * i + j) * QK + 128 * c:(7 * i + j) * QK + 128 * c + 128]
                res = _dot(_unpack(o), _unpack(w if odd else side.gate(step, w)), NN)
                if odd:
                    side.done(step, res)
                return res
            return _block(_strassen(product))

        xt = view(x_v, t, T)

        def emit(cs, q, r, res):
            for k, c in enumerate(cs):
                for n in range(2):
                    rows, c0 = slice(q * TH, (q + 1) * TH), r * HK + n * QK + 128 * c
                    h_v[slot][rows, c0:c0 + 128] = (res[:, 256 * k + 128 * n:256 * k + 128 * n + 128]
                                                    + xt[rows, c0:c0 + 128].astype(F32))
                made.add(("h", slot, q, r, c))

        for cs in ((0,), (1,)) if OUT_ORDER == 0 else ((0, 1),):
            _strassen_rows_first(lambda i: jnp.concatenate([inner(i, c) for c in cs], axis=1),
                                 lambda q, r, res: emit(cs, q, r, res))

    def phase2(u, carry):
        for i in range(4):
            stage_copy(i, u).wait()
        never = u < 0
        side = _Side(never, lambda rel, gap: min(rel + 2 * gap, 97) if rel < 98 else
                     rel + gap if rel + gap <= 155 else 2 * (rel + gap - 155) - 1)
        st = {"route": carry}
        tp = jnp.maximum(2 * u - 1, 0)
        early = len(LN2_PLANS[2])
        order = []

        def ln2(slot, t, valid, k0, key):
            def job(k, a):
                k += k0
                hs = {("h", slot, k // 8, r, c) for r in range(2) for c in range(2)}
                assert made >= hs or key == 0
                best = yield from finish_rows(h_v[slot], k, t, valid, st, never, a)
                assert key > 0 or not made & hs
                order.append((key, k))
                assert order == sorted(order)
                return best
            return job

        side.add(LN2_PLANS[0], ln2(1, tp, u > 0, early, 0))
        side.add(LN2_PLANS[1], ln2(0, 2 * u, None, 0, 1))
        side.add(LN2_PLANS[2], ln2(1, 2 * u + 1, None, 0, 2))

        def packer(i, dst, n):
            left = [n]

            def job(k, a):
                if i < 2:
                    yield from pack_rows(stage_v[i], dst, (k // 2) * 16, (0, D)[k % 2], (D, FM - D)[k % 2], never, a)
                else:
                    yield from pack_rows(stage_v[i], dst, k * 16, 0, D, never, a)
                left[0] -= 1
                if not left[0]:
                    stage_copy(i, jnp.minimum(u + 1, NQ - 1)).start()
                    n0 = stage_v[i].shape[0] - 16
                    side.deps.setdefault(PACK_DUE[i], []).append(stage_v[i][n0:n0 + 8, 0:128].astype(F32))
            return job

        for i in range(2):
            side.add(PACK_PLANS[i], packer(i, view((wgp_v, wup_v)[i], u, D // NQ // 2), len(PACK_PLANS[i])))
            d0 = pl.multiple_of(u * (DQ // 2) + i * (DQA // 2), 8)
            side.add(PACKD_PLANS[i], packer(2 + i, wdp_v.at[pl.ds(d0, 8 * len(PACKD_PLANS[i])), :],
                                            len(PACKD_PLANS[i])))
            for g in range(4):
                step = 107 + 28 * i + 7 * g + G_LAG
                wrap = lambda x: x if x < 156 else 2 * (x - 156) + 1
                side.hooks.setdefault(wrap(step), []).append(
                    lambda i=i, g=g, due=wrap(step + O_DUE): attn_blocks(i, g, side.deps.setdefault(due, [])))
            for c in range(2):
                side.add(O2_PLANS[2 * i + c], o_blocks(i, c, never))
        for i in range(2):
            feat_stage(side, 100 + 28 * i, 0, xs_tile(2 * u + i), lambda p, pr: q_pair(p, i, pr),
                       2 * u if i == 0 else None)
        for i in range(2):
            out_proj(side, 49 * i, 2 * u + i, i)
        side.check()

        @pl.when(u == 0)
        def _():
            o_copy(0, T, 0).start()

        @pl.when(u > 0)
        def _():
            o_copy(pl.multiple_of(tp * T, T), 2 * T, u).start()

        return st["route"]

    wg_copy.wait()
    wu_copy.wait()
    wd_copy.wait()
    route = lax.fori_loop(
        0, NT_ // 2, phase2,
        jnp.full((8, 128), KEY_MIN, jnp.int32))
    st = {"route": route}
    for k in range(len(LN2_PLANS[2]), T // LNC):
        now(finish_rows(h_v[1], k, NT_ - 1, None, st))
    o_copy(S - T, T, NT_).start()

    best = st["route"]
    for shift in (4, 2, 1):
        best = jnp.maximum(best, pltpu.roll(best, shift, 0))
    idx_s = (S - 1) - (best[0, 0] & (S - 1))
    gate = _lane_tile(jax.nn.sigmoid(pltpu.bitcast(_ordered(best & -65536), F32)), D // 128)
    blk = pl.multiple_of((idx_s >> 4) << 4, 16)
    pair = jnp.broadcast_to(hn_v[pl.ds(idx_s >> 1, 1), :], (8, D))
    x8 = pltpu.bitcast(jnp.where((idx_s & 1) == 1, pair & jnp.uint32(0xFFFF0000), pair << 16), F32)
    xs = jnp.concatenate([x8, x8], axis=0).astype(BF16)
    acts, anchors = [], []

    def park(v, half):
        n = v.shape[0] // 128
        for i in range(n):
            z_v[i, :, 128 * half:128 * half + 128] = v[128 * i:128 * i + 128, :]
        return jnp.concatenate([z_v[i, :, 128 * half:128 * half + 128] for i in range(n)], axis=0)

    for c0 in range(0, FM, 128):
        g = _dot(xs, _unpack(wgp_v[:, c0:c0 + 128]), NN)[0:8, :]
        u = _dot(xs, _unpack(wup_v[:, c0:c0 + 128]), NN)[0:8, :]
        anchors += [g, u]
        acts.append(g * jax.nn.sigmoid(g) * u)
    xb = park(_col_broadcast(x8), 0)
    g, u = [_sublane_allreduce(_vpu_matvec(
        xb, lambda g: w[8 * g:8 * g + 8, :].astype(F32), never0,
        anchors[i * MOE_NA // 2:(i + 1) * MOE_NA // 2], MOE_LAGS[0])) for i, w in enumerate((wg_v, wu_v))]
    acts.append(g * jax.nn.sigmoid(g) * u)
    a = jnp.concatenate(acts, axis=1)
    am = jnp.concatenate([a[:, FVD:], a[:, FVD:]], axis=0).astype(BF16)
    ys, anchors = [], anchors[MOE_NA:]
    for k0 in range(0, FF - FVD, 512):
        k1 = min(k0 + 512, FF - FVD)
        yk = _dot(am[:, k0:k1], _unpack(wdp_v[k0 // 2:k1 // 2, 0:D]), NN)[0:8, :]
        ys.append(yk)
        anchors += [yk[:, c:c + 128] for c in range(128, D, 256)]
    ys.append(_sublane_allreduce(_vpu_matvec(
        park(_col_broadcast(a[:, :FVD]), 1), lambda g: wd_v[8 * g:8 * g + 8, :].astype(F32), never0,
        anchors[:-MOE_ND], MOE_LAGS[1])))
    y = _tree(jnp.add, ys) * gate
    y = jnp.concatenate([y, y], axis=0)
    sel = lax.broadcasted_iota(jnp.int32, (16, 1), 0) == (idx_s - blk)
    patch_v[...] = (o_v[pl.ds(blk, 16), :].astype(F32) + jnp.where(sel, y, 0.0)).astype(BF16)
    o_copy(0, T, 0).wait()
    for u in range(1, NT_ // 2):
        o_copy((2 * u - 1) * T, 2 * T, u).wait()
    o_copy(S - T, T, NT_).wait()
    pc = pltpu.make_async_copy(patch_v, out_hbm.at[pl.ds(blk, 16), :], sem.at[SM + 3])
    pc.start()
    for i in range(4):
        stage_copy(i, NQ - 1).wait()
    pc.wait()


@jax.jit
def pallas_sequential_preLN__linear_kernel_hedgehog__moe_arch_mod__prompt_kernel(
    A_x: jax.Array,
    A_wqkv: jax.Array,
    A_w_phi: jax.Array,
    A_wo: jax.Array,
    B_x: jax.Array,
    B_w_r: jax.Array,
    B_w_gate: jax.Array,
    B_w_up: jax.Array,
    B_w_down: jax.Array,
):
    del B_x
    hbm = pl.BlockSpec(memory_space=pl.ANY)
    out = pl.pallas_call(
        _kernel,
        out_shape=jax.ShapeDtypeStruct((S, D), BF16),
        in_specs=[hbm] * 8,
        out_specs=hbm,
        scratch_shapes=[
            pltpu.VMEM((S, D), BF16),
            pltpu.VMEM((T, D), U32),
            pltpu.VMEM((NT_ * TH // 2, SW), U32),
            pltpu.VMEM((NT_ * HK // 2, 128), U32),
            pltpu.VMEM((3 * NC, D, RC), BF16),
            [pltpu.VMEM((D // 2, D), U32)] * 3,
            [pltpu.VMEM((HK // 2, 7 * HK), U32)] * 3,
            pltpu.VMEM((H, DH, DH), BF16),
            pltpu.VMEM((8 * 64, 128), U32),
            pltpu.VMEM((4, QK, D), BF16),
            pltpu.VMEM((QK // 2, 49 * QK + 128), U32),
            pltpu.VMEM((D,), BF16),
            pltpu.VMEM((8, D), F32),
            pltpu.VMEM((NPAIR, 64, 128), F32),
            pltpu.VMEM((NPAIR * 32, 128), U32),
            pltpu.VMEM((NPAIR, 128, T), F32),
            pltpu.VMEM((NPAIR, 128, 128), F32),
            [pltpu.VMEM((NPAIR * 64, T), U32)] * 2,
            [pltpu.VMEM((TH // 2, 7 * HK), U32)] * 2,
            [pltpu.VMEM((TH // 4, 49 * QK), U32)] * 2,
            [pltpu.VMEM((T, D), F32)] * 2,
            pltpu.VMEM((S // 2, D), U32),
            pltpu.VMEM((S, D), BF16),
            pltpu.VMEM((D, FV), BF16),
            pltpu.VMEM((D, FV), BF16),
            pltpu.VMEM((FVD, D), BF16),
            [pltpu.VMEM((D // NQ + 16, FM), BF16), pltpu.VMEM((D // NQ + 16, FM), BF16),
             pltpu.VMEM((DQA + 16, D), BF16), pltpu.VMEM((DQ - DQA + 16, D), BF16)],
            pltpu.VMEM((D // 2, FM), U32),
            pltpu.VMEM((D // 2, FM), U32),
            pltpu.VMEM(((FF - FVD) // 2, D + 128), U32),
            pltpu.VMEM((16, D), BF16),
            pltpu.SemaphoreType.DMA((6 + 3 * NC + NT_ + 16,)),
        ],
        compiler_params=pltpu.CompilerParams(vmem_limit_bytes=100 * 1024 * 1024,
                                             disable_semaphore_checks=True, disable_bounds_checks=True),
        name="hedgehog_mod",
    )(
        A_x.reshape(S, D),
        A_wqkv,
        A_w_phi,
        A_wo.reshape(4, QK, D),
        B_w_r,
        B_w_gate,
        B_w_up,
        B_w_down,
    )
    return out.reshape(1, S, D)
```

```python
import math

import jax
import jax.numpy as jnp
from jax import lax
import jax.experimental.pallas as pl
import jax.experimental.pallas.tpu as pltpu

F32 = jnp.float32
BF16 = jnp.bfloat16
U32 = jnp.uint32

S = 2048
D = 1024
H = 32
DH = 32
FF = 3584
NPAIR = H // 2
LOG2E = 1.4426950408889634
LN_EPS = 1e-5
KEY_MIN = -2 ** 31

T = 256
TH = T // 2
NT_ = S // T
RC = 256
NC = D // RC
PPC = RC // 64
LNC = 16

FV = 10 * 128
FM = FF - FV
FVD = 8 * 128
NQ = NT_ // 2
DQ = (FF - FVD) // NQ
WO_ROWS = 96
QK = D // 4
HK = D // 2
SW = 8 * HK


def _spread(n, a, b, due=None):
    rel = [round(a + (b - a) * k / (n - 1), 3) for k in range(n)]
    return tuple((r, None if due is None else math.ceil(r) + due) for r in rel)


LN1_PLANS = (((0.072, 7), (0.452, 7), (2.8, 9), (4.2, 11), (5.323, 12), (7.125, 13), (8.42, 16), (9.93, 16),
    (11.174, 18), (11.723, 19), (13.877, 22), (15.466, 23), (16.77, 23), (18.221, 25), (19.564, 26), (21.5,
    27)), ((-1.151, 5), (1.211, 7), (1.804, 8), (3.369, 9), (5.17, 11), (5.924, 14), (8.015, 14), (9.695, 17),
    (10.176, 17), (11.93, 19), (13.665, 19), (15.339, 22), (16.785, 22), (18.546, 25), (19.47, 26), (21.122,
    27)))
PRO_LN_PLANS0 = ((None, 4), (None, 7), (0.12, 5), (0.555, 5), (1.7, 6), (2.168, 6), (3.001, None), (4.239,
    None))
PRO_LN_PLANS1 = ((None, 4), (None, 5), (-0.516, None), (0.246, 6), (1.046, 6), (2.1, 7), (3.001, 7), (3.003,
    6))
PRO_K_PLANS0 = ((0.388, None), (0.863, None), (1.721, None), (2.715, None), (2.982, None), (3.948, None),
    (5.473, None), (5.989, None))
PRO_K_PLANS1 = ((-0.866, None), (0.636, None), (1.962, None), (2.951, None), (3.554, None), (4.106, None),
    (4.699, None), (5.223, None))
PRO_X0_PLAN = ((20.049, None), (21.671, None), (23.071, None), (23.684, None), (25.371, None), (25.791, None),
    (26.566, None), (27.089, None))
PRO_W_PLANS0 = ((3.2, None), (3.488, None), (3.771, None), (4.235, None), (4.92, None), (5.413, None), (6.114,
    None), (6.485, None))
PRO_W_PLANS1 = ((4.846, None), (5.235, None), (6.531, None))
PRO_W_PLANS2 = ((6.626, None), (7.329, None), (8.074, None), (9.011, None), (9.904, None), (10.947, None),
    (12.625, None), (13.232, None), (14.27, None), (15.036, None), (16.142, None), (17.035, None), (18.379,
    None), (18.82, None), (19.316, None), (20.753, None), (21.341, None), (22.294, None), (23.106, None),
    (25.173, None))
PRO_K_PLANS2 = ((21.924, None), (22.415, None), (24.003, None), (24.086, None), (24.582, None), (25.771,
    None), (26.668, None), (27.134, None))
PRO_V_PLANS = (((None, None), (None, None), (None, None), (None, None), (None, None), (None, None), (None,
    None), (None, None), (-4.983, 0), (-4.771, 1), (-4.658, 2), (-3.398, 2), (-3.155, 2), (-2.921, 2),
    (-2.695, 3), (-2.355, 3), (-1.874, 4), (-1.535, 4), (-1.124, 4), (-0.925, 4), (-0.706, 4), (0.261, 6),
    (0.532, 7), (0.573, 6), (1.247, 7), (1.4, 7), (2.688, 9), (2.727, 7), (3.012, 8), (3.087, 9), (4.289, 9),
    (4.937, 10)), ((5.897, None), (7.691, None), (9.854, None), (12.014, None), (14.264, None), (15.069,
    None), (17.339, None), (20.836, None)), ((0.0, None), (1.776, None), (3.418, None), (4.808, None)),
    ((20.132, None), (21.451, None), (22.762, None), (23.333, None)), ((16.059, None), (20.449, None),
    (20.497, None), (21.893, None), (22.449, None), (23.173, None), (25.224, None), (25.836, None), (-0.337,
    None), (-0.164, None), (0.63, None), (2.709, None), (2.857, None), (3.639, None), (4.338, None), (4.918,
    None), (5.332, None), (6.91, None), (7.587, None), (8.953, None), (9.24, None), (10.232, None), (11.175,
    None), (12.0, None), (12.57, None), (13.783, None), (14.312, None), (14.773, None), (16.402, None),
    (16.81, None), (17.502, None), (19.159, None)))
END_PLANS = (((-0.162, None), (2.011, None), (3.829, None), (5.62, None), (6.909, None), (8.134, None),
    (10.634, None), (12.371, None), (13.954, None), (15.538, None), (16.797, None), (19.352, None), (20.737,
    None), (23.183, None), (23.393, None), (25.88, None)), ((100.308, None), (101.389, None), (102.104, None),
    (0.409, None), (1.005, None), (2.198, None), (2.898, None), (4.205, None), (5.131, None), (6.022, None),
    (7.291, None), (7.974, None), (8.425, None), (10.079, None), (11.3, None), (11.768, None), (12.903, None),
    (13.561, None), (14.696, None), (15.687, None), (17.565, None), (18.013, None), (18.596, None), (19.613,
    None), (20.25, None), (21.235, None), (22.366, None), (23.06, None), (24.673, None), (25.256, None),
    (25.849, None)))
WO_PLANS = (((0.245, None), (6.671, None), (13.134, None), (18.635, None), (25.68, None)), ((-26.952, None),
    (-20.774, None), (-16.958, None), (-12.341, None), (-8.3, None), (-2.883, None), (1.607, None), (6.233,
    None), (10.547, None), (15.312, None), (19.974, None), (24.229, None)), ((-27.525, None), (-22.089, None),
    (-18.962, None), (-14.225, None), (-9.98, None), (-6.618, None), (-2.09, None)))
LN2_PLANS = (((-0.5, 12), (1.385, 15), (5.612, 19), (6.544, 21), (11.772, 24), (14.638, 27), (17.452, 29),
    (19.2, 33), (23.964, 36), (26.706, 40), (29.685, 42), (33.006, 45)), ((35.739, 47), (38.936, 51), (41.779,
    54), (45.752, 57), (47.863, 61), (50.474, 62), (53.833, 66), (56.742, 69), (61.708, 72), (62.833, 75),
    (65.713, 78), (68.926, 81), (71.975, 82), (74.997, 86), (78.06, 90), (81.109, 92)), ((84.217, None),
    (87.649, None), (89.543, None), (90.236, None)))
O2_PLANS = (((131.357, None), (134.449, None), (137.05, None), (137.656, None), (138.539, None), (140.057,
    None), (144.16, None)), ((141.38, None), (145.789, None), (145.843, None), (146.882, None), (149.928,
    None), (152.324, None), (153.261, None)), ((12.503, None), (22.336, None), (31.211, None), (39.891, None),
    (47.762, None), (57.333, None), (66.0, None)), ((27.948, None), (36.312, None), (43.877, None), (51.105,
    None), (58.218, None), (67.954, None), (76.139, None)))
PACK_PLANS = (((100.502, None), (101.244, None), (102.208, None), (102.296, None), (103.427, None), (104.874,
    None), (105.862, None), (106.631, None), (107.838, None), (108.106, None), (109.264, None), (109.501,
    None), (110.296, None), (111.052, None), (111.166, None), (111.529, None), (114.039, None), (114.221,
    None), (115.251, None), (116.905, None), (117.775, None), (118.037, None), (118.466, None), (118.897,
    None), (121.059, None), (121.33, None), (121.354, None), (122.756, None), (123.403, None), (124.242,
    None), (124.673, None), (125.882, None)), ((128.281, None), (128.956, None), (131.04, None), (131.514,
    None), (131.968, None), (132.242, None), (132.835, None), (133.941, None), (135.423, None), (136.25,
    None), (136.936, None), (137.657, None), (138.836, None), (139.06, None), (140.343, None), (141.492,
    None), (142.08, None), (142.473, None), (143.694, None), (143.8, None), (144.137, None), (146.083, None),
    (146.911, None), (147.792, None), (148.441, None), (149.019, None), (149.771, None), (150.598, None),
    (151.737, None), (152.598, None), (153.829, None), (154.519, None)))
PACKD_PLANS = (((1.12, None), (1.495, None), (4.36, None), (5.329, None), (7.571, None), (9.451, None),
    (9.782, None), (11.222, None), (12.795, None), (14.02, None), (14.575, None), (15.831, None), (19.475,
    None), (20.868, None), (21.935, None), (22.323, None), (25.31, None), (26.102, None), (28.561, None),
    (30.197, None), (31.978, None), (33.481, None)), ((35.02, None), (36.791, None), (38.947, None), (39.775,
    None), (42.179, None), (42.661, None), (46.568, None), (46.704, None), (49.436, None), (51.509, None),
    (51.641, None), (52.889, None), (53.189, None), (55.672, None), (56.222, None), (58.458, None), (59.773,
    None), (60, None)))
PACK_DUE = (130, 5, 39, 64)
DQA = 16 * len(PACKD_PLANS[0])
G_LAG = 5
D_LAG = 1
PLAIN_V0 = 1
OC_PIN = 1
LN2_GAPS = (1.13, 1.5, 0.2)
LN2_SPLIT = 4
PACK_W = 512
GAP_PACK = 0.2
LN1_GAPS = (1, 1.25)
GAP_PRO = 0.13
GAP_X = 0.2
GAP_WO = 0.2
GAP_O2 = 0.26
OUT_ORDER = 1
O_DUE = 6
MOE_NA = 36
MOE_ND = 2
MOE_LAGS = (2, 2)
STAGGER = 8

NN = (((1,), (0,)), ((), ()))
NT = (((1,), (1,)), ((), ()))


def _dot(a, b, dims):
    return lax.dot_general(a, b, dims, preferred_element_type=F32)


def _recip(x):
    return pl.reciprocal(x, approx=False, full_range=False)


def _pack(x):
    return pltpu.bitcast(x, U32)


def _unpack(x):
    return pltpu.bitcast(x, BF16)


def _strassen_lhs(a11, a12, a21, a22):
    return [a21 + a22, a22, a11 + a12, a11, a11 + a22, a12 - a22, a21 - a11]


def _strassen_rhs(b11, b12, b21, b22):
    return [b11, b21 - b11, b22, b12 - b22, b11 + b22, b21 + b22, b11 + b12]


def _strassen(product):
    m2 = product(0)
    m4 = product(1)
    c21 = m2 + m4
    m5 = product(2)
    u11 = m4 - m5
    m3 = product(3)
    c12 = m3 + m5
    u22 = m3 - m2
    m1 = product(4)
    u11 = u11 + m1
    u22 = u22 + m1
    c11 = product(5) + u11
    c22 = product(6) + u22
    return [[c11, c12], [c21, c22]]


def _strassen_rows_first(product, emit):
    m5 = product(2)
    m3 = product(3)
    emit(0, 1, m3 + m5)
    m4 = product(1)
    u11 = m4 - m5
    m1 = product(4)
    u11 = u11 + m1
    u22 = m3 + m1
    emit(0, 0, product(5) + u11)
    m2 = product(0)
    emit(1, 0, m2 + m4)
    u22 = u22 - m2
    emit(1, 1, product(6) + u22)


def _ordered(bits):
    return bits ^ ((bits >> 31) & 0x7FFF0000)


def _block(rows):
    return jnp.concatenate([jnp.concatenate(r, axis=1) for r in rows], axis=0)


def _pair_allreduce(a, op):
    a = op(a, pltpu.roll(a, 2, 0))
    return op(a, pltpu.roll(a, 4, 0))


def _tree(op, xs):
    xs = list(xs)
    while len(xs) > 1:
        nxt = [op(xs[i], xs[i + 1]) for i in range(0, len(xs) - 1, 2)]
        if len(xs) % 2:
            nxt.append(xs[-1])
        xs = nxt
    return xs[0]


def _pair_logits(sl, j):
    sub = lax.broadcasted_iota(jnp.int32, sl[0].shape, 0)
    if j < 3:
        head = jnp.where(sub < 2, 0.0, sl[(0, 1, 16)[j]])
    else:
        head = jnp.where(sub < 2, sl[0], jnp.where(sub < 4, pltpu.roll(sl[1], 2, 0),
                                                   jnp.where(sub < 6, pltpu.roll(sl[16], 4, 0), 0.0)))
    r0 = (2, 9, 17, 24)[j]
    return [head] + list(sl[r0:r0 + 7])


def _dual_exp(sl):
    mx = _pair_allreduce(_tree(jnp.maximum, sl), jnp.maximum)
    mn = _pair_allreduce(_tree(jnp.minimum, sl), jnp.minimum)
    ep = [jnp.exp2(s - mx) for s in sl]
    en = [jnp.exp2(mn - s) for s in sl]
    sp = _pair_allreduce(_tree(jnp.add, ep), jnp.add)
    sn = _pair_allreduce(_tree(jnp.add, en), jnp.add)
    return ep, en, sp, sn


def _after(x, never, anchor):
    if anchor is None:
        return x
    d = jnp.concatenate([anchor] * (x.shape[0] // 8), axis=0)
    if x.shape[1] == 128:
        return jnp.where(never, d, x)
    return jnp.concatenate([jnp.where(never, d, x[:, :128]), x[:, 128:]], axis=1)


def _gate(x, never, deps):
    for i, dep in enumerate(deps):
        d = jnp.broadcast_to(dep, (8, 128))
        if x.dtype != F32:
            d = pltpu.bitcast(d, x.dtype)
        blk = jnp.where(never, d, x[8 * i:8 * i + 8, :128])
        if x.shape[1] > 128:
            blk = jnp.concatenate([blk, x[8 * i:8 * i + 8, 128:]], axis=1)
        parts = ([x[:8 * i, :]] if i else []) + [blk, x[8 * i + 8:, :]]
        x = jnp.concatenate(parts, axis=0)
    return x


def _lane_fold(a):
    return _tree(jnp.add, [a[:, 128 * i:128 * i + 128] for i in range(a.shape[1] // 128)])


def _row_sum(a):
    return jnp.sum(_lane_fold(a), axis=-1, keepdims=True)


def _lane_tile(a, n):
    return a if n == 1 else jnp.concatenate([a] * n, axis=1)


def _sublane_allreduce(a):
    a = a + pltpu.roll(a, 4, 0)
    a = a + pltpu.roll(a, 2, 0)
    return a + pltpu.roll(a, 1, 0)


def _col_broadcast(row8):
    return jnp.concatenate([row8] * 16, axis=0).astype(BF16).T.astype(F32)


def _vpu_matvec(xb, w_rows, never, anchors, lag):
    ng = xb.shape[0] // 8
    acc, hist = None, []
    for g in range(ng):
        dep = anchors[(g * len(anchors)) // ng]
        if g >= lag:
            dep = dep + hist[g - lag]
        x = jnp.where(never, dep, xb[8 * g:8 * g + 8, :])
        w = w_rows(g)
        t = w * _lane_tile(x, w.shape[1] // 128)
        acc = t if acc is None else acc + t
        c = 128 * (g % (w.shape[1] // 128))
        hist.append(acc[:, c:c + 128])
    return acc


class _Side:
    def __init__(self, never, later=lambda rel, gap: rel + gap):
        self.never = never
        self.later = later
        self.jobs = []
        self.deps = {}
        self.hooks = {}

    def add(self, plan, fn):
        for k, (rel, due) in enumerate(plan):
            if rel is None:
                self._run(None, due, fn, k, None)
            else:
                self.jobs.append((rel, due, fn, k))

    def _run(self, rel, due, fn, k, anchor):
        gen = fn if hasattr(fn, "send") else fn(k, anchor)
        dep = gen
        if hasattr(gen, "send"):
            try:
                while True:
                    gap = gen.send(anchor) if gen is fn or rel is None and dep is None else next(gen)
                    if rel is not None:
                        self.jobs.append((self.later(rel, gap), due, gen, k))
                        return
                    dep = None
            except StopIteration as stop:
                dep = stop.value
        if due is not None:
            self.deps.setdefault(due, []).append(dep)

    def check(self):
        assert not self.jobs and not self.deps and not self.hooks

    def gate(self, step, x):
        return _gate(x, self.never, self.deps.pop(step, []))

    def done(self, step, res):
        m = res.shape[0] // 8
        while True:
            ready = [j for j in self.jobs if step - 1 < j[0] <= step]
            if not ready:
                break
            job = min(ready, key=lambda j: j[0])
            self.jobs.remove(job)
            g = m - 1 - int((step - job[0]) * m)
            self._run(*job, res[8 * g:8 * g + 8, res.shape[1] - 128:])
        for fn in self.hooks.pop(step, []):
            fn()


def _kernel(x_hbm, wqkv_hbm, wphi_hbm, wo_hbm, wr_hbm, wg_hbm, wu_hbm, wd_hbm, out_hbm,
            x_v, xn_v, xs_v, lead_v, wraw_v, wt_v, ws_v, wphi_v, a_v, woraw_v, wos_v, wrraw_v, wr_v,
            kvacc_v, kvbf_v, z_v, zb_v, phi_v, oc_v, oc2_v, h_v, hn_v, o_v, wg_v, wu_v, wd_v, stage_v,
            wgp_v, wup_v, wdp_v, patch_v,
            sem):
    SX, SQ, SO, SM = 0, 6, 6 + 3 * NC, 6 + 3 * NC + NT_ + 1

    def x_copy(i):
        h0, h1 = ((0, 1), (1, 2), (3, 4), (4, 8), (8, 2 * NT_), (2, 3))[i]
        rows = pl.ds(h0 * TH, (h1 - h0) * TH)
        return pltpu.make_async_copy(x_hbm.at[rows, :], x_v.at[rows, :], sem.at[SX + i])

    def k0_copy(s):
        return pltpu.make_async_copy(wqkv_hbm.at[:, pl.ds(D + s * 128, 128)],
                                     wraw_v.at[NC, :, pl.ds(s * 128, 128)], sem.at[(SM + 7, SQ + NC)[s]])

    def w_copy(j, c):
        return pltpu.make_async_copy(wqkv_hbm.at[:, pl.ds(j * D + c * RC, RC)], wraw_v.at[j * NC + c],
                                     sem.at[SQ + j * NC + c])

    def wphi_copy(i):
        h0, h1 = ((0, 8), (16, 24), (8, 16), (24, H))[i]
        return pltpu.make_async_copy(wphi_hbm.at[pl.ds(h0, h1 - h0)], wphi_v.at[pl.ds(h0, h1 - h0)],
                                     sem.at[(SM + 4, SM + 8, SM + 9, SM + 14)[i]])

    wr_copy = pltpu.make_async_copy(wr_hbm, wrraw_v, sem.at[SM + 5])

    def wo_copy(i):
        rows = pl.ds(0, WO_ROWS) if i == 0 else pl.ds(WO_ROWS, QK - WO_ROWS)
        return pltpu.make_async_copy(wo_hbm.at[:, rows, :], woraw_v.at[:, rows, :], sem.at[(SM + 6, SM + 15)[i]])

    wg_copy = pltpu.make_async_copy(wg_hbm.at[:, pl.ds(FM, FV)], wg_v, sem.at[SM + 0])
    wu_copy = pltpu.make_async_copy(wu_hbm.at[:, pl.ds(FM, FV)], wu_v, sem.at[SM + 1])
    wd_copy = pltpu.make_async_copy(wd_hbm.at[pl.ds(0, FVD), :], wd_v, sem.at[SM + 2])

    def stage_copy(i, q):
        if i < 2:
            r0 = q * (D // NQ)
            r0 = r0 if isinstance(r0, int) else pl.multiple_of(r0, D // NQ)
            src = (wg_hbm, wu_hbm)[i].at[pl.ds(r0, D // NQ), pl.ds(0, FM)]
        else:
            r0 = FVD + q * DQ + (i - 2) * DQA
            r0 = r0 if isinstance(r0, int) else pl.multiple_of(r0, 16)
            src = wd_hbm.at[pl.ds(r0, (DQA, DQ - DQA)[i - 2]), :]
        return pltpu.make_async_copy(src, stage_v[i].at[pl.ds(0, src.shape[0]), :], sem.at[SM + 10 + i])

    wphi_copy(0).start()
    k0_copy(0).start()
    x_copy(0).start()
    k0_copy(1).start()
    x_copy(1).start()
    wphi_copy(1).start()
    w_copy(1, 2).start()

    made = set()

    def view(ref, i, n, off=0):
        r0 = off + i * n
        return ref.at[pl.ds(r0 if isinstance(r0, int) else pl.multiple_of(r0, math.gcd(n, off)), n), :]

    def put_blocks(dst, r0, fn, m11, m12, m21, m22, never, a, skip=(), base=0, pitch=HK, gap=None):
        for c0 in range(0, m11.shape[1], 128):
            if c0:
                a = yield gap or GAP_PRO
            d11, d22 = m11[:, c0:c0 + 128], m22[:, c0:c0 + 128]
            if a is not None:
                d = jnp.concatenate([a, a], axis=0)
                d11, d22 = jnp.where(never, d, d11), jnp.where(never, d, d22)
            blocks = fn(d11, m12[:, c0:c0 + 128], m21[:, c0:c0 + 128], d22)
            for i, b in enumerate(blocks):
                if i not in skip:
                    dst[r0:r0 + 8, base + i * pitch + c0:base + i * pitch + c0 + 128] = _pack(b.astype(BF16))

    def rows16(ref, r0, c0=0, w=D):
        return _unpack(ref[r0:r0 + 8, c0:c0 + w]).astype(F32)

    def x_blocks(t, k, lo, hi, never, a, gap=None):
        yield from put_blocks(view(xs_v, t, TH // 2), k * LNC // 2, _strassen_rhs,
                              lo[:, :HK], hi[:, :HK], lo[:, HK:], hi[:, HK:], never, a, gap=gap)
        if isinstance(t, int):
            made.add(("xs", t, k))

    def ln_rows(t, k, n, never=None, anchor=None, plain=False):
        wide = lambda c, a: _lane_tile(_after(jnp.broadcast_to(c, (n, 128)), never, a), D // 128)
        x = _after(view(x_v, t, T)[k * n:(k + 1) * n, :].astype(F32), never, anchor)
        s1 = _row_sum(x)
        anchor = yield LN1_GAPS[0]
        xc = x - wide(s1 * (1.0 / D), anchor)
        rstd = lax.rsqrt(_row_sum(xc * xc) * (1.0 / D) + LN_EPS)
        anchor = yield LN1_GAPS[1]
        xn = xc * wide(rstd, anchor)
        if plain:
            xn_v[k * n // 2:(k + 1) * n // 2, :] = _pack(xn.astype(BF16))
        elif k * n < TH:
            xn_v[(T + k * n) // 2:(T + (k + 1) * n) // 2, :] = _pack(xn.astype(BF16))
        else:
            yield from x_blocks(t, k - TH // LNC, rows16(xn_v, (TH + k * n) // 2), xn, never, anchor, GAP_X)
        return _tree(jnp.add, [rstd[8 * i:8 * i + 8, :] for i in range(min(n, LNC) // 8)])

    def now(gen):
        try:
            while True:
                next(gen)
        except StopIteration as stop:
            return stop.value

    def late_x_blocks(t):
        return lambda k, a: x_blocks(t, k, rows16(xn_v, t * T // 2 + 8 * k),
                                     rows16(xn_v, (t * T + TH) // 2 + 8 * k), never0, a)

    def xn_tile(t):
        return _unpack(xn_v[t * T // 2:(t + 1) * T // 2, :])

    def xs_tile(t):
        assert not isinstance(t, int) or t > 1 or made >= {("xs", t, k) for k in range(8)}
        return _unpack(view(xs_v, t, TH // 2)[:, 0:7 * HK])

    def expand_wphi(c):
        w = wphi_v[8 * c:8 * c + 8].reshape(8 * DH, DH).astype(F32).T
        bits = pltpu.bitcast(w, U32)
        head = lax.broadcasted_iota(jnp.int32, (DH, 128), 1) >> 5
        for s in range(2):
            b = bits[:, 128 * s:128 * s + 128]
            for j in range(2):
                r0 = 64 * (2 * c + s) + 32 * j
                a_v[r0:r0 + 32, :] = jnp.where(head == 2 * j, b >> 16,
                                               jnp.where(head == 2 * j + 1, b, jnp.uint32(0)))

    wphi_copy(0).wait()
    expand_wphi(0)
    h_v[1][...] = jnp.zeros((T, D), F32)
    if OC_PIN:
        for ref in oc_v + oc2_v:
            ref[0:8, 0:128] = jnp.zeros((8, 128), U32)
    for ref in stage_v:
        ref[ref.shape[0] - 16:, 0:128] = jnp.zeros((16, 128), BF16)

    def v_transpose(k, a):
        q, r0 = (k // 8) + 4 * (k % 2), 256 * (k % 8 // 2)
        w = wraw_v[2 * NC + q // 2, r0:r0 + 256, (q % 2) * 128:(q % 2) * 128 + 128]
        if a is not None:
            w = _unpack(jnp.where(never0, jnp.concatenate([pltpu.bitcast(a, U32)] * 16, axis=0), _pack(w)))
        wt = _pack(w.T)
        wt_v[2][64 * q:64 * q + 64, r0:r0 + 256] = wt
        made.add(("vt", k))
        return pltpu.bitcast(wt[56:64, 128:256], F32)

    def fold_pairs(j, c, s, side=None, step0=None):
        g0 = 64 * (2 * c + s)
        g0 = g0 if isinstance(g0, int) else pl.multiple_of(g0, 64)
        res = _dot(_unpack(a_v[pl.ds(g0, 64), :]), wraw_v[j * NC + c, :, s * 128:(s + 1) * 128], NT)
        if side is not None:
            side.done(step0 + 2 * s, res[:, :D // 2])
            side.done(step0 + 2 * s + 1, res[:, D // 2:])
        sub = lax.broadcasted_iota(jnp.int32, (8, D), 0)
        out = []
        for q in range(2):
            base = _pair_allreduce(jnp.where(sub < 2, res[64 * q:64 * q + 8, :], 0.0), jnp.add)
            out.append([(res[64 * q + 8 * i:64 * q + 8 * i + 8, :] - base) * LOG2E for i in range(8)])
        return out

    def share(z, z3, k):
        sub = lax.broadcasted_iota(jnp.int32, (8, D), 0)
        return jnp.where(sub < 2, pltpu.roll(z3, 8 - 2 * k, 0), z)

    def packed(slabs):
        return _pack(jnp.concatenate(slabs, axis=0).astype(BF16))

    def fold(j, c, side=None, step0=None):
        p0, p1 = fold_pairs(j, c, 0, side, step0)
        p2, p3 = fold_pairs(j, c, 1, side, step0)
        sl = ([share(p0[0], p3[0], 1), share(p1[0], p3[0], 2)] + p0[1:] + p1[1:]
              + [share(p2[0], p3[0], 3)] + p2[1:] + p3[1:])
        zero = jnp.zeros((8, D), F32)
        even, odd = sl + [zero], [zero] + sl
        r0 = 8 * ((31 * c) // 2)
        is_odd = c % 2 == 1
        if isinstance(c, int):
            sl = odd if is_odd else even
        else:
            r0 = pl.multiple_of(r0, 8)
            sl = [jnp.where(is_odd, o, e) for o, e in zip(odd, even)]
        win = wt_v[j].at[pl.ds(r0, 128), :]
        win[8:128, :] = packed(sl[2:])
        first = packed(sl[:2])
        if is_odd is not False:
            keep = lax.broadcasted_iota(jnp.int32, (8, D), 0) < jnp.where(is_odd, 4, 0)
            first = jnp.where(keep, win[0:8, :], first)
        win[0:8, :] = first
        made.update(("fold", j, q) for q in ([c] if isinstance(c, int) else range(3)))

    def w_blocks(j, k0=0):
        def job(k, a):
            k += k0
            assert made >= ({("vt", 8 * (k // 8) + q) for q in range(8)} if j == 2 else
                            {("fold", j, q) for q in ((0, 2) if k < 15 else range(4))})
            lo, hi = rows16(wt_v[j], 8 * k), rows16(wt_v[j], (256 if j == 2 else 248) + 8 * k)
            yield from put_blocks(ws_v[j], 8 * k, _strassen_lhs, lo[:, :HK], lo[:, HK:], hi[:, :HK], hi[:, HK:],
                                  never0, a, skip=(1, 3))
            made.add(("ws", j, k))
        return job

    def k_pair(p, slot, pr, c0, never=None):
        first = ("z", pr, c0) not in made
        for n in range(c0, c0 + p[0].shape[1], 128):
            assert first == (("z", pr, n) not in made)
            made.update({("z", pr, n), ("phi", slot, pr, n)})
        ep, en, sp, sn = _dual_exp(p)
        inv = _recip(sp * sn)
        scale = (sn * inv, sp * inv)
        es = ep + en
        cols = slice(c0, c0 + p[0].shape[1])
        n = 16 if never is None else 16 // STAGGER
        last = None
        for q in range(16 // n):
            sc = scale
            if last is not None:
                sc = [jnp.where(never, last, x) for x in scale]
            phi = jnp.concatenate([es[i] * sc[i // 8] for i in range(q * n, (q + 1) * n)], axis=0)
            rows = slice(8 * q * n, 8 * (q + 1) * n)
            z = phi if first else z_v[pr, rows, cols] + phi
            z_v[pr, rows, cols] = z
            phi_v[slot][64 * pr + 4 * q * n:64 * pr + 4 * (q + 1) * n, cols] = _pack(phi.astype(BF16))
            last = z[8 * n - 8:, :]

    def kv_update(vts, slot, g, first, publish=False):
        for q, vt in enumerate(vts):
            for j in range(2):
                pr = 2 * g + 8 * q + j
                assert made >= {("phi", slot, pr, 0), ("phi", slot, pr, 128)}
                upd = _dot(vt[64 * j:64 * j + 64, :].astype(BF16), _unpack(phi_v[slot][64 * pr:64 * pr + 64, :]), NT)
                acc = upd if first else kvacc_v[pr] + upd
                kvacc_v[pr] = acc
                if publish:
                    odd = -(lax.broadcasted_iota(jnp.int32, (32, 128), 1) & 1)
                    bits = pltpu.bitcast(acc, jnp.int32) & jnp.concatenate([~odd, odd], axis=0)
                    kvbf_v[32 * pr:32 * pr + 32, :] = _pack(pltpu.bitcast(bits, F32).astype(BF16))

    def save_lead(t):
        view(lead_v, t, HK // 2)[...] = _pack(_unpack(view(xs_v, t, TH // 2)[:, 0:HK]).T)

    def proj_feat(side, step0, c, xn):
        r0 = 8 * ((31 * c) // 2)
        w = wt_v[1][r0:r0 + 128, :]
        quarters = []
        for n in range(2):
            for m in range(2):
                step = step0 + 2 * n + m
                wq = _unpack(side.gate(step, w[:64, :] if m == 0 else w[64:, :]))
                res = _dot(wq, xn[n * TH:(n + 1) * TH, :], NT)
                side.done(step, res)
                quarters.append(res)
        res = jnp.concatenate(
            [jnp.concatenate([quarters[0], quarters[2]], axis=1),
             jnp.concatenate([quarters[1], quarters[3]], axis=1)], axis=0)
        sl = [res[8 * i:8 * i + 8, :] for i in range(res.shape[0] // 8)]
        return sl[c % 2:31 + c % 2]

    def proj_unit(side, step0, j, b, xs, lead=None, plain=None):
        r1 = 64 * b + (64 if j == 2 or b < 3 else 56)
        assert made >= ({("vt", 8 * b + q) for q in range(8)} if plain is not None else
                        {("ws", j, k) for k in range(8 * b, r1 // 8)})
        if plain is not None:
            out = []
            for q in range(2):
                row = []
                for n in range(2):
                    steps = range((0, 2, 4, 5)[2 * q + n], (2, 4, 5, 7)[2 * q + n])
                    deps = [d for i in steps for d in side.deps.pop(step0 + i, [])]
                    w = _gate(wt_v[2][256 * q + 64 * b:256 * q + r1, :], side.never, deps)
                    res = _dot(_unpack(w), plain[n * TH:(n + 1) * TH, :], NT)
                    for i in steps:
                        side.done(step0 + i, res)
                    row.append(res)
                out.append(jnp.concatenate(row, axis=1))
            return out

        def product(i):
            off = 256 if j == 2 else 248
            w = (wt_v[j][off + 64 * b:off + r1, HK:] if i == 1 else wt_v[j][64 * b:r1, :HK] if i == 3
                 else ws_v[j][64 * b:r1, i * HK:(i + 1) * HK])
            w = _unpack(side.gate(step0 + i, w))
            if lead is not None and i == 0:
                res = _dot(w, _unpack(view(lead_v, lead, HK // 2)[...]), NN)
            else:
                res = _dot(w, xs[:, i * HK:(i + 1) * HK], NT)
            side.done(step0 + i, res)
            return res
        return [jnp.concatenate(row, axis=1) for row in _strassen(product)]

    def feat_stage(side, step0, j, xs, pair_fn, lead=None, units=range(4), sl=None, hold=None):
        sl = sl or [[], []]
        for b in units:
            for q, res in enumerate(proj_unit(side, step0 + 7 * b, j, b, xs, lead if b == units[0] else None)):
                sl[q] += [res[8 * i:8 * i + 8, :] for i in range(res.shape[0] // 8)]
            for q in (1, 0):
                for jj in (2 * (b % 2), 2 * (b % 2) + 1):
                    if b != hold:
                        pair_fn(_pair_logits(sl[q][31 * (b // 2):], jj), 8 * q + 4 * (b // 2) + jj)
        return sl

    def v_stage(side, xs, slot, first, publish, lead, plain=None):
        pending = None
        for g in range(4):
            if pending is not None:
                side.hooks.setdefault(7 * g + D_LAG, []).append(lambda p=pending: kv_update(*p))
            pending = (proj_unit(side, 7 * g, 2, g, xs, lead if g == 0 else None, plain if g < PLAIN_V0 else None),
                       slot, g, first, publish)
        side.check()
        return pending

    def pack_rows(src, dst, r0, c0, cols, never, a):
        for c in range(c0, c0 + cols, PACK_W):
            if c > c0:
                a = yield GAP_PACK
            w = min(PACK_W, c0 + cols - c)
            v = src[r0:r0 + 16, c:c + w].astype(F32)
            v = jnp.concatenate([jnp.where(never, _lane_tile(a, w // 128), v[0:8, :]), v[8:16, :]], axis=0)
            dst[r0 // 2:r0 // 2 + 8, c:c + w] = _pack(v.astype(BF16))

    def stash_at(i, k, n):
        return zb_v.at[4 * i + 2 * (k // 16) + n, pl.ds(8 * (k % 16), 8), :]

    def stash(i, sl):
        for k, v in enumerate(sl):
            for n in range(2):
                stash_at(i, k, n)[...] = v[:, 128 * n:128 * n + 128]

    def stashed_k(i, slot, c):
        def job(k, a):
            j, n = k // 2, k % 2
            p = _pair_logits([stash_at(i, q, n)[...] for q in range(16 if j < 2 else 31)], j)
            k_pair([_after(p[0], never0, a)] + p[1:], slot, c * PPC + j, 128 * n, never0)
        return job

    def first_rows(k0, k1, n):
        xn = _unpack(xn_v[n * TH // 2:(n + 1) * TH // 2, :])
        ks = [k for k in range(k0, k1)]
        w = jnp.concatenate([wt_v[1][4 * (k % 32):4 * (k % 32) + 8, :] for k in ks[::2]], axis=0)
        res = _dot(_unpack(w), xn, NT)
        for q, k in enumerate(ks):
            if k % 32 < 31:
                stash_at(0, k % 32, n)[...] = res[8 * q:8 * q + 8, :]

    k0_copy(0).wait()
    x_copy(0).wait()
    wphi_copy(2).start()
    x_copy(5).start()
    w_copy(1, 1).start()
    wphi_copy(3).start()
    x_copy(2).start()
    p0, p1 = fold_pairs(1, 0, 0)
    wt_v[1][8:64, :] = packed(p0[1:] + p1[1:])
    h_v[0][0:8, :] = p0[0]
    h_v[0][8:16, :] = p1[0]
    never0 = now(ln_rows(0, 0, TH, plain=True))[0, 0] < 0.0
    first_rows(2, 16, 0)

    k0_copy(1).wait()
    x_copy(1).wait()
    wphi_copy(1).wait()
    w_copy(1, 3).start()
    for c in (0, 2, 1, 3):
        w_copy(2, c).start()
    p2, p3 = fold_pairs(1, 0, 1)
    wt_v[1][0:8, :] = packed([share(h_v[0][0:8, :], p3[0], 1), share(h_v[0][8:16, :], p3[0], 2)])
    wt_v[1][64:128, :] = packed([share(p2[0], p3[0], 3)] + p2[1:] + p3[1:] + [jnp.zeros((8, D), F32)])
    made.add(("fold", 1, 0))
    now(ln_rows(0, 1, TH, plain=True))
    first_rows(16, 34, 0)
    first_rows(0, 16, 1)
    first_rows(16, 32, 1)
    expand_wphi(2)

    def slow(end):
        return lambda rel, gap: min(rel + (gap / 2 if 3 <= rel < 7 else gap), end)

    for c, prev in ((2, 0), (1, 2)):
        w_copy(1, c).wait()
        wphi_copy(4 - c).wait()
        side = _Side(never0, slow(7))
        if c == 1:
            x_copy(5).wait()
            side.add(PRO_LN_PLANS0, lambda k, a: ln_rows(1, k, LNC, never0, a))
        expand_wphi(5 - 2 * c)
        side.add((PRO_W_PLANS0, PRO_W_PLANS1)[2 - c], w_blocks(1, (2 - c) * len(PRO_W_PLANS0)))
        side.add((PRO_K_PLANS0, PRO_K_PLANS1)[2 - c], stashed_k(prev, 0, prev))
        fold(1, c, side, 0)
        stash(c, proj_feat(side, 4, c, xn_tile(0)))
        side.check()

    x_copy(2).wait()
    w_copy(1, 3).wait()
    x_copy(3).start()
    w_copy(0, 0).start()
    wo_copy(0).start()
    x_copy(4).start()
    side = _Side(never0, slow(28))
    side.add(PRO_LN_PLANS1, lambda k, a: ln_rows(1, k + 8, LNC, never0, a))
    side.add(PRO_W_PLANS2, w_blocks(1, 31 - len(PRO_W_PLANS2)))
    side.add(PRO_K_PLANS2, stashed_k(1, 0, 1))
    side.add(PRO_X0_PLAN, late_x_blocks(0))
    fold(1, 3, side, 0)
    stash(3, proj_feat(side, 4, 3, xn_tile(0)))
    k1 = lambda p, pr: k_pair(p, 1, pr, 0, never0)
    for q, sl in enumerate(feat_stage(side, 8, 1, xs_tile(1), k1, units=range(3), hold=2)):
        stash(2 * q, sl[31:])
    side.check()
    save_lead(1)

    for c in range(NC):
        w_copy(2, c).wait()
    side = _Side(never0, lambda rel, gap: min(rel + gap, 27))
    side.add(PRO_V_PLANS[0], v_transpose)
    side.add(PRO_V_PLANS[1], stashed_k(3, 0, 3))
    side.add(PRO_V_PLANS[2], stashed_k(0, 1, 1))
    side.add(PRO_V_PLANS[3], stashed_k(2, 1, 3))
    side.add(PRO_V_PLANS[4], w_blocks(2))
    sl = [[None] * 31 + [jnp.concatenate([stash_at(2 * q, k, n)[...] for n in range(2)], axis=1) for k in range(17)]
          for q in range(2)]
    feat_stage(side, -28, 1, xs_tile(1), k1, 1, units=range(3, 4), sl=sl)
    kv_update(*v_stage(side, xs_tile(0), 0, True, False, None, xn_tile(0)))
    save_lead(0)
    for c in range(1, NC):
        w_copy(0, c).start()
    wo_copy(1).start()
    wr_copy.start()
    for i in range(4):
        stage_copy(i, 0).start()
    wg_copy.start()
    wu_copy.start()
    wd_copy.start()
    for r0 in (0, 248):
        wt_v[0][r0:r0 + 8, :] = jnp.zeros((8, D), U32)

    def phase1(u, carry):
        never = u < 0

        @pl.when(u == 0)
        def _():
            x_copy(3).wait()
            w_copy(0, 0).wait()
            wo_copy(0).wait()

        @pl.when(u == 1)
        def _():
            x_copy(4).wait()
            w_copy(0, 1).wait()
            w_copy(0, 2).wait()
            wo_copy(1).wait()

        def wo_blocks(k0):
            def job(k, a):
                k += k0
                r, c, part = k // 4, 128 * (k // 2 % 2), k % 2
                r0 = u * ((QK - WO_ROWS) // 2)
                dst = wos_v.at[pl.ds(pl.multiple_of(r0 // 2, 8), WO_ROWS // 2), :]

                def piece(kq, nq):
                    src = woraw_v.at[kq, pl.ds(pl.multiple_of(r0, 16), WO_ROWS), :]
                    return src[16 * r:16 * r + 16, nq * QK + c:nq * QK + c + 128].astype(F32)
                outer = [_strassen_rhs(piece(ki, ni), piece(ki, 2 + ni), piece(2 + ki, ni), piece(2 + ki, 2 + ni))
                         for ki in range(2) for ni in range(2)]
                for i in range(4) if part == 0 else range(4, 7):
                    if i % 4:
                        a = yield GAP_WO
                    yield from put_blocks(dst, 8 * r, _strassen_rhs, *[o[i] for o in outer], never, a,
                                          base=7 * i * QK + c, pitch=QK)
            return job

        xs = xs_tile(2 * u + 1)
        side = _Side(never, lambda rel, gap: min(rel + gap, 27))
        for i in range(2):
            t = 2 * u + 2 + i
            if i == 0:
                side.add(LN1_PLANS[0], lambda k, a: ln_rows(2 * u + 2, k, LNC, never, a))
                side.add(WO_PLANS[0], wo_blocks(0))
            pending = v_stage(side, xs, 1 - i, False, False, t - 1 if i == 0 else None)
            xs = xs_tile(t)
            side = _Side(never, lambda rel, gap, end=(27, -1)[i]: min(rel + gap, end))
            if i == 0:
                side.add(LN1_PLANS[1], lambda k, a: ln_rows(2 * u + 3, k, LNC, never, a))
                side.add(WO_PLANS[1], wo_blocks(len(WO_PLANS[0])))
            else:
                side.add(WO_PLANS[2], wo_blocks(24 - len(WO_PLANS[2])))
            side.hooks[-28 + D_LAG] = [lambda p=pending: kv_update(*p)]
            feat_stage(side, -28, 1, xs, lambda p, pr: k_pair(p, i, pr, 0, never if i == 1 else None))
            save_lead(t)
        side.check()
        fold(0, u)
        return carry

    lax.fori_loop(0, (NT_ - 2) // 2, phase1, 0)

    w_copy(0, 3).wait()
    wr_copy.wait()
    side = _Side(never0, lambda rel, gap: min(rel + gap, 27 if rel < 98 else 103))

    def z_final(k, a):
        zb_v[k] = jnp.broadcast_to(_row_sum(_after(z_v[k], never0, a)), (128, 128))

    side.add(END_PLANS[0], z_final)
    side.add(END_PLANS[1], w_blocks(0))
    side.hooks[0] = [lambda: fold(0, 3, side, 100)]
    kv_update(*v_stage(side, xs_tile(NT_ - 1), 1, False, True, NT_ - 1))
    wr_v[...] = jnp.broadcast_to(wrraw_v[...].reshape(1, D).astype(F32), (8, D))

    def o_copy(r0, n, i):
        return pltpu.make_async_copy(o_v.at[pl.ds(r0, n), :], out_hbm.at[pl.ds(r0, n), :], sem.at[SO + i])

    def finish_rows(h_ref, k, t, valid, st, never=None, anchor=None):
        r0 = t * T + k * LNC
        rows = slice(k * LNC, (k + 1) * LNC)
        m = jnp.broadcast_to(_row_sum(_after(h_ref[rows, :], never, anchor)) * (1.0 / D), (LNC, 128))
        rstd, r = [], []
        for i in range(LNC // 8):
            anchor = yield LN2_GAPS[2] if i else LN2_GAPS[0]
            mi = _after(m[8 * i:8 * i + 8, :], never, anchor)
            hc = h_ref[k * LNC + 8 * i:k * LNC + 8 * i + 8, :] - _lane_tile(mi, D // 128)
            rs = lax.rsqrt(_row_sum(hc * hc) * (1.0 / D) + LN_EPS)
            r.append((_row_sum(hc * wr_v[...]) * rs + 0.0).astype(BF16).astype(F32))
            rstd.append(jnp.broadcast_to(rs, (8, 128)))
        rstd = jnp.concatenate(rstd, axis=0)
        w = D if never is None else D // LN2_SPLIT
        for c in range(0, D, w):
            anchor = yield LN2_GAPS[2] if c else LN2_GAPS[1]
            h = h_ref[rows, c:c + w]
            hn = (h - _lane_tile(_after(m, never, anchor), w // 128)) * _lane_tile(rstd, w // 128)
            view(hn_v, t, T // 2)[k * LNC // 2:(k + 1) * LNC // 2, c:c + w] = _pack(hn.astype(BF16))
            view(o_v, t, T)[rows, c:c + w] = (hn + h).astype(BF16)
        best = st["route"]
        sub = lax.broadcasted_iota(jnp.int32, (8, 128), 0)
        for i, ri in enumerate(r):
            key = _ordered(pltpu.bitcast(jnp.broadcast_to(ri, (8, 128)), jnp.int32)) | ((S - 1 - r0 - 8 * i) - sub)
            if valid is not None:
                key = jnp.where(valid, key, KEY_MIN)
            best = jnp.maximum(best, key)
        st["route"] = best
        return pltpu.bitcast(best, F32)

    def q_pair(p, slot, pr):
        ep, en, sp, sn = _dual_exp(p)
        zz = [_lane_tile(zb_v[pr, 8 * i:8 * i + 8, :], T // 128) for i in range(16)]
        ap = _pair_allreduce(_tree(jnp.add, [ep[i] * zz[i] for i in range(8)]), jnp.add)
        an = _pair_allreduce(_tree(jnp.add, [en[i] * zz[8 + i] for i in range(8)]), jnp.add)
        inv = _recip(ap * sn + (an + 1e-6 * sn) * sp)
        rp = sn * inv
        rn = sp * inv
        phi = jnp.concatenate([e * rp for e in ep] + [e * rn for e in en], axis=0)
        phi_v[slot][64 * pr:64 * pr + 64, :] = _pack(phi.astype(BF16))

    held = []

    def attn_blocks(slot, g, deps):
        res = [_dot(_unpack(kvbf_v[32 * pr:32 * pr + 32, :]), _unpack(phi_v[slot][64 * pr:64 * pr + 64, :]), NN)
               for pr in (2 * g, 2 * g + 8, 2 * g + 1, 2 * g + 9)]
        lo, hi = jnp.concatenate(res[0::2], axis=0), jnp.concatenate(res[1::2], axis=0)
        blocks = [(i, g, b) for i, b in enumerate(_strassen_lhs(lo[:, :TH], hi[:, :TH], lo[:, TH:], hi[:, TH:]))]
        if g % 2 == 0:
            held.append(blocks.pop())
        else:
            blocks.append(held.pop())
        ot = _pack(jnp.concatenate([b for _, _, b in blocks], axis=1).astype(BF16).T)
        for q, (i, n, _) in enumerate(blocks):
            oc_v[slot][:, i * HK + 128 * n:i * HK + 128 * n + 128] = ot[q * TH // 2:(q + 1) * TH // 2, :]
            made.add(("oc", slot, i, n))
            if q % 2:
                deps.append(pltpu.bitcast(ot[(q + 1) * TH // 2 - 8:(q + 1) * TH // 2, :], F32))

    def o_blocks(slot, c, never):
        def job(k, a):
            k = (2, 3, 1, 4, 5, 0, 6)[k]
            assert made >= {("oc", slot, k, c), ("oc", slot, k, c + 2)}
            for r in range(4):
                if r:
                    a = yield GAP_O2
                m = [rows16(oc_v[slot], 8 * r + 32 * q, k * HK + n * QK + 128 * c, 128)
                     for q in range(2) for n in range(2)]
                yield from put_blocks(oc2_v[slot], 8 * r, _strassen_lhs, *m, never, a, skip=(1, 3),
                                      base=7 * k * QK + 128 * c, pitch=QK)
            made.add(("oc2", slot, k, c))
        return job

    def out_proj(side, step0, t, slot):
        count = [0]

        def inner(i, c):
            assert made >= {("oc2", slot, i, 0), ("oc2", slot, i, 1)}

            def product(j):
                step, odd = step0 + count[0] // 2, count[0] % 2
                count[0] += 1
                o = (oc_v[slot][32:64, i * HK + QK:(i + 1) * HK] if j == 1 else
                     oc_v[slot][0:32, i * HK:i * HK + QK] if j == 3 else
                     oc2_v[slot][:, (7 * i + j) * QK:(7 * i + j + 1) * QK])
                w = wos_v[:, (7 * i + j) * QK + 128 * c:(7 * i + j) * QK + 128 * c + 128]
                res = _dot(_unpack(o), _unpack(w if odd else side.gate(step, w)), NN)
                if odd:
                    side.done(step, res)
                return res
            return _block(_strassen(product))

        xt = view(x_v, t, T)

        def emit(cs, q, r, res):
            for k, c in enumerate(cs):
                for n in range(2):
                    rows, c0 = slice(q * TH, (q + 1) * TH), r * HK + n * QK + 128 * c
                    h_v[slot][rows, c0:c0 + 128] = (res[:, 256 * k + 128 * n:256 * k + 128 * n + 128]
                                                    + xt[rows, c0:c0 + 128].astype(F32))
                made.add(("h", slot, q, r, c))

        for cs in ((0,), (1,)) if OUT_ORDER == 0 else ((0, 1),):
            _strassen_rows_first(lambda i: jnp.concatenate([inner(i, c) for c in cs], axis=1),
                                 lambda q, r, res: emit(cs, q, r, res))

    def phase2(u, carry):
        for i in range(4):
            stage_copy(i, u).wait()
        never = u < 0
        side = _Side(never, lambda rel, gap: min(rel + 2 * gap, 97) if rel < 98 else
                     rel + gap if rel + gap <= 155 else 2 * (rel + gap - 155) - 1)
        st = {"route": carry}
        tp = jnp.maximum(2 * u - 1, 0)
        early = len(LN2_PLANS[2])
        order = []

        def ln2(slot, t, valid, k0, key):
            def job(k, a):
                k += k0
                hs = {("h", slot, k // 8, r, c) for r in range(2) for c in range(2)}
                assert made >= hs or key == 0
                best = yield from finish_rows(h_v[slot], k, t, valid, st, never, a)
                assert key > 0 or not made & hs
                order.append((key, k))
                assert order == sorted(order)
                return best
            return job

        side.add(LN2_PLANS[0], ln2(1, tp, u > 0, early, 0))
        side.add(LN2_PLANS[1], ln2(0, 2 * u, None, 0, 1))
        side.add(LN2_PLANS[2], ln2(1, 2 * u + 1, None, 0, 2))

        def packer(i, dst, n):
            left = [n]

            def job(k, a):
                if i < 2:
                    yield from pack_rows(stage_v[i], dst, (k // 2) * 16, (0, D)[k % 2], (D, FM - D)[k % 2], never, a)
                else:
                    yield from pack_rows(stage_v[i], dst, k * 16, 0, D, never, a)
                left[0] -= 1
                if not left[0]:
                    stage_copy(i, jnp.minimum(u + 1, NQ - 1)).start()
                    n0 = stage_v[i].shape[0] - 16
                    side.deps.setdefault(PACK_DUE[i], []).append(stage_v[i][n0:n0 + 8, 0:128].astype(F32))
            return job

        for i in range(2):
            side.add(PACK_PLANS[i], packer(i, view((wgp_v, wup_v)[i], u, D // NQ // 2), len(PACK_PLANS[i])))
            d0 = pl.multiple_of(u * (DQ // 2) + i * (DQA // 2), 8)
            side.add(PACKD_PLANS[i], packer(2 + i, wdp_v.at[pl.ds(d0, 8 * len(PACKD_PLANS[i])), :],
                                            len(PACKD_PLANS[i])))
            for g in range(4):
                step = 107 + 28 * i + 7 * g + G_LAG
                wrap = lambda x: x if x < 156 else 2 * (x - 156) + 1
                side.hooks.setdefault(wrap(step), []).append(
                    lambda i=i, g=g, due=wrap(step + O_DUE): attn_blocks(i, g, side.deps.setdefault(due, [])))
            for c in range(2):
                side.add(O2_PLANS[2 * i + c], o_blocks(i, c, never))
        for i in range(2):
            feat_stage(side, 100 + 28 * i, 0, xs_tile(2 * u + i), lambda p, pr: q_pair(p, i, pr),
                       2 * u if i == 0 else None)
        for i in range(2):
            out_proj(side, 49 * i, 2 * u + i, i)
        side.check()

        @pl.when(u == 0)
        def _():
            o_copy(0, T, 0).start()

        @pl.when(u > 0)
        def _():
            o_copy(pl.multiple_of(tp * T, T), 2 * T, u).start()

        return st["route"]

    wg_copy.wait()
    wu_copy.wait()
    wd_copy.wait()
    route = lax.fori_loop(
        0, NT_ // 2, phase2,
        jnp.full((8, 128), KEY_MIN, jnp.int32))
    st = {"route": route}
    for k in range(len(LN2_PLANS[2]), T // LNC):
        now(finish_rows(h_v[1], k, NT_ - 1, None, st))
    o_copy(S - T, T, NT_).start()

    best = st["route"]
    for shift in (4, 2, 1):
        best = jnp.maximum(best, pltpu.roll(best, shift, 0))
    idx_s = (S - 1) - (best[0, 0] & (S - 1))
    gate = _lane_tile(jax.nn.sigmoid(pltpu.bitcast(_ordered(best & -65536), F32)), D // 128)
    blk = pl.multiple_of((idx_s >> 4) << 4, 16)
    pair = jnp.broadcast_to(hn_v[pl.ds(idx_s >> 1, 1), :], (8, D))
    x8 = pltpu.bitcast(jnp.where((idx_s & 1) == 1, pair & jnp.uint32(0xFFFF0000), pair << 16), F32)
    xs = jnp.concatenate([x8, x8], axis=0).astype(BF16)
    acts, anchors = [], []

    def park(v, half):
        n = v.shape[0] // 128
        for i in range(n):
            z_v[i, :, 128 * half:128 * half + 128] = v[128 * i:128 * i + 128, :]
        return jnp.concatenate([z_v[i, :, 128 * half:128 * half + 128] for i in range(n)], axis=0)

    for c0 in range(0, FM, 128):
        g = _dot(xs, _unpack(wgp_v[:, c0:c0 + 128]), NN)[0:8, :]
        u = _dot(xs, _unpack(wup_v[:, c0:c0 + 128]), NN)[0:8, :]
        anchors += [g, u]
        acts.append(g * jax.nn.sigmoid(g) * u)
    xb = park(_col_broadcast(x8), 0)
    g, u = [_sublane_allreduce(_vpu_matvec(
        xb, lambda g: w[8 * g:8 * g + 8, :].astype(F32), never0,
        anchors[i * MOE_NA // 2:(i + 1) * MOE_NA // 2], MOE_LAGS[0])) for i, w in enumerate((wg_v, wu_v))]
    acts.append(g * jax.nn.sigmoid(g) * u)
    a = jnp.concatenate(acts, axis=1)
    am = jnp.concatenate([a[:, FVD:], a[:, FVD:]], axis=0).astype(BF16)
    ys, anchors = [], anchors[MOE_NA:]
    for k0 in range(0, FF - FVD, 512):
        k1 = min(k0 + 512, FF - FVD)
        yk = _dot(am[:, k0:k1], _unpack(wdp_v[k0 // 2:k1 // 2, 0:D]), NN)[0:8, :]
        ys.append(yk)
        anchors += [yk[:, c:c + 128] for c in range(128, D, 256)]
    ys.append(_sublane_allreduce(_vpu_matvec(
        park(_col_broadcast(a[:, :FVD]), 1), lambda g: wd_v[8 * g:8 * g + 8, :].astype(F32), never0,
        anchors[:-MOE_ND], MOE_LAGS[1])))
    y = _tree(jnp.add, ys) * gate
    y = jnp.concatenate([y, y], axis=0)
    sel = lax.broadcasted_iota(jnp.int32, (16, 1), 0) == (idx_s - blk)
    patch_v[...] = (o_v[pl.ds(blk, 16), :].astype(F32) + jnp.where(sel, y, 0.0)).astype(BF16)
    o_copy(0, T, 0).wait()
    for u in range(1, NT_ // 2):
        o_copy((2 * u - 1) * T, 2 * T, u).wait()
    o_copy(S - T, T, NT_).wait()
    pc = pltpu.make_async_copy(patch_v, out_hbm.at[pl.ds(blk, 16), :], sem.at[SM + 3])
    pc.start()
    for i in range(4):
        stage_copy(i, NQ - 1).wait()
    pc.wait()


@jax.jit
def pallas_sequential_preLN__linear_kernel_hedgehog__moe_arch_mod__prompt_kernel(
    A_x: jax.Array,
    A_wqkv: jax.Array,
    A_w_phi: jax.Array,
    A_wo: jax.Array,
    B_x: jax.Array,
    B_w_r: jax.Array,
    B_w_gate: jax.Array,
    B_w_up: jax.Array,
    B_w_down: jax.Array,
):
    del B_x
    hbm = pl.BlockSpec(memory_space=pl.ANY)
    out = pl.pallas_call(
        _kernel,
        out_shape=jax.ShapeDtypeStruct((S, D), BF16),
        in_specs=[hbm] * 8,
        out_specs=hbm,
        scratch_shapes=[
            pltpu.VMEM((S, D), BF16),
            pltpu.VMEM(((T + TH) // 2, D), U32),
            pltpu.VMEM((NT_ * TH // 2, SW), U32),
            pltpu.VMEM((NT_ * HK // 2, 128), U32),
            pltpu.VMEM((3 * NC, D, RC), BF16),
            [pltpu.VMEM((D // 2, D), U32)] * 3,
            [pltpu.VMEM((HK // 2, 7 * HK), U32)] * 3,
            pltpu.VMEM((H, DH, DH), BF16),
            pltpu.VMEM((8 * 64, 128), U32),
            pltpu.VMEM((4, QK, D), BF16),
            pltpu.VMEM((QK // 2, 49 * QK + 128), U32),
            pltpu.VMEM((D,), BF16),
            pltpu.VMEM((8, D), F32),
            pltpu.VMEM((NPAIR, 64, 128), F32),
            pltpu.VMEM((NPAIR * 32, 128), U32),
            pltpu.VMEM((NPAIR, 128, T), F32),
            pltpu.VMEM((NPAIR, 128, 128), F32),
            [pltpu.VMEM((NPAIR * 64, T), U32)] * 2,
            [pltpu.VMEM((TH // 2, 7 * HK), U32)] * 2,
            [pltpu.VMEM((TH // 4, 49 * QK), U32)] * 2,
            [pltpu.VMEM((T, D), F32)] * 2,
            pltpu.VMEM((S // 2, D), U32),
            pltpu.VMEM((S, D), BF16),
            pltpu.VMEM((D, FV), BF16),
            pltpu.VMEM((D, FV), BF16),
            pltpu.VMEM((FVD, D), BF16),
            [pltpu.VMEM((D // NQ + 16, FM), BF16), pltpu.VMEM((D // NQ + 16, FM), BF16),
             pltpu.VMEM((DQA + 16, D), BF16), pltpu.VMEM((DQ - DQA + 16, D), BF16)],
            pltpu.VMEM((D // 2, FM), U32),
            pltpu.VMEM((D // 2, FM), U32),
            pltpu.VMEM(((FF - FVD) // 2, D + 128), U32),
            pltpu.VMEM((16, D), BF16),
            pltpu.SemaphoreType.DMA((6 + 3 * NC + NT_ + 17,)),
        ],
        compiler_params=pltpu.CompilerParams(vmem_limit_bytes=100 * 1024 * 1024,
                                             disable_semaphore_checks=True, disable_bounds_checks=True),
        name="hedgehog_mod",
    )(
        A_x.reshape(S, D),
        A_wqkv,
        A_w_phi,
        A_wo.reshape(4, QK, D),
        B_w_r,
        B_w_gate,
        B_w_up,
        B_w_down,
    )
    return out.reshape(1, S, D)
```

```python
import math

import jax
import jax.numpy as jnp
from jax import lax
import jax.experimental.pallas as pl
import jax.experimental.pallas.tpu as pltpu

F32 = jnp.float32
BF16 = jnp.bfloat16
U32 = jnp.uint32

S = 2048
D = 1024
H = 32
DH = 32
FF = 3584
NPAIR = H // 2
LOG2E = 1.4426950408889634
LN_EPS = 1e-5
KEY_MIN = -2 ** 31

T = 256
TH = T // 2
NT_ = S // T
RC = 256
NC = D // RC
PPC = RC // 64
LNC = 16

FV = 10 * 128
FM = FF - FV
FVD = 8 * 128
NQ = NT_ // 2
DQ = (FF - FVD) // NQ
WO_ROWS = 96
QK = D // 4
HK = D // 2
SW = 8 * HK


def _spread(n, a, b, due=None):
    rel = [round(a + (b - a) * k / (n - 1), 3) for k in range(n)]
    return tuple((r, None if due is None else math.ceil(r) + due) for r in rel)


LN1_PLANS = (((0.095, 7), (0.452, 8), (2.855, 10), (4.2, 11), (5.323, 12), (7.125, 13), (8.42, 16), (9.93,
    16), (11.174, 18), (11.928, 19), (13.877, 22), (15.466, 23), (16.77, 23), (18.221, 25), (19.564, 26),
    (21.5, 27)), ((-1.151, 4), (1.211, 7), (1.804, 8), (3.43, 9), (5.504, 11), (5.924, 14), (8.015, 14),
    (9.695, 17), (10.176, 17), (11.93, 19), (13.665, 19), (15.339, 22), (16.395, 22), (18.546, 25), (19.409,
    26), (21.079, 27)))
PRO_LN_PLANS0 = ((None, 4), (None, 7), (0.12, 5), (0.555, 5), (1.7, 6), (2.168, 6), (3.297, None), (4.239,
    None))
PRO_LN_PLANS1 = ((None, 4), (None, 5), (-0.516, None), (0.246, 6), (1.046, 6), (2.1, 7), (3.001, 7), (3.003,
    6))
PRO_K_PLANS0 = ((0.388, None), (0.863, None), (1.721, None), (2.715, None), (2.982, None), (3.948, None),
    (5.473, None), (5.989, None))
PRO_K_PLANS1 = ((-0.866, None), (0.636, None), (1.962, None), (2.951, None), (3.554, None), (4.106, None),
    (4.699, None), (5.223, None))
PRO_X0_PLAN = ((20.049, None), (21.671, None), (23.071, None), (23.684, None), (25.371, None), (26.097, None),
    (26.566, None), (27.089, None))
PRO_W_PLANS0 = ((3.2, None), (3.488, None), (3.771, None), (4.235, None), (4.92, None), (5.413, None), (6.114,
    None), (6.485, None))
PRO_W_PLANS1 = ((4.846, None), (5.235, None), (6.531, None))
PRO_W_PLANS2 = ((6.626, None), (7.329, None), (8.074, None), (9.011, None), (9.904, None), (10.947, None),
    (12.625, None), (13.232, None), (14.27, None), (15.036, None), (16.142, None), (17.035, None), (18.379,
    None), (19.306, None), (19.316, None), (20.753, None), (21.341, None), (22.294, None), (23.106, None),
    (25.173, None))
PRO_K_PLANS2 = ((21.924, None), (22.415, None), (24.003, None), (24.127, None), (24.582, None), (25.771,
    None), (26.668, None), (27.134, None))
PRO_V_PLANS = (((None, None), (None, None), (None, None), (None, None), (None, None), (None, None), (None,
    None), (None, None), (-4.983, 0), (-4.771, 1), (-4.658, 2), (-3.398, 2), (-3.155, 2), (-2.921, 2),
    (-2.499, 3), (-2.355, 3), (-1.874, 4), (-1.535, 4), (-1.024, 4), (-0.927, 4), (-0.706, 4), (0.24, 6),
    (0.481, 7), (0.668, 6), (1.247, 7), (1.4, 7), (2.688, 9), (2.727, 7), (3.012, 8), (3.087, 9), (4.289, 9),
    (4.924, 10)), ((5.897, None), (7.691, None), (10.048, None), (12.014, None), (13.868, None), (15.456,
    None), (17.412, None), (20.836, None)), ((0.0, None), (1.776, None), (3.418, None), (4.808, None)),
    ((19.45, None), (21.451, None), (22.925, None), (23.333, None)), ((16.059, None), (20.449, None), (20.497,
    None), (21.79, None), (22.449, None), (22.572, None), (25.109, None), (25.686, None), (-0.337, None),
    (-0.164, None), (0.488, None), (2.709, None), (2.857, None), (3.639, None), (4.322, None), (4.918, None),
    (5.207, None), (6.91, None), (7.587, None), (8.953, None), (9.24, None), (10.232, None), (11.175, None),
    (11.993, None), (12.583, None), (13.787, None), (14.312, None), (14.817, None), (16.402, None), (16.81,
    None), (17.304, None), (19.292, None)))
END_PLANS = (((-0.162, None), (2.011, None), (3.829, None), (5.62, None), (6.909, None), (8.156, None),
    (10.634, None), (12.371, None), (13.954, None), (15.538, None), (16.797, None), (19.352, None), (20.737,
    None), (23.183, None), (23.393, None), (25.88, None)), ((100.308, None), (101.389, None), (102.104, None),
    (0.409, None), (1.005, None), (2.198, None), (2.898, None), (4.205, None), (5.131, None), (6.022, None),
    (7.291, None), (7.974, None), (8.425, None), (9.982, None), (11.3, None), (11.768, None), (12.903, None),
    (13.561, None), (14.696, None), (15.687, None), (17.565, None), (18.013, None), (18.596, None), (19.613,
    None), (20.25, None), (21.235, None), (22.366, None), (23.06, None), (24.673, None), (25.256, None),
    (26.011, None)))
WO_PLANS = (((0.245, None), (6.671, None), (13.134, None), (18.635, None), (24.922, None)), ((-26.952, None),
    (-21.248, None), (-16.958, None), (-12.341, None), (-8.3, None), (-2.883, None), (1.607, None), (6.233,
    None), (10.547, None), (15.312, None), (19.974, None), (24.229, None)), ((-27.707, None), (-22.089, None),
    (-18.962, None), (-14.225, None), (-9.98, None), (-6.618, None), (-2.09, None)))
LN2_PLANS = (((-0.5, 12), (1.385, 15), (5.416, 19), (6.544, 21), (11.772, 24), (14.638, 27), (17.452, 29),
    (19.2, 33), (23.964, 36), (26.706, 40), (29.685, 42), (33.006, 46)), ((35.739, 47), (38.936, 51), (41.779,
    54), (45.752, 57), (47.863, 61), (50.474, 62), (53.833, 66), (56.742, 69), (61.708, 72), (62.833, 75),
    (65.713, 78), (68.926, 82), (71.975, 82), (74.997, 86), (78.06, 90), (81.109, 92)), ((84.217, None),
    (87.649, None), (89.543, None), (90.236, None)))
O2_PLANS = (((131.357, None), (134.449, None), (137.05, None), (137.656, None), (138.539, None), (140.057,
    None), (144.16, None)), ((141.38, None), (145.789, None), (145.843, None), (146.882, None), (149.928,
    None), (152.324, None), (153.261, None)), ((12.503, None), (22.336, None), (31.211, None), (39.891, None),
    (47.762, None), (57.333, None), (66.0, None)), ((27.948, None), (36.312, None), (43.877, None), (50.771,
    None), (58.218, None), (67.954, None), (76.139, None)))
PACK_PLANS = (((100.502, None), (101.244, None), (102.208, None), (102.296, None), (103.427, None), (104.874,
    None), (105.862, None), (106.631, None), (107.838, None), (108.106, None), (109.264, None), (109.501,
    None), (110.296, None), (111.052, None), (111.166, None), (111.529, None), (114.039, None), (114.221,
    None), (115.251, None), (116.905, None), (117.839, None), (118.037, None), (118.466, None), (118.897,
    None), (121.059, None), (121.33, None), (121.354, None), (122.756, None), (123.403, None), (124.242,
    None), (124.673, None), (125.882, None)), ((128.281, None), (128.956, None), (131.04, None), (131.514,
    None), (131.968, None), (132.242, None), (132.835, None), (133.941, None), (135.423, None), (136.25,
    None), (136.936, None), (137.657, None), (138.836, None), (139.06, None), (140.343, None), (141.492,
    None), (142.08, None), (142.473, None), (143.694, None), (143.8, None), (144.137, None), (146.083, None),
    (146.911, None), (147.792, None), (148.441, None), (149.019, None), (149.771, None), (150.598, None),
    (151.737, None), (152.598, None), (153.829, None), (154.519, None)))
PACKD_PLANS = (((1.12, None), (1.633, None), (4.36, None), (5.329, None), (7.571, None), (9.451, None),
    (9.782, None), (11.103, None), (12.795, None), (14.02, None), (14.575, None), (15.831, None), (19.475,
    None), (20.868, None), (21.935, None), (22.323, None), (25.31, None), (26.102, None), (28.561, None),
    (30.197, None), (31.978, None), (33.481, None)), ((35.02, None), (36.791, None), (38.947, None), (39.775,
    None), (42.179, None), (42.661, None), (46.568, None), (46.704, None), (49.436, None), (51.509, None),
    (51.641, None), (52.889, None), (53.189, None), (55.672, None), (56.222, None), (58.458, None), (59.773,
    None), (60, None)))
PACK_DUE = (130, 5, 39, 64)
DQA = 16 * len(PACKD_PLANS[0])
G_LAG = 5
D_LAG = 1
PLAIN_V0 = 1
OC_PIN = 1
LN2_GAPS = (1.13, 1.5, 0.2)
LN2_SPLIT = 4
PACK_W = 512
GAP_PACK = 0.2
LN1_GAPS = (1, 1.25)
GAP_PRO = 0.13
GAP_X = 0.2
GAP_WO = 0.2
GAP_O2 = 0.26
OUT_ORDER = 1
O_DUE = 6
MOE_NA = 36
MOE_ND = 2
MOE_LAGS = (2, 2)
STAGGER = 8

NN = (((1,), (0,)), ((), ()))
NT = (((1,), (1,)), ((), ()))


def _dot(a, b, dims):
    return lax.dot_general(a, b, dims, preferred_element_type=F32)


def _recip(x):
    return pl.reciprocal(x, approx=False, full_range=False)


def _pack(x):
    return pltpu.bitcast(x, U32)


def _unpack(x):
    return pltpu.bitcast(x, BF16)


def _strassen_lhs(a11, a12, a21, a22):
    return [a21 + a22, a22, a11 + a12, a11, a11 + a22, a12 - a22, a21 - a11]


def _strassen_rhs(b11, b12, b21, b22):
    return [b11, b21 - b11, b22, b12 - b22, b11 + b22, b21 + b22, b11 + b12]


def _strassen(product):
    m2 = product(0)
    m4 = product(1)
    c21 = m2 + m4
    m5 = product(2)
    u11 = m4 - m5
    m3 = product(3)
    c12 = m3 + m5
    u22 = m3 - m2
    m1 = product(4)
    u11 = u11 + m1
    u22 = u22 + m1
    c11 = product(5) + u11
    c22 = product(6) + u22
    return [[c11, c12], [c21, c22]]


def _strassen_rows_first(product, emit):
    m5 = product(2)
    m3 = product(3)
    emit(0, 1, m3 + m5)
    m4 = product(1)
    u11 = m4 - m5
    m1 = product(4)
    u11 = u11 + m1
    u22 = m3 + m1
    emit(0, 0, product(5) + u11)
    m2 = product(0)
    emit(1, 0, m2 + m4)
    u22 = u22 - m2
    emit(1, 1, product(6) + u22)


def _ordered(bits):
    return bits ^ ((bits >> 31) & 0x7FFF0000)


def _block(rows):
    return jnp.concatenate([jnp.concatenate(r, axis=1) for r in rows], axis=0)


def _pair_allreduce(a, op):
    a = op(a, pltpu.roll(a, 2, 0))
    return op(a, pltpu.roll(a, 4, 0))


def _tree(op, xs):
    xs = list(xs)
    while len(xs) > 1:
        nxt = [op(xs[i], xs[i + 1]) for i in range(0, len(xs) - 1, 2)]
        if len(xs) % 2:
            nxt.append(xs[-1])
        xs = nxt
    return xs[0]


def _pair_logits(sl, j):
    sub = lax.broadcasted_iota(jnp.int32, sl[0].shape, 0)
    if j < 3:
        head = jnp.where(sub < 2, 0.0, sl[(0, 1, 16)[j]])
    else:
        head = jnp.where(sub < 2, sl[0], jnp.where(sub < 4, pltpu.roll(sl[1], 2, 0),
                                                   jnp.where(sub < 6, pltpu.roll(sl[16], 4, 0), 0.0)))
    r0 = (2, 9, 17, 24)[j]
    return [head] + list(sl[r0:r0 + 7])


def _dual_exp(sl):
    mx = _pair_allreduce(_tree(jnp.maximum, sl), jnp.maximum)
    mn = _pair_allreduce(_tree(jnp.minimum, sl), jnp.minimum)
    ep = [jnp.exp2(s - mx) for s in sl]
    en = [jnp.exp2(mn - s) for s in sl]
    sp = _pair_allreduce(_tree(jnp.add, ep), jnp.add)
    sn = _pair_allreduce(_tree(jnp.add, en), jnp.add)
    return ep, en, sp, sn


def _after(x, never, anchor):
    if anchor is None:
        return x
    d = jnp.concatenate([anchor] * (x.shape[0] // 8), axis=0)
    if x.shape[1] == 128:
        return jnp.where(never, d, x)
    return jnp.concatenate([jnp.where(never, d, x[:, :128]), x[:, 128:]], axis=1)


def _gate(x, never, deps):
    for i, dep in enumerate(deps):
        d = jnp.broadcast_to(dep, (8, 128))
        if x.dtype != F32:
            d = pltpu.bitcast(d, x.dtype)
        blk = jnp.where(never, d, x[8 * i:8 * i + 8, :128])
        if x.shape[1] > 128:
            blk = jnp.concatenate([blk, x[8 * i:8 * i + 8, 128:]], axis=1)
        parts = ([x[:8 * i, :]] if i else []) + [blk, x[8 * i + 8:, :]]
        x = jnp.concatenate(parts, axis=0)
    return x


def _lane_fold(a):
    return _tree(jnp.add, [a[:, 128 * i:128 * i + 128] for i in range(a.shape[1] // 128)])


def _row_sum(a):
    return jnp.sum(_lane_fold(a), axis=-1, keepdims=True)


def _lane_tile(a, n):
    return a if n == 1 else jnp.concatenate([a] * n, axis=1)


def _sublane_allreduce(a):
    a = a + pltpu.roll(a, 4, 0)
    a = a + pltpu.roll(a, 2, 0)
    return a + pltpu.roll(a, 1, 0)


def _col_broadcast(row8):
    return jnp.concatenate([row8] * 16, axis=0).astype(BF16).T.astype(F32)


def _vpu_matvec(xb, w_rows, never, anchors, lag):
    ng = xb.shape[0] // 8
    acc, hist = None, []
    for g in range(ng):
        dep = anchors[(g * len(anchors)) // ng]
        if g >= lag:
            dep = dep + hist[g - lag]
        x = jnp.where(never, dep, xb[8 * g:8 * g + 8, :])
        w = w_rows(g)
        t = w * _lane_tile(x, w.shape[1] // 128)
        acc = t if acc is None else acc + t
        c = 128 * (g % (w.shape[1] // 128))
        hist.append(acc[:, c:c + 128])
    return acc


class _Side:
    def __init__(self, never, later=lambda rel, gap: rel + gap):
        self.never = never
        self.later = later
        self.jobs = []
        self.deps = {}
        self.hooks = {}

    def add(self, plan, fn):
        for k, (rel, due) in enumerate(plan):
            if rel is None:
                self._run(None, due, fn, k, None)
            else:
                self.jobs.append((rel, due, fn, k))

    def _run(self, rel, due, fn, k, anchor):
        gen = fn if hasattr(fn, "send") else fn(k, anchor)
        dep = gen
        if hasattr(gen, "send"):
            try:
                while True:
                    gap = gen.send(anchor) if gen is fn or rel is None and dep is None else next(gen)
                    if rel is not None:
                        self.jobs.append((self.later(rel, gap), due, gen, k))
                        return
                    dep = None
            except StopIteration as stop:
                dep = stop.value
        if due is not None:
            self.deps.setdefault(due, []).append(dep)

    def check(self):
        assert not self.jobs and not self.deps and not self.hooks

    def gate(self, step, x):
        return _gate(x, self.never, self.deps.pop(step, []))

    def done(self, step, res):
        m = res.shape[0] // 8
        while True:
            ready = [j for j in self.jobs if step - 1 < j[0] <= step]
            if not ready:
                break
            job = min(ready, key=lambda j: j[0])
            self.jobs.remove(job)
            g = m - 1 - int((step - job[0]) * m)
            self._run(*job, res[8 * g:8 * g + 8, res.shape[1] - 128:])
        for fn in self.hooks.pop(step, []):
            fn()


def _kernel(x_hbm, wqkv_hbm, wphi_hbm, wo_hbm, wr_hbm, wg_hbm, wu_hbm, wd_hbm, out_hbm,
            x_v, xn_v, xs_v, lead_v, wraw_v, wt_v, ws_v, wphi_v, a_v, woraw_v, wos_v, wrraw_v, wr_v,
            kvacc_v, kvbf_v, z_v, zb_v, phi_v, oc_v, oc2_v, h_v, hn_v, o_v, wg_v, wu_v, wd_v, stage_v,
            wgp_v, wup_v, wdp_v, patch_v,
            sem):
    SX, SQ, SO, SM = 0, 6, 6 + 3 * NC, 6 + 3 * NC + NT_ + 1

    def x_copy(i):
        h0, h1 = ((0, 1), (1, 2), (3, 4), (4, 8), (8, 2 * NT_), (2, 3))[i]
        rows = pl.ds(h0 * TH, (h1 - h0) * TH)
        return pltpu.make_async_copy(x_hbm.at[rows, :], x_v.at[rows, :], sem.at[SX + i])

    def k0_copy(s):
        return pltpu.make_async_copy(wqkv_hbm.at[:, pl.ds(D + s * 128, 128)],
                                     wraw_v.at[NC, :, pl.ds(s * 128, 128)], sem.at[(SM + 7, SQ + NC)[s]])

    def w_copy(j, c):
        return pltpu.make_async_copy(wqkv_hbm.at[:, pl.ds(j * D + c * RC, RC)], wraw_v.at[j * NC + c],
                                     sem.at[SQ + j * NC + c])

    def wphi_copy(i):
        h0, h1 = ((0, 8), (16, 24), (8, 16), (24, H))[i]
        return pltpu.make_async_copy(wphi_hbm.at[pl.ds(h0, h1 - h0)], wphi_v.at[pl.ds(h0, h1 - h0)],
                                     sem.at[(SM + 4, SM + 8, SM + 9, SM + 14)[i]])

    wr_copy = pltpu.make_async_copy(wr_hbm, wrraw_v, sem.at[SM + 5])

    def wo_copy(i):
        rows = pl.ds(0, WO_ROWS) if i == 0 else pl.ds(WO_ROWS, QK - WO_ROWS)
        return pltpu.make_async_copy(wo_hbm.at[:, rows, :], woraw_v.at[:, rows, :], sem.at[(SM + 6, SM + 15)[i]])

    wg_copy = pltpu.make_async_copy(wg_hbm.at[:, pl.ds(FM, FV)], wg_v, sem.at[SM + 0])
    wu_copy = pltpu.make_async_copy(wu_hbm.at[:, pl.ds(FM, FV)], wu_v, sem.at[SM + 1])
    wd_copy = pltpu.make_async_copy(wd_hbm.at[pl.ds(0, FVD), :], wd_v, sem.at[SM + 2])

    def stage_copy(i, q):
        if i < 2:
            r0 = q * (D // NQ)
            r0 = r0 if isinstance(r0, int) else pl.multiple_of(r0, D // NQ)
            src = (wg_hbm, wu_hbm)[i].at[pl.ds(r0, D // NQ), pl.ds(0, FM)]
        else:
            r0 = FVD + q * DQ + (i - 2) * DQA
            r0 = r0 if isinstance(r0, int) else pl.multiple_of(r0, 16)
            src = wd_hbm.at[pl.ds(r0, (DQA, DQ - DQA)[i - 2]), :]
        return pltpu.make_async_copy(src, stage_v[i].at[pl.ds(0, src.shape[0]), :], sem.at[SM + 10 + i])

    wphi_copy(0).start()
    k0_copy(0).start()
    x_copy(0).start()
    k0_copy(1).start()
    x_copy(1).start()
    wphi_copy(1).start()
    w_copy(1, 2).start()

    made = set()

    def view(ref, i, n, off=0):
        r0 = off + i * n
        return ref.at[pl.ds(r0 if isinstance(r0, int) else pl.multiple_of(r0, math.gcd(n, off)), n), :]

    def put_blocks(dst, r0, fn, m11, m12, m21, m22, never, a, skip=(), base=0, pitch=HK, gap=None):
        for c0 in range(0, m11.shape[1], 128):
            if c0:
                a = yield gap or GAP_PRO
            d11, d22 = m11[:, c0:c0 + 128], m22[:, c0:c0 + 128]
            if a is not None:
                d = jnp.concatenate([a, a], axis=0)
                d11, d22 = jnp.where(never, d, d11), jnp.where(never, d, d22)
            blocks = fn(d11, m12[:, c0:c0 + 128], m21[:, c0:c0 + 128], d22)
            for i, b in enumerate(blocks):
                if i not in skip:
                    dst[r0:r0 + 8, base + i * pitch + c0:base + i * pitch + c0 + 128] = _pack(b.astype(BF16))

    def rows16(ref, r0, c0=0, w=D):
        return _unpack(ref[r0:r0 + 8, c0:c0 + w]).astype(F32)

    def x_blocks(t, k, lo, hi, never, a, gap=None):
        yield from put_blocks(view(xs_v, t, TH // 2), k * LNC // 2, _strassen_rhs,
                              lo[:, :HK], hi[:, :HK], lo[:, HK:], hi[:, HK:], never, a, gap=gap)
        if isinstance(t, int):
            made.add(("xs", t, k))

    def ln_rows(t, k, n, never=None, anchor=None, plain=False):
        wide = lambda c, a: _lane_tile(_after(jnp.broadcast_to(c, (n, 128)), never, a), D // 128)
        x = _after(view(x_v, t, T)[k * n:(k + 1) * n, :].astype(F32), never, anchor)
        s1 = _row_sum(x)
        anchor = yield LN1_GAPS[0]
        xc = x - wide(s1 * (1.0 / D), anchor)
        rstd = lax.rsqrt(_row_sum(xc * xc) * (1.0 / D) + LN_EPS)
        anchor = yield LN1_GAPS[1]
        xn = xc * wide(rstd, anchor)
        if plain:
            xn_v[k * n // 2:(k + 1) * n // 2, :] = _pack(xn.astype(BF16))
        elif k * n < TH:
            xn_v[(T + k * n) // 2:(T + (k + 1) * n) // 2, :] = _pack(xn.astype(BF16))
        else:
            yield from x_blocks(t, k - TH // LNC, rows16(xn_v, (TH + k * n) // 2), xn, never, anchor, GAP_X)
        return _tree(jnp.add, [rstd[8 * i:8 * i + 8, :] for i in range(min(n, LNC) // 8)])

    def now(gen):
        try:
            while True:
                next(gen)
        except StopIteration as stop:
            return stop.value

    def late_x_blocks(t):
        return lambda k, a: x_blocks(t, k, rows16(xn_v, t * T // 2 + 8 * k),
                                     rows16(xn_v, (t * T + TH) // 2 + 8 * k), never0, a)

    def xn_tile(t):
        return _unpack(xn_v[t * T // 2:(t + 1) * T // 2, :])

    def xs_tile(t):
        assert not isinstance(t, int) or t > 1 or made >= {("xs", t, k) for k in range(8)}
        return _unpack(view(xs_v, t, TH // 2)[:, 0:7 * HK])

    def expand_wphi(c):
        w = wphi_v[8 * c:8 * c + 8].reshape(8 * DH, DH).astype(F32).T
        bits = pltpu.bitcast(w, U32)
        head = lax.broadcasted_iota(jnp.int32, (DH, 128), 1) >> 5
        for s in range(2):
            b = bits[:, 128 * s:128 * s + 128]
            for j in range(2):
                r0 = 64 * (2 * c + s) + 32 * j
                a_v[r0:r0 + 32, :] = jnp.where(head == 2 * j, b >> 16,
                                               jnp.where(head == 2 * j + 1, b, jnp.uint32(0)))

    wphi_copy(0).wait()
    expand_wphi(0)
    h_v[1][...] = jnp.zeros((T, D), F32)
    if OC_PIN:
        for ref in oc_v + oc2_v:
            ref[0:8, 0:128] = jnp.zeros((8, 128), U32)
    for ref in stage_v:
        ref[ref.shape[0] - 16:, 0:128] = jnp.zeros((16, 128), BF16)

    def v_transpose(k, a):
        q, r0 = (k // 8) + 4 * (k % 2), 256 * (k % 8 // 2)
        w = wraw_v[2 * NC + q // 2, r0:r0 + 256, (q % 2) * 128:(q % 2) * 128 + 128]
        if a is not None:
            w = _unpack(jnp.where(never0, jnp.concatenate([pltpu.bitcast(a, U32)] * 16, axis=0), _pack(w)))
        wt = _pack(w.T)
        wt_v[2][64 * q:64 * q + 64, r0:r0 + 256] = wt
        made.add(("vt", k))
        return pltpu.bitcast(wt[56:64, 128:256], F32)

    def fold_pairs(j, c, s, side=None, step0=None):
        g0 = 64 * (2 * c + s)
        g0 = g0 if isinstance(g0, int) else pl.multiple_of(g0, 64)
        res = _dot(_unpack(a_v[pl.ds(g0, 64), :]), wraw_v[j * NC + c, :, s * 128:(s + 1) * 128], NT)
        if side is not None:
            side.done(step0 + 2 * s, res[:, :D // 2])
            side.done(step0 + 2 * s + 1, res[:, D // 2:])
        sub = lax.broadcasted_iota(jnp.int32, (8, D), 0)
        out = []
        for q in range(2):
            base = _pair_allreduce(jnp.where(sub < 2, res[64 * q:64 * q + 8, :], 0.0), jnp.add)
            out.append([(res[64 * q + 8 * i:64 * q + 8 * i + 8, :] - base) * LOG2E for i in range(8)])
        return out

    def share(z, z3, k):
        sub = lax.broadcasted_iota(jnp.int32, (8, D), 0)
        return jnp.where(sub < 2, pltpu.roll(z3, 8 - 2 * k, 0), z)

    def packed(slabs):
        return _pack(jnp.concatenate(slabs, axis=0).astype(BF16))

    def fold(j, c, side=None, step0=None):
        p0, p1 = fold_pairs(j, c, 0, side, step0)
        p2, p3 = fold_pairs(j, c, 1, side, step0)
        sl = ([share(p0[0], p3[0], 1), share(p1[0], p3[0], 2)] + p0[1:] + p1[1:]
              + [share(p2[0], p3[0], 3)] + p2[1:] + p3[1:])
        zero = jnp.zeros((8, D), F32)
        even, odd = sl + [zero], [zero] + sl
        r0 = 8 * ((31 * c) // 2)
        is_odd = c % 2 == 1
        if isinstance(c, int):
            sl = odd if is_odd else even
        else:
            r0 = pl.multiple_of(r0, 8)
            sl = [jnp.where(is_odd, o, e) for o, e in zip(odd, even)]
        win = wt_v[j].at[pl.ds(r0, 128), :]
        win[8:128, :] = packed(sl[2:])
        first = packed(sl[:2])
        if is_odd is not False:
            keep = lax.broadcasted_iota(jnp.int32, (8, D), 0) < jnp.where(is_odd, 4, 0)
            first = jnp.where(keep, win[0:8, :], first)
        win[0:8, :] = first
        made.update(("fold", j, q) for q in ([c] if isinstance(c, int) else range(3)))

    def w_blocks(j, k0=0):
        def job(k, a):
            k += k0
            assert made >= ({("vt", 8 * (k // 8) + q) for q in range(8)} if j == 2 else
                            {("fold", j, q) for q in ((0, 2) if k < 15 else range(4))})
            lo, hi = rows16(wt_v[j], 8 * k), rows16(wt_v[j], (256 if j == 2 else 248) + 8 * k)
            yield from put_blocks(ws_v[j], 8 * k, _strassen_lhs, lo[:, :HK], lo[:, HK:], hi[:, :HK], hi[:, HK:],
                                  never0, a, skip=(1, 3))
            made.add(("ws", j, k))
        return job

    def k_pair(p, slot, pr, c0, never=None):
        first = ("z", pr, c0) not in made
        for n in range(c0, c0 + p[0].shape[1], 128):
            assert first == (("z", pr, n) not in made)
            made.update({("z", pr, n), ("phi", slot, pr, n)})
        ep, en, sp, sn = _dual_exp(p)
        inv = _recip(sp * sn)
        scale = (sn * inv, sp * inv)
        es = ep + en
        cols = slice(c0, c0 + p[0].shape[1])
        n = 16 if never is None else 16 // STAGGER
        last = None
        for q in range(16 // n):
            sc = scale
            if last is not None:
                sc = [jnp.where(never, last, x) for x in scale]
            phi = jnp.concatenate([es[i] * sc[i // 8] for i in range(q * n, (q + 1) * n)], axis=0)
            rows = slice(8 * q * n, 8 * (q + 1) * n)
            z = phi if first else z_v[pr, rows, cols] + phi
            z_v[pr, rows, cols] = z
            phi_v[slot][64 * pr + 4 * q * n:64 * pr + 4 * (q + 1) * n, cols] = _pack(phi.astype(BF16))
            last = z[8 * n - 8:, :]

    def kv_update(vts, slot, g, first, publish=False):
        for q, vt in enumerate(vts):
            for j in range(2):
                pr = 2 * g + 8 * q + j
                assert made >= {("phi", slot, pr, 0), ("phi", slot, pr, 128)}
                upd = _dot(vt[64 * j:64 * j + 64, :].astype(BF16), _unpack(phi_v[slot][64 * pr:64 * pr + 64, :]), NT)
                acc = upd if first else kvacc_v[pr] + upd
                kvacc_v[pr] = acc
                if publish:
                    odd = -(lax.broadcasted_iota(jnp.int32, (32, 128), 1) & 1)
                    bits = pltpu.bitcast(acc, jnp.int32) & jnp.concatenate([~odd, odd], axis=0)
                    kvbf_v[32 * pr:32 * pr + 32, :] = _pack(pltpu.bitcast(bits, F32).astype(BF16))

    def save_lead(t):
        view(lead_v, t, HK // 2)[...] = _pack(_unpack(view(xs_v, t, TH // 2)[:, 0:HK]).T)

    def proj_feat(side, step0, c, xn):
        r0 = 8 * ((31 * c) // 2)
        w = wt_v[1][r0:r0 + 128, :]
        quarters = []
        for n in range(2):
            for m in range(2):
                step = step0 + 2 * n + m
                wq = _unpack(side.gate(step, w[:64, :] if m == 0 else w[64:, :]))
                res = _dot(wq, xn[n * TH:(n + 1) * TH, :], NT)
                side.done(step, res)
                quarters.append(res)
        res = jnp.concatenate(
            [jnp.concatenate([quarters[0], quarters[2]], axis=1),
             jnp.concatenate([quarters[1], quarters[3]], axis=1)], axis=0)
        sl = [res[8 * i:8 * i + 8, :] for i in range(res.shape[0] // 8)]
        return sl[c % 2:31 + c % 2]

    def proj_unit(side, step0, j, b, xs, lead=None, plain=None):
        r1 = 64 * b + (64 if j == 2 or b < 3 else 56)
        assert made >= ({("vt", 8 * b + q) for q in range(8)} if plain is not None else
                        {("ws", j, k) for k in range(8 * b, r1 // 8)})
        if plain is not None:
            out = []
            for q in range(2):
                row = []
                for n in range(2):
                    steps = range((0, 2, 4, 5)[2 * q + n], (2, 4, 5, 7)[2 * q + n])
                    deps = [d for i in steps for d in side.deps.pop(step0 + i, [])]
                    w = _gate(wt_v[2][256 * q + 64 * b:256 * q + r1, :], side.never, deps)
                    res = _dot(_unpack(w), plain[n * TH:(n + 1) * TH, :], NT)
                    for i in steps:
                        side.done(step0 + i, res)
                    row.append(res)
                out.append(jnp.concatenate(row, axis=1))
            return out

        def product(i):
            off = 256 if j == 2 else 248
            w = (wt_v[j][off + 64 * b:off + r1, HK:] if i == 1 else wt_v[j][64 * b:r1, :HK] if i == 3
                 else ws_v[j][64 * b:r1, i * HK:(i + 1) * HK])
            w = _unpack(side.gate(step0 + i, w))
            if lead is not None and i == 0:
                res = _dot(w, _unpack(view(lead_v, lead, HK // 2)[...]), NN)
            else:
                res = _dot(w, xs[:, i * HK:(i + 1) * HK], NT)
            side.done(step0 + i, res)
            return res
        return [jnp.concatenate(row, axis=1) for row in _strassen(product)]

    def feat_stage(side, step0, j, xs, pair_fn, lead=None, units=range(4), sl=None, hold=None):
        sl = sl or [[], []]
        for b in units:
            for q, res in enumerate(proj_unit(side, step0 + 7 * b, j, b, xs, lead if b == units[0] else None)):
                sl[q] += [res[8 * i:8 * i + 8, :] for i in range(res.shape[0] // 8)]
            for q in (1, 0):
                for jj in (2 * (b % 2), 2 * (b % 2) + 1):
                    if b != hold:
                        pair_fn(_pair_logits(sl[q][31 * (b // 2):], jj), 8 * q + 4 * (b // 2) + jj)
        return sl

    def v_stage(side, xs, slot, first, publish, lead, plain=None):
        pending = None
        for g in range(4):
            if pending is not None:
                side.hooks.setdefault(7 * g + D_LAG, []).append(lambda p=pending: kv_update(*p))
            pending = (proj_unit(side, 7 * g, 2, g, xs, lead if g == 0 else None, plain if g < PLAIN_V0 else None),
                       slot, g, first, publish)
        side.check()
        return pending

    def pack_rows(src, dst, r0, c0, cols, never, a):
        for c in range(c0, c0 + cols, PACK_W):
            if c > c0:
                a = yield GAP_PACK
            w = min(PACK_W, c0 + cols - c)
            v = src[r0:r0 + 16, c:c + w].astype(F32)
            v = jnp.concatenate([jnp.where(never, _lane_tile(a, w // 128), v[0:8, :]), v[8:16, :]], axis=0)
            dst[r0 // 2:r0 // 2 + 8, c:c + w] = _pack(v.astype(BF16))

    def stash_at(i, k, n):
        return zb_v.at[4 * i + 2 * (k // 16) + n, pl.ds(8 * (k % 16), 8), :]

    def stash(i, sl):
        for k, v in enumerate(sl):
            for n in range(2):
                stash_at(i, k, n)[...] = v[:, 128 * n:128 * n + 128]

    def stashed_k(i, slot, c):
        def job(k, a):
            j, n = k // 2, k % 2
            p = _pair_logits([stash_at(i, q, n)[...] for q in range(16 if j < 2 else 31)], j)
            k_pair([_after(p[0], never0, a)] + p[1:], slot, c * PPC + j, 128 * n, never0)
        return job

    def first_rows(k0, k1, n):
        xn = _unpack(xn_v[n * TH // 2:(n + 1) * TH // 2, :])
        ks = [k for k in range(k0, k1)]
        w = jnp.concatenate([wt_v[1][4 * (k % 32):4 * (k % 32) + 8, :] for k in ks[::2]], axis=0)
        res = _dot(_unpack(w), xn, NT)
        for q, k in enumerate(ks):
            if k % 32 < 31:
                stash_at(0, k % 32, n)[...] = res[8 * q:8 * q + 8, :]

    k0_copy(0).wait()
    x_copy(0).wait()
    wphi_copy(2).start()
    x_copy(5).start()
    w_copy(1, 1).start()
    wphi_copy(3).start()
    x_copy(2).start()
    p0, p1 = fold_pairs(1, 0, 0)
    wt_v[1][8:64, :] = packed(p0[1:] + p1[1:])
    h_v[0][0:8, :] = p0[0]
    h_v[0][8:16, :] = p1[0]
    never0 = now(ln_rows(0, 0, TH, plain=True))[0, 0] < 0.0
    first_rows(2, 16, 0)

    k0_copy(1).wait()
    x_copy(1).wait()
    wphi_copy(1).wait()
    w_copy(1, 3).start()
    for c in (0, 2, 1, 3):
        w_copy(2, c).start()
    p2, p3 = fold_pairs(1, 0, 1)
    wt_v[1][0:8, :] = packed([share(h_v[0][0:8, :], p3[0], 1), share(h_v[0][8:16, :], p3[0], 2)])
    wt_v[1][64:128, :] = packed([share(p2[0], p3[0], 3)] + p2[1:] + p3[1:] + [jnp.zeros((8, D), F32)])
    made.add(("fold", 1, 0))
    now(ln_rows(0, 1, TH, plain=True))
    first_rows(16, 34, 0)
    first_rows(0, 16, 1)
    first_rows(16, 32, 1)
    expand_wphi(2)

    def slow(end):
        return lambda rel, gap: min(rel + (gap / 2 if 3 <= rel < 7 else gap), end)

    for c, prev in ((2, 0), (1, 2)):
        w_copy(1, c).wait()
        wphi_copy(4 - c).wait()
        side = _Side(never0, slow(7))
        if c == 1:
            x_copy(5).wait()
            side.add(PRO_LN_PLANS0, lambda k, a: ln_rows(1, k, LNC, never0, a))
        expand_wphi(5 - 2 * c)
        side.add((PRO_W_PLANS0, PRO_W_PLANS1)[2 - c], w_blocks(1, (2 - c) * len(PRO_W_PLANS0)))
        side.add((PRO_K_PLANS0, PRO_K_PLANS1)[2 - c], stashed_k(prev, 0, prev))
        fold(1, c, side, 0)
        stash(c, proj_feat(side, 4, c, xn_tile(0)))
        side.check()

    x_copy(2).wait()
    w_copy(1, 3).wait()
    x_copy(3).start()
    w_copy(0, 0).start()
    wo_copy(0).start()
    x_copy(4).start()
    side = _Side(never0, slow(28))
    side.add(PRO_LN_PLANS1, lambda k, a: ln_rows(1, k + 8, LNC, never0, a))
    side.add(PRO_W_PLANS2, w_blocks(1, 31 - len(PRO_W_PLANS2)))
    side.add(PRO_K_PLANS2, stashed_k(1, 0, 1))
    side.add(PRO_X0_PLAN, late_x_blocks(0))
    fold(1, 3, side, 0)
    stash(3, proj_feat(side, 4, 3, xn_tile(0)))
    k1 = lambda p, pr: k_pair(p, 1, pr, 0, never0)
    for q, sl in enumerate(feat_stage(side, 8, 1, xs_tile(1), k1, units=range(3), hold=2)):
        stash(2 * q, sl[31:])
    side.check()
    save_lead(1)

    for c in range(NC):
        w_copy(2, c).wait()
    side = _Side(never0, lambda rel, gap: min(rel + gap, 27))
    side.add(PRO_V_PLANS[0], v_transpose)
    side.add(PRO_V_PLANS[1], stashed_k(3, 0, 3))
    side.add(PRO_V_PLANS[2], stashed_k(0, 1, 1))
    side.add(PRO_V_PLANS[3], stashed_k(2, 1, 3))
    side.add(PRO_V_PLANS[4], w_blocks(2))
    sl = [[None] * 31 + [jnp.concatenate([stash_at(2 * q, k, n)[...] for n in range(2)], axis=1) for k in range(17)]
          for q in range(2)]
    feat_stage(side, -28, 1, xs_tile(1), k1, 1, units=range(3, 4), sl=sl)
    kv_update(*v_stage(side, xs_tile(0), 0, True, False, None, xn_tile(0)))
    save_lead(0)
    for c in range(1, NC):
        w_copy(0, c).start()
    wo_copy(1).start()
    wr_copy.start()
    for i in range(4):
        stage_copy(i, 0).start()
    wg_copy.start()
    wu_copy.start()
    wd_copy.start()
    for r0 in (0, 248):
        wt_v[0][r0:r0 + 8, :] = jnp.zeros((8, D), U32)

    def phase1(u, carry):
        never = u < 0

        @pl.when(u == 0)
        def _():
            x_copy(3).wait()
            w_copy(0, 0).wait()
            wo_copy(0).wait()

        @pl.when(u == 1)
        def _():
            x_copy(4).wait()
            w_copy(0, 1).wait()
            w_copy(0, 2).wait()
            wo_copy(1).wait()

        def wo_blocks(k0):
            def job(k, a):
                k += k0
                r, c, part = k // 4, 128 * (k // 2 % 2), k % 2
                r0 = u * ((QK - WO_ROWS) // 2)
                dst = wos_v.at[pl.ds(pl.multiple_of(r0 // 2, 8), WO_ROWS // 2), :]

                def piece(kq, nq):
                    src = woraw_v.at[kq, pl.ds(pl.multiple_of(r0, 16), WO_ROWS), :]
                    return src[16 * r:16 * r + 16, nq * QK + c:nq * QK + c + 128].astype(F32)
                outer = [_strassen_rhs(piece(ki, ni), piece(ki, 2 + ni), piece(2 + ki, ni), piece(2 + ki, 2 + ni))
                         for ki in range(2) for ni in range(2)]
                for i in range(4) if part == 0 else range(4, 7):
                    if i % 4:
                        a = yield GAP_WO
                    yield from put_blocks(dst, 8 * r, _strassen_rhs, *[o[i] for o in outer], never, a,
                                          base=7 * i * QK + c, pitch=QK)
            return job

        xs = xs_tile(2 * u + 1)
        side = _Side(never, lambda rel, gap: min(rel + gap, 27))
        for i in range(2):
            t = 2 * u + 2 + i
            if i == 0:
                side.add(LN1_PLANS[0], lambda k, a: ln_rows(2 * u + 2, k, LNC, never, a))
                side.add(WO_PLANS[0], wo_blocks(0))
            pending = v_stage(side, xs, 1 - i, False, False, t - 1 if i == 0 else None)
            xs = xs_tile(t)
            side = _Side(never, lambda rel, gap, end=(27, -1)[i]: min(rel + gap, end))
            if i == 0:
                side.add(LN1_PLANS[1], lambda k, a: ln_rows(2 * u + 3, k, LNC, never, a))
                side.add(WO_PLANS[1], wo_blocks(len(WO_PLANS[0])))
            else:
                side.add(WO_PLANS[2], wo_blocks(24 - len(WO_PLANS[2])))
            side.hooks[-28 + D_LAG] = [lambda p=pending: kv_update(*p)]
            feat_stage(side, -28, 1, xs, lambda p, pr: k_pair(p, i, pr, 0, never if i == 1 else None))
            save_lead(t)
        side.check()
        fold(0, u)
        return carry

    lax.fori_loop(0, (NT_ - 2) // 2, phase1, 0)

    w_copy(0, 3).wait()
    wr_copy.wait()
    side = _Side(never0, lambda rel, gap: min(rel + gap, 27 if rel < 98 else 103))

    def z_final(k, a):
        zb_v[k] = jnp.broadcast_to(_row_sum(_after(z_v[k], never0, a)), (128, 128))

    side.add(END_PLANS[0], z_final)
    side.add(END_PLANS[1], w_blocks(0))
    side.hooks[0] = [lambda: fold(0, 3, side, 100)]
    kv_update(*v_stage(side, xs_tile(NT_ - 1), 1, False, True, NT_ - 1))
    wr_v[...] = jnp.broadcast_to(wrraw_v[...].reshape(1, D).astype(F32), (8, D))

    def o_copy(r0, n, i):
        return pltpu.make_async_copy(o_v.at[pl.ds(r0, n), :], out_hbm.at[pl.ds(r0, n), :], sem.at[SO + i])

    def finish_rows(h_ref, k, t, valid, st, never=None, anchor=None):
        r0 = t * T + k * LNC
        rows = slice(k * LNC, (k + 1) * LNC)
        m = jnp.broadcast_to(_row_sum(_after(h_ref[rows, :], never, anchor)) * (1.0 / D), (LNC, 128))
        rstd, r = [], []
        for i in range(LNC // 8):
            anchor = yield LN2_GAPS[2] if i else LN2_GAPS[0]
            mi = _after(m[8 * i:8 * i + 8, :], never, anchor)
            hc = h_ref[k * LNC + 8 * i:k * LNC + 8 * i + 8, :] - _lane_tile(mi, D // 128)
            rs = lax.rsqrt(_row_sum(hc * hc) * (1.0 / D) + LN_EPS)
            r.append((_row_sum(hc * wr_v[...]) * rs + 0.0).astype(BF16).astype(F32))
            rstd.append(jnp.broadcast_to(rs, (8, 128)))
        rstd = jnp.concatenate(rstd, axis=0)
        w = D if never is None else D // LN2_SPLIT
        for c in range(0, D, w):
            anchor = yield LN2_GAPS[2] if c else LN2_GAPS[1]
            h = h_ref[rows, c:c + w]
            hn = (h - _lane_tile(_after(m, never, anchor), w // 128)) * _lane_tile(rstd, w // 128)
            view(hn_v, t, T // 2)[k * LNC // 2:(k + 1) * LNC // 2, c:c + w] = _pack(hn.astype(BF16))
            view(o_v, t, T)[rows, c:c + w] = (hn + h).astype(BF16)
        best = st["route"]
        sub = lax.broadcasted_iota(jnp.int32, (8, 128), 0)
        for i, ri in enumerate(r):
            key = _ordered(pltpu.bitcast(jnp.broadcast_to(ri, (8, 128)), jnp.int32)) | ((S - 1 - r0 - 8 * i) - sub)
            if valid is not None:
                key = jnp.where(valid, key, KEY_MIN)
            best = jnp.maximum(best, key)
        st["route"] = best
        return pltpu.bitcast(best, F32)

    def q_pair(p, slot, pr):
        ep, en, sp, sn = _dual_exp(p)
        zz = [_lane_tile(zb_v[pr, 8 * i:8 * i + 8, :], T // 128) for i in range(16)]
        ap = _pair_allreduce(_tree(jnp.add, [ep[i] * zz[i] for i in range(8)]), jnp.add)
        an = _pair_allreduce(_tree(jnp.add, [en[i] * zz[8 + i] for i in range(8)]), jnp.add)
        inv = _recip(ap * sn + (an + 1e-6 * sn) * sp)
        rp = sn * inv
        rn = sp * inv
        phi = jnp.concatenate([e * rp for e in ep] + [e * rn for e in en], axis=0)
        phi_v[slot][64 * pr:64 * pr + 64, :] = _pack(phi.astype(BF16))

    held = []

    def attn_blocks(slot, g, deps):
        res = [_dot(_unpack(kvbf_v[32 * pr:32 * pr + 32, :]), _unpack(phi_v[slot][64 * pr:64 * pr + 64, :]), NN)
               for pr in (2 * g, 2 * g + 8, 2 * g + 1, 2 * g + 9)]
        lo, hi = jnp.concatenate(res[0::2], axis=0), jnp.concatenate(res[1::2], axis=0)
        blocks = [(i, g, b) for i, b in enumerate(_strassen_lhs(lo[:, :TH], hi[:, :TH], lo[:, TH:], hi[:, TH:]))]
        if g % 2 == 0:
            held.append(blocks.pop())
        else:
            blocks.append(held.pop())
        ot = _pack(jnp.concatenate([b for _, _, b in blocks], axis=1).astype(BF16).T)
        for q, (i, n, _) in enumerate(blocks):
            oc_v[slot][:, i * HK + 128 * n:i * HK + 128 * n + 128] = ot[q * TH // 2:(q + 1) * TH // 2, :]
            made.add(("oc", slot, i, n))
            if q % 2:
                deps.append(pltpu.bitcast(ot[(q + 1) * TH // 2 - 8:(q + 1) * TH // 2, :], F32))

    def o_blocks(slot, c, never):
        def job(k, a):
            k = (2, 3, 1, 4, 5, 0, 6)[k]
            assert made >= {("oc", slot, k, c), ("oc", slot, k, c + 2)}
            for r in range(4):
                if r:
                    a = yield GAP_O2
                m = [rows16(oc_v[slot], 8 * r + 32 * q, k * HK + n * QK + 128 * c, 128)
                     for q in range(2) for n in range(2)]
                yield from put_blocks(oc2_v[slot], 8 * r, _strassen_lhs, *m, never, a, skip=(1, 3),
                                      base=7 * k * QK + 128 * c, pitch=QK)
            made.add(("oc2", slot, k, c))
        return job

    def out_proj(side, step0, t, slot):
        count = [0]

        def inner(i, c):
            assert made >= {("oc2", slot, i, 0), ("oc2", slot, i, 1)}

            def product(j):
                step, odd = step0 + count[0] // 2, count[0] % 2
                count[0] += 1
                o = (oc_v[slot][32:64, i * HK + QK:(i + 1) * HK] if j == 1 else
                     oc_v[slot][0:32, i * HK:i * HK + QK] if j == 3 else
                     oc2_v[slot][:, (7 * i + j) * QK:(7 * i + j + 1) * QK])
                w = wos_v[:, (7 * i + j) * QK + 128 * c:(7 * i + j) * QK + 128 * c + 128]
                res = _dot(_unpack(o), _unpack(w if odd else side.gate(step, w)), NN)
                if odd:
                    side.done(step, res)
                return res
            return _block(_strassen(product))

        xt = view(x_v, t, T)

        def emit(cs, q, r, res):
            for k, c in enumerate(cs):
                for n in range(2):
                    rows, c0 = slice(q * TH, (q + 1) * TH), r * HK + n * QK + 128 * c
                    h_v[slot][rows, c0:c0 + 128] = (res[:, 256 * k + 128 * n:256 * k + 128 * n + 128]
                                                    + xt[rows, c0:c0 + 128].astype(F32))
                made.add(("h", slot, q, r, c))

        for cs in ((0,), (1,)) if OUT_ORDER == 0 else ((0, 1),):
            _strassen_rows_first(lambda i: jnp.concatenate([inner(i, c) for c in cs], axis=1),
                                 lambda q, r, res: emit(cs, q, r, res))

    def phase2(u, carry):
        for i in range(4):
            stage_copy(i, u).wait()
        never = u < 0
        side = _Side(never, lambda rel, gap: min(rel + 2 * gap, 97) if rel < 98 else
                     rel + gap if rel + gap <= 155 else 2 * (rel + gap - 155) - 1)
        st = {"route": carry}
        tp = jnp.maximum(2 * u - 1, 0)
        early = len(LN2_PLANS[2])
        order = []

        def ln2(slot, t, valid, k0, key):
            def job(k, a):
                k += k0
                hs = {("h", slot, k // 8, r, c) for r in range(2) for c in range(2)}
                assert made >= hs or key == 0
                best = yield from finish_rows(h_v[slot], k, t, valid, st, never, a)
                assert key > 0 or not made & hs
                order.append((key, k))
                assert order == sorted(order)
                return best
            return job

        side.add(LN2_PLANS[0], ln2(1, tp, u > 0, early, 0))
        side.add(LN2_PLANS[1], ln2(0, 2 * u, None, 0, 1))
        side.add(LN2_PLANS[2], ln2(1, 2 * u + 1, None, 0, 2))

        def packer(i, dst, n):
            left = [n]

            def job(k, a):
                if i < 2:
                    yield from pack_rows(stage_v[i], dst, (k // 2) * 16, (0, D)[k % 2], (D, FM - D)[k % 2], never, a)
                else:
                    yield from pack_rows(stage_v[i], dst, k * 16, 0, D, never, a)
                left[0] -= 1
                if not left[0]:
                    stage_copy(i, jnp.minimum(u + 1, NQ - 1)).start()
                    n0 = stage_v[i].shape[0] - 16
                    side.deps.setdefault(PACK_DUE[i], []).append(stage_v[i][n0:n0 + 8, 0:128].astype(F32))
            return job

        for i in range(2):
            side.add(PACK_PLANS[i], packer(i, view((wgp_v, wup_v)[i], u, D // NQ // 2), len(PACK_PLANS[i])))
            d0 = pl.multiple_of(u * (DQ // 2) + i * (DQA // 2), 8)
            side.add(PACKD_PLANS[i], packer(2 + i, wdp_v.at[pl.ds(d0, 8 * len(PACKD_PLANS[i])), :],
                                            len(PACKD_PLANS[i])))
            for g in range(4):
                step = 107 + 28 * i + 7 * g + G_LAG
                wrap = lambda x: x if x < 156 else 2 * (x - 156) + 1
                side.hooks.setdefault(wrap(step), []).append(
                    lambda i=i, g=g, due=wrap(step + O_DUE): attn_blocks(i, g, side.deps.setdefault(due, [])))
            for c in range(2):
                side.add(O2_PLANS[2 * i + c], o_blocks(i, c, never))
        for i in range(2):
            feat_stage(side, 100 + 28 * i, 0, xs_tile(2 * u + i), lambda p, pr: q_pair(p, i, pr),
                       2 * u if i == 0 else None)
        for i in range(2):
            out_proj(side, 49 * i, 2 * u + i, i)
        side.check()

        @pl.when(u == 0)
        def _():
            o_copy(0, T, 0).start()

        @pl.when(u > 0)
        def _():
            o_copy(pl.multiple_of(tp * T, T), 2 * T, u).start()

        return st["route"]

    wg_copy.wait()
    wu_copy.wait()
    wd_copy.wait()
    route = lax.fori_loop(
        0, NT_ // 2, phase2,
        jnp.full((8, 128), KEY_MIN, jnp.int32))
    st = {"route": route}
    for k in range(len(LN2_PLANS[2]), T // LNC):
        now(finish_rows(h_v[1], k, NT_ - 1, None, st))
    o_copy(S - T, T, NT_).start()

    best = st["route"]
    for shift in (4, 2, 1):
        best = jnp.maximum(best, pltpu.roll(best, shift, 0))
    idx_s = (S - 1) - (best[0, 0] & (S - 1))
    gate = _lane_tile(jax.nn.sigmoid(pltpu.bitcast(_ordered(best & -65536), F32)), D // 128)
    blk = pl.multiple_of((idx_s >> 4) << 4, 16)
    pair = jnp.broadcast_to(hn_v[pl.ds(idx_s >> 1, 1), :], (8, D))
    x8 = pltpu.bitcast(jnp.where((idx_s & 1) == 1, pair & jnp.uint32(0xFFFF0000), pair << 16), F32)
    xs = jnp.concatenate([x8, x8], axis=0).astype(BF16)
    acts, anchors = [], []

    def park(v, half):
        n = v.shape[0] // 128
        for i in range(n):
            z_v[i, :, 128 * half:128 * half + 128] = v[128 * i:128 * i + 128, :]
        return jnp.concatenate([z_v[i, :, 128 * half:128 * half + 128] for i in range(n)], axis=0)

    for c0 in range(0, FM, 128):
        g = _dot(xs, _unpack(wgp_v[:, c0:c0 + 128]), NN)[0:8, :]
        u = _dot(xs, _unpack(wup_v[:, c0:c0 + 128]), NN)[0:8, :]
        anchors += [g, u]
        acts.append(g * jax.nn.sigmoid(g) * u)
    xb = park(_col_broadcast(x8), 0)
    g, u = [_sublane_allreduce(_vpu_matvec(
        xb, lambda g: w[8 * g:8 * g + 8, :].astype(F32), never0,
        anchors[i * MOE_NA // 2:(i + 1) * MOE_NA // 2], MOE_LAGS[0])) for i, w in enumerate((wg_v, wu_v))]
    acts.append(g * jax.nn.sigmoid(g) * u)
    a = jnp.concatenate(acts, axis=1)
    am = jnp.concatenate([a[:, FVD:], a[:, FVD:]], axis=0).astype(BF16)
    ys, anchors = [], anchors[MOE_NA:]
    for k0 in range(0, FF - FVD, 512):
        k1 = min(k0 + 512, FF - FVD)
        yk = _dot(am[:, k0:k1], _unpack(wdp_v[k0 // 2:k1 // 2, 0:D]), NN)[0:8, :]
        ys.append(yk)
        anchors += [yk[:, c:c + 128] for c in range(128, D, 256)]
    ys.append(_sublane_allreduce(_vpu_matvec(
        park(_col_broadcast(a[:, :FVD]), 1), lambda g: wd_v[8 * g:8 * g + 8, :].astype(F32), never0,
        anchors[:-MOE_ND], MOE_LAGS[1])))
    y = _tree(jnp.add, ys) * gate
    y = jnp.concatenate([y, y], axis=0)
    sel = lax.broadcasted_iota(jnp.int32, (16, 1), 0) == (idx_s - blk)
    patch_v[...] = (o_v[pl.ds(blk, 16), :].astype(F32) + jnp.where(sel, y, 0.0)).astype(BF16)
    o_copy(0, T, 0).wait()
    for u in range(1, NT_ // 2):
        o_copy((2 * u - 1) * T, 2 * T, u).wait()
    o_copy(S - T, T, NT_).wait()
    pc = pltpu.make_async_copy(patch_v, out_hbm.at[pl.ds(blk, 16), :], sem.at[SM + 3])
    pc.start()
    for i in range(4):
        stage_copy(i, NQ - 1).wait()
    pc.wait()


@jax.jit
def pallas_sequential_preLN__linear_kernel_hedgehog__moe_arch_mod__prompt_kernel(
    A_x: jax.Array,
    A_wqkv: jax.Array,
    A_w_phi: jax.Array,
    A_wo: jax.Array,
    B_x: jax.Array,
    B_w_r: jax.Array,
    B_w_gate: jax.Array,
    B_w_up: jax.Array,
    B_w_down: jax.Array,
):
    del B_x
    hbm = pl.BlockSpec(memory_space=pl.ANY)
    out = pl.pallas_call(
        _kernel,
        out_shape=jax.ShapeDtypeStruct((S, D), BF16),
        in_specs=[hbm] * 8,
        out_specs=hbm,
        scratch_shapes=[
            pltpu.VMEM((S, D), BF16),
            pltpu.VMEM(((T + TH) // 2, D), U32),
            pltpu.VMEM((NT_ * TH // 2, SW), U32),
            pltpu.VMEM((NT_ * HK // 2, 128), U32),
            pltpu.VMEM((3 * NC, D, RC), BF16),
            [pltpu.VMEM((D // 2, D), U32)] * 3,
            [pltpu.VMEM((HK // 2, 7 * HK), U32)] * 3,
            pltpu.VMEM((H, DH, DH), BF16),
            pltpu.VMEM((8 * 64, 128), U32),
            pltpu.VMEM((4, QK, D), BF16),
            pltpu.VMEM((QK // 2, 49 * QK + 128), U32),
            pltpu.VMEM((D,), BF16),
            pltpu.VMEM((8, D), F32),
            pltpu.VMEM((NPAIR, 64, 128), F32),
            pltpu.VMEM((NPAIR * 32, 128), U32),
            pltpu.VMEM((NPAIR, 128, T), F32),
            pltpu.VMEM((NPAIR, 128, 128), F32),
            [pltpu.VMEM((NPAIR * 64, T), U32)] * 2,
            [pltpu.VMEM((TH // 2, 7 * HK), U32)] * 2,
            [pltpu.VMEM((TH // 4, 49 * QK), U32)] * 2,
            [pltpu.VMEM((T, D), F32)] * 2,
            pltpu.VMEM((S // 2, D), U32),
            pltpu.VMEM((S, D), BF16),
            pltpu.VMEM((D, FV), BF16),
            pltpu.VMEM((D, FV), BF16),
            pltpu.VMEM((FVD, D), BF16),
            [pltpu.VMEM((D // NQ + 16, FM), BF16), pltpu.VMEM((D // NQ + 16, FM), BF16),
             pltpu.VMEM((DQA + 16, D), BF16), pltpu.VMEM((DQ - DQA + 16, D), BF16)],
            pltpu.VMEM((D // 2, FM), U32),
            pltpu.VMEM((D // 2, FM), U32),
            pltpu.VMEM(((FF - FVD) // 2, D + 128), U32),
            pltpu.VMEM((16, D), BF16),
            pltpu.SemaphoreType.DMA((6 + 3 * NC + NT_ + 17,)),
        ],
        compiler_params=pltpu.CompilerParams(vmem_limit_bytes=100 * 1024 * 1024,
                                             disable_semaphore_checks=True, disable_bounds_checks=True),
        name="hedgehog_mod",
    )(
        A_x.reshape(S, D),
        A_wqkv,
        A_w_phi,
        A_wo.reshape(4, QK, D),
        B_w_r,
        B_w_gate,
        B_w_up,
        B_w_down,
    )
    return out.reshape(1, S, D)
```

```python
import math

import jax
import jax.numpy as jnp
from jax import lax
import jax.experimental.pallas as pl
import jax.experimental.pallas.tpu as pltpu

F32 = jnp.float32
BF16 = jnp.bfloat16
U32 = jnp.uint32

S = 2048
D = 1024
H = 32
DH = 32
FF = 3584
NPAIR = H // 2
LOG2E = 1.4426950408889634
LN_EPS = 1e-5
KEY_MIN = -2 ** 31

T = 256
TH = T // 2
NT_ = S // T
RC = 256
NC = D // RC
PPC = RC // 64
LNC = 16

FV = 10 * 128
FM = FF - FV
FVD = 8 * 128
NQ = NT_ // 2
DQ = (FF - FVD) // NQ
WO_ROWS = 96
QK = D // 4
HK = D // 2
SW = 8 * HK


LN1_PLANS = (((0.095, 7), (0.452, 8), (2.855, 10), (4.2, 11), (5.323, 12), (7.125, 13), (8.42, 16), (9.93,
    16), (11.174, 18), (11.928, 19), (13.877, 22), (15.466, 23), (16.77, 23), (18.221, 25), (19.564, 26),
    (21.5, 27)), ((-1.151, 4), (1.211, 7), (1.804, 8), (3.43, 9), (5.504, 11), (5.924, 14), (8.015, 14),
    (9.695, 17), (10.176, 17), (11.93, 19), (13.665, 19), (15.339, 22), (16.395, 22), (18.546, 25), (19.409,
    26), (21.079, 27)))
PRO_LN_PLANS0 = ((None, 4), (None, 7), (0.12, 5), (0.555, 5), (1.7, 6), (2.168, 6), (3.297, None), (4.239,
    None))
PRO_LN_PLANS1 = ((None, 4), (None, 5), (-0.516, None), (0.246, 6), (1.046, 6), (2.1, 7), (3.001, 7), (3.003,
    6))
PRO_K_PLANS0 = ((0.388, None), (0.863, None), (1.721, None), (2.715, None), (2.982, None), (3.948, None),
    (5.473, None), (5.989, None))
PRO_K_PLANS1 = ((-0.866, None), (0.636, None), (1.962, None), (2.951, None), (3.554, None), (4.106, None),
    (4.699, None), (5.223, None))
PRO_X0_PLAN = ((20.049, None), (21.671, None), (23.071, None), (23.684, None), (25.371, None), (26.097, None),
    (26.566, None), (27.089, None))
PRO_W_PLANS0 = ((3.2, None), (3.488, None), (3.771, None), (4.235, None), (4.92, None), (5.413, None), (6.114,
    None), (6.485, None))
PRO_W_PLANS1 = ((4.846, None), (5.235, None), (6.531, None))
PRO_W_PLANS2 = ((6.626, None), (7.329, None), (8.074, None), (9.011, None), (9.904, None), (10.947, None),
    (12.625, None), (13.232, None), (14.27, None), (15.036, None), (16.142, None), (17.035, None), (18.379,
    None), (19.306, None), (19.316, None), (20.753, None), (21.341, None), (22.294, None), (23.106, None),
    (25.173, None))
PRO_K_PLANS2 = ((21.924, None), (22.415, None), (24.003, None), (24.127, None), (24.582, None), (25.771,
    None), (26.668, None), (27.134, None))
PRO_V_PLANS = (((None, None), (None, None), (None, None), (None, None), (None, None), (None, None), (None,
    None), (None, None), (-4.983, 0), (-4.771, 1), (-4.658, 2), (-3.398, 2), (-3.155, 2), (-2.921, 2),
    (-2.499, 3), (-2.355, 3), (-1.874, 4), (-1.535, 4), (-1.024, 4), (-0.927, 4), (-0.706, 4), (0.24, 6),
    (0.481, 7), (0.668, 6), (1.247, 7), (1.4, 7), (2.688, 9), (2.727, 7), (3.012, 8), (3.087, 9), (4.289, 9),
    (4.924, 10)), ((5.897, None), (7.691, None), (10.048, None), (12.014, None), (13.868, None), (15.456,
    None), (17.412, None), (20.836, None)), ((0.0, None), (1.776, None), (3.418, None), (4.808, None)),
    ((19.45, None), (21.451, None), (22.925, None), (23.333, None)), ((16.059, None), (20.449, None), (20.497,
    None), (21.79, None), (22.449, None), (22.572, None), (25.109, None), (25.686, None), (-0.337, None),
    (-0.164, None), (0.488, None), (2.709, None), (2.857, None), (3.639, None), (4.322, None), (4.918, None),
    (5.207, None), (6.91, None), (7.587, None), (8.953, None), (9.24, None), (10.232, None), (11.175, None),
    (11.993, None), (12.583, None), (13.787, None), (14.312, None), (14.817, None), (16.402, None), (16.81,
    None), (17.304, None), (19.292, None)))
END_PLANS = (((-0.162, None), (2.011, None), (3.829, None), (5.62, None), (6.909, None), (8.156, None),
    (10.634, None), (12.371, None), (13.954, None), (15.538, None), (16.797, None), (19.352, None), (20.737,
    None), (23.183, None), (23.393, None), (25.88, None)), ((100.308, None), (101.389, None), (102.104, None),
    (0.409, None), (1.005, None), (2.198, None), (2.898, None), (4.205, None), (5.131, None), (6.022, None),
    (7.291, None), (7.974, None), (8.425, None), (9.982, None), (11.3, None), (11.768, None), (12.903, None),
    (13.561, None), (14.696, None), (15.687, None), (17.565, None), (18.013, None), (18.596, None), (19.613,
    None), (20.25, None), (21.235, None), (22.366, None), (23.06, None), (24.673, None), (25.256, None),
    (26.011, None)))
WO_PLANS = (((0.245, None), (6.671, None), (13.134, None), (18.635, None), (24.922, None)), ((-26.952, None),
    (-21.248, None), (-16.958, None), (-12.341, None), (-8.3, None), (-2.883, None), (1.607, None), (6.233,
    None), (10.547, None), (15.312, None), (19.974, None), (24.229, None)), ((-27.707, None), (-22.089, None),
    (-18.962, None), (-14.225, None), (-9.98, None), (-6.618, None), (-2.09, None)))
LN2_PLANS = (((-0.5, 12), (1.385, 15), (5.416, 19), (6.544, 21), (11.772, 24), (14.638, 27), (17.452, 29),
    (19.2, 33), (23.964, 36), (26.706, 40), (29.685, 42), (33.006, 46)), ((35.739, 47), (38.936, 51), (41.779,
    54), (45.752, 57), (47.863, 61), (50.474, 62), (53.833, 66), (56.742, 69), (61.708, 72), (62.833, 75),
    (65.713, 78), (68.926, 82), (71.975, 82), (74.997, 86), (78.06, 90), (81.109, 92)), ((84.217, None),
    (87.649, None), (89.543, None), (90.236, None)))
O2_PLANS = (((131.357, None), (134.449, None), (137.05, None), (137.656, None), (138.539, None), (140.057,
    None), (144.16, None)), ((141.38, None), (145.789, None), (145.843, None), (146.882, None), (149.928,
    None), (152.324, None), (153.261, None)), ((12.503, None), (22.336, None), (31.211, None), (39.891, None),
    (47.762, None), (57.333, None), (66.0, None)), ((27.948, None), (36.312, None), (43.877, None), (50.771,
    None), (58.218, None), (67.954, None), (76.139, None)))
PACK_PLANS = (((100.502, None), (101.244, None), (102.208, None), (102.296, None), (103.427, None), (104.874,
    None), (105.862, None), (106.631, None), (107.838, None), (108.106, None), (109.264, None), (109.501,
    None), (110.296, None), (111.052, None), (111.166, None), (111.529, None), (114.039, None), (114.221,
    None), (115.251, None), (116.905, None), (117.839, None), (118.037, None), (118.466, None), (118.897,
    None), (121.059, None), (121.33, None), (121.354, None), (122.756, None), (123.403, None), (124.242,
    None), (124.673, None), (125.882, None)), ((128.281, None), (128.956, None), (131.04, None), (131.514,
    None), (131.968, None), (132.242, None), (132.835, None), (133.941, None), (135.423, None), (136.25,
    None), (136.936, None), (137.657, None), (138.836, None), (139.06, None), (140.343, None), (141.492,
    None), (142.08, None), (142.473, None), (143.694, None), (143.8, None), (144.137, None), (146.083, None),
    (146.911, None), (147.792, None), (148.441, None), (149.019, None), (149.771, None), (150.598, None),
    (151.737, None), (152.598, None), (153.829, None), (154.519, None)))
PACKD_PLANS = (((1.12, None), (1.633, None), (4.36, None), (5.329, None), (7.571, None), (9.451, None),
    (9.782, None), (11.103, None), (12.795, None), (14.02, None), (14.575, None), (15.831, None), (19.475,
    None), (20.868, None), (21.935, None), (22.323, None), (25.31, None), (26.102, None), (28.561, None),
    (30.197, None), (31.978, None), (33.481, None)), ((35.02, None), (36.791, None), (38.947, None), (39.775,
    None), (42.179, None), (42.661, None), (46.568, None), (46.704, None), (49.436, None), (51.509, None),
    (51.641, None), (52.889, None), (53.189, None), (55.672, None), (56.222, None), (58.458, None), (59.773,
    None), (60, None)))
PACK_DUE = (130, 5, 39, 64)
DQA = 16 * len(PACKD_PLANS[0])
G_LAG = 5
D_LAG = 1
PLAIN_V0 = 1
LN2_GAPS = (1.13, 1.5, 0.2)
LN2_SPLIT = 4
PACK_W = 512
GAP_PACK = 0.2
LN1_GAPS = (1, 1.25)
GAP_PRO = 0.13
GAP_X = 0.2
GAP_WO = 0.2
GAP_O2 = 0.26
O_DUE = 6
MOE_NA = 36
MOE_ND = 2
MOE_LAGS = (2, 2)
STAGGER = 8

NN = (((1,), (0,)), ((), ()))
NT = (((1,), (1,)), ((), ()))


def _dot(a, b, dims):
    return lax.dot_general(a, b, dims, preferred_element_type=F32)


def _recip(x):
    return pl.reciprocal(x, approx=False, full_range=False)


def _pack(x):
    return pltpu.bitcast(x, U32)


def _unpack(x):
    return pltpu.bitcast(x, BF16)


def _strassen_lhs(a11, a12, a21, a22):
    return [a21 + a22, a22, a11 + a12, a11, a11 + a22, a12 - a22, a21 - a11]


def _strassen_rhs(b11, b12, b21, b22):
    return [b11, b21 - b11, b22, b12 - b22, b11 + b22, b21 + b22, b11 + b12]


def _strassen(product):
    m2 = product(0)
    m4 = product(1)
    c21 = m2 + m4
    m5 = product(2)
    u11 = m4 - m5
    m3 = product(3)
    c12 = m3 + m5
    u22 = m3 - m2
    m1 = product(4)
    u11 = u11 + m1
    u22 = u22 + m1
    c11 = product(5) + u11
    c22 = product(6) + u22
    return [[c11, c12], [c21, c22]]


def _strassen_rows_first(product, emit):
    m5 = product(2)
    m3 = product(3)
    emit(0, 1, m3 + m5)
    m4 = product(1)
    u11 = m4 - m5
    m1 = product(4)
    u11 = u11 + m1
    u22 = m3 + m1
    emit(0, 0, product(5) + u11)
    m2 = product(0)
    emit(1, 0, m2 + m4)
    u22 = u22 - m2
    emit(1, 1, product(6) + u22)


def _ordered(bits):
    return bits ^ ((bits >> 31) & 0x7FFF0000)


def _block(rows):
    return jnp.concatenate([jnp.concatenate(r, axis=1) for r in rows], axis=0)


def _pair_allreduce(a, op):
    a = op(a, pltpu.roll(a, 2, 0))
    return op(a, pltpu.roll(a, 4, 0))


def _tree(op, xs):
    xs = list(xs)
    while len(xs) > 1:
        nxt = [op(xs[i], xs[i + 1]) for i in range(0, len(xs) - 1, 2)]
        if len(xs) % 2:
            nxt.append(xs[-1])
        xs = nxt
    return xs[0]


def _pair_logits(sl, j):
    sub = lax.broadcasted_iota(jnp.int32, sl[0].shape, 0)
    if j < 3:
        head = jnp.where(sub < 2, 0.0, sl[(0, 1, 16)[j]])
    else:
        head = jnp.where(sub < 2, sl[0], jnp.where(sub < 4, pltpu.roll(sl[1], 2, 0),
                                                   jnp.where(sub < 6, pltpu.roll(sl[16], 4, 0), 0.0)))
    r0 = (2, 9, 17, 24)[j]
    return [head] + list(sl[r0:r0 + 7])


def _dual_exp(sl):
    mx = _pair_allreduce(_tree(jnp.maximum, sl), jnp.maximum)
    mn = _pair_allreduce(_tree(jnp.minimum, sl), jnp.minimum)
    ep = [jnp.exp2(s - mx) for s in sl]
    en = [jnp.exp2(mn - s) for s in sl]
    sp = _pair_allreduce(_tree(jnp.add, ep), jnp.add)
    sn = _pair_allreduce(_tree(jnp.add, en), jnp.add)
    return ep, en, sp, sn


def _after(x, never, anchor):
    if anchor is None:
        return x
    d = jnp.concatenate([anchor] * (x.shape[0] // 8), axis=0)
    if x.shape[1] == 128:
        return jnp.where(never, d, x)
    return jnp.concatenate([jnp.where(never, d, x[:, :128]), x[:, 128:]], axis=1)


def _gate(x, never, deps):
    for i, dep in enumerate(deps):
        d = jnp.broadcast_to(dep, (8, 128))
        if x.dtype != F32:
            d = pltpu.bitcast(d, x.dtype)
        blk = jnp.where(never, d, x[8 * i:8 * i + 8, :128])
        if x.shape[1] > 128:
            blk = jnp.concatenate([blk, x[8 * i:8 * i + 8, 128:]], axis=1)
        parts = ([x[:8 * i, :]] if i else []) + [blk, x[8 * i + 8:, :]]
        x = jnp.concatenate(parts, axis=0)
    return x


def _lane_fold(a):
    return _tree(jnp.add, [a[:, 128 * i:128 * i + 128] for i in range(a.shape[1] // 128)])


def _row_sum(a):
    return jnp.sum(_lane_fold(a), axis=-1, keepdims=True)


def _lane_tile(a, n):
    return a if n == 1 else jnp.concatenate([a] * n, axis=1)


def _sublane_allreduce(a):
    a = a + pltpu.roll(a, 4, 0)
    a = a + pltpu.roll(a, 2, 0)
    return a + pltpu.roll(a, 1, 0)


def _col_broadcast(row8):
    return jnp.concatenate([row8] * 16, axis=0).astype(BF16).T.astype(F32)


def _vpu_matvec(xb, w_rows, never, anchors, lag):
    ng = xb.shape[0] // 8
    acc, hist = None, []
    for g in range(ng):
        dep = anchors[(g * len(anchors)) // ng]
        if g >= lag:
            dep = dep + hist[g - lag]
        x = jnp.where(never, dep, xb[8 * g:8 * g + 8, :])
        w = w_rows(g)
        t = w * _lane_tile(x, w.shape[1] // 128)
        acc = t if acc is None else acc + t
        c = 128 * (g % (w.shape[1] // 128))
        hist.append(acc[:, c:c + 128])
    return acc


class _Side:
    def __init__(self, never, later=lambda rel, gap: rel + gap):
        self.never = never
        self.later = later
        self.jobs = []
        self.deps = {}
        self.hooks = {}

    def add(self, plan, fn):
        for k, (rel, due) in enumerate(plan):
            if rel is None:
                self._run(None, due, fn, k, None)
            else:
                self.jobs.append((rel, due, fn, k))

    def _run(self, rel, due, fn, k, anchor):
        gen = fn if hasattr(fn, "send") else fn(k, anchor)
        dep = gen
        if hasattr(gen, "send"):
            try:
                while True:
                    gap = gen.send(anchor) if gen is fn or rel is None and dep is None else next(gen)
                    if rel is not None:
                        self.jobs.append((self.later(rel, gap), due, gen, k))
                        return
                    dep = None
            except StopIteration as stop:
                dep = stop.value
        if due is not None:
            self.deps.setdefault(due, []).append(dep)

    def check(self):
        assert not self.jobs and not self.deps and not self.hooks

    def gate(self, step, x):
        return _gate(x, self.never, self.deps.pop(step, []))

    def done(self, step, res):
        m = res.shape[0] // 8
        while True:
            ready = [j for j in self.jobs if step - 1 < j[0] <= step]
            if not ready:
                break
            job = min(ready, key=lambda j: j[0])
            self.jobs.remove(job)
            g = m - 1 - int((step - job[0]) * m)
            self._run(*job, res[8 * g:8 * g + 8, res.shape[1] - 128:])
        for fn in self.hooks.pop(step, []):
            fn()


def _kernel(x_hbm, wqkv_hbm, wphi_hbm, wo_hbm, wr_hbm, wg_hbm, wu_hbm, wd_hbm, out_hbm,
            x_v, xn_v, xs_v, lead_v, wraw_v, wt_v, ws_v, wphi_v, a_v, woraw_v, wos_v, wrraw_v, wr_v,
            kvacc_v, kvbf_v, z_v, zb_v, phi_v, oc_v, oc2_v, h_v, hn_v, o_v, wg_v, wu_v, wd_v, stage_v,
            wgp_v, wup_v, wdp_v, patch_v,
            sem):
    SX, SQ, SO, SM = 0, 6, 6 + 3 * NC, 6 + 3 * NC + NT_ + 1

    def x_copy(i):
        h0, h1 = ((0, 1), (1, 2), (3, 4), (4, 8), (8, 2 * NT_), (2, 3))[i]
        rows = pl.ds(h0 * TH, (h1 - h0) * TH)
        return pltpu.make_async_copy(x_hbm.at[rows, :], x_v.at[rows, :], sem.at[SX + i])

    def k0_copy(s):
        return pltpu.make_async_copy(wqkv_hbm.at[:, pl.ds(D + s * 128, 128)],
                                     wraw_v.at[NC, :, pl.ds(s * 128, 128)], sem.at[(SM + 7, SQ + NC)[s]])

    def w_copy(j, c):
        return pltpu.make_async_copy(wqkv_hbm.at[:, pl.ds(j * D + c * RC, RC)], wraw_v.at[j * NC + c],
                                     sem.at[SQ + j * NC + c])

    def wphi_copy(i):
        h0, h1 = ((0, 8), (16, 24), (8, 16), (24, H))[i]
        return pltpu.make_async_copy(wphi_hbm.at[pl.ds(h0, h1 - h0)], wphi_v.at[pl.ds(h0, h1 - h0)],
                                     sem.at[(SM + 4, SM + 8, SM + 9, SM + 14)[i]])

    wr_copy = pltpu.make_async_copy(wr_hbm, wrraw_v, sem.at[SM + 5])

    def wo_copy(i):
        rows = pl.ds(0, WO_ROWS) if i == 0 else pl.ds(WO_ROWS, QK - WO_ROWS)
        return pltpu.make_async_copy(wo_hbm.at[:, rows, :], woraw_v.at[:, rows, :], sem.at[(SM + 6, SM + 15)[i]])

    wg_copy = pltpu.make_async_copy(wg_hbm.at[:, pl.ds(FM, FV)], wg_v, sem.at[SM + 0])
    wu_copy = pltpu.make_async_copy(wu_hbm.at[:, pl.ds(FM, FV)], wu_v, sem.at[SM + 1])
    wd_copy = pltpu.make_async_copy(wd_hbm.at[pl.ds(0, FVD), :], wd_v, sem.at[SM + 2])

    def stage_copy(i, q):
        if i < 2:
            r0 = q * (D // NQ)
            r0 = r0 if isinstance(r0, int) else pl.multiple_of(r0, D // NQ)
            src = (wg_hbm, wu_hbm)[i].at[pl.ds(r0, D // NQ), pl.ds(0, FM)]
        else:
            r0 = FVD + q * DQ + (i - 2) * DQA
            r0 = r0 if isinstance(r0, int) else pl.multiple_of(r0, 16)
            src = wd_hbm.at[pl.ds(r0, (DQA, DQ - DQA)[i - 2]), :]
        return pltpu.make_async_copy(src, stage_v[i].at[pl.ds(0, src.shape[0]), :], sem.at[SM + 10 + i])

    wphi_copy(0).start()
    k0_copy(0).start()
    x_copy(0).start()
    k0_copy(1).start()
    x_copy(1).start()
    wphi_copy(1).start()
    w_copy(1, 2).start()

    made = set()

    def view(ref, i, n, off=0):
        r0 = off + i * n
        return ref.at[pl.ds(r0 if isinstance(r0, int) else pl.multiple_of(r0, math.gcd(n, off)), n), :]

    def put_blocks(dst, r0, fn, m11, m12, m21, m22, never, a, skip=(), base=0, pitch=HK, gap=None):
        for c0 in range(0, m11.shape[1], 128):
            if c0:
                a = yield gap or GAP_PRO
            d11, d22 = m11[:, c0:c0 + 128], m22[:, c0:c0 + 128]
            if a is not None:
                d = jnp.concatenate([a, a], axis=0)
                d11, d22 = jnp.where(never, d, d11), jnp.where(never, d, d22)
            blocks = fn(d11, m12[:, c0:c0 + 128], m21[:, c0:c0 + 128], d22)
            for i, b in enumerate(blocks):
                if i not in skip:
                    dst[r0:r0 + 8, base + i * pitch + c0:base + i * pitch + c0 + 128] = _pack(b.astype(BF16))

    def rows16(ref, r0, c0=0, w=D):
        return _unpack(ref[r0:r0 + 8, c0:c0 + w]).astype(F32)

    def x_blocks(t, k, lo, hi, never, a, gap=None):
        yield from put_blocks(view(xs_v, t, TH // 2), k * LNC // 2, _strassen_rhs,
                              lo[:, :HK], hi[:, :HK], lo[:, HK:], hi[:, HK:], never, a, gap=gap)
        if isinstance(t, int):
            made.add(("xs", t, k))

    def ln_rows(t, k, n, never=None, anchor=None, plain=False):
        wide = lambda c, a: _lane_tile(_after(jnp.broadcast_to(c, (n, 128)), never, a), D // 128)
        x = _after(view(x_v, t, T)[k * n:(k + 1) * n, :].astype(F32), never, anchor)
        s1 = _row_sum(x)
        anchor = yield LN1_GAPS[0]
        xc = x - wide(s1 * (1.0 / D), anchor)
        rstd = lax.rsqrt(_row_sum(xc * xc) * (1.0 / D) + LN_EPS)
        anchor = yield LN1_GAPS[1]
        xn = xc * wide(rstd, anchor)
        if plain:
            xn_v[k * n // 2:(k + 1) * n // 2, :] = _pack(xn.astype(BF16))
        elif k * n < TH:
            xn_v[(T + k * n) // 2:(T + (k + 1) * n) // 2, :] = _pack(xn.astype(BF16))
        else:
            yield from x_blocks(t, k - TH // LNC, rows16(xn_v, (TH + k * n) // 2), xn, never, anchor, GAP_X)
        return _tree(jnp.add, [rstd[8 * i:8 * i + 8, :] for i in range(min(n, LNC) // 8)])

    def now(gen):
        try:
            while True:
                next(gen)
        except StopIteration as stop:
            return stop.value

    def late_x_blocks(t):
        return lambda k, a: x_blocks(t, k, rows16(xn_v, t * T // 2 + 8 * k),
                                     rows16(xn_v, (t * T + TH) // 2 + 8 * k), never0, a)

    def xn_tile(t):
        return _unpack(xn_v[t * T // 2:(t + 1) * T // 2, :])

    def xs_tile(t):
        assert not isinstance(t, int) or t > 1 or made >= {("xs", t, k) for k in range(8)}
        return _unpack(view(xs_v, t, TH // 2)[:, 0:7 * HK])

    def expand_wphi(c):
        w = wphi_v[8 * c:8 * c + 8].reshape(8 * DH, DH).astype(F32).T
        bits = pltpu.bitcast(w, U32)
        head = lax.broadcasted_iota(jnp.int32, (DH, 128), 1) >> 5
        for s in range(2):
            b = bits[:, 128 * s:128 * s + 128]
            for j in range(2):
                r0 = 64 * (2 * c + s) + 32 * j
                a_v[r0:r0 + 32, :] = jnp.where(head == 2 * j, b >> 16,
                                               jnp.where(head == 2 * j + 1, b, jnp.uint32(0)))

    wphi_copy(0).wait()
    expand_wphi(0)
    h_v[1][...] = jnp.zeros((T, D), F32)
    for ref in oc_v + oc2_v:
        ref[0:8, 0:128] = jnp.zeros((8, 128), U32)
    for ref in stage_v:
        ref[ref.shape[0] - 16:, 0:128] = jnp.zeros((16, 128), BF16)

    def v_transpose(k, a):
        q, r0 = (k // 8) + 4 * (k % 2), 256 * (k % 8 // 2)
        w = wraw_v[2 * NC + q // 2, r0:r0 + 256, (q % 2) * 128:(q % 2) * 128 + 128]
        if a is not None:
            w = _unpack(jnp.where(never0, jnp.concatenate([pltpu.bitcast(a, U32)] * 16, axis=0), _pack(w)))
        wt = _pack(w.T)
        wt_v[2][64 * q:64 * q + 64, r0:r0 + 256] = wt
        made.add(("vt", k))
        return pltpu.bitcast(wt[56:64, 128:256], F32)

    def fold_pairs(j, c, s, side=None, step0=None):
        g0 = 64 * (2 * c + s)
        g0 = g0 if isinstance(g0, int) else pl.multiple_of(g0, 64)
        res = _dot(_unpack(a_v[pl.ds(g0, 64), :]), wraw_v[j * NC + c, :, s * 128:(s + 1) * 128], NT)
        if side is not None:
            side.done(step0 + 2 * s, res[:, :D // 2])
            side.done(step0 + 2 * s + 1, res[:, D // 2:])
        sub = lax.broadcasted_iota(jnp.int32, (8, D), 0)
        out = []
        for q in range(2):
            base = _pair_allreduce(jnp.where(sub < 2, res[64 * q:64 * q + 8, :], 0.0), jnp.add)
            out.append([(res[64 * q + 8 * i:64 * q + 8 * i + 8, :] - base) * LOG2E for i in range(8)])
        return out

    def share(z, z3, k):
        sub = lax.broadcasted_iota(jnp.int32, (8, D), 0)
        return jnp.where(sub < 2, pltpu.roll(z3, 8 - 2 * k, 0), z)

    def packed(slabs):
        return _pack(jnp.concatenate(slabs, axis=0).astype(BF16))

    def fold(j, c, side=None, step0=None):
        p0, p1 = fold_pairs(j, c, 0, side, step0)
        p2, p3 = fold_pairs(j, c, 1, side, step0)
        sl = ([share(p0[0], p3[0], 1), share(p1[0], p3[0], 2)] + p0[1:] + p1[1:]
              + [share(p2[0], p3[0], 3)] + p2[1:] + p3[1:])
        zero = jnp.zeros((8, D), F32)
        even, odd = sl + [zero], [zero] + sl
        r0 = 8 * ((31 * c) // 2)
        is_odd = c % 2 == 1
        if isinstance(c, int):
            sl = odd if is_odd else even
        else:
            r0 = pl.multiple_of(r0, 8)
            sl = [jnp.where(is_odd, o, e) for o, e in zip(odd, even)]
        win = wt_v[j].at[pl.ds(r0, 128), :]
        win[8:128, :] = packed(sl[2:])
        first = packed(sl[:2])
        if is_odd is not False:
            keep = lax.broadcasted_iota(jnp.int32, (8, D), 0) < jnp.where(is_odd, 4, 0)
            first = jnp.where(keep, win[0:8, :], first)
        win[0:8, :] = first
        made.update(("fold", j, q) for q in ([c] if isinstance(c, int) else range(3)))

    def w_blocks(j, k0=0):
        def job(k, a):
            k += k0
            assert made >= ({("vt", 8 * (k // 8) + q) for q in range(8)} if j == 2 else
                            {("fold", j, q) for q in ((0, 2) if k < 15 else range(4))})
            lo, hi = rows16(wt_v[j], 8 * k), rows16(wt_v[j], (256 if j == 2 else 248) + 8 * k)
            yield from put_blocks(ws_v[j], 8 * k, _strassen_lhs, lo[:, :HK], lo[:, HK:], hi[:, :HK], hi[:, HK:],
                                  never0, a, skip=(1, 3))
            made.add(("ws", j, k))
        return job

    def k_pair(p, slot, pr, c0, never=None):
        first = ("z", pr, c0) not in made
        for n in range(c0, c0 + p[0].shape[1], 128):
            assert first == (("z", pr, n) not in made)
            made.update({("z", pr, n), ("phi", slot, pr, n)})
        ep, en, sp, sn = _dual_exp(p)
        inv = _recip(sp * sn)
        scale = (sn * inv, sp * inv)
        es = ep + en
        cols = slice(c0, c0 + p[0].shape[1])
        n = 16 if never is None else 16 // STAGGER
        last = None
        for q in range(16 // n):
            sc = scale
            if last is not None:
                sc = [jnp.where(never, last, x) for x in scale]
            phi = jnp.concatenate([es[i] * sc[i // 8] for i in range(q * n, (q + 1) * n)], axis=0)
            rows = slice(8 * q * n, 8 * (q + 1) * n)
            z = phi if first else z_v[pr, rows, cols] + phi
            z_v[pr, rows, cols] = z
            phi_v[slot][64 * pr + 4 * q * n:64 * pr + 4 * (q + 1) * n, cols] = _pack(phi.astype(BF16))
            last = z[8 * n - 8:, :]

    def kv_update(vts, slot, g, first, publish=False):
        for q, vt in enumerate(vts):
            for j in range(2):
                pr = 2 * g + 8 * q + j
                assert made >= {("phi", slot, pr, 0), ("phi", slot, pr, 128)}
                upd = _dot(vt[64 * j:64 * j + 64, :].astype(BF16), _unpack(phi_v[slot][64 * pr:64 * pr + 64, :]), NT)
                acc = upd if first else kvacc_v[pr] + upd
                kvacc_v[pr] = acc
                if publish:
                    odd = -(lax.broadcasted_iota(jnp.int32, (32, 128), 1) & 1)
                    bits = pltpu.bitcast(acc, jnp.int32) & jnp.concatenate([~odd, odd], axis=0)
                    kvbf_v[32 * pr:32 * pr + 32, :] = _pack(pltpu.bitcast(bits, F32).astype(BF16))

    def save_lead(t):
        view(lead_v, t, HK // 2)[...] = _pack(_unpack(view(xs_v, t, TH // 2)[:, 0:HK]).T)

    def proj_feat(side, step0, c, xn):
        r0 = 8 * ((31 * c) // 2)
        w = wt_v[1][r0:r0 + 128, :]
        quarters = []
        for n in range(2):
            for m in range(2):
                step = step0 + 2 * n + m
                wq = _unpack(side.gate(step, w[:64, :] if m == 0 else w[64:, :]))
                res = _dot(wq, xn[n * TH:(n + 1) * TH, :], NT)
                side.done(step, res)
                quarters.append(res)
        res = jnp.concatenate(
            [jnp.concatenate([quarters[0], quarters[2]], axis=1),
             jnp.concatenate([quarters[1], quarters[3]], axis=1)], axis=0)
        sl = [res[8 * i:8 * i + 8, :] for i in range(res.shape[0] // 8)]
        return sl[c % 2:31 + c % 2]

    def proj_unit(side, step0, j, b, xs, lead=None, plain=None):
        r1 = 64 * b + (64 if j == 2 or b < 3 else 56)
        assert made >= ({("vt", 8 * b + q) for q in range(8)} if plain is not None else
                        {("ws", j, k) for k in range(8 * b, r1 // 8)})
        if plain is not None:
            out = []
            for q in range(2):
                row = []
                for n in range(2):
                    steps = range((0, 2, 4, 5)[2 * q + n], (2, 4, 5, 7)[2 * q + n])
                    deps = [d for i in steps for d in side.deps.pop(step0 + i, [])]
                    w = _gate(wt_v[2][256 * q + 64 * b:256 * q + r1, :], side.never, deps)
                    res = _dot(_unpack(w), plain[n * TH:(n + 1) * TH, :], NT)
                    for i in steps:
                        side.done(step0 + i, res)
                    row.append(res)
                out.append(jnp.concatenate(row, axis=1))
            return out

        def product(i):
            off = 256 if j == 2 else 248
            w = (wt_v[j][off + 64 * b:off + r1, HK:] if i == 1 else wt_v[j][64 * b:r1, :HK] if i == 3
                 else ws_v[j][64 * b:r1, i * HK:(i + 1) * HK])
            w = _unpack(side.gate(step0 + i, w))
            if lead is not None and i == 0:
                res = _dot(w, _unpack(view(lead_v, lead, HK // 2)[...]), NN)
            else:
                res = _dot(w, xs[:, i * HK:(i + 1) * HK], NT)
            side.done(step0 + i, res)
            return res
        return [jnp.concatenate(row, axis=1) for row in _strassen(product)]

    def feat_stage(side, step0, j, xs, pair_fn, lead=None, units=range(4), sl=None, hold=None):
        sl = sl or [[], []]
        for b in units:
            for q, res in enumerate(proj_unit(side, step0 + 7 * b, j, b, xs, lead if b == units[0] else None)):
                sl[q] += [res[8 * i:8 * i + 8, :] for i in range(res.shape[0] // 8)]
            for q in (1, 0):
                for jj in (2 * (b % 2), 2 * (b % 2) + 1):
                    if b != hold:
                        pair_fn(_pair_logits(sl[q][31 * (b // 2):], jj), 8 * q + 4 * (b // 2) + jj)
        return sl

    def v_stage(side, xs, slot, first, publish, lead, plain=None):
        pending = None
        for g in range(4):
            if pending is not None:
                side.hooks.setdefault(7 * g + D_LAG, []).append(lambda p=pending: kv_update(*p))
            pending = (proj_unit(side, 7 * g, 2, g, xs, lead if g == 0 else None, plain if g < PLAIN_V0 else None),
                       slot, g, first, publish)
        side.check()
        return pending

    def pack_rows(src, dst, r0, c0, cols, never, a):
        for c in range(c0, c0 + cols, PACK_W):
            if c > c0:
                a = yield GAP_PACK
            w = min(PACK_W, c0 + cols - c)
            v = src[r0:r0 + 16, c:c + w].astype(F32)
            v = jnp.concatenate([jnp.where(never, _lane_tile(a, w // 128), v[0:8, :]), v[8:16, :]], axis=0)
            dst[r0 // 2:r0 // 2 + 8, c:c + w] = _pack(v.astype(BF16))

    def stash_at(i, k, n):
        return zb_v.at[4 * i + 2 * (k // 16) + n, pl.ds(8 * (k % 16), 8), :]

    def stash(i, sl):
        for k, v in enumerate(sl):
            for n in range(2):
                stash_at(i, k, n)[...] = v[:, 128 * n:128 * n + 128]

    def stashed_k(i, slot, c):
        def job(k, a):
            j, n = k // 2, k % 2
            p = _pair_logits([stash_at(i, q, n)[...] for q in range(16 if j < 2 else 31)], j)
            k_pair([_after(p[0], never0, a)] + p[1:], slot, c * PPC + j, 128 * n, never0)
        return job

    def first_rows(k0, k1, n):
        xn = _unpack(xn_v[n * TH // 2:(n + 1) * TH // 2, :])
        ks = [k for k in range(k0, k1)]
        w = jnp.concatenate([wt_v[1][4 * (k % 32):4 * (k % 32) + 8, :] for k in ks[::2]], axis=0)
        res = _dot(_unpack(w), xn, NT)
        for q, k in enumerate(ks):
            if k % 32 < 31:
                stash_at(0, k % 32, n)[...] = res[8 * q:8 * q + 8, :]

    k0_copy(0).wait()
    x_copy(0).wait()
    wphi_copy(2).start()
    x_copy(5).start()
    w_copy(1, 1).start()
    wphi_copy(3).start()
    x_copy(2).start()
    p0, p1 = fold_pairs(1, 0, 0)
    wt_v[1][8:64, :] = packed(p0[1:] + p1[1:])
    h_v[0][0:8, :] = p0[0]
    h_v[0][8:16, :] = p1[0]
    never0 = now(ln_rows(0, 0, TH, plain=True))[0, 0] < 0.0
    first_rows(2, 16, 0)

    k0_copy(1).wait()
    x_copy(1).wait()
    wphi_copy(1).wait()
    w_copy(1, 3).start()
    for c in (0, 2, 1, 3):
        w_copy(2, c).start()
    p2, p3 = fold_pairs(1, 0, 1)
    wt_v[1][0:8, :] = packed([share(h_v[0][0:8, :], p3[0], 1), share(h_v[0][8:16, :], p3[0], 2)])
    wt_v[1][64:128, :] = packed([share(p2[0], p3[0], 3)] + p2[1:] + p3[1:] + [jnp.zeros((8, D), F32)])
    made.add(("fold", 1, 0))
    now(ln_rows(0, 1, TH, plain=True))
    first_rows(16, 34, 0)
    first_rows(0, 16, 1)
    first_rows(16, 32, 1)
    expand_wphi(2)

    def slow(end):
        return lambda rel, gap: min(rel + (gap / 2 if 3 <= rel < 7 else gap), end)

    for c, prev in ((2, 0), (1, 2)):
        w_copy(1, c).wait()
        wphi_copy(4 - c).wait()
        side = _Side(never0, slow(7))
        if c == 1:
            x_copy(5).wait()
            side.add(PRO_LN_PLANS0, lambda k, a: ln_rows(1, k, LNC, never0, a))
        expand_wphi(5 - 2 * c)
        side.add((PRO_W_PLANS0, PRO_W_PLANS1)[2 - c], w_blocks(1, (2 - c) * len(PRO_W_PLANS0)))
        side.add((PRO_K_PLANS0, PRO_K_PLANS1)[2 - c], stashed_k(prev, 0, prev))
        fold(1, c, side, 0)
        stash(c, proj_feat(side, 4, c, xn_tile(0)))
        side.check()

    x_copy(2).wait()
    w_copy(1, 3).wait()
    x_copy(3).start()
    w_copy(0, 0).start()
    wo_copy(0).start()
    x_copy(4).start()
    side = _Side(never0, slow(28))
    side.add(PRO_LN_PLANS1, lambda k, a: ln_rows(1, k + 8, LNC, never0, a))
    side.add(PRO_W_PLANS2, w_blocks(1, 31 - len(PRO_W_PLANS2)))
    side.add(PRO_K_PLANS2, stashed_k(1, 0, 1))
    side.add(PRO_X0_PLAN, late_x_blocks(0))
    fold(1, 3, side, 0)
    stash(3, proj_feat(side, 4, 3, xn_tile(0)))
    k1 = lambda p, pr: k_pair(p, 1, pr, 0, never0)
    for q, sl in enumerate(feat_stage(side, 8, 1, xs_tile(1), k1, units=range(3), hold=2)):
        stash(2 * q, sl[31:])
    side.check()
    save_lead(1)

    for c in range(NC):
        w_copy(2, c).wait()
    side = _Side(never0, lambda rel, gap: min(rel + gap, 27))
    side.add(PRO_V_PLANS[0], v_transpose)
    side.add(PRO_V_PLANS[1], stashed_k(3, 0, 3))
    side.add(PRO_V_PLANS[2], stashed_k(0, 1, 1))
    side.add(PRO_V_PLANS[3], stashed_k(2, 1, 3))
    side.add(PRO_V_PLANS[4], w_blocks(2))
    sl = [[None] * 31 + [jnp.concatenate([stash_at(2 * q, k, n)[...] for n in range(2)], axis=1) for k in range(17)]
          for q in range(2)]
    feat_stage(side, -28, 1, xs_tile(1), k1, 1, units=range(3, 4), sl=sl)
    kv_update(*v_stage(side, xs_tile(0), 0, True, False, None, xn_tile(0)))
    save_lead(0)
    for c in range(1, NC):
        w_copy(0, c).start()
    wo_copy(1).start()
    wr_copy.start()
    for i in range(4):
        stage_copy(i, 0).start()
    wg_copy.start()
    wu_copy.start()
    wd_copy.start()
    for r0 in (0, 248):
        wt_v[0][r0:r0 + 8, :] = jnp.zeros((8, D), U32)

    def phase1(u, carry):
        never = u < 0

        @pl.when(u == 0)
        def _():
            x_copy(3).wait()
            w_copy(0, 0).wait()
            wo_copy(0).wait()

        @pl.when(u == 1)
        def _():
            x_copy(4).wait()
            w_copy(0, 1).wait()
            w_copy(0, 2).wait()
            wo_copy(1).wait()

        def wo_blocks(k0):
            def job(k, a):
                k += k0
                r, c, part = k // 4, 128 * (k // 2 % 2), k % 2
                r0 = u * ((QK - WO_ROWS) // 2)
                dst = wos_v.at[pl.ds(pl.multiple_of(r0 // 2, 8), WO_ROWS // 2), :]

                def piece(kq, nq):
                    src = woraw_v.at[kq, pl.ds(pl.multiple_of(r0, 16), WO_ROWS), :]
                    return src[16 * r:16 * r + 16, nq * QK + c:nq * QK + c + 128].astype(F32)
                outer = [_strassen_rhs(piece(ki, ni), piece(ki, 2 + ni), piece(2 + ki, ni), piece(2 + ki, 2 + ni))
                         for ki in range(2) for ni in range(2)]
                for i in range(4) if part == 0 else range(4, 7):
                    if i % 4:
                        a = yield GAP_WO
                    yield from put_blocks(dst, 8 * r, _strassen_rhs, *[o[i] for o in outer], never, a,
                                          base=7 * i * QK + c, pitch=QK)
            return job

        xs = xs_tile(2 * u + 1)
        side = _Side(never, lambda rel, gap: min(rel + gap, 27))
        for i in range(2):
            t = 2 * u + 2 + i
            if i == 0:
                side.add(LN1_PLANS[0], lambda k, a: ln_rows(2 * u + 2, k, LNC, never, a))
                side.add(WO_PLANS[0], wo_blocks(0))
            pending = v_stage(side, xs, 1 - i, False, False, t - 1 if i == 0 else None)
            xs = xs_tile(t)
            side = _Side(never, lambda rel, gap, end=(27, -1)[i]: min(rel + gap, end))
            if i == 0:
                side.add(LN1_PLANS[1], lambda k, a: ln_rows(2 * u + 3, k, LNC, never, a))
                side.add(WO_PLANS[1], wo_blocks(len(WO_PLANS[0])))
            else:
                side.add(WO_PLANS[2], wo_blocks(24 - len(WO_PLANS[2])))
            side.hooks[-28 + D_LAG] = [lambda p=pending: kv_update(*p)]
            feat_stage(side, -28, 1, xs, lambda p, pr: k_pair(p, i, pr, 0, never if i == 1 else None))
            save_lead(t)
        side.check()
        fold(0, u)
        return carry

    lax.fori_loop(0, (NT_ - 2) // 2, phase1, 0)

    w_copy(0, 3).wait()
    wr_copy.wait()
    side = _Side(never0, lambda rel, gap: min(rel + gap, 27 if rel < 98 else 103))

    def z_final(k, a):
        zb_v[k] = jnp.broadcast_to(_row_sum(_after(z_v[k], never0, a)), (128, 128))

    side.add(END_PLANS[0], z_final)
    side.add(END_PLANS[1], w_blocks(0))
    side.hooks[0] = [lambda: fold(0, 3, side, 100)]
    kv_update(*v_stage(side, xs_tile(NT_ - 1), 1, False, True, NT_ - 1))
    wr_v[...] = jnp.broadcast_to(wrraw_v[...].reshape(1, D).astype(F32), (8, D))

    def o_copy(r0, n, i):
        return pltpu.make_async_copy(o_v.at[pl.ds(r0, n), :], out_hbm.at[pl.ds(r0, n), :], sem.at[SO + i])

    def finish_rows(h_ref, k, t, valid, st, never=None, anchor=None):
        r0 = t * T + k * LNC
        rows = slice(k * LNC, (k + 1) * LNC)
        m = jnp.broadcast_to(_row_sum(_after(h_ref[rows, :], never, anchor)) * (1.0 / D), (LNC, 128))
        rstd, r = [], []
        for i in range(LNC // 8):
            anchor = yield LN2_GAPS[2] if i else LN2_GAPS[0]
            mi = _after(m[8 * i:8 * i + 8, :], never, anchor)
            hc = h_ref[k * LNC + 8 * i:k * LNC + 8 * i + 8, :] - _lane_tile(mi, D // 128)
            rs = lax.rsqrt(_row_sum(hc * hc) * (1.0 / D) + LN_EPS)
            r.append((_row_sum(hc * wr_v[...]) * rs + 0.0).astype(BF16).astype(F32))
            rstd.append(jnp.broadcast_to(rs, (8, 128)))
        rstd = jnp.concatenate(rstd, axis=0)
        w = D if never is None else D // LN2_SPLIT
        for c in range(0, D, w):
            anchor = yield LN2_GAPS[2] if c else LN2_GAPS[1]
            h = h_ref[rows, c:c + w]
            hn = (h - _lane_tile(_after(m, never, anchor), w // 128)) * _lane_tile(rstd, w // 128)
            view(hn_v, t, T // 2)[k * LNC // 2:(k + 1) * LNC // 2, c:c + w] = _pack(hn.astype(BF16))
            view(o_v, t, T)[rows, c:c + w] = (hn + h).astype(BF16)
        best = st["route"]
        sub = lax.broadcasted_iota(jnp.int32, (8, 128), 0)
        for i, ri in enumerate(r):
            key = _ordered(pltpu.bitcast(jnp.broadcast_to(ri, (8, 128)), jnp.int32)) | ((S - 1 - r0 - 8 * i) - sub)
            if valid is not None:
                key = jnp.where(valid, key, KEY_MIN)
            best = jnp.maximum(best, key)
        st["route"] = best
        return pltpu.bitcast(best, F32)

    def q_pair(p, slot, pr):
        ep, en, sp, sn = _dual_exp(p)
        zz = [_lane_tile(zb_v[pr, 8 * i:8 * i + 8, :], T // 128) for i in range(16)]
        ap = _pair_allreduce(_tree(jnp.add, [ep[i] * zz[i] for i in range(8)]), jnp.add)
        an = _pair_allreduce(_tree(jnp.add, [en[i] * zz[8 + i] for i in range(8)]), jnp.add)
        inv = _recip(ap * sn + (an + 1e-6 * sn) * sp)
        rp = sn * inv
        rn = sp * inv
        phi = jnp.concatenate([e * rp for e in ep] + [e * rn for e in en], axis=0)
        phi_v[slot][64 * pr:64 * pr + 64, :] = _pack(phi.astype(BF16))

    held = []

    def attn_blocks(slot, g, deps):
        res = [_dot(_unpack(kvbf_v[32 * pr:32 * pr + 32, :]), _unpack(phi_v[slot][64 * pr:64 * pr + 64, :]), NN)
               for pr in (2 * g, 2 * g + 8, 2 * g + 1, 2 * g + 9)]
        lo, hi = jnp.concatenate(res[0::2], axis=0), jnp.concatenate(res[1::2], axis=0)
        blocks = [(i, g, b) for i, b in enumerate(_strassen_lhs(lo[:, :TH], hi[:, :TH], lo[:, TH:], hi[:, TH:]))]
        if g % 2 == 0:
            held.append(blocks.pop())
        else:
            blocks.append(held.pop())
        ot = _pack(jnp.concatenate([b for _, _, b in blocks], axis=1).astype(BF16).T)
        for q, (i, n, _) in enumerate(blocks):
            oc_v[slot][:, i * HK + 128 * n:i * HK + 128 * n + 128] = ot[q * TH // 2:(q + 1) * TH // 2, :]
            made.add(("oc", slot, i, n))
            if q % 2:
                deps.append(pltpu.bitcast(ot[(q + 1) * TH // 2 - 8:(q + 1) * TH // 2, :], F32))

    def o_blocks(slot, c, never):
        def job(k, a):
            k = (2, 3, 1, 4, 5, 0, 6)[k]
            assert made >= {("oc", slot, k, c), ("oc", slot, k, c + 2)}
            for r in range(4):
                if r:
                    a = yield GAP_O2
                m = [rows16(oc_v[slot], 8 * r + 32 * q, k * HK + n * QK + 128 * c, 128)
                     for q in range(2) for n in range(2)]
                yield from put_blocks(oc2_v[slot], 8 * r, _strassen_lhs, *m, never, a, skip=(1, 3),
                                      base=7 * k * QK + 128 * c, pitch=QK)
            made.add(("oc2", slot, k, c))
        return job

    def out_proj(side, step0, t, slot):
        count = [0]

        def inner(i, c):
            assert made >= {("oc2", slot, i, 0), ("oc2", slot, i, 1)}

            def product(j):
                step, odd = step0 + count[0] // 2, count[0] % 2
                count[0] += 1
                o = (oc_v[slot][32:64, i * HK + QK:(i + 1) * HK] if j == 1 else
                     oc_v[slot][0:32, i * HK:i * HK + QK] if j == 3 else
                     oc2_v[slot][:, (7 * i + j) * QK:(7 * i + j + 1) * QK])
                w = wos_v[:, (7 * i + j) * QK + 128 * c:(7 * i + j) * QK + 128 * c + 128]
                res = _dot(_unpack(o), _unpack(w if odd else side.gate(step, w)), NN)
                if odd:
                    side.done(step, res)
                return res
            return _block(_strassen(product))

        xt = view(x_v, t, T)

        def emit(q, r, res):
            for c in range(2):
                for n in range(2):
                    rows, c0 = slice(q * TH, (q + 1) * TH), r * HK + n * QK + 128 * c
                    h_v[slot][rows, c0:c0 + 128] = (res[:, 256 * c + 128 * n:256 * c + 128 * n + 128]
                                                    + xt[rows, c0:c0 + 128].astype(F32))
            made.add(("h", slot, q, r))

        _strassen_rows_first(lambda i: jnp.concatenate([inner(i, c) for c in range(2)], axis=1), emit)

    def phase2(u, carry):
        for i in range(4):
            stage_copy(i, u).wait()
        never = u < 0
        side = _Side(never, lambda rel, gap: min(rel + 2 * gap, 97) if rel < 98 else
                     rel + gap if rel + gap <= 155 else 2 * (rel + gap - 155) - 1)
        st = {"route": carry}
        tp = jnp.maximum(2 * u - 1, 0)
        early = len(LN2_PLANS[2])

        def ln2(slot, t, valid, k0, key):
            def job(k, a):
                k += k0
                hs = {("h", slot, k // 8, r) for r in range(2)}
                assert made >= hs or key == 0
                best = yield from finish_rows(h_v[slot], k, t, valid, st, never, a)
                assert key > 0 or not made & hs
                return best
            return job

        side.add(LN2_PLANS[0], ln2(1, tp, u > 0, early, 0))
        side.add(LN2_PLANS[1], ln2(0, 2 * u, None, 0, 1))
        side.add(LN2_PLANS[2], ln2(1, 2 * u + 1, None, 0, 2))

        def packer(i, dst, n):
            left = [n]

            def job(k, a):
                if i < 2:
                    yield from pack_rows(stage_v[i], dst, (k // 2) * 16, (0, D)[k % 2], (D, FM - D)[k % 2], never, a)
                else:
                    yield from pack_rows(stage_v[i], dst, k * 16, 0, D, never, a)
                left[0] -= 1
                if not left[0]:
                    stage_copy(i, jnp.minimum(u + 1, NQ - 1)).start()
                    n0 = stage_v[i].shape[0] - 16
                    side.deps.setdefault(PACK_DUE[i], []).append(stage_v[i][n0:n0 + 8, 0:128].astype(F32))
            return job

        for i in range(2):
            side.add(PACK_PLANS[i], packer(i, view((wgp_v, wup_v)[i], u, D // NQ // 2), len(PACK_PLANS[i])))
            d0 = pl.multiple_of(u * (DQ // 2) + i * (DQA // 2), 8)
            side.add(PACKD_PLANS[i], packer(2 + i, wdp_v.at[pl.ds(d0, 8 * len(PACKD_PLANS[i])), :],
                                            len(PACKD_PLANS[i])))
            for g in range(4):
                step = 107 + 28 * i + 7 * g + G_LAG
                wrap = lambda x: x if x < 156 else 2 * (x - 156) + 1
                side.hooks.setdefault(wrap(step), []).append(
                    lambda i=i, g=g, due=wrap(step + O_DUE): attn_blocks(i, g, side.deps.setdefault(due, [])))
            for c in range(2):
                side.add(O2_PLANS[2 * i + c], o_blocks(i, c, never))
        for i in range(2):
            feat_stage(side, 100 + 28 * i, 0, xs_tile(2 * u + i), lambda p, pr: q_pair(p, i, pr),
                       2 * u if i == 0 else None)
        for i in range(2):
            out_proj(side, 49 * i, 2 * u + i, i)
        side.check()

        @pl.when(u == 0)
        def _():
            o_copy(0, T, 0).start()

        @pl.when(u > 0)
        def _():
            o_copy(pl.multiple_of(tp * T, T), 2 * T, u).start()

        return st["route"]

    wg_copy.wait()
    wu_copy.wait()
    wd_copy.wait()
    route = lax.fori_loop(
        0, NT_ // 2, phase2,
        jnp.full((8, 128), KEY_MIN, jnp.int32))
    st = {"route": route}
    for k in range(len(LN2_PLANS[2]), T // LNC):
        now(finish_rows(h_v[1], k, NT_ - 1, None, st))
    o_copy(S - T, T, NT_).start()

    best = st["route"]
    for shift in (4, 2, 1):
        best = jnp.maximum(best, pltpu.roll(best, shift, 0))
    idx_s = (S - 1) - (best[0, 0] & (S - 1))
    gate = _lane_tile(jax.nn.sigmoid(pltpu.bitcast(_ordered(best & -65536), F32)), D // 128)
    blk = pl.multiple_of(jnp.clip((idx_s >> 4) << 4, 0, S - 16), 16)
    pair = jnp.broadcast_to(hn_v[pl.ds(jnp.clip(idx_s >> 1, 0, S // 2 - 1), 1), :], (8, D))
    x8 = pltpu.bitcast(jnp.where((idx_s & 1) == 1, pair & jnp.uint32(0xFFFF0000), pair << 16), F32)
    xs = jnp.concatenate([x8, x8], axis=0).astype(BF16)
    acts, anchors = [], []

    def park(v, half):
        n = v.shape[0] // 128
        for i in range(n):
            z_v[i, :, 128 * half:128 * half + 128] = v[128 * i:128 * i + 128, :]
        return jnp.concatenate([z_v[i, :, 128 * half:128 * half + 128] for i in range(n)], axis=0)

    for c0 in range(0, FM, 128):
        g = _dot(xs, _unpack(wgp_v[:, c0:c0 + 128]), NN)[0:8, :]
        u = _dot(xs, _unpack(wup_v[:, c0:c0 + 128]), NN)[0:8, :]
        anchors += [g, u]
        acts.append(g * jax.nn.sigmoid(g) * u)
    xb = park(_col_broadcast(x8), 0)
    g, u = [_sublane_allreduce(_vpu_matvec(
        xb, lambda g: w[8 * g:8 * g + 8, :].astype(F32), never0,
        anchors[i * MOE_NA // 2:(i + 1) * MOE_NA // 2], MOE_LAGS[0])) for i, w in enumerate((wg_v, wu_v))]
    acts.append(g * jax.nn.sigmoid(g) * u)
    a = jnp.concatenate(acts, axis=1)
    am = jnp.concatenate([a[:, FVD:], a[:, FVD:]], axis=0).astype(BF16)
    ys, anchors = [], anchors[MOE_NA:]
    for k0 in range(0, FF - FVD, 512):
        k1 = min(k0 + 512, FF - FVD)
        yk = _dot(am[:, k0:k1], _unpack(wdp_v[k0 // 2:k1 // 2, 0:D]), NN)[0:8, :]
        ys.append(yk)
        anchors += [yk[:, c:c + 128] for c in range(128, D, 256)]
    ys.append(_sublane_allreduce(_vpu_matvec(
        park(_col_broadcast(a[:, :FVD]), 1), lambda g: wd_v[8 * g:8 * g + 8, :].astype(F32), never0,
        anchors[:-MOE_ND], MOE_LAGS[1])))
    y = _tree(jnp.add, ys) * gate
    y = jnp.concatenate([y, y], axis=0)
    sel = lax.broadcasted_iota(jnp.int32, (16, 1), 0) == (idx_s - blk)
    patch_v[...] = (o_v[pl.ds(blk, 16), :].astype(F32) + jnp.where(sel, y, 0.0)).astype(BF16)
    o_copy(0, T, 0).wait()
    for u in range(1, NT_ // 2):
        o_copy((2 * u - 1) * T, 2 * T, u).wait()
    o_copy(S - T, T, NT_).wait()
    pc = pltpu.make_async_copy(patch_v, out_hbm.at[pl.ds(blk, 16), :], sem.at[SM + 3])
    pc.start()
    for i in range(4):
        stage_copy(i, NQ - 1).wait()
    pc.wait()


@jax.jit
def pallas_sequential_preLN__linear_kernel_hedgehog__moe_arch_mod__prompt_kernel(
    A_x: jax.Array,
    A_wqkv: jax.Array,
    A_w_phi: jax.Array,
    A_wo: jax.Array,
    B_x: jax.Array,
    B_w_r: jax.Array,
    B_w_gate: jax.Array,
    B_w_up: jax.Array,
    B_w_down: jax.Array,
):
    del B_x
    hbm = pl.BlockSpec(memory_space=pl.ANY)
    out = pl.pallas_call(
        _kernel,
        out_shape=jax.ShapeDtypeStruct((S, D), BF16),
        in_specs=[hbm] * 8,
        out_specs=hbm,
        scratch_shapes=[
            pltpu.VMEM((S, D), BF16),
            pltpu.VMEM(((T + TH) // 2, D), U32),
            pltpu.VMEM((NT_ * TH // 2, SW), U32),
            pltpu.VMEM((NT_ * HK // 2, 128), U32),
            pltpu.VMEM((3 * NC, D, RC), BF16),
            [pltpu.VMEM((D // 2, D), U32)] * 3,
            [pltpu.VMEM((HK // 2, 7 * HK), U32)] * 3,
            pltpu.VMEM((H, DH, DH), BF16),
            pltpu.VMEM((8 * 64, 128), U32),
            pltpu.VMEM((4, QK, D), BF16),
            pltpu.VMEM((QK // 2, 49 * QK + 128), U32),
            pltpu.VMEM((D,), BF16),
            pltpu.VMEM((8, D), F32),
            pltpu.VMEM((NPAIR, 64, 128), F32),
            pltpu.VMEM((NPAIR * 32, 128), U32),
            pltpu.VMEM((NPAIR, 128, T), F32),
            pltpu.VMEM((NPAIR, 128, 128), F32),
            [pltpu.VMEM((NPAIR * 64, T), U32)] * 2,
            [pltpu.VMEM((TH // 2, 7 * HK), U32)] * 2,
            [pltpu.VMEM((TH // 4, 49 * QK), U32)] * 2,
            [pltpu.VMEM((T, D), F32)] * 2,
            pltpu.VMEM((S // 2, D), U32),
            pltpu.VMEM((S, D), BF16),
            pltpu.VMEM((D, FV), BF16),
            pltpu.VMEM((D, FV), BF16),
            pltpu.VMEM((FVD, D), BF16),
            [pltpu.VMEM((D // NQ + 16, FM), BF16), pltpu.VMEM((D // NQ + 16, FM), BF16),
             pltpu.VMEM((DQA + 16, D), BF16), pltpu.VMEM((DQ - DQA + 16, D), BF16)],
            pltpu.VMEM((D // 2, FM), U32),
            pltpu.VMEM((D // 2, FM), U32),
            pltpu.VMEM(((FF - FVD) // 2, D + 128), U32),
            pltpu.VMEM((16, D), BF16),
            pltpu.SemaphoreType.DMA((6 + 3 * NC + NT_ + 17,)),
        ],
        compiler_params=pltpu.CompilerParams(vmem_limit_bytes=100 * 1024 * 1024,
                                             disable_semaphore_checks=True, disable_bounds_checks=True),
        name="hedgehog_mod",
    )(
        A_x.reshape(S, D),
        A_wqkv,
        A_w_phi,
        A_wo.reshape(4, QK, D),
        B_w_r,
        B_w_gate,
        B_w_up,
        B_w_down,
    )
    return out.reshape(1, S, D)
```

```python
import math

import jax
import jax.numpy as jnp
from jax import lax
import jax.experimental.pallas as pl
import jax.experimental.pallas.tpu as pltpu

F32 = jnp.float32
BF16 = jnp.bfloat16
U32 = jnp.uint32

S = 2048
D = 1024
H = 32
DH = 32
FF = 3584
NPAIR = H // 2
LOG2E = 1.4426950408889634
LN_EPS = 1e-5
KEY_MIN = -2 ** 31

T = 256
TH = T // 2
NT_ = S // T
RC = 256
NC = D // RC
PPC = RC // 64
LNC = 16

FV = 10 * 128
FM = FF - FV
FVD = 8 * 128
NQ = NT_ // 2
DQ = (FF - FVD) // NQ
WO_ROWS = 96
QK = D // 4
HK = D // 2
SW = 8 * HK


LN1_PLANS = (((0.095, 7), (0.452, 8), (2.855, 10), (4.2, 11), (5.323, 12), (7.125, 13), (8.42, 16), (9.93,
    16), (11.174, 18), (11.928, 19), (13.877, 22), (15.466, 23), (16.77, 23), (18.221, 25), (19.564, 26),
    (21.5, 27)), ((-1.151, 4), (1.211, 7), (1.804, 8), (3.43, 9), (5.504, 11), (5.924, 14), (8.015, 14),
    (9.695, 17), (10.176, 17), (11.93, 19), (13.665, 19), (15.339, 22), (16.395, 22), (18.546, 25), (19.409,
    26), (21.079, 27)))
PRO_LN_PLANS0 = ((None, 4), (None, 7), (0.12, 5), (0.555, 5), (1.7, 6), (2.168, 6), (3.297, None), (4.239,
    None))
PRO_LN_PLANS1 = ((None, 4), (None, 5), (-0.516, None), (0.246, 6), (1.046, 6), (2.1, 7), (3.001, 7), (3.003,
    6))
PRO_K_PLANS0 = ((0.388, None), (0.863, None), (1.721, None), (2.715, None), (2.982, None), (3.948, None),
    (5.473, None), (5.989, None))
PRO_K_PLANS1 = ((-0.866, None), (0.636, None), (1.962, None), (2.951, None), (3.554, None), (4.106, None),
    (4.699, None), (5.223, None))
PRO_X0_PLAN = ((20.049, None), (21.671, None), (23.071, None), (23.684, None), (25.371, None), (26.097, None),
    (26.566, None), (27.089, None))
PRO_W_PLANS0 = ((3.2, None), (3.488, None), (3.771, None), (4.235, None), (4.92, None), (5.413, None), (6.114,
    None), (6.485, None))
PRO_W_PLANS1 = ((4.846, None), (5.235, None), (6.531, None))
PRO_W_PLANS2 = ((6.626, None), (7.329, None), (8.074, None), (9.011, None), (9.904, None), (10.947, None),
    (12.625, None), (13.232, None), (14.27, None), (15.036, None), (16.142, None), (17.035, None), (18.379,
    None), (19.306, None), (19.316, None), (20.753, None), (21.341, None), (22.294, None), (23.106, None),
    (25.173, None))
PRO_K_PLANS2 = ((21.924, None), (22.415, None), (24.003, None), (24.127, None), (24.582, None), (25.771,
    None), (26.668, None), (27.134, None))
PRO_V_PLANS = (((None, None), (None, None), (None, None), (None, None), (None, None), (None, None), (None,
    None), (None, None), (-4.983, 0), (-4.771, 1), (-4.658, 2), (-3.398, 2), (-3.155, 2), (-2.921, 2),
    (-2.499, 3), (-2.355, 3), (-1.874, 4), (-1.535, 4), (-1.024, 4), (-0.927, 4), (-0.706, 4), (0.24, 6),
    (0.481, 7), (0.668, 6), (1.247, 7), (1.4, 7), (2.688, 9), (2.727, 7), (3.012, 8), (3.087, 9), (4.289, 9),
    (4.924, 10)), ((5.897, None), (7.691, None), (10.048, None), (12.014, None), (13.868, None), (15.456,
    None), (17.412, None), (20.836, None)), ((0.0, None), (1.776, None), (3.418, None), (4.808, None)),
    ((19.45, None), (21.451, None), (22.925, None), (23.333, None)), ((16.059, None), (20.449, None), (20.497,
    None), (21.79, None), (22.449, None), (22.572, None), (25.109, None), (25.686, None), (-0.337, None),
    (-0.164, None), (0.488, None), (2.709, None), (2.857, None), (3.639, None), (4.322, None), (4.918, None),
    (5.207, None), (6.91, None), (7.587, None), (8.953, None), (9.24, None), (10.232, None), (11.175, None),
    (11.993, None), (12.583, None), (13.787, None), (14.312, None), (14.817, None), (16.402, None), (16.81,
    None), (17.304, None), (19.292, None)))
END_PLANS = (((-0.162, None), (2.011, None), (3.829, None), (5.62, None), (6.909, None), (8.156, None),
    (10.634, None), (12.371, None), (13.954, None), (15.538, None), (16.797, None), (19.352, None), (20.737,
    None), (23.183, None), (23.393, None), (25.88, None)), ((100.308, None), (101.389, None), (102.104, None),
    (0.409, None), (1.005, None), (2.198, None), (2.898, None), (4.205, None), (5.131, None), (6.022, None),
    (7.291, None), (7.974, None), (8.425, None), (9.982, None), (11.3, None), (11.768, None), (12.903, None),
    (13.561, None), (14.696, None), (15.687, None), (17.565, None), (18.013, None), (18.596, None), (19.613,
    None), (20.25, None), (21.235, None), (22.366, None), (23.06, None), (24.673, None), (25.256, None),
    (26.011, None)))
WO_PLANS = (((0.245, None), (6.671, None), (13.134, None), (18.635, None), (24.922, None)), ((-26.952, None),
    (-21.248, None), (-16.958, None), (-12.341, None), (-8.3, None), (-2.883, None), (1.607, None), (6.233,
    None), (10.547, None), (15.312, None), (19.974, None), (24.229, None)), ((-27.707, None), (-22.089, None),
    (-18.962, None), (-14.225, None), (-9.98, None), (-6.618, None), (-2.09, None)))
LN2_PLANS = (((-0.9, 12), (1.365, 15), (5.416, 19), (5.782, 21), (11.172, 24), (14.638, 27), (17.452, 29),
    (19.2, 33), (23.916, 36), (26.706, 40), (29.431, 42), (33.006, 46)), ((35.739, 47), (38.937, 51), (41.779,
    54), (45.752, 57), (47.863, 61), (50.474, 62), (53.833, 66), (56.742, 69), (61.708, 72), (62.833, 75),
    (65.346, 77), (68.926, 83), (71.975, 82), (74.997, 86), (78.06, 90), (81.178, 92)), ((84.39, None),
    (87.649, None), (89.394, None), (89.543, None)))
O2_PLANS = (((130.451, None), (134.449, None), (137.05, None), (137.656, None), (138.539, None), (140.057,
    None), (144.16, None)), ((141.38, None), (145.789, None), (145.843, None), (146.882, None), (149.928,
    None), (152.029, None), (152.297, None)), ((13.193, None), (22.336, None), (31.211, None), (39.891, None),
    (47.762, None), (56.772, None), (66.0, None)), ((27.948, None), (36.312, None), (43.877, None), (51.401,
    None), (58.218, None), (67.954, None), (76.139, None)))
PACK_PLANS = (((100.689, None), (101.244, None), (102.208, None), (102.296, None), (103.427, None), (104.581,
    None), (105.862, None), (106.631, None), (107.838, None), (108.106, None), (109.264, None), (109.501,
    None), (110.393, None), (111.052, None), (111.166, None), (111.572, None), (114.039, None), (114.221,
    None), (115.251, None), (116.905, None), (117.839, None), (118.037, None), (118.466, None), (118.897,
    None), (121.059, None), (121.354, None), (121.429, None), (122.756, None), (123.403, None), (124.242,
    None), (124.9, None), (125.882, None)), ((128.281, None), (128.956, None), (131.04, None), (131.514,
    None), (131.968, None), (132.635, None), (132.835, None), (133.941, None), (135.423, None), (136.25,
    None), (136.936, None), (137.657, None), (138.658, None), (139.06, None), (140.343, None), (141.492,
    None), (142.08, None), (142.473, None), (143.602, None), (143.8, None), (144.137, None), (146.083, None),
    (146.911, None), (147.792, None), (148.441, None), (148.723, None), (149.954, None), (151.061, None),
    (151.737, None), (152.867, None), (153.829, None), (154.519, None)))
PACKD_PLANS = (((0.956, None), (1.633, None), (4.36, None), (5.329, None), (7.571, None), (9.451, None),
    (9.768, None), (11.103, None), (12.795, None), (13.625, None), (14.575, None), (14.855, None), (19.475,
    None), (20.868, None), (21.935, None), (22.323, None), (25.31, None), (26.102, None), (28.561, None),
    (30.197, None), (31.978, None), (33.481, None)), ((34.174, None), (36.791, None), (38.947, None), (39.775,
    None), (42.179, None), (42.661, None), (46.568, None), (46.608, None), (49.436, None), (51.509, None),
    (51.641, None), (52.889, None), (53.189, None), (55.672, None), (56.222, None), (58.458, None), (60,
    None), (60, None)))
PACK_DUE = (130, 5, 39, 64)
DQA = 16 * len(PACKD_PLANS[0])
G_LAG = 5
D_LAG = 1
PLAIN_V0 = 1
LN2_GAPS = (1.13, 1.5, 0.2)
LN2_SPLIT = 4
PACK_W = 512
GAP_PACK = 0.2
LN1_GAPS = (1, 1.25)
GAP_PRO = 0.13
GAP_X = 0.2
GAP_WO = 0.2
GAP_O2 = 0.26
O_DUE = 6
MOE_NA = 36
MOE_ND = 2
MOE_LAGS = (2, 2)
STAGGER = 8

NN = (((1,), (0,)), ((), ()))
NT = (((1,), (1,)), ((), ()))


def _dot(a, b, dims):
    return lax.dot_general(a, b, dims, preferred_element_type=F32)


def _recip(x):
    return pl.reciprocal(x, approx=False, full_range=False)


def _pack(x):
    return pltpu.bitcast(x, U32)


def _unpack(x):
    return pltpu.bitcast(x, BF16)


def _strassen_lhs(a11, a12, a21, a22):
    return [a21 + a22, a22, a11 + a12, a11, a11 + a22, a12 - a22, a21 - a11]


def _strassen_rhs(b11, b12, b21, b22):
    return [b11, b21 - b11, b22, b12 - b22, b11 + b22, b21 + b22, b11 + b12]


def _strassen(product):
    m2 = product(0)
    m4 = product(1)
    c21 = m2 + m4
    m5 = product(2)
    u11 = m4 - m5
    m3 = product(3)
    c12 = m3 + m5
    u22 = m3 - m2
    m1 = product(4)
    u11 = u11 + m1
    u22 = u22 + m1
    c11 = product(5) + u11
    c22 = product(6) + u22
    return [[c11, c12], [c21, c22]]


def _strassen_rows_first(product, emit):
    m5 = product(2)
    m3 = product(3)
    emit(0, 1, m3 + m5)
    m4 = product(1)
    u11 = m4 - m5
    m1 = product(4)
    u11 = u11 + m1
    u22 = m3 + m1
    emit(0, 0, product(5) + u11)
    m2 = product(0)
    emit(1, 0, m2 + m4)
    u22 = u22 - m2
    emit(1, 1, product(6) + u22)


def _ordered(bits):
    return bits ^ ((bits >> 31) & 0x7FFF0000)


def _block(rows):
    return jnp.concatenate([jnp.concatenate(r, axis=1) for r in rows], axis=0)


def _pair_allreduce(a, op):
    a = op(a, pltpu.roll(a, 2, 0))
    return op(a, pltpu.roll(a, 4, 0))


def _tree(op, xs):
    xs = list(xs)
    while len(xs) > 1:
        nxt = [op(xs[i], xs[i + 1]) for i in range(0, len(xs) - 1, 2)]
        if len(xs) % 2:
            nxt.append(xs[-1])
        xs = nxt
    return xs[0]


def _pair_logits(sl, j):
    sub = lax.broadcasted_iota(jnp.int32, sl[0].shape, 0)
    if j < 3:
        head = jnp.where(sub < 2, 0.0, sl[(0, 1, 16)[j]])
    else:
        head = jnp.where(sub < 2, sl[0], jnp.where(sub < 4, pltpu.roll(sl[1], 2, 0),
                                                   jnp.where(sub < 6, pltpu.roll(sl[16], 4, 0), 0.0)))
    r0 = (2, 9, 17, 24)[j]
    return [head] + list(sl[r0:r0 + 7])


def _dual_exp(sl):
    mx = _pair_allreduce(_tree(jnp.maximum, sl), jnp.maximum)
    mn = _pair_allreduce(_tree(jnp.minimum, sl), jnp.minimum)
    ep = [jnp.exp2(s - mx) for s in sl]
    en = [jnp.exp2(mn - s) for s in sl]
    sp = _pair_allreduce(_tree(jnp.add, ep), jnp.add)
    sn = _pair_allreduce(_tree(jnp.add, en), jnp.add)
    return ep, en, sp, sn


def _after(x, never, anchor):
    if anchor is None:
        return x
    d = jnp.concatenate([anchor] * (x.shape[0] // 8), axis=0)
    if x.shape[1] == 128:
        return jnp.where(never, d, x)
    return jnp.concatenate([jnp.where(never, d, x[:, :128]), x[:, 128:]], axis=1)


def _gate(x, never, deps):
    for i, dep in enumerate(deps):
        d = jnp.broadcast_to(dep, (8, 128))
        if x.dtype != F32:
            d = pltpu.bitcast(d, x.dtype)
        blk = jnp.where(never, d, x[8 * i:8 * i + 8, :128])
        if x.shape[1] > 128:
            blk = jnp.concatenate([blk, x[8 * i:8 * i + 8, 128:]], axis=1)
        parts = ([x[:8 * i, :]] if i else []) + [blk, x[8 * i + 8:, :]]
        x = jnp.concatenate(parts, axis=0)
    return x


def _lane_fold(a):
    return _tree(jnp.add, [a[:, 128 * i:128 * i + 128] for i in range(a.shape[1] // 128)])


def _row_sum(a):
    return jnp.sum(_lane_fold(a), axis=-1, keepdims=True)


def _lane_tile(a, n):
    return a if n == 1 else jnp.concatenate([a] * n, axis=1)


def _sublane_allreduce(a):
    a = a + pltpu.roll(a, 4, 0)
    a = a + pltpu.roll(a, 2, 0)
    return a + pltpu.roll(a, 1, 0)


def _col_broadcast(row8):
    return jnp.concatenate([row8] * 16, axis=0).astype(BF16).T.astype(F32)


def _vpu_matvec(xb, w_rows, never, anchors, lag):
    ng = xb.shape[0] // 8
    acc, hist = None, []
    for g in range(ng):
        dep = anchors[(g * len(anchors)) // ng]
        if g >= lag:
            dep = dep + hist[g - lag]
        x = jnp.where(never, dep, xb[8 * g:8 * g + 8, :])
        w = w_rows(g)
        t = w * _lane_tile(x, w.shape[1] // 128)
        acc = t if acc is None else acc + t
        c = 128 * (g % (w.shape[1] // 128))
        hist.append(acc[:, c:c + 128])
    return acc


class _Side:
    def __init__(self, never, later=lambda rel, gap: rel + gap):
        self.never = never
        self.later = later
        self.jobs = []
        self.deps = {}
        self.hooks = {}

    def add(self, plan, fn):
        for k, (rel, due) in enumerate(plan):
            if rel is None:
                self._run(None, due, fn, k, None)
            else:
                self.jobs.append((rel, due, fn, k))

    def _run(self, rel, due, fn, k, anchor):
        gen = fn if hasattr(fn, "send") else fn(k, anchor)
        dep = gen
        if hasattr(gen, "send"):
            try:
                while True:
                    gap = gen.send(anchor) if gen is fn or rel is None and dep is None else next(gen)
                    if rel is not None:
                        self.jobs.append((self.later(rel, gap), due, gen, k))
                        return
                    dep = None
            except StopIteration as stop:
                dep = stop.value
        if due is not None:
            self.deps.setdefault(due, []).append(dep)

    def check(self):
        assert not self.jobs and not self.deps and not self.hooks

    def gate(self, step, x):
        return _gate(x, self.never, self.deps.pop(step, []))

    def done(self, step, res):
        m = res.shape[0] // 8
        while True:
            ready = [j for j in self.jobs if step - 1 < j[0] <= step]
            if not ready:
                break
            job = min(ready, key=lambda j: j[0])
            self.jobs.remove(job)
            g = m - 1 - int((step - job[0]) * m)
            self._run(*job, res[8 * g:8 * g + 8, res.shape[1] - 128:])
        for fn in self.hooks.pop(step, []):
            fn()


def _kernel(x_hbm, wqkv_hbm, wphi_hbm, wo_hbm, wr_hbm, wg_hbm, wu_hbm, wd_hbm, out_hbm,
            x_v, xn_v, xs_v, lead_v, wraw_v, wt_v, ws_v, wphi_v, a_v, woraw_v, wos_v, wrraw_v, wr_v,
            kvacc_v, kvbf_v, z_v, zb_v, phi_v, oc_v, oc2_v, h_v, hn_v, o_v, wg_v, wu_v, wd_v, stage_v,
            wgp_v, wup_v, wdp_v, patch_v,
            sem):
    SX, SQ, SO, SM = 0, 6, 6 + 3 * NC, 6 + 3 * NC + NT_ + 1

    def x_copy(i):
        h0, h1 = ((0, 1), (1, 2), (3, 4), (4, 8), (8, 2 * NT_), (2, 3))[i]
        rows = pl.ds(h0 * TH, (h1 - h0) * TH)
        return pltpu.make_async_copy(x_hbm.at[rows, :], x_v.at[rows, :], sem.at[SX + i])

    def k0_copy(s):
        return pltpu.make_async_copy(wqkv_hbm.at[:, pl.ds(D + s * 128, 128)],
                                     wraw_v.at[NC, :, pl.ds(s * 128, 128)], sem.at[(SM + 7, SQ + NC)[s]])

    def w_copy(j, c):
        return pltpu.make_async_copy(wqkv_hbm.at[:, pl.ds(j * D + c * RC, RC)], wraw_v.at[j * NC + c],
                                     sem.at[SQ + j * NC + c])

    def wphi_copy(i):
        h0, h1 = ((0, 8), (16, 24), (8, 16), (24, H))[i]
        return pltpu.make_async_copy(wphi_hbm.at[pl.ds(h0, h1 - h0)], wphi_v.at[pl.ds(h0, h1 - h0)],
                                     sem.at[(SM + 4, SM + 8, SM + 9, SM + 14)[i]])

    wr_copy = pltpu.make_async_copy(wr_hbm, wrraw_v, sem.at[SM + 5])

    def wo_copy(i):
        rows = pl.ds(0, WO_ROWS) if i == 0 else pl.ds(WO_ROWS, QK - WO_ROWS)
        return pltpu.make_async_copy(wo_hbm.at[:, rows, :], woraw_v.at[:, rows, :], sem.at[(SM + 6, SM + 15)[i]])

    wg_copy = pltpu.make_async_copy(wg_hbm.at[:, pl.ds(FM, FV)], wg_v, sem.at[SM + 0])
    wu_copy = pltpu.make_async_copy(wu_hbm.at[:, pl.ds(FM, FV)], wu_v, sem.at[SM + 1])
    wd_copy = pltpu.make_async_copy(wd_hbm.at[pl.ds(0, FVD), :], wd_v, sem.at[SM + 2])

    def stage_copy(i, q):
        if i < 2:
            r0 = q * (D // NQ)
            r0 = r0 if isinstance(r0, int) else pl.multiple_of(r0, D // NQ)
            src = (wg_hbm, wu_hbm)[i].at[pl.ds(r0, D // NQ), pl.ds(0, FM)]
        else:
            r0 = FVD + q * DQ + (i - 2) * DQA
            r0 = r0 if isinstance(r0, int) else pl.multiple_of(r0, 16)
            src = wd_hbm.at[pl.ds(r0, (DQA, DQ - DQA)[i - 2]), :]
        return pltpu.make_async_copy(src, stage_v[i].at[pl.ds(0, src.shape[0]), :], sem.at[SM + 10 + i])

    wphi_copy(0).start()
    k0_copy(0).start()
    x_copy(0).start()
    k0_copy(1).start()
    x_copy(1).start()
    wphi_copy(1).start()
    w_copy(1, 2).start()

    made = set()

    def view(ref, i, n, off=0):
        r0 = off + i * n
        return ref.at[pl.ds(r0 if isinstance(r0, int) else pl.multiple_of(r0, math.gcd(n, off)), n), :]

    def put_blocks(dst, r0, fn, m11, m12, m21, m22, never, a, skip=(), base=0, pitch=HK, gap=None):
        for c0 in range(0, m11.shape[1], 128):
            if c0:
                a = yield gap or GAP_PRO
            d11, d22 = m11[:, c0:c0 + 128], m22[:, c0:c0 + 128]
            if a is not None:
                d = jnp.concatenate([a, a], axis=0)
                d11, d22 = jnp.where(never, d, d11), jnp.where(never, d, d22)
            blocks = fn(d11, m12[:, c0:c0 + 128], m21[:, c0:c0 + 128], d22)
            for i, b in enumerate(blocks):
                if i not in skip:
                    dst[r0:r0 + 8, base + i * pitch + c0:base + i * pitch + c0 + 128] = _pack(b.astype(BF16))

    def rows16(ref, r0, c0=0, w=D):
        return _unpack(ref[r0:r0 + 8, c0:c0 + w]).astype(F32)

    def x_blocks(t, k, lo, hi, never, a, gap=None):
        yield from put_blocks(view(xs_v, t, TH // 2), k * LNC // 2, _strassen_rhs,
                              lo[:, :HK], hi[:, :HK], lo[:, HK:], hi[:, HK:], never, a, gap=gap)
        if isinstance(t, int):
            made.add(("xs", t, k))

    def ln_rows(t, k, n, never=None, anchor=None, plain=False):
        wide = lambda c, a: _lane_tile(_after(jnp.broadcast_to(c, (n, 128)), never, a), D // 128)
        x = _after(view(x_v, t, T)[k * n:(k + 1) * n, :].astype(F32), never, anchor)
        s1 = _row_sum(x)
        anchor = yield LN1_GAPS[0]
        xc = x - wide(s1 * (1.0 / D), anchor)
        rstd = lax.rsqrt(_row_sum(xc * xc) * (1.0 / D) + LN_EPS)
        anchor = yield LN1_GAPS[1]
        xn = xc * wide(rstd, anchor)
        if plain:
            xn_v[k * n // 2:(k + 1) * n // 2, :] = _pack(xn.astype(BF16))
        elif k * n < TH:
            xn_v[(T + k * n) // 2:(T + (k + 1) * n) // 2, :] = _pack(xn.astype(BF16))
        else:
            yield from x_blocks(t, k - TH // LNC, rows16(xn_v, (TH + k * n) // 2), xn, never, anchor, GAP_X)
        return _tree(jnp.add, [rstd[8 * i:8 * i + 8, :] for i in range(min(n, LNC) // 8)])

    def now(gen):
        try:
            while True:
                next(gen)
        except StopIteration as stop:
            return stop.value

    def late_x_blocks(t):
        return lambda k, a: x_blocks(t, k, rows16(xn_v, t * T // 2 + 8 * k),
                                     rows16(xn_v, (t * T + TH) // 2 + 8 * k), never0, a)

    def xn_tile(t):
        return _unpack(xn_v[t * T // 2:(t + 1) * T // 2, :])

    def xs_tile(t):
        assert not isinstance(t, int) or t > 1 or made >= {("xs", t, k) for k in range(8)}
        return _unpack(view(xs_v, t, TH // 2)[:, 0:7 * HK])

    def expand_wphi(c):
        w = wphi_v[8 * c:8 * c + 8].reshape(8 * DH, DH).astype(F32).T
        bits = pltpu.bitcast(w, U32)
        head = lax.broadcasted_iota(jnp.int32, (DH, 128), 1) >> 5
        for s in range(2):
            b = bits[:, 128 * s:128 * s + 128]
            for j in range(2):
                r0 = 64 * (2 * c + s) + 32 * j
                a_v[r0:r0 + 32, :] = jnp.where(head == 2 * j, b >> 16,
                                               jnp.where(head == 2 * j + 1, b, jnp.uint32(0)))

    wphi_copy(0).wait()
    expand_wphi(0)
    h_v[1][...] = jnp.zeros((T, D), F32)
    for ref in oc_v + oc2_v:
        ref[0:8, 0:128] = jnp.zeros((8, 128), U32)
    for ref in stage_v:
        ref[ref.shape[0] - 16:, 0:128] = jnp.zeros((16, 128), BF16)

    def v_transpose(k, a):
        q, r0 = (k // 8) + 4 * (k % 2), 256 * (k % 8 // 2)
        w = wraw_v[2 * NC + q // 2, r0:r0 + 256, (q % 2) * 128:(q % 2) * 128 + 128]
        if a is not None:
            w = _unpack(jnp.where(never0, jnp.concatenate([pltpu.bitcast(a, U32)] * 16, axis=0), _pack(w)))
        wt = _pack(w.T)
        wt_v[2][64 * q:64 * q + 64, r0:r0 + 256] = wt
        made.add(("vt", k))
        return pltpu.bitcast(wt[56:64, 128:256], F32)

    def fold_pairs(j, c, s, side=None, step0=None):
        g0 = 64 * (2 * c + s)
        g0 = g0 if isinstance(g0, int) else pl.multiple_of(g0, 64)
        res = _dot(_unpack(a_v[pl.ds(g0, 64), :]), wraw_v[j * NC + c, :, s * 128:(s + 1) * 128], NT)
        if side is not None:
            side.done(step0 + 2 * s, res[:, :D // 2])
            side.done(step0 + 2 * s + 1, res[:, D // 2:])
        sub = lax.broadcasted_iota(jnp.int32, (8, D), 0)
        out = []
        for q in range(2):
            base = _pair_allreduce(jnp.where(sub < 2, res[64 * q:64 * q + 8, :], 0.0), jnp.add)
            out.append([(res[64 * q + 8 * i:64 * q + 8 * i + 8, :] - base) * LOG2E for i in range(8)])
        return out

    def share(z, z3, k):
        sub = lax.broadcasted_iota(jnp.int32, (8, D), 0)
        return jnp.where(sub < 2, pltpu.roll(z3, 8 - 2 * k, 0), z)

    def packed(slabs):
        return _pack(jnp.concatenate(slabs, axis=0).astype(BF16))

    def fold(j, c, side=None, step0=None):
        p0, p1 = fold_pairs(j, c, 0, side, step0)
        p2, p3 = fold_pairs(j, c, 1, side, step0)
        sl = ([share(p0[0], p3[0], 1), share(p1[0], p3[0], 2)] + p0[1:] + p1[1:]
              + [share(p2[0], p3[0], 3)] + p2[1:] + p3[1:])
        zero = jnp.zeros((8, D), F32)
        even, odd = sl + [zero], [zero] + sl
        r0 = 8 * ((31 * c) // 2)
        is_odd = c % 2 == 1
        if isinstance(c, int):
            sl = odd if is_odd else even
        else:
            r0 = pl.multiple_of(r0, 8)
            sl = [jnp.where(is_odd, o, e) for o, e in zip(odd, even)]
        win = wt_v[j].at[pl.ds(r0, 128), :]
        win[8:128, :] = packed(sl[2:])
        first = packed(sl[:2])
        if is_odd is not False:
            keep = lax.broadcasted_iota(jnp.int32, (8, D), 0) < jnp.where(is_odd, 4, 0)
            first = jnp.where(keep, win[0:8, :], first)
        win[0:8, :] = first
        made.update(("fold", j, q) for q in ([c] if isinstance(c, int) else range(3)))

    def w_blocks(j, k0=0):
        def job(k, a):
            k += k0
            assert made >= ({("vt", 8 * (k // 8) + q) for q in range(8)} if j == 2 else
                            {("fold", j, q) for q in ((0, 2) if k < 15 else range(4))})
            lo, hi = rows16(wt_v[j], 8 * k), rows16(wt_v[j], (256 if j == 2 else 248) + 8 * k)
            yield from put_blocks(ws_v[j], 8 * k, _strassen_lhs, lo[:, :HK], lo[:, HK:], hi[:, :HK], hi[:, HK:],
                                  never0, a, skip=(1, 3))
            made.add(("ws", j, k))
        return job

    def k_pair(p, slot, pr, c0, never=None):
        first = ("z", pr, c0) not in made
        for n in range(c0, c0 + p[0].shape[1], 128):
            assert first == (("z", pr, n) not in made)
            made.update({("z", pr, n), ("phi", slot, pr, n)})
        ep, en, sp, sn = _dual_exp(p)
        inv = _recip(sp * sn)
        scale = (sn * inv, sp * inv)
        es = ep + en
        cols = slice(c0, c0 + p[0].shape[1])
        n = 16 if never is None else 16 // STAGGER
        last = None
        for q in range(16 // n):
            sc = scale
            if last is not None:
                sc = [jnp.where(never, last, x) for x in scale]
            phi = jnp.concatenate([es[i] * sc[i // 8] for i in range(q * n, (q + 1) * n)], axis=0)
            rows = slice(8 * q * n, 8 * (q + 1) * n)
            z = phi if first else z_v[pr, rows, cols] + phi
            z_v[pr, rows, cols] = z
            phi_v[slot][64 * pr + 4 * q * n:64 * pr + 4 * (q + 1) * n, cols] = _pack(phi.astype(BF16))
            last = z[8 * n - 8:, :]

    def kv_update(vts, slot, g, first, publish=False):
        for q, vt in enumerate(vts):
            for j in range(2):
                pr = 2 * g + 8 * q + j
                assert made >= {("phi", slot, pr, 0), ("phi", slot, pr, 128)}
                upd = _dot(vt[64 * j:64 * j + 64, :].astype(BF16), _unpack(phi_v[slot][64 * pr:64 * pr + 64, :]), NT)
                acc = upd if first else kvacc_v[pr] + upd
                kvacc_v[pr] = acc
                if publish:
                    odd = -(lax.broadcasted_iota(jnp.int32, (32, 128), 1) & 1)
                    bits = pltpu.bitcast(acc, jnp.int32) & jnp.concatenate([~odd, odd], axis=0)
                    kvbf_v[32 * pr:32 * pr + 32, :] = _pack(pltpu.bitcast(bits, F32).astype(BF16))

    def save_lead(t):
        view(lead_v, t, HK // 2)[...] = _pack(_unpack(view(xs_v, t, TH // 2)[:, 0:HK]).T)

    def proj_feat(side, step0, c, xn):
        r0 = 8 * ((31 * c) // 2)
        w = wt_v[1][r0:r0 + 128, :]
        quarters = []
        for n in range(2):
            for m in range(2):
                step = step0 + 2 * n + m
                wq = _unpack(side.gate(step, w[:64, :] if m == 0 else w[64:, :]))
                res = _dot(wq, xn[n * TH:(n + 1) * TH, :], NT)
                side.done(step, res)
                quarters.append(res)
        res = jnp.concatenate(
            [jnp.concatenate([quarters[0], quarters[2]], axis=1),
             jnp.concatenate([quarters[1], quarters[3]], axis=1)], axis=0)
        sl = [res[8 * i:8 * i + 8, :] for i in range(res.shape[0] // 8)]
        return sl[c % 2:31 + c % 2]

    def proj_unit(side, step0, j, b, xs, lead=None, plain=None):
        r1 = 64 * b + (64 if j == 2 or b < 3 else 56)
        assert made >= ({("vt", 8 * b + q) for q in range(8)} if plain is not None else
                        {("ws", j, k) for k in range(8 * b, r1 // 8)})
        if plain is not None:
            out = []
            for q in range(2):
                row = []
                for n in range(2):
                    steps = range((0, 2, 4, 5)[2 * q + n], (2, 4, 5, 7)[2 * q + n])
                    deps = [d for i in steps for d in side.deps.pop(step0 + i, [])]
                    w = _gate(wt_v[2][256 * q + 64 * b:256 * q + r1, :], side.never, deps)
                    res = _dot(_unpack(w), plain[n * TH:(n + 1) * TH, :], NT)
                    for i in steps:
                        side.done(step0 + i, res)
                    row.append(res)
                out.append(jnp.concatenate(row, axis=1))
            return out

        def product(i):
            off = 256 if j == 2 else 248
            w = (wt_v[j][off + 64 * b:off + r1, HK:] if i == 1 else wt_v[j][64 * b:r1, :HK] if i == 3
                 else ws_v[j][64 * b:r1, i * HK:(i + 1) * HK])
            w = _unpack(side.gate(step0 + i, w))
            if lead is not None and i == 0:
                res = _dot(w, _unpack(view(lead_v, lead, HK // 2)[...]), NN)
            else:
                res = _dot(w, xs[:, i * HK:(i + 1) * HK], NT)
            side.done(step0 + i, res)
            return res
        return [jnp.concatenate(row, axis=1) for row in _strassen(product)]

    def feat_stage(side, step0, j, xs, pair_fn, lead=None, units=range(4), sl=None, hold=None):
        sl = sl or [[], []]
        for b in units:
            for q, res in enumerate(proj_unit(side, step0 + 7 * b, j, b, xs, lead if b == units[0] else None)):
                sl[q] += [res[8 * i:8 * i + 8, :] for i in range(res.shape[0] // 8)]
            for q in (1, 0):
                for jj in (2 * (b % 2), 2 * (b % 2) + 1):
                    if b != hold:
                        pair_fn(_pair_logits(sl[q][31 * (b // 2):], jj), 8 * q + 4 * (b // 2) + jj)
        return sl

    def v_stage(side, xs, slot, first, publish, lead, plain=None):
        pending = None
        for g in range(4):
            if pending is not None:
                side.hooks.setdefault(7 * g + D_LAG, []).append(lambda p=pending: kv_update(*p))
            pending = (proj_unit(side, 7 * g, 2, g, xs, lead if g == 0 else None, plain if g < PLAIN_V0 else None),
                       slot, g, first, publish)
        side.check()
        return pending

    def pack_rows(src, dst, r0, c0, cols, never, a):
        for c in range(c0, c0 + cols, PACK_W):
            if c > c0:
                a = yield GAP_PACK
            w = min(PACK_W, c0 + cols - c)
            v = src[r0:r0 + 16, c:c + w].astype(F32)
            v = jnp.concatenate([jnp.where(never, _lane_tile(a, w // 128), v[0:8, :]), v[8:16, :]], axis=0)
            dst[r0 // 2:r0 // 2 + 8, c:c + w] = _pack(v.astype(BF16))

    def stash_at(i, k, n):
        return zb_v.at[4 * i + 2 * (k // 16) + n, pl.ds(8 * (k % 16), 8), :]

    def stash(i, sl):
        for k, v in enumerate(sl):
            for n in range(2):
                stash_at(i, k, n)[...] = v[:, 128 * n:128 * n + 128]

    def stashed_k(i, slot, c):
        def job(k, a):
            j, n = k // 2, k % 2
            p = _pair_logits([stash_at(i, q, n)[...] for q in range(16 if j < 2 else 31)], j)
            k_pair([_after(p[0], never0, a)] + p[1:], slot, c * PPC + j, 128 * n, never0)
        return job

    def first_rows(k0, k1, n):
        xn = _unpack(xn_v[n * TH // 2:(n + 1) * TH // 2, :])
        ks = [k for k in range(k0, k1)]
        w = jnp.concatenate([wt_v[1][4 * (k % 32):4 * (k % 32) + 8, :] for k in ks[::2]], axis=0)
        res = _dot(_unpack(w), xn, NT)
        for q, k in enumerate(ks):
            if k % 32 < 31:
                stash_at(0, k % 32, n)[...] = res[8 * q:8 * q + 8, :]

    k0_copy(0).wait()
    x_copy(0).wait()
    wphi_copy(2).start()
    x_copy(5).start()
    w_copy(1, 1).start()
    wphi_copy(3).start()
    x_copy(2).start()
    p0, p1 = fold_pairs(1, 0, 0)
    wt_v[1][8:64, :] = packed(p0[1:] + p1[1:])
    h_v[0][0:8, :] = p0[0]
    h_v[0][8:16, :] = p1[0]
    never0 = now(ln_rows(0, 0, TH, plain=True))[0, 0] < 0.0
    first_rows(2, 16, 0)

    k0_copy(1).wait()
    x_copy(1).wait()
    wphi_copy(1).wait()
    w_copy(1, 3).start()
    for c in (0, 2, 1, 3):
        w_copy(2, c).start()
    p2, p3 = fold_pairs(1, 0, 1)
    wt_v[1][0:8, :] = packed([share(h_v[0][0:8, :], p3[0], 1), share(h_v[0][8:16, :], p3[0], 2)])
    wt_v[1][64:128, :] = packed([share(p2[0], p3[0], 3)] + p2[1:] + p3[1:] + [jnp.zeros((8, D), F32)])
    made.add(("fold", 1, 0))
    now(ln_rows(0, 1, TH, plain=True))
    first_rows(16, 34, 0)
    first_rows(0, 16, 1)
    first_rows(16, 32, 1)
    expand_wphi(2)

    def slow(end):
        return lambda rel, gap: min(rel + (gap / 2 if 3 <= rel < 7 else gap), end)

    for c, prev in ((2, 0), (1, 2)):
        w_copy(1, c).wait()
        wphi_copy(4 - c).wait()
        side = _Side(never0, slow(7))
        if c == 1:
            x_copy(5).wait()
            side.add(PRO_LN_PLANS0, lambda k, a: ln_rows(1, k, LNC, never0, a))
        expand_wphi(5 - 2 * c)
        side.add((PRO_W_PLANS0, PRO_W_PLANS1)[2 - c], w_blocks(1, (2 - c) * len(PRO_W_PLANS0)))
        side.add((PRO_K_PLANS0, PRO_K_PLANS1)[2 - c], stashed_k(prev, 0, prev))
        fold(1, c, side, 0)
        stash(c, proj_feat(side, 4, c, xn_tile(0)))
        side.check()

    x_copy(2).wait()
    w_copy(1, 3).wait()
    x_copy(3).start()
    w_copy(0, 0).start()
    wo_copy(0).start()
    x_copy(4).start()
    side = _Side(never0, slow(28))
    side.add(PRO_LN_PLANS1, lambda k, a: ln_rows(1, k + 8, LNC, never0, a))
    side.add(PRO_W_PLANS2, w_blocks(1, 31 - len(PRO_W_PLANS2)))
    side.add(PRO_K_PLANS2, stashed_k(1, 0, 1))
    side.add(PRO_X0_PLAN, late_x_blocks(0))
    fold(1, 3, side, 0)
    stash(3, proj_feat(side, 4, 3, xn_tile(0)))
    k1 = lambda p, pr: k_pair(p, 1, pr, 0, never0)
    for q, sl in enumerate(feat_stage(side, 8, 1, xs_tile(1), k1, units=range(3), hold=2)):
        stash(2 * q, sl[31:])
    side.check()
    save_lead(1)

    for c in range(NC):
        w_copy(2, c).wait()
    side = _Side(never0, lambda rel, gap: min(rel + gap, 27))
    side.add(PRO_V_PLANS[0], v_transpose)
    side.add(PRO_V_PLANS[1], stashed_k(3, 0, 3))
    side.add(PRO_V_PLANS[2], stashed_k(0, 1, 1))
    side.add(PRO_V_PLANS[3], stashed_k(2, 1, 3))
    side.add(PRO_V_PLANS[4], w_blocks(2))
    sl = [[None] * 31 + [jnp.concatenate([stash_at(2 * q, k, n)[...] for n in range(2)], axis=1) for k in range(17)]
          for q in range(2)]
    feat_stage(side, -28, 1, xs_tile(1), k1, 1, units=range(3, 4), sl=sl)
    kv_update(*v_stage(side, xs_tile(0), 0, True, False, None, xn_tile(0)))
    save_lead(0)
    for c in range(1, NC):
        w_copy(0, c).start()
    wo_copy(1).start()
    wr_copy.start()
    for i in range(4):
        stage_copy(i, 0).start()
    wg_copy.start()
    wu_copy.start()
    wd_copy.start()
    for r0 in (0, 248):
        wt_v[0][r0:r0 + 8, :] = jnp.zeros((8, D), U32)

    def phase1(u, carry):
        never = u < 0

        @pl.when(u == 0)
        def _():
            x_copy(3).wait()
            w_copy(0, 0).wait()
            wo_copy(0).wait()

        @pl.when(u == 1)
        def _():
            x_copy(4).wait()
            w_copy(0, 1).wait()
            w_copy(0, 2).wait()
            wo_copy(1).wait()

        def wo_blocks(k0):
            def job(k, a):
                k += k0
                r, c, part = k // 4, 128 * (k // 2 % 2), k % 2
                r0 = u * ((QK - WO_ROWS) // 2)
                dst = wos_v.at[pl.ds(pl.multiple_of(r0 // 2, 8), WO_ROWS // 2), :]

                def piece(kq, nq):
                    src = woraw_v.at[kq, pl.ds(pl.multiple_of(r0, 16), WO_ROWS), :]
                    return src[16 * r:16 * r + 16, nq * QK + c:nq * QK + c + 128].astype(F32)
                outer = [_strassen_rhs(piece(ki, ni), piece(ki, 2 + ni), piece(2 + ki, ni), piece(2 + ki, 2 + ni))
                         for ki in range(2) for ni in range(2)]
                for i in range(4) if part == 0 else range(4, 7):
                    if i % 4:
                        a = yield GAP_WO
                    yield from put_blocks(dst, 8 * r, _strassen_rhs, *[o[i] for o in outer], never, a,
                                          base=7 * i * QK + c, pitch=QK)
            return job

        xs = xs_tile(2 * u + 1)
        side = _Side(never, lambda rel, gap: min(rel + gap, 27))
        for i in range(2):
            t = 2 * u + 2 + i
            if i == 0:
                side.add(LN1_PLANS[0], lambda k, a: ln_rows(2 * u + 2, k, LNC, never, a))
                side.add(WO_PLANS[0], wo_blocks(0))
            pending = v_stage(side, xs, 1 - i, False, False, t - 1 if i == 0 else None)
            xs = xs_tile(t)
            side = _Side(never, lambda rel, gap, end=(27, -1)[i]: min(rel + gap, end))
            if i == 0:
                side.add(LN1_PLANS[1], lambda k, a: ln_rows(2 * u + 3, k, LNC, never, a))
                side.add(WO_PLANS[1], wo_blocks(len(WO_PLANS[0])))
            else:
                side.add(WO_PLANS[2], wo_blocks(24 - len(WO_PLANS[2])))
            side.hooks[-28 + D_LAG] = [lambda p=pending: kv_update(*p)]
            feat_stage(side, -28, 1, xs, lambda p, pr: k_pair(p, i, pr, 0, never if i == 1 else None))
            save_lead(t)
        side.check()
        fold(0, u)
        return carry

    lax.fori_loop(0, (NT_ - 2) // 2, phase1, 0)

    w_copy(0, 3).wait()
    wr_copy.wait()
    side = _Side(never0, lambda rel, gap: min(rel + gap, 27 if rel < 98 else 103))

    def z_final(k, a):
        zb_v[k] = jnp.broadcast_to(_row_sum(_after(z_v[k], never0, a)), (128, 128))

    side.add(END_PLANS[0], z_final)
    side.add(END_PLANS[1], w_blocks(0))
    side.hooks[0] = [lambda: fold(0, 3, side, 100)]
    kv_update(*v_stage(side, xs_tile(NT_ - 1), 1, False, True, NT_ - 1))
    wr_v[...] = jnp.broadcast_to(wrraw_v[...].reshape(1, D).astype(F32), (8, D))

    def o_copy(r0, n, i):
        return pltpu.make_async_copy(o_v.at[pl.ds(r0, n), :], out_hbm.at[pl.ds(r0, n), :], sem.at[SO + i])

    def finish_rows(h_ref, k, t, valid, st, never=None, anchor=None):
        r0 = t * T + k * LNC
        rows = slice(k * LNC, (k + 1) * LNC)
        m = jnp.broadcast_to(_row_sum(_after(h_ref[rows, :], never, anchor)) * (1.0 / D), (LNC, 128))
        rstd, r = [], []
        for i in range(LNC // 8):
            anchor = yield LN2_GAPS[2] if i else LN2_GAPS[0]
            mi = _after(m[8 * i:8 * i + 8, :], never, anchor)
            hc = h_ref[k * LNC + 8 * i:k * LNC + 8 * i + 8, :] - _lane_tile(mi, D // 128)
            rs = lax.rsqrt(_row_sum(hc * hc) * (1.0 / D) + LN_EPS)
            r.append((_row_sum(hc * wr_v[...]) * rs + 0.0).astype(BF16).astype(F32))
            rstd.append(jnp.broadcast_to(rs, (8, 128)))
        rstd = jnp.concatenate(rstd, axis=0)
        w = D if never is None else D // LN2_SPLIT
        for c in range(0, D, w):
            anchor = yield LN2_GAPS[2] if c else LN2_GAPS[1]
            h = h_ref[rows, c:c + w]
            hn = (h - _lane_tile(_after(m, never, anchor), w // 128)) * _lane_tile(rstd, w // 128)
            view(hn_v, t, T // 2)[k * LNC // 2:(k + 1) * LNC // 2, c:c + w] = _pack(hn.astype(BF16))
            view(o_v, t, T)[rows, c:c + w] = (hn + h).astype(BF16)
        best = st["route"]
        sub = lax.broadcasted_iota(jnp.int32, (8, 128), 0)
        for i, ri in enumerate(r):
            key = _ordered(pltpu.bitcast(jnp.broadcast_to(ri, (8, 128)), jnp.int32)) | ((S - 1 - r0 - 8 * i) - sub)
            if valid is not None:
                key = jnp.where(valid, key, KEY_MIN)
            best = jnp.maximum(best, key)
        st["route"] = best
        return pltpu.bitcast(best, F32)

    def q_pair(p, slot, pr):
        ep, en, sp, sn = _dual_exp(p)
        zz = [_lane_tile(zb_v[pr, 8 * i:8 * i + 8, :], T // 128) for i in range(16)]
        ap = _pair_allreduce(_tree(jnp.add, [ep[i] * zz[i] for i in range(8)]), jnp.add)
        an = _pair_allreduce(_tree(jnp.add, [en[i] * zz[8 + i] for i in range(8)]), jnp.add)
        inv = _recip(ap * sn + (an + 1e-6 * sn) * sp)
        rp = sn * inv
        rn = sp * inv
        phi = jnp.concatenate([e * rp for e in ep] + [e * rn for e in en], axis=0)
        phi_v[slot][64 * pr:64 * pr + 64, :] = _pack(phi.astype(BF16))

    held = []

    def attn_blocks(slot, g, deps):
        res = [_dot(_unpack(kvbf_v[32 * pr:32 * pr + 32, :]), _unpack(phi_v[slot][64 * pr:64 * pr + 64, :]), NN)
               for pr in (2 * g, 2 * g + 8, 2 * g + 1, 2 * g + 9)]
        lo, hi = jnp.concatenate(res[0::2], axis=0), jnp.concatenate(res[1::2], axis=0)
        blocks = [(i, g, b) for i, b in enumerate(_strassen_lhs(lo[:, :TH], hi[:, :TH], lo[:, TH:], hi[:, TH:]))]
        if g % 2 == 0:
            held.append(blocks.pop())
        else:
            blocks.append(held.pop())
        ot = _pack(jnp.concatenate([b for _, _, b in blocks], axis=1).astype(BF16).T)
        for q, (i, n, _) in enumerate(blocks):
            oc_v[slot][:, i * HK + 128 * n:i * HK + 128 * n + 128] = ot[q * TH // 2:(q + 1) * TH // 2, :]
            made.add(("oc", slot, i, n))
            if q % 2:
                deps.append(pltpu.bitcast(ot[(q + 1) * TH // 2 - 8:(q + 1) * TH // 2, :], F32))

    def o_blocks(slot, c, never):
        def job(k, a):
            k = (2, 3, 1, 4, 5, 0, 6)[k]
            assert made >= {("oc", slot, k, c), ("oc", slot, k, c + 2)}
            for r in range(4):
                if r:
                    a = yield GAP_O2
                m = [rows16(oc_v[slot], 8 * r + 32 * q, k * HK + n * QK + 128 * c, 128)
                     for q in range(2) for n in range(2)]
                yield from put_blocks(oc2_v[slot], 8 * r, _strassen_lhs, *m, never, a, skip=(1, 3),
                                      base=7 * k * QK + 128 * c, pitch=QK)
            made.add(("oc2", slot, k, c))
        return job

    def out_proj(side, step0, t, slot):
        count = [0]

        def inner(i, c):
            assert made >= {("oc2", slot, i, 0), ("oc2", slot, i, 1)}

            def product(j):
                step, odd = step0 + count[0] // 2, count[0] % 2
                count[0] += 1
                o = (oc_v[slot][32:64, i * HK + QK:(i + 1) * HK] if j == 1 else
                     oc_v[slot][0:32, i * HK:i * HK + QK] if j == 3 else
                     oc2_v[slot][:, (7 * i + j) * QK:(7 * i + j + 1) * QK])
                w = wos_v[:, (7 * i + j) * QK + 128 * c:(7 * i + j) * QK + 128 * c + 128]
                res = _dot(_unpack(o), _unpack(w if odd else side.gate(step, w)), NN)
                if odd:
                    side.done(step, res)
                return res
            return _block(_strassen(product))

        xt = view(x_v, t, T)

        def emit(q, r, res):
            for c in range(2):
                for n in range(2):
                    rows, c0 = slice(q * TH, (q + 1) * TH), r * HK + n * QK + 128 * c
                    h_v[slot][rows, c0:c0 + 128] = (res[:, 256 * c + 128 * n:256 * c + 128 * n + 128]
                                                    + xt[rows, c0:c0 + 128].astype(F32))
            made.add(("h", slot, q, r))

        _strassen_rows_first(lambda i: jnp.concatenate([inner(i, c) for c in range(2)], axis=1), emit)

    def phase2(u, carry):
        made.difference_update({m for m in made if m[0] in ("h", "oc", "oc2")})
        for i in range(4):
            stage_copy(i, u).wait()
        never = u < 0
        side = _Side(never, lambda rel, gap: min(rel + 2 * gap, 97) if rel < 98 else
                     rel + gap if rel + gap <= 155 else 2 * (rel + gap - 155) - 1)
        st = {"route": carry}
        tp = jnp.maximum(2 * u - 1, 0)
        early = len(LN2_PLANS[2])

        def ln2(slot, t, valid, k0, key):
            def job(k, a):
                k += k0
                hs = {("h", slot, k // 8, r) for r in range(2)}
                assert made >= hs or key == 0
                best = yield from finish_rows(h_v[slot], k, t, valid, st, never, a)
                assert key > 0 or not made & hs
                return best
            return job

        side.add(LN2_PLANS[0], ln2(1, tp, u > 0, early, 0))
        side.add(LN2_PLANS[1], ln2(0, 2 * u, None, 0, 1))
        side.add(LN2_PLANS[2], ln2(1, 2 * u + 1, None, 0, 2))

        def packer(i, dst, n):
            left = [n]

            def job(k, a):
                if i < 2:
                    yield from pack_rows(stage_v[i], dst, (k // 2) * 16, (0, D)[k % 2], (D, FM - D)[k % 2], never, a)
                else:
                    yield from pack_rows(stage_v[i], dst, k * 16, 0, D, never, a)
                left[0] -= 1
                if not left[0]:
                    stage_copy(i, jnp.minimum(u + 1, NQ - 1)).start()
                    n0 = stage_v[i].shape[0] - 16
                    side.deps.setdefault(PACK_DUE[i], []).append(stage_v[i][n0:n0 + 8, 0:128].astype(F32))
            return job

        for i in range(2):
            side.add(PACK_PLANS[i], packer(i, view((wgp_v, wup_v)[i], u, D // NQ // 2), len(PACK_PLANS[i])))
            d0 = pl.multiple_of(u * (DQ // 2) + i * (DQA // 2), 8)
            side.add(PACKD_PLANS[i], packer(2 + i, wdp_v.at[pl.ds(d0, 8 * len(PACKD_PLANS[i])), :],
                                            len(PACKD_PLANS[i])))
            for g in range(4):
                step = 107 + 28 * i + 7 * g + G_LAG
                wrap = lambda x: x if x < 156 else 2 * (x - 156) + 1
                side.hooks.setdefault(wrap(step), []).append(
                    lambda i=i, g=g, due=wrap(step + O_DUE): attn_blocks(i, g, side.deps.setdefault(due, [])))
            for c in range(2):
                side.add(O2_PLANS[2 * i + c], o_blocks(i, c, never))
        for i in range(2):
            feat_stage(side, 100 + 28 * i, 0, xs_tile(2 * u + i), lambda p, pr: q_pair(p, i, pr),
                       2 * u if i == 0 else None)
        for i in range(2):
            out_proj(side, 49 * i, 2 * u + i, i)
        side.check()

        @pl.when(u == 0)
        def _():
            o_copy(0, T, 0).start()

        @pl.when(u > 0)
        def _():
            o_copy(pl.multiple_of(tp * T, T), 2 * T, u).start()

        return st["route"]

    wg_copy.wait()
    wu_copy.wait()
    wd_copy.wait()
    route = lax.fori_loop(
        0, NT_ // 2, phase2,
        jnp.full((8, 128), KEY_MIN, jnp.int32))
    st = {"route": route}
    for k in range(len(LN2_PLANS[2]), T // LNC):
        now(finish_rows(h_v[1], k, NT_ - 1, None, st))
    o_copy(S - T, T, NT_).start()

    best = st["route"]
    for shift in (4, 2, 1):
        best = jnp.maximum(best, pltpu.roll(best, shift, 0))
    idx_s = (S - 1) - (best[0, 0] & (S - 1))
    gate = _lane_tile(jax.nn.sigmoid(pltpu.bitcast(_ordered(best & -65536), F32)), D // 128)
    blk = pl.multiple_of(jnp.clip((idx_s >> 4) << 4, 0, S - 16), 16)
    pair = jnp.broadcast_to(hn_v[pl.ds(jnp.clip(idx_s >> 1, 0, S // 2 - 1), 1), :], (8, D))
    x8 = pltpu.bitcast(jnp.where((idx_s & 1) == 1, pair & jnp.uint32(0xFFFF0000), pair << 16), F32)
    xs = jnp.concatenate([x8, x8], axis=0).astype(BF16)
    acts, anchors = [], []

    def park(v, half):
        n = v.shape[0] // 128
        for i in range(n):
            z_v[i, :, 128 * half:128 * half + 128] = v[128 * i:128 * i + 128, :]
        return jnp.concatenate([z_v[i, :, 128 * half:128 * half + 128] for i in range(n)], axis=0)

    for c0 in range(0, FM, 128):
        g = _dot(xs, _unpack(wgp_v[:, c0:c0 + 128]), NN)[0:8, :]
        u = _dot(xs, _unpack(wup_v[:, c0:c0 + 128]), NN)[0:8, :]
        anchors += [g, u]
        acts.append(g * jax.nn.sigmoid(g) * u)
    xb = park(_col_broadcast(x8), 0)
    g, u = [_sublane_allreduce(_vpu_matvec(
        xb, lambda g: w[8 * g:8 * g + 8, :].astype(F32), never0,
        anchors[i * MOE_NA // 2:(i + 1) * MOE_NA // 2], MOE_LAGS[0])) for i, w in enumerate((wg_v, wu_v))]
    acts.append(g * jax.nn.sigmoid(g) * u)
    a = jnp.concatenate(acts, axis=1)
    am = jnp.concatenate([a[:, FVD:], a[:, FVD:]], axis=0).astype(BF16)
    ys, anchors = [], anchors[MOE_NA:]
    for k0 in range(0, FF - FVD, 512):
        k1 = min(k0 + 512, FF - FVD)
        yk = _dot(am[:, k0:k1], _unpack(wdp_v[k0 // 2:k1 // 2, 0:D]), NN)[0:8, :]
        ys.append(yk)
        anchors += [yk[:, c:c + 128] for c in range(128, D, 256)]
    ys.append(_sublane_allreduce(_vpu_matvec(
        park(_col_broadcast(a[:, :FVD]), 1), lambda g: wd_v[8 * g:8 * g + 8, :].astype(F32), never0,
        anchors[:-MOE_ND], MOE_LAGS[1])))
    y = _tree(jnp.add, ys) * gate
    y = jnp.concatenate([y, y], axis=0)
    sel = lax.broadcasted_iota(jnp.int32, (16, 1), 0) == (idx_s - blk)
    patch_v[...] = (o_v[pl.ds(blk, 16), :].astype(F32) + jnp.where(sel, y, 0.0)).astype(BF16)
    o_copy(0, T, 0).wait()
    for u in range(1, NT_ // 2):
        o_copy((2 * u - 1) * T, 2 * T, u).wait()
    o_copy(S - T, T, NT_).wait()
    pc = pltpu.make_async_copy(patch_v, out_hbm.at[pl.ds(blk, 16), :], sem.at[SM + 3])
    pc.start()
    for i in range(4):
        stage_copy(i, NQ - 1).wait()
    pc.wait()


@jax.jit
def pallas_sequential_preLN__linear_kernel_hedgehog__moe_arch_mod__prompt_kernel(
    A_x: jax.Array,
    A_wqkv: jax.Array,
    A_w_phi: jax.Array,
    A_wo: jax.Array,
    B_x: jax.Array,
    B_w_r: jax.Array,
    B_w_gate: jax.Array,
    B_w_up: jax.Array,
    B_w_down: jax.Array,
):
    del B_x
    hbm = pl.BlockSpec(memory_space=pl.ANY)
    out = pl.pallas_call(
        _kernel,
        out_shape=jax.ShapeDtypeStruct((S, D), BF16),
        in_specs=[hbm] * 8,
        out_specs=hbm,
        scratch_shapes=[
            pltpu.VMEM((S, D), BF16),
            pltpu.VMEM(((T + TH) // 2, D), U32),
            pltpu.VMEM((NT_ * TH // 2, SW), U32),
            pltpu.VMEM((NT_ * HK // 2, 128), U32),
            pltpu.VMEM((3 * NC, D, RC), BF16),
            [pltpu.VMEM((D // 2, D), U32)] * 3,
            [pltpu.VMEM((HK // 2, 7 * HK), U32)] * 3,
            pltpu.VMEM((H, DH, DH), BF16),
            pltpu.VMEM((8 * 64, 128), U32),
            pltpu.VMEM((4, QK, D), BF16),
            pltpu.VMEM((QK // 2, 49 * QK + 128), U32),
            pltpu.VMEM((D,), BF16),
            pltpu.VMEM((8, D), F32),
            pltpu.VMEM((NPAIR, 64, 128), F32),
            pltpu.VMEM((NPAIR * 32, 128), U32),
            pltpu.VMEM((NPAIR, 128, T), F32),
            pltpu.VMEM((NPAIR, 128, 128), F32),
            [pltpu.VMEM((NPAIR * 64, T), U32)] * 2,
            [pltpu.VMEM((TH // 2, 7 * HK), U32)] * 2,
            [pltpu.VMEM((TH // 4, 49 * QK), U32)] * 2,
            [pltpu.VMEM((T, D), F32)] * 2,
            pltpu.VMEM((S // 2, D), U32),
            pltpu.VMEM((S, D), BF16),
            pltpu.VMEM((D, FV), BF16),
            pltpu.VMEM((D, FV), BF16),
            pltpu.VMEM((FVD, D), BF16),
            [pltpu.VMEM((D // NQ + 16, FM), BF16), pltpu.VMEM((D // NQ + 16, FM), BF16),
             pltpu.VMEM((DQA + 16, D), BF16), pltpu.VMEM((DQ - DQA + 16, D), BF16)],
            pltpu.VMEM((D // 2, FM), U32),
            pltpu.VMEM((D // 2, FM), U32),
            pltpu.VMEM(((FF - FVD) // 2, D + 128), U32),
            pltpu.VMEM((16, D), BF16),
            pltpu.SemaphoreType.DMA((6 + 3 * NC + NT_ + 17,)),
        ],
        compiler_params=pltpu.CompilerParams(vmem_limit_bytes=100 * 1024 * 1024,
                                             disable_semaphore_checks=True, disable_bounds_checks=True),
        name="hedgehog_mod",
    )(
        A_x.reshape(S, D),
        A_wqkv,
        A_w_phi,
        A_wo.reshape(4, QK, D),
        B_w_r,
        B_w_gate,
        B_w_up,
        B_w_down,
    )
    return out.reshape(1, S, D)
```

```python
import math

import jax
import jax.numpy as jnp
from jax import lax
import jax.experimental.pallas as pl
import jax.experimental.pallas.tpu as pltpu

F32 = jnp.float32
BF16 = jnp.bfloat16
U32 = jnp.uint32

S = 2048
D = 1024
H = 32
DH = 32
FF = 3584
NPAIR = H // 2
LOG2E = 1.4426950408889634
LN_EPS = 1e-5
KEY_MIN = -2 ** 31

T = 256
TH = T // 2
NT_ = S // T
RC = 256
NC = D // RC
PPC = RC // 64
LNC = 16

FV = 10 * 128
FM = FF - FV
FVD = 8 * 128
NQ = NT_ // 2
DQ = (FF - FVD) // NQ
WO_ROWS = 96
QK = D // 4
HK = D // 2
SW = 8 * HK


LN1_PLANS = (((0.095, 7), (0.452, 8), (2.855, 10), (4.2, 11), (5.319, 11), (7.125, 13), (8.42, 16), (9.93,
    16), (11.174, 17), (11.928, 20), (13.877, 22), (15.466, 23), (16.77, 23), (18.221, 25), (19.528, 26),
    (21.5, 27)), ((-1.151, 4), (1.227, 7), (1.804, 8), (3.43, 9), (5.504, 11), (5.922, 14), (8.015, 14),
    (9.666, 17), (10.176, 17), (12.035, 19), (13.665, 19), (15.339, 22), (16.395, 22), (18.546, 25), (19.409,
    26), (21.079, 27)))
PRO_LN_PLANS0 = ((None, 4), (None, 7), (0.12, 5), (0.555, 5), (1.7, 6), (2.168, 6), (3.297, None), (4.239,
    None))
PRO_LN_PLANS1 = ((None, 4), (None, 5), (-0.516, None), (0.246, 6), (1.046, 6), (2.1, 7), (3.001, 7), (3.003,
    6))
PRO_K_PLANS0 = ((0.388, None), (0.863, None), (1.721, None), (2.715, None), (2.982, None), (3.948, None),
    (5.473, None), (5.989, None))
PRO_K_PLANS1 = ((-0.866, None), (0.636, None), (1.962, None), (2.951, None), (3.554, None), (4.106, None),
    (4.699, None), (5.223, None))
PRO_X0_PLAN = ((20.049, None), (21.671, None), (23.071, None), (23.684, None), (25.371, None), (26.097, None),
    (26.566, None), (27.089, None))
PRO_W_PLANS0 = ((3.2, None), (3.488, None), (3.771, None), (4.235, None), (4.92, None), (5.413, None), (6.114,
    None), (6.485, None))
PRO_W_PLANS1 = ((4.846, None), (5.235, None), (6.531, None))
PRO_W_PLANS2 = ((6.626, None), (7.329, None), (8.074, None), (9.011, None), (9.904, None), (10.947, None),
    (12.625, None), (13.232, None), (14.27, None), (15.036, None), (16.142, None), (17.035, None), (18.379,
    None), (19.306, None), (19.316, None), (20.753, None), (21.341, None), (22.294, None), (23.106, None),
    (25.173, None))
PRO_K_PLANS2 = ((21.924, None), (22.415, None), (24.003, None), (24.127, None), (24.582, None), (25.771,
    None), (26.668, None), (27.134, None))
PRO_V_PLANS = (((None, None), (None, None), (None, None), (None, None), (None, None), (None, None), (None,
    None), (None, None), (-4.983, 0), (-4.771, 1), (-4.658, 2), (-3.398, 2), (-3.155, 2), (-2.921, 2),
    (-2.499, 3), (-2.355, 3), (-1.874, 4), (-1.535, 4), (-1.024, 4), (-0.927, 4), (-0.706, 4), (0.24, 6),
    (0.481, 7), (0.668, 6), (1.247, 7), (1.4, 7), (2.688, 9), (2.727, 7), (3.012, 8), (3.087, 9), (4.289, 9),
    (4.924, 10)), ((5.897, None), (7.691, None), (10.048, None), (12.014, None), (13.868, None), (15.456,
    None), (17.412, None), (20.836, None)), ((0.0, None), (1.776, None), (3.418, None), (4.808, None)),
    ((19.45, None), (21.451, None), (22.925, None), (23.333, None)), ((16.059, None), (20.449, None), (20.497,
    None), (21.79, None), (22.449, None), (22.572, None), (25.109, None), (25.686, None), (-0.337, None),
    (-0.164, None), (0.488, None), (2.709, None), (2.857, None), (3.639, None), (4.322, None), (4.918, None),
    (5.207, None), (6.91, None), (7.587, None), (8.953, None), (9.24, None), (10.232, None), (11.175, None),
    (11.993, None), (12.583, None), (13.787, None), (14.312, None), (14.817, None), (16.402, None), (16.81,
    None), (17.304, None), (19.292, None)))
END_PLANS = (((-0.162, None), (2.011, None), (3.829, None), (5.62, None), (6.909, None), (8.156, None),
    (10.634, None), (12.371, None), (13.954, None), (15.538, None), (16.797, None), (19.352, None), (20.737,
    None), (23.183, None), (23.393, None), (25.88, None)), ((100.308, None), (101.389, None), (102.104, None),
    (0.409, None), (1.005, None), (2.198, None), (2.898, None), (4.205, None), (5.131, None), (6.022, None),
    (7.291, None), (7.974, None), (8.425, None), (9.982, None), (11.3, None), (11.768, None), (12.903, None),
    (13.561, None), (14.696, None), (15.687, None), (17.565, None), (18.013, None), (18.596, None), (19.613,
    None), (20.25, None), (21.235, None), (22.366, None), (23.06, None), (24.673, None), (25.256, None),
    (26.011, None)))
WO_PLANS = (((0.245, None), (6.671, None), (13.503, None), (18.706, None), (24.618, None)), ((-26.952, None),
    (-21.248, None), (-17.185, None), (-12.341, None), (-8.3, None), (-2.883, None), (1.471, None), (6.233,
    None), (10.547, None), (15.312, None), (19.869, None), (24.052, None)), ((-27.707, None), (-22.089, None),
    (-18.962, None), (-14.225, None), (-9.98, None), (-6.503, None), (-2.606, None)))
LN2_PLANS = (((-0.9, 12), (1.365, 15), (5.416, 19), (5.782, 21), (11.172, 24), (14.638, 27), (17.452, 29),
    (19.2, 33), (23.916, 36), (26.706, 40), (29.431, 42), (33.006, 46)), ((35.739, 47), (38.937, 51), (41.779,
    54), (45.752, 57), (47.863, 61), (50.474, 62), (53.833, 66), (56.742, 69), (61.708, 72), (62.833, 75),
    (65.346, 77), (68.926, 83), (71.975, 82), (74.997, 86), (78.06, 90), (81.178, 92)), ((84.39, None),
    (87.649, None), (89.394, None), (89.543, None)))
O2_PLANS = (((130.451, None), (134.449, None), (137.05, None), (137.656, None), (138.539, None), (140.057,
    None), (144.16, None)), ((141.38, None), (145.789, None), (145.843, None), (146.882, None), (149.928,
    None), (152.029, None), (152.297, None)), ((13.193, None), (22.336, None), (31.211, None), (39.891, None),
    (47.762, None), (56.772, None), (66.0, None)), ((27.948, None), (36.312, None), (43.877, None), (51.401,
    None), (58.218, None), (67.954, None), (76.139, None)))
PACK_PLANS = (((100.689, None), (101.244, None), (102.208, None), (102.296, None), (103.427, None), (104.581,
    None), (105.862, None), (106.631, None), (107.838, None), (108.106, None), (109.264, None), (109.501,
    None), (110.393, None), (111.052, None), (111.166, None), (111.572, None), (114.039, None), (114.221,
    None), (115.251, None), (116.905, None), (117.839, None), (118.037, None), (118.466, None), (118.897,
    None), (121.059, None), (121.354, None), (121.429, None), (122.756, None), (123.403, None), (124.242,
    None), (124.9, None), (125.882, None)), ((128.281, None), (128.956, None), (131.04, None), (131.514,
    None), (131.968, None), (132.635, None), (132.835, None), (133.941, None), (135.423, None), (136.25,
    None), (136.936, None), (137.657, None), (138.658, None), (139.06, None), (140.343, None), (141.492,
    None), (142.08, None), (142.473, None), (143.602, None), (143.8, None), (144.137, None), (146.083, None),
    (146.911, None), (147.792, None), (148.441, None), (148.723, None), (149.954, None), (151.061, None),
    (151.737, None), (152.867, None), (153.829, None), (154.519, None)))
PACKD_PLANS = (((0.956, None), (1.633, None), (4.36, None), (5.329, None), (7.571, None), (9.451, None),
    (9.768, None), (11.103, None), (12.795, None), (13.625, None), (14.575, None), (14.855, None), (19.475,
    None), (20.868, None), (21.935, None), (22.323, None), (25.31, None), (26.102, None), (28.561, None),
    (30.197, None), (31.978, None), (33.481, None)), ((34.174, None), (36.791, None), (38.947, None), (39.775,
    None), (42.179, None), (42.661, None), (46.568, None), (46.608, None), (49.436, None), (51.509, None),
    (51.641, None), (52.889, None), (53.189, None), (55.672, None), (56.222, None), (58.458, None), (60,
    None), (60, None)))
PACK_DUE = (130, 5, 39, 64)
DQA = 16 * len(PACKD_PLANS[0])
G_LAG = 5
D_LAG = 1
PLAIN_V0 = 1
LN2_GAPS = (1.13, 1.5, 0.2)
LN2_SPLIT = 4
PACK_W = 512
GAP_PACK = 0.2
LN1_GAPS = (1, 1.25, 0.2)
LOOP_GAPS = (1, 1.25, 0.2)
GAP_PRO = 0.13
GAP_WO = 0.2
GAP_O2 = 0.26
O_DUE = 6
MOE_NA = 36
MOE_ND = 2
MOE_LAGS = (2, 2)
STAGGER = 8

NN = (((1,), (0,)), ((), ()))
NT = (((1,), (1,)), ((), ()))


def _dot(a, b, dims):
    return lax.dot_general(a, b, dims, preferred_element_type=F32)


def _recip(x):
    return pl.reciprocal(x, approx=False, full_range=False)


def _pack(x):
    return pltpu.bitcast(x, U32)


def _unpack(x):
    return pltpu.bitcast(x, BF16)


def _strassen_lhs(a11, a12, a21, a22):
    return [a21 + a22, a22, a11 + a12, a11, a11 + a22, a12 - a22, a21 - a11]


def _strassen_rhs(b11, b12, b21, b22):
    return [b11, b21 - b11, b22, b12 - b22, b11 + b22, b21 + b22, b11 + b12]


def _strassen(product):
    m2 = product(0)
    m4 = product(1)
    c21 = m2 + m4
    m5 = product(2)
    u11 = m4 - m5
    m3 = product(3)
    c12 = m3 + m5
    u22 = m3 - m2
    m1 = product(4)
    u11 = u11 + m1
    u22 = u22 + m1
    c11 = product(5) + u11
    c22 = product(6) + u22
    return [[c11, c12], [c21, c22]]


def _strassen_rows_first(product, emit):
    m5 = product(2)
    m3 = product(3)
    emit(0, 1, m3 + m5)
    m4 = product(1)
    u11 = m4 - m5
    m1 = product(4)
    u11 = u11 + m1
    u22 = m3 + m1
    emit(0, 0, product(5) + u11)
    m2 = product(0)
    emit(1, 0, m2 + m4)
    u22 = u22 - m2
    emit(1, 1, product(6) + u22)


def _ordered(bits):
    return bits ^ ((bits >> 31) & 0x7FFF0000)


def _block(rows):
    return jnp.concatenate([jnp.concatenate(r, axis=1) for r in rows], axis=0)


def _pair_allreduce(a, op):
    a = op(a, pltpu.roll(a, 2, 0))
    return op(a, pltpu.roll(a, 4, 0))


def _tree(op, xs):
    xs = list(xs)
    while len(xs) > 1:
        nxt = [op(xs[i], xs[i + 1]) for i in range(0, len(xs) - 1, 2)]
        if len(xs) % 2:
            nxt.append(xs[-1])
        xs = nxt
    return xs[0]


def _pair_logits(sl, j):
    sub = lax.broadcasted_iota(jnp.int32, sl[0].shape, 0)
    if j < 3:
        head = jnp.where(sub < 2, 0.0, sl[(0, 1, 16)[j]])
    else:
        head = jnp.where(sub < 2, sl[0], jnp.where(sub < 4, pltpu.roll(sl[1], 2, 0),
                                                   jnp.where(sub < 6, pltpu.roll(sl[16], 4, 0), 0.0)))
    r0 = (2, 9, 17, 24)[j]
    return [head] + list(sl[r0:r0 + 7])


def _dual_exp(sl):
    mx = _pair_allreduce(_tree(jnp.maximum, sl), jnp.maximum)
    mn = _pair_allreduce(_tree(jnp.minimum, sl), jnp.minimum)
    ep = [jnp.exp2(s - mx) for s in sl]
    en = [jnp.exp2(mn - s) for s in sl]
    sp = _pair_allreduce(_tree(jnp.add, ep), jnp.add)
    sn = _pair_allreduce(_tree(jnp.add, en), jnp.add)
    return ep, en, sp, sn


def _after(x, never, anchor):
    if anchor is None:
        return x
    d = jnp.concatenate([anchor] * (x.shape[0] // 8), axis=0)
    if x.shape[1] == 128:
        return jnp.where(never, d, x)
    return jnp.concatenate([jnp.where(never, d, x[:, :128]), x[:, 128:]], axis=1)


def _gate(x, never, deps):
    for i, dep in enumerate(deps):
        d = jnp.broadcast_to(dep, (8, 128))
        if x.dtype != F32:
            d = pltpu.bitcast(d, x.dtype)
        blk = jnp.where(never, d, x[8 * i:8 * i + 8, :128])
        if x.shape[1] > 128:
            blk = jnp.concatenate([blk, x[8 * i:8 * i + 8, 128:]], axis=1)
        parts = ([x[:8 * i, :]] if i else []) + [blk, x[8 * i + 8:, :]]
        x = jnp.concatenate(parts, axis=0)
    return x


def _lane_fold(a):
    return _tree(jnp.add, [a[:, 128 * i:128 * i + 128] for i in range(a.shape[1] // 128)])


def _row_sum(a):
    return jnp.sum(_lane_fold(a), axis=-1, keepdims=True)


def _lane_tile(a, n):
    return a if n == 1 else jnp.concatenate([a] * n, axis=1)


def _sublane_allreduce(a):
    a = a + pltpu.roll(a, 4, 0)
    a = a + pltpu.roll(a, 2, 0)
    return a + pltpu.roll(a, 1, 0)


def _col_broadcast(row8):
    return jnp.concatenate([row8] * 16, axis=0).astype(BF16).T.astype(F32)


def _vpu_matvec(xb, w_rows, never, anchors, lag):
    ng = xb.shape[0] // 8
    acc, hist = None, []
    for g in range(ng):
        dep = anchors[(g * len(anchors)) // ng]
        if g >= lag:
            dep = dep + hist[g - lag]
        x = jnp.where(never, dep, xb[8 * g:8 * g + 8, :])
        w = w_rows(g)
        t = w * _lane_tile(x, w.shape[1] // 128)
        acc = t if acc is None else acc + t
        c = 128 * (g % (w.shape[1] // 128))
        hist.append(acc[:, c:c + 128])
    return acc


class _Side:
    def __init__(self, never, later=lambda rel, gap: rel + gap):
        self.never = never
        self.later = later
        self.jobs = []
        self.deps = {}
        self.hooks = {}

    def add(self, plan, fn):
        for k, (rel, due) in enumerate(plan):
            if rel is None:
                self._run(None, due, fn, k, None)
            else:
                self.jobs.append((rel, due, fn, k))

    def _run(self, rel, due, fn, k, anchor):
        gen = fn if hasattr(fn, "send") else fn(k, anchor)
        dep = gen
        if hasattr(gen, "send"):
            try:
                while True:
                    gap = gen.send(anchor) if gen is fn or rel is None and dep is None else next(gen)
                    if rel is not None:
                        self.jobs.append((self.later(rel, gap), due, gen, k))
                        return
                    dep = None
            except StopIteration as stop:
                dep = stop.value
        if due is not None:
            self.deps.setdefault(due, []).append(dep)

    def check(self):
        assert not self.jobs and not self.deps and not self.hooks

    def gate(self, step, x):
        return _gate(x, self.never, self.deps.pop(step, []))

    def done(self, step, res):
        m = res.shape[0] // 8
        while True:
            ready = [j for j in self.jobs if step - 1 < j[0] <= step]
            if not ready:
                break
            job = min(ready, key=lambda j: j[0])
            self.jobs.remove(job)
            g = m - 1 - int((step - job[0]) * m)
            self._run(*job, res[8 * g:8 * g + 8, res.shape[1] - 128:])
        for fn in self.hooks.pop(step, []):
            fn()


def _kernel(x_hbm, wqkv_hbm, wphi_hbm, wo_hbm, wr_hbm, wg_hbm, wu_hbm, wd_hbm, out_hbm,
            x_v, xn_v, xs_v, lead_v, wraw_v, wt_v, ws_v, wphi_v, a_v, woraw_v, wos_v, wrraw_v, wr_v,
            kvacc_v, kvbf_v, z_v, zb_v, phi_v, oc_v, oc2_v, h_v, hn_v, o_v, wg_v, wu_v, wd_v, stage_v,
            wgp_v, wup_v, wdp_v, patch_v,
            sem):
    SX, SQ, SO, SM = 0, 6, 6 + 3 * NC, 6 + 3 * NC + NT_ + 1

    def x_copy(i):
        h0, h1 = ((0, 1), (1, 2), (3, 4), (4, 8), (8, 2 * NT_), (2, 3))[i]
        rows = pl.ds(h0 * TH, (h1 - h0) * TH)
        return pltpu.make_async_copy(x_hbm.at[rows, :], x_v.at[rows, :], sem.at[SX + i])

    def k0_copy(s):
        return pltpu.make_async_copy(wqkv_hbm.at[:, pl.ds(D + s * 128, 128)],
                                     wraw_v.at[NC, :, pl.ds(s * 128, 128)], sem.at[(SM + 7, SQ + NC)[s]])

    def w_copy(j, c):
        return pltpu.make_async_copy(wqkv_hbm.at[:, pl.ds(j * D + c * RC, RC)], wraw_v.at[j * NC + c],
                                     sem.at[SQ + j * NC + c])

    def wphi_copy(i):
        h0, h1 = ((0, 8), (16, 24), (8, 16), (24, H))[i]
        return pltpu.make_async_copy(wphi_hbm.at[pl.ds(h0, h1 - h0)], wphi_v.at[pl.ds(h0, h1 - h0)],
                                     sem.at[(SM + 4, SM + 8, SM + 9, SM + 14)[i]])

    wr_copy = pltpu.make_async_copy(wr_hbm, wrraw_v, sem.at[SM + 5])

    def wo_copy(i):
        rows = pl.ds(0, WO_ROWS) if i == 0 else pl.ds(WO_ROWS, QK - WO_ROWS)
        return pltpu.make_async_copy(wo_hbm.at[:, rows, :], woraw_v.at[:, rows, :], sem.at[(SM + 6, SM + 15)[i]])

    wg_copy = pltpu.make_async_copy(wg_hbm.at[:, pl.ds(FM, FV)], wg_v, sem.at[SM + 0])
    wu_copy = pltpu.make_async_copy(wu_hbm.at[:, pl.ds(FM, FV)], wu_v, sem.at[SM + 1])
    wd_copy = pltpu.make_async_copy(wd_hbm.at[pl.ds(0, FVD), :], wd_v, sem.at[SM + 2])

    def stage_copy(i, q):
        if i < 2:
            r0 = q * (D // NQ)
            r0 = r0 if isinstance(r0, int) else pl.multiple_of(r0, D // NQ)
            src = (wg_hbm, wu_hbm)[i].at[pl.ds(r0, D // NQ), pl.ds(0, FM)]
        else:
            r0 = FVD + q * DQ + (i - 2) * DQA
            r0 = r0 if isinstance(r0, int) else pl.multiple_of(r0, 16)
            src = wd_hbm.at[pl.ds(r0, (DQA, DQ - DQA)[i - 2]), :]
        return pltpu.make_async_copy(src, stage_v[i].at[pl.ds(0, src.shape[0]), :], sem.at[SM + 10 + i])

    wphi_copy(0).start()
    k0_copy(0).start()
    x_copy(0).start()
    k0_copy(1).start()
    x_copy(1).start()
    wphi_copy(1).start()
    w_copy(1, 2).start()

    made = set()

    def view(ref, i, n, off=0):
        r0 = off + i * n
        return ref.at[pl.ds(r0 if isinstance(r0, int) else pl.multiple_of(r0, math.gcd(n, off)), n), :]

    def xs_view(t, par):
        return view(xs_v[par], t >> 1, TH // 2)

    def put_blocks(dst, r0, fn, m11, m12, m21, m22, never, a, skip=(), base=0, pitch=HK, gap=None):
        for c0 in range(0, m11.shape[1], 128):
            if c0:
                a = yield gap or GAP_PRO
            d11, d22 = m11[:, c0:c0 + 128], m22[:, c0:c0 + 128]
            if a is not None:
                d = jnp.concatenate([a, a], axis=0)
                d11, d22 = jnp.where(never, d, d11), jnp.where(never, d, d22)
            blocks = fn(d11, m12[:, c0:c0 + 128], m21[:, c0:c0 + 128], d22)
            for i, b in enumerate(blocks):
                if i not in skip:
                    dst[r0:r0 + 8, base + i * pitch + c0:base + i * pitch + c0 + 128] = _pack(b.astype(BF16))

    def rows16(ref, r0, c0=0, w=D):
        return _unpack(ref[r0:r0 + 8, c0:c0 + w]).astype(F32)

    def x_blocks(t, par, k, lo, hi, never, a, gap=None):
        yield from put_blocks(xs_view(t, par), k * LNC // 2, _strassen_rhs,
                              lo[:, :HK], hi[:, :HK], lo[:, HK:], hi[:, HK:], never, a, gap=gap)
        if isinstance(t, int):
            made.add(("xs", t, k))

    def ln_rows(t, par, k, n, never=None, anchor=None, plain=False):
        wide = lambda c, a: _lane_tile(_after(jnp.broadcast_to(c, (n, 128)), never, a), D // 128)
        x = _after(view(x_v, t, T)[k * n:(k + 1) * n, :].astype(F32), never, anchor)
        s1 = _row_sum(x)
        gaps = LN1_GAPS if isinstance(t, int) else LOOP_GAPS
        anchor = yield gaps[0]
        xc = x - wide(s1 * (1.0 / D), anchor)
        rstd = lax.rsqrt(_row_sum(xc * xc) * (1.0 / D) + LN_EPS)
        anchor = yield gaps[1]
        xn = xc * wide(rstd, anchor)
        if plain:
            xn_v[k * n // 2:(k + 1) * n // 2, :] = _pack(xn.astype(BF16))
        elif k * n < TH:
            xn_v[(T + k * n) // 2:(T + (k + 1) * n) // 2, :] = _pack(xn.astype(BF16))
        else:
            yield from x_blocks(t, par, k - TH // LNC, rows16(xn_v, (TH + k * n) // 2), xn, never, anchor, gaps[2])
        return _tree(jnp.add, [rstd[8 * i:8 * i + 8, :] for i in range(min(n, LNC) // 8)])

    def now(gen):
        try:
            while True:
                next(gen)
        except StopIteration as stop:
            return stop.value

    def late_x_blocks(t):
        return lambda k, a: x_blocks(t, t % 2, k, rows16(xn_v, t * T // 2 + 8 * k),
                                     rows16(xn_v, (t * T + TH) // 2 + 8 * k), never0, a)

    def xn_tile(t):
        return _unpack(xn_v[t * T // 2:(t + 1) * T // 2, :])

    def xs_tile(t, par):
        assert not isinstance(t, int) or t > 1 or made >= {("xs", t, k) for k in range(8)}
        return _unpack(xs_view(t, par)[:, 0:7 * HK])

    def expand_wphi(c):
        w = wphi_v[8 * c:8 * c + 8].reshape(8 * DH, DH).astype(F32).T
        bits = pltpu.bitcast(w, U32)
        head = lax.broadcasted_iota(jnp.int32, (DH, 128), 1) >> 5
        for s in range(2):
            b = bits[:, 128 * s:128 * s + 128]
            for j in range(2):
                r0 = 64 * (2 * c + s) + 32 * j
                a_v[r0:r0 + 32, :] = jnp.where(head == 2 * j, b >> 16,
                                               jnp.where(head == 2 * j + 1, b, jnp.uint32(0)))

    wphi_copy(0).wait()
    expand_wphi(0)
    h_v[1][...] = jnp.zeros((T, D), F32)
    for ref in oc_v + oc2_v:
        ref[0:8, 0:128] = jnp.zeros((8, 128), U32)
    for ref in stage_v:
        ref[ref.shape[0] - 16:, 0:128] = jnp.zeros((16, 128), BF16)

    def v_transpose(k, a):
        q, r0 = (k // 8) + 4 * (k % 2), 256 * (k % 8 // 2)
        w = wraw_v[2 * NC + q // 2, r0:r0 + 256, (q % 2) * 128:(q % 2) * 128 + 128]
        if a is not None:
            w = _unpack(jnp.where(never0, jnp.concatenate([pltpu.bitcast(a, U32)] * 16, axis=0), _pack(w)))
        wt = _pack(w.T)
        wt_v[2][64 * q:64 * q + 64, r0:r0 + 256] = wt
        made.add(("vt", k))
        return pltpu.bitcast(wt[56:64, 128:256], F32)

    def fold_pairs(j, c, s, side=None, step0=None):
        g0 = 64 * (2 * c + s)
        g0 = g0 if isinstance(g0, int) else pl.multiple_of(g0, 64)
        res = _dot(_unpack(a_v[pl.ds(g0, 64), :]), wraw_v[j * NC + c, :, s * 128:(s + 1) * 128], NT)
        if side is not None:
            side.done(step0 + 2 * s, res[:, :D // 2])
            side.done(step0 + 2 * s + 1, res[:, D // 2:])
        sub = lax.broadcasted_iota(jnp.int32, (8, D), 0)
        out = []
        for q in range(2):
            base = _pair_allreduce(jnp.where(sub < 2, res[64 * q:64 * q + 8, :], 0.0), jnp.add)
            out.append([(res[64 * q + 8 * i:64 * q + 8 * i + 8, :] - base) * LOG2E for i in range(8)])
        return out

    def share(z, z3, k):
        sub = lax.broadcasted_iota(jnp.int32, (8, D), 0)
        return jnp.where(sub < 2, pltpu.roll(z3, 8 - 2 * k, 0), z)

    def packed(slabs):
        return _pack(jnp.concatenate(slabs, axis=0).astype(BF16))

    def fold(j, c, side=None, step0=None):
        p0, p1 = fold_pairs(j, c, 0, side, step0)
        p2, p3 = fold_pairs(j, c, 1, side, step0)
        sl = ([share(p0[0], p3[0], 1), share(p1[0], p3[0], 2)] + p0[1:] + p1[1:]
              + [share(p2[0], p3[0], 3)] + p2[1:] + p3[1:])
        zero = jnp.zeros((8, D), F32)
        even, odd = sl + [zero], [zero] + sl
        r0 = 8 * ((31 * c) // 2)
        is_odd = c % 2 == 1
        if isinstance(c, int):
            sl = odd if is_odd else even
        else:
            r0 = pl.multiple_of(r0, 8)
            sl = [jnp.where(is_odd, o, e) for o, e in zip(odd, even)]
        win = wt_v[j].at[pl.ds(r0, 128), :]
        win[8:128, :] = packed(sl[2:])
        first = packed(sl[:2])
        if is_odd is not False:
            keep = lax.broadcasted_iota(jnp.int32, (8, D), 0) < jnp.where(is_odd, 4, 0)
            first = jnp.where(keep, win[0:8, :], first)
        win[0:8, :] = first
        made.update(("fold", j, q) for q in ([c] if isinstance(c, int) else range(3)))

    def w_blocks(j, k0=0):
        def job(k, a):
            k += k0
            assert made >= ({("vt", 8 * (k // 8) + q) for q in range(8)} if j == 2 else
                            {("fold", j, q) for q in ((0, 2) if k < 15 else range(4))})
            lo, hi = rows16(wt_v[j], 8 * k), rows16(wt_v[j], (256 if j == 2 else 248) + 8 * k)
            yield from put_blocks(ws_v[j], 8 * k, _strassen_lhs, lo[:, :HK], lo[:, HK:], hi[:, :HK], hi[:, HK:],
                                  never0, a, skip=(1, 3))
            made.add(("ws", j, k))
        return job

    def k_pair(p, slot, pr, c0, never=None):
        first = ("z", pr, c0) not in made
        for n in range(c0, c0 + p[0].shape[1], 128):
            assert first == (("z", pr, n) not in made)
            made.update({("z", pr, n), ("phi", slot, pr, n)})
        ep, en, sp, sn = _dual_exp(p)
        inv = _recip(sp * sn)
        scale = (sn * inv, sp * inv)
        es = ep + en
        cols = slice(c0, c0 + p[0].shape[1])
        n = 16 if never is None else 16 // STAGGER
        last = None
        for q in range(16 // n):
            sc = scale
            if last is not None:
                sc = [jnp.where(never, last, x) for x in scale]
            phi = jnp.concatenate([es[i] * sc[i // 8] for i in range(q * n, (q + 1) * n)], axis=0)
            rows = slice(8 * q * n, 8 * (q + 1) * n)
            z = phi if first else z_v[pr, rows, cols] + phi
            z_v[pr, rows, cols] = z
            phi_v[slot][64 * pr + 4 * q * n:64 * pr + 4 * (q + 1) * n, cols] = _pack(phi.astype(BF16))
            last = z[8 * n - 8:, :]

    def kv_update(vts, slot, g, first, publish=False):
        for q, vt in enumerate(vts):
            for j in range(2):
                pr = 2 * g + 8 * q + j
                assert made >= {("phi", slot, pr, 0), ("phi", slot, pr, 128)}
                upd = _dot(vt[64 * j:64 * j + 64, :].astype(BF16), _unpack(phi_v[slot][64 * pr:64 * pr + 64, :]), NT)
                acc = upd if first else kvacc_v[pr] + upd
                kvacc_v[pr] = acc
                if publish:
                    odd = -(lax.broadcasted_iota(jnp.int32, (32, 128), 1) & 1)
                    bits = pltpu.bitcast(acc, jnp.int32) & jnp.concatenate([~odd, odd], axis=0)
                    kvbf_v[32 * pr:32 * pr + 32, :] = _pack(pltpu.bitcast(bits, F32).astype(BF16))

    def save_lead(t, par):
        view(lead_v, t, HK // 2)[...] = _pack(_unpack(xs_view(t, par)[:, 0:HK]).T)

    def proj_feat(side, step0, c, xn):
        r0 = 8 * ((31 * c) // 2)
        w = wt_v[1][r0:r0 + 128, :]
        quarters = []
        for n in range(2):
            for m in range(2):
                step = step0 + 2 * n + m
                wq = _unpack(side.gate(step, w[:64, :] if m == 0 else w[64:, :]))
                res = _dot(wq, xn[n * TH:(n + 1) * TH, :], NT)
                side.done(step, res)
                quarters.append(res)
        res = jnp.concatenate(
            [jnp.concatenate([quarters[0], quarters[2]], axis=1),
             jnp.concatenate([quarters[1], quarters[3]], axis=1)], axis=0)
        sl = [res[8 * i:8 * i + 8, :] for i in range(res.shape[0] // 8)]
        return sl[c % 2:31 + c % 2]

    def proj_unit(side, step0, j, b, xs, lead=None, plain=None):
        r1 = 64 * b + (64 if j == 2 or b < 3 else 56)
        assert made >= ({("vt", 8 * b + q) for q in range(8)} if plain is not None else
                        {("ws", j, k) for k in range(8 * b, r1 // 8)})
        if plain is not None:
            out = []
            for q in range(2):
                row = []
                for n in range(2):
                    steps = range((0, 2, 4, 5)[2 * q + n], (2, 4, 5, 7)[2 * q + n])
                    deps = [d for i in steps for d in side.deps.pop(step0 + i, [])]
                    w = _gate(wt_v[2][256 * q + 64 * b:256 * q + r1, :], side.never, deps)
                    res = _dot(_unpack(w), plain[n * TH:(n + 1) * TH, :], NT)
                    for i in steps:
                        side.done(step0 + i, res)
                    row.append(res)
                out.append(jnp.concatenate(row, axis=1))
            return out

        def product(i):
            off = 256 if j == 2 else 248
            w = (wt_v[j][off + 64 * b:off + r1, HK:] if i == 1 else wt_v[j][64 * b:r1, :HK] if i == 3
                 else ws_v[j][64 * b:r1, i * HK:(i + 1) * HK])
            w = _unpack(side.gate(step0 + i, w))
            if lead is not None and i == 0:
                res = _dot(w, _unpack(view(lead_v, lead, HK // 2)[...]), NN)
            else:
                res = _dot(w, xs[:, i * HK:(i + 1) * HK], NT)
            side.done(step0 + i, res)
            return res
        return [jnp.concatenate(row, axis=1) for row in _strassen(product)]

    def feat_stage(side, step0, j, xs, pair_fn, lead=None, units=range(4), sl=None, hold=None):
        sl = sl or [[], []]
        for b in units:
            for q, res in enumerate(proj_unit(side, step0 + 7 * b, j, b, xs, lead if b == units[0] else None)):
                sl[q] += [res[8 * i:8 * i + 8, :] for i in range(res.shape[0] // 8)]
            for q in (1, 0):
                for jj in (2 * (b % 2), 2 * (b % 2) + 1):
                    if b != hold:
                        pair_fn(_pair_logits(sl[q][31 * (b // 2):], jj), 8 * q + 4 * (b // 2) + jj)
        return sl

    def v_stage(side, xs, slot, first, publish, lead, plain=None):
        pending = None
        for g in range(4):
            if pending is not None:
                side.hooks.setdefault(7 * g + D_LAG, []).append(lambda p=pending: kv_update(*p))
            pending = (proj_unit(side, 7 * g, 2, g, xs, lead if g == 0 else None, plain if g < PLAIN_V0 else None),
                       slot, g, first, publish)
        side.check()
        return pending

    def pack_rows(src, dst, r0, c0, cols, never, a):
        for c in range(c0, c0 + cols, PACK_W):
            if c > c0:
                a = yield GAP_PACK
            w = min(PACK_W, c0 + cols - c)
            v = src[r0:r0 + 16, c:c + w].astype(F32)
            v = jnp.concatenate([jnp.where(never, _lane_tile(a, w // 128), v[0:8, :]), v[8:16, :]], axis=0)
            dst[r0 // 2:r0 // 2 + 8, c:c + w] = _pack(v.astype(BF16))

    def stash_at(i, k, n):
        return zb_v.at[4 * i + 2 * (k // 16) + n, pl.ds(8 * (k % 16), 8), :]

    def stash(i, sl):
        for k, v in enumerate(sl):
            for n in range(2):
                stash_at(i, k, n)[...] = v[:, 128 * n:128 * n + 128]

    def stashed_k(i, slot, c):
        def job(k, a):
            j, n = k // 2, k % 2
            p = _pair_logits([stash_at(i, q, n)[...] for q in range(16 if j < 2 else 31)], j)
            k_pair([_after(p[0], never0, a)] + p[1:], slot, c * PPC + j, 128 * n, never0)
        return job

    def first_rows(k0, k1, n):
        xn = _unpack(xn_v[n * TH // 2:(n + 1) * TH // 2, :])
        ks = [k for k in range(k0, k1)]
        w = jnp.concatenate([wt_v[1][4 * (k % 32):4 * (k % 32) + 8, :] for k in ks[::2]], axis=0)
        res = _dot(_unpack(w), xn, NT)
        for q, k in enumerate(ks):
            if k % 32 < 31:
                stash_at(0, k % 32, n)[...] = res[8 * q:8 * q + 8, :]

    k0_copy(0).wait()
    x_copy(0).wait()
    wphi_copy(2).start()
    x_copy(5).start()
    w_copy(1, 1).start()
    wphi_copy(3).start()
    x_copy(2).start()
    p0, p1 = fold_pairs(1, 0, 0)
    wt_v[1][8:64, :] = packed(p0[1:] + p1[1:])
    h_v[0][0:8, :] = p0[0]
    h_v[0][8:16, :] = p1[0]
    never0 = now(ln_rows(0, 0, 0, TH, plain=True))[0, 0] < 0.0
    first_rows(2, 16, 0)

    k0_copy(1).wait()
    x_copy(1).wait()
    wphi_copy(1).wait()
    w_copy(1, 3).start()
    for c in (0, 2, 1, 3):
        w_copy(2, c).start()
    p2, p3 = fold_pairs(1, 0, 1)
    wt_v[1][0:8, :] = packed([share(h_v[0][0:8, :], p3[0], 1), share(h_v[0][8:16, :], p3[0], 2)])
    wt_v[1][64:128, :] = packed([share(p2[0], p3[0], 3)] + p2[1:] + p3[1:] + [jnp.zeros((8, D), F32)])
    made.add(("fold", 1, 0))
    now(ln_rows(0, 0, 1, TH, plain=True))
    first_rows(16, 34, 0)
    first_rows(0, 16, 1)
    first_rows(16, 32, 1)
    expand_wphi(2)

    def slow(end):
        return lambda rel, gap: min(rel + (gap / 2 if 3 <= rel < 7 else gap), end)

    for c, prev in ((2, 0), (1, 2)):
        w_copy(1, c).wait()
        wphi_copy(4 - c).wait()
        side = _Side(never0, slow(7))
        if c == 1:
            x_copy(5).wait()
            side.add(PRO_LN_PLANS0, lambda k, a: ln_rows(1, 1, k, LNC, never0, a))
        expand_wphi(5 - 2 * c)
        side.add((PRO_W_PLANS0, PRO_W_PLANS1)[2 - c], w_blocks(1, (2 - c) * len(PRO_W_PLANS0)))
        side.add((PRO_K_PLANS0, PRO_K_PLANS1)[2 - c], stashed_k(prev, 0, prev))
        fold(1, c, side, 0)
        stash(c, proj_feat(side, 4, c, xn_tile(0)))
        side.check()

    x_copy(2).wait()
    w_copy(1, 3).wait()
    x_copy(3).start()
    w_copy(0, 0).start()
    wo_copy(0).start()
    x_copy(4).start()
    side = _Side(never0, slow(28))
    side.add(PRO_LN_PLANS1, lambda k, a: ln_rows(1, 1, k + 8, LNC, never0, a))
    side.add(PRO_W_PLANS2, w_blocks(1, 31 - len(PRO_W_PLANS2)))
    side.add(PRO_K_PLANS2, stashed_k(1, 0, 1))
    side.add(PRO_X0_PLAN, late_x_blocks(0))
    fold(1, 3, side, 0)
    stash(3, proj_feat(side, 4, 3, xn_tile(0)))
    k1 = lambda p, pr: k_pair(p, 1, pr, 0, never0)
    for q, sl in enumerate(feat_stage(side, 8, 1, xs_tile(1, 1), k1, units=range(3), hold=2)):
        stash(2 * q, sl[31:])
    side.check()
    save_lead(1, 1)

    for c in range(NC):
        w_copy(2, c).wait()
    side = _Side(never0, lambda rel, gap: min(rel + gap, 27))
    side.add(PRO_V_PLANS[0], v_transpose)
    side.add(PRO_V_PLANS[1], stashed_k(3, 0, 3))
    side.add(PRO_V_PLANS[2], stashed_k(0, 1, 1))
    side.add(PRO_V_PLANS[3], stashed_k(2, 1, 3))
    side.add(PRO_V_PLANS[4], w_blocks(2))
    sl = [[None] * 31 + [jnp.concatenate([stash_at(2 * q, k, n)[...] for n in range(2)], axis=1) for k in range(17)]
          for q in range(2)]
    feat_stage(side, -28, 1, xs_tile(1, 1), k1, 1, units=range(3, 4), sl=sl)
    kv_update(*v_stage(side, xs_tile(0, 0), 0, True, False, None, xn_tile(0)))
    save_lead(0, 0)
    for c in range(1, NC):
        w_copy(0, c).start()
    wo_copy(1).start()
    wr_copy.start()
    for i in range(4):
        stage_copy(i, 0).start()
    wg_copy.start()
    wu_copy.start()
    wd_copy.start()
    for r0 in (0, 248):
        wt_v[0][r0:r0 + 8, :] = jnp.zeros((8, D), U32)

    def phase1(u, carry):
        never = u < 0

        @pl.when(u == 0)
        def _():
            x_copy(3).wait()
            w_copy(0, 0).wait()
            wo_copy(0).wait()

        @pl.when(u == 1)
        def _():
            x_copy(4).wait()
            w_copy(0, 1).wait()
            w_copy(0, 2).wait()
            wo_copy(1).wait()

        def wo_blocks(k0):
            def job(k, a):
                k += k0
                r, c, part = k // 4, 128 * (k // 2 % 2), k % 2
                r0 = u * ((QK - WO_ROWS) // 2)
                dst = wos_v.at[pl.ds(pl.multiple_of(r0 // 2, 8), WO_ROWS // 2), :]

                def piece(kq, nq):
                    src = woraw_v.at[kq, pl.ds(pl.multiple_of(r0, 16), WO_ROWS), :]
                    return src[16 * r:16 * r + 16, nq * QK + c:nq * QK + c + 128].astype(F32)
                outer = [_strassen_rhs(piece(ki, ni), piece(ki, 2 + ni), piece(2 + ki, ni), piece(2 + ki, 2 + ni))
                         for ki in range(2) for ni in range(2)]
                for i in range(4) if part == 0 else range(4, 7):
                    if i % 4:
                        a = yield GAP_WO
                    yield from put_blocks(dst, 8 * r, _strassen_rhs, *[o[i] for o in outer], never, a,
                                          base=7 * i * QK + c, pitch=QK)
            return job

        xs = xs_tile(2 * u + 1, 1)
        side = _Side(never, lambda rel, gap: min(rel + gap, 27))
        for i in range(2):
            t = 2 * u + 2 + i
            if i == 0:
                side.add(LN1_PLANS[0], lambda k, a: ln_rows(2 * u + 2, 0, k, LNC, never, a))
                side.add(WO_PLANS[0], wo_blocks(0))
            pending = v_stage(side, xs, 1 - i, False, False, t - 1 if i == 0 else None)
            xs = xs_tile(t, i)
            side = _Side(never, lambda rel, gap, end=(27, -1)[i]: min(rel + gap, end))
            if i == 0:
                side.add(LN1_PLANS[1], lambda k, a: ln_rows(2 * u + 3, 1, k, LNC, never, a))
                side.add(WO_PLANS[1], wo_blocks(len(WO_PLANS[0])))
            else:
                side.add(WO_PLANS[2], wo_blocks(24 - len(WO_PLANS[2])))
            side.hooks[-28 + D_LAG] = [lambda p=pending: kv_update(*p)]
            feat_stage(side, -28, 1, xs, lambda p, pr: k_pair(p, i, pr, 0, never if i == 1 else None))
            save_lead(t, i)
        side.check()
        fold(0, u)
        return carry

    lax.fori_loop(0, (NT_ - 2) // 2, phase1, 0)

    w_copy(0, 3).wait()
    wr_copy.wait()
    side = _Side(never0, lambda rel, gap: min(rel + gap, 27 if rel < 98 else 103))

    def z_final(k, a):
        zb_v[k] = jnp.broadcast_to(_row_sum(_after(z_v[k], never0, a)), (128, 128))

    side.add(END_PLANS[0], z_final)
    side.add(END_PLANS[1], w_blocks(0))
    side.hooks[0] = [lambda: fold(0, 3, side, 100)]
    kv_update(*v_stage(side, xs_tile(NT_ - 1, 1), 1, False, True, NT_ - 1))
    wr_v[...] = jnp.broadcast_to(wrraw_v[...].reshape(1, D).astype(F32), (8, D))

    def o_copy(r0, n, i):
        return pltpu.make_async_copy(o_v.at[pl.ds(r0, n), :], out_hbm.at[pl.ds(r0, n), :], sem.at[SO + i])

    def finish_rows(h_ref, k, t, valid, st, never=None, anchor=None):
        r0 = t * T + k * LNC
        rows = slice(k * LNC, (k + 1) * LNC)
        m = jnp.broadcast_to(_row_sum(_after(h_ref[rows, :], never, anchor)) * (1.0 / D), (LNC, 128))
        rstd, r = [], []
        for i in range(LNC // 8):
            anchor = yield LN2_GAPS[2] if i else LN2_GAPS[0]
            mi = _after(m[8 * i:8 * i + 8, :], never, anchor)
            hc = h_ref[k * LNC + 8 * i:k * LNC + 8 * i + 8, :] - _lane_tile(mi, D // 128)
            rs = lax.rsqrt(_row_sum(hc * hc) * (1.0 / D) + LN_EPS)
            r.append((_row_sum(hc * wr_v[...]) * rs + 0.0).astype(BF16).astype(F32))
            rstd.append(jnp.broadcast_to(rs, (8, 128)))
        rstd = jnp.concatenate(rstd, axis=0)
        w = D if never is None else D // LN2_SPLIT
        for c in range(0, D, w):
            anchor = yield LN2_GAPS[2] if c else LN2_GAPS[1]
            h = h_ref[rows, c:c + w]
            hn = (h - _lane_tile(_after(m, never, anchor), w // 128)) * _lane_tile(rstd, w // 128)
            view(hn_v, t, T // 2)[k * LNC // 2:(k + 1) * LNC // 2, c:c + w] = _pack(hn.astype(BF16))
            view(o_v, t, T)[rows, c:c + w] = (hn + h).astype(BF16)
        best = st["route"]
        sub = lax.broadcasted_iota(jnp.int32, (8, 128), 0)
        for i, ri in enumerate(r):
            key = _ordered(pltpu.bitcast(jnp.broadcast_to(ri, (8, 128)), jnp.int32)) | ((S - 1 - r0 - 8 * i) - sub)
            if valid is not None:
                key = jnp.where(valid, key, KEY_MIN)
            best = jnp.maximum(best, key)
        st["route"] = best
        return pltpu.bitcast(best, F32)

    def q_pair(p, slot, pr):
        ep, en, sp, sn = _dual_exp(p)
        zz = [_lane_tile(zb_v[pr, 8 * i:8 * i + 8, :], T // 128) for i in range(16)]
        ap = _pair_allreduce(_tree(jnp.add, [ep[i] * zz[i] for i in range(8)]), jnp.add)
        an = _pair_allreduce(_tree(jnp.add, [en[i] * zz[8 + i] for i in range(8)]), jnp.add)
        inv = _recip(ap * sn + (an + 1e-6 * sn) * sp)
        rp = sn * inv
        rn = sp * inv
        phi = jnp.concatenate([e * rp for e in ep] + [e * rn for e in en], axis=0)
        phi_v[slot][64 * pr:64 * pr + 64, :] = _pack(phi.astype(BF16))

    held = []

    def attn_blocks(slot, g, deps):
        res = [_dot(_unpack(kvbf_v[32 * pr:32 * pr + 32, :]), _unpack(phi_v[slot][64 * pr:64 * pr + 64, :]), NN)
               for pr in (2 * g, 2 * g + 8, 2 * g + 1, 2 * g + 9)]
        lo, hi = jnp.concatenate(res[0::2], axis=0), jnp.concatenate(res[1::2], axis=0)
        blocks = [(i, g, b) for i, b in enumerate(_strassen_lhs(lo[:, :TH], hi[:, :TH], lo[:, TH:], hi[:, TH:]))]
        if g % 2 == 0:
            held.append(blocks.pop())
        else:
            blocks.append(held.pop())
        ot = _pack(jnp.concatenate([b for _, _, b in blocks], axis=1).astype(BF16).T)
        for q, (i, n, _) in enumerate(blocks):
            oc_v[slot][:, i * HK + 128 * n:i * HK + 128 * n + 128] = ot[q * TH // 2:(q + 1) * TH // 2, :]
            made.add(("oc", slot, i, n))
            if q % 2:
                deps.append(pltpu.bitcast(ot[(q + 1) * TH // 2 - 8:(q + 1) * TH // 2, :], F32))

    def o_blocks(slot, c, never):
        def job(k, a):
            k = (2, 3, 1, 4, 5, 0, 6)[k]
            assert made >= {("oc", slot, k, c), ("oc", slot, k, c + 2)}
            for r in range(4):
                if r:
                    a = yield GAP_O2
                m = [rows16(oc_v[slot], 8 * r + 32 * q, k * HK + n * QK + 128 * c, 128)
                     for q in range(2) for n in range(2)]
                yield from put_blocks(oc2_v[slot], 8 * r, _strassen_lhs, *m, never, a, skip=(1, 3),
                                      base=7 * k * QK + 128 * c, pitch=QK)
            made.add(("oc2", slot, k, c))
        return job

    def out_proj(side, step0, t, slot):
        count = [0]

        def inner(i, c):
            assert made >= {("oc2", slot, i, 0), ("oc2", slot, i, 1)}

            def product(j):
                step, odd = step0 + count[0] // 2, count[0] % 2
                count[0] += 1
                o = (oc_v[slot][32:64, i * HK + QK:(i + 1) * HK] if j == 1 else
                     oc_v[slot][0:32, i * HK:i * HK + QK] if j == 3 else
                     oc2_v[slot][:, (7 * i + j) * QK:(7 * i + j + 1) * QK])
                w = wos_v[:, (7 * i + j) * QK + 128 * c:(7 * i + j) * QK + 128 * c + 128]
                res = _dot(_unpack(o), _unpack(w if odd else side.gate(step, w)), NN)
                if odd:
                    side.done(step, res)
                return res
            return _block(_strassen(product))

        xt = view(x_v, t, T)

        def emit(q, r, res):
            for c in range(2):
                for n in range(2):
                    rows, c0 = slice(q * TH, (q + 1) * TH), r * HK + n * QK + 128 * c
                    h_v[slot][rows, c0:c0 + 128] = (res[:, 256 * c + 128 * n:256 * c + 128 * n + 128]
                                                    + xt[rows, c0:c0 + 128].astype(F32))
            made.add(("h", slot, q, r))

        _strassen_rows_first(lambda i: jnp.concatenate([inner(i, c) for c in range(2)], axis=1), emit)

    def phase2(u, carry):
        made.difference_update({m for m in made if m[0] in ("h", "oc", "oc2")})
        for i in range(4):
            stage_copy(i, u).wait()
        never = u < 0
        side = _Side(never, lambda rel, gap: min(rel + 2 * gap, 97) if rel < 98 else
                     rel + gap if rel + gap <= 155 else 2 * (rel + gap - 155) - 1)
        st = {"route": carry}
        tp = jnp.maximum(2 * u - 1, 0)
        early = len(LN2_PLANS[2])

        def ln2(slot, t, valid, k0, key):
            def job(k, a):
                k += k0
                hs = {("h", slot, k // 8, r) for r in range(2)}
                assert made >= hs or key == 0
                best = yield from finish_rows(h_v[slot], k, t, valid, st, never, a)
                assert key > 0 or not made & hs
                return best
            return job

        side.add(LN2_PLANS[0], ln2(1, tp, u > 0, early, 0))
        side.add(LN2_PLANS[1], ln2(0, 2 * u, None, 0, 1))
        side.add(LN2_PLANS[2], ln2(1, 2 * u + 1, None, 0, 2))

        def packer(i, dst, n):
            left = [n]

            def job(k, a):
                if i < 2:
                    yield from pack_rows(stage_v[i], dst, (k // 2) * 16, (0, D)[k % 2], (D, FM - D)[k % 2], never, a)
                else:
                    yield from pack_rows(stage_v[i], dst, k * 16, 0, D, never, a)
                left[0] -= 1
                if not left[0]:
                    stage_copy(i, jnp.minimum(u + 1, NQ - 1)).start()
                    n0 = stage_v[i].shape[0] - 16
                    side.deps.setdefault(PACK_DUE[i], []).append(stage_v[i][n0:n0 + 8, 0:128].astype(F32))
            return job

        for i in range(2):
            side.add(PACK_PLANS[i], packer(i, view((wgp_v, wup_v)[i], u, D // NQ // 2), len(PACK_PLANS[i])))
            d0 = pl.multiple_of(u * (DQ // 2) + i * (DQA // 2), 8)
            side.add(PACKD_PLANS[i], packer(2 + i, wdp_v.at[pl.ds(d0, 8 * len(PACKD_PLANS[i])), :],
                                            len(PACKD_PLANS[i])))
            for g in range(4):
                step = 107 + 28 * i + 7 * g + G_LAG
                wrap = lambda x: x if x < 156 else 2 * (x - 156) + 1
                side.hooks.setdefault(wrap(step), []).append(
                    lambda i=i, g=g, due=wrap(step + O_DUE): attn_blocks(i, g, side.deps.setdefault(due, [])))
            for c in range(2):
                side.add(O2_PLANS[2 * i + c], o_blocks(i, c, never))
        for i in range(2):
            feat_stage(side, 100 + 28 * i, 0, xs_tile(2 * u + i, i), lambda p, pr: q_pair(p, i, pr),
                       2 * u if i == 0 else None)
        for i in range(2):
            out_proj(side, 49 * i, 2 * u + i, i)
        side.check()

        @pl.when(u == 0)
        def _():
            o_copy(0, T, 0).start()

        @pl.when(u > 0)
        def _():
            o_copy(pl.multiple_of(tp * T, T), 2 * T, u).start()

        return st["route"]

    wg_copy.wait()
    wu_copy.wait()
    wd_copy.wait()
    route = lax.fori_loop(
        0, NT_ // 2, phase2,
        jnp.full((8, 128), KEY_MIN, jnp.int32))
    st = {"route": route}
    for k in range(len(LN2_PLANS[2]), T // LNC):
        now(finish_rows(h_v[1], k, NT_ - 1, None, st))
    o_copy(S - T, T, NT_).start()

    best = st["route"]
    for shift in (4, 2, 1):
        best = jnp.maximum(best, pltpu.roll(best, shift, 0))
    idx_s = (S - 1) - (best[0, 0] & (S - 1))
    gate = _lane_tile(jax.nn.sigmoid(pltpu.bitcast(_ordered(best & -65536), F32)), D // 128)
    blk = pl.multiple_of(jnp.clip((idx_s >> 4) << 4, 0, S - 16), 16)
    pair = jnp.broadcast_to(hn_v[pl.ds(jnp.clip(idx_s >> 1, 0, S // 2 - 1), 1), :], (8, D))
    x8 = pltpu.bitcast(jnp.where((idx_s & 1) == 1, pair & jnp.uint32(0xFFFF0000), pair << 16), F32)
    xs = jnp.concatenate([x8, x8], axis=0).astype(BF16)
    acts, anchors = [], []

    def park(v, half):
        n = v.shape[0] // 128
        for i in range(n):
            z_v[i, :, 128 * half:128 * half + 128] = v[128 * i:128 * i + 128, :]
        return jnp.concatenate([z_v[i, :, 128 * half:128 * half + 128] for i in range(n)], axis=0)

    for c0 in range(0, FM, 128):
        g = _dot(xs, _unpack(wgp_v[:, c0:c0 + 128]), NN)[0:8, :]
        u = _dot(xs, _unpack(wup_v[:, c0:c0 + 128]), NN)[0:8, :]
        anchors += [g, u]
        acts.append(g * jax.nn.sigmoid(g) * u)
    xb = park(_col_broadcast(x8), 0)
    g, u = [_sublane_allreduce(_vpu_matvec(
        xb, lambda g: w[8 * g:8 * g + 8, :].astype(F32), never0,
        anchors[i * MOE_NA // 2:(i + 1) * MOE_NA // 2], MOE_LAGS[0])) for i, w in enumerate((wg_v, wu_v))]
    acts.append(g * jax.nn.sigmoid(g) * u)
    a = jnp.concatenate(acts, axis=1)
    am = jnp.concatenate([a[:, FVD:], a[:, FVD:]], axis=0).astype(BF16)
    ys, anchors = [], anchors[MOE_NA:]
    for k0 in range(0, FF - FVD, 512):
        k1 = min(k0 + 512, FF - FVD)
        yk = _dot(am[:, k0:k1], _unpack(wdp_v[k0 // 2:k1 // 2, 0:D]), NN)[0:8, :]
        ys.append(yk)
        anchors += [yk[:, c:c + 128] for c in range(128, D, 256)]
    ys.append(_sublane_allreduce(_vpu_matvec(
        park(_col_broadcast(a[:, :FVD]), 1), lambda g: wd_v[8 * g:8 * g + 8, :].astype(F32), never0,
        anchors[:-MOE_ND], MOE_LAGS[1])))
    y = _tree(jnp.add, ys) * gate
    y = jnp.concatenate([y, y], axis=0)
    sel = lax.broadcasted_iota(jnp.int32, (16, 1), 0) == (idx_s - blk)
    patch_v[...] = (o_v[pl.ds(blk, 16), :].astype(F32) + jnp.where(sel, y, 0.0)).astype(BF16)
    o_copy(0, T, 0).wait()
    for u in range(1, NT_ // 2):
        o_copy((2 * u - 1) * T, 2 * T, u).wait()
    o_copy(S - T, T, NT_).wait()
    pc = pltpu.make_async_copy(patch_v, out_hbm.at[pl.ds(blk, 16), :], sem.at[SM + 3])
    pc.start()
    for i in range(4):
        stage_copy(i, NQ - 1).wait()
    pc.wait()


@jax.jit
def pallas_sequential_preLN__linear_kernel_hedgehog__moe_arch_mod__prompt_kernel(
    A_x: jax.Array,
    A_wqkv: jax.Array,
    A_w_phi: jax.Array,
    A_wo: jax.Array,
    B_x: jax.Array,
    B_w_r: jax.Array,
    B_w_gate: jax.Array,
    B_w_up: jax.Array,
    B_w_down: jax.Array,
):
    del B_x
    hbm = pl.BlockSpec(memory_space=pl.ANY)
    out = pl.pallas_call(
        _kernel,
        out_shape=jax.ShapeDtypeStruct((S, D), BF16),
        in_specs=[hbm] * 8,
        out_specs=hbm,
        scratch_shapes=[
            pltpu.VMEM((S, D), BF16),
            pltpu.VMEM(((T + TH) // 2, D), U32),
            [pltpu.VMEM((NT_ * TH // 4, SW), U32)] * 2,
            pltpu.VMEM((NT_ * HK // 2, 128), U32),
            pltpu.VMEM((3 * NC, D, RC), BF16),
            [pltpu.VMEM((D // 2, D), U32)] * 3,
            [pltpu.VMEM((HK // 2, 7 * HK), U32)] * 3,
            pltpu.VMEM((H, DH, DH), BF16),
            pltpu.VMEM((8 * 64, 128), U32),
            pltpu.VMEM((4, QK, D), BF16),
            pltpu.VMEM((QK // 2, 49 * QK + 128), U32),
            pltpu.VMEM((D,), BF16),
            pltpu.VMEM((8, D), F32),
            pltpu.VMEM((NPAIR, 64, 128), F32),
            pltpu.VMEM((NPAIR * 32, 128), U32),
            pltpu.VMEM((NPAIR, 128, T), F32),
            pltpu.VMEM((NPAIR, 128, 128), F32),
            [pltpu.VMEM((NPAIR * 64, T), U32)] * 2,
            [pltpu.VMEM((TH // 2, 7 * HK), U32)] * 2,
            [pltpu.VMEM((TH // 4, 49 * QK), U32)] * 2,
            [pltpu.VMEM((T, D), F32)] * 2,
            pltpu.VMEM((S // 2, D), U32),
            pltpu.VMEM((S, D), BF16),
            pltpu.VMEM((D, FV), BF16),
            pltpu.VMEM((D, FV), BF16),
            pltpu.VMEM((FVD, D), BF16),
            [pltpu.VMEM((D // NQ + 16, FM), BF16), pltpu.VMEM((D // NQ + 16, FM), BF16),
             pltpu.VMEM((DQA + 16, D), BF16), pltpu.VMEM((DQ - DQA + 16, D), BF16)],
            pltpu.VMEM((D // 2, FM), U32),
            pltpu.VMEM((D // 2, FM), U32),
            pltpu.VMEM(((FF - FVD) // 2, D + 128), U32),
            pltpu.VMEM((16, D), BF16),
            pltpu.SemaphoreType.DMA((6 + 3 * NC + NT_ + 17,)),
        ],
        compiler_params=pltpu.CompilerParams(vmem_limit_bytes=100 * 1024 * 1024,
                                             disable_semaphore_checks=True, disable_bounds_checks=True),
        name="hedgehog_mod",
    )(
        A_x.reshape(S, D),
        A_wqkv,
        A_w_phi,
        A_wo.reshape(4, QK, D),
        B_w_r,
        B_w_gate,
        B_w_up,
        B_w_down,
    )
    return out.reshape(1, S, D)
```
